```python
import jax
import jax.numpy as jnp

def _softmax(x, axis=-1):
    return jax.nn.softmax(x, axis=axis)

def _gelu(x):
    return jax.nn.gelu(x, approximate=True)

def _silu(x):
    return jax.nn.silu(x)

def _sigmoid(x):
    return jax.nn.sigmoid(x)

def _layernorm(x, axis=-1, eps=1e-05):
    m = jnp.mean(x, axis=axis, keepdims=True)
    v = jnp.var(x, axis=axis, keepdims=True)
    return (x - m) / jnp.sqrt(v + eps)

def _scatter_add(tgt, idx, src, axis=0):
    return tgt.at[idx].add(src)

def _segment_sum(src, seg, n):
    return jax.ops.segment_sum(src, seg, n)

class _Rng:

    def __init__(self, key):
        self._k = key

    def _next(self):
        self._k, sub = jax.random.split(self._k)
        return sub

    def normal(self, shape):
        return jax.random.normal(self._next(), shape, dtype=jnp.bfloat16)

    def randint(self, lo, hi, shape):
        return jax.random.randint(self._next(), shape, lo, hi, dtype=jnp.int32)

    def uniform(self, shape, lo=0.0, hi=1.0):
        return jax.random.uniform(self._next(), shape, jnp.bfloat16, lo, hi)

    def permutation(self, n):
        return jax.random.permutation(self._next(), n)
kernel_name = 'adaLN_cond__memory_aug_recurrent_mem_tr__mixer_s_mlp__prompt'

def setup_inputs():
    _rng = _Rng(jax.random.key(int.from_bytes(__import__("os").urandom(4), "little")))
    _w = lambda a: (lambda t: t.astype(jnp.bfloat16) if jnp.issubdtype(t.dtype, jnp.floating) else t)(jnp.asarray(a))

    def _A_setup():
        B, S, Dm = (1, 2048, 1024)
        H, Dh = (32, 128)
        M, seg = (8, 32)
        seg = min(seg, S)
        S = S // seg * seg
        return {'x': _w((lambda *s: _rng.normal(s) * 0.05)(B, S, Dm)), 'mem0': _w((lambda *s: _rng.normal(s) * 0.05)(B, M, Dm)), 'Wq': _w((lambda *s: _rng.normal(s) * 0.05)(Dm, H, Dh) * Dm ** (-0.5)), 'Wk': _w((lambda *s: _rng.normal(s) * 0.05)(Dm, H, Dh) * Dm ** (-0.5)), 'Wv': _w((lambda *s: _rng.normal(s) * 0.05)(Dm, H, Dh) * Dm ** (-0.5)), 'Wo': _w((lambda *s: _rng.normal(s) * 0.05)(H, Dh, Dm) * (H * Dh) ** (-0.5)), 'seg_len': seg}
    _A_in = _A_setup()

    def _B_setup():
        B, S, D, F = (1, 2048, 1024, 3584)
        return {'x': _w((lambda *s: _rng.normal(s) * 0.05)(B, S, D)), 'w1': _w((lambda *s: _rng.normal(s) * 0.05)(D, D) * D ** (-0.5)), 'w2': _w((lambda *s: _rng.normal(s) * 0.05)(D, D) * D ** (-0.5)), 'w3': _w((lambda *s: _rng.normal(s) * 0.05)(D, F) * D ** (-0.5)), 'w4': _w((lambda *s: _rng.normal(s) * 0.05)(F, D) * F ** (-0.5))}
    _B_in = _B_setup()
    return {'A_x': _A_in['x'], 'A_mem0': _A_in['mem0'], 'A_Wq': _A_in['Wq'], 'A_Wk': _A_in['Wk'], 'A_Wv': _A_in['Wv'], 'A_Wo': _A_in['Wo'], 'A_seg_len': _A_in['seg_len'], 'B_x': _B_in['x'], 'B_w1': _B_in['w1'], 'B_w2': _B_in['w2'], 'B_w3': _B_in['w3'], 'B_w4': _B_in['w4'], 'c': _w((lambda *s: _rng.normal(s) * 0.05)(1, 1024)), 'w_mod': _w((lambda *s: _rng.normal(s) * 0.05)(1024, 6 * 1024) * 1024 ** (-0.5))}

def reference(A_x, A_mem0, A_Wq, A_Wk, A_Wv, A_Wo, A_seg_len, B_x, B_w1, B_w2, B_w3, B_w4, c, w_mod):

    def _A_ref(x, mem0, Wq, Wk, Wv, Wo, seg_len):
        B, S, Dm = x.shape
        H, Dh = (Wq.shape[1], Wq.shape[2])
        M = mem0.shape[1]
        scale = Dh ** (-0.5)
        n_seg = S // seg_len
        L = M + seg_len
        idx = jnp.arange(L)
        mask = (idx[:, None] < M) | (idx[:, None] >= idx[None, :])
        mem = mem0
        outs = []
        for s in range(n_seg):
            xs = x[:, s * seg_len:(s + 1) * seg_len, :].copy()
            h = jnp.concatenate([mem, xs], axis=1)
            q = jnp.einsum('btd,dhe->bhte', h, Wq)
            k = jnp.einsum('btd,dhe->bhte', h, Wk)
            v = jnp.einsum('btd,dhe->bhte', h, Wv)
            scores = jnp.einsum('bhqe,bhke->bhqk', q, k) * scale
            scores = jnp.where(mask[None, None], scores, -1000000000.0)
            p = _softmax(scores, axis=-1)
            o = jnp.einsum('bhqk,bhke->bhqe', p, v)
            o = jnp.einsum('bhte,hed->btd', o, Wo)
            mem = o[:, :M, :].copy()
            outs.append(o[:, M:, :])
        return jnp.concatenate(outs, axis=1)

    def _B_ref(x, w1, w2, w3, w4):
        B, S, D = x.shape
        h = _gelu(_layernorm(x, axis=-1) @ w1)
        c = D // 4
        g0 = jnp.pad(h[:, :, 0 * c:1 * c], ((0, 0), (1, 0), (0, 0)))[:, :S, :]
        g1 = jnp.pad(h[:, :, 1 * c:2 * c], ((0, 0), (0, 1), (0, 0)))[:, 1:, :]
        g2 = jnp.pad(h[:, :, 2 * c:3 * c], ((0, 0), (2, 0), (0, 0)))[:, :S, :]
        g3 = jnp.pad(h[:, :, 3 * c:], ((0, 0), (0, 2), (0, 0)))[:, 2:, :]
        hs = jnp.concatenate([g0, g1, g2, g3], axis=-1) @ w2
        x1 = x + hs
        h2 = _gelu(_layernorm(x1, axis=-1) @ w3) @ w4
        return x1 + h2
    x = A_x
    mod = (_silu(c) @ w_mod).reshape(c.shape[0], 6, 1, -1)
    sa, ca, ga, sb, cb, gb = (mod[:, 0].copy(), mod[:, 1].copy(), mod[:, 2].copy(), mod[:, 3].copy(), mod[:, 4].copy(), mod[:, 5].copy())
    h = _layernorm(x, axis=-1) * (1 + ca) + sa
    x = x + ga * _A_ref(h, A_mem0, A_Wq, A_Wk, A_Wv, A_Wo, A_seg_len)
    h = _layernorm(x, axis=-1) * (1 + cb) + sb
    x = x + gb * _B_ref(h, B_w1, B_w2, B_w3, B_w4)
    return x
```

```python
import functools

import jax
import jax.numpy as jnp
from jax import lax
import jax.experimental.pallas as pl
import jax.experimental.pallas.tpu as pltpu

bf16, f32, u32 = jnp.bfloat16, jnp.float32, jnp.uint32

S, D, H, E, M, SEG, F = 2048, 1024, 32, 128, 8, 32, 3584
NSEG = S // SEG
NP = H // 2
TC = SEG - M
HG = 8
NG = H // HG
TB = 256
NB = S // TB
FC = 512
EPS = 1e-5
SCALE = E ** -0.5


def _pk(x):
    return pltpu.bitcast(x.astype(bf16), u32)


def _up(x):
    return pltpu.bitcast(x, bf16)


def _dot(a, b):
    return jnp.dot(a, b, preferred_element_type=f32)


def _ln(x):
    m = jnp.mean(x, axis=-1, keepdims=True)
    xc = x - m
    v = jnp.mean(xc * xc, axis=-1, keepdims=True)
    return xc * lax.rsqrt(v + EPS)


def _gelu(x):
    c = 0.7978845608028654
    return 0.5 * x * (1.0 + jnp.tanh(c * (x + 0.044715 * (x * x * x))))


def _mask_fill():
    n = 2 * (M + SEG)
    r = lax.broadcasted_iota(jnp.int32, (n, n), 0)
    c = lax.broadcasted_iota(jnp.int32, (n, n), 1)

    def headpos(i):
        head = jnp.where(i < 64, i >> 5, (i - 64) >> 3)
        pos = jnp.where(i < 64, i & 31, 32 + (i & 7))
        return head, pos

    hr, pr = headpos(r)
    hc, pc = headpos(c)
    same = hr == hc
    valid = same & ((pr < M) | (pr >= pc))
    return jnp.where(valid, 0.0, jnp.where(same, -1e9, -jnp.inf)).astype(f32)


def _kernel(x_hbm, mem0_ref, wq_hbm, wk_hbm, wv_hbm, wo_hbm, w1_hbm, w2_hbm, w3_hbm,
            w4_hbm, c_ref, wm_hbm,
            out_hbm,
            x_s, xpre_s, hpre_s, wm_s, sq, sk, sv, wq_s, wk_s, wv_s, wo_s,
            w1_s, w2_s, w3_s, w4_s, pre_s, mod_s, mem_s, hn_s, aout_s, fill_s,
            x2_s, hb_s, t_s, y_s, u_s, o_s, sems):
    w_hbm = (wq_hbm, wk_hbm, wv_hbm)
    stg = (sq, sk, sv)
    w_s = (wq_s, wk_s, wv_s)

    SEM_XPRE, SEM_WM, SEM_STG, SEM_X, SEM_WO, SEM_W1, SEM_W2, SEM_W3, SEM_W4, SEM_OUT = (
        0, 1, 2, 5, 6, 7, 8, 9, 10, 11)

    def copy(src, dst, k):
        return pltpu.make_async_copy(src, dst, sems.at[k])

    def w_copy(t, g):
        return copy(w_hbm[t].at[:, pl.ds(pl.multiple_of(g * HG, HG), HG), :], stg[t], SEM_STG + t)

    def mod_row(k):
        return mod_s[0:1, k * D:(k + 1) * D]

    cp_xpre = copy(x_hbm.at[:, TC:SEG, :], xpre_s, SEM_XPRE)
    cp_wm0 = copy(wm_hbm.at[:, 0:2 * D], wm_s.at[:, 0:2 * D], SEM_WM)
    cp_xpre.start()
    cp_wm0.start()
    for t in range(3):
        w_copy(t, 0).start()

    fill_s[...] = _mask_fill()
    mem_s[...] = mem0_ref[...].astype(f32)
    mod_s[...] = jnp.zeros(mod_s.shape, f32)
    aout_s[...] = jnp.zeros(aout_s.shape, f32)
    t_s[0:8, :] = jnp.zeros((8, D), f32)
    t_s[S + 8:S + 16, :] = jnp.zeros((8, D), f32)

    cf = c_ref[...].astype(f32)
    sc = cf * (1.0 / (1.0 + jnp.exp(-cf)))
    sc8 = jnp.broadcast_to(sc, (8, D)).astype(bf16)

    cp_wm0.wait()
    mod_s[:, 0:2 * D] = _dot(sc8, wm_s[:, 0:2 * D])

    def modulate_a(xr):
        return _ln(xr) * (1.0 + mod_row(1)) + mod_row(0)

    cp_xpre.wait()

    def hpre_body(i, carry):
        xr = xpre_s[pl.ds(pl.multiple_of(i * 8, 8), 8)].astype(f32).reshape(64, D)
        hpre_s[pl.ds(pl.multiple_of(i * 32, 32), 32), :] = _pk(modulate_a(xr))
        return carry

    lax.fori_loop(0, NSEG // 8, hpre_body, 0)

    def relayout(t, g, part, nparts):
        n = 16
        per = D // nparts
        for i in range(per // n):
            d0 = part * per + i * n
            v = jnp.swapaxes(stg[t][d0:d0 + n], 0, 1)
            w_s[t][pl.ds(g * HG, HG), d0 // 2:(d0 + n) // 2, :] = pltpu.bitcast(v, u32)

    w_copy(0, 0).wait()
    relayout(0, 0, 0, 1)

    MB = 128

    def pre_pair(t, g, pp):
        ys = []
        for hh in range(2):
            w = _up(w_s[t][g * HG + 2 * pp + hh])
            ys.append(jnp.concatenate(
                [_dot(_up(hpre_s[mb * MB // 2:(mb + 1) * MB // 2, :]), w)
                 for mb in range(NSEG * M // MB)], axis=0).reshape(NSEG, M, E))
        y = jnp.concatenate(ys, axis=1)
        pre_s[t * NP + g * (HG // 2) + pp] = pltpu.bitcast(y.astype(bf16), u32)

    def p1_body(g, carry):
        gn = jnp.minimum(g + 1, NG - 1)
        for t in range(3):
            tn = (t + 1) % 3
            @pl.when(g + 1 < NG)
            def _():
                w_copy(t, gn).start()

            if t == 0:
                for j in range(2):
                    jj = 2 * g + j
                    copy(wo_hbm.at[:, pl.ds(pl.multiple_of(jj * E, E), E)], wo_s.at[jj],
                         SEM_WO).start()
            elif t == 1:
                r = pl.ds(pl.multiple_of(g * (NSEG // NG), NSEG // NG), NSEG // NG)
                copy(x_hbm.at[r], x_s.at[r], SEM_X).start()
                r1 = pl.ds(pl.multiple_of(g * (D // NG), D // NG), D // NG)
                copy(w1_hbm.at[r1], w1_s.at[r1], SEM_W1).start()

            if t < 2:
                w_copy(tn, g).wait()
                gr = g
            else:
                @pl.when(g + 1 < NG)
                def _():
                    w_copy(tn, gn).wait()
                gr = gn
            for pp in range(HG // 2):
                relayout(tn, gr, pp, HG // 2)
                pre_pair(t, g, pp)
        return carry

    lax.fori_loop(0, NG, p1_body, 0)

    copy(wo_s, wo_s, SEM_WO).wait()
    copy(x_s, x_s, SEM_X).wait()
    copy(w1_s, w1_s, SEM_W1).wait()
    cp_wm1 = copy(wm_hbm.at[:, 2 * D:6 * D], wm_s, SEM_WM)
    cp_w2 = copy(w2_hbm, w2_s, SEM_W2)
    cp_w3 = copy(w3_hbm, w3_s, SEM_W3)
    cp_w4 = copy(w4_hbm, w4_s, SEM_W4)
    cp_wm1.start()
    cp_w2.start()
    cp_w3.start()
    cp_w4.start()

    def h_rows(s):
        return modulate_a(x_s[s, 0:TC, :].astype(f32))

    hn_s[...] = h_rows(0)

    def chain_step(s, mem, htok, odef_prev):
        hs = jnp.concatenate([mem, htok], axis=0).astype(bf16)
        qkv = [[None] * 3 for _ in range(NP)]
        ps = [None] * NP
        os_ = [None] * H
        odef = [None] * H

        def proj(p):
            for t in range(3):
                a = _dot(hs, _up(w_s[t][2 * p]))
                b = _dot(hs, _up(w_s[t][2 * p + 1]))
                qkv[p][t] = _up(jnp.concatenate([_pk(a), _pk(b), pre_s[t * NP + p, s]], axis=0))

        def scores(p):
            sc_ = lax.dot_general(qkv[p][0], qkv[p][1], (((1,), (1,)), ((), ())),
                                  preferred_element_type=f32)
            fill = fill_s[...]
            sc_ = jnp.where(fill == 0.0, sc_ * SCALE, fill)
            m = jnp.max(sc_, axis=-1, keepdims=True)
            e = jnp.exp(sc_ - m)
            l = jnp.sum(e, axis=-1, keepdims=True)
            r = pl.reciprocal(l, approx=True)
            r = r * (2.0 - l * r)
            ps[p] = (e * r).astype(bf16)

        def fin(p):
            o = _dot(ps[p], qkv[p][2])
            for hh in range(2):
                h = 2 * p + hh
                rows = o[32 * hh:32 * hh + 32]
                odef[h] = o[64 + 8 * hh:72 + 8 * hh]
                if odef_prev is not None:
                    rows = jnp.concatenate([rows, odef_prev[h], odef[h]], axis=0)
                os_[h] = _pk(rows)

        acc = [None] * 8

        def wo(h0, h1, js):
            lhs = _up(jnp.concatenate(os_[h0:h1], axis=1))
            for j in js:
                part = _dot(lhs, wo_s[j, h0 * E:h1 * E, :])
                acc[j] = part if acc[j] is None else part + acc[j]

        for p in range(NP):
            proj(p)
            if p >= 1:
                scores(p - 1)
            if p >= 3:
                fin(p - 3)
        wo(0, 24, range(0, 2))
        scores(NP - 1)
        fin(NP - 3)
        wo(0, 24, range(2, 3))
        fin(NP - 2)
        wo(0, 24, range(3, 5))
        fin(NP - 1)
        wo(0, 24, range(5, 8))
        wo(24, 32, range(8))
        return jnp.concatenate(acc, axis=1), odef

    def mixer_in(i):
        r = pl.ds(pl.multiple_of(i * 64, 64), 64)
        xr = x_s[pl.ds(2 * i, 2)].astype(f32).reshape(2 * SEG, D)
        x2 = xr + mod_row(2) * aout_s[...]
        x2_s[r, :] = x2.astype(bf16)
        hb = _ln(x2) * (1.0 + mod_row(4)) + mod_row(3)
        hb_s[r, :] = hb.astype(bf16)
        t = _gelu(_dot(_ln(hb).astype(bf16), w1_s[...]))
        t_s[pl.ds(pl.multiple_of(i * 64 + 8, 8), 64), :] = t

    def p2_body(i, carry):
        @pl.when(i == 1)
        def _():
            cp_wm1.wait()
            mod_s[:, 2 * D:6 * D] = _dot(sc8, wm_s[...])

        sa_ = 2 * i
        sb_ = 2 * i + 1
        hb_tok = h_rows(sb_)
        oa, odef_a = chain_step(sa_, mem_s[...], hn_s[...], None)
        mixer_in(jnp.maximum(i - 1, 0))
        ob, _ = chain_step(sb_, oa[0:M], hb_tok, odef_a)
        mem_s[...] = ob[0:M]
        aout_s[0:TC, :] = oa[M:SEG]
        aout_s[TC:SEG, :] = ob[SEG:SEG + M]
        aout_s[SEG:SEG + TC, :] = ob[M:SEG]
        aout_s[SEG + TC:2 * SEG, :] = ob[SEG + M:SEG + 2 * M]
        hn_s[...] = h_rows(jnp.minimum(sb_ + 1, NSEG - 1))
        return carry

    lax.fori_loop(0, NSEG // 2, p2_body, 0)
    mixer_in(NSEG // 2 - 1)

    cp_w2.wait()
    cp_w3.wait()
    cp_w4.wait()

    def mix(j):
        r0 = pl.multiple_of(j * TB, TB)
        q = D // 4
        parts = []
        for k, sh in enumerate((-1, 1, -2, 2)):
            tt = t_s[pl.ds(r0, TB + 16), k * q:(k + 1) * q]
            parts.append(tt[8 + sh:8 + sh + TB])
        g = jnp.concatenate(parts, axis=1).astype(bf16)
        x1 = hb_s[pl.ds(r0, TB), :].astype(f32) + _dot(g, w2_s[...])
        return x1

    def out_copy(j, slot):
        return copy(o_s.at[slot], out_hbm.at[pl.ds(pl.multiple_of(j * TB, TB), TB)], SEM_OUT + slot)

    x1_0 = mix(0)
    y_s[...] = _pk(_ln(x1_0))
    hb_s[0:TB, :] = x1_0.astype(bf16)

    def p3_body(j, carry):
        slot = j % 2

        @pl.when(j >= 2)
        def _():
            out_copy(j - 2, slot).wait()

        r = pl.ds(pl.multiple_of(j * TB, TB), TB)
        for cidx in range(F // FC):
            u = _gelu(_dot(_up(y_s[...]), w3_s[:, cidx * FC:(cidx + 1) * FC]))
            u_s[:, cidx * FC:(cidx + 1) * FC] = _pk(u)
        base = x2_s[r, :].astype(f32) + mod_row(5) * hb_s[r, :].astype(f32)
        jn = jnp.minimum(j + 1, NB - 1)
        x1n = mix(jn)
        h2 = _dot(_up(u_s[...]), w4_s[...])
        o_s[slot] = (base + mod_row(5) * h2).astype(bf16)
        y_s[...] = _pk(_ln(x1n))
        hb_s[pl.ds(pl.multiple_of(jn * TB, TB), TB), :] = x1n.astype(bf16)
        out_copy(j, slot).start()
        return carry

    lax.fori_loop(0, NB, p3_body, 0)
    out_copy(NB - 2, 0).wait()
    out_copy(NB - 1, 1).wait()


@functools.partial(jax.jit, static_argnames=("A_seg_len",))
def pallas_adaLN_cond__memory_aug_recurrent_mem_tr__mixer_s_mlp__prompt_kernel(
    A_x: jax.Array,
    A_mem0: jax.Array,
    A_Wq: jax.Array,
    A_Wk: jax.Array,
    A_Wv: jax.Array,
    A_Wo: jax.Array,
    A_seg_len,
    B_x: jax.Array,
    B_w1: jax.Array,
    B_w2: jax.Array,
    B_w3: jax.Array,
    B_w4: jax.Array,
    c: jax.Array,
    w_mod: jax.Array,
):
    assert A_seg_len == SEG and A_x.shape == (1, S, D) and A_mem0.shape == (1, M, D)
    hbm = pl.BlockSpec(memory_space=pl.ANY)
    vmem = pl.BlockSpec(memory_space=pltpu.VMEM)
    scratch = [
        pltpu.VMEM((NSEG, SEG, D), bf16),
        pltpu.VMEM((NSEG, M, D), bf16),
        pltpu.VMEM((NSEG * M // 2, D), u32),
        pltpu.VMEM((D, 4 * D), bf16),
        pltpu.VMEM((D, HG, E), bf16),
        pltpu.VMEM((D, HG, E), bf16),
        pltpu.VMEM((D, HG, E), bf16),
        pltpu.VMEM((H, D // 2, E), u32),
        pltpu.VMEM((H, D // 2, E), u32),
        pltpu.VMEM((H, D // 2, E), u32),
        pltpu.VMEM((D // E, H * E, E), bf16),
        pltpu.VMEM((D, D), bf16),
        pltpu.VMEM((D, D), bf16),
        pltpu.VMEM((D, F), bf16),
        pltpu.VMEM((F, D), bf16),
        pltpu.VMEM((3 * NP, NSEG, M, E), u32),
        pltpu.VMEM((8, 6 * D), f32),
        pltpu.VMEM((M, D), f32),
        pltpu.VMEM((TC, D), f32),
        pltpu.VMEM((2 * SEG, D), f32),
        pltpu.VMEM((2 * (M + SEG), 2 * (M + SEG)), f32),
        pltpu.VMEM((S, D), bf16),
        pltpu.VMEM((S, D), bf16),
        pltpu.VMEM((S + 16, D), f32),
        pltpu.VMEM((TB // 2, D), u32),
        pltpu.VMEM((TB // 2, F), u32),
        pltpu.VMEM((2, TB, D), bf16),
        pltpu.SemaphoreType.DMA((13,)),
    ]
    out = pl.pallas_call(
        _kernel,
        out_shape=jax.ShapeDtypeStruct((S, D), bf16),
        in_specs=[hbm, vmem, hbm, hbm, hbm, hbm, hbm, hbm, hbm, hbm, vmem, hbm],
        out_specs=hbm,
        scratch_shapes=scratch,
        compiler_params=pltpu.CompilerParams(vmem_limit_bytes=126 * 1024 * 1024),
    )(A_x.reshape(NSEG, SEG, D), A_mem0.reshape(M, D), A_Wq, A_Wk, A_Wv,
      A_Wo.reshape(H * E, D), B_w1, B_w2, B_w3, B_w4, c, w_mod)
    return out.reshape(1, S, D)
```

```python
import functools

import jax
import jax.numpy as jnp
from jax import lax
import jax.experimental.pallas as pl
import jax.experimental.pallas.tpu as pltpu

bf16, f32, u32 = jnp.bfloat16, jnp.float32, jnp.uint32

S, D, H, E, M, SEG, F = 2048, 1024, 32, 128, 8, 32, 3584
NSEG = S // SEG
NP = H // 2
TC = SEG - M
HG = 8
NG = H // HG
TB = 256
NB = S // TB
FC = 512
RL_ROWS = 16
EPS = 1e-5
SCALE = E ** -0.5
_PHASES = "123"


def _pk(x):
    return pltpu.bitcast(x.astype(bf16), u32)


def _up(x):
    return pltpu.bitcast(x, bf16)


def _dot(a, b):
    return jnp.dot(a, b, preferred_element_type=f32)


def _ln(x):
    m = jnp.mean(x, axis=-1, keepdims=True)
    xc = x - m
    v = jnp.mean(xc * xc, axis=-1, keepdims=True)
    return xc * lax.rsqrt(v + EPS)


def _gelu(x):
    c = 0.7978845608028654
    return 0.5 * x * (1.0 + jnp.tanh(c * (x + 0.044715 * (x * x * x))))


def _mask_fill():
    n = 2 * (M + SEG)
    r = lax.broadcasted_iota(jnp.int32, (n, n), 0)
    c = lax.broadcasted_iota(jnp.int32, (n, n), 1)

    def headpos(i):
        head = jnp.where(i < 64, i >> 5, (i - 64) >> 3)
        pos = jnp.where(i < 64, i & 31, 32 + (i & 7))
        return head, pos

    hr, pr = headpos(r)
    hc, pc = headpos(c)
    same = hr == hc
    valid = same & ((pr < M) | (pr >= pc))
    return jnp.where(valid, 0.0, jnp.where(same, -1e9, -jnp.inf)).astype(f32)


def _kernel(x_hbm, mem0_ref, wq_hbm, wk_hbm, wv_hbm, wo_hbm, w1_hbm, w2_hbm, w3_hbm,
            w4_hbm, c_ref, wm_hbm,
            out_hbm,
            x_s, xpre_s, hpre_s, wm_s, sq, sk, sv, wq_s, wk_s, wv_s, wo_s,
            w1_s, w2_s, w3_s, w4_s, pre_s, mod_s, mem_s, hn_s, aout_s, fill_s,
            x2_s, hb_s, t_s, y_s, u_s, o_s, zero_s, so, s1, sems):
    w_hbm = (wq_hbm, wk_hbm, wv_hbm)
    stg = (sq, sk, sv)
    w_s = (wq_s, wk_s, wv_s)

    SEM_XPRE, SEM_WM, SEM_STG, SEM_X, SEM_WO, SEM_W1, SEM_W2, SEM_W3, SEM_W4, SEM_OUT = (
        0, 1, 2, 5, 6, 7, 8, 9, 10, 11)

    def copy(src, dst, k):
        return pltpu.make_async_copy(src, dst, sems.at[k])

    def w_copy(t, g):
        return copy(w_hbm[t].at[:, pl.ds(pl.multiple_of(g * HG, HG), HG), :], stg[t], SEM_STG + t)

    def mod_row(k):
        return mod_s[0:1, k * D:(k + 1) * D]

    cp_xpre = copy(x_hbm.at[:, TC:SEG, :], xpre_s, SEM_XPRE)
    cp_wm0 = copy(wm_hbm.at[:, 0:2 * D], wm_s.at[:, 0:2 * D], SEM_WM)
    cp_xpre.start()
    cp_wm0.start()
    for t in range(3):
        w_copy(t, 0).start()

    zero_s[...] = jnp.zeros(zero_s.shape, u32)
    fill_s[...] = _mask_fill()
    mem_s[...] = mem0_ref[...].astype(f32)
    mod_s[...] = jnp.zeros(mod_s.shape, f32)
    aout_s[...] = jnp.zeros(aout_s.shape, f32)
    t_s[0:8, :] = jnp.zeros((8, D), f32)
    t_s[S + 8:S + 16, :] = jnp.zeros((8, D), f32)

    cf = c_ref[...].astype(f32)
    sc = cf * (1.0 / (1.0 + jnp.exp(-cf)))
    sc8 = jnp.broadcast_to(sc, (8, D)).astype(bf16)

    cp_wm0.wait()
    mod_s[:, 0:2 * D] = _dot(sc8, wm_s[:, 0:2 * D])

    def modulate_a(xr):
        return _ln(xr) * (1.0 + mod_row(1)) + mod_row(0)

    cp_xpre.wait()

    def hpre_body(i, carry):
        xr = xpre_s[pl.ds(pl.multiple_of(i * 8, 8), 8)].astype(f32).reshape(64, D)
        hpre_s[pl.ds(pl.multiple_of(i * 32, 32), 32), :] = _pk(modulate_a(xr))
        return carry

    lax.fori_loop(0, NSEG // 8, hpre_body, 0)

    def relayout(t, g, i):
        n = RL_ROWS
        d0 = i * n
        v = pltpu.bitcast(jnp.swapaxes(stg[t][d0:d0 + n], 0, 1), u32)
        w_s[t][pl.ds(g * HG, HG), d0 // 2:(d0 + n) // 2, :] = v
        z = v[0]
        for h in range(1, HG):
            z = z | v[h]
        return z

    def repack(src, dst, g, i):
        v = pltpu.bitcast(src[16 * i:16 * i + 16, :], u32)
        dst[pl.ds(pl.multiple_of(g * (src.shape[0] // 2) + 8 * i, 8), 8), :] = v
        z = v[:, 0:E]
        for j in range(1, D // E):
            z = z | v[:, j * E:(j + 1) * E]
        return z

    w_copy(0, 0).wait()
    for i in range(D // RL_ROWS):
        relayout(0, 0, i)

    MB = 128

    def pre_pair(t, g, pp, side):
        ys = []
        for hh in range(2):
            blocks = []
            for mb in range(NSEG * M // MB):
                w = w_s[t][g * HG + 2 * pp + hh]
                za, zb = side(), side()
                w = jnp.concatenate([w[0:8] | za, w[8:256], w[256:264] | zb, w[264:]], axis=0)
                blocks.append(_dot(_up(hpre_s[mb * MB // 2:(mb + 1) * MB // 2, :]), _up(w)))
            ys.append(jnp.concatenate(blocks, axis=0).reshape(NSEG, M, E))
        y = jnp.concatenate(ys, axis=1)
        pre_s[t * NP + g * (HG // 2) + pp] = pltpu.bitcast(y.astype(bf16), u32)

    def p1_body(g, carry):
        gn = jnp.minimum(g + 1, NG - 1)
        no, n1 = H * E // NG, D // NG
        cp_wo = copy(wo_hbm.at[pl.ds(pl.multiple_of(g * no, no), no)], so, SEM_WO)
        cp_w1 = copy(w1_hbm.at[pl.ds(pl.multiple_of(g * n1, n1), n1)], s1, SEM_W1)
        for t in range(3):
            tn = (t + 1) % 3
            @pl.when(g + 1 < NG)
            def _():
                w_copy(t, gn).start()

            if t == 0:
                cp_wo.start()
                cp_w1.start()
            elif t == 1:
                r = pl.ds(pl.multiple_of(g * (NSEG // NG), NSEG // NG), NSEG // NG)
                copy(x_hbm.at[r], x_s.at[r], SEM_X).start()

            if t < 2:
                w_copy(tn, g).wait()
                gr = g
            else:
                cp_wo.wait()
                cp_w1.wait()

                @pl.when(g + 1 < NG)
                def _():
                    w_copy(tn, gn).wait()
                gr = gn
            units = iter(range(D // RL_ROWS))

            def side():
                i = next(units)
                z = relayout(tn, gr, i)
                if t == 2:
                    z = z | repack(so, wo_s, g, i)
                    if i % 4 == 0:
                        z = z | repack(s1, w1_s, g, i // 4)
                return z & zero_s[...]

            for pp in range(HG // 2):
                pre_pair(t, g, pp, side)
        return carry

    lax.fori_loop(0, NG, p1_body, 0)

    copy(x_s, x_s, SEM_X).wait()
    cp_wm1 = copy(wm_hbm.at[:, 2 * D:6 * D], wm_s, SEM_WM)
    cp_w2 = copy(w2_hbm, w2_s, SEM_W2)
    cp_w3 = copy(w3_hbm, w3_s, SEM_W3)
    cp_w4 = copy(w4_hbm, w4_s, SEM_W4)
    cp_wm1.start()
    cp_w2.start()
    cp_w3.start()
    cp_w4.start()

    def h_rows(s):
        return modulate_a(x_s[s, 0:TC, :].astype(f32))

    hn_s[...] = h_rows(0)

    def chain_step(s, mem, htok, odef_prev):
        hs = jnp.concatenate([mem, htok], axis=0).astype(bf16)
        qkv = [[None] * 3 for _ in range(NP)]
        ps = [None] * NP
        os_ = [None] * H
        odef = [None] * H

        def proj(p):
            for t in range(3):
                a = _dot(hs, _up(w_s[t][2 * p]))
                b = _dot(hs, _up(w_s[t][2 * p + 1]))
                qkv[p][t] = _up(jnp.concatenate([_pk(a), _pk(b), pre_s[t * NP + p, s]], axis=0))

        def scores(p):
            sc_ = lax.dot_general(qkv[p][0], qkv[p][1], (((1,), (1,)), ((), ())),
                                  preferred_element_type=f32)
            fill = fill_s[...]
            sc_ = jnp.where(fill == 0.0, sc_ * SCALE, fill)
            m = jnp.max(sc_, axis=-1, keepdims=True)
            e = jnp.exp(sc_ - m)
            l = jnp.sum(e, axis=-1, keepdims=True)
            r = pl.reciprocal(l, approx=True)
            r = r * (2.0 - l * r)
            ps[p] = (e * r).astype(bf16)

        def fin(p):
            o = _dot(ps[p], qkv[p][2])
            for hh in range(2):
                h = 2 * p + hh
                rows = o[32 * hh:32 * hh + 32]
                odef[h] = o[64 + 8 * hh:72 + 8 * hh]
                if odef_prev is not None:
                    rows = jnp.concatenate([rows, odef_prev[h], odef[h]], axis=0)
                os_[h] = _pk(rows)

        acc = [None] * 8

        def wo(h0, h1, js):
            lhs = _up(jnp.concatenate(os_[h0:h1], axis=1))
            for j in js:
                part = _dot(lhs, _up(wo_s[h0 * E // 2:h1 * E // 2, j * E:(j + 1) * E]))
                acc[j] = part if acc[j] is None else part + acc[j]

        for p in range(NP):
            proj(p)
            if p >= 1:
                scores(p - 1)
            if p >= 3:
                fin(p - 3)
        wo(0, 24, range(0, 2))
        scores(NP - 1)
        fin(NP - 3)
        wo(0, 24, range(2, 3))
        fin(NP - 2)
        wo(0, 24, range(3, 5))
        fin(NP - 1)
        wo(0, 24, range(5, 8))
        wo(24, 32, range(8))
        return jnp.concatenate(acc, axis=1), odef

    def mixer_in(i):
        r = pl.ds(pl.multiple_of(i * 64, 64), 64)
        xr = x_s[pl.ds(2 * i, 2)].astype(f32).reshape(2 * SEG, D)
        x2 = xr + mod_row(2) * aout_s[...]
        x2_s[r, :] = x2.astype(bf16)
        hb = _ln(x2) * (1.0 + mod_row(4)) + mod_row(3)
        hb_s[r, :] = hb.astype(bf16)
        t = _gelu(_dot(_ln(hb).astype(bf16), _up(w1_s[...])))
        t_s[pl.ds(pl.multiple_of(i * 64 + 8, 8), 64), :] = t

    def p2_body(i, carry):
        @pl.when(i == 1)
        def _():
            cp_wm1.wait()
            mod_s[:, 2 * D:6 * D] = _dot(sc8, wm_s[...])

        sa_ = 2 * i
        sb_ = 2 * i + 1
        hb_tok = h_rows(sb_)
        oa, odef_a = chain_step(sa_, mem_s[...], hn_s[...], None)
        mixer_in(jnp.maximum(i - 1, 0))
        ob, _ = chain_step(sb_, oa[0:M], hb_tok, odef_a)
        mem_s[...] = ob[0:M]
        aout_s[0:TC, :] = oa[M:SEG]
        aout_s[TC:SEG, :] = ob[SEG:SEG + M]
        aout_s[SEG:SEG + TC, :] = ob[M:SEG]
        aout_s[SEG + TC:2 * SEG, :] = ob[SEG + M:SEG + 2 * M]
        hn_s[...] = h_rows(jnp.minimum(sb_ + 1, NSEG - 1))
        return carry

    if "2" in _PHASES:
        lax.fori_loop(0, NSEG // 2, p2_body, 0)
        mixer_in(NSEG // 2 - 1)
    else:
        cp_wm1.wait()
        cpd = copy(pre_s.at[0], pre_s.at[1], SEM_WM)
        cpd.start()
        cpd.wait()

    cp_w2.wait()
    cp_w3.wait()
    cp_w4.wait()

    def mix(j):
        r0 = pl.multiple_of(j * TB, TB)
        q = D // 4
        parts = []
        for k, sh in enumerate((-1, 1, -2, 2)):
            tt = t_s[pl.ds(r0, TB + 16), k * q:(k + 1) * q]
            parts.append(tt[8 + sh:8 + sh + TB])
        g = jnp.concatenate(parts, axis=1).astype(bf16)
        x1 = hb_s[pl.ds(r0, TB), :].astype(f32) + _dot(g, w2_s[...])
        return x1

    def out_copy(j, slot):
        return copy(o_s.at[slot], out_hbm.at[pl.ds(pl.multiple_of(j * TB, TB), TB)], SEM_OUT + slot)

    if "3" not in _PHASES:
        return

    x1_0 = mix(0)
    y_s[...] = _pk(_ln(x1_0))
    hb_s[0:TB, :] = x1_0.astype(bf16)

    def p3_body(j, carry):
        slot = j % 2

        @pl.when(j >= 2)
        def _():
            out_copy(j - 2, slot).wait()

        r = pl.ds(pl.multiple_of(j * TB, TB), TB)
        for cidx in range(F // FC):
            u = _gelu(_dot(_up(y_s[...]), w3_s[:, cidx * FC:(cidx + 1) * FC]))
            u_s[:, cidx * FC:(cidx + 1) * FC] = _pk(u)
        base = x2_s[r, :].astype(f32) + mod_row(5) * hb_s[r, :].astype(f32)
        jn = jnp.minimum(j + 1, NB - 1)
        x1n = mix(jn)
        h2 = _dot(_up(u_s[...]), w4_s[...])
        o_s[slot] = (base + mod_row(5) * h2).astype(bf16)
        y_s[...] = _pk(_ln(x1n))
        hb_s[pl.ds(pl.multiple_of(jn * TB, TB), TB), :] = x1n.astype(bf16)
        out_copy(j, slot).start()
        return carry

    lax.fori_loop(0, NB, p3_body, 0)
    out_copy(NB - 2, 0).wait()
    out_copy(NB - 1, 1).wait()


@functools.partial(jax.jit, static_argnames=("A_seg_len",))
def pallas_adaLN_cond__memory_aug_recurrent_mem_tr__mixer_s_mlp__prompt_kernel(
    A_x: jax.Array,
    A_mem0: jax.Array,
    A_Wq: jax.Array,
    A_Wk: jax.Array,
    A_Wv: jax.Array,
    A_Wo: jax.Array,
    A_seg_len,
    B_x: jax.Array,
    B_w1: jax.Array,
    B_w2: jax.Array,
    B_w3: jax.Array,
    B_w4: jax.Array,
    c: jax.Array,
    w_mod: jax.Array,
):
    assert A_seg_len == SEG and A_x.shape == (1, S, D) and A_mem0.shape == (1, M, D)
    hbm = pl.BlockSpec(memory_space=pl.ANY)
    vmem = pl.BlockSpec(memory_space=pltpu.VMEM)
    scratch = [
        pltpu.VMEM((NSEG, SEG, D), bf16),
        pltpu.VMEM((NSEG, M, D), bf16),
        pltpu.VMEM((NSEG * M // 2, D), u32),
        pltpu.VMEM((D, 4 * D), bf16),
        pltpu.VMEM((D, HG, E), bf16),
        pltpu.VMEM((D, HG, E), bf16),
        pltpu.VMEM((D, HG, E), bf16),
        pltpu.VMEM((H, D // 2, E), u32),
        pltpu.VMEM((H, D // 2, E), u32),
        pltpu.VMEM((H, D // 2, E), u32),
        pltpu.VMEM((H * E // 2, D), u32),
        pltpu.VMEM((D // 2, D), u32),
        pltpu.VMEM((D, D), bf16),
        pltpu.VMEM((D, F), bf16),
        pltpu.VMEM((F, D), bf16),
        pltpu.VMEM((3 * NP, NSEG, M, E), u32),
        pltpu.VMEM((8, 6 * D), f32),
        pltpu.VMEM((M, D), f32),
        pltpu.VMEM((TC, D), f32),
        pltpu.VMEM((2 * SEG, D), f32),
        pltpu.VMEM((2 * (M + SEG), 2 * (M + SEG)), f32),
        pltpu.VMEM((S, D), bf16),
        pltpu.VMEM((S, D), bf16),
        pltpu.VMEM((S + 16, D), f32),
        pltpu.VMEM((TB // 2, D), u32),
        pltpu.VMEM((TB // 2, F), u32),
        pltpu.VMEM((2, TB, D), bf16),
        pltpu.VMEM((8, E), u32),
        pltpu.VMEM((H * E // NG, D), bf16),
        pltpu.VMEM((D // NG, D), bf16),
        pltpu.SemaphoreType.DMA((13,)),
    ]
    out = pl.pallas_call(
        _kernel,
        out_shape=jax.ShapeDtypeStruct((S, D), bf16),
        in_specs=[hbm, vmem, hbm, hbm, hbm, hbm, hbm, hbm, hbm, hbm, vmem, hbm],
        out_specs=hbm,
        scratch_shapes=scratch,
        compiler_params=pltpu.CompilerParams(vmem_limit_bytes=126 * 1024 * 1024),
    )(A_x.reshape(NSEG, SEG, D), A_mem0.reshape(M, D), A_Wq, A_Wk, A_Wv,
      A_Wo.reshape(H * E, D), B_w1, B_w2, B_w3, B_w4, c, w_mod)
    return out.reshape(1, S, D)
```

```python
import functools

import jax
import jax.numpy as jnp
from jax import lax
import jax.experimental.pallas as pl
import jax.experimental.pallas.tpu as pltpu

bf16, f32, u32 = jnp.bfloat16, jnp.float32, jnp.uint32

S, D, H, E, M, SEG, F = 2048, 1024, 32, 128, 8, 32, 3584
NSEG = S // SEG
NP = H // 2
TC = SEG - M
HG = 8
NG = H // HG
TB = 128
NB = S // TB
FC = 512
NC = 3 * NG
BGR = 512
EPS = 1e-5
SCALE = E ** -0.5
_PHASES = "123"
_SCOPES = False
_N2 = NSEG // 2
_N3 = NB


def _scoped(name, fn):
    def wrapped(*a):
        if not _SCOPES:
            return fn(*a)
        with jax.named_scope(name):
            return fn(*a)
    return wrapped


def _pk(x):
    return pltpu.bitcast(x.astype(bf16), u32)


def _up(x):
    return pltpu.bitcast(x, bf16)


def _dot(a, b):
    return jnp.dot(a, b, preferred_element_type=f32)


def _ln(x):
    m = jnp.mean(x, axis=-1, keepdims=True)
    xc = x - m
    v = jnp.mean(xc * xc, axis=-1, keepdims=True)
    return xc * lax.rsqrt(v + EPS)


def _gelu(x):
    c = 0.7978845608028654
    return 0.5 * x * (1.0 + jnp.tanh(c * (x + 0.044715 * (x * x * x))))


def _mask_fill():
    n = 2 * (M + SEG)
    r = lax.broadcasted_iota(jnp.int32, (n, n), 0)
    c = lax.broadcasted_iota(jnp.int32, (n, n), 1)

    def headpos(i):
        head = jnp.where(i < 64, i >> 5, (i - 64) >> 3)
        pos = jnp.where(i < 64, i & 31, 32 + (i & 7))
        return head, pos

    hr, pr = headpos(r)
    hc, pc = headpos(c)
    same = hr == hc
    valid = same & ((pr < M) | (pr >= pc))
    return jnp.where(valid, 0.0, jnp.where(same, -1e9, -jnp.inf)).astype(f32)


def _kernel(x_hbm, mem0_hbm, wq_hbm, wk_hbm, wv_hbm, wo_hbm, w1_hbm, w2_hbm, w3_hbm,
            w4_hbm, c_hbm, wm_hbm,
            out_hbm,
            x_s, xpre_s, hpre_s, wm_s, stg, w_s, wo1_s,
            w2_s, w3_s, w4_s, pre_s, mod_s, mem_s, hn_s, aout_s, fill_s,
            x2_s, hb_s, t_s, y_s, u_s, o_s, zero_s, bg, c_s, mem0_s, sems):
    w_hbm = (wq_hbm, wk_hbm, wv_hbm)

    (SEM_C, SEM_MEM, SEM_XPRE, SEM_X, SEM_W2, SEM_W3, SEM_W4, SEM_STG, SEM_BG, SEM_OUT,
     SEM_WM) = (0, 1, 2, 3, 4, 5, 6, 7, 9, 11, 13)

    def copy(src, dst, k):
        return pltpu.make_async_copy(src, dst, sems.at[k])

    def w_copy(t, g, slot):
        return copy(w_hbm[t].at[:, pl.ds(pl.multiple_of(g * HG, HG), HG), :], stg.at[slot],
                    SEM_STG + slot)

    def bg_copy(src, b, slot):
        return copy(src.at[pl.ds(pl.multiple_of(b * BGR, BGR), BGR)], bg.at[slot], SEM_BG + slot)

    def mod_row(k):
        return mod_s[0:1, k * D:(k + 1) * D]

    def relayout(slot, c, i):
        v = pltpu.bitcast(jnp.swapaxes(stg[slot, pl.ds(i * 16, 16)], 0, 1), u32)
        r = i * 8 if isinstance(i, int) else pl.multiple_of(i * 8, 8)
        w_s[pl.ds(c * HG, HG), pl.ds(r, 8), :] = v
        z = v[0]
        for h in range(1, HG):
            z = z | v[h]
        return z

    def repack(slot, b, i):
        v = pltpu.bitcast(bg[slot, 16 * i:16 * i + 16, :], u32)
        wo1_s[pl.ds(pl.multiple_of(b * (BGR // 2) + 8 * i, 8), 8), :] = v
        z = v[:, 0:E]
        for j in range(1, D // E):
            z = z | v[:, j * E:(j + 1) * E]
        return z

    HD = D // 2
    cp_c = copy(c_hbm, c_s, SEM_C)
    cp_mem = copy(mem0_hbm, mem0_s, SEM_MEM)
    cp_xpre = copy(x_hbm.at[:, TC:SEG, :], xpre_s, SEM_XPRE)
    wm_cols = (0, D, HD, D + HD)
    cp_wm = [copy(wm_hbm.at[:, c0:c0 + HD], wm_s.at[:, c0:c0 + HD], SEM_WM + k)
             for k, c0 in enumerate(wm_cols)]
    w_copy(0, 0, 0).start()
    cp_xpre.start()
    cp_c.start()
    cp_mem.start()
    for cp in cp_wm:
        cp.start()
    w_copy(0, 1, 1).start()

    zero_s[...] = jnp.zeros(zero_s.shape, u32)
    fill_s[...] = _mask_fill()
    mod_s[...] = jnp.zeros(mod_s.shape, f32)
    aout_s[...] = jnp.zeros(aout_s.shape, f32)
    bg[1] = jnp.zeros(bg.shape[1:], bf16)

    w_copy(0, 0, 0).wait()

    def rl0_body(i, carry):
        for k in range(4):
            relayout(0, 0, 4 * i + k)
        return carry

    lax.fori_loop(0, D // 64, rl0_body, 0)

    cp_xpre.wait()

    def npre_body(i, carry):
        xr = xpre_s[pl.ds(pl.multiple_of(i * 8, 8), 8)].astype(f32).reshape(64, D)
        t_s[pl.ds(pl.multiple_of(i * 64, 64), 64), :] = _ln(xr)
        return carry

    lax.fori_loop(0, NSEG // 8, _scoped("npre", npre_body), 0)

    cp_c.wait()
    cp_mem.wait()
    mem_s[...] = mem0_s[...].astype(f32)
    cf = c_s[...].astype(f32)
    sc = cf * (1.0 / (1.0 + jnp.exp(-cf)))
    sc8 = jnp.broadcast_to(sc, (8, D)).astype(bf16)

    for half in range(2):
        for k in (2 * half, 2 * half + 1):
            c0 = wm_cols[k]
            cp_wm[k].wait()
            mod_s[:, c0:c0 + HD] = _dot(sc8, wm_s[:, c0:c0 + HD])
        cols = slice(half * HD, (half + 1) * HD)
        shift = mod_s[0:1, half * HD:(half + 1) * HD]
        scale1 = 1.0 + mod_s[0:1, D + half * HD:D + (half + 1) * HD]
        hpre_s[:, cols] = _pk(t_s[0:NSEG * M, cols] * scale1 + shift)

    t_s[0:8, :] = jnp.zeros((8, D), f32)
    t_s[S + 8:S + 16, :] = jnp.zeros((8, D), f32)

    def modulate_a(xr):
        return _ln(xr) * (1.0 + mod_row(1)) + mod_row(0)

    MB = 128
    cp_x = copy(x_hbm, x_s, SEM_X)
    cp_wm1 = copy(wm_hbm.at[:, 2 * D:6 * D], wm_s, SEM_WM)
    cp_w2 = copy(w2_hbm, w2_s, SEM_W2)
    cp_w3 = copy(w3_hbm, w3_s, SEM_W3)
    cp_w4 = copy(w4_hbm, w4_s, SEM_W4)

    def pre_pair(c, pp, side):
        ys = []
        for hh in range(2):
            blocks = []
            for mb in range(NSEG * M // MB):
                h = c * HG + 2 * pp + hh
                za = side() & zero_s[...]
                lo = w_s[h, 0:256, :]
                zb = side() & zero_s[...]
                hi = w_s[h, 256:512, :]
                w = jnp.concatenate([lo[0:8] | za, lo[8:], hi[0:8] | zb, hi[8:]], axis=0)
                blocks.append(_dot(_up(hpre_s[mb * MB // 2:(mb + 1) * MB // 2, :]), _up(w)))
            ys.append(jnp.concatenate(blocks, axis=0).reshape(NSEG, M, E))
        y = jnp.concatenate(ys, axis=1)
        pre_s[c * (HG // 2) + pp] = pltpu.bitcast(y.astype(bf16), u32)

    NWO = H * E // BGR
    NBG = NWO + D // BGR

    def p1_body(c, carry):
        slot = c % 2
        b = jnp.clip(c - 1, 0, NBG - 1)
        bslot = jnp.where(c == 0, 1, b % 2)

        for t in range(3):
            @pl.when((c + 2) // NG == t)
            def _():
                w_copy(t, (c + 2) % NG, slot).start()

        @pl.when(c < NWO)
        def _():
            bg_copy(wo_hbm, c, slot).start()

        @pl.when(jnp.logical_and(c >= NWO, c < NBG))
        def _():
            bg_copy(w1_hbm, c - NWO, slot).start()

        @pl.when(c == NC - 2)
        def _():
            cp_x.start()

        @pl.when(c == NC - 1)
        def _():
            cp_wm1.start()

        @pl.when(jnp.logical_and(c >= 1, c <= NBG))
        def _():
            bg_copy(wo_hbm, 0, bslot).wait()

        @pl.when(c + 1 < NC)
        def _():
            w_copy(0, 0, 1 - slot).wait()

        units = iter(range(D // 16))

        def side():
            i = next(units)
            z = relayout(1 - slot, c + 1, i)
            if i % 2 == 0:
                z = z | repack(bslot, b, i // 2)
            return z

        for pp in range(HG // 2):
            pre_pair(c, pp, side)
        return carry

    lax.fori_loop(0, NC, _scoped("p1", p1_body), 0)
    cp_x.wait()

    def h_rows(s):
        return modulate_a(x_s[s, 0:TC, :].astype(f32))

    hn_s[...] = h_rows(0)

    def chain_step(s, mem, htok, odef_prev):
        hs = jnp.concatenate([mem, htok], axis=0).astype(bf16)
        qkv = [[None] * 3 for _ in range(NP)]
        ps = [None] * NP
        os_ = [None] * H
        odef = [None] * H

        def proj(p):
            for t in range(3):
                a = _dot(hs, _up(w_s[t * H + 2 * p]))
                b = _dot(hs, _up(w_s[t * H + 2 * p + 1]))
                qkv[p][t] = _up(jnp.concatenate([_pk(a), _pk(b), pre_s[t * NP + p, s]], axis=0))

        def scores(p):
            sc_ = lax.dot_general(qkv[p][0], qkv[p][1], (((1,), (1,)), ((), ())),
                                  preferred_element_type=f32)
            fill = fill_s[...]
            sc_ = jnp.where(fill == 0.0, sc_ * SCALE, fill)
            m = jnp.max(sc_, axis=-1, keepdims=True)
            e = jnp.exp(sc_ - m)
            l = jnp.sum(e, axis=-1, keepdims=True)
            r = pl.reciprocal(l, approx=True)
            r = r * (2.0 - l * r)
            ps[p] = (e * r).astype(bf16)

        def fin(p):
            o = _dot(ps[p], qkv[p][2])
            for hh in range(2):
                h = 2 * p + hh
                rows = o[32 * hh:32 * hh + 32]
                odef[h] = o[64 + 8 * hh:72 + 8 * hh]
                if odef_prev is not None:
                    rows = jnp.concatenate([rows, odef_prev[h], odef[h]], axis=0)
                os_[h] = _pk(rows)

        acc = [None] * 8

        def wo(h0, h1, js):
            lhs = _up(jnp.concatenate(os_[h0:h1], axis=1))
            for j in js:
                part = _dot(lhs, _up(wo1_s[h0 * E // 2:h1 * E // 2, j * E:(j + 1) * E]))
                acc[j] = part if acc[j] is None else part + acc[j]

        for p in range(NP):
            proj(p)
            if p >= 1:
                scores(p - 1)
            if p >= 3:
                fin(p - 3)
        wo(0, 24, range(0, 2))
        scores(NP - 1)
        fin(NP - 3)
        wo(0, 24, range(2, 3))
        fin(NP - 2)
        wo(0, 24, range(3, 5))
        fin(NP - 1)
        wo(0, 24, range(5, 8))
        wo(24, 32, range(8))
        return jnp.concatenate(acc, axis=1), odef

    def mixer_in(i):
        r = pl.ds(pl.multiple_of(i * 64, 64), 64)
        xr = x_s[pl.ds(2 * i, 2)].astype(f32).reshape(2 * SEG, D)
        x2 = xr + mod_row(2) * aout_s[...]
        x2_s[r, :] = x2.astype(bf16)
        hb = _ln(x2) * (1.0 + mod_row(4)) + mod_row(3)
        hb_s[r, :] = hb.astype(bf16)
        t = _gelu(_dot(_ln(hb).astype(bf16), _up(wo1_s[H * E // 2:, :])))
        t_s[pl.ds(pl.multiple_of(i * 64 + 8, 8), 64), :] = t

    def p2_body(i, carry):
        @pl.when(i == 1)
        def _():
            cp_wm1.wait()
            mod_s[:, 2 * D:6 * D] = _dot(sc8, wm_s[...])

        @pl.when(i == 3)
        def _():
            cp_w2.start()
            cp_w3.start()
            cp_w4.start()

        sa_ = 2 * i
        sb_ = 2 * i + 1
        hb_tok = h_rows(sb_)
        oa, odef_a = chain_step(sa_, mem_s[...], hn_s[...], None)
        mixer_in(jnp.maximum(i - 1, 0))
        ob, _ = chain_step(sb_, oa[0:M], hb_tok, odef_a)
        mem_s[...] = ob[0:M]
        aout_s[0:TC, :] = oa[M:SEG]
        aout_s[TC:SEG, :] = ob[SEG:SEG + M]
        aout_s[SEG:SEG + TC, :] = ob[M:SEG]
        aout_s[SEG + TC:2 * SEG, :] = ob[SEG + M:SEG + 2 * M]
        hn_s[...] = h_rows(jnp.minimum(sb_ + 1, NSEG - 1))
        return carry

    if "2" in _PHASES:
        lax.fori_loop(0, _N2, _scoped("p2", p2_body), 0)
        mixer_in(NSEG // 2 - 1)
    else:
        cp_w2.start()
        cp_w3.start()
        cp_w4.start()
        cp_wm1.wait()
        cpd = copy(pre_s.at[0], pre_s.at[1], SEM_WM)
        cpd.start()
        cpd.wait()

    cp_w2.wait()
    cp_w3.wait()
    cp_w4.wait()

    def mix(j):
        r0 = pl.multiple_of(j * TB, TB)
        q = D // 4
        parts = []
        for k, sh in enumerate((-1, 1, -2, 2)):
            tt = t_s[pl.ds(r0, TB + 16), k * q:(k + 1) * q]
            parts.append(tt[8 + sh:8 + sh + TB])
        g = jnp.concatenate(parts, axis=1).astype(bf16)
        x1 = hb_s[pl.ds(r0, TB), :].astype(f32) + _dot(g, w2_s[...])
        return x1

    def out_copy(j, slot):
        return copy(o_s.at[slot], out_hbm.at[pl.ds(pl.multiple_of(j * TB, TB), TB)], SEM_OUT + slot)

    if "3" not in _PHASES:
        return

    x1_0 = mix(0)
    y_s[...] = _pk(_ln(x1_0))
    hb_s[0:TB, :] = x1_0.astype(bf16)

    def p3_body(j, carry):
        slot = j % 2

        @pl.when(j >= 2)
        def _():
            out_copy(j - 2, slot).wait()

        r = pl.ds(pl.multiple_of(j * TB, TB), TB)
        for cidx in range(F // FC):
            u = _gelu(_dot(_up(y_s[...]), w3_s[:, cidx * FC:(cidx + 1) * FC]))
            u_s[:, cidx * FC:(cidx + 1) * FC] = _pk(u)
        base = x2_s[r, :].astype(f32) + mod_row(5) * hb_s[r, :].astype(f32)
        jn = jnp.minimum(j + 1, NB - 1)
        x1n = mix(jn)
        h2 = _dot(_up(u_s[...]), w4_s[...])
        o_s[slot] = (base + mod_row(5) * h2).astype(bf16)
        y_s[...] = _pk(_ln(x1n))
        hb_s[pl.ds(pl.multiple_of(jn * TB, TB), TB), :] = x1n.astype(bf16)
        out_copy(j, slot).start()
        return carry

    lax.fori_loop(0, _N3, _scoped("p3", p3_body), 0)
    out_copy(NB - 2, 0).wait()
    out_copy(NB - 1, 1).wait()


@functools.partial(jax.jit, static_argnames=("A_seg_len",))
def pallas_adaLN_cond__memory_aug_recurrent_mem_tr__mixer_s_mlp__prompt_kernel(
    A_x: jax.Array,
    A_mem0: jax.Array,
    A_Wq: jax.Array,
    A_Wk: jax.Array,
    A_Wv: jax.Array,
    A_Wo: jax.Array,
    A_seg_len,
    B_x: jax.Array,
    B_w1: jax.Array,
    B_w2: jax.Array,
    B_w3: jax.Array,
    B_w4: jax.Array,
    c: jax.Array,
    w_mod: jax.Array,
):
    assert A_seg_len == SEG and A_x.shape == (1, S, D) and A_mem0.shape == (1, M, D)
    hbm = pl.BlockSpec(memory_space=pl.ANY)
    scratch = [
        pltpu.VMEM((NSEG, SEG, D), bf16),
        pltpu.VMEM((NSEG, M, D), bf16),
        pltpu.VMEM((NSEG * M // 2, D), u32),
        pltpu.VMEM((D, 4 * D), bf16),
        pltpu.VMEM((2, D, HG, E), bf16),
        pltpu.VMEM((3 * H + HG, D // 2, E), u32),
        pltpu.VMEM(((H * E + D) // 2, D), u32),
        pltpu.VMEM((D, D), bf16),
        pltpu.VMEM((D, F), bf16),
        pltpu.VMEM((F, D), bf16),
        pltpu.VMEM((3 * NP, NSEG, M, E), u32),
        pltpu.VMEM((8, 6 * D), f32),
        pltpu.VMEM((M, D), f32),
        pltpu.VMEM((TC, D), f32),
        pltpu.VMEM((2 * SEG, D), f32),
        pltpu.VMEM((2 * (M + SEG), 2 * (M + SEG)), f32),
        pltpu.VMEM((S, D), bf16),
        pltpu.VMEM((S, D), bf16),
        pltpu.VMEM((S + 16, D), f32),
        pltpu.VMEM((TB // 2, D), u32),
        pltpu.VMEM((TB // 2, F), u32),
        pltpu.VMEM((2, TB, D), bf16),
        pltpu.VMEM((8, E), u32),
        pltpu.VMEM((2, BGR, D), bf16),
        pltpu.VMEM((1, D), bf16),
        pltpu.VMEM((M, D), bf16),
        pltpu.SemaphoreType.DMA((17,)),
    ]
    out = pl.pallas_call(
        _kernel,
        out_shape=jax.ShapeDtypeStruct((S, D), bf16),
        in_specs=[hbm] * 12,
        out_specs=hbm,
        scratch_shapes=scratch,
        compiler_params=pltpu.CompilerParams(vmem_limit_bytes=126 * 1024 * 1024),
    )(A_x.reshape(NSEG, SEG, D), A_mem0.reshape(M, D), A_Wq, A_Wk, A_Wv,
      A_Wo.reshape(H * E, D), B_w1, B_w2, B_w3, B_w4, c, w_mod)
    return out.reshape(1, S, D)
```

```python
import functools

import jax
import jax.numpy as jnp
from jax import lax
import jax.experimental.pallas as pl
import jax.experimental.pallas.tpu as pltpu

bf16, f32, u32 = jnp.bfloat16, jnp.float32, jnp.uint32

S, D, H, E, M, SEG, F = 2048, 1024, 32, 128, 8, 32, 3584
NSEG = S // SEG
NP = H // 2
TC = SEG - M
HG = 8
NG = H // HG
TB = 128
NB = S // TB
FC = 512
NC = 3 * NG
BGR = 512
NR = 2 * (M + SEG)
XT = 1
EPS = 1e-5
SCALE = E ** -0.5
_PHASES = "123"
_SCOPES = False
_N2 = NSEG // 2
_N3 = NB


def _scoped(name, fn):
    def wrapped(*a):
        if not _SCOPES:
            return fn(*a)
        with jax.named_scope(name):
            return fn(*a)
    return wrapped


def _pk(x):
    return pltpu.bitcast(x.astype(bf16), u32)


def _up(x):
    return pltpu.bitcast(x, bf16)


def _dot(a, b):
    return jnp.dot(a, b, preferred_element_type=f32)


def _ln(x):
    m = jnp.mean(x, axis=-1, keepdims=True)
    xc = x - m
    v = jnp.mean(xc * xc, axis=-1, keepdims=True)
    return xc * lax.rsqrt(v + EPS)


def _gelu(x):
    c = 0.7978845608028654
    return 0.5 * x * (1.0 + jnp.tanh(c * (x + 0.044715 * (x * x * x))))


def _mask_fill():
    shape = (NR, E if XT else NR)
    r = lax.broadcasted_iota(jnp.int32, shape, 0)
    c = lax.broadcasted_iota(jnp.int32, shape, 1)

    def headpos(i):
        head = jnp.where(i < 64, i >> 5, (i - 64) >> 3)
        pos = jnp.where(i < 64, i & 31, 32 + (i & 7))
        return head, pos

    hr, pr = headpos(r)
    hc, pc = headpos(c)
    same = hr == hc
    valid = same & ((pr < M) | (pr >= pc))
    return jnp.where(valid, 0.0, jnp.where(same, -1e9, -jnp.inf)).astype(f32)


def _kernel(x_hbm, mem0_hbm, wq_hbm, wk_hbm, wv_hbm, wo_hbm, w1_hbm, w2_hbm, w3_hbm,
            w4_hbm, c_hbm, wm_hbm,
            out_hbm,
            x_s, xpre_s, hpre_s, wm_s, stg, w_s, wo1_s,
            w2_s, w3_s, w4_s, pre_s, mod_s, mem_s, hn_s, aout_s, fill_s,
            x2_s, hb_s, t_s, y_s, u_s, o_s, zero_s, bg, c_s, mem0_s, sems):
    w_hbm = (wq_hbm, wk_hbm, wv_hbm)

    (SEM_C, SEM_MEM, SEM_XPRE, SEM_X, SEM_W2, SEM_W3, SEM_W4, SEM_STG, SEM_BG, SEM_OUT,
     SEM_WM) = (0, 1, 2, 3, 4, 5, 6, 7, 9, 11, 13)

    def copy(src, dst, k):
        return pltpu.make_async_copy(src, dst, sems.at[k])

    def w_copy(t, g, slot):
        return copy(w_hbm[t].at[:, pl.ds(pl.multiple_of(g * HG, HG), HG), :], stg.at[slot],
                    SEM_STG + slot)

    def bg_copy(src, b, slot):
        return copy(src.at[pl.ds(pl.multiple_of(b * BGR, BGR), BGR)], bg.at[slot], SEM_BG + slot)

    def mod_row(k):
        return mod_s[0:1, k * D:(k + 1) * D]

    def relayout(slot, c, i):
        v = pltpu.bitcast(jnp.swapaxes(stg[slot, pl.ds(i * 16, 16)], 0, 1), u32)
        r = i * 8 if isinstance(i, int) else pl.multiple_of(i * 8, 8)
        w_s[pl.ds(c * HG, HG), pl.ds(r, 8), :] = v
        z = v[0]
        for h in range(1, HG):
            z = z | v[h]
        return z

    def repack(slot, b, i):
        v = pltpu.bitcast(bg[slot, 16 * i:16 * i + 16, :], u32)
        wo1_s[pl.ds(pl.multiple_of(b * (BGR // 2) + 8 * i, 8), 8), :] = v
        z = v[:, 0:E]
        for j in range(1, D // E):
            z = z | v[:, j * E:(j + 1) * E]
        return z

    HD = D // 2
    cp_c = copy(c_hbm, c_s, SEM_C)
    cp_mem = copy(mem0_hbm, mem0_s, SEM_MEM)
    cp_xpre = copy(x_hbm.at[:, TC:SEG, :], xpre_s, SEM_XPRE)
    wm_cols = (0, D, HD, D + HD)
    cp_wm = [copy(wm_hbm.at[:, c0:c0 + HD], wm_s.at[:, c0:c0 + HD], SEM_WM + k)
             for k, c0 in enumerate(wm_cols)]
    w_copy(0, 0, 0).start()
    cp_xpre.start()
    cp_c.start()
    cp_mem.start()
    for cp in cp_wm:
        cp.start()
    w_copy(0, 1, 1).start()

    zero_s[...] = jnp.zeros(zero_s.shape, u32)
    fill_s[...] = _mask_fill()
    mod_s[...] = jnp.zeros(mod_s.shape, f32)
    aout_s[...] = jnp.zeros(aout_s.shape, f32)
    bg[1] = jnp.zeros(bg.shape[1:], bf16)

    w_copy(0, 0, 0).wait()

    def rl0_body(i, carry):
        for k in range(4):
            relayout(0, 0, 4 * i + k)
        return carry

    lax.fori_loop(0, D // 64, rl0_body, 0)

    cp_xpre.wait()

    def npre_body(i, carry):
        xr = xpre_s[pl.ds(pl.multiple_of(i * 8, 8), 8)].astype(f32).reshape(64, D)
        t_s[pl.ds(pl.multiple_of(i * 64, 64), 64), :] = _ln(xr)
        return carry

    lax.fori_loop(0, NSEG // 8, _scoped("npre", npre_body), 0)

    cp_c.wait()
    cp_mem.wait()
    mem_s[...] = mem0_s[...].astype(f32)
    cf = c_s[...].astype(f32)
    sc = cf * (1.0 / (1.0 + jnp.exp(-cf)))
    sc8 = jnp.broadcast_to(sc, (8, D)).astype(bf16)

    for half in range(2):
        for k in (2 * half, 2 * half + 1):
            c0 = wm_cols[k]
            cp_wm[k].wait()
            mod_s[:, c0:c0 + HD] = _dot(sc8, wm_s[:, c0:c0 + HD])
        cols = slice(half * HD, (half + 1) * HD)
        shift = mod_s[0:1, half * HD:(half + 1) * HD]
        scale1 = 1.0 + mod_s[0:1, D + half * HD:D + (half + 1) * HD]
        hpre_s[:, cols] = _pk(t_s[0:NSEG * M, cols] * scale1 + shift)

    t_s[0:8, :] = jnp.zeros((8, D), f32)
    t_s[S + 8:S + 16, :] = jnp.zeros((8, D), f32)

    def modulate_a(xr):
        return _ln(xr) * (1.0 + mod_row(1)) + mod_row(0)

    MB = 128
    cp_x = copy(x_hbm, x_s, SEM_X)
    cp_wm1 = copy(wm_hbm.at[:, 2 * D:6 * D], wm_s, SEM_WM)
    cp_w2 = copy(w2_hbm, w2_s, SEM_W2)
    cp_w3 = copy(w3_hbm, w3_s, SEM_W3)
    cp_w4 = copy(w4_hbm, w4_s, SEM_W4)

    def pre_pair(c, pp, side):
        ys = []
        for hh in range(2):
            blocks = []
            for mb in range(NSEG * M // MB):
                h = c * HG + 2 * pp + hh
                za = side() & zero_s[...]
                lo = w_s[h, 0:256, :]
                zb = side() & zero_s[...]
                hi = w_s[h, 256:512, :]
                w = jnp.concatenate([lo[0:8] | za, lo[8:], hi[0:8] | zb, hi[8:]], axis=0)
                blocks.append(_dot(_up(hpre_s[mb * MB // 2:(mb + 1) * MB // 2, :]), _up(w)))
            ys.append(jnp.concatenate(blocks, axis=0).reshape(NSEG, M, E))
        y = jnp.concatenate(ys, axis=1)
        pre_s[c * (HG // 2) + pp] = pltpu.bitcast(y.astype(bf16), u32)

    NWO = H * E // BGR
    NBG = NWO + D // BGR

    def p1_body(c, carry):
        slot = c % 2
        b = jnp.clip(c - 1, 0, NBG - 1)
        bslot = jnp.where(c == 0, 1, b % 2)

        for t in range(3):
            @pl.when((c + 2) // NG == t)
            def _():
                w_copy(t, (c + 2) % NG, slot).start()

        @pl.when(c < NWO)
        def _():
            bg_copy(wo_hbm, c, slot).start()

        @pl.when(jnp.logical_and(c >= NWO, c < NBG))
        def _():
            bg_copy(w1_hbm, c - NWO, slot).start()

        @pl.when(c == NC - 2)
        def _():
            cp_x.start()

        @pl.when(c == NC - 1)
        def _():
            cp_wm1.start()

        @pl.when(jnp.logical_and(c >= 1, c <= NBG))
        def _():
            bg_copy(wo_hbm, 0, bslot).wait()

        @pl.when(c + 1 < NC)
        def _():
            w_copy(0, 0, 1 - slot).wait()

        units = iter(range(D // 16))

        def side():
            i = next(units)
            z = relayout(1 - slot, c + 1, i)
            if i % 2 == 0:
                z = z | repack(bslot, b, i // 2)
            return z

        for pp in range(HG // 2):
            pre_pair(c, pp, side)
        return carry

    lax.fori_loop(0, NC, _scoped("p1", p1_body), 0)
    cp_x.wait()

    def h_rows(s):
        return modulate_a(x_s[s, 0:TC, :].astype(f32))

    hn_s[...] = h_rows(0)

    def chain_step(s, mem, htok, odef_prev):
        hs = jnp.concatenate([mem, htok], axis=0).astype(bf16)
        qkv = [[None] * 3 for _ in range(NP)]
        ps = [None] * NP
        os_ = [None] * H
        odef = [None] * H

        def proj(p):
            for t in range(3):
                a = _dot(hs, _up(w_s[t * H + 2 * p]))
                b = _dot(hs, _up(w_s[t * H + 2 * p + 1]))
                pre = pre_s[t * NP + p, s]
                if t == 1 and XT:
                    kf = jnp.concatenate([a, b, _up(pre).astype(f32), jnp.zeros((E - NR, E), f32)],
                                         axis=0)
                    qkv[p][t] = kf.T.astype(bf16)
                    continue
                parts = [_pk(a), _pk(b), pre]
                if t == 2 and XT:
                    parts += [zero_s[...] if XT == 2 else jnp.zeros((8, E), u32)] * ((E - NR) // 16)
                qkv[p][t] = _up(jnp.concatenate(parts, axis=0))

        def scores(p):
            if XT:
                sc_ = _dot(qkv[p][0], qkv[p][1])
            else:
                sc_ = lax.dot_general(qkv[p][0], qkv[p][1], (((1,), (1,)), ((), ())),
                                      preferred_element_type=f32)
            fill = fill_s[...]
            sc_ = jnp.where(fill == 0.0, sc_ * SCALE, fill)
            m = jnp.max(sc_, axis=-1, keepdims=True)
            e = jnp.exp(sc_ - m)
            l = jnp.sum(e, axis=-1, keepdims=True)
            r = pl.reciprocal(l, approx=True)
            r = r * (2.0 - l * r)
            ps[p] = (e * r).astype(bf16)

        def fin(p):
            o = _dot(ps[p], qkv[p][2])
            for hh in range(2):
                h = 2 * p + hh
                rows = o[32 * hh:32 * hh + 32]
                odef[h] = o[64 + 8 * hh:72 + 8 * hh]
                if odef_prev is not None:
                    rows = jnp.concatenate([rows, odef_prev[h], odef[h]], axis=0)
                os_[h] = _pk(rows)

        acc = [None] * 8

        def wo(h0, h1, js):
            lhs = _up(jnp.concatenate(os_[h0:h1], axis=1))
            for j in js:
                part = _dot(lhs, _up(wo1_s[h0 * E // 2:h1 * E // 2, j * E:(j + 1) * E]))
                acc[j] = part if acc[j] is None else part + acc[j]

        for p in range(NP):
            proj(p)
            if p >= 1:
                scores(p - 1)
            if p >= 3:
                fin(p - 3)
        wo(0, 24, range(0, 2))
        scores(NP - 1)
        fin(NP - 3)
        wo(0, 24, range(2, 3))
        fin(NP - 2)
        wo(0, 24, range(3, 5))
        fin(NP - 1)
        wo(0, 24, range(5, 8))
        wo(24, 32, range(8))
        return jnp.concatenate(acc, axis=1), odef

    def mixer_in(i):
        r = pl.ds(pl.multiple_of(i * 64, 64), 64)
        xr = x_s[pl.ds(2 * i, 2)].astype(f32).reshape(2 * SEG, D)
        x2 = xr + mod_row(2) * aout_s[...]
        x2_s[r, :] = x2.astype(bf16)
        hb = _ln(x2) * (1.0 + mod_row(4)) + mod_row(3)
        hb_s[r, :] = hb.astype(bf16)
        t = _gelu(_dot(_ln(hb).astype(bf16), _up(wo1_s[H * E // 2:, :])))
        t_s[pl.ds(pl.multiple_of(i * 64 + 8, 8), 64), :] = t

    def p2_body(i, carry):
        @pl.when(i == 1)
        def _():
            cp_wm1.wait()
            mod_s[:, 2 * D:6 * D] = _dot(sc8, wm_s[...])

        @pl.when(i == 3)
        def _():
            cp_w2.start()
            cp_w3.start()
            cp_w4.start()

        sa_ = 2 * i
        sb_ = 2 * i + 1
        hb_tok = h_rows(sb_)
        oa, odef_a = chain_step(sa_, mem_s[...], hn_s[...], None)
        mixer_in(jnp.maximum(i - 1, 0))
        ob, _ = chain_step(sb_, oa[0:M], hb_tok, odef_a)
        mem_s[...] = ob[0:M]
        aout_s[0:TC, :] = oa[M:SEG]
        aout_s[TC:SEG, :] = ob[SEG:SEG + M]
        aout_s[SEG:SEG + TC, :] = ob[M:SEG]
        aout_s[SEG + TC:2 * SEG, :] = ob[SEG + M:SEG + 2 * M]
        hn_s[...] = h_rows(jnp.minimum(sb_ + 1, NSEG - 1))
        return carry

    if "2" in _PHASES:
        lax.fori_loop(0, _N2, _scoped("p2", p2_body), 0)
        mixer_in(NSEG // 2 - 1)
    else:
        cp_w2.start()
        cp_w3.start()
        cp_w4.start()
        cp_wm1.wait()
        cpd = copy(pre_s.at[0], pre_s.at[1], SEM_WM)
        cpd.start()
        cpd.wait()

    cp_w2.wait()
    cp_w3.wait()
    cp_w4.wait()

    def mix(j):
        r0 = pl.multiple_of(j * TB, TB)
        q = D // 4
        parts = []
        for k, sh in enumerate((-1, 1, -2, 2)):
            tt = t_s[pl.ds(r0, TB + 16), k * q:(k + 1) * q]
            parts.append(tt[8 + sh:8 + sh + TB])
        g = jnp.concatenate(parts, axis=1).astype(bf16)
        x1 = hb_s[pl.ds(r0, TB), :].astype(f32) + _dot(g, w2_s[...])
        return x1

    def out_copy(j, slot):
        return copy(o_s.at[slot], out_hbm.at[pl.ds(pl.multiple_of(j * TB, TB), TB)], SEM_OUT + slot)

    if "3" not in _PHASES:
        return

    x1_0 = mix(0)
    y_s[...] = _pk(_ln(x1_0))
    hb_s[0:TB, :] = x1_0.astype(bf16)

    def p3_body(j, carry):
        slot = j % 2

        @pl.when(j >= 2)
        def _():
            out_copy(j - 2, slot).wait()

        r = pl.ds(pl.multiple_of(j * TB, TB), TB)
        for cidx in range(F // FC):
            u = _gelu(_dot(_up(y_s[...]), w3_s[:, cidx * FC:(cidx + 1) * FC]))
            u_s[:, cidx * FC:(cidx + 1) * FC] = _pk(u)
        base = x2_s[r, :].astype(f32) + mod_row(5) * hb_s[r, :].astype(f32)
        jn = jnp.minimum(j + 1, NB - 1)
        x1n = mix(jn)
        h2 = _dot(_up(u_s[...]), w4_s[...])
        o_s[slot] = (base + mod_row(5) * h2).astype(bf16)
        y_s[...] = _pk(_ln(x1n))
        hb_s[pl.ds(pl.multiple_of(jn * TB, TB), TB), :] = x1n.astype(bf16)
        out_copy(j, slot).start()
        return carry

    lax.fori_loop(0, _N3, _scoped("p3", p3_body), 0)
    out_copy(NB - 2, 0).wait()
    out_copy(NB - 1, 1).wait()


@functools.partial(jax.jit, static_argnames=("A_seg_len",))
def pallas_adaLN_cond__memory_aug_recurrent_mem_tr__mixer_s_mlp__prompt_kernel(
    A_x: jax.Array,
    A_mem0: jax.Array,
    A_Wq: jax.Array,
    A_Wk: jax.Array,
    A_Wv: jax.Array,
    A_Wo: jax.Array,
    A_seg_len,
    B_x: jax.Array,
    B_w1: jax.Array,
    B_w2: jax.Array,
    B_w3: jax.Array,
    B_w4: jax.Array,
    c: jax.Array,
    w_mod: jax.Array,
):
    assert A_seg_len == SEG and A_x.shape == (1, S, D) and A_mem0.shape == (1, M, D)
    hbm = pl.BlockSpec(memory_space=pl.ANY)
    scratch = [
        pltpu.VMEM((NSEG, SEG, D), bf16),
        pltpu.VMEM((NSEG, M, D), bf16),
        pltpu.VMEM((NSEG * M // 2, D), u32),
        pltpu.VMEM((D, 4 * D), bf16),
        pltpu.VMEM((2, D, HG, E), bf16),
        pltpu.VMEM((3 * H + HG, D // 2, E), u32),
        pltpu.VMEM(((H * E + D) // 2, D), u32),
        pltpu.VMEM((D, D), bf16),
        pltpu.VMEM((D, F), bf16),
        pltpu.VMEM((F, D), bf16),
        pltpu.VMEM((3 * NP, NSEG, M, E), u32),
        pltpu.VMEM((8, 6 * D), f32),
        pltpu.VMEM((M, D), f32),
        pltpu.VMEM((TC, D), f32),
        pltpu.VMEM((2 * SEG, D), f32),
        pltpu.VMEM((NR, E if XT else NR), f32),
        pltpu.VMEM((S, D), bf16),
        pltpu.VMEM((S, D), bf16),
        pltpu.VMEM((S + 16, D), f32),
        pltpu.VMEM((TB // 2, D), u32),
        pltpu.VMEM((TB // 2, F), u32),
        pltpu.VMEM((2, TB, D), bf16),
        pltpu.VMEM((8, E), u32),
        pltpu.VMEM((2, BGR, D), bf16),
        pltpu.VMEM((1, D), bf16),
        pltpu.VMEM((M, D), bf16),
        pltpu.SemaphoreType.DMA((17,)),
    ]
    out = pl.pallas_call(
        _kernel,
        out_shape=jax.ShapeDtypeStruct((S, D), bf16),
        in_specs=[hbm] * 12,
        out_specs=hbm,
        scratch_shapes=scratch,
        compiler_params=pltpu.CompilerParams(vmem_limit_bytes=126 * 1024 * 1024),
    )(A_x.reshape(NSEG, SEG, D), A_mem0.reshape(M, D), A_Wq, A_Wk, A_Wv,
      A_Wo.reshape(H * E, D), B_w1, B_w2, B_w3, B_w4, c, w_mod)
    return out.reshape(1, S, D)
```

```python
import functools

import jax
import jax.numpy as jnp
from jax import lax
import jax.experimental.pallas as pl
import jax.experimental.pallas.tpu as pltpu

bf16, f32, u32 = jnp.bfloat16, jnp.float32, jnp.uint32

S, D, H, E, M, SEG, F = 2048, 1024, 32, 128, 8, 32, 3584
NSEG = S // SEG
NP = H // 2
TC = SEG - M
HG = 8
NG = H // HG
TB = 128
NB = S // TB
FC = 512
NC = 3 * NG
BGR = 512
NR = 2 * (M + SEG)
HS_REF = 0
LAG_S = 1
LAG_O = 3
ORDER = 2
PINS = ()
EPS = 1e-5
SCALE = E ** -0.5
_PHASES = "123"
_SCOPES = False
_N2 = NSEG // 2
_N3 = NB


def _scoped(name, fn):
    def wrapped(*a):
        if not _SCOPES:
            return fn(*a)
        with jax.named_scope(name):
            return fn(*a)
    return wrapped


def _pk(x):
    return pltpu.bitcast(x.astype(bf16), u32)


def _up(x):
    return pltpu.bitcast(x, bf16)


def _dot(a, b):
    return jnp.dot(a, b, preferred_element_type=f32)


def _ln(x):
    m = jnp.mean(x, axis=-1, keepdims=True)
    xc = x - m
    v = jnp.mean(xc * xc, axis=-1, keepdims=True)
    return xc * lax.rsqrt(v + EPS)


def _gelu(x):
    c = 0.7978845608028654
    return 0.5 * x * (1.0 + jnp.tanh(c * (x + 0.044715 * (x * x * x))))


def _mask_fill():
    shape = (NR, E)
    r = lax.broadcasted_iota(jnp.int32, shape, 0)
    c = lax.broadcasted_iota(jnp.int32, shape, 1)

    def headpos(i):
        head = jnp.where(i < 64, i >> 5, (i - 64) >> 3)
        pos = jnp.where(i < 64, i & 31, 32 + (i & 7))
        return head, pos

    hr, pr = headpos(r)
    hc, pc = headpos(c)
    same = hr == hc
    valid = same & ((pr < M) | (pr >= pc))
    return jnp.where(valid, 0.0, jnp.where(same, -1e9, -jnp.inf)).astype(f32)


def _kernel(x_hbm, mem0_hbm, wq_hbm, wk_hbm, wv_hbm, wo_hbm, w1_hbm, w2_hbm, w3_hbm,
            w4_hbm, c_hbm, wm_hbm,
            out_hbm,
            x_s, xpre_s, hpre_s, wm_s, stg, w_s, wo1_s,
            w2_s, w3_s, w4_s, pre_s, mod_s, mem_s, hn_s, aout_s, fill_s,
            x2_s, hb_s, t_s, y_s, u_s, o_s, zero_s, bg, c_s, mem0_s, hs_s, sems):
    w_hbm = (wq_hbm, wk_hbm, wv_hbm)

    (SEM_C, SEM_MEM, SEM_XPRE, SEM_X, SEM_W2, SEM_W3, SEM_W4, SEM_STG, SEM_BG, SEM_OUT,
     SEM_WM) = (0, 1, 2, 3, 4, 5, 6, 7, 9, 11, 13)

    def copy(src, dst, k):
        return pltpu.make_async_copy(src, dst, sems.at[k])

    def w_copy(t, g, slot):
        return copy(w_hbm[t].at[:, pl.ds(pl.multiple_of(g * HG, HG), HG), :], stg.at[slot],
                    SEM_STG + slot)

    def bg_copy(src, b, slot):
        return copy(src.at[pl.ds(pl.multiple_of(b * BGR, BGR), BGR)], bg.at[slot], SEM_BG + slot)

    def mod_row(k):
        return mod_s[0:1, k * D:(k + 1) * D]

    def relayout(slot, c, i):
        v = pltpu.bitcast(jnp.swapaxes(stg[slot, pl.ds(i * 16, 16)], 0, 1), u32)
        r = i * 8 if isinstance(i, int) else pl.multiple_of(i * 8, 8)
        w_s[pl.ds(c * HG, HG), pl.ds(r, 8), :] = v
        z = v[0]
        for h in range(1, HG):
            z = z | v[h]
        return z

    def repack(slot, b, i):
        v = pltpu.bitcast(bg[slot, 16 * i:16 * i + 16, :], u32)
        wo1_s[pl.ds(pl.multiple_of(b * (BGR // 2) + 8 * i, 8), 8), :] = v
        z = v[:, 0:E]
        for j in range(1, D // E):
            z = z | v[:, j * E:(j + 1) * E]
        return z

    HD = D // 2
    cp_c = copy(c_hbm, c_s, SEM_C)
    cp_mem = copy(mem0_hbm, mem0_s, SEM_MEM)
    cp_xpre = copy(x_hbm.at[:, TC:SEG, :], xpre_s, SEM_XPRE)
    wm_cols = (0, D, HD, D + HD)
    cp_wm = [copy(wm_hbm.at[:, c0:c0 + HD], wm_s.at[:, c0:c0 + HD], SEM_WM + k)
             for k, c0 in enumerate(wm_cols)]
    w_copy(0, 0, 0).start()
    cp_xpre.start()
    cp_c.start()
    cp_mem.start()
    for cp in cp_wm:
        cp.start()
    w_copy(0, 1, 1).start()

    zero_s[...] = jnp.zeros(zero_s.shape, u32)
    fill_s[...] = _mask_fill()
    mod_s[...] = jnp.zeros(mod_s.shape, f32)
    aout_s[...] = jnp.zeros(aout_s.shape, f32)
    bg[1] = jnp.zeros(bg.shape[1:], bf16)

    w_copy(0, 0, 0).wait()

    def rl0_body(i, carry):
        for k in range(4):
            relayout(0, 0, 4 * i + k)
        return carry

    lax.fori_loop(0, D // 64, rl0_body, 0)

    cp_xpre.wait()

    def npre_body(i, carry):
        xr = xpre_s[pl.ds(pl.multiple_of(i * 8, 8), 8)].astype(f32).reshape(64, D)
        t_s[pl.ds(pl.multiple_of(i * 64, 64), 64), :] = _ln(xr)
        return carry

    lax.fori_loop(0, NSEG // 8, _scoped("npre", npre_body), 0)

    cp_c.wait()
    cp_mem.wait()
    mem_s[...] = mem0_s[...].astype(f32)
    cf = c_s[...].astype(f32)
    sc = cf * (1.0 / (1.0 + jnp.exp(-cf)))
    sc8 = jnp.broadcast_to(sc, (8, D)).astype(bf16)

    for half in range(2):
        for k in (2 * half, 2 * half + 1):
            c0 = wm_cols[k]
            cp_wm[k].wait()
            mod_s[:, c0:c0 + HD] = _dot(sc8, wm_s[:, c0:c0 + HD])
        cols = slice(half * HD, (half + 1) * HD)
        shift = mod_s[0:1, half * HD:(half + 1) * HD]
        scale1 = 1.0 + mod_s[0:1, D + half * HD:D + (half + 1) * HD]
        hpre_s[:, cols] = _pk(t_s[0:NSEG * M, cols] * scale1 + shift)

    t_s[0:8, :] = jnp.zeros((8, D), f32)
    t_s[S + 8:S + 16, :] = jnp.zeros((8, D), f32)

    def modulate_a(xr):
        return _ln(xr) * (1.0 + mod_row(1)) + mod_row(0)

    MB = 128
    cp_x = copy(x_hbm, x_s, SEM_X)
    cp_wm1 = copy(wm_hbm.at[:, 2 * D:6 * D], wm_s, SEM_WM)
    cp_w2 = copy(w2_hbm, w2_s, SEM_W2)
    cp_w3 = copy(w3_hbm, w3_s, SEM_W3)
    cp_w4 = copy(w4_hbm, w4_s, SEM_W4)

    def pre_pair(c, pp, side):
        ys = []
        for hh in range(2):
            blocks = []
            for mb in range(NSEG * M // MB):
                h = c * HG + 2 * pp + hh
                za = side() & zero_s[...]
                lo = w_s[h, 0:256, :]
                zb = side() & zero_s[...]
                hi = w_s[h, 256:512, :]
                w = jnp.concatenate([lo[0:8] | za, lo[8:], hi[0:8] | zb, hi[8:]], axis=0)
                blocks.append(_dot(_up(hpre_s[mb * MB // 2:(mb + 1) * MB // 2, :]), _up(w)))
            ys.append(jnp.concatenate(blocks, axis=0).reshape(NSEG, M, E))
        y = jnp.concatenate(ys, axis=1)
        pre_s[c * (HG // 2) + pp] = pltpu.bitcast(y.astype(bf16), u32)

    NWO = H * E // BGR
    NBG = NWO + D // BGR

    def p1_body(c, carry):
        slot = c % 2
        b = jnp.clip(c - 1, 0, NBG - 1)
        bslot = jnp.where(c == 0, 1, b % 2)

        for t in range(3):
            @pl.when((c + 2) // NG == t)
            def _():
                w_copy(t, (c + 2) % NG, slot).start()

        @pl.when(c < NWO)
        def _():
            bg_copy(wo_hbm, c, slot).start()

        @pl.when(jnp.logical_and(c >= NWO, c < NBG))
        def _():
            bg_copy(w1_hbm, c - NWO, slot).start()

        @pl.when(c == NC - 2)
        def _():
            cp_x.start()

        @pl.when(c == NC - 1)
        def _():
            cp_wm1.start()

        @pl.when(jnp.logical_and(c >= 1, c <= NBG))
        def _():
            bg_copy(wo_hbm, 0, bslot).wait()

        @pl.when(c + 1 < NC)
        def _():
            w_copy(0, 0, 1 - slot).wait()

        units = iter(range(D // 16))

        def side():
            i = next(units)
            z = relayout(1 - slot, c + 1, i)
            if i % 2 == 0:
                z = z | repack(bslot, b, i // 2)
            return z

        for pp in range(HG // 2):
            pre_pair(c, pp, side)
        return carry

    lax.fori_loop(0, NC, _scoped("p1", p1_body), 0)
    cp_x.wait()

    def h_rows(s):
        return modulate_a(x_s[s, 0:TC, :].astype(f32))

    hn_s[...] = h_rows(0)

    def chain_step(s, mem, htok, odef_prev, pins=None):
        hs_v = jnp.concatenate([mem, htok], axis=0).astype(bf16)
        if HS_REF:
            hs_r = hs_s.at[0 if odef_prev is None else 1]
            hs_r[...] = pltpu.bitcast(hs_v, u32)
        qkv = [[None] * 3 for _ in range(NP)]
        ps = [None] * NP
        os_ = [None] * H
        odef = [None] * H

        def proj(p, ts=(0, 1, 2)):
            for t in ts:
                wa = w_s[t * H + 2 * p]
                if pins and t == 0 and p in pins:
                    wa = jnp.concatenate([wa[0:8] | (pins[p]() & zero_s[...]), wa[8:]], axis=0)
                a = _dot(_up(hs_r[...]) if HS_REF else hs_v, _up(wa))
                b = _dot(_up(hs_r[...]) if HS_REF else hs_v, _up(w_s[t * H + 2 * p + 1]))
                pre = pre_s[t * NP + p, s]
                if t == 1:
                    kf = jnp.concatenate([a, b, _up(pre).astype(f32), jnp.zeros((E - NR, E), f32)],
                                         axis=0)
                    qkv[p][t] = kf.T.astype(bf16)
                    continue
                parts = [_pk(a), _pk(b), pre]
                if t == 2:
                    parts.append(jnp.zeros(((E - NR) // 2, E), u32))
                qkv[p][t] = _up(jnp.concatenate(parts, axis=0))

        def scores(p):
            sc_ = _dot(qkv[p][0], qkv[p][1])
            fill = fill_s[...]
            sc_ = jnp.where(fill == 0.0, sc_ * SCALE, fill)
            m = jnp.max(sc_, axis=-1, keepdims=True)
            e = jnp.exp(sc_ - m)
            l = jnp.sum(e, axis=-1, keepdims=True)
            r = pl.reciprocal(l, approx=True)
            r = r * (2.0 - l * r)
            ps[p] = (e * r).astype(bf16)

        def fin(p):
            o = _dot(ps[p], qkv[p][2])
            for hh in range(2):
                h = 2 * p + hh
                rows = o[32 * hh:32 * hh + 32]
                odef[h] = o[64 + 8 * hh:72 + 8 * hh]
                if odef_prev is not None:
                    rows = jnp.concatenate([rows, odef_prev[h], odef[h]], axis=0)
                os_[h] = _pk(rows)

        acc = [None] * 8

        def wo(h0, h1, js):
            lhs = _up(jnp.concatenate(os_[h0:h1], axis=1))
            for j in js:
                part = _dot(lhs, _up(wo1_s[h0 * E // 2:h1 * E // 2, j * E:(j + 1) * E]))
                acc[j] = part if acc[j] is None else part + acc[j]

        for p in range(NP):
            if ORDER == 0:
                proj(p)
                if p >= LAG_S:
                    scores(p - LAG_S)
                if p >= LAG_O:
                    fin(p - LAG_O)
            elif ORDER == 1:
                proj(p, (1, 0))
                if p >= LAG_O:
                    fin(p - LAG_O)
                proj(p, (2,))
                if p >= LAG_S:
                    scores(p - LAG_S)
            elif ORDER == 2:
                proj(p, (1,))
                if p >= LAG_S:
                    scores(p - LAG_S)
                proj(p, (0,))
                if p >= LAG_O:
                    fin(p - LAG_O)
                proj(p, (2,))
            else:
                proj(p, (1, 0, 2))
                if p >= LAG_O:
                    fin(p - LAG_O)
                if p >= LAG_S:
                    scores(p - LAG_S)
        tail = []
        for k in range(LAG_O):
            step = []
            if NP - LAG_S + k < NP:
                step.append(functools.partial(scores, NP - LAG_S + k))
            step.append(functools.partial(fin, NP - LAG_O + k))
            tail.append(step)
        hsplit = min(24, 2 * (NP - LAG_O))
        cuts = {3: (2, 3, 5), 2: (2, 5), 4: (1, 2, 4, 6), 5: (1, 2, 3, 4, 6)}[LAG_O]
        j0 = 0
        for k, step in enumerate(tail):
            wo(0, hsplit, range(j0, cuts[k]))
            j0 = cuts[k]
            for f in step:
                f()
        wo(0, hsplit, range(j0, 8))
        wo(hsplit, H, range(8))
        return jnp.concatenate(acc, axis=1), odef

    def mixer_prep(i, k, n):
        r = pl.ds(pl.multiple_of(i * 64 + k * n, n), n)
        if n == 64:
            xr = x_s[pl.ds(2 * i, 2)].astype(f32).reshape(2 * SEG, D)
        else:
            r0 = (k * n) % SEG
            xr = x_s[2 * i + (k * n) // SEG, r0:r0 + n, :].astype(f32)
        x2 = xr + mod_row(2) * aout_s[k * n:(k + 1) * n, :]
        x2_s[r, :] = x2.astype(bf16)
        hb = _ln(x2) * (1.0 + mod_row(4)) + mod_row(3)
        hb_s[r, :] = hb.astype(bf16)
        return _pk(_ln(hb)) if n < 64 else _ln(hb).astype(bf16)

    def mixer_mm(i, lhs):
        t = _gelu(_dot(lhs, _up(wo1_s[H * E // 2:, :])))
        t_s[pl.ds(pl.multiple_of(i * 64 + 8, 8), 64), :] = t

    def mixer_in(i):
        mixer_mm(i, mixer_prep(i, 0, 64))

    def p2_body(i, carry):
        @pl.when(i == 1)
        def _():
            cp_wm1.wait()
            mod_s[:, 2 * D:6 * D] = _dot(sc8, wm_s[...])

        @pl.when(i == 3)
        def _():
            cp_w2.start()
            cp_w3.start()
            cp_w4.start()

        sa_ = 2 * i
        sb_ = 2 * i + 1
        hb_tok = h_rows(sb_)
        ip = jnp.maximum(i - 1, 0)
        if PINS:
            n = 64 // len(PINS)
            pieces = [None] * len(PINS)

            def pin(k):
                v = pieces[k] = mixer_prep(ip, k, n)
                z = v[0:8, 0:E]
                for rr in range(n // 16):
                    for j in range(D // E):
                        if rr or j:
                            z = z | v[8 * rr:8 * rr + 8, j * E:(j + 1) * E]
                return z

            pins = {p: functools.partial(pin, k) for k, p in enumerate(PINS)}
            oa, odef_a = chain_step(sa_, mem_s[...], hn_s[...], None, pins)
            mixer_mm(ip, _up(jnp.concatenate(pieces, axis=0)))
        else:
            oa, odef_a = chain_step(sa_, mem_s[...], hn_s[...], None)
            mixer_in(ip)
        ob, _ = chain_step(sb_, oa[0:M], hb_tok, odef_a)
        mem_s[...] = ob[0:M]
        aout_s[0:TC, :] = oa[M:SEG]
        aout_s[TC:SEG, :] = ob[SEG:SEG + M]
        aout_s[SEG:SEG + TC, :] = ob[M:SEG]
        aout_s[SEG + TC:2 * SEG, :] = ob[SEG + M:SEG + 2 * M]
        hn_s[...] = h_rows(jnp.minimum(sb_ + 1, NSEG - 1))
        return carry

    if "2" in _PHASES:
        lax.fori_loop(0, _N2, _scoped("p2", p2_body), 0)
        mixer_in(NSEG // 2 - 1)
    else:
        cp_w2.start()
        cp_w3.start()
        cp_w4.start()
        cp_wm1.wait()
        cpd = copy(pre_s.at[0], pre_s.at[1], SEM_WM)
        cpd.start()
        cpd.wait()

    cp_w2.wait()
    cp_w3.wait()
    cp_w4.wait()

    def mix(j):
        r0 = pl.multiple_of(j * TB, TB)
        q = D // 4
        parts = []
        for k, sh in enumerate((-1, 1, -2, 2)):
            tt = t_s[pl.ds(r0, TB + 16), k * q:(k + 1) * q]
            parts.append(tt[8 + sh:8 + sh + TB])
        g = jnp.concatenate(parts, axis=1).astype(bf16)
        x1 = hb_s[pl.ds(r0, TB), :].astype(f32) + _dot(g, w2_s[...])
        return x1

    def out_copy(j, slot):
        return copy(o_s.at[slot], out_hbm.at[pl.ds(pl.multiple_of(j * TB, TB), TB)], SEM_OUT + slot)

    if "3" not in _PHASES:
        return

    x1_0 = mix(0)
    y_s[...] = _pk(_ln(x1_0))
    hb_s[0:TB, :] = x1_0.astype(bf16)

    def p3_body(j, carry):
        slot = j % 2

        @pl.when(j >= 2)
        def _():
            out_copy(j - 2, slot).wait()

        r = pl.ds(pl.multiple_of(j * TB, TB), TB)
        for cidx in range(F // FC):
            u = _gelu(_dot(_up(y_s[...]), w3_s[:, cidx * FC:(cidx + 1) * FC]))
            u_s[:, cidx * FC:(cidx + 1) * FC] = _pk(u)
        base = x2_s[r, :].astype(f32) + mod_row(5) * hb_s[r, :].astype(f32)
        jn = jnp.minimum(j + 1, NB - 1)
        x1n = mix(jn)
        h2 = _dot(_up(u_s[...]), w4_s[...])
        o_s[slot] = (base + mod_row(5) * h2).astype(bf16)
        y_s[...] = _pk(_ln(x1n))
        hb_s[pl.ds(pl.multiple_of(jn * TB, TB), TB), :] = x1n.astype(bf16)
        out_copy(j, slot).start()
        return carry

    lax.fori_loop(0, _N3, _scoped("p3", p3_body), 0)
    out_copy(NB - 2, 0).wait()
    out_copy(NB - 1, 1).wait()


@functools.partial(jax.jit, static_argnames=("A_seg_len",))
def pallas_adaLN_cond__memory_aug_recurrent_mem_tr__mixer_s_mlp__prompt_kernel(
    A_x: jax.Array,
    A_mem0: jax.Array,
    A_Wq: jax.Array,
    A_Wk: jax.Array,
    A_Wv: jax.Array,
    A_Wo: jax.Array,
    A_seg_len,
    B_x: jax.Array,
    B_w1: jax.Array,
    B_w2: jax.Array,
    B_w3: jax.Array,
    B_w4: jax.Array,
    c: jax.Array,
    w_mod: jax.Array,
):
    assert A_seg_len == SEG and A_x.shape == (1, S, D) and A_mem0.shape == (1, M, D)
    hbm = pl.BlockSpec(memory_space=pl.ANY)
    scratch = [
        pltpu.VMEM((NSEG, SEG, D), bf16),
        pltpu.VMEM((NSEG, M, D), bf16),
        pltpu.VMEM((NSEG * M // 2, D), u32),
        pltpu.VMEM((D, 4 * D), bf16),
        pltpu.VMEM((2, D, HG, E), bf16),
        pltpu.VMEM((3 * H + HG, D // 2, E), u32),
        pltpu.VMEM(((H * E + D) // 2, D), u32),
        pltpu.VMEM((D, D), bf16),
        pltpu.VMEM((D, F), bf16),
        pltpu.VMEM((F, D), bf16),
        pltpu.VMEM((3 * NP, NSEG, M, E), u32),
        pltpu.VMEM((8, 6 * D), f32),
        pltpu.VMEM((M, D), f32),
        pltpu.VMEM((TC, D), f32),
        pltpu.VMEM((2 * SEG, D), f32),
        pltpu.VMEM((NR, E), f32),
        pltpu.VMEM((S, D), bf16),
        pltpu.VMEM((S, D), bf16),
        pltpu.VMEM((S + 16, D), f32),
        pltpu.VMEM((TB // 2, D), u32),
        pltpu.VMEM((TB // 2, F), u32),
        pltpu.VMEM((2, TB, D), bf16),
        pltpu.VMEM((8, E), u32),
        pltpu.VMEM((2, BGR, D), bf16),
        pltpu.VMEM((1, D), bf16),
        pltpu.VMEM((M, D), bf16),
        pltpu.VMEM((2, 16, D), u32),
        pltpu.SemaphoreType.DMA((17,)),
    ]
    out = pl.pallas_call(
        _kernel,
        out_shape=jax.ShapeDtypeStruct((S, D), bf16),
        in_specs=[hbm] * 12,
        out_specs=hbm,
        scratch_shapes=scratch,
        compiler_params=pltpu.CompilerParams(vmem_limit_bytes=126 * 1024 * 1024),
    )(A_x.reshape(NSEG, SEG, D), A_mem0.reshape(M, D), A_Wq, A_Wk, A_Wv,
      A_Wo.reshape(H * E, D), B_w1, B_w2, B_w3, B_w4, c, w_mod)
    return out.reshape(1, S, D)
```

```python
import functools

import jax
import jax.numpy as jnp
from jax import lax
import jax.experimental.pallas as pl
import jax.experimental.pallas.tpu as pltpu

bf16, f32, u32 = jnp.bfloat16, jnp.float32, jnp.uint32

S, D, H, E, M, SEG, F = 2048, 1024, 32, 128, 8, 32, 3584
NSEG = S // SEG
NP = H // 2
TC = SEG - M
HG = 8
NG = H // HG
TB = 128
NB = S // TB
FC = 512
NC = 3 * NG
WMC = 384
BGR = 512
NR = 2 * (M + SEG)
LAG_S = 1
LAG_O = 3
ORDER = 2
EPS = 1e-5
SCALE = E ** -0.5
_SCOPES = False
_N2 = NSEG // 2
_N3 = NB


def _scoped(name, fn):
    def wrapped(*a):
        if not _SCOPES:
            return fn(*a)
        with jax.named_scope(name):
            return fn(*a)
    return wrapped


def _pk(x):
    return pltpu.bitcast(x.astype(bf16), u32)


def _up(x):
    return pltpu.bitcast(x, bf16)


def _dot(a, b):
    return jnp.dot(a, b, preferred_element_type=f32)


def _ln(x):
    m = jnp.mean(x, axis=-1, keepdims=True)
    xc = x - m
    v = jnp.mean(xc * xc, axis=-1, keepdims=True)
    return xc * lax.rsqrt(v + EPS)


def _gelu(x):
    c = 0.7978845608028654
    return 0.5 * x * (1.0 + jnp.tanh(c * (x + 0.044715 * (x * x * x))))


def _mask_fill():
    shape = (NR, E)
    r = lax.broadcasted_iota(jnp.int32, shape, 0)
    c = lax.broadcasted_iota(jnp.int32, shape, 1)

    def headpos(i):
        head = jnp.where(i < 64, i >> 5, (i - 64) >> 3)
        pos = jnp.where(i < 64, i & 31, 32 + (i & 7))
        return head, pos

    hr, pr = headpos(r)
    hc, pc = headpos(c)
    same = hr == hc
    valid = same & ((pr < M) | (pr >= pc))
    return jnp.where(valid, 0.0, jnp.where(same, -1e9, -jnp.inf)).astype(f32)


def _kernel(x_hbm, mem0_hbm, wq_hbm, wk_hbm, wv_hbm, wo_hbm, w1_hbm, w2_hbm, w3_hbm,
            w4_hbm, c_hbm, wm_hbm,
            out_hbm,
            x_s, xpre_s, hpre_s, wm_s, stg, w_s, wo1_s,
            w2_s, w3_s, w4_s, pre_s, mod_s, mem_s, hn_s, aout_s, fill_s,
            x2_s, hb_s, t_s, y_s, u_s, o_s, zero_s, bg, c_s, mem0_s, wmr, modt_s, sems):
    w_hbm = (wq_hbm, wk_hbm, wv_hbm)

    (SEM_C, SEM_MEM, SEM_XPRE, SEM_X, SEM_W2, SEM_W3, SEM_W4, SEM_STG, SEM_BG, SEM_OUT,
     SEM_WMR, SEM_WM) = (0, 1, 2, 3, 4, 5, 6, 7, 9, 11, 13, 15)

    def copy(src, dst, k):
        return pltpu.make_async_copy(src, dst, sems.at[k])

    def w_copy(t, g, slot):
        return copy(w_hbm[t].at[:, pl.ds(pl.multiple_of(g * HG, HG), HG), :], stg.at[slot],
                    SEM_STG + slot)

    def bg_copy(src, b, slot):
        return copy(src.at[pl.ds(pl.multiple_of(b * BGR, BGR), BGR)], bg.at[slot], SEM_BG + slot)

    def wmr_tile(k):
        return jnp.minimum(k * (WMC // E), (4 * D - WMC) // E)

    def wmr_copy(k, slot):
        c0 = pl.multiple_of(2 * D + wmr_tile(k) * E, E)
        return copy(wm_hbm.at[:, pl.ds(c0, WMC)], wmr.at[slot], SEM_WMR + slot)

    def mod_row(k):
        return mod_s[0:1, k * D:(k + 1) * D]

    def relayout(slot, c, i):
        v = pltpu.bitcast(jnp.swapaxes(stg[slot, pl.ds(i * 16, 16)], 0, 1), u32)
        r = i * 8 if isinstance(i, int) else pl.multiple_of(i * 8, 8)
        w_s[pl.ds(c * HG, HG), pl.ds(r, 8), :] = v
        z = v[0]
        for h in range(1, HG):
            z = z | v[h]
        return z

    def repack(slot, b, i):
        v = pltpu.bitcast(bg[slot, 16 * i:16 * i + 16, :], u32)
        wo1_s[pl.ds(pl.multiple_of(b * (BGR // 2) + 8 * i, 8), 8), :] = v
        z = v[:, 0:E]
        for j in range(1, D // E):
            z = z | v[:, j * E:(j + 1) * E]
        return z

    HD = D // 2
    cp_c = copy(c_hbm, c_s, SEM_C)
    cp_mem = copy(mem0_hbm, mem0_s, SEM_MEM)
    cp_xpre = copy(x_hbm.at[:, TC:SEG, :], xpre_s, SEM_XPRE)
    wm_cols = (0, D, HD, D + HD)
    cp_wm = [copy(wm_hbm.at[:, c0:c0 + HD], wm_s.at[:, c0:c0 + HD], SEM_WM + k)
             for k, c0 in enumerate(wm_cols)]
    w_copy(0, 0, 0).start()
    cp_xpre.start()
    cp_c.start()
    cp_mem.start()
    for cp in cp_wm:
        cp.start()
    w_copy(0, 1, 1).start()

    zero_s[...] = jnp.zeros(zero_s.shape, u32)
    fill_s[...] = _mask_fill()
    aout_s[...] = jnp.zeros(aout_s.shape, f32)
    bg[1] = jnp.zeros(bg.shape[1:], bf16)
    wmr[1] = jnp.zeros(wmr.shape[1:], bf16)

    w_copy(0, 0, 0).wait()

    def rl0_body(i, carry):
        for k in range(4):
            relayout(0, 0, 4 * i + k)
        return carry

    lax.fori_loop(0, D // 64, rl0_body, 0)
    w_copy(0, 2, 0).start()
    bg_copy(wo_hbm, 0, 0).start()
    wmr_copy(0, 0).start()

    cp_xpre.wait()

    def npre_body(i, carry):
        xr = xpre_s[pl.ds(pl.multiple_of(i * 8, 8), 8)].astype(f32).reshape(64, D)
        t_s[pl.ds(pl.multiple_of(i * 64, 64), 64), :] = _ln(xr)
        return carry

    lax.fori_loop(0, NSEG // 8, _scoped("npre", npre_body), 0)

    cp_c.wait()
    cp_mem.wait()
    mem_s[...] = mem0_s[...].astype(f32)
    cf = c_s[...].astype(f32)
    sc = cf * (1.0 / (1.0 + jnp.exp(-cf)))
    sc8 = jnp.broadcast_to(sc, (8, D)).astype(bf16)

    for half in range(2):
        for k in (2 * half, 2 * half + 1):
            c0 = wm_cols[k]
            cp_wm[k].wait()
            mod_s[:, c0:c0 + HD] = _dot(sc8, wm_s[:, c0:c0 + HD])
        cols = slice(half * HD, (half + 1) * HD)
        shift = mod_s[0:1, half * HD:(half + 1) * HD]
        scale1 = 1.0 + mod_s[0:1, D + half * HD:D + (half + 1) * HD]
        hpre_s[:, cols] = _pk(t_s[0:NSEG * M, cols] * scale1 + shift)

    t_s[0:8, :] = jnp.zeros((8, D), f32)
    t_s[S + 8:S + 16, :] = jnp.zeros((8, D), f32)

    def modulate_a(xr):
        return _ln(xr) * (1.0 + mod_row(1)) + mod_row(0)

    MB = 128
    cp_x = copy(x_hbm, x_s, SEM_X)
    cp_w2 = copy(w2_hbm, w2_s, SEM_W2)
    cp_w3 = copy(w3_hbm, w3_s, SEM_W3)
    cp_w4 = copy(w4_hbm, w4_s, SEM_W4)

    def pre_pair(c, pp, side, extra):
        ys = []
        for hh in range(2):
            blocks = []
            for mb in range(NSEG * M // MB):
                h = c * HG + 2 * pp + hh
                halves = []
                for k in range(2):
                    z = side()
                    w = w_s[h, k * 256:(k + 1) * 256, :]
                    if z is not None:
                        w = jnp.concatenate([w[0:8] | (z & zero_s[...]), w[8:]], axis=0)
                    halves.append(w)
                w = jnp.concatenate(halves, axis=0)
                blocks.append(_dot(_up(hpre_s[mb * MB // 2:(mb + 1) * MB // 2, :]), _up(w)))
            ys.append(jnp.concatenate(blocks, axis=0).reshape(NSEG, M, E))
            extra()
        y = jnp.concatenate(ys, axis=1)
        pre_s[c * (HG // 2) + pp] = pltpu.bitcast(y.astype(bf16), u32)

    NWO = H * E // BGR
    NBG = NWO + D // BGR

    def p1_body(c, carry):
        slot = c % 2
        pslot = 1 - slot
        b = jnp.clip(c - 1, 0, NBG - 1)
        bslot = jnp.where(c == 0, 1, b % 2)

        @pl.when(jnp.logical_and(c >= 1, c <= NBG))
        def _():
            bg_copy(wo_hbm, 0, bslot).wait()

        @pl.when(c >= 1)
        def _():
            wmr_copy(0, pslot).wait()

        @pl.when(c + 1 < NC)
        def _():
            w_copy(0, 0, pslot).wait()

        units = iter(range(-1, D // 16))

        def side():
            i = next(units)
            if i < 0:
                return None
            z = relayout(pslot, c + 1, i)
            if i % 2 == 0:
                z = z | repack(bslot, b, i // 2)
            return z

        mt = wmr_tile(jnp.maximum(c - 1, 0))
        halves = iter(range(2 * HG))
        part = [None]

        def extra():
            k = next(halves)
            j, hf = k // 2, k % 2
            if j >= WMC // E:
                return
            y = _dot(sc8[:, hf * HD:(hf + 1) * HD],
                     wmr[pslot, hf * HD:(hf + 1) * HD, j * E:(j + 1) * E])
            if hf == 0:
                part[0] = y
            else:
                modt_s[mt + j] = y + part[0]

        for pp in range(HG // 2):
            pre_pair(c, pp, side, extra)
        side()

        for t in range(3):
            @pl.when((c + 3) // NG == t)
            def _():
                w_copy(t, (c + 3) % NG, pslot).start()

        @pl.when(c + 1 < NWO)
        def _():
            bg_copy(wo_hbm, c + 1, pslot).start()

        @pl.when(jnp.logical_and(c + 1 >= NWO, c + 1 < NBG))
        def _():
            bg_copy(w1_hbm, c + 1 - NWO, pslot).start()

        @pl.when(c + 2 < NC)
        def _():
            wmr_copy(c + 1, pslot).start()

        @pl.when(c == NC - 3)
        def _():
            cp_x.start()

        return carry

    lax.fori_loop(0, NC, _scoped("p1", p1_body), 0)
    mod_s[:, 2 * D:6 * D] = jnp.concatenate([modt_s[j] for j in range(4 * D // E)], axis=1)
    cp_w2.start()
    cp_w3.start()
    cp_w4.start()
    cp_x.wait()

    def h_rows(s):
        return modulate_a(x_s[s, 0:TC, :].astype(f32))

    hn_s[...] = h_rows(0)

    def chain_step(s, mem, htok, odef_prev):
        hs = jnp.concatenate([mem, htok], axis=0).astype(bf16)
        qkv = [[None] * 3 for _ in range(NP)]
        ps = [None] * NP
        os_ = [None] * H
        odef = [None] * H

        def proj(p, ts=(0, 1, 2)):
            for t in ts:
                a = _dot(hs, _up(w_s[t * H + 2 * p]))
                b = _dot(hs, _up(w_s[t * H + 2 * p + 1]))
                pre = pre_s[t * NP + p, s]
                if t == 1:
                    kf = jnp.concatenate([a, b, _up(pre).astype(f32), jnp.zeros((E - NR, E), f32)],
                                         axis=0)
                    qkv[p][t] = kf.T.astype(bf16)
                    continue
                parts = [_pk(a), _pk(b), pre]
                if t == 2:
                    parts.append(jnp.zeros(((E - NR) // 2, E), u32))
                qkv[p][t] = _up(jnp.concatenate(parts, axis=0))

        def scores(p):
            sc_ = _dot(qkv[p][0], qkv[p][1])
            fill = fill_s[...]
            sc_ = jnp.where(fill == 0.0, sc_ * SCALE, fill)
            m = jnp.max(sc_, axis=-1, keepdims=True)
            e = jnp.exp(sc_ - m)
            l = jnp.sum(e, axis=-1, keepdims=True)
            r = pl.reciprocal(l, approx=True)
            r = r * (2.0 - l * r)
            ps[p] = (e * r).astype(bf16)

        def fin(p):
            o = _dot(ps[p], qkv[p][2])
            for hh in range(2):
                h = 2 * p + hh
                rows = o[32 * hh:32 * hh + 32]
                odef[h] = o[64 + 8 * hh:72 + 8 * hh]
                if odef_prev is not None:
                    rows = jnp.concatenate([rows, odef_prev[h], odef[h]], axis=0)
                os_[h] = _pk(rows)

        acc = [None] * 8

        def wo(h0, h1, js):
            lhs = _up(jnp.concatenate(os_[h0:h1], axis=1))
            for j in js:
                part = _dot(lhs, _up(wo1_s[h0 * E // 2:h1 * E // 2, j * E:(j + 1) * E]))
                acc[j] = part if acc[j] is None else part + acc[j]

        for p in range(NP):
            if ORDER == 0:
                proj(p)
                if p >= LAG_S:
                    scores(p - LAG_S)
                if p >= LAG_O:
                    fin(p - LAG_O)
            elif ORDER == 1:
                proj(p, (1, 0))
                if p >= LAG_O:
                    fin(p - LAG_O)
                proj(p, (2,))
                if p >= LAG_S:
                    scores(p - LAG_S)
            elif ORDER == 2:
                proj(p, (1,))
                if p >= LAG_S:
                    scores(p - LAG_S)
                proj(p, (0,))
                if p >= LAG_O:
                    fin(p - LAG_O)
                proj(p, (2,))
            else:
                proj(p, (1, 0, 2))
                if p >= LAG_O:
                    fin(p - LAG_O)
                if p >= LAG_S:
                    scores(p - LAG_S)
        tail = []
        for k in range(LAG_O):
            step = []
            if NP - LAG_S + k < NP:
                step.append(functools.partial(scores, NP - LAG_S + k))
            step.append(functools.partial(fin, NP - LAG_O + k))
            tail.append(step)
        hsplit = min(24, 2 * (NP - LAG_O))
        cuts = {3: (2, 3, 5), 2: (2, 5), 4: (1, 2, 4, 6), 5: (1, 2, 3, 4, 6)}[LAG_O]
        j0 = 0
        for k, step in enumerate(tail):
            wo(0, hsplit, range(j0, cuts[k]))
            j0 = cuts[k]
            for f in step:
                f()
        wo(0, hsplit, range(j0, 8))
        wo(hsplit, H, range(8))
        return jnp.concatenate(acc, axis=1), odef

    def mixer_prep(i):
        r = pl.ds(i * 64 if isinstance(i, int) else pl.multiple_of(i * 64, 64), 64)
        xr = x_s[pl.ds(2 * i, 2)].astype(f32).reshape(2 * SEG, D)
        x2 = xr + mod_row(2) * aout_s[...]
        x2_s[r, :] = x2.astype(bf16)
        hb = _ln(x2) * (1.0 + mod_row(4)) + mod_row(3)
        hb_s[r, :] = hb.astype(bf16)
        return _ln(hb).astype(bf16)

    def mixer_mm(i, lhs):
        t = _gelu(_dot(lhs, _up(wo1_s[H * E // 2:, :])))
        r0 = i * 64 + 8
        t_s[pl.ds(r0 if isinstance(i, int) else pl.multiple_of(r0, 8), 64), :] = t

    def p2_body(i, carry):
        sa_ = 2 * i
        sb_ = 2 * i + 1
        hb_tok = h_rows(sb_)
        oa, odef_a = chain_step(sa_, mem_s[...], hn_s[...], None)
        ip = jnp.maximum(i - 1, 0)
        mixer_mm(ip, mixer_prep(ip))
        ob, _ = chain_step(sb_, oa[0:M], hb_tok, odef_a)
        mem_s[...] = ob[0:M]
        aout_s[0:TC, :] = oa[M:SEG]
        aout_s[TC:SEG, :] = ob[SEG:SEG + M]
        aout_s[SEG:SEG + TC, :] = ob[M:SEG]
        aout_s[SEG + TC:2 * SEG, :] = ob[SEG + M:SEG + 2 * M]
        hn_s[...] = h_rows(jnp.minimum(sb_ + 1, NSEG - 1))
        return carry

    lax.fori_loop(0, _N2, _scoped("p2", p2_body), 0)

    cp_w2.wait()
    cp_w3.wait()
    cp_w4.wait()

    def mix(j):
        r0 = j * TB if isinstance(j, int) else pl.multiple_of(j * TB, TB)
        q = D // 4
        parts = []
        for k, sh in enumerate((-1, 1, -2, 2)):
            tt = t_s[pl.ds(r0, TB + 16), k * q:(k + 1) * q]
            parts.append(tt[8 + sh:8 + sh + TB])
        g = jnp.concatenate(parts, axis=1).astype(bf16)
        x1 = hb_s[pl.ds(r0, TB), :].astype(f32) + _dot(g, w2_s[...])
        return x1

    def out_copy(j, slot):
        return copy(o_s.at[slot], out_hbm.at[pl.ds(pl.multiple_of(j * TB, TB), TB)], SEM_OUT + slot)

    lhs_last = mixer_prep(NSEG // 2 - 1)
    x1_0 = mix(0)
    mixer_mm(NSEG // 2 - 1, lhs_last)
    y_s[...] = _pk(_ln(x1_0))
    hb_s[0:TB, :] = x1_0.astype(bf16)

    def p3_body(j, carry):
        slot = j % 2

        @pl.when(j >= 2)
        def _():
            out_copy(j - 2, slot).wait()

        r = pl.ds(pl.multiple_of(j * TB, TB), TB)
        for cidx in range(F // FC):
            u = _gelu(_dot(_up(y_s[...]), w3_s[:, cidx * FC:(cidx + 1) * FC]))
            u_s[:, cidx * FC:(cidx + 1) * FC] = _pk(u)
        base = x2_s[r, :].astype(f32) + mod_row(5) * hb_s[r, :].astype(f32)
        jn = jnp.minimum(j + 1, NB - 1)
        x1n = mix(jn)
        h2 = _dot(_up(u_s[...]), w4_s[...])
        o_s[slot] = (base + mod_row(5) * h2).astype(bf16)
        y_s[...] = _pk(_ln(x1n))
        hb_s[pl.ds(pl.multiple_of(jn * TB, TB), TB), :] = x1n.astype(bf16)
        out_copy(j, slot).start()
        return carry

    lax.fori_loop(0, _N3, _scoped("p3", p3_body), 0)
    out_copy(NB - 2, 0).wait()
    out_copy(NB - 1, 1).wait()


@functools.partial(jax.jit, static_argnames=("A_seg_len",))
def pallas_adaLN_cond__memory_aug_recurrent_mem_tr__mixer_s_mlp__prompt_kernel(
    A_x: jax.Array,
    A_mem0: jax.Array,
    A_Wq: jax.Array,
    A_Wk: jax.Array,
    A_Wv: jax.Array,
    A_Wo: jax.Array,
    A_seg_len,
    B_x: jax.Array,
    B_w1: jax.Array,
    B_w2: jax.Array,
    B_w3: jax.Array,
    B_w4: jax.Array,
    c: jax.Array,
    w_mod: jax.Array,
):
    assert A_seg_len == SEG and A_x.shape == (1, S, D) and A_mem0.shape == (1, M, D)
    hbm = pl.BlockSpec(memory_space=pl.ANY)
    scratch = [
        pltpu.VMEM((NSEG, SEG, D), bf16),
        pltpu.VMEM((NSEG, M, D), bf16),
        pltpu.VMEM((NSEG * M // 2, D), u32),
        pltpu.VMEM((D, 2 * D), bf16),
        pltpu.VMEM((2, D, HG, E), bf16),
        pltpu.VMEM((3 * H + HG, D // 2, E), u32),
        pltpu.VMEM(((H * E + D) // 2, D), u32),
        pltpu.VMEM((D, D), bf16),
        pltpu.VMEM((D, F), bf16),
        pltpu.VMEM((F, D), bf16),
        pltpu.VMEM((3 * NP, NSEG, M, E), u32),
        pltpu.VMEM((8, 6 * D), f32),
        pltpu.VMEM((M, D), f32),
        pltpu.VMEM((TC, D), f32),
        pltpu.VMEM((2 * SEG, D), f32),
        pltpu.VMEM((NR, E), f32),
        pltpu.VMEM((S, D), bf16),
        pltpu.VMEM((S, D), bf16),
        pltpu.VMEM((S + 16, D), f32),
        pltpu.VMEM((TB // 2, D), u32),
        pltpu.VMEM((TB // 2, F), u32),
        pltpu.VMEM((2, TB, D), bf16),
        pltpu.VMEM((8, E), u32),
        pltpu.VMEM((2, BGR, D), bf16),
        pltpu.VMEM((1, D), bf16),
        pltpu.VMEM((M, D), bf16),
        pltpu.VMEM((2, D, WMC), bf16),
        pltpu.VMEM((4 * D // E, 8, E), f32),
        pltpu.SemaphoreType.DMA((19,)),
    ]
    out = pl.pallas_call(
        _kernel,
        out_shape=jax.ShapeDtypeStruct((S, D), bf16),
        in_specs=[hbm] * 12,
        out_specs=hbm,
        scratch_shapes=scratch,
        compiler_params=pltpu.CompilerParams(vmem_limit_bytes=126 * 1024 * 1024),
    )(A_x.reshape(NSEG, SEG, D), A_mem0.reshape(M, D), A_Wq, A_Wk, A_Wv,
      A_Wo.reshape(H * E, D), B_w1, B_w2, B_w3, B_w4, c, w_mod)
    return out.reshape(1, S, D)
```

```python
import functools

import jax
import jax.numpy as jnp
from jax import lax
import jax.experimental.pallas as pl
import jax.experimental.pallas.tpu as pltpu

bf16, f32, u32 = jnp.bfloat16, jnp.float32, jnp.uint32

S, D, H, E, M, SEG, F = 2048, 1024, 32, 128, 8, 32, 3584
NSEG = S // SEG
NP = H // 2
TC = SEG - M
HG = 8
NG = H // HG
TB = 128
NB = S // TB
FC = 512
NC = 3 * NG
WMC = 384
BGR = 512
NR = 2 * (M + SEG)
LAG_S = 1
LAG_O = 3
ORDER = 2
EPS = 1e-5
SCALE = E ** -0.5
_SCOPES = False
_N2 = NSEG // 2


def _scoped(name, fn):
    def wrapped(*a):
        if not _SCOPES:
            return fn(*a)
        with jax.named_scope(name):
            return fn(*a)
    return wrapped


def _pk(x):
    return pltpu.bitcast(x.astype(bf16), u32)


def _up(x):
    return pltpu.bitcast(x, bf16)


def _dot(a, b):
    return jnp.dot(a, b, preferred_element_type=f32)


def _ln(x):
    m = jnp.mean(x, axis=-1, keepdims=True)
    xc = x - m
    v = jnp.mean(xc * xc, axis=-1, keepdims=True)
    return xc * lax.rsqrt(v + EPS)


def _gelu(x):
    c = 0.7978845608028654
    return 0.5 * x * (1.0 + jnp.tanh(c * (x + 0.044715 * (x * x * x))))


def _mask_fill():
    shape = (NR, E)
    r = lax.broadcasted_iota(jnp.int32, shape, 0)
    c = lax.broadcasted_iota(jnp.int32, shape, 1)

    def headpos(i):
        head = jnp.where(i < 64, i >> 5, (i - 64) >> 3)
        pos = jnp.where(i < 64, i & 31, 32 + (i & 7))
        return head, pos

    hr, pr = headpos(r)
    hc, pc = headpos(c)
    same = hr == hc
    valid = same & ((pr < M) | (pr >= pc))
    return jnp.where(valid, 0.0, jnp.where(same, -1e9, -jnp.inf)).astype(f32)


def _kernel(x_hbm, mem0_hbm, wq_hbm, wk_hbm, wv_hbm, wo_hbm, w1_hbm, w2_hbm, w3_hbm,
            w4_hbm, c_hbm, wm_hbm,
            out_hbm,
            x_s, xpre_s, hpre_s, wm_s, stg, w_s, wo1_s,
            w2_s, w3_s, w4_s, pre_s, mod_s, mem_s, hn_s, aout_s, fill_s,
            x2_s, hb_s, t_s, y_s, u_s, o_s, zero_s, bg, c_s, mem0_s, wmr, modt_s, sems):
    w_hbm = (wq_hbm, wk_hbm, wv_hbm)

    (SEM_C, SEM_MEM, SEM_XPRE, SEM_X, SEM_W2, SEM_W3, SEM_W4, SEM_STG, SEM_BG, SEM_OUT,
     SEM_WMR, SEM_WM) = (0, 1, 2, 3, 4, 5, 6, 7, 9, 11, 13, 15)

    def copy(src, dst, k):
        return pltpu.make_async_copy(src, dst, sems.at[k])

    def w_copy(t, g, slot):
        return copy(w_hbm[t].at[:, pl.ds(pl.multiple_of(g * HG, HG), HG), :], stg.at[slot],
                    SEM_STG + slot)

    def bg_copy(src, b, slot):
        return copy(src.at[pl.ds(pl.multiple_of(b * BGR, BGR), BGR)], bg.at[slot], SEM_BG + slot)

    def wmr_tile(k):
        return jnp.minimum(k * (WMC // E), (4 * D - WMC) // E)

    def wmr_copy(k, slot):
        c0 = pl.multiple_of(2 * D + wmr_tile(k) * E, E)
        return copy(wm_hbm.at[:, pl.ds(c0, WMC)], wmr.at[slot], SEM_WMR + slot)

    def mod_row(k):
        return mod_s[0:1, k * D:(k + 1) * D]

    def relayout(slot, c, i):
        v = pltpu.bitcast(jnp.swapaxes(stg[slot, pl.ds(i * 16, 16)], 0, 1), u32)
        r = i * 8 if isinstance(i, int) else pl.multiple_of(i * 8, 8)
        w_s[pl.ds(c * HG, HG), pl.ds(r, 8), :] = v
        z = v[0]
        for h in range(1, HG):
            z = z | v[h]
        return z

    def repack(slot, b, i):
        v = pltpu.bitcast(bg[slot, 16 * i:16 * i + 16, :], u32)
        wo1_s[pl.ds(pl.multiple_of(b * (BGR // 2) + 8 * i, 8), 8), :] = v
        z = v[:, 0:E]
        for j in range(1, D // E):
            z = z | v[:, j * E:(j + 1) * E]
        return z

    HD = D // 2
    cp_c = copy(c_hbm, c_s, SEM_C)
    cp_mem = copy(mem0_hbm, mem0_s, SEM_MEM)
    cp_xpre = copy(x_hbm.at[:, TC:SEG, :], xpre_s, SEM_XPRE)
    wm_cols = (0, D, HD, D + HD)
    cp_wm = [copy(wm_hbm.at[:, c0:c0 + HD], wm_s.at[:, c0:c0 + HD], SEM_WM + k)
             for k, c0 in enumerate(wm_cols)]
    w_copy(0, 0, 0).start()
    cp_xpre.start()
    cp_c.start()
    cp_mem.start()
    for cp in cp_wm:
        cp.start()
    w_copy(0, 1, 1).start()

    zero_s[...] = jnp.zeros(zero_s.shape, u32)
    fill_s[...] = _mask_fill()
    aout_s[...] = jnp.zeros(aout_s.shape, f32)
    bg[1] = jnp.zeros(bg.shape[1:], bf16)
    wmr[1] = jnp.zeros(wmr.shape[1:], bf16)

    w_copy(0, 0, 0).wait()

    def rl0_body(i, carry):
        for k in range(4):
            relayout(0, 0, 4 * i + k)
        return carry

    lax.fori_loop(0, D // 64, rl0_body, 0)
    w_copy(0, 2, 0).start()
    bg_copy(wo_hbm, 0, 0).start()
    wmr_copy(0, 0).start()

    cp_xpre.wait()

    def npre_body(i, carry):
        xr = xpre_s[pl.ds(pl.multiple_of(i * 8, 8), 8)].astype(f32).reshape(64, D)
        t_s[pl.ds(pl.multiple_of(i * 64, 64), 64), :] = _ln(xr)
        return carry

    lax.fori_loop(0, NSEG // 8, _scoped("npre", npre_body), 0)

    cp_c.wait()
    cp_mem.wait()
    mem_s[...] = mem0_s[...].astype(f32)
    cf = c_s[...].astype(f32)
    sc = cf * (1.0 / (1.0 + jnp.exp(-cf)))
    sc8 = jnp.broadcast_to(sc, (8, D)).astype(bf16)

    for half in range(2):
        for k in (2 * half, 2 * half + 1):
            c0 = wm_cols[k]
            cp_wm[k].wait()
            mod_s[:, c0:c0 + HD] = _dot(sc8, wm_s[:, c0:c0 + HD])
        cols = slice(half * HD, (half + 1) * HD)
        shift = mod_s[0:1, half * HD:(half + 1) * HD]
        scale1 = 1.0 + mod_s[0:1, D + half * HD:D + (half + 1) * HD]
        hpre_s[:, cols] = _pk(t_s[0:NSEG * M, cols] * scale1 + shift)

    t_s[0:8, :] = jnp.zeros((8, D), f32)
    t_s[S + 8:S + 16, :] = jnp.zeros((8, D), f32)

    def modulate_a(xr):
        return _ln(xr) * (1.0 + mod_row(1)) + mod_row(0)

    MB = 128
    cp_x = copy(x_hbm, x_s, SEM_X)
    cp_w2 = copy(w2_hbm, w2_s, SEM_W2)
    cp_w3 = copy(w3_hbm, w3_s, SEM_W3)
    cp_w4 = copy(w4_hbm, w4_s, SEM_W4)

    def pre_pair(c, pp, side, extra):
        ys = []
        for hh in range(2):
            blocks = []
            for mb in range(NSEG * M // MB):
                h = c * HG + 2 * pp + hh
                halves = []
                for k in range(2):
                    z = side()
                    w = w_s[h, k * 256:(k + 1) * 256, :]
                    if z is not None:
                        w = jnp.concatenate([w[0:8] | (z & zero_s[...]), w[8:]], axis=0)
                    halves.append(w)
                w = jnp.concatenate(halves, axis=0)
                blocks.append(_dot(_up(hpre_s[mb * MB // 2:(mb + 1) * MB // 2, :]), _up(w)))
            ys.append(jnp.concatenate(blocks, axis=0).reshape(NSEG, M, E))
            extra()
        y = jnp.concatenate(ys, axis=1)
        pre_s[c * (HG // 2) + pp] = pltpu.bitcast(y.astype(bf16), u32)

    NWO = H * E // BGR
    NBG = NWO + D // BGR

    def p1_body(c, carry):
        slot = c % 2
        pslot = 1 - slot
        b = jnp.clip(c - 1, 0, NBG - 1)
        bslot = jnp.where(c == 0, 1, b % 2)

        @pl.when(jnp.logical_and(c >= 1, c <= NBG))
        def _():
            bg_copy(wo_hbm, 0, bslot).wait()

        @pl.when(c >= 1)
        def _():
            wmr_copy(0, pslot).wait()

        @pl.when(c + 1 < NC)
        def _():
            w_copy(0, 0, pslot).wait()

        units = iter(range(-1, D // 16))

        def side():
            i = next(units)
            if i < 0:
                return None
            z = relayout(pslot, c + 1, i)
            if i % 2 == 0:
                z = z | repack(bslot, b, i // 2)
            return z

        mt = wmr_tile(jnp.maximum(c - 1, 0))
        halves = iter(range(2 * HG))
        part = [None]

        def extra():
            k = next(halves)
            j, hf = k // 2, k % 2
            if j >= WMC // E:
                return
            y = _dot(sc8[:, hf * HD:(hf + 1) * HD],
                     wmr[pslot, hf * HD:(hf + 1) * HD, j * E:(j + 1) * E])
            if hf == 0:
                part[0] = y
            else:
                modt_s[mt + j] = y + part[0]

        for pp in range(HG // 2):
            pre_pair(c, pp, side, extra)
        side()

        for t in range(3):
            @pl.when((c + 3) // NG == t)
            def _():
                w_copy(t, (c + 3) % NG, pslot).start()

        @pl.when(c + 1 < NWO)
        def _():
            bg_copy(wo_hbm, c + 1, pslot).start()

        @pl.when(jnp.logical_and(c + 1 >= NWO, c + 1 < NBG))
        def _():
            bg_copy(w1_hbm, c + 1 - NWO, pslot).start()

        @pl.when(c + 2 < NC)
        def _():
            wmr_copy(c + 1, pslot).start()

        @pl.when(c == NC - 3)
        def _():
            cp_x.start()

        return carry

    lax.fori_loop(0, NC, _scoped("p1", p1_body), 0)
    mod_s[:, 2 * D:6 * D] = jnp.concatenate([modt_s[j] for j in range(4 * D // E)], axis=1)
    cp_w2.start()
    cp_w3.start()
    cp_w4.start()
    cp_x.wait()

    def h_rows(s):
        return modulate_a(x_s[s, 0:TC, :].astype(f32))

    hn_s[...] = h_rows(0)

    def chain_step(s, mem, htok, odef_prev):
        hs = jnp.concatenate([mem, htok], axis=0).astype(bf16)
        qkv = [[None] * 3 for _ in range(NP)]
        ps = [None] * NP
        os_ = [None] * H
        odef = [None] * H

        def proj(p, ts=(0, 1, 2)):
            for t in ts:
                a = _dot(hs, _up(w_s[t * H + 2 * p]))
                b = _dot(hs, _up(w_s[t * H + 2 * p + 1]))
                pre = pre_s[t * NP + p, s]
                if t == 1:
                    kf = jnp.concatenate([a, b, _up(pre).astype(f32), jnp.zeros((E - NR, E), f32)],
                                         axis=0)
                    qkv[p][t] = kf.T.astype(bf16)
                    continue
                parts = [_pk(a), _pk(b), pre]
                if t == 2:
                    parts.append(jnp.zeros(((E - NR) // 2, E), u32))
                qkv[p][t] = _up(jnp.concatenate(parts, axis=0))

        def scores(p):
            sc_ = _dot(qkv[p][0], qkv[p][1])
            fill = fill_s[...]
            sc_ = jnp.where(fill == 0.0, sc_ * SCALE, fill)
            m = jnp.max(sc_, axis=-1, keepdims=True)
            e = jnp.exp(sc_ - m)
            l = jnp.sum(e, axis=-1, keepdims=True)
            r = pl.reciprocal(l, approx=True)
            r = r * (2.0 - l * r)
            ps[p] = (e * r).astype(bf16)

        def fin(p):
            o = _dot(ps[p], qkv[p][2])
            for hh in range(2):
                h = 2 * p + hh
                rows = o[32 * hh:32 * hh + 32]
                odef[h] = o[64 + 8 * hh:72 + 8 * hh]
                if odef_prev is not None:
                    rows = jnp.concatenate([rows, odef_prev[h], odef[h]], axis=0)
                os_[h] = _pk(rows)

        acc = [None] * 8

        def wo(h0, h1, js):
            lhs = _up(jnp.concatenate(os_[h0:h1], axis=1))
            for j in js:
                part = _dot(lhs, _up(wo1_s[h0 * E // 2:h1 * E // 2, j * E:(j + 1) * E]))
                acc[j] = part if acc[j] is None else part + acc[j]

        for p in range(NP):
            if ORDER == 0:
                proj(p)
                if p >= LAG_S:
                    scores(p - LAG_S)
                if p >= LAG_O:
                    fin(p - LAG_O)
            elif ORDER == 1:
                proj(p, (1, 0))
                if p >= LAG_O:
                    fin(p - LAG_O)
                proj(p, (2,))
                if p >= LAG_S:
                    scores(p - LAG_S)
            elif ORDER == 2:
                proj(p, (1,))
                if p >= LAG_S:
                    scores(p - LAG_S)
                proj(p, (0,))
                if p >= LAG_O:
                    fin(p - LAG_O)
                proj(p, (2,))
            else:
                proj(p, (1, 0, 2))
                if p >= LAG_O:
                    fin(p - LAG_O)
                if p >= LAG_S:
                    scores(p - LAG_S)
        tail = []
        for k in range(LAG_O):
            step = []
            if NP - LAG_S + k < NP:
                step.append(functools.partial(scores, NP - LAG_S + k))
            step.append(functools.partial(fin, NP - LAG_O + k))
            tail.append(step)
        hsplit = min(24, 2 * (NP - LAG_O))
        cuts = {3: (2, 3, 5), 2: (2, 5), 4: (1, 2, 4, 6), 5: (1, 2, 3, 4, 6)}[LAG_O]
        j0 = 0
        for k, step in enumerate(tail):
            wo(0, hsplit, range(j0, cuts[k]))
            j0 = cuts[k]
            for f in step:
                f()
        wo(0, hsplit, range(j0, 8))
        wo(hsplit, H, range(8))
        return jnp.concatenate(acc, axis=1), odef

    def mixer_prep(i):
        r = pl.ds(i * 64 if isinstance(i, int) else pl.multiple_of(i * 64, 64), 64)
        xr = x_s[pl.ds(2 * i, 2)].astype(f32).reshape(2 * SEG, D)
        x2 = xr + mod_row(2) * aout_s[...]
        x2_s[r, :] = x2.astype(bf16)
        hb = _ln(x2) * (1.0 + mod_row(4)) + mod_row(3)
        hb_s[r, :] = hb.astype(bf16)
        return _ln(hb).astype(bf16)

    def mixer_mm(i, lhs):
        t = _gelu(_dot(lhs, _up(wo1_s[H * E // 2:, :])))
        r0 = i * 64 + 8
        t_s[pl.ds(r0 if isinstance(i, int) else pl.multiple_of(r0, 8), 64), :] = t

    def p2_body(i, carry):
        sa_ = 2 * i
        sb_ = 2 * i + 1
        hb_tok = h_rows(sb_)
        oa, odef_a = chain_step(sa_, mem_s[...], hn_s[...], None)
        ip = jnp.maximum(i - 1, 0)
        mixer_mm(ip, mixer_prep(ip))
        ob, _ = chain_step(sb_, oa[0:M], hb_tok, odef_a)
        mem_s[...] = ob[0:M]
        aout_s[0:TC, :] = oa[M:SEG]
        aout_s[TC:SEG, :] = ob[SEG:SEG + M]
        aout_s[SEG:SEG + TC, :] = ob[M:SEG]
        aout_s[SEG + TC:2 * SEG, :] = ob[SEG + M:SEG + 2 * M]
        hn_s[...] = h_rows(jnp.minimum(sb_ + 1, NSEG - 1))
        return carry

    lax.fori_loop(0, _N2, _scoped("p2", p2_body), 0)

    cp_w2.wait()
    cp_w3.wait()
    cp_w4.wait()

    def mix(j):
        r0 = j * TB if isinstance(j, int) else pl.multiple_of(j * TB, TB)
        q = D // 4
        parts = []
        for k, sh in enumerate((-1, 1, -2, 2)):
            tt = t_s[pl.ds(r0, TB + 16), k * q:(k + 1) * q]
            parts.append(tt[8 + sh:8 + sh + TB])
        g = jnp.concatenate(parts, axis=1).astype(bf16)
        x1 = hb_s[pl.ds(r0, TB), :].astype(f32) + _dot(g, w2_s[...])
        return x1

    def out_copy(j, slot):
        r0 = j * TB if isinstance(j, int) else pl.multiple_of(j * TB, TB)
        return copy(o_s.at[slot], out_hbm.at[pl.ds(r0, TB)], SEM_OUT + slot)

    lhs_last = mixer_prep(NSEG // 2 - 1)
    x1_0 = mix(0)
    mixer_mm(NSEG // 2 - 1, lhs_last)
    y_s[...] = _pk(_ln(x1_0))
    hb_s[0:TB, :] = x1_0.astype(bf16)

    def mlp_block(j, last):
        slot = j % 2
        r = pl.ds(j * TB if last else pl.multiple_of(j * TB, TB), TB)
        for cidx in range(F // FC):
            u = _gelu(_dot(_up(y_s[...]), w3_s[:, cidx * FC:(cidx + 1) * FC]))
            u_s[:, cidx * FC:(cidx + 1) * FC] = _pk(u)
        base = x2_s[r, :].astype(f32) + mod_row(5) * hb_s[r, :].astype(f32)
        if last:
            ks = F - FC
            h2 = _dot(_up(u_s[:, 0:ks]), w4_s[0:ks, :])
            h2 = _dot(_up(u_s[:, ks:F]), w4_s[ks:F, :]) + h2
        else:
            x1n = mix(j + 1)
            h2 = _dot(_up(u_s[...]), w4_s[...])
        o_s[slot] = (base + mod_row(5) * h2).astype(bf16)
        if not last:
            y_s[...] = _pk(_ln(x1n))
            hb_s[pl.ds(pl.multiple_of((j + 1) * TB, TB), TB), :] = x1n.astype(bf16)
        out_copy(j, slot).start()

    def p3_body(j, carry):
        @pl.when(j >= 2)
        def _():
            out_copy(j - 2, j % 2).wait()

        mlp_block(j, False)
        return carry

    lax.fori_loop(0, NB - 1, _scoped("p3", p3_body), 0)
    out_copy(NB - 3, (NB - 3) % 2).wait()
    mlp_block(NB - 1, True)
    out_copy(NB - 2, (NB - 2) % 2).wait()
    out_copy(NB - 1, (NB - 1) % 2).wait()


@functools.partial(jax.jit, static_argnames=("A_seg_len",))
def pallas_adaLN_cond__memory_aug_recurrent_mem_tr__mixer_s_mlp__prompt_kernel(
    A_x: jax.Array,
    A_mem0: jax.Array,
    A_Wq: jax.Array,
    A_Wk: jax.Array,
    A_Wv: jax.Array,
    A_Wo: jax.Array,
    A_seg_len,
    B_x: jax.Array,
    B_w1: jax.Array,
    B_w2: jax.Array,
    B_w3: jax.Array,
    B_w4: jax.Array,
    c: jax.Array,
    w_mod: jax.Array,
):
    assert A_seg_len == SEG and A_x.shape == (1, S, D) and A_mem0.shape == (1, M, D)
    hbm = pl.BlockSpec(memory_space=pl.ANY)
    scratch = [
        pltpu.VMEM((NSEG, SEG, D), bf16),
        pltpu.VMEM((NSEG, M, D), bf16),
        pltpu.VMEM((NSEG * M // 2, D), u32),
        pltpu.VMEM((D, 2 * D), bf16),
        pltpu.VMEM((2, D, HG, E), bf16),
        pltpu.VMEM((3 * H + HG, D // 2, E), u32),
        pltpu.VMEM(((H * E + D) // 2, D), u32),
        pltpu.VMEM((D, D), bf16),
        pltpu.VMEM((D, F), bf16),
        pltpu.VMEM((F, D), bf16),
        pltpu.VMEM((3 * NP, NSEG, M, E), u32),
        pltpu.VMEM((8, 6 * D), f32),
        pltpu.VMEM((M, D), f32),
        pltpu.VMEM((TC, D), f32),
        pltpu.VMEM((2 * SEG, D), f32),
        pltpu.VMEM((NR, E), f32),
        pltpu.VMEM((S, D), bf16),
        pltpu.VMEM((S, D), bf16),
        pltpu.VMEM((S + 16, D), f32),
        pltpu.VMEM((TB // 2, D), u32),
        pltpu.VMEM((TB // 2, F), u32),
        pltpu.VMEM((2, TB, D), bf16),
        pltpu.VMEM((8, E), u32),
        pltpu.VMEM((2, BGR, D), bf16),
        pltpu.VMEM((1, D), bf16),
        pltpu.VMEM((M, D), bf16),
        pltpu.VMEM((2, D, WMC), bf16),
        pltpu.VMEM((4 * D // E, 8, E), f32),
        pltpu.SemaphoreType.DMA((19,)),
    ]
    out = pl.pallas_call(
        _kernel,
        out_shape=jax.ShapeDtypeStruct((S, D), bf16),
        in_specs=[hbm] * 12,
        out_specs=hbm,
        scratch_shapes=scratch,
        compiler_params=pltpu.CompilerParams(vmem_limit_bytes=126 * 1024 * 1024),
    )(A_x.reshape(NSEG, SEG, D), A_mem0.reshape(M, D), A_Wq, A_Wk, A_Wv,
      A_Wo.reshape(H * E, D), B_w1, B_w2, B_w3, B_w4, c, w_mod)
    return out.reshape(1, S, D)
```

```python
import functools

import jax
import jax.numpy as jnp
from jax import lax
import jax.experimental.pallas as pl
import jax.experimental.pallas.tpu as pltpu

bf16, f32, u32 = jnp.bfloat16, jnp.float32, jnp.uint32

S, D, H, E, M, SEG, F = 2048, 1024, 32, 128, 8, 32, 3584
NSEG = S // SEG
NP = H // 2
TC = SEG - M
HG = 8
NG = H // HG
TB = 128
NB = S // TB
FH = F // 2
NF = FH // E
G4R = FH // 16
NC = 3 * NG
WMC = 384
BGR = 512
NR = 2 * (M + SEG)
NO_BOUNDS = True
PIN_ROWS = 512
LAG_S = 1
LAG_O = 3
ORDER = 2
EPS = 1e-5
SCALE = E ** -0.5
_SCOPES = False
_N2 = NSEG // 2


def _scoped(name, fn):
    def wrapped(*a):
        if not _SCOPES:
            return fn(*a)
        with jax.named_scope(name):
            return fn(*a)
    return wrapped


def _pk(x):
    return pltpu.bitcast(x.astype(bf16), u32)


def _up(x):
    return pltpu.bitcast(x, bf16)


def _dot(a, b):
    return jnp.dot(a, b, preferred_element_type=f32)


def _ln(x):
    m = jnp.mean(x, axis=-1, keepdims=True)
    xc = x - m
    v = jnp.mean(xc * xc, axis=-1, keepdims=True)
    return xc * lax.rsqrt(v + EPS)


def _gelu(x):
    c = 0.7978845608028654
    return 0.5 * x * (1.0 + jnp.tanh(c * (x + 0.044715 * (x * x * x))))


def _lhs_set(a11, a12, a21, a22):
    return (a11 + a22, a21 + a22, a11, a22, a11 + a12, a21 - a11, a12 - a22)


def _rhs_set(b11, b12, b21, b22):
    return (b11 + b22, b11, b12 - b22, b21 - b11, b22, b11 + b12, b21 + b22)


def _strassen(m):
    m1 = m(0)
    m2 = m(1)
    c22 = m1 - m2
    m3 = m(2)
    c22 = c22 + m3
    c22 = m(5) + c22
    m4 = m(3)
    c21 = m2 + m4
    c11 = m1 + m4
    m5 = m(4)
    c12 = m3 + m5
    c11 = c11 - m5
    c11 = m(6) + c11
    return c11, c12, c21, c22


def _mask_fill():
    shape = (NR, E)
    r = lax.broadcasted_iota(jnp.int32, shape, 0)
    c = lax.broadcasted_iota(jnp.int32, shape, 1)

    def headpos(i):
        head = jnp.where(i < 64, i >> 5, (i - 64) >> 3)
        pos = jnp.where(i < 64, i & 31, 32 + (i & 7))
        return head, pos

    hr, pr = headpos(r)
    hc, pc = headpos(c)
    same = hr == hc
    valid = same & ((pr < M) | (pr >= pc))
    return jnp.where(valid, 0.0, jnp.where(same, -1e9, -jnp.inf)).astype(f32)


def _kernel(x_hbm, mem0_hbm, wq_hbm, wk_hbm, wv_hbm, wo_hbm, w1_hbm, w2_hbm, w3_hbm,
            w4_hbm, c_hbm, wm_hbm,
            out_hbm,
            x_s, xpre_s, hpre_s, wm_s, stg, w_s, wo1_s,
            w2_s, t3_s, t4_s, g3, g4, pre_s, mod_s, mem_s, hn_s, aout_s, fill_s,
            x2_s, hb_s, t_s, y_s, u_s, o_s, zero_s, bg, c_s, mem0_s, wmr, modt_s, sems):
    w_hbm = (wq_hbm, wk_hbm, wv_hbm)

    (SEM_C, SEM_MEM, SEM_XPRE, SEM_X, SEM_W2, SEM_STG, SEM_BG, SEM_OUT,
     SEM_WMR, SEM_G3, SEM_G4, SEM_WM) = (0, 1, 2, 3, 4, 5, 7, 9, 11, 13, 15, 17)

    def copy(src, dst, k):
        return pltpu.make_async_copy(src, dst, sems.at[k])

    def w_copy(t, g, slot):
        return copy(w_hbm[t].at[:, pl.ds(pl.multiple_of(g * HG, HG), HG), :], stg.at[slot],
                    SEM_STG + slot)

    def bg_copy(src, b, slot):
        return copy(src.at[pl.ds(pl.multiple_of(b * BGR, BGR), BGR)], bg.at[slot], SEM_BG + slot)

    def wmr_tile(k):
        return jnp.minimum(k * (WMC // E), (4 * D - WMC) // E)

    def wmr_copy(k, slot):
        c0 = pl.multiple_of(2 * D + wmr_tile(k) * E, E)
        return copy(wm_hbm.at[:, pl.ds(c0, WMC)], wmr.at[slot], SEM_WMR + slot)

    def aligned(x, n):
        return x if isinstance(x, int) else pl.multiple_of(x, n)

    def g3_copy(k, slot):
        return copy(w3_hbm.at[:, pl.ds(aligned(k * 16, 16), 16), :], g3.at[slot], SEM_G3 + slot)

    def g4_copy(k, slot):
        return copy(w4_hbm.at[:, pl.ds(aligned((k // 2) * G4R, 16), G4R),
                              pl.ds(aligned((k % 2) * (D // 2), E), D // 2)],
                    g4.at[slot], SEM_G4 + slot)

    def rhs_job(src, slot, r0, c1, c2, dst, q, row):
        blk = [src[slot, kh, r0:r0 + 16, cc * E:(cc + 1) * E].astype(f32)
               for kh in range(2) for cc in (c1, c2)]
        z = None
        for n, v in enumerate(_rhs_set(*blk)):
            v = _pk(v)
            dst[n, q, pl.ds(pl.multiple_of(row, 8), 8), :] = v
            z = v if z is None else z | v
        return z

    def mod_row(k):
        return mod_s[0:1, k * D:(k + 1) * D]

    def relayout(slot, c, i):
        v = pltpu.bitcast(jnp.swapaxes(stg[slot, pl.ds(i * 16, 16)], 0, 1), u32)
        r = i * 8 if isinstance(i, int) else pl.multiple_of(i * 8, 8)
        w_s[pl.ds(c * HG, HG), pl.ds(r, 8), :] = v
        z = v[0]
        for h in range(1, HG):
            z = z | v[h]
        return z

    def repack(slot, b, i):
        v = pltpu.bitcast(bg[slot, 16 * i:16 * i + 16, :], u32)
        wo1_s[pl.ds(pl.multiple_of(b * (BGR // 2) + 8 * i, 8), 8), :] = v
        z = v[:, 0:E]
        for j in range(1, D // E):
            z = z | v[:, j * E:(j + 1) * E]
        return z

    HD = D // 2
    cp_c = copy(c_hbm, c_s, SEM_C)
    cp_mem = copy(mem0_hbm, mem0_s, SEM_MEM)
    cp_xpre = copy(x_hbm.at[:, TC:SEG, :], xpre_s, SEM_XPRE)
    wm_cols = (0, D, HD, D + HD)
    cp_wm = [copy(wm_hbm.at[:, c0:c0 + HD], wm_s.at[:, c0:c0 + HD], SEM_WM + k)
             for k, c0 in enumerate(wm_cols)]
    w_copy(0, 0, 0).start()
    cp_xpre.start()
    cp_c.start()
    cp_mem.start()
    for cp in cp_wm:
        cp.start()
    w_copy(0, 1, 1).start()

    zero_s[...] = jnp.zeros(zero_s.shape, u32)
    fill_s[...] = _mask_fill()
    aout_s[...] = jnp.zeros(aout_s.shape, f32)
    bg[1] = jnp.zeros(bg.shape[1:], bf16)
    wmr[1] = jnp.zeros(wmr.shape[1:], bf16)

    w_copy(0, 0, 0).wait()

    def rl0_body(i, carry):
        for k in range(4):
            relayout(0, 0, 4 * i + k)
        return carry

    lax.fori_loop(0, D // 64, rl0_body, 0)
    w_copy(0, 2, 0).start()
    bg_copy(wo_hbm, 0, 0).start()
    wmr_copy(0, 0).start()

    cp_xpre.wait()

    def npre_body(i, carry):
        xr = xpre_s[pl.ds(pl.multiple_of(i * 8, 8), 8)].astype(f32).reshape(64, D)
        t_s[pl.ds(pl.multiple_of(i * 64, 64), 64), :] = _ln(xr)
        return carry

    lax.fori_loop(0, NSEG // 8, _scoped("npre", npre_body), 0)

    cp_c.wait()
    cp_mem.wait()
    mem_s[...] = mem0_s[...].astype(f32)
    cf = c_s[...].astype(f32)
    sc = cf * (1.0 / (1.0 + jnp.exp(-cf)))
    sc8 = jnp.broadcast_to(sc, (8, D)).astype(bf16)

    for half in range(2):
        for k in (2 * half, 2 * half + 1):
            c0 = wm_cols[k]
            cp_wm[k].wait()
            mod_s[:, c0:c0 + HD] = _dot(sc8, wm_s[:, c0:c0 + HD])
        cols = slice(half * HD, (half + 1) * HD)
        shift = mod_s[0:1, half * HD:(half + 1) * HD]
        scale1 = 1.0 + mod_s[0:1, D + half * HD:D + (half + 1) * HD]
        hpre_s[:, cols] = _pk(t_s[0:NSEG * M, cols] * scale1 + shift)

    t_s[0:8, :] = jnp.zeros((8, D), f32)
    t_s[S + 8:S + 16, :] = jnp.zeros((8, D), f32)

    def modulate_a(xr):
        return _ln(xr) * (1.0 + mod_row(1)) + mod_row(0)

    MB = 128
    cp_x = copy(x_hbm, x_s, SEM_X)
    cp_w2 = copy(w2_hbm, w2_s, SEM_W2)

    def pre_pair(c, pp, side, extra):
        ys = []
        for hh in range(2):
            blocks = []
            for mb in range(NSEG * M // MB):
                h = c * HG + 2 * pp + hh
                halves = []
                for k in range(2):
                    z = side()
                    w = w_s[h, k * 256:(k + 1) * 256, :]
                    if z is not None:
                        w = jnp.concatenate([w[0:8] | (z & zero_s[...]), w[8:]], axis=0)
                    halves.append(w)
                w = jnp.concatenate(halves, axis=0)
                blocks.append(_dot(_up(hpre_s[mb * MB // 2:(mb + 1) * MB // 2, :]), _up(w)))
            ys.append(jnp.concatenate(blocks, axis=0).reshape(NSEG, M, E))
            extra()
        y = jnp.concatenate(ys, axis=1)
        pre_s[c * (HG // 2) + pp] = pltpu.bitcast(y.astype(bf16), u32)

    NWO = H * E // BGR
    NBG = NWO + D // BGR

    def p1_body(c, carry):
        slot = c % 2
        pslot = 1 - slot
        b = jnp.clip(c - 1, 0, NBG - 1)
        bslot = jnp.where(c == 0, 1, b % 2)

        @pl.when(jnp.logical_and(c >= 1, c <= NBG))
        def _():
            bg_copy(wo_hbm, 0, bslot).wait()

        @pl.when(c >= 1)
        def _():
            wmr_copy(0, pslot).wait()

        @pl.when(c + 1 < NC)
        def _():
            w_copy(0, 0, pslot).wait()

        units = iter(range(-1, D // 16))

        def side():
            i = next(units)
            if i < 0:
                return None
            z = relayout(pslot, c + 1, i)
            if i % 2 == 0:
                z = z | repack(bslot, b, i // 2)
            return z

        mt = wmr_tile(jnp.maximum(c - 1, 0))
        halves = iter(range(2 * HG))
        part = [None]

        def extra():
            k = next(halves)
            j, hf = k // 2, k % 2
            if j >= WMC // E:
                return
            y = _dot(sc8[:, hf * HD:(hf + 1) * HD],
                     wmr[pslot, hf * HD:(hf + 1) * HD, j * E:(j + 1) * E])
            if hf == 0:
                part[0] = y
            else:
                modt_s[mt + j] = y + part[0]

        for pp in range(HG // 2):
            pre_pair(c, pp, side, extra)
        side()

        for t in range(3):
            @pl.when((c + 3) // NG == t)
            def _():
                w_copy(t, (c + 3) % NG, pslot).start()

        @pl.when(c + 1 < NWO)
        def _():
            bg_copy(wo_hbm, c + 1, pslot).start()

        @pl.when(jnp.logical_and(c + 1 >= NWO, c + 1 < NBG))
        def _():
            bg_copy(w1_hbm, c + 1 - NWO, pslot).start()

        @pl.when(c + 2 < NC)
        def _():
            wmr_copy(c + 1, pslot).start()

        @pl.when(c == NC - 3)
        def _():
            cp_x.start()

        return carry

    lax.fori_loop(0, NC, _scoped("p1", p1_body), 0)
    mod_s[:, 2 * D:6 * D] = jnp.concatenate([modt_s[j] for j in range(4 * D // E)], axis=1)
    for k in range(2):
        g3_copy(k, k).start()
        g4_copy(k, k).start()
    cp_w2.start()
    cp_x.wait()

    def h_rows(s):
        return modulate_a(x_s[s, 0:TC, :].astype(f32))

    hn_s[...] = h_rows(0)

    def chain_step(s, mem, htok, odef_prev, jobs=()):
        hs = jnp.concatenate([mem, htok], axis=0).astype(bf16)
        qkv = [[None] * 3 for _ in range(NP)]
        ps = [None] * NP
        os_ = [None] * H
        odef = [None] * H

        def proj(p, ts=(0, 1, 2)):
            for t in ts:
                a = _dot(hs, _up(w_s[t * H + 2 * p]))
                b = _dot(hs, _up(w_s[t * H + 2 * p + 1]))
                pre = pre_s[t * NP + p, s]
                if t == 1:
                    kf = jnp.concatenate([a, b, _up(pre).astype(f32), jnp.zeros((E - NR, E), f32)],
                                         axis=0)
                    qkv[p][t] = kf.T.astype(bf16)
                    continue
                parts = [_pk(a), _pk(b), pre]
                if t == 2:
                    parts.append(jnp.zeros(((E - NR) // 2, E), u32))
                qkv[p][t] = _up(jnp.concatenate(parts, axis=0))

        def scores(p):
            sc_ = _dot(qkv[p][0], qkv[p][1])
            fill = fill_s[...]
            sc_ = jnp.where(fill == 0.0, sc_ * SCALE, fill)
            m = jnp.max(sc_, axis=-1, keepdims=True)
            e = jnp.exp(sc_ - m)
            l = jnp.sum(e, axis=-1, keepdims=True)
            r = pl.reciprocal(l, approx=True)
            r = r * (2.0 - l * r)
            ps[p] = (e * r).astype(bf16)

        def fin(p):
            o = _dot(ps[p], qkv[p][2])
            for hh in range(2):
                h = 2 * p + hh
                rows = o[32 * hh:32 * hh + 32]
                odef[h] = o[64 + 8 * hh:72 + 8 * hh]
                if odef_prev is not None:
                    rows = jnp.concatenate([rows, odef_prev[h], odef[h]], axis=0)
                os_[h] = _pk(rows)

        acc = [None] * 8
        jobs = iter(jobs)

        def wo(h0, h1, js):
            lhs = _up(jnp.concatenate(os_[h0:h1], axis=1))
            for j in js:
                ws = []
                for r0 in range(h0 * E // 2, h1 * E // 2, PIN_ROWS):
                    job = next(jobs, None)
                    z = None if job is None else job()
                    w = wo1_s[r0:r0 + PIN_ROWS, j * E:(j + 1) * E]
                    if z is not None:
                        w = jnp.concatenate([w[0:8] | (z & zero_s[...]), w[8:]], axis=0)
                    ws.append(w)
                part = _dot(lhs, _up(jnp.concatenate(ws, axis=0)))
                acc[j] = part if acc[j] is None else part + acc[j]

        for p in range(NP):
            if ORDER == 0:
                proj(p)
                if p >= LAG_S:
                    scores(p - LAG_S)
                if p >= LAG_O:
                    fin(p - LAG_O)
            elif ORDER == 1:
                proj(p, (1, 0))
                if p >= LAG_O:
                    fin(p - LAG_O)
                proj(p, (2,))
                if p >= LAG_S:
                    scores(p - LAG_S)
            elif ORDER == 2:
                proj(p, (1,))
                if p >= LAG_S:
                    scores(p - LAG_S)
                proj(p, (0,))
                if p >= LAG_O:
                    fin(p - LAG_O)
                proj(p, (2,))
            else:
                proj(p, (1, 0, 2))
                if p >= LAG_O:
                    fin(p - LAG_O)
                if p >= LAG_S:
                    scores(p - LAG_S)
        tail = []
        for k in range(LAG_O):
            step = []
            if NP - LAG_S + k < NP:
                step.append(functools.partial(scores, NP - LAG_S + k))
            step.append(functools.partial(fin, NP - LAG_O + k))
            tail.append(step)
        hsplit = min(24, 2 * (NP - LAG_O))
        cuts = {3: (2, 3, 5), 2: (2, 5), 4: (1, 2, 4, 6), 5: (1, 2, 3, 4, 6)}[LAG_O]
        j0 = 0
        for k, step in enumerate(tail):
            wo(0, hsplit, range(j0, cuts[k]))
            j0 = cuts[k]
            for f in step:
                f()
        wo(0, hsplit, range(j0, 8))
        wo(hsplit, H, range(8))
        return jnp.concatenate(acc, axis=1), odef

    def mixer_prep(i):
        r = pl.ds(i * 64 if isinstance(i, int) else pl.multiple_of(i * 64, 64), 64)
        xr = x_s[pl.ds(2 * i, 2)].astype(f32).reshape(2 * SEG, D)
        x2 = xr + mod_row(2) * aout_s[...]
        x2_s[r, :] = x2.astype(bf16)
        hb = _ln(x2) * (1.0 + mod_row(4)) + mod_row(3)
        hb_s[r, :] = hb.astype(bf16)
        return _ln(hb).astype(bf16)

    def mixer_mm(i, lhs):
        t = _gelu(_dot(lhs, _up(wo1_s[H * E // 2:, :])))
        r0 = i * 64 + 8
        t_s[pl.ds(r0 if isinstance(i, int) else pl.multiple_of(r0, 8), 64), :] = t

    def p2_body(i, carry):
        slot = i % 2
        g3_copy(0, slot).wait()
        g4_copy(0, slot).wait()
        jobs = []
        for q in range(NF):
            jobs.append(functools.partial(rhs_job, g3, slot, 0, q, NF + q, t3_s, q, i * 8))
            rt, e = q // 2, q % 2
            jobs.append(functools.partial(rhs_job, g4, slot, 16 * rt, e, 2 + e, t4_s, 2 * slot + e,
                                          (i // 2) * (G4R // 2) + 8 * rt))

        sa_ = 2 * i
        sb_ = 2 * i + 1
        hb_tok = h_rows(sb_)
        oa, odef_a = chain_step(sa_, mem_s[...], hn_s[...], None)
        ip = jnp.maximum(i - 1, 0)
        mixer_mm(ip, mixer_prep(ip))
        ob, _ = chain_step(sb_, oa[0:M], hb_tok, odef_a, jobs)
        mem_s[...] = ob[0:M]
        aout_s[0:TC, :] = oa[M:SEG]
        aout_s[TC:SEG, :] = ob[SEG:SEG + M]
        aout_s[SEG:SEG + TC, :] = ob[M:SEG]
        aout_s[SEG + TC:2 * SEG, :] = ob[SEG + M:SEG + 2 * M]
        hn_s[...] = h_rows(jnp.minimum(sb_ + 1, NSEG - 1))

        @pl.when(i + 2 < NSEG // 2)
        def _():
            g3_copy(i + 2, slot).start()
            g4_copy(i + 2, slot).start()

        return carry

    lax.fori_loop(0, _N2, _scoped("p2", p2_body), 0)

    cp_w2.wait()

    def mix(j):
        r0 = j * TB if isinstance(j, int) else pl.multiple_of(j * TB, TB)
        q = D // 4
        parts = []
        for k, sh in enumerate((-1, 1, -2, 2)):
            tt = t_s[pl.ds(r0, TB + 16), k * q:(k + 1) * q]
            parts.append(tt[8 + sh:8 + sh + TB])
        g = jnp.concatenate(parts, axis=1).astype(bf16)
        x1 = hb_s[pl.ds(r0, TB), :].astype(f32) + _dot(g, w2_s[...])
        return x1

    def out_copy(j, slot):
        r0 = j * TB if isinstance(j, int) else pl.multiple_of(j * TB, TB)
        return copy(o_s.at[slot], out_hbm.at[pl.ds(r0, TB)], SEM_OUT + slot)

    TH = TB // 2

    def put_y(x1):
        y = _ln(x1)
        for n, v in enumerate(_lhs_set(y[:TH, :HD], y[:TH, HD:], y[TH:, :HD], y[TH:, HD:])):
            y_s[n] = _pk(v)

    lhs_last = mixer_prep(NSEG // 2 - 1)
    x1_0 = mix(0)
    mixer_mm(NSEG // 2 - 1, lhs_last)
    put_y(x1_0)
    hb_s[0:TB, :] = x1_0.astype(bf16)

    def mlp_block(j, last):
        slot = j % 2
        r0 = aligned(j * TB, TB)
        for q in range(NF):
            cs = _strassen(lambda n: _dot(_up(y_s[n]), _up(t3_s[n, q])))
            for n, v in enumerate(_lhs_set(*[_gelu(cc) for cc in cs])):
                u_s[n, :, q * E:(q + 1) * E] = _pk(v)
        if not last:
            x1n = mix(j + 1)
        for q in range(D // E // 2):
            if last and q == 0:
                ks = FH - 2 * E
                head = [_dot(_up(u_s[n, :, 0:ks]), _up(t4_s[n, q, 0:ks // 2, :])) for n in range(7)]
                cs = _strassen(lambda n: _dot(_up(u_s[n, :, ks:FH]), _up(t4_s[n, q, ks // 2:, :]))
                               + head[n])
            else:
                cs = _strassen(lambda n: _dot(_up(u_s[n]), _up(t4_s[n, q])))
            ct = 4 * (q // 2) + q % 2
            for k, cc in enumerate(cs):
                rr = pl.ds(r0 + (k // 2) * TH, TH)
                cols = slice((ct + 2 * (k % 2)) * E, (ct + 2 * (k % 2) + 1) * E)
                gb = mod_s[0:1, 5 * D + cols.start:5 * D + cols.stop]
                o_s[slot, (k // 2) * TH:(k // 2 + 1) * TH, cols] = (
                    x2_s[rr, cols].astype(f32)
                    + gb * (hb_s[rr, cols].astype(f32) + cc)).astype(bf16)
        if not last:
            put_y(x1n)
            hb_s[pl.ds(pl.multiple_of((j + 1) * TB, TB), TB), :] = x1n.astype(bf16)
        out_copy(j, slot).start()

    def p3_body(j, carry):
        @pl.when(j >= 2)
        def _():
            out_copy(j - 2, j % 2).wait()

        mlp_block(j, False)
        return carry

    lax.fori_loop(0, NB - 1, _scoped("p3", p3_body), 0)
    out_copy(NB - 3, (NB - 3) % 2).wait()
    mlp_block(NB - 1, True)
    out_copy(NB - 2, (NB - 2) % 2).wait()
    out_copy(NB - 1, (NB - 1) % 2).wait()


@jax.jit
def pallas_adaLN_cond__memory_aug_recurrent_mem_tr__mixer_s_mlp__prompt_kernel(
    A_x: jax.Array,
    A_mem0: jax.Array,
    A_Wq: jax.Array,
    A_Wk: jax.Array,
    A_Wv: jax.Array,
    A_Wo: jax.Array,
    A_seg_len,
    B_x: jax.Array,
    B_w1: jax.Array,
    B_w2: jax.Array,
    B_w3: jax.Array,
    B_w4: jax.Array,
    c: jax.Array,
    w_mod: jax.Array,
):
    del A_seg_len, B_x
    assert A_x.shape == (1, S, D) and A_mem0.shape == (1, M, D)
    hbm = pl.BlockSpec(memory_space=pl.ANY)
    scratch = [
        pltpu.VMEM((NSEG, SEG, D), bf16),
        pltpu.VMEM((NSEG, M, D), bf16),
        pltpu.VMEM((NSEG * M // 2, D), u32),
        pltpu.VMEM((D, 2 * D), bf16),
        pltpu.VMEM((2, D, HG, E), bf16),
        pltpu.VMEM((3 * H + HG, D // 2, E), u32),
        pltpu.VMEM(((H * E + D) // 2, D), u32),
        pltpu.VMEM((D, D), bf16),
        pltpu.VMEM((7, NF, D // 4, E), u32),
        pltpu.VMEM((7, D // E // 2, FH // 2, E), u32),
        pltpu.VMEM((2, 2, 16, F), bf16),
        pltpu.VMEM((2, 2, G4R, D // 2), bf16),
        pltpu.VMEM((3 * NP, NSEG, M, E), u32),
        pltpu.VMEM((8, 6 * D), f32),
        pltpu.VMEM((M, D), f32),
        pltpu.VMEM((TC, D), f32),
        pltpu.VMEM((2 * SEG, D), f32),
        pltpu.VMEM((NR, E), f32),
        pltpu.VMEM((S, D), bf16),
        pltpu.VMEM((S, D), bf16),
        pltpu.VMEM((S + 16, D), f32),
        pltpu.VMEM((7, TB // 4, D // 2), u32),
        pltpu.VMEM((7, TB // 4, FH), u32),
        pltpu.VMEM((2, TB, D), bf16),
        pltpu.VMEM((8, E), u32),
        pltpu.VMEM((2, BGR, D), bf16),
        pltpu.VMEM((1, D), bf16),
        pltpu.VMEM((M, D), bf16),
        pltpu.VMEM((2, D, WMC), bf16),
        pltpu.VMEM((4 * D // E, 8, E), f32),
        pltpu.SemaphoreType.DMA((21,)),
    ]
    out = pl.pallas_call(
        _kernel,
        out_shape=jax.ShapeDtypeStruct((S, D), bf16),
        in_specs=[hbm] * 12,
        out_specs=hbm,
        scratch_shapes=scratch,
        compiler_params=pltpu.CompilerParams(vmem_limit_bytes=126 * 1024 * 1024,
                                             disable_bounds_checks=NO_BOUNDS),
    )(A_x.reshape(NSEG, SEG, D), A_mem0.reshape(M, D), A_Wq, A_Wk, A_Wv,
      A_Wo.reshape(H * E, D), B_w1, B_w2, B_w3.reshape(2, D // 2, F),
      B_w4.reshape(2, FH, D), c, w_mod)
    return out.reshape(1, S, D)
```

```python
import functools

import jax
import jax.numpy as jnp
from jax import lax
import jax.experimental.pallas as pl
import jax.experimental.pallas.tpu as pltpu

bf16, f32, u32 = jnp.bfloat16, jnp.float32, jnp.uint32

S, D, H, E, M, SEG, F = 2048, 1024, 32, 128, 8, 32, 3584
NSEG = S // SEG
NP = H // 2
TC = SEG - M
HG = 8
NG = H // HG
TB = 128
NB = S // TB
FH = F // 2
NF = FH // E
G4R = 64
NI = NSEG // 2
NQ = D // E // 2
NC = 3 * NG
WMC = 384
BGR = 512
NR = 2 * (M + SEG)
NO_BOUNDS = True
PIN_ROWS = 256
Y_AT = (0, 3, 6, 9)
G_AT = 4
LAG_S = 1
LAG_O = 3
ORDER = 2
EPS = 1e-5
SCALE = E ** -0.5
_SCOPES = False
_N2 = NSEG // 2


def _scoped(name, fn):
    def wrapped(*a):
        if not _SCOPES:
            return fn(*a)
        with jax.named_scope(name):
            return fn(*a)
    return wrapped


def _pk(x):
    return pltpu.bitcast(x.astype(bf16), u32)


def _up(x):
    return pltpu.bitcast(x, bf16)


def _dot(a, b):
    return jnp.dot(a, b, preferred_element_type=f32)


def _ln(x):
    m = jnp.mean(x, axis=-1, keepdims=True)
    xc = x - m
    v = jnp.mean(xc * xc, axis=-1, keepdims=True)
    return xc * lax.rsqrt(v + EPS)


def _gelu(x):
    c = 0.7978845608028654
    return 0.5 * x * (1.0 + jnp.tanh(c * (x + 0.044715 * (x * x * x))))


def _lhs_set(a11, a12, a21, a22):
    return (a11 + a22, a21 + a22, a11, a22, a11 + a12, a21 - a11, a12 - a22)


def _rhs_set(b11, b12, b21, b22):
    return (b11 + b22, b11, b12 - b22, b21 - b11, b22, b11 + b12, b21 + b22)


def _strassen(m):
    m1 = m(0)
    m2 = m(1)
    c22 = m1 - m2
    m3 = m(2)
    c22 = c22 + m3
    c22 = m(5) + c22
    m4 = m(3)
    c21 = m2 + m4
    c11 = m1 + m4
    m5 = m(4)
    c12 = m3 + m5
    c11 = c11 - m5
    c11 = m(6) + c11
    return c11, c12, c21, c22


def _mask_fill():
    shape = (NR, E)
    r = lax.broadcasted_iota(jnp.int32, shape, 0)
    c = lax.broadcasted_iota(jnp.int32, shape, 1)

    def headpos(i):
        head = jnp.where(i < 64, i >> 5, (i - 64) >> 3)
        pos = jnp.where(i < 64, i & 31, 32 + (i & 7))
        return head, pos

    hr, pr = headpos(r)
    hc, pc = headpos(c)
    same = hr == hc
    valid = same & ((pr < M) | (pr >= pc))
    return jnp.where(valid, 0.0, jnp.where(same, -1e9, -jnp.inf)).astype(f32)


def _kernel(x_hbm, mem0_hbm, wq_hbm, wk_hbm, wv_hbm, wo_hbm, w1_hbm, w2_hbm, w3_hbm,
            w4_hbm, c_hbm, wm_hbm,
            out_hbm,
            x_s, xpre_s, hpre_s, wm_s, stg, w_s, wo1_s,
            t2_s, t3_s, t4_s, g2, g3, g4, pre_s, mod_s, mem_s, hn_s, aout_s, fill_s,
            x2_s, hb_s, t_s, x1_s, g_s, y_s, u_s, o_s, zero_s, bg, c_s, mem0_s, wmr, modt_s, sems):
    w_hbm = (wq_hbm, wk_hbm, wv_hbm)

    (SEM_C, SEM_MEM, SEM_XPRE, SEM_X, SEM_STG, SEM_BG, SEM_OUT,
     SEM_WMR, SEM_G2, SEM_G3, SEM_G4, SEM_WM) = (0, 1, 2, 3, 4, 6, 8, 10, 12, 14, 16, 18)

    def copy(src, dst, k):
        return pltpu.make_async_copy(src, dst, sems.at[k])

    def w_copy(t, g, slot):
        return copy(w_hbm[t].at[:, pl.ds(pl.multiple_of(g * HG, HG), HG), :], stg.at[slot],
                    SEM_STG + slot)

    def bg_copy(src, b, slot):
        return copy(src.at[pl.ds(pl.multiple_of(b * BGR, BGR), BGR)], bg.at[slot], SEM_BG + slot)

    def wmr_tile(k):
        return jnp.minimum(k * (WMC // E), (4 * D - WMC) // E)

    def wmr_copy(k, slot):
        c0 = pl.multiple_of(2 * D + wmr_tile(k) * E, E)
        return copy(wm_hbm.at[:, pl.ds(c0, WMC)], wmr.at[slot], SEM_WMR + slot)

    def aligned(x, n):
        return x if isinstance(x, int) else pl.multiple_of(x, n)

    def clamp(k, hi):
        return min(k, hi) if isinstance(k, int) else jnp.minimum(k, hi)

    def mlp_w_copies(k, slot):
        r = pl.ds(aligned(clamp(k, NI - 1) * 16, 16), 16)
        r4 = pl.ds(aligned(clamp(k, FH // G4R - 1) * G4R, 16), G4R)
        return (copy(w2_hbm.at[:, r, :], g2.at[slot], SEM_G2 + slot),
                copy(w3_hbm.at[:, r, :], g3.at[slot], SEM_G3 + slot),
                copy(w4_hbm.at[:, r4, :], g4.at[slot], SEM_G4 + slot))

    def pinned(w, job):
        if job is None:
            return w()
        z = job() & zero_s[...]
        w = w()
        return jnp.concatenate([w[0:8] | z, w[8:]], axis=0)

    def rhs_job(src, slot, r0, c1, c2, dst, q, row):
        blk = [src[slot, kh, r0:r0 + 16, cc * E:(cc + 1) * E].astype(f32)
               for kh in range(2) for cc in (c1, c2)]
        z = None
        for n, v in enumerate(_rhs_set(*blk)):
            v = _pk(v)
            dst[n, q, pl.ds(pl.multiple_of(row, 8), 8), :] = v
            z = v if z is None else z | v
        return z

    def mod_row(k):
        return mod_s[0:1, k * D:(k + 1) * D]

    def relayout(slot, c, i):
        v = pltpu.bitcast(jnp.swapaxes(stg[slot, pl.ds(i * 16, 16)], 0, 1), u32)
        r = i * 8 if isinstance(i, int) else pl.multiple_of(i * 8, 8)
        w_s[pl.ds(c * HG, HG), pl.ds(r, 8), :] = v
        z = v[0]
        for h in range(1, HG):
            z = z | v[h]
        return z

    def repack(slot, b, i):
        v = pltpu.bitcast(bg[slot, 16 * i:16 * i + 16, :], u32)
        wo1_s[pl.ds(pl.multiple_of(b * (BGR // 2) + 8 * i, 8), 8), :] = v
        z = v[:, 0:E]
        for j in range(1, D // E):
            z = z | v[:, j * E:(j + 1) * E]
        return z

    HD = D // 2
    cp_c = copy(c_hbm, c_s, SEM_C)
    cp_mem = copy(mem0_hbm, mem0_s, SEM_MEM)
    cp_xpre = copy(x_hbm.at[:, TC:SEG, :], xpre_s, SEM_XPRE)
    wm_cols = (0, D, HD, D + HD)
    cp_wm = [copy(wm_hbm.at[:, c0:c0 + HD], wm_s.at[:, c0:c0 + HD], SEM_WM + k)
             for k, c0 in enumerate(wm_cols)]
    w_copy(0, 0, 0).start()
    cp_xpre.start()
    cp_c.start()
    cp_mem.start()
    for cp in cp_wm:
        cp.start()
    w_copy(0, 1, 1).start()

    zero_s[...] = jnp.zeros(zero_s.shape, u32)
    fill_s[...] = _mask_fill()
    aout_s[...] = jnp.zeros(aout_s.shape, f32)
    bg[1] = jnp.zeros(bg.shape[1:], bf16)
    wmr[1] = jnp.zeros(wmr.shape[1:], bf16)

    w_copy(0, 0, 0).wait()

    def rl0_body(i, carry):
        for k in range(4):
            relayout(0, 0, 4 * i + k)
        return carry

    lax.fori_loop(0, D // 64, rl0_body, 0)
    w_copy(0, 2, 0).start()
    bg_copy(wo_hbm, 0, 0).start()
    wmr_copy(0, 0).start()

    cp_xpre.wait()

    def npre_body(i, carry):
        xr = xpre_s[pl.ds(pl.multiple_of(i * 8, 8), 8)].astype(f32).reshape(64, D)
        t_s[pl.ds(pl.multiple_of(i * 64, 64), 64), :] = _ln(xr)
        return carry

    lax.fori_loop(0, NSEG // 8, _scoped("npre", npre_body), 0)

    cp_c.wait()
    cp_mem.wait()
    mem_s[...] = mem0_s[...].astype(f32)
    cf = c_s[...].astype(f32)
    sc = cf * (1.0 / (1.0 + jnp.exp(-cf)))
    sc8 = jnp.broadcast_to(sc, (8, D)).astype(bf16)

    for half in range(2):
        for k in (2 * half, 2 * half + 1):
            c0 = wm_cols[k]
            cp_wm[k].wait()
            mod_s[:, c0:c0 + HD] = _dot(sc8, wm_s[:, c0:c0 + HD])
        cols = slice(half * HD, (half + 1) * HD)
        shift = mod_s[0:1, half * HD:(half + 1) * HD]
        scale1 = 1.0 + mod_s[0:1, D + half * HD:D + (half + 1) * HD]
        hpre_s[:, cols] = _pk(t_s[0:NSEG * M, cols] * scale1 + shift)

    t_s[0:8, :] = jnp.zeros((8, D), f32)
    t_s[S + 8:S + 16, :] = jnp.zeros((8, D), f32)

    def modulate_a(xr):
        return _ln(xr) * (1.0 + mod_row(1)) + mod_row(0)

    MB = 128
    cp_x = copy(x_hbm, x_s, SEM_X)

    def pre_pair(c, pp, side, extra):
        ys = []
        for hh in range(2):
            blocks = []
            for mb in range(NSEG * M // MB):
                h = c * HG + 2 * pp + hh
                halves = []
                for k in range(2):
                    z = side()
                    w = w_s[h, k * 256:(k + 1) * 256, :]
                    if z is not None:
                        w = jnp.concatenate([w[0:8] | (z & zero_s[...]), w[8:]], axis=0)
                    halves.append(w)
                w = jnp.concatenate(halves, axis=0)
                blocks.append(_dot(_up(hpre_s[mb * MB // 2:(mb + 1) * MB // 2, :]), _up(w)))
            ys.append(jnp.concatenate(blocks, axis=0).reshape(NSEG, M, E))
            extra()
        y = jnp.concatenate(ys, axis=1)
        pre_s[c * (HG // 2) + pp] = pltpu.bitcast(y.astype(bf16), u32)

    NWO = H * E // BGR
    NBG = NWO + D // BGR

    def p1_body(c, carry):
        slot = c % 2
        pslot = 1 - slot
        b = jnp.clip(c - 1, 0, NBG - 1)
        bslot = jnp.where(c == 0, 1, b % 2)

        @pl.when(jnp.logical_and(c >= 1, c <= NBG))
        def _():
            bg_copy(wo_hbm, 0, bslot).wait()

        @pl.when(c >= 1)
        def _():
            wmr_copy(0, pslot).wait()

        @pl.when(c + 1 < NC)
        def _():
            w_copy(0, 0, pslot).wait()

        units = iter(range(-1, D // 16))

        def side():
            i = next(units)
            if i < 0:
                return None
            z = relayout(pslot, c + 1, i)
            if i % 2 == 0:
                z = z | repack(bslot, b, i // 2)
            return z

        mt = wmr_tile(jnp.maximum(c - 1, 0))
        halves = iter(range(2 * HG))
        part = [None]

        def extra():
            k = next(halves)
            j, hf = k // 2, k % 2
            if j >= WMC // E:
                return
            y = _dot(sc8[:, hf * HD:(hf + 1) * HD],
                     wmr[pslot, hf * HD:(hf + 1) * HD, j * E:(j + 1) * E])
            if hf == 0:
                part[0] = y
            else:
                modt_s[mt + j] = y + part[0]

        for pp in range(HG // 2):
            pre_pair(c, pp, side, extra)
        side()

        for t in range(3):
            @pl.when((c + 3) // NG == t)
            def _():
                w_copy(t, (c + 3) % NG, pslot).start()

        @pl.when(c + 1 < NWO)
        def _():
            bg_copy(wo_hbm, c + 1, pslot).start()

        @pl.when(jnp.logical_and(c + 1 >= NWO, c + 1 < NBG))
        def _():
            bg_copy(w1_hbm, c + 1 - NWO, pslot).start()

        @pl.when(c + 2 < NC)
        def _():
            wmr_copy(c + 1, pslot).start()

        @pl.when(c == NC - 3)
        def _():
            cp_x.start()

        @pl.when(c == NC - 2)
        def _():
            for k in range(2):
                for cp in mlp_w_copies(k, k):
                    cp.start()

        return carry

    lax.fori_loop(0, NC, _scoped("p1", p1_body), 0)
    mod_s[:, 2 * D:6 * D] = jnp.concatenate([modt_s[j] for j in range(4 * D // E)], axis=1)
    cp_x.wait()

    def h_rows(s):
        return modulate_a(x_s[s, 0:TC, :].astype(f32))

    hn_s[...] = h_rows(0)

    def chain_step(s, mem, htok, odef_prev, jobs=()):
        hs = jnp.concatenate([mem, htok], axis=0).astype(bf16)
        qkv = [[None] * 3 for _ in range(NP)]
        ps = [None] * NP
        os_ = [None] * H
        odef = [None] * H

        def proj(p, ts=(0, 1, 2)):
            for t in ts:
                a = _dot(hs, _up(w_s[t * H + 2 * p]))
                b = _dot(hs, _up(w_s[t * H + 2 * p + 1]))
                pre = pre_s[t * NP + p, s]
                if t == 1:
                    kf = jnp.concatenate([a, b, _up(pre).astype(f32), jnp.zeros((E - NR, E), f32)],
                                         axis=0)
                    qkv[p][t] = kf.T.astype(bf16)
                    continue
                parts = [_pk(a), _pk(b), pre]
                if t == 2:
                    parts.append(jnp.zeros(((E - NR) // 2, E), u32))
                qkv[p][t] = _up(jnp.concatenate(parts, axis=0))

        def scores(p):
            sc_ = _dot(qkv[p][0], qkv[p][1])
            fill = fill_s[...]
            sc_ = jnp.where(fill == 0.0, sc_ * SCALE, fill)
            m = jnp.max(sc_, axis=-1, keepdims=True)
            e = jnp.exp(sc_ - m)
            l = jnp.sum(e, axis=-1, keepdims=True)
            r = pl.reciprocal(l, approx=True)
            r = r * (2.0 - l * r)
            ps[p] = (e * r).astype(bf16)

        def fin(p):
            o = _dot(ps[p], qkv[p][2])
            for hh in range(2):
                h = 2 * p + hh
                rows = o[32 * hh:32 * hh + 32]
                odef[h] = o[64 + 8 * hh:72 + 8 * hh]
                if odef_prev is not None:
                    rows = jnp.concatenate([rows, odef_prev[h], odef[h]], axis=0)
                os_[h] = _pk(rows)

        acc = [None] * 8
        jobs = iter(jobs)

        def wo(h0, h1, js):
            lhs = _up(jnp.concatenate(os_[h0:h1], axis=1))
            for j in js:
                ws = []
                for r0 in range(h0 * E // 2, h1 * E // 2, PIN_ROWS):
                    ws.append(pinned(lambda: wo1_s[r0:r0 + PIN_ROWS, j * E:(j + 1) * E],
                                     next(jobs, None)))
                part = _dot(lhs, _up(jnp.concatenate(ws, axis=0)))
                acc[j] = part if acc[j] is None else part + acc[j]

        for p in range(NP):
            if ORDER == 0:
                proj(p)
                if p >= LAG_S:
                    scores(p - LAG_S)
                if p >= LAG_O:
                    fin(p - LAG_O)
            elif ORDER == 1:
                proj(p, (1, 0))
                if p >= LAG_O:
                    fin(p - LAG_O)
                proj(p, (2,))
                if p >= LAG_S:
                    scores(p - LAG_S)
            elif ORDER == 2:
                proj(p, (1,))
                if p >= LAG_S:
                    scores(p - LAG_S)
                proj(p, (0,))
                if p >= LAG_O:
                    fin(p - LAG_O)
                proj(p, (2,))
            else:
                proj(p, (1, 0, 2))
                if p >= LAG_O:
                    fin(p - LAG_O)
                if p >= LAG_S:
                    scores(p - LAG_S)
        tail = []
        for k in range(LAG_O):
            step = []
            if NP - LAG_S + k < NP:
                step.append(functools.partial(scores, NP - LAG_S + k))
            step.append(functools.partial(fin, NP - LAG_O + k))
            tail.append(step)
        hsplit = min(24, 2 * (NP - LAG_O))
        cuts = {3: (2, 3, 5), 2: (2, 5), 4: (1, 2, 4, 6), 5: (1, 2, 3, 4, 6)}[LAG_O]
        j0 = 0
        for k, step in enumerate(tail):
            wo(0, hsplit, range(j0, cuts[k]))
            j0 = cuts[k]
            for f in step:
                f()
        wo(0, hsplit, range(j0, 8))
        wo(hsplit, H, range(8))
        return jnp.concatenate(acc, axis=1), odef

    def mixer_prep(i):
        r = pl.ds(i * 64 if isinstance(i, int) else pl.multiple_of(i * 64, 64), 64)
        xr = x_s[pl.ds(2 * i, 2)].astype(f32).reshape(2 * SEG, D)
        x2 = xr + mod_row(2) * aout_s[...]
        x2_s[r, :] = x2.astype(bf16)
        hb = _ln(x2) * (1.0 + mod_row(4)) + mod_row(3)
        hb_s[r, :] = hb.astype(bf16)
        return _ln(hb).astype(bf16)

    def mixer_mm(i, lhs):
        t = _gelu(_dot(lhs, _up(wo1_s[H * E // 2:, :])))
        r0 = i * 64 + 8
        t_s[pl.ds(r0 if isinstance(i, int) else pl.multiple_of(r0, 8), 64), :] = t

    def p2_body(i, carry):
        slot = i & 1
        for cp in mlp_w_copies(0, slot):
            cp.wait()
        work = [functools.partial(rhs_job, g3, slot, 0, q, NF + q, t3_s, q, i * 8)
                for q in range(NF)]
        work += [functools.partial(rhs_job, g2, slot, 0, q, NQ + q, t2_s, q, i * 8)
                 for q in range(NQ)]
        row4 = clamp(i, FH // G4R - 1) * (G4R // 2)
        work += [functools.partial(rhs_job, g4, slot, 16 * rt, q, NQ + q, t4_s, q, row4 + 8 * rt)
                 for rt in range(G4R // 16) for q in range(NQ)]
        npin = 60
        jobs = [None] * npin
        for k, job in enumerate(work):
            jobs[1 + k * (npin - 1) // len(work)] = job

        sa_ = 2 * i
        sb_ = 2 * i + 1
        hb_tok = h_rows(sb_)
        oa, odef_a = chain_step(sa_, mem_s[...], hn_s[...], None)
        ip = jnp.maximum(i - 1, 0)
        mixer_mm(ip, mixer_prep(ip))
        ob, _ = chain_step(sb_, oa[0:M], hb_tok, odef_a, jobs)
        mem_s[...] = ob[0:M]
        aout_s[0:TC, :] = oa[M:SEG]
        aout_s[TC:SEG, :] = ob[SEG:SEG + M]
        aout_s[SEG:SEG + TC, :] = ob[M:SEG]
        aout_s[SEG + TC:2 * SEG, :] = ob[SEG + M:SEG + 2 * M]
        hn_s[...] = h_rows(jnp.minimum(sb_ + 1, NSEG - 1))
        for cp in mlp_w_copies(i + 2, slot):
            cp.start()
        return carry

    lax.fori_loop(0, _N2, _scoped("p2", p2_body), 0)

    for k in range(2):
        for cp in mlp_w_copies(0, k):
            cp.wait()

    TH = TB // 2
    SHIFT = (-1, -1, 1, 1, -2, -2, 2, 2)

    def after(x, anchor):
        if anchor is None:
            return x
        z = pltpu.bitcast(pltpu.bitcast(anchor[0:8], u32) & zero_s[...], f32)
        z = jnp.concatenate([z] * (x.shape[0] // 8), axis=0)
        return jnp.concatenate([x[:, 0:E] + z, x[:, E:]], axis=1) if x.shape[1] > E else x + z

    def g_job(j, rt, q, n=16, anchor=None):
        blk = []
        for hf in range(2):
            for ct in (q, NQ + q):
                win = t_s[pl.ds(aligned(j * TB + hf * TH + rt * n, 16), n + 16), ct * E:(ct + 1) * E]
                blk.append(win[8 + SHIFT[ct]:8 + SHIFT[ct] + n])
        blk[0] = after(blk[0], anchor)
        blk[3] = after(blk[3], anchor)
        for k, v in enumerate(_lhs_set(*blk)):
            g_s[k, rt * n // 2:(rt + 1) * n // 2, q * E:(q + 1) * E] = _pk(v)

    def mix(j):
        r0 = aligned(j * TB, TB)
        for q in range(NQ):
            cs = _strassen(lambda n: _dot(_up(g_s[n]), _up(t2_s[n, q])))
            for k, cc in enumerate(cs):
                rr = pl.ds(r0 + (k // 2) * TH, TH)
                c0 = (q + NQ * (k % 2)) * E
                x1 = hb_s[rr, c0:c0 + E].astype(f32) + cc
                x1_s[(k // 2) * TH:(k // 2 + 1) * TH, c0:c0 + E] = x1
                hb_s[rr, c0:c0 + E] = x1.astype(bf16)

    def out_copy(j, slot):
        return copy(o_s.at[slot], out_hbm.at[pl.ds(aligned(j * TB, TB), TB)], SEM_OUT + slot)

    prev_y = [None]

    def put_y(rt=0, n=TH, anchor=None):
        if anchor is not None and rt > 0:
            anchor = anchor[0:8] + prev_y[0]
        ya = _ln(after(x1_s[rt * n:(rt + 1) * n, :], anchor))
        yb = _ln(after(x1_s[TH + rt * n:TH + (rt + 1) * n, :], anchor))
        sets = _lhs_set(ya[:, :HD], ya[:, HD:], yb[:, :HD], yb[:, HD:])
        prev_y[0] = sets[0][0:8, 0:E] + sets[0][8:16, 0:E]
        for k, v in enumerate(sets):
            y_s[k, rt * n // 2:(rt + 1) * n // 2, :] = _pk(v)

    lhs_last = mixer_prep(NI - 1)
    for q in range(NQ):
        g_job(0, 0, q, TH)
    mix(0)
    mixer_mm(NI - 1, lhs_last)
    put_y()
    for q in range(NQ):
        g_job(1, 0, q, TH)

    def mlp_block(j, last):
        slot = j & 1
        r0 = aligned(j * TB, TB)
        for q in range(NF):
            cs = _strassen(lambda n: _dot(_up(y_s[n]), _up(t3_s[n, q])))
            for n, v in enumerate(_lhs_set(*[_gelu(cc) for cc in cs])):
                u_s[n, :, q * E:(q + 1) * E] = _pk(v)
        jobs = {}
        if not last:
            mix(j + 1)
            jn = clamp(j + 2, NB - 1)
            for rt in range(TH // 16):
                jobs[Y_AT[rt]] = functools.partial(put_y, rt, 16)
            free = [k for k in range(G_AT, 7 * NQ) if k not in jobs]
            for k in range(TH // 16 * NQ):
                jobs[free[k]] = functools.partial(g_job, jn, k // NQ, k % NQ, 16)

        def prod(n, q):
            m = _dot(_up(u_s[n]), _up(t4_s[n, q]))
            job = jobs.get(count[0])
            count[0] += 1
            if job is not None:
                job(anchor=m)
            return m

        count = [0]
        for q in range(NQ):
            if last and q == 0:
                ks = FH - 2 * E
                head = [_dot(_up(u_s[n, :, 0:ks]), _up(t4_s[n, q, 0:ks // 2, :])) for n in range(7)]
                cs = _strassen(lambda n: _dot(_up(u_s[n, :, ks:FH]), _up(t4_s[n, q, ks // 2:, :]))
                               + head[n])
            else:
                cs = _strassen(lambda n: prod(n, q))
            for k, cc in enumerate(cs):
                rr = pl.ds(r0 + (k // 2) * TH, TH)
                c0 = (q + NQ * (k % 2)) * E
                gb = mod_s[0:1, 5 * D + c0:5 * D + c0 + E]
                o_s[slot, (k // 2) * TH:(k // 2 + 1) * TH, c0:c0 + E] = (
                    x2_s[rr, c0:c0 + E].astype(f32)
                    + gb * (hb_s[rr, c0:c0 + E].astype(f32) + cc)).astype(bf16)
        out_copy(j, slot).start()

    def p3_body(j, carry):
        @pl.when(j >= 2)
        def _():
            out_copy(j - 2, j & 1).wait()

        mlp_block(j, False)
        return carry

    lax.fori_loop(0, NB - 1, _scoped("p3", p3_body), 0)
    out_copy(NB - 3, (NB - 3) % 2).wait()
    mlp_block(NB - 1, True)
    out_copy(NB - 2, (NB - 2) % 2).wait()
    out_copy(NB - 1, (NB - 1) % 2).wait()


@jax.jit
def pallas_adaLN_cond__memory_aug_recurrent_mem_tr__mixer_s_mlp__prompt_kernel(
    A_x: jax.Array,
    A_mem0: jax.Array,
    A_Wq: jax.Array,
    A_Wk: jax.Array,
    A_Wv: jax.Array,
    A_Wo: jax.Array,
    A_seg_len,
    B_x: jax.Array,
    B_w1: jax.Array,
    B_w2: jax.Array,
    B_w3: jax.Array,
    B_w4: jax.Array,
    c: jax.Array,
    w_mod: jax.Array,
):
    del A_seg_len, B_x
    assert A_x.shape == (1, S, D) and A_mem0.shape == (1, M, D)
    hbm = pl.BlockSpec(memory_space=pl.ANY)
    scratch = [
        pltpu.VMEM((NSEG, SEG, D), bf16),
        pltpu.VMEM((NSEG, M, D), bf16),
        pltpu.VMEM((NSEG * M // 2, D), u32),
        pltpu.VMEM((D, 2 * D), bf16),
        pltpu.VMEM((2, D, HG, E), bf16),
        pltpu.VMEM((3 * H + HG, D // 2, E), u32),
        pltpu.VMEM(((H * E + D) // 2, D), u32),
        pltpu.VMEM((7, NQ, D // 4, E), u32),
        pltpu.VMEM((7, NF, D // 4, E), u32),
        pltpu.VMEM((7, NQ, FH // 2, E), u32),
        pltpu.VMEM((2, 2, 16, D), bf16),
        pltpu.VMEM((2, 2, 16, F), bf16),
        pltpu.VMEM((2, 2, G4R, D), bf16),
        pltpu.VMEM((3 * NP, NSEG, M, E), u32),
        pltpu.VMEM((8, 6 * D), f32),
        pltpu.VMEM((M, D), f32),
        pltpu.VMEM((TC, D), f32),
        pltpu.VMEM((2 * SEG, D), f32),
        pltpu.VMEM((NR, E), f32),
        pltpu.VMEM((S, D), bf16),
        pltpu.VMEM((S, D), bf16),
        pltpu.VMEM((S + 16, D), f32),
        pltpu.VMEM((TB, D), f32),
        pltpu.VMEM((7, TB // 4, D // 2), u32),
        pltpu.VMEM((7, TB // 4, D // 2), u32),
        pltpu.VMEM((7, TB // 4, FH), u32),
        pltpu.VMEM((2, TB, D), bf16),
        pltpu.VMEM((8, E), u32),
        pltpu.VMEM((2, BGR, D), bf16),
        pltpu.VMEM((1, D), bf16),
        pltpu.VMEM((M, D), bf16),
        pltpu.VMEM((2, D, WMC), bf16),
        pltpu.VMEM((4 * D // E, 8, E), f32),
        pltpu.SemaphoreType.DMA((22,)),
    ]
    out = pl.pallas_call(
        _kernel,
        out_shape=jax.ShapeDtypeStruct((S, D), bf16),
        in_specs=[hbm] * 12,
        out_specs=hbm,
        scratch_shapes=scratch,
        compiler_params=pltpu.CompilerParams(vmem_limit_bytes=126 * 1024 * 1024,
                                             disable_bounds_checks=NO_BOUNDS),
    )(A_x.reshape(NSEG, SEG, D), A_mem0.reshape(M, D), A_Wq, A_Wk, A_Wv,
      A_Wo.reshape(H * E, D), B_w1, B_w2.reshape(2, D // 2, D), B_w3.reshape(2, D // 2, F),
      B_w4.reshape(2, FH, D), c, w_mod)
    return out.reshape(1, S, D)
```

```python
import functools

import jax
import jax.numpy as jnp
from jax import lax
import jax.experimental.pallas as pl
import jax.experimental.pallas.tpu as pltpu

bf16, f32, u32 = jnp.bfloat16, jnp.float32, jnp.uint32

S, D, H, E, M, SEG, F = 2048, 1024, 32, 128, 8, 32, 3584
NSEG = S // SEG
NP = H // 2
TC = SEG - M
HG = 8
NG = H // HG
TB = 128
NB = S // TB
FH = F // 2
NF = FH // E
G4R = 64
NI = NSEG // 2
NQ = D // E // 2
NC = 3 * NG
BGR = 512
HD = D // 2
X0 = 4
NR = 2 * (M + SEG)
NO_BOUNDS = True
PIN_ROWS = 256
Y_AT = (0, 7, 14, 21)
G_AT = 2
SORD = 0
FINE = 1
JGROUP = 1
P1_TAIL = 5
P1_LAG = 4
LAG_S = 1
LAG_O = 3
ORDER = 2
EPS = 1e-5
SCALE = E ** -0.5
_SCOPES = False
_N2 = NSEG // 2


def _scoped(name, fn):
    def wrapped(*a):
        if not _SCOPES:
            return fn(*a)
        with jax.named_scope(name):
            return fn(*a)
    return wrapped


def _pk(x):
    return pltpu.bitcast(x.astype(bf16), u32)


def _up(x):
    return pltpu.bitcast(x, bf16)


def _ct(k):
    return slice(k * E, (k + 1) * E)


def _dot(a, b):
    return jnp.dot(a, b, preferred_element_type=f32)


def _ln(x):
    m = jnp.mean(x, axis=-1, keepdims=True)
    xc = x - m
    v = jnp.mean(xc * xc, axis=-1, keepdims=True)
    return xc * lax.rsqrt(v + EPS)


def _gelu(x):
    c = 0.7978845608028654
    return 0.5 * x * (1.0 + jnp.tanh(c * (x + 0.044715 * (x * x * x))))


def _lhs_set(a11, a12, a21, a22):
    return (a11 + a22, a21 + a22, a11, a22, a11 + a12, a21 - a11, a12 - a22)


def _rhs_set(b11, b12, b21, b22):
    return (b11 + b22, b11, b12 - b22, b21 - b11, b22, b11 + b12, b21 + b22)


def _strassen(m):
    if SORD == 0:
        m1 = m(0)
        m2 = m(1)
        c22 = m1 - m2
        m3 = m(2)
        c22 = c22 + m3
        c22 = m(5) + c22
        m4 = m(3)
        c21 = m2 + m4
        c11 = m1 + m4
        m5 = m(4)
        c12 = m3 + m5
        c11 = c11 - m5
        c11 = m(6) + c11
    else:
        m2 = m(1)
        c22 = m(5) - m2
        m4 = m(3)
        c21 = m2 + m4
        m1 = m(0)
        c22 = c22 + m1
        c11 = m4 + m1
        m3 = m(2)
        c22 = c22 + m3
        m5 = m(4)
        c12 = m3 + m5
        c11 = c11 - m5
        c11 = m(6) + c11
    return c11, c12, c21, c22


def _mask_fill():
    shape = (NR, E)
    r = lax.broadcasted_iota(jnp.int32, shape, 0)
    c = lax.broadcasted_iota(jnp.int32, shape, 1)

    def headpos(i):
        head = jnp.where(i < 64, i >> 5, (i - 64) >> 3)
        pos = jnp.where(i < 64, i & 31, 32 + (i & 7))
        return head, pos

    hr, pr = headpos(r)
    hc, pc = headpos(c)
    same = hr == hc
    valid = same & ((pr < M) | (pr >= pc))
    return jnp.where(valid, 0.0, jnp.where(same, -1e9, -jnp.inf)).astype(f32)


def _kernel(x_hbm, mem0_hbm, wq_hbm, wk_hbm, wv_hbm, wo_hbm, w1_hbm, w2_hbm, w3_hbm,
            w4_hbm, c_hbm, wm_hbm,
            out_hbm,
            x_s, xpre_s, hpre_s, wm_s, stg, w_s, wo1_s,
            t2_s, t3_s, t4_s, g2, g3, g4, pre_s, mod_s, mem_s, hn_s, aout_s, fill_s,
            x2_s, hb_s, t_s, x1_s, g_s, y_s, u_s, o_s, zero_s, bg, c_s, mem0_s, sems):
    w_hbm = (wq_hbm, wk_hbm, wv_hbm)

    (SEM_C, SEM_MEM, SEM_XPRE, SEM_X, SEM_STG, SEM_BG, SEM_OUT,
     SEM_WMR, SEM_G2, SEM_G3, SEM_G4, SEM_WM) = (0, 1, 2, 3, 4, 6, 8, 10, 12, 14, 16, 18)

    def copy(src, dst, k):
        return pltpu.make_async_copy(src, dst, sems.at[k])

    def w_copy(t, g, slot):
        return copy(w_hbm[t].at[:, pl.ds(pl.multiple_of(g * HG, HG), HG), :], stg.at[slot],
                    SEM_STG + slot)

    def bg_copy(src, b, slot):
        return copy(src.at[pl.ds(pl.multiple_of(b * BGR, BGR), BGR)], bg.at[slot], SEM_BG + slot)

    def wm_copy(src_tile, dst_tile, sem):
        return copy(wm_hbm.at[:, pl.ds(aligned(src_tile * E, E), E)], wm_s.at[dst_tile], sem)

    def wm_wait(t0, n, sem):
        copy(wm_s.at[t0:t0 + n], wm_s.at[t0:t0 + n], sem).wait()

    def aligned(x, n):
        return x if isinstance(x, int) else pl.multiple_of(x, n)

    def clamp(k, hi):
        return min(k, hi) if isinstance(k, int) else jnp.minimum(k, hi)

    def mlp_w_copies(k, slot):
        r = pl.ds(aligned(clamp(k, NI - 1) * 16, 16), 16)
        r4 = pl.ds(aligned(clamp(k, FH // G4R - 1) * G4R, 16), G4R)
        return (copy(w2_hbm.at[:, r, :], g2.at[slot], SEM_G2 + slot),
                copy(w3_hbm.at[:, r, :], g3.at[slot], SEM_G3 + slot),
                copy(w4_hbm.at[:, r4, :], g4.at[slot], SEM_G4 + slot))

    def pinned(w, job):
        if job is None:
            return w()
        z = job() & zero_s[...]
        w = w()
        return jnp.concatenate([w[0:8] | z, w[8:]], axis=0)

    def after(x, anchor):
        if anchor is None:
            return x
        z = pltpu.bitcast(pltpu.bitcast(anchor[0:8], u32) & zero_s[...], f32)
        z = jnp.concatenate([z] * (x.shape[0] // 8), axis=0)
        return jnp.concatenate([x[:, 0:E] + z, x[:, E:]], axis=1) if x.shape[1] > E else x + z

    def rhs_job(src, slot, r0, c1, c2, dst, q, row):
        blk = [src[slot, kh, r0:r0 + 16, cc * E:(cc + 1) * E].astype(f32)
               for kh in range(2) for cc in (c1, c2)]
        z = None
        for n, v in enumerate(_rhs_set(*blk)):
            v = _pk(v)
            dst[n, pl.ds(pl.multiple_of(row, 8), 8), _ct(q)] = v
            z = v if z is None else z | v
        return z

    def mod_row(k):
        return mod_s[0:1, k * D:(k + 1) * D]

    def relayout_jobs(slot, c, i):
        memo = []
        r = aligned(i * 8, 8)

        def job(j, z=None):
            if not memo:
                for d0 in (i * 16, HD + i * 16):
                    memo.append(jnp.swapaxes(pltpu.bitcast(stg[slot, pl.ds(d0, 16)], u32), 0, 1))
            blk = []
            for kh in range(2):
                u = memo[kh][j]
                if z is not None:
                    u = u | jnp.concatenate([z, z], axis=0)
                blk.append(pltpu.bitcast(u << 16, f32))
                blk.append(pltpu.bitcast(u & jnp.uint32(0xFFFF0000), f32))
            for k, v in enumerate(blk):
                w_s.at[c][pl.ds((k // 2) * (D // 4) + r, 8), _ct(2 * j + k % 2)] = _pk(v)
            for n, v in enumerate(_rhs_set(*blk)):
                if n not in (1, 4):
                    t4_s.at[n][pl.ds(aligned(slot * (D // 4) + i * 8, 8), 8), _ct(j)] = _pk(v)

        return [functools.partial(job, j) for j in range(HG // 2)]

    def repack(slot, b, i, z):
        v = pltpu.bitcast(bg[slot, 16 * i:16 * i + 16, :], u32)
        v = v | jnp.concatenate([z] * (D // E), axis=1)
        wo1_s[pl.ds(pl.multiple_of(b * (BGR // 2) + 8 * i, 8), 8), :] = v

    cp_c = copy(c_hbm, c_s, SEM_C)
    cp_mem = copy(mem0_hbm, mem0_s, SEM_MEM)
    cp_xpre = copy(x_hbm.at[:, TC:SEG, :], xpre_s, SEM_XPRE)
    w_copy(0, 0, 0).start()
    cp_xpre.start()
    cp_c.start()
    cp_mem.start()
    for k in range(2 * D // E):
        wm_copy(k, k, SEM_WM + k // 4).start()
    w_copy(0, 1, 1).start()

    zero_s[...] = jnp.zeros(zero_s.shape, u32)
    fill_s[...] = _mask_fill()
    aout_s[...] = jnp.zeros(aout_s.shape, f32)
    bg[1] = jnp.zeros(bg.shape[1:], bf16)

    w_copy(0, 0, 0).wait()

    def rl0_body(i, carry):
        for job in relayout_jobs(0, 0, i):
            job()
        return carry

    lax.fori_loop(0, D // 32, rl0_body, 0)
    w_copy(0, 2, 0).start()
    bg_copy(wo_hbm, 0, 0).start()

    cp_xpre.wait()

    def npre_body(i, carry):
        xr = xpre_s[pl.ds(pl.multiple_of(i * 8, 8), 8)].astype(f32).reshape(64, D)
        t_s[pl.ds(pl.multiple_of(i * 64, 64), 64), :] = _ln(xr)
        return carry

    lax.fori_loop(0, NSEG // 8, _scoped("npre", npre_body), 0)

    cp_c.wait()
    cp_mem.wait()
    mem_s[...] = mem0_s[...].astype(f32)
    cf = c_s[...].astype(f32)
    sc = cf * (1.0 / (1.0 + jnp.exp(-cf)))
    sc8 = jnp.broadcast_to(sc, (8, D)).astype(bf16)

    def mod_tiles(t0, n, dst_tile):
        for k in range(n):
            mod_s[:, (dst_tile + k) * E:(dst_tile + k + 1) * E] = _dot(sc8, wm_s[t0 + k])

    for k in range(4):
        wm_wait(4 * k, 4, SEM_WM + k)
        mod_tiles(4 * k, 4, 4 * k)

    PH = NSEG * M // 2

    def hpre_body(i, carry):
        h = [t_s[pl.ds(pl.multiple_of(hf * PH + i * 16, 16), 16), :] * (1.0 + mod_row(1)) + mod_row(0)
             for hf in range(2)]
        for n, v in enumerate(_lhs_set(h[0][:, :HD], h[0][:, HD:], h[1][:, :HD], h[1][:, HD:])):
            hpre_s.at[n][pl.ds(pl.multiple_of(i * 8, 8), 8), :] = _pk(v)
        return carry

    lax.fori_loop(0, PH // 16, _scoped("hpre", hpre_body), 0)

    t_s[0:8, :] = jnp.zeros((8, D), f32)
    t_s[S + 8:S + 16, :] = jnp.zeros((8, D), f32)

    def modulate_a(xr):
        return _ln(xr) * (1.0 + mod_row(1)) + mod_row(0)

    MB = 64

    def x_copy(k):
        r = slice(0, X0) if k == 0 else slice(X0, NSEG)
        return copy(x_hbm.at[r], x_s.at[r], SEM_XPRE if k == 0 else SEM_X)

    NWO = H * E // BGR
    NBG = NWO + D // BGR

    def p1_body(c, carry):
        slot = c & 1
        pslot = 1 - slot
        b = jnp.clip(c - 1, 0, NBG - 1)
        bslot = jnp.where(c == 0, 1, b & 1)

        @pl.when(jnp.logical_and(c >= 1, c <= NBG))
        def _():
            bg_copy(wo_hbm, 0, bslot).wait()

        @pl.when(c + 1 < NC)
        def _():
            w_copy(0, 0, pslot).wait()

        work = []
        for i in range(D // 32):
            js = relayout_jobs(pslot, c + 1, i)
            work += [js[k:k + JGROUP] for k in range(0, len(js), JGROUP)]
            work.append([functools.partial(repack, bslot, b, i)])
        npin = 7 * (HG // 2) * (PH // MB)
        jobs = [[] for _ in range(npin)]
        for k, group in enumerate(work):
            pos = k * (npin - P1_TAIL) * 8 // len(work)
            jobs[pos // 8] += [(job, pos % 8 if FINE else 0) for job in group]
        jobs = iter(jobs)

        def prod(n, q, mb):
            if n == 1:
                w = w_s[c, 0:D // 4, _ct(2 * q)]
            elif n == 4:
                w = w_s[c, D // 4:D // 2, _ct(2 * q + 1)]
            else:
                w = t4_s[n, pl.ds(pl.multiple_of(slot * (D // 4), D // 4), D // 4), _ct(q)]
            m = _dot(_up(hpre_s[n, mb * MB // 2:(mb + 1) * MB // 2, :]), _up(w))
            pending.append(m)
            if len(pending) > P1_LAG:
                anchor = pltpu.bitcast(pending.pop(0), u32)
                for job, g in next(jobs):
                    job(anchor[8 * g:8 * g + 8] & zero_s[...])
            return m

        pending = []
        ns = MB // M
        for q in range(HG // 2):
            for mb in range(PH // MB):
                cs = _strassen(lambda n: prod(n, q, mb))
                for hf in range(2):
                    y = jnp.concatenate([cs[2 * hf + k][sg * M:(sg + 1) * M]
                                         for sg in range(ns) for k in range(2)], axis=0)
                    s0 = hf * (NSEG // 2) + mb * ns
                    pre_s.at[c][s0 * M:(s0 + ns) * M, _ct(q)] = _pk(y)

        for t in range(3):
            @pl.when((c + 3) >> 2 == t)
            def _():
                w_copy(t, (c + 3) & 3, pslot).start()

        @pl.when(c + 1 < NWO)
        def _():
            bg_copy(wo_hbm, c + 1, pslot).start()

        @pl.when(jnp.logical_and(c + 1 >= NWO, c + 1 < NBG))
        def _():
            bg_copy(w1_hbm, c + 1 - NWO, pslot).start()

        @pl.when(c == NC - 3)
        def _():
            def issue(k, carry2):
                wm_copy(2 * D // E + k, k, SEM_WMR).start()
                return carry2

            x_copy(0).start()
            for k in range(2):
                for cp in mlp_w_copies(k, k):
                    cp.start()
            lax.fori_loop(0, 3 * D // E, issue, 0)

        return carry

    lax.fori_loop(0, NC, _scoped("p1", p1_body), 0)
    x_copy(1).start()
    for k in range(3 * D // E, 4 * D // E):
        wm_copy(2 * D // E + k, k, SEM_WM).start()
    x_copy(0).wait()
    wm_wait(0, 3 * D // E, SEM_WMR)
    mod_tiles(0, 3 * D // E, 2 * D // E)

    def h_rows(s):
        return modulate_a(x_s[s, 0:TC, :].astype(f32))

    hn_s[...] = h_rows(0)

    def chain_step(s, mem, htok, odef_prev, jobs=()):
        hs = jnp.concatenate([mem, htok], axis=0).astype(bf16)
        qkv = [[None] * 3 for _ in range(NP)]
        ps = [None] * NP
        os_ = [None] * H
        odef = [None] * H

        def proj(p, ts=(0, 1, 2)):
            for t in ts:
                c, q = t * NG + p // (HG // 2), p % (HG // 2)
                a = _dot(hs, _up(w_s[c, :, _ct(2 * q)]))
                b = _dot(hs, _up(w_s[c, :, _ct(2 * q + 1)]))
                pre = pre_s[c, pl.ds(pl.multiple_of(s * M, M), M), _ct(q)]
                if t == 1:
                    kf = jnp.concatenate([a, b, _up(pre).astype(f32), jnp.zeros((E - NR, E), f32)],
                                         axis=0)
                    qkv[p][t] = kf.T.astype(bf16)
                    continue
                parts = [_pk(a), _pk(b), pre]
                if t == 2:
                    parts.append(jnp.zeros(((E - NR) // 2, E), u32))
                qkv[p][t] = _up(jnp.concatenate(parts, axis=0))

        def scores(p):
            sc_ = _dot(qkv[p][0], qkv[p][1])
            fill = fill_s[...]
            sc_ = jnp.where(fill == 0.0, sc_ * SCALE, fill)
            m = jnp.max(sc_, axis=-1, keepdims=True)
            e = jnp.exp(sc_ - m)
            l = jnp.sum(e, axis=-1, keepdims=True)
            r = pl.reciprocal(l, approx=True)
            r = r * (2.0 - l * r)
            ps[p] = (e * r).astype(bf16)

        def fin(p):
            o = _dot(ps[p], qkv[p][2])
            for hh in range(2):
                h = 2 * p + hh
                rows = o[32 * hh:32 * hh + 32]
                odef[h] = o[64 + 8 * hh:72 + 8 * hh]
                if odef_prev is not None:
                    rows = jnp.concatenate([rows, odef_prev[h], odef[h]], axis=0)
                os_[h] = _pk(rows)

        acc = [None] * 8
        jobs = iter(jobs)

        def wo(h0, h1, js):
            lhs = _up(jnp.concatenate(os_[h0:h1], axis=1))
            for j in js:
                ws = []
                for r0 in range(h0 * E // 2, h1 * E // 2, PIN_ROWS):
                    ws.append(pinned(lambda: wo1_s[r0:r0 + PIN_ROWS, j * E:(j + 1) * E],
                                     next(jobs, None)))
                part = _dot(lhs, _up(jnp.concatenate(ws, axis=0)))
                acc[j] = part if acc[j] is None else part + acc[j]

        for p in range(NP):
            if ORDER == 0:
                proj(p)
                if p >= LAG_S:
                    scores(p - LAG_S)
                if p >= LAG_O:
                    fin(p - LAG_O)
            elif ORDER == 1:
                proj(p, (1, 0))
                if p >= LAG_O:
                    fin(p - LAG_O)
                proj(p, (2,))
                if p >= LAG_S:
                    scores(p - LAG_S)
            elif ORDER == 2:
                proj(p, (1,))
                if p >= LAG_S:
                    scores(p - LAG_S)
                proj(p, (0,))
                if p >= LAG_O:
                    fin(p - LAG_O)
                proj(p, (2,))
            else:
                proj(p, (1, 0, 2))
                if p >= LAG_O:
                    fin(p - LAG_O)
                if p >= LAG_S:
                    scores(p - LAG_S)
        tail = []
        for k in range(LAG_O):
            step = []
            if NP - LAG_S + k < NP:
                step.append(functools.partial(scores, NP - LAG_S + k))
            step.append(functools.partial(fin, NP - LAG_O + k))
            tail.append(step)
        hsplit = min(24, 2 * (NP - LAG_O))
        cuts = {3: (2, 3, 5), 2: (2, 5), 4: (1, 2, 4, 6), 5: (1, 2, 3, 4, 6)}[LAG_O]
        j0 = 0
        for k, step in enumerate(tail):
            wo(0, hsplit, range(j0, cuts[k]))
            j0 = cuts[k]
            for f in step:
                f()
        wo(0, hsplit, range(j0, 8))
        wo(hsplit, H, range(8))
        return jnp.concatenate(acc, axis=1), odef

    def mixer_prep(i, k=0, n=64, anchor=None):
        r = pl.ds(aligned(i * 64 + k * n, 16), n)
        if n == 64:
            xr = x_s[pl.ds(2 * i, 2)].astype(f32).reshape(2 * SEG, D)
        else:
            r0 = (k * n) % SEG
            xr = x_s[2 * i + (k * n) // SEG, r0:r0 + n, :].astype(f32)
        x2 = xr + mod_row(2) * after(aout_s[k * n:(k + 1) * n, :], anchor)
        x2_s[r, :] = x2.astype(bf16)
        hb = _ln(x2) * (1.0 + mod_row(4)) + mod_row(3)
        hb_s[r, :] = hb.astype(bf16)
        return _ln(hb)

    def mixer_mm(i, lhs):
        t = _gelu(_dot(lhs, _up(wo1_s[H * E // 2:, :])))
        r0 = i * 64 + 8
        t_s[pl.ds(r0 if isinstance(i, int) else pl.multiple_of(r0, 8), 64), :] = t

    def p2_body(i, carry):
        slot = i & 1
        for cp in mlp_w_copies(0, slot):
            cp.wait()

        @pl.when(i == 1)
        def _():
            x_copy(1).wait()

        work = [functools.partial(rhs_job, g3, slot, 0, q, NF + q, t3_s, q, i * 8)
                for q in range(NF)]
        work += [functools.partial(rhs_job, g2, slot, 0, q, NQ + q, t2_s, q, i * 8)
                 for q in range(NQ)]
        row4 = clamp(i, FH // G4R - 1) * (G4R // 2)
        work += [functools.partial(rhs_job, g4, slot, 16 * rt, q, NQ + q, t4_s, q, row4 + 8 * rt)
                 for rt in range(G4R // 16) for q in range(NQ)]
        npin = 60
        jobs = [None] * npin
        for k, job in enumerate(work):
            jobs[1 + k * (npin - 1) // len(work)] = job

        sa_ = 2 * i
        sb_ = 2 * i + 1
        hb_tok = h_rows(sb_)
        oa, odef_a = chain_step(sa_, mem_s[...], hn_s[...], None)
        ip = jnp.maximum(i - 1, 0)
        mixer_mm(ip, mixer_prep(ip).astype(bf16))
        ob, _ = chain_step(sb_, oa[0:M], hb_tok, odef_a, jobs)
        mem_s[...] = ob[0:M]
        aout_s[0:TC, :] = oa[M:SEG]
        aout_s[TC:SEG, :] = ob[SEG:SEG + M]
        aout_s[SEG:SEG + TC, :] = ob[M:SEG]
        aout_s[SEG + TC:2 * SEG, :] = ob[SEG + M:SEG + 2 * M]
        hn_s[...] = h_rows(jnp.minimum(sb_ + 1, NSEG - 1))
        for cp in mlp_w_copies(i + 2, slot):
            cp.start()
        return carry

    lax.fori_loop(0, _N2, _scoped("p2", p2_body), 0)

    for k in range(2):
        for cp in mlp_w_copies(0, k):
            cp.wait()

    TH = TB // 2
    SHIFT = (-1, -1, 1, 1, -2, -2, 2, 2)

    def g_job(j, rt, q, n=16, anchor=None):
        blk = []
        for hf in range(2):
            for ct in (q, NQ + q):
                win = t_s[pl.ds(aligned(j * TB + hf * TH + rt * n, 16), n + 16), ct * E:(ct + 1) * E]
                blk.append(win[8 + SHIFT[ct]:8 + SHIFT[ct] + n])
        blk[0] = after(blk[0], anchor)
        blk[3] = after(blk[3], anchor)
        for k, v in enumerate(_lhs_set(*blk)):
            g_s.at[k][rt * n // 2:(rt + 1) * n // 2, q * E:(q + 1) * E] = _pk(v)

    def mix(j):
        r0 = aligned(j * TB, TB)
        for q in range(NQ):
            cs = _strassen(lambda n: _dot(_up(g_s[n]), _up(t2_s[n, :, _ct(q)])))
            for k, cc in enumerate(cs):
                rr = pl.ds(r0 + (k // 2) * TH, TH)
                c0 = (q + NQ * (k % 2)) * E
                x1 = hb_s[rr, c0:c0 + E].astype(f32) + cc
                x1_s[(k // 2) * TH:(k // 2 + 1) * TH, c0:c0 + E] = x1
                hb_s[rr, c0:c0 + E] = x1.astype(bf16)

    def out_copy(j, slot):
        return copy(o_s.at[slot], out_hbm.at[pl.ds(aligned(j * TB, TB), TB)], SEM_OUT + slot)

    prev_y = [None]

    def put_y(rt=0, n=TH, anchor=None):
        if anchor is not None and rt > 0:
            anchor = anchor[0:8] + prev_y[0]
        ya = _ln(after(x1_s[rt * n:(rt + 1) * n, :], anchor))
        yb = _ln(after(x1_s[TH + rt * n:TH + (rt + 1) * n, :], anchor))
        sets = _lhs_set(ya[:, :HD], ya[:, HD:], yb[:, :HD], yb[:, HD:])
        prev_y[0] = sets[0][0:8, 0:E] + sets[0][8:16, 0:E]
        for k, v in enumerate(sets):
            y_s.at[k][rt * n // 2:(rt + 1) * n // 2, :] = _pk(v)

    wm_wait(3 * D // E, D // E, SEM_WM)
    mod_tiles(3 * D // E, D // E, 5 * D // E)
    lhs_last = mixer_prep(NI - 1).astype(bf16)
    for q in range(NQ):
        g_job(0, 0, q, TH)
    mix(0)
    mixer_mm(NI - 1, lhs_last)
    put_y()
    for q in range(NQ):
        g_job(1, 0, q, TH)

    def mlp_block(j, last):
        slot = j & 1
        r0 = aligned(j * TB, TB)
        for q in range(NF):
            cs = _strassen(lambda n: _dot(_up(y_s[n]), _up(t3_s[n, :, _ct(q)])))
            for n, v in enumerate(_lhs_set(*[_gelu(cc) for cc in cs])):
                u_s.at[n][:, q * E:(q + 1) * E] = _pk(v)
        jobs = {}
        if not last:
            mix(j + 1)
            jn = clamp(j + 2, NB - 1)
            for rt in range(TH // 16):
                jobs[Y_AT[rt]] = functools.partial(put_y, rt, 16)
            free = [k for k in range(G_AT, 7 * NQ) if k not in jobs]
            for k in range(TH // 16 * NQ):
                jobs[free[k]] = functools.partial(g_job, jn, k // NQ, k % NQ, 16)

        def prod(n, q):
            m = _dot(_up(u_s[n]), _up(t4_s[n, :, _ct(q)]))
            job = jobs.get(count[0])
            count[0] += 1
            if job is not None:
                job(anchor=m)
            return m

        count = [0]
        for q in range(NQ):
            if last and q == 0:
                ks = FH - 2 * E
                head = [_dot(_up(u_s[n, :, 0:ks]), _up(t4_s[n, 0:ks // 2, _ct(q)])) for n in range(7)]
                cs = _strassen(lambda n: _dot(_up(u_s[n, :, ks:FH]), _up(t4_s[n, ks // 2:, _ct(q)]))
                               + head[n])
            else:
                cs = _strassen(lambda n: prod(n, q))
            for k, cc in enumerate(cs):
                rr = pl.ds(r0 + (k // 2) * TH, TH)
                c0 = (q + NQ * (k % 2)) * E
                gb = mod_s[0:1, 5 * D + c0:5 * D + c0 + E]
                o_s[slot, (k // 2) * TH:(k // 2 + 1) * TH, c0:c0 + E] = (
                    x2_s[rr, c0:c0 + E].astype(f32)
                    + gb * (hb_s[rr, c0:c0 + E].astype(f32) + cc)).astype(bf16)
        out_copy(j, slot).start()

    def p3_body(j, carry):
        @pl.when(j >= 2)
        def _():
            out_copy(j - 2, j & 1).wait()

        mlp_block(j, False)
        return carry

    lax.fori_loop(0, NB - 1, _scoped("p3", p3_body), 0)
    out_copy(NB - 3, (NB - 3) % 2).wait()
    mlp_block(NB - 1, True)
    out_copy(NB - 2, (NB - 2) % 2).wait()
    out_copy(NB - 1, (NB - 1) % 2).wait()


@jax.jit
def pallas_adaLN_cond__memory_aug_recurrent_mem_tr__mixer_s_mlp__prompt_kernel(
    A_x: jax.Array,
    A_mem0: jax.Array,
    A_Wq: jax.Array,
    A_Wk: jax.Array,
    A_Wv: jax.Array,
    A_Wo: jax.Array,
    A_seg_len,
    B_x: jax.Array,
    B_w1: jax.Array,
    B_w2: jax.Array,
    B_w3: jax.Array,
    B_w4: jax.Array,
    c: jax.Array,
    w_mod: jax.Array,
):
    del A_seg_len, B_x
    assert A_x.shape == (1, S, D) and A_mem0.shape == (1, M, D)
    hbm = pl.BlockSpec(memory_space=pl.ANY)
    scratch = [
        pltpu.VMEM((NSEG, SEG, D), bf16),
        pltpu.VMEM((NSEG, M, D), bf16),
        pltpu.VMEM((7, NSEG * M // 4, D // 2), u32),
        pltpu.VMEM((4 * D // E, D, E), bf16),
        pltpu.VMEM((2, D, HG, E), bf16),
        pltpu.VMEM((NC + 1, D // 2, HG * E), u32),
        pltpu.VMEM(((H * E + D) // 2, D), u32),
        pltpu.VMEM((7, D // 4, D // 2), u32),
        pltpu.VMEM((7, D // 4, FH), u32),
        pltpu.VMEM((7, FH // 2, D // 2), u32),
        pltpu.VMEM((2, 2, 16, D), bf16),
        pltpu.VMEM((2, 2, 16, F), bf16),
        pltpu.VMEM((2, 2, G4R, D), bf16),
        pltpu.VMEM((NC, NSEG * M, HG // 2 * E), u32),
        pltpu.VMEM((8, 6 * D), f32),
        pltpu.VMEM((M, D), f32),
        pltpu.VMEM((TC, D), f32),
        pltpu.VMEM((2 * SEG, D), f32),
        pltpu.VMEM((NR, E), f32),
        pltpu.VMEM((S, D), bf16),
        pltpu.VMEM((S, D), bf16),
        pltpu.VMEM((S + 16, D), f32),
        pltpu.VMEM((TB, D), f32),
        pltpu.VMEM((7, TB // 4, D // 2), u32),
        pltpu.VMEM((7, TB // 4, D // 2), u32),
        pltpu.VMEM((7, TB // 4, FH), u32),
        pltpu.VMEM((2, TB, D), bf16),
        pltpu.VMEM((8, E), u32),
        pltpu.VMEM((2, BGR, D), bf16),
        pltpu.VMEM((1, D), bf16),
        pltpu.VMEM((M, D), bf16),
        pltpu.SemaphoreType.DMA((22,)),
    ]
    out = pl.pallas_call(
        _kernel,
        out_shape=jax.ShapeDtypeStruct((S, D), bf16),
        in_specs=[hbm] * 12,
        out_specs=hbm,
        scratch_shapes=scratch,
        compiler_params=pltpu.CompilerParams(vmem_limit_bytes=126 * 1024 * 1024,
                                             disable_bounds_checks=NO_BOUNDS),
    )(A_x.reshape(NSEG, SEG, D), A_mem0.reshape(M, D), A_Wq, A_Wk, A_Wv,
      A_Wo.reshape(H * E, D), B_w1, B_w2.reshape(2, D // 2, D), B_w3.reshape(2, D // 2, F),
      B_w4.reshape(2, FH, D), c, w_mod)
    return out.reshape(1, S, D)
```

```python
import functools

import jax
import jax.numpy as jnp
from jax import lax
import jax.experimental.pallas as pl
import jax.experimental.pallas.tpu as pltpu

bf16, f32, u32 = jnp.bfloat16, jnp.float32, jnp.uint32

S, D, H, E, M, SEG, F = 2048, 1024, 32, 128, 8, 32, 3584
NSEG = S // SEG
NP = H // 2
TC = SEG - M
HG = 8
NG = H // HG
TB = 128
NB = S // TB
FH = F // 2
NF = FH // E
G4R = 64
NI = NSEG // 2
NQ = D // E // 2
NC = 3 * NG
BGR = 512
HD = D // 2
X0 = 4
NR = 2 * (M + SEG)
NO_BOUNDS = True
PIN_ROWS = 256
Y_AT = (0, 7, 14, 21)
G_AT = 2
SORD = 0
FINE = 1
JGROUP = 1
P1_TAIL = 5
P1_LAG = 4
LAG_S = 1
LAG_O = 3
ORDER = 2
EPS = 1e-5
SCALE = E ** -0.5
_SCOPES = False
_N2 = NSEG // 2


def _scoped(name, fn):
    def wrapped(*a):
        if not _SCOPES:
            return fn(*a)
        with jax.named_scope(name):
            return fn(*a)
    return wrapped


def _pk(x):
    return pltpu.bitcast(x.astype(bf16), u32)


def _up(x):
    return pltpu.bitcast(x, bf16)


def _ct(k):
    return slice(k * E, (k + 1) * E)


def _dot(a, b):
    return jnp.dot(a, b, preferred_element_type=f32)


def _ln(x):
    m = jnp.mean(x, axis=-1, keepdims=True)
    xc = x - m
    v = jnp.mean(xc * xc, axis=-1, keepdims=True)
    return xc * lax.rsqrt(v + EPS)


def _gelu(x):
    c = 0.7978845608028654
    return 0.5 * x * (1.0 + jnp.tanh(c * (x + 0.044715 * (x * x * x))))


def _lhs_set(a11, a12, a21, a22):
    return (a11 + a22, a21 + a22, a11, a22, a11 + a12, a21 - a11, a12 - a22)


def _rhs_set(b11, b12, b21, b22):
    return (b11 + b22, b11, b12 - b22, b21 - b11, b22, b11 + b12, b21 + b22)


def _strassen(m):
    if SORD == 0:
        m1 = m(0)
        m2 = m(1)
        c22 = m1 - m2
        m3 = m(2)
        c22 = c22 + m3
        c22 = m(5) + c22
        m4 = m(3)
        c21 = m2 + m4
        c11 = m1 + m4
        m5 = m(4)
        c12 = m3 + m5
        c11 = c11 - m5
        c11 = m(6) + c11
    else:
        m2 = m(1)
        c22 = m(5) - m2
        m4 = m(3)
        c21 = m2 + m4
        m1 = m(0)
        c22 = c22 + m1
        c11 = m4 + m1
        m3 = m(2)
        c22 = c22 + m3
        m5 = m(4)
        c12 = m3 + m5
        c11 = c11 - m5
        c11 = m(6) + c11
    return c11, c12, c21, c22


def _mask_fill():
    shape = (NR, E)
    r = lax.broadcasted_iota(jnp.int32, shape, 0)
    c = lax.broadcasted_iota(jnp.int32, shape, 1)

    def headpos(i):
        head = jnp.where(i < 64, i >> 5, (i - 64) >> 3)
        pos = jnp.where(i < 64, i & 31, 32 + (i & 7))
        return head, pos

    hr, pr = headpos(r)
    hc, pc = headpos(c)
    same = hr == hc
    valid = same & ((pr < M) | (pr >= pc))
    return jnp.where(valid, 0.0, jnp.where(same, -1e9, -jnp.inf)).astype(f32)


def _kernel(x_hbm, mem0_hbm, wq_hbm, wk_hbm, wv_hbm, wo_hbm, w1_hbm, w2_hbm, w3_hbm,
            w4_hbm, c_hbm, wm_hbm,
            out_hbm,
            x_s, xpre_s, hpre_s, wm_s, stg, w_s, wo1_s,
            t2_s, t3_s, t4_s, g2, g3, g4, pre_s, mod_s, mem_s, hn_s, aout_s, fill_s,
            x2_s, hb_s, t_s, x1_s, g_s, y_s, u_s, o_s, zero_s, bg, c_s, mem0_s, sems):
    w_hbm = (wq_hbm, wk_hbm, wv_hbm)

    (SEM_C, SEM_MEM, SEM_XPRE, SEM_X, SEM_STG, SEM_BG, SEM_OUT,
     SEM_WMR, SEM_G2, SEM_G3, SEM_G4, SEM_WM) = (0, 1, 2, 3, 4, 6, 8, 10, 12, 14, 16, 18)

    def copy(src, dst, k):
        return pltpu.make_async_copy(src, dst, sems.at[k])

    def w_copy(t, g, slot):
        return copy(w_hbm[t].at[:, pl.ds(pl.multiple_of(g * HG, HG), HG), :], stg.at[slot],
                    SEM_STG + slot)

    def bg_copy(src, b, slot):
        return copy(src.at[pl.ds(pl.multiple_of(b * BGR, BGR), BGR)], bg.at[slot], SEM_BG + slot)

    def wm_copy(src_tile, dst_tile, sem):
        return copy(wm_hbm.at[:, pl.ds(aligned(src_tile * E, E), E)], wm_s.at[dst_tile], sem)

    def wm_wait(t0, n, sem):
        copy(wm_s.at[t0:t0 + n], wm_s.at[t0:t0 + n], sem).wait()

    def aligned(x, n):
        return x if isinstance(x, int) else pl.multiple_of(x, n)

    def clamp(k, hi):
        return min(k, hi) if isinstance(k, int) else jnp.minimum(k, hi)

    def mlp_w_copies(k, slot):
        r = pl.ds(aligned(clamp(k, NI - 1) * 16, 16), 16)
        r4 = pl.ds(aligned(clamp(k, FH // G4R - 1) * G4R, 16), G4R)
        return (copy(w2_hbm.at[:, r, :], g2.at[slot], SEM_G2 + slot),
                copy(w3_hbm.at[:, r, :], g3.at[slot], SEM_G3 + slot),
                copy(w4_hbm.at[:, r4, :], g4.at[slot], SEM_G4 + slot))

    def pinned(w, job):
        if job is None:
            return w()
        z = job() & zero_s[...]
        w = w()
        return jnp.concatenate([w[0:8] | z, w[8:]], axis=0)

    def after(x, anchor):
        if anchor is None:
            return x
        z = pltpu.bitcast(pltpu.bitcast(anchor[0:8], u32) & zero_s[...], f32)
        z = jnp.concatenate([z] * (x.shape[0] // 8), axis=0)
        return jnp.concatenate([x[:, 0:E] + z, x[:, E:]], axis=1) if x.shape[1] > E else x + z

    def rhs_job(src, slot, r0, c1, c2, dst, q, row):
        blk = [src[slot, kh, r0:r0 + 16, cc * E:(cc + 1) * E].astype(f32)
               for kh in range(2) for cc in (c1, c2)]
        z = None
        for n, v in enumerate(_rhs_set(*blk)):
            v = _pk(v)
            dst[n, pl.ds(pl.multiple_of(row, 8), 8), _ct(q)] = v
            z = v if z is None else z | v
        return z

    def mod_row(k):
        return mod_s[0:1, k * D:(k + 1) * D]

    def tq_place(c, n):
        if n == 1:
            return w_s.at[c], 0, None
        if n == 4:
            return w_s.at[c], D // 4, None
        if n == 6:
            return pre_s.at[c + 1], 0, 0
        k = (0, 2, 3, 5).index(n)
        return w_s.at[c + 2], (k // 2) * (D // 4), (k % 2) * (HG // 2)

    def relayout_jobs(slot, c, i):
        memo = []
        r = aligned(i * 8, 8)

        def job(j, z=None):
            if not memo:
                for d0 in (i * 16, HD + i * 16):
                    memo.append(jnp.swapaxes(pltpu.bitcast(stg[slot, pl.ds(d0, 16)], u32), 0, 1))
            blk = []
            for kh in range(2):
                u = memo[kh][j]
                if z is not None:
                    u = u | jnp.concatenate([z, z], axis=0)
                blk.append(pltpu.bitcast(u << 16, f32))
                blk.append(pltpu.bitcast(u & jnp.uint32(0xFFFF0000), f32))
            for k, v in enumerate(blk):
                w_s.at[c][pl.ds((k // 2) * (D // 4) + r, 8), _ct(2 * j + k % 2)] = _pk(v)
            for n, v in enumerate(_rhs_set(*blk)):
                if n not in (1, 4):
                    ref, r0, c0 = tq_place(c, n)
                    ref[pl.ds(r0 + r, 8), _ct(c0 + j)] = _pk(v)

        return [functools.partial(job, j) for j in range(HG // 2)]

    def repack(slot, b, i, z):
        v = pltpu.bitcast(bg[slot, 16 * i:16 * i + 16, :], u32)
        v = v | jnp.concatenate([z] * (D // E), axis=1)
        wo1_s[pl.ds(pl.multiple_of(b * (BGR // 2) + 8 * i, 8), 8), :] = v

    cp_c = copy(c_hbm, c_s, SEM_C)
    cp_mem = copy(mem0_hbm, mem0_s, SEM_MEM)
    cp_xpre = copy(x_hbm.at[:, TC:SEG, :], xpre_s, SEM_XPRE)
    w_copy(0, 0, 0).start()
    cp_xpre.start()
    cp_c.start()
    cp_mem.start()
    for k in range(2 * D // E):
        wm_copy(k, k, SEM_WM + k // 4).start()
    w_copy(0, 1, 1).start()

    zero_s[...] = jnp.zeros(zero_s.shape, u32)
    fill_s[...] = _mask_fill()
    aout_s[...] = jnp.zeros(aout_s.shape, f32)
    bg[1] = jnp.zeros(bg.shape[1:], bf16)

    w_copy(0, 0, 0).wait()

    def rl0_body(i, carry):
        for job in relayout_jobs(0, 0, i):
            job()
        return carry

    lax.fori_loop(0, D // 32, rl0_body, 0)
    w_copy(0, 2, 0).start()
    bg_copy(wo_hbm, 0, 0).start()

    cp_xpre.wait()

    def npre_body(i, carry):
        xr = xpre_s[pl.ds(pl.multiple_of(i * 8, 8), 8)].astype(f32).reshape(64, D)
        t_s[pl.ds(pl.multiple_of(i * 64, 64), 64), :] = _ln(xr)
        return carry

    lax.fori_loop(0, NSEG // 8, _scoped("npre", npre_body), 0)

    cp_c.wait()
    cp_mem.wait()
    mem_s[...] = mem0_s[...].astype(f32)
    cf = c_s[...].astype(f32)
    sc = cf * (1.0 / (1.0 + jnp.exp(-cf)))
    sc8 = jnp.broadcast_to(sc, (8, D)).astype(bf16)

    def mod_tiles(t0, n, dst_tile):
        for k in range(n):
            mod_s[:, (dst_tile + k) * E:(dst_tile + k + 1) * E] = _dot(sc8, wm_s[t0 + k])

    for k in range(4):
        wm_wait(4 * k, 4, SEM_WM + k)
        mod_tiles(4 * k, 4, 4 * k)

    PH = NSEG * M // 2

    def hpre_body(i, carry):
        h = [t_s[pl.ds(pl.multiple_of(hf * PH + i * 16, 16), 16), :] * (1.0 + mod_row(1)) + mod_row(0)
             for hf in range(2)]
        for n, v in enumerate(_lhs_set(h[0][:, :HD], h[0][:, HD:], h[1][:, :HD], h[1][:, HD:])):
            hpre_s.at[n][pl.ds(pl.multiple_of(i * 8, 8), 8), :] = _pk(v)
        return carry

    lax.fori_loop(0, PH // 16, _scoped("hpre", hpre_body), 0)

    t_s[0:8, :] = jnp.zeros((8, D), f32)
    t_s[S + 8:S + 16, :] = jnp.zeros((8, D), f32)

    def modulate_a(xr):
        return _ln(xr) * (1.0 + mod_row(1)) + mod_row(0)

    MB = 64

    def x_copy(k):
        r = slice(0, X0) if k == 0 else slice(X0, NSEG)
        return copy(x_hbm.at[r], x_s.at[r], SEM_XPRE if k == 0 else SEM_X)

    NWO = H * E // BGR
    NBG = NWO + D // BGR

    def p1_body(c, carry):
        slot = c & 1
        pslot = 1 - slot
        b = jnp.clip(c - 1, 0, NBG - 1)
        bslot = jnp.where(c == 0, 1, b & 1)

        @pl.when(jnp.logical_and(c >= 1, c <= NBG))
        def _():
            bg_copy(wo_hbm, 0, bslot).wait()

        @pl.when(c + 1 < NC)
        def _():
            w_copy(0, 0, pslot).wait()

        work = []
        for i in range(D // 32):
            js = relayout_jobs(pslot, c + 1, i)
            work += [js[k:k + JGROUP] for k in range(0, len(js), JGROUP)]
            work.append([functools.partial(repack, bslot, b, i)])
        npin = 7 * (HG // 2) * (PH // MB)
        jobs = [[] for _ in range(npin)]
        for k, group in enumerate(work):
            pos = k * (npin - P1_TAIL) * 8 // len(work)
            jobs[pos // 8] += [(job, pos % 8 if FINE else 0) for job in group]
        jobs = iter(jobs)

        def prod(n, q, mb):
            ref, r0, c0 = tq_place(c, n)
            w = ref[r0:r0 + D // 4, _ct(2 * q + (n == 4) if c0 is None else c0 + q)]
            m = _dot(_up(hpre_s[n, mb * MB // 2:(mb + 1) * MB // 2, :]), _up(w))
            pending.append(m)
            if len(pending) > P1_LAG:
                anchor = pltpu.bitcast(pending.pop(0), u32)
                for job, g in next(jobs):
                    job(anchor[8 * g:8 * g + 8] & zero_s[...])
            return m

        pending = []
        ns = MB // M
        for q in range(HG // 2):
            for mb in range(PH // MB):
                cs = _strassen(lambda n: prod(n, q, mb))
                for hf in range(2):
                    y = jnp.concatenate([cs[2 * hf + k][sg * M:(sg + 1) * M]
                                         for sg in range(ns) for k in range(2)], axis=0)
                    s0 = hf * (NSEG // 2) + mb * ns
                    pre_s.at[c][s0 * M:(s0 + ns) * M, _ct(q)] = _pk(y)

        for t in range(3):
            @pl.when((c + 3) >> 2 == t)
            def _():
                w_copy(t, (c + 3) & 3, pslot).start()

        @pl.when(c + 1 < NWO)
        def _():
            bg_copy(wo_hbm, c + 1, pslot).start()

        @pl.when(jnp.logical_and(c + 1 >= NWO, c + 1 < NBG))
        def _():
            bg_copy(w1_hbm, c + 1 - NWO, pslot).start()

        @pl.when(c == NC - 3)
        def _():
            def issue(k, carry2):
                wm_copy(2 * D // E + k, k, SEM_WMR).start()
                return carry2

            x_copy(0).start()
            for k in range(2):
                for cp in mlp_w_copies(k, k):
                    cp.start()
            lax.fori_loop(0, 3 * D // E, issue, 0)

        return carry

    lax.fori_loop(0, NC, _scoped("p1", p1_body), 0)
    x_copy(1).start()
    x_copy(0).wait()
    wm_wait(0, 3 * D // E, SEM_WMR)
    mod_tiles(0, 3 * D // E, 2 * D // E)
    for k in range(D // E):
        wm_copy(5 * D // E + k, k, SEM_WM).start()

    def h_rows(s):
        return modulate_a(x_s[s, 0:TC, :].astype(f32))

    hn_s[...] = h_rows(0)

    def chain_step(s, mem, htok, odef_prev, jobs=()):
        hs = jnp.concatenate([mem, htok], axis=0).astype(bf16)
        qkv = [[None] * 3 for _ in range(NP)]
        ps = [None] * NP
        os_ = [None] * H
        odef = [None] * H

        def proj(p, ts=(0, 1, 2)):
            for t in ts:
                c, q = t * NG + p // (HG // 2), p % (HG // 2)
                a = _dot(hs, _up(w_s[c, :, _ct(2 * q)]))
                b = _dot(hs, _up(w_s[c, :, _ct(2 * q + 1)]))
                pre = pre_s[c, pl.ds(pl.multiple_of(s * M, M), M), _ct(q)]
                if t == 1:
                    kf = jnp.concatenate([a, b, _up(pre).astype(f32), jnp.zeros((E - NR, E), f32)],
                                         axis=0)
                    qkv[p][t] = kf.T.astype(bf16)
                    continue
                parts = [_pk(a), _pk(b), pre]
                if t == 2:
                    parts.append(jnp.zeros(((E - NR) // 2, E), u32))
                qkv[p][t] = _up(jnp.concatenate(parts, axis=0))

        def scores(p):
            sc_ = _dot(qkv[p][0], qkv[p][1])
            fill = fill_s[...]
            sc_ = jnp.where(fill == 0.0, sc_ * SCALE, fill)
            m = jnp.max(sc_, axis=-1, keepdims=True)
            e = jnp.exp(sc_ - m)
            l = jnp.sum(e, axis=-1, keepdims=True)
            r = pl.reciprocal(l, approx=True)
            r = r * (2.0 - l * r)
            ps[p] = (e * r).astype(bf16)

        def fin(p):
            o = _dot(ps[p], qkv[p][2])
            for hh in range(2):
                h = 2 * p + hh
                rows = o[32 * hh:32 * hh + 32]
                odef[h] = o[64 + 8 * hh:72 + 8 * hh]
                if odef_prev is not None:
                    rows = jnp.concatenate([rows, odef_prev[h], odef[h]], axis=0)
                os_[h] = _pk(rows)

        acc = [None] * 8
        jobs = iter(jobs)

        def wo(h0, h1, js):
            lhs = _up(jnp.concatenate(os_[h0:h1], axis=1))
            for j in js:
                ws = []
                for r0 in range(h0 * E // 2, h1 * E // 2, PIN_ROWS):
                    ws.append(pinned(lambda: wo1_s[r0:r0 + PIN_ROWS, j * E:(j + 1) * E],
                                     next(jobs, None)))
                part = _dot(lhs, _up(jnp.concatenate(ws, axis=0)))
                acc[j] = part if acc[j] is None else part + acc[j]

        for p in range(NP):
            if ORDER == 0:
                proj(p)
                if p >= LAG_S:
                    scores(p - LAG_S)
                if p >= LAG_O:
                    fin(p - LAG_O)
            elif ORDER == 1:
                proj(p, (1, 0))
                if p >= LAG_O:
                    fin(p - LAG_O)
                proj(p, (2,))
                if p >= LAG_S:
                    scores(p - LAG_S)
            elif ORDER == 2:
                proj(p, (1,))
                if p >= LAG_S:
                    scores(p - LAG_S)
                proj(p, (0,))
                if p >= LAG_O:
                    fin(p - LAG_O)
                proj(p, (2,))
            else:
                proj(p, (1, 0, 2))
                if p >= LAG_O:
                    fin(p - LAG_O)
                if p >= LAG_S:
                    scores(p - LAG_S)
        tail = []
        for k in range(LAG_O):
            step = []
            if NP - LAG_S + k < NP:
                step.append(functools.partial(scores, NP - LAG_S + k))
            step.append(functools.partial(fin, NP - LAG_O + k))
            tail.append(step)
        hsplit = min(24, 2 * (NP - LAG_O))
        cuts = {3: (2, 3, 5), 2: (2, 5), 4: (1, 2, 4, 6), 5: (1, 2, 3, 4, 6)}[LAG_O]
        j0 = 0
        for k, step in enumerate(tail):
            wo(0, hsplit, range(j0, cuts[k]))
            j0 = cuts[k]
            for f in step:
                f()
        wo(0, hsplit, range(j0, 8))
        wo(hsplit, H, range(8))
        return jnp.concatenate(acc, axis=1), odef

    def mixer_prep(i, k=0, n=64, anchor=None):
        r = pl.ds(aligned(i * 64 + k * n, 16), n)
        if n == 64:
            xr = x_s[pl.ds(2 * i, 2)].astype(f32).reshape(2 * SEG, D)
        else:
            r0 = (k * n) % SEG
            xr = x_s[2 * i + (k * n) // SEG, r0:r0 + n, :].astype(f32)
        x2 = xr + mod_row(2) * after(aout_s[k * n:(k + 1) * n, :], anchor)
        x2_s[r, :] = x2.astype(bf16)
        hb = _ln(x2) * (1.0 + mod_row(4)) + mod_row(3)
        hb_s[r, :] = hb.astype(bf16)
        return _ln(hb)

    def mixer_mm(i, lhs):
        t = _gelu(_dot(lhs, _up(wo1_s[H * E // 2:, :])))
        r0 = i * 64 + 8
        t_s[pl.ds(r0 if isinstance(i, int) else pl.multiple_of(r0, 8), 64), :] = t

    def p2_body(i, carry):
        slot = i & 1
        for cp in mlp_w_copies(0, slot):
            cp.wait()

        @pl.when(i == 1)
        def _():
            x_copy(1).wait()

        work = [functools.partial(rhs_job, g3, slot, 0, q, NF + q, t3_s, q, i * 8)
                for q in range(NF)]
        work += [functools.partial(rhs_job, g2, slot, 0, q, NQ + q, t2_s, q, i * 8)
                 for q in range(NQ)]
        row4 = clamp(i, FH // G4R - 1) * (G4R // 2)
        work += [functools.partial(rhs_job, g4, slot, 16 * rt, q, NQ + q, t4_s, q, row4 + 8 * rt)
                 for rt in range(G4R // 16) for q in range(NQ)]
        npin = 60
        jobs = [None] * npin
        for k, job in enumerate(work):
            jobs[1 + k * (npin - 1) // len(work)] = job

        sa_ = 2 * i
        sb_ = 2 * i + 1
        hb_tok = h_rows(sb_)
        oa, odef_a = chain_step(sa_, mem_s[...], hn_s[...], None)
        ip = jnp.maximum(i - 1, 0)
        mixer_mm(ip, mixer_prep(ip).astype(bf16))
        ob, _ = chain_step(sb_, oa[0:M], hb_tok, odef_a, jobs)
        mem_s[...] = ob[0:M]
        aout_s[0:TC, :] = oa[M:SEG]
        aout_s[TC:SEG, :] = ob[SEG:SEG + M]
        aout_s[SEG:SEG + TC, :] = ob[M:SEG]
        aout_s[SEG + TC:2 * SEG, :] = ob[SEG + M:SEG + 2 * M]
        hn_s[...] = h_rows(jnp.minimum(sb_ + 1, NSEG - 1))
        for cp in mlp_w_copies(i + 2, slot):
            cp.start()
        return carry

    lax.fori_loop(0, _N2, _scoped("p2", p2_body), 0)

    for k in range(2):
        for cp in mlp_w_copies(0, k):
            cp.wait()

    TH = TB // 2
    SHIFT = (-1, -1, 1, 1, -2, -2, 2, 2)

    def g_job(j, rt, q, n=16, anchor=None):
        blk = []
        for hf in range(2):
            for ct in (q, NQ + q):
                win = t_s[pl.ds(aligned(j * TB + hf * TH + rt * n, 16), n + 16), ct * E:(ct + 1) * E]
                blk.append(win[8 + SHIFT[ct]:8 + SHIFT[ct] + n])
        blk[0] = after(blk[0], anchor)
        blk[3] = after(blk[3], anchor)
        for k, v in enumerate(_lhs_set(*blk)):
            g_s.at[k][rt * n // 2:(rt + 1) * n // 2, q * E:(q + 1) * E] = _pk(v)

    def mix(j):
        r0 = aligned(j * TB, TB)
        for q in range(NQ):
            cs = _strassen(lambda n: _dot(_up(g_s[n]), _up(t2_s[n, :, _ct(q)])))
            for k, cc in enumerate(cs):
                rr = pl.ds(r0 + (k // 2) * TH, TH)
                c0 = (q + NQ * (k % 2)) * E
                x1 = hb_s[rr, c0:c0 + E].astype(f32) + cc
                x1_s[(k // 2) * TH:(k // 2 + 1) * TH, c0:c0 + E] = x1
                hb_s[rr, c0:c0 + E] = x1.astype(bf16)

    def out_copy(j, slot):
        return copy(o_s.at[slot], out_hbm.at[pl.ds(aligned(j * TB, TB), TB)], SEM_OUT + slot)

    prev_y = [None]

    def put_y(rt=0, n=TH, anchor=None):
        if anchor is not None and rt > 0:
            anchor = anchor[0:8] + prev_y[0]
        ya = _ln(after(x1_s[rt * n:(rt + 1) * n, :], anchor))
        yb = _ln(after(x1_s[TH + rt * n:TH + (rt + 1) * n, :], anchor))
        sets = _lhs_set(ya[:, :HD], ya[:, HD:], yb[:, :HD], yb[:, HD:])
        prev_y[0] = sets[0][0:8, 0:E] + sets[0][8:16, 0:E]
        for k, v in enumerate(sets):
            y_s.at[k][rt * n // 2:(rt + 1) * n // 2, :] = _pk(v)

    wm_wait(0, D // E, SEM_WM)
    mod_tiles(0, D // E, 5 * D // E)
    lhs_last = mixer_prep(NI - 1).astype(bf16)
    for q in range(NQ):
        g_job(0, 0, q, TH)
    mix(0)
    mixer_mm(NI - 1, lhs_last)
    put_y()
    for q in range(NQ):
        g_job(1, 0, q, TH)

    def mlp_block(j, last):
        slot = j & 1
        r0 = aligned(j * TB, TB)
        for q in range(NF):
            cs = _strassen(lambda n: _dot(_up(y_s[n]), _up(t3_s[n, :, _ct(q)])))
            for n, v in enumerate(_lhs_set(*[_gelu(cc) for cc in cs])):
                u_s.at[n][:, q * E:(q + 1) * E] = _pk(v)
        jobs = {}
        if not last:
            mix(j + 1)
            jn = clamp(j + 2, NB - 1)
            for rt in range(TH // 16):
                jobs[Y_AT[rt]] = functools.partial(put_y, rt, 16)
            free = [k for k in range(G_AT, 7 * NQ) if k not in jobs]
            for k in range(TH // 16 * NQ):
                jobs[free[k]] = functools.partial(g_job, jn, k // NQ, k % NQ, 16)

        def prod(n, q):
            m = _dot(_up(u_s[n]), _up(t4_s[n, :, _ct(q)]))
            job = jobs.get(count[0])
            count[0] += 1
            if job is not None:
                job(anchor=m)
            return m

        count = [0]
        for q in range(NQ):
            if last and q == 0:
                ks = FH - 2 * E
                head = [_dot(_up(u_s[n, :, 0:ks]), _up(t4_s[n, 0:ks // 2, _ct(q)])) for n in range(7)]
                cs = _strassen(lambda n: _dot(_up(u_s[n, :, ks:FH]), _up(t4_s[n, ks // 2:, _ct(q)]))
                               + head[n])
            else:
                cs = _strassen(lambda n: prod(n, q))
            for k, cc in enumerate(cs):
                rr = pl.ds(r0 + (k // 2) * TH, TH)
                c0 = (q + NQ * (k % 2)) * E
                gb = mod_s[0:1, 5 * D + c0:5 * D + c0 + E]
                o_s[slot, (k // 2) * TH:(k // 2 + 1) * TH, c0:c0 + E] = (
                    x2_s[rr, c0:c0 + E].astype(f32)
                    + gb * (hb_s[rr, c0:c0 + E].astype(f32) + cc)).astype(bf16)
        out_copy(j, slot).start()

    def p3_body(j, carry):
        @pl.when(j >= 2)
        def _():
            out_copy(j - 2, j & 1).wait()

        mlp_block(j, False)
        return carry

    lax.fori_loop(0, NB - 1, _scoped("p3", p3_body), 0)
    out_copy(NB - 3, (NB - 3) % 2).wait()
    mlp_block(NB - 1, True)
    out_copy(NB - 2, (NB - 2) % 2).wait()
    out_copy(NB - 1, (NB - 1) % 2).wait()


@jax.jit
def pallas_adaLN_cond__memory_aug_recurrent_mem_tr__mixer_s_mlp__prompt_kernel(
    A_x: jax.Array,
    A_mem0: jax.Array,
    A_Wq: jax.Array,
    A_Wk: jax.Array,
    A_Wv: jax.Array,
    A_Wo: jax.Array,
    A_seg_len,
    B_x: jax.Array,
    B_w1: jax.Array,
    B_w2: jax.Array,
    B_w3: jax.Array,
    B_w4: jax.Array,
    c: jax.Array,
    w_mod: jax.Array,
):
    del A_seg_len, B_x
    assert A_x.shape == (1, S, D) and A_mem0.shape == (1, M, D)
    hbm = pl.BlockSpec(memory_space=pl.ANY)
    scratch = [
        pltpu.VMEM((NSEG, SEG, D), bf16),
        pltpu.VMEM((NSEG, M, D), bf16),
        pltpu.VMEM((7, NSEG * M // 4, D // 2), u32),
        pltpu.VMEM((3 * D // E, D, E), bf16),
        pltpu.VMEM((2, D, HG, E), bf16),
        pltpu.VMEM((NC + 3, D // 2, HG * E), u32),
        pltpu.VMEM(((H * E + D) // 2, D), u32),
        pltpu.VMEM((7, D // 4, D // 2), u32),
        pltpu.VMEM((7, D // 4, FH), u32),
        pltpu.VMEM((7, FH // 2, D // 2), u32),
        pltpu.VMEM((2, 2, 16, D), bf16),
        pltpu.VMEM((2, 2, 16, F), bf16),
        pltpu.VMEM((2, 2, G4R, D), bf16),
        pltpu.VMEM((NC + 2, NSEG * M, HG // 2 * E), u32),
        pltpu.VMEM((8, 6 * D), f32),
        pltpu.VMEM((M, D), f32),
        pltpu.VMEM((TC, D), f32),
        pltpu.VMEM((2 * SEG, D), f32),
        pltpu.VMEM((NR, E), f32),
        pltpu.VMEM((S, D), bf16),
        pltpu.VMEM((S, D), bf16),
        pltpu.VMEM((S + 16, D), f32),
        pltpu.VMEM((TB, D), f32),
        pltpu.VMEM((7, TB // 4, D // 2), u32),
        pltpu.VMEM((7, TB // 4, D // 2), u32),
        pltpu.VMEM((7, TB // 4, FH), u32),
        pltpu.VMEM((2, TB, D), bf16),
        pltpu.VMEM((8, E), u32),
        pltpu.VMEM((2, BGR, D), bf16),
        pltpu.VMEM((1, D), bf16),
        pltpu.VMEM((M, D), bf16),
        pltpu.SemaphoreType.DMA((22,)),
    ]
    out = pl.pallas_call(
        _kernel,
        out_shape=jax.ShapeDtypeStruct((S, D), bf16),
        in_specs=[hbm] * 12,
        out_specs=hbm,
        scratch_shapes=scratch,
        compiler_params=pltpu.CompilerParams(vmem_limit_bytes=126 * 1024 * 1024,
                                             disable_bounds_checks=NO_BOUNDS),
    )(A_x.reshape(NSEG, SEG, D), A_mem0.reshape(M, D), A_Wq, A_Wk, A_Wv,
      A_Wo.reshape(H * E, D), B_w1, B_w2.reshape(2, D // 2, D), B_w3.reshape(2, D // 2, F),
      B_w4.reshape(2, FH, D), c, w_mod)
    return out.reshape(1, S, D)
```

```python
import functools

import jax
import jax.numpy as jnp
from jax import lax
import jax.experimental.pallas as pl
import jax.experimental.pallas.tpu as pltpu

bf16, f32, u32 = jnp.bfloat16, jnp.float32, jnp.uint32

S, D, H, E, M, SEG, F = 2048, 1024, 32, 128, 8, 32, 3584
NSEG = S // SEG
NP = H // 2
TC = SEG - M
HG = 8
NG = H // HG
TB = 128
NB = S // TB
FH = F // 2
NF = FH // E
G4R = 64
NI = NSEG // 2
NQ = D // E // 2
NC = 3 * NG
BGR = 384
G1R = 48
HD = D // 2
X0 = 4
NR = 2 * (M + SEG)
NO_BOUNDS = True
PIN_ROWS = 256
Y_AT = (0, 7, 14, 21)
G_AT = 2
PREP_AT = (1, 4)
SORD = 0
FINE = 1
JGROUP = 1
P1_TAIL = 5
P1_LAG = 4
LAG_S = 1
LAG_O = 3
ORDER = 2
EPS = 1e-5
SCALE = E ** -0.5
_SCOPES = False
_N2 = NSEG // 2


def _scoped(name, fn):
    def wrapped(*a):
        if not _SCOPES:
            return fn(*a)
        with jax.named_scope(name):
            return fn(*a)
    return wrapped


def _pk(x):
    return pltpu.bitcast(x.astype(bf16), u32)


def _up(x):
    return pltpu.bitcast(x, bf16)


def _ct(k):
    return slice(k * E, (k + 1) * E)


def _dot(a, b):
    return jnp.dot(a, b, preferred_element_type=f32)


def _ln(x):
    m = jnp.mean(x, axis=-1, keepdims=True)
    xc = x - m
    v = jnp.mean(xc * xc, axis=-1, keepdims=True)
    return xc * lax.rsqrt(v + EPS)


def _gelu(x):
    c = 0.7978845608028654
    return 0.5 * x * (1.0 + jnp.tanh(c * (x + 0.044715 * (x * x * x))))


def _lhs_set(a11, a12, a21, a22):
    return (a11 + a22, a21 + a22, a11, a22, a11 + a12, a21 - a11, a12 - a22)


def _rhs_set(b11, b12, b21, b22):
    return (b11 + b22, b11, b12 - b22, b21 - b11, b22, b11 + b12, b21 + b22)


def _strassen(m):
    if SORD == 0:
        m1 = m(0)
        m2 = m(1)
        c22 = m1 - m2
        m3 = m(2)
        c22 = c22 + m3
        c22 = m(5) + c22
        m4 = m(3)
        c21 = m2 + m4
        c11 = m1 + m4
        m5 = m(4)
        c12 = m3 + m5
        c11 = c11 - m5
        c11 = m(6) + c11
    else:
        m2 = m(1)
        c22 = m(5) - m2
        m4 = m(3)
        c21 = m2 + m4
        m1 = m(0)
        c22 = c22 + m1
        c11 = m4 + m1
        m3 = m(2)
        c22 = c22 + m3
        m5 = m(4)
        c12 = m3 + m5
        c11 = c11 - m5
        c11 = m(6) + c11
    return c11, c12, c21, c22


def _mask_fill():
    shape = (NR, E)
    r = lax.broadcasted_iota(jnp.int32, shape, 0)
    c = lax.broadcasted_iota(jnp.int32, shape, 1)

    def headpos(i):
        head = jnp.where(i < 64, i >> 5, (i - 64) >> 3)
        pos = jnp.where(i < 64, i & 31, 32 + (i & 7))
        return head, pos

    hr, pr = headpos(r)
    hc, pc = headpos(c)
    same = hr == hc
    valid = same & ((pr < M) | (pr >= pc))
    return jnp.where(valid, 0.0, jnp.where(same, -1e9, -jnp.inf)).astype(f32)


def _kernel(x_hbm, mem0_hbm, wq_hbm, wk_hbm, wv_hbm, wo_hbm, w1_hbm, w2_hbm, w3_hbm,
            w4_hbm, c_hbm, wm_hbm,
            out_hbm,
            x_s, xpre_s, hpre_s, wm_s, stg, w_s, wo_s,
            t1_s, g1, t2_s, t3_s, t4_s, g2, g3, g4, pre_s, mod_s, mem_s, hn_s, aout_s, fill_s,
            x2_s, hb_s, t_s, l1_s, x1_s, g_s, y_s, u_s, o_s, zero_s, bg, c_s, mem0_s, sems):
    w_hbm = (wq_hbm, wk_hbm, wv_hbm)

    (SEM_C, SEM_MEM, SEM_XPRE, SEM_X, SEM_STG, SEM_BG, SEM_OUT,
     SEM_WMR, SEM_G2, SEM_G3, SEM_G4, SEM_WM, SEM_G1) = (0, 1, 2, 3, 4, 6, 8, 10, 12, 14, 16, 18, 22)

    def copy(src, dst, k):
        return pltpu.make_async_copy(src, dst, sems.at[k])

    def w_copy(t, g, slot):
        return copy(w_hbm[t].at[:, pl.ds(pl.multiple_of(g * HG, HG), HG), :], stg.at[slot],
                    SEM_STG + slot)

    def bg_rows(k):
        return clamp(k * BGR, H * E - BGR), clamp(k * G1R, HD - G1R)

    def bg_copies(k, slot):
        ro, r1 = bg_rows(k)
        return (copy(wo_hbm.at[pl.ds(aligned(ro, 16), BGR)], bg.at[slot], SEM_BG + slot),
                copy(w1_hbm.at[:, pl.ds(aligned(r1, 16), G1R), :], g1.at[slot], SEM_G1 + slot))

    def wm_copy(src_tile, dst_tile, sem):
        return copy(wm_hbm.at[:, pl.ds(aligned(src_tile * E, E), E)], wm_s.at[dst_tile], sem)

    def wm_wait(t0, n, sem):
        copy(wm_s.at[t0:t0 + n], wm_s.at[t0:t0 + n], sem).wait()

    def aligned(x, n):
        return x if isinstance(x, int) else pl.multiple_of(x, n)

    def clamp(k, hi):
        return min(k, hi) if isinstance(k, int) else jnp.minimum(k, hi)

    def mlp_w_copies(k, slot):
        r = pl.ds(aligned(clamp(k, NI - 1) * 16, 16), 16)
        r4 = pl.ds(aligned(clamp(k, FH // G4R - 1) * G4R, 16), G4R)
        return (copy(w2_hbm.at[:, r, :], g2.at[slot], SEM_G2 + slot),
                copy(w3_hbm.at[:, r, :], g3.at[slot], SEM_G3 + slot),
                copy(w4_hbm.at[:, r4, :], g4.at[slot], SEM_G4 + slot))

    def pinned(w, job):
        if job is None:
            return w()
        z = job() & zero_s[...]
        w = w()
        return jnp.concatenate([w[0:8] | z, w[8:]], axis=0)

    def after(x, anchor):
        if anchor is None:
            return x
        z = pltpu.bitcast(pltpu.bitcast(anchor[0:8], u32) & zero_s[...], f32)
        z = jnp.concatenate([z] * (x.shape[0] // 8), axis=0)
        return jnp.concatenate([x[:, 0:E] + z, x[:, E:]], axis=1) if x.shape[1] > E else x + z

    def rhs_job(src, slot, r0, c1, c2, dst, q, row, z=None):
        blk = [src[slot, kh, r0:r0 + 16, cc * E:(cc + 1) * E].astype(f32)
               for kh in range(2) for cc in (c1, c2)]
        if z is not None:
            zf = pltpu.bitcast(jnp.concatenate([z, z], axis=0), f32)
            blk[0] = blk[0] + zf
            blk[3] = blk[3] + zf
        sets = _rhs_set(*blk)
        for n, v in enumerate(sets):
            dst.at[n][pl.ds(pl.multiple_of(row, 8), 8), _ct(q)] = _pk(v)
        out = pltpu.bitcast(sets[2], u32) | pltpu.bitcast(sets[3], u32)
        return out[0:8] | out[8:16]

    def mod_row(k):
        return mod_s[0:1, k * D:(k + 1) * D]

    def tq_place(c, n):
        if n == 1:
            return w_s.at[c], 0, None
        if n == 4:
            return w_s.at[c], D // 4, None
        if n == 6:
            return pre_s.at[c + 1], 0, 0
        k = (0, 2, 3, 5).index(n)
        return w_s.at[c + 2], (k // 2) * (D // 4), (k % 2) * (HG // 2)

    def relayout_jobs(slot, c, i):
        memo = []
        r = aligned(i * 8, 8)

        def job(j, z=None):
            if not memo:
                for d0 in (i * 16, HD + i * 16):
                    memo.append(jnp.swapaxes(pltpu.bitcast(stg[slot, pl.ds(d0, 16)], u32), 0, 1))
            blk = []
            for kh in range(2):
                u = memo[kh][j]
                if z is not None:
                    u = u | jnp.concatenate([z, z], axis=0)
                blk.append(pltpu.bitcast(u << 16, f32))
                blk.append(pltpu.bitcast(u & jnp.uint32(0xFFFF0000), f32))
            for k, v in enumerate(blk):
                w_s.at[c][pl.ds((k // 2) * (D // 4) + r, 8), _ct(2 * j + k % 2)] = _pk(v)
            for n, v in enumerate(_rhs_set(*blk)):
                if n not in (1, 4):
                    ref, r0, c0 = tq_place(c, n)
                    ref[pl.ds(r0 + r, 8), _ct(c0 + j)] = _pk(v)

        return [functools.partial(job, j) for j in range(HG // 2)]

    def repack(slot, row, i, z):
        v = pltpu.bitcast(bg[slot, 16 * i:16 * i + 16, :], u32)
        v = v | jnp.concatenate([z] * (D // E), axis=1)
        wo_s[pl.ds(pl.multiple_of(row + 8 * i, 8), 8), :] = v

    cp_c = copy(c_hbm, c_s, SEM_C)
    cp_mem = copy(mem0_hbm, mem0_s, SEM_MEM)
    cp_xpre = copy(x_hbm.at[:, TC:SEG, :], xpre_s, SEM_XPRE)
    w_copy(0, 0, 0).start()
    cp_xpre.start()
    cp_c.start()
    cp_mem.start()
    for k in range(2 * D // E):
        wm_copy(k, k, SEM_WM + k // 4).start()
    w_copy(0, 1, 1).start()

    zero_s[...] = jnp.zeros(zero_s.shape, u32)
    fill_s[...] = _mask_fill()
    aout_s[...] = jnp.zeros(aout_s.shape, f32)
    l1_s[...] = jnp.zeros(l1_s.shape, u32)
    bg[1] = jnp.zeros(bg.shape[1:], bf16)
    g1[1] = jnp.zeros(g1.shape[1:], bf16)

    w_copy(0, 0, 0).wait()

    def rl0_body(i, carry):
        for job in relayout_jobs(0, 0, i):
            job()
        return carry

    lax.fori_loop(0, D // 32, rl0_body, 0)
    w_copy(0, 2, 0).start()
    for cp in bg_copies(0, 0):
        cp.start()

    cp_xpre.wait()

    def npre_body(i, carry):
        xr = xpre_s[pl.ds(pl.multiple_of(i * 8, 8), 8)].astype(f32).reshape(64, D)
        t_s[pl.ds(pl.multiple_of(i * 64, 64), 64), :] = _ln(xr)
        return carry

    lax.fori_loop(0, NSEG // 8, _scoped("npre", npre_body), 0)

    cp_c.wait()
    cp_mem.wait()
    mem_s[...] = mem0_s[...].astype(f32)
    cf = c_s[...].astype(f32)
    sc = cf * (1.0 / (1.0 + jnp.exp(-cf)))
    sc8 = jnp.broadcast_to(sc, (8, D)).astype(bf16)

    def mod_tiles(t0, n, dst_tile):
        for k in range(n):
            mod_s[:, (dst_tile + k) * E:(dst_tile + k + 1) * E] = _dot(sc8, wm_s[t0 + k])

    for k in range(4):
        wm_wait(4 * k, 4, SEM_WM + k)
        mod_tiles(4 * k, 4, 4 * k)

    PH = NSEG * M // 2

    def hpre_body(i, carry):
        h = [t_s[pl.ds(pl.multiple_of(hf * PH + i * 16, 16), 16), :] * (1.0 + mod_row(1)) + mod_row(0)
             for hf in range(2)]
        for n, v in enumerate(_lhs_set(h[0][:, :HD], h[0][:, HD:], h[1][:, :HD], h[1][:, HD:])):
            hpre_s.at[n][pl.ds(pl.multiple_of(i * 8, 8), 8), :] = _pk(v)
        return carry

    lax.fori_loop(0, PH // 16, _scoped("hpre", hpre_body), 0)

    t_s[0:8, :] = jnp.zeros((8, D), f32)
    t_s[S + 8:S + 16, :] = jnp.zeros((8, D), f32)

    def modulate_a(xr):
        return _ln(xr) * (1.0 + mod_row(1)) + mod_row(0)

    MB = 64

    def x_copy(k):
        r = slice(0, X0) if k == 0 else slice(X0, NSEG)
        return copy(x_hbm.at[r], x_s.at[r], SEM_XPRE if k == 0 else SEM_X)


    def p1_body(c, carry):
        slot = c & 1
        pslot = 1 - slot
        ro, r1 = bg_rows(jnp.maximum(c - 1, 0))

        @pl.when(c >= 1)
        def _():
            for cp in bg_copies(0, pslot):
                cp.wait()

        @pl.when(c + 1 < NC)
        def _():
            w_copy(0, 0, pslot).wait()

        small = [functools.partial(repack, pslot, ro >> 1, i) for i in range(BGR // 16)]
        small += [functools.partial(rhs_job, g1, pslot, 16 * rt, q, NQ + q, t1_s, q, (r1 >> 1) + 8 * rt)
                  for rt in range(G1R // 16) for q in range(NQ)]
        work = []
        nu = D // 32
        for i in range(nu):
            js = relayout_jobs(pslot, c + 1, i)
            work += [js[k:k + JGROUP] for k in range(0, len(js), JGROUP)]
            work += [[job] for job in small[i * len(small) // nu:(i + 1) * len(small) // nu]]
        npin = 7 * (HG // 2) * (PH // MB)
        jobs = [[] for _ in range(npin)]
        for k, group in enumerate(work):
            pos = k * (npin - P1_TAIL) * 8 // len(work)
            jobs[pos // 8] += [(job, pos % 8 if FINE else 0) for job in group]
        jobs = iter(jobs)

        def prod(n, q, mb):
            ref, r0, c0 = tq_place(c, n)
            w = ref[r0:r0 + D // 4, _ct(2 * q + (n == 4) if c0 is None else c0 + q)]
            m = _dot(_up(hpre_s[n, mb * MB // 2:(mb + 1) * MB // 2, :]), _up(w))
            pending.append(m)
            if len(pending) > P1_LAG:
                anchor = pltpu.bitcast(pending.pop(0), u32)
                for job, g in next(jobs):
                    job(anchor[8 * g:8 * g + 8] & zero_s[...])
            return m

        pending = []
        ns = MB // M
        for q in range(HG // 2):
            for mb in range(PH // MB):
                cs = _strassen(lambda n: prod(n, q, mb))
                for hf in range(2):
                    y = jnp.concatenate([cs[2 * hf + k][sg * M:(sg + 1) * M]
                                         for sg in range(ns) for k in range(2)], axis=0)
                    s0 = hf * (NSEG // 2) + mb * ns
                    pre_s.at[c][s0 * M:(s0 + ns) * M, _ct(q)] = _pk(y)

        for t in range(3):
            @pl.when((c + 3) >> 2 == t)
            def _():
                w_copy(t, (c + 3) & 3, pslot).start()

        @pl.when(c + 2 < NC)
        def _():
            for cp in bg_copies(c + 1, pslot):
                cp.start()

        @pl.when(c < NC - 3)
        def _():
            wm_copy(2 * D // E + c, c, SEM_WMR).start()

        @pl.when(c == NC - 3)
        def _():
            def issue(k, carry2):
                wm_copy(2 * D // E + k, k, SEM_WMR).start()
                return carry2

            x_copy(0).start()
            for k in range(2):
                for cp in mlp_w_copies(k, k):
                    cp.start()
            lax.fori_loop(NC - 3, 3 * D // E, issue, 0)

        return carry

    lax.fori_loop(0, NC, _scoped("p1", p1_body), 0)
    x_copy(1).start()
    x_copy(0).wait()
    wm_wait(0, 3 * D // E, SEM_WMR)
    mod_tiles(0, 3 * D // E, 2 * D // E)
    for k in range(D // E):
        wm_copy(5 * D // E + k, k, SEM_WM).start()

    def h_rows(s):
        return modulate_a(x_s[s, 0:TC, :].astype(f32))

    hn_s[...] = h_rows(0)

    def chain_step(s, mem, htok, odef_prev, jobs=(), hooks=None):
        hs = jnp.concatenate([mem, htok], axis=0).astype(bf16)
        qkv = [[None] * 3 for _ in range(NP)]
        ps = [None] * NP
        os_ = [None] * H
        odef = [None] * H

        def proj(p, ts=(0, 1, 2)):
            for t in ts:
                c, q = t * NG + p // (HG // 2), p % (HG // 2)
                a = _dot(hs, _up(w_s[c, :, _ct(2 * q)]))
                b = _dot(hs, _up(w_s[c, :, _ct(2 * q + 1)]))
                pre = pre_s[c, pl.ds(pl.multiple_of(s * M, M), M), _ct(q)]
                if t == 1:
                    kf = jnp.concatenate([a, b, _up(pre).astype(f32), jnp.zeros((E - NR, E), f32)],
                                         axis=0)
                    qkv[p][t] = kf.T.astype(bf16)
                    continue
                parts = [_pk(a), _pk(b), pre]
                if t == 2:
                    parts.append(jnp.zeros(((E - NR) // 2, E), u32))
                qkv[p][t] = _up(jnp.concatenate(parts, axis=0))

        def scores(p):
            sc_ = _dot(qkv[p][0], qkv[p][1])
            fill = fill_s[...]
            sc_ = jnp.where(fill == 0.0, sc_ * SCALE, fill)
            m = jnp.max(sc_, axis=-1, keepdims=True)
            e = jnp.exp(sc_ - m)
            l = jnp.sum(e, axis=-1, keepdims=True)
            r = pl.reciprocal(l, approx=True)
            r = r * (2.0 - l * r)
            ps[p] = (e * r).astype(bf16)

        def fin(p):
            o = _dot(ps[p], qkv[p][2])
            for hh in range(2):
                h = 2 * p + hh
                rows = o[32 * hh:32 * hh + 32]
                odef[h] = o[64 + 8 * hh:72 + 8 * hh]
                if odef_prev is not None:
                    rows = jnp.concatenate([rows, odef_prev[h], odef[h]], axis=0)
                os_[h] = _pk(rows)

        acc = [None] * 8
        jobs = iter(jobs)

        def wo(h0, h1, js):
            lhs = _up(jnp.concatenate(os_[h0:h1], axis=1))
            for j in js:
                ws = []
                for r0 in range(h0 * E // 2, h1 * E // 2, PIN_ROWS):
                    ws.append(pinned(lambda: wo_s[r0:r0 + PIN_ROWS, j * E:(j + 1) * E],
                                     next(jobs, None)))
                part = _dot(lhs, _up(jnp.concatenate(ws, axis=0)))
                if hooks and acc[j] is None and j in hooks:
                    hooks[j](part)
                acc[j] = part if acc[j] is None else part + acc[j]

        for p in range(NP):
            if ORDER == 0:
                proj(p)
                if p >= LAG_S:
                    scores(p - LAG_S)
                if p >= LAG_O:
                    fin(p - LAG_O)
            elif ORDER == 1:
                proj(p, (1, 0))
                if p >= LAG_O:
                    fin(p - LAG_O)
                proj(p, (2,))
                if p >= LAG_S:
                    scores(p - LAG_S)
            elif ORDER == 2:
                proj(p, (1,))
                if p >= LAG_S:
                    scores(p - LAG_S)
                proj(p, (0,))
                if p >= LAG_O:
                    fin(p - LAG_O)
                proj(p, (2,))
            else:
                proj(p, (1, 0, 2))
                if p >= LAG_O:
                    fin(p - LAG_O)
                if p >= LAG_S:
                    scores(p - LAG_S)
        tail = []
        for k in range(LAG_O):
            step = []
            if NP - LAG_S + k < NP:
                step.append(functools.partial(scores, NP - LAG_S + k))
            step.append(functools.partial(fin, NP - LAG_O + k))
            tail.append(step)
        hsplit = min(24, 2 * (NP - LAG_O))
        cuts = {3: (2, 3, 5), 2: (2, 5), 4: (1, 2, 4, 6), 5: (1, 2, 3, 4, 6)}[LAG_O]
        j0 = 0
        for k, step in enumerate(tail):
            wo(0, hsplit, range(j0, cuts[k]))
            j0 = cuts[k]
            for f in step:
                f()
        wo(0, hsplit, range(j0, 8))
        wo(hsplit, H, range(8))
        return jnp.concatenate(acc, axis=1), odef

    def mixer_prep(i, k=0, n=SEG, anchor=None):
        ys = []
        for hf in range(2):
            r0 = hf * SEG + k * n
            r = pl.ds(aligned(i * 64 + r0, 16), n)
            xr = x_s[2 * i + hf, k * n:(k + 1) * n, :].astype(f32)
            x2 = xr + mod_row(2) * after(aout_s[r0:r0 + n, :], anchor)
            x2_s[r, :] = x2.astype(bf16)
            hb = _ln(x2) * (1.0 + mod_row(4)) + mod_row(3)
            hb_s[r, :] = hb.astype(bf16)
            ys.append(_ln(hb))
        sets = _lhs_set(ys[0][:, :HD], ys[0][:, HD:], ys[1][:, :HD], ys[1][:, HD:])
        for m, v in enumerate(sets):
            l1_s.at[m][k * n // 2:(k + 1) * n // 2, :] = _pk(v)
        return sets[0][0:8, 0:E] + sets[0][8:16, 0:E]

    def mixer_mm(i):
        for q in range(NQ):
            cs = _strassen(lambda n: _dot(_up(l1_s[n]), _up(t1_s[n, :, _ct(q)])))
            for k, cc in enumerate(cs):
                r0 = aligned(i * 64 + 8 + (k // 2) * SEG, 8)
                t_s[pl.ds(r0, SEG), _ct(q + NQ * (k % 2))] = _gelu(cc)

    def p2_body(i, carry):
        slot = i & 1
        for cp in mlp_w_copies(0, slot):
            cp.wait()

        @pl.when(i == 1)
        def _():
            x_copy(1).wait()

        work = [functools.partial(rhs_job, g3, slot, 0, q, NF + q, t3_s, q, i * 8)
                for q in range(NF)]
        work += [functools.partial(rhs_job, g2, slot, 0, q, NQ + q, t2_s, q, i * 8)
                 for q in range(NQ)]
        row4 = clamp(i, FH // G4R - 1) * (G4R // 2)
        work += [functools.partial(rhs_job, g4, slot, 16 * rt, q, NQ + q, t4_s, q, row4 + 8 * rt)
                 for rt in range(G4R // 16) for q in range(NQ)]
        npin = 60
        jobs = [None] * npin
        for k, job in enumerate(work):
            jobs[1 + k * (npin - 1) // len(work)] = job

        sa_ = 2 * i
        sb_ = 2 * i + 1
        hb_tok = h_rows(sb_)
        oa, odef_a = chain_step(sa_, mem_s[...], hn_s[...], None)
        mixer_mm(jnp.maximum(i - 2, 0))
        prev = [None]

        def hook(k, anchor):
            if k > 0:
                anchor = anchor[0:8] + prev[0]
            prev[0] = mixer_prep(jnp.maximum(i - 1, 0), k, 16, anchor)

        hooks = {j: functools.partial(hook, k) for k, j in enumerate(PREP_AT)}
        ob, _ = chain_step(sb_, oa[0:M], hb_tok, odef_a, jobs, hooks)
        mem_s[...] = ob[0:M]
        aout_s[0:TC, :] = oa[M:SEG]
        aout_s[TC:SEG, :] = ob[SEG:SEG + M]
        aout_s[SEG:SEG + TC, :] = ob[M:SEG]
        aout_s[SEG + TC:2 * SEG, :] = ob[SEG + M:SEG + 2 * M]
        hn_s[...] = h_rows(jnp.minimum(sb_ + 1, NSEG - 1))
        for cp in mlp_w_copies(i + 2, slot):
            cp.start()
        return carry

    lax.fori_loop(0, _N2, _scoped("p2", p2_body), 0)

    TH = TB // 2
    SHIFT = (-1, -1, 1, 1, -2, -2, 2, 2)

    def g_job(j, rt, q, n=16, anchor=None):
        blk = []
        for hf in range(2):
            for ct in (q, NQ + q):
                win = t_s[pl.ds(aligned(j * TB + hf * TH + rt * n, 16), n + 16), ct * E:(ct + 1) * E]
                blk.append(win[8 + SHIFT[ct]:8 + SHIFT[ct] + n])
        blk[0] = after(blk[0], anchor)
        blk[3] = after(blk[3], anchor)
        for k, v in enumerate(_lhs_set(*blk)):
            g_s.at[k][rt * n // 2:(rt + 1) * n // 2, q * E:(q + 1) * E] = _pk(v)

    def mix(j):
        r0 = aligned(j * TB, TB)
        for q in range(NQ):
            cs = _strassen(lambda n: _dot(_up(g_s[n]), _up(t2_s[n, :, _ct(q)])))
            for k, cc in enumerate(cs):
                rr = pl.ds(r0 + (k // 2) * TH, TH)
                c0 = (q + NQ * (k % 2)) * E
                x1 = hb_s[rr, c0:c0 + E].astype(f32) + cc
                x1_s[(k // 2) * TH:(k // 2 + 1) * TH, c0:c0 + E] = x1
                hb_s[rr, c0:c0 + E] = x1.astype(bf16)

    def out_copy(j, slot):
        return copy(o_s.at[slot], out_hbm.at[pl.ds(aligned(j * TB, TB), TB)], SEM_OUT + slot)

    prev_y = [None]

    def put_y(rt=0, n=TH, anchor=None):
        if anchor is not None and rt > 0:
            anchor = anchor[0:8] + prev_y[0]
        ya = _ln(after(x1_s[rt * n:(rt + 1) * n, :], anchor))
        yb = _ln(after(x1_s[TH + rt * n:TH + (rt + 1) * n, :], anchor))
        sets = _lhs_set(ya[:, :HD], ya[:, HD:], yb[:, :HD], yb[:, HD:])
        prev_y[0] = sets[0][0:8, 0:E] + sets[0][8:16, 0:E]
        for k, v in enumerate(sets):
            y_s.at[k][rt * n // 2:(rt + 1) * n // 2, :] = _pk(v)

    wm_wait(0, D // E, SEM_WM)
    mod_tiles(0, D // E, 5 * D // E)
    mixer_mm(NI - 2)
    mixer_prep(NI - 1)
    for q in range(NQ):
        g_job(0, 0, q, TH)
    mix(0)
    mixer_mm(NI - 1)
    put_y()
    for q in range(NQ):
        g_job(1, 0, q, TH)

    def mlp_block(j, last):
        slot = j & 1
        r0 = aligned(j * TB, TB)
        for q in range(NF):
            cs = _strassen(lambda n: _dot(_up(y_s[n]), _up(t3_s[n, :, _ct(q)])))
            for n, v in enumerate(_lhs_set(*[_gelu(cc) for cc in cs])):
                u_s.at[n][:, q * E:(q + 1) * E] = _pk(v)
        jobs = {}
        if not last:
            mix(j + 1)
            jn = clamp(j + 2, NB - 1)
            for rt in range(TH // 16):
                jobs[Y_AT[rt]] = functools.partial(put_y, rt, 16)
            free = [k for k in range(G_AT, 7 * NQ) if k not in jobs]
            for k in range(TH // 16 * NQ):
                jobs[free[k]] = functools.partial(g_job, jn, k // NQ, k % NQ, 16)

        def prod(n, q):
            m = _dot(_up(u_s[n]), _up(t4_s[n, :, _ct(q)]))
            job = jobs.get(count[0])
            count[0] += 1
            if job is not None:
                job(anchor=m)
            return m

        count = [0]
        for q in range(NQ):
            if last and q == 0:
                ks = FH - 2 * E
                head = [_dot(_up(u_s[n, :, 0:ks]), _up(t4_s[n, 0:ks // 2, _ct(q)])) for n in range(7)]
                cs = _strassen(lambda n: _dot(_up(u_s[n, :, ks:FH]), _up(t4_s[n, ks // 2:, _ct(q)]))
                               + head[n])
            else:
                cs = _strassen(lambda n: prod(n, q))
            for k, cc in enumerate(cs):
                rr = pl.ds(r0 + (k // 2) * TH, TH)
                c0 = (q + NQ * (k % 2)) * E
                gb = mod_s[0:1, 5 * D + c0:5 * D + c0 + E]
                o_s[slot, (k // 2) * TH:(k // 2 + 1) * TH, c0:c0 + E] = (
                    x2_s[rr, c0:c0 + E].astype(f32)
                    + gb * (hb_s[rr, c0:c0 + E].astype(f32) + cc)).astype(bf16)
        out_copy(j, slot).start()

    def p3_body(j, carry):
        @pl.when(j >= 2)
        def _():
            out_copy(j - 2, j & 1).wait()

        mlp_block(j, False)
        return carry

    lax.fori_loop(0, NB - 1, _scoped("p3", p3_body), 0)
    for k in range(2):
        for cp in mlp_w_copies(0, k):
            cp.wait()
    out_copy(NB - 3, (NB - 3) % 2).wait()
    mlp_block(NB - 1, True)
    out_copy(NB - 2, (NB - 2) % 2).wait()
    out_copy(NB - 1, (NB - 1) % 2).wait()


@jax.jit
def pallas_adaLN_cond__memory_aug_recurrent_mem_tr__mixer_s_mlp__prompt_kernel(
    A_x: jax.Array,
    A_mem0: jax.Array,
    A_Wq: jax.Array,
    A_Wk: jax.Array,
    A_Wv: jax.Array,
    A_Wo: jax.Array,
    A_seg_len,
    B_x: jax.Array,
    B_w1: jax.Array,
    B_w2: jax.Array,
    B_w3: jax.Array,
    B_w4: jax.Array,
    c: jax.Array,
    w_mod: jax.Array,
):
    del A_seg_len, B_x
    assert A_x.shape == (1, S, D) and A_mem0.shape == (1, M, D)
    hbm = pl.BlockSpec(memory_space=pl.ANY)
    scratch = [
        pltpu.VMEM((NSEG, SEG, D), bf16),
        pltpu.VMEM((NSEG, M, D), bf16),
        pltpu.VMEM((7, NSEG * M // 4, D // 2), u32),
        pltpu.VMEM((3 * D // E, D, E), bf16),
        pltpu.VMEM((2, D, HG, E), bf16),
        pltpu.VMEM((NC + 3, D // 2, HG * E), u32),
        pltpu.VMEM((H * E // 2, D), u32),
        pltpu.VMEM((7, D // 4, D // 2), u32),
        pltpu.VMEM((2, 2, G1R, D), bf16),
        pltpu.VMEM((7, D // 4, D // 2), u32),
        pltpu.VMEM((7, D // 4, FH), u32),
        pltpu.VMEM((7, FH // 2, D // 2), u32),
        pltpu.VMEM((2, 2, 16, D), bf16),
        pltpu.VMEM((2, 2, 16, F), bf16),
        pltpu.VMEM((2, 2, G4R, D), bf16),
        pltpu.VMEM((NC + 2, NSEG * M, HG // 2 * E), u32),
        pltpu.VMEM((8, 6 * D), f32),
        pltpu.VMEM((M, D), f32),
        pltpu.VMEM((TC, D), f32),
        pltpu.VMEM((2 * SEG, D), f32),
        pltpu.VMEM((NR, E), f32),
        pltpu.VMEM((S, D), bf16),
        pltpu.VMEM((S, D), bf16),
        pltpu.VMEM((S + 16, D), f32),
        pltpu.VMEM((7, SEG // 2, D // 2), u32),
        pltpu.VMEM((TB, D), f32),
        pltpu.VMEM((7, TB // 4, D // 2), u32),
        pltpu.VMEM((7, TB // 4, D // 2), u32),
        pltpu.VMEM((7, TB // 4, FH), u32),
        pltpu.VMEM((2, TB, D), bf16),
        pltpu.VMEM((8, E), u32),
        pltpu.VMEM((2, BGR, D), bf16),
        pltpu.VMEM((1, D), bf16),
        pltpu.VMEM((M, D), bf16),
        pltpu.SemaphoreType.DMA((24,)),
    ]
    out = pl.pallas_call(
        _kernel,
        out_shape=jax.ShapeDtypeStruct((S, D), bf16),
        in_specs=[hbm] * 12,
        out_specs=hbm,
        scratch_shapes=scratch,
        compiler_params=pltpu.CompilerParams(vmem_limit_bytes=126 * 1024 * 1024,
                                             disable_bounds_checks=NO_BOUNDS),
    )(A_x.reshape(NSEG, SEG, D), A_mem0.reshape(M, D), A_Wq, A_Wk, A_Wv,
      A_Wo.reshape(H * E, D), B_w1.reshape(2, D // 2, D), B_w2.reshape(2, D // 2, D), B_w3.reshape(2, D // 2, F),
      B_w4.reshape(2, FH, D), c, w_mod)
    return out.reshape(1, S, D)
```

```python
import functools

import jax
import jax.numpy as jnp
from jax import lax
import jax.experimental.pallas as pl
import jax.experimental.pallas.tpu as pltpu

bf16, f32, u32 = jnp.bfloat16, jnp.float32, jnp.uint32

S, D, H, E, M, SEG, F = 2048, 1024, 32, 128, 8, 32, 3584
NSEG = S // SEG
NP = H // 2
TC = SEG - M
HG = 8
NG = H // HG
TB = 128
NB = S // TB
FH = F // 2
NF = FH // E
G4R = 64
NI = NSEG // 2
NQ = D // E // 2
NC = 3 * NG
BGR = 384
G1R = 48
HD = D // 2
X0 = 4
NR = 2 * (M + SEG)
NO_BOUNDS = True
PIN_ROWS = 256
Y_AT = (0, 7, 14, 21)
G_AT = 2
PREP_AT = (0, 1, 3, 4)
PREP_CH = 2
SORD = 0
FINE = 1
JGROUP = 1
P1_TAIL = 5
P1_LAG = 4
LAG_S = 1
LAG_O = 3
ORDER = 2
EPS = 1e-5
SCALE = E ** -0.5
_SCOPES = False
_N2 = NSEG // 2


def _scoped(name, fn):
    def wrapped(*a):
        if not _SCOPES:
            return fn(*a)
        with jax.named_scope(name):
            return fn(*a)
    return wrapped


def _pk(x):
    return pltpu.bitcast(x.astype(bf16), u32)


def _up(x):
    return pltpu.bitcast(x, bf16)


def _ct(k):
    return slice(k * E, (k + 1) * E)


def _dot(a, b):
    return jnp.dot(a, b, preferred_element_type=f32)


def _ln(x):
    m = jnp.mean(x, axis=-1, keepdims=True)
    xc = x - m
    v = jnp.mean(xc * xc, axis=-1, keepdims=True)
    return xc * lax.rsqrt(v + EPS)


def _gelu(x):
    c = 0.7978845608028654
    return 0.5 * x * (1.0 + jnp.tanh(c * (x + 0.044715 * (x * x * x))))


def _lhs_set(a11, a12, a21, a22):
    return (a11 + a22, a21 + a22, a11, a22, a11 + a12, a21 - a11, a12 - a22)


def _rhs_set(b11, b12, b21, b22):
    return (b11 + b22, b11, b12 - b22, b21 - b11, b22, b11 + b12, b21 + b22)


def _strassen(m):
    if SORD == 0:
        m1 = m(0)
        m2 = m(1)
        c22 = m1 - m2
        m3 = m(2)
        c22 = c22 + m3
        c22 = m(5) + c22
        m4 = m(3)
        c21 = m2 + m4
        c11 = m1 + m4
        m5 = m(4)
        c12 = m3 + m5
        c11 = c11 - m5
        c11 = m(6) + c11
    else:
        m2 = m(1)
        c22 = m(5) - m2
        m4 = m(3)
        c21 = m2 + m4
        m1 = m(0)
        c22 = c22 + m1
        c11 = m4 + m1
        m3 = m(2)
        c22 = c22 + m3
        m5 = m(4)
        c12 = m3 + m5
        c11 = c11 - m5
        c11 = m(6) + c11
    return c11, c12, c21, c22


def _mask_fill():
    shape = (NR, E)
    r = lax.broadcasted_iota(jnp.int32, shape, 0)
    c = lax.broadcasted_iota(jnp.int32, shape, 1)

    def headpos(i):
        head = jnp.where(i < 64, i >> 5, (i - 64) >> 3)
        pos = jnp.where(i < 64, i & 31, 32 + (i & 7))
        return head, pos

    hr, pr = headpos(r)
    hc, pc = headpos(c)
    same = hr == hc
    valid = same & ((pr < M) | (pr >= pc))
    return jnp.where(valid, 0.0, jnp.where(same, -1e9, -jnp.inf)).astype(f32)


def _kernel(x_hbm, mem0_hbm, wq_hbm, wk_hbm, wv_hbm, wo_hbm, w1_hbm, w2_hbm, w3_hbm,
            w4_hbm, c_hbm, wm_hbm,
            out_hbm,
            x_s, xpre_s, hpre_s, wm_s, stg, w_s, wo_s,
            t1_s, g1, t2_s, t3_s, t4_s, g2, g3, g4, pre_s, mod_s, mem_s, hn_s, aout_s, fill_s,
            x2_s, hb_s, t_s, l1_s, x1_s, g_s, y_s, u_s, o_s, zero_s, bg, c_s, mem0_s, sems):
    w_hbm = (wq_hbm, wk_hbm, wv_hbm)

    (SEM_C, SEM_MEM, SEM_XPRE, SEM_X, SEM_STG, SEM_BG, SEM_OUT,
     SEM_WMR, SEM_G2, SEM_G3, SEM_G4, SEM_WM, SEM_G1) = (0, 1, 2, 3, 4, 6, 8, 10, 12, 14, 16, 18, 22)

    def copy(src, dst, k):
        return pltpu.make_async_copy(src, dst, sems.at[k])

    def w_copy(t, g, slot):
        return copy(w_hbm[t].at[:, pl.ds(pl.multiple_of(g * HG, HG), HG), :], stg.at[slot],
                    SEM_STG + slot)

    def bg_rows(k):
        return clamp(k * BGR, H * E - BGR), clamp(k * G1R, HD - G1R)

    def bg_copies(k, slot):
        ro, r1 = bg_rows(k)
        return (copy(wo_hbm.at[pl.ds(aligned(ro, 16), BGR)], bg.at[slot], SEM_BG + slot),
                copy(w1_hbm.at[:, pl.ds(aligned(r1, 16), G1R), :], g1.at[slot], SEM_G1 + slot))

    def wm_copy(src_tile, dst_tile, sem):
        return copy(wm_hbm.at[:, pl.ds(aligned(src_tile * E, E), E)], wm_s.at[dst_tile], sem)

    def wm_wait(t0, n, sem):
        copy(wm_s.at[t0:t0 + n], wm_s.at[t0:t0 + n], sem).wait()

    def aligned(x, n):
        return x if isinstance(x, int) else pl.multiple_of(x, n)

    def clamp(k, hi):
        return min(k, hi) if isinstance(k, int) else jnp.minimum(k, hi)

    def mlp_w_copies(k, slot):
        r = pl.ds(aligned(clamp(k, NI - 1) * 16, 16), 16)
        r4 = pl.ds(aligned(clamp(k, FH // G4R - 1) * G4R, 16), G4R)
        return (copy(w2_hbm.at[:, r, :], g2.at[slot], SEM_G2 + slot),
                copy(w3_hbm.at[:, r, :], g3.at[slot], SEM_G3 + slot),
                copy(w4_hbm.at[:, r4, :], g4.at[slot], SEM_G4 + slot))

    def pinned(w, job):
        if job is None:
            return w()
        z = job() & zero_s[...]
        w = w()
        return jnp.concatenate([w[0:8] | z, w[8:]], axis=0)

    def after(x, anchor):
        if anchor is None:
            return x
        z = pltpu.bitcast(pltpu.bitcast(anchor[0:8], u32) & zero_s[...], f32)
        z = jnp.concatenate([z] * (x.shape[0] // 8), axis=0)
        return jnp.concatenate([x[:, 0:E] + z, x[:, E:]], axis=1) if x.shape[1] > E else x + z

    def rhs_job(src, slot, r0, c1, c2, dst, q, row, z=None):
        blk = [src[slot, kh, r0:r0 + 16, cc * E:(cc + 1) * E].astype(f32)
               for kh in range(2) for cc in (c1, c2)]
        if z is not None:
            zf = pltpu.bitcast(jnp.concatenate([z, z], axis=0), f32)
            blk[0] = blk[0] + zf
            blk[3] = blk[3] + zf
        sets = _rhs_set(*blk)
        for n, v in enumerate(sets):
            dst.at[n][pl.ds(pl.multiple_of(row, 8), 8), _ct(q)] = _pk(v)
        out = pltpu.bitcast(sets[2], u32) | pltpu.bitcast(sets[3], u32)
        return out[0:8] | out[8:16]

    def mod_rows(k, n, c0=0, w=D):
        return jnp.concatenate([mod_s[:, k * D + c0:k * D + c0 + w]] * (n // 8), axis=0)

    def tq_place(c, n):
        if n == 1:
            return w_s.at[c], 0, None
        if n == 4:
            return w_s.at[c], D // 4, None
        if n == 6:
            return pre_s.at[c + 1], 0, 0
        k = (0, 2, 3, 5).index(n)
        return w_s.at[c + 2], (k // 2) * (D // 4), (k % 2) * (HG // 2)

    def relayout_jobs(slot, c, i):
        memo = []
        r = aligned(i * 8, 8)

        def job(j, z=None):
            if not memo:
                for d0 in (i * 16, HD + i * 16):
                    memo.append(jnp.swapaxes(pltpu.bitcast(stg[slot, pl.ds(d0, 16)], u32), 0, 1))
            blk = []
            for kh in range(2):
                u = memo[kh][j]
                if z is not None:
                    u = u | jnp.concatenate([z, z], axis=0)
                blk.append(pltpu.bitcast(u << 16, f32))
                blk.append(pltpu.bitcast(u & jnp.uint32(0xFFFF0000), f32))
            for k, v in enumerate(blk):
                w_s.at[c][pl.ds((k // 2) * (D // 4) + r, 8), _ct(2 * j + k % 2)] = _pk(v)
            for n, v in enumerate(_rhs_set(*blk)):
                if n not in (1, 4):
                    ref, r0, c0 = tq_place(c, n)
                    ref[pl.ds(r0 + r, 8), _ct(c0 + j)] = _pk(v)

        return [functools.partial(job, j) for j in range(HG // 2)]

    def repack(slot, row, i, z):
        v = pltpu.bitcast(bg[slot, 16 * i:16 * i + 16, :], u32)
        v = v | jnp.concatenate([z] * (D // E), axis=1)
        wo_s[pl.ds(pl.multiple_of(row + 8 * i, 8), 8), :] = v

    cp_c = copy(c_hbm, c_s, SEM_C)
    cp_mem = copy(mem0_hbm, mem0_s, SEM_MEM)
    cp_xpre = copy(x_hbm.at[:, TC:SEG, :], xpre_s, SEM_XPRE)
    w_copy(0, 0, 0).start()
    cp_xpre.start()
    cp_c.start()
    cp_mem.start()
    for k in range(2 * D // E):
        wm_copy(k, k, SEM_WM + k // 4).start()
    w_copy(0, 1, 1).start()

    zero_s[...] = jnp.zeros(zero_s.shape, u32)
    fill_s[...] = _mask_fill()
    aout_s[...] = jnp.zeros(aout_s.shape, f32)
    l1_s[...] = jnp.zeros(l1_s.shape, u32)
    bg[1] = jnp.zeros(bg.shape[1:], bf16)
    g1[1] = jnp.zeros(g1.shape[1:], bf16)

    w_copy(0, 0, 0).wait()

    def rl0_body(i, carry):
        for job in relayout_jobs(0, 0, i):
            job()
        return carry

    lax.fori_loop(0, D // 32, rl0_body, 0)
    w_copy(0, 2, 0).start()
    for cp in bg_copies(0, 0):
        cp.start()

    cp_xpre.wait()

    def npre_body(i, carry):
        xr = xpre_s[pl.ds(pl.multiple_of(i * 8, 8), 8)].astype(f32).reshape(64, D)
        t_s[pl.ds(pl.multiple_of(i * 64, 64), 64), :] = _ln(xr)
        return carry

    lax.fori_loop(0, NSEG // 8, _scoped("npre", npre_body), 0)

    cp_c.wait()
    cp_mem.wait()
    mem_s[...] = mem0_s[...].astype(f32)
    cf = c_s[...].astype(f32)
    sc = cf * (1.0 / (1.0 + jnp.exp(-cf)))
    sc8 = jnp.broadcast_to(sc, (8, D)).astype(bf16)

    def mod_tiles(t0, n, dst_tile):
        for k in range(n):
            v = _dot(sc8, wm_s[t0 + k])
            if (dst_tile + k) // (D // E) in (1, 4):
                v = 1.0 + v
            mod_s[:, _ct(dst_tile + k)] = v

    for k in range(4):
        wm_wait(4 * k, 4, SEM_WM + k)
        mod_tiles(4 * k, 4, 4 * k)

    PH = NSEG * M // 2

    def hpre_body(i, carry):
        h = [t_s[pl.ds(pl.multiple_of(hf * PH + i * 16, 16), 16), :] * mod_rows(1, 16) + mod_rows(0, 16)
             for hf in range(2)]
        for n, v in enumerate(_lhs_set(h[0][:, :HD], h[0][:, HD:], h[1][:, :HD], h[1][:, HD:])):
            hpre_s.at[n][pl.ds(pl.multiple_of(i * 8, 8), 8), :] = _pk(v)
        return carry

    lax.fori_loop(0, PH // 16, _scoped("hpre", hpre_body), 0)

    t_s[0:8, :] = jnp.zeros((8, D), f32)
    t_s[S + 8:S + 16, :] = jnp.zeros((8, D), f32)

    def modulate_a(xr):
        return _ln(xr) * mod_rows(1, xr.shape[0]) + mod_rows(0, xr.shape[0])

    MB = 64

    def x_copy(k):
        r = slice(0, X0) if k == 0 else slice(X0, NSEG)
        return copy(x_hbm.at[r], x_s.at[r], SEM_XPRE if k == 0 else SEM_X)


    def p1_body(c, carry):
        slot = c & 1
        pslot = 1 - slot
        ro, r1 = bg_rows(jnp.maximum(c - 1, 0))

        @pl.when(c >= 1)
        def _():
            for cp in bg_copies(0, pslot):
                cp.wait()

        @pl.when(c + 1 < NC)
        def _():
            w_copy(0, 0, pslot).wait()

        small = [functools.partial(repack, pslot, ro >> 1, i) for i in range(BGR // 16)]
        small += [functools.partial(rhs_job, g1, pslot, 16 * rt, q, NQ + q, t1_s, q, (r1 >> 1) + 8 * rt)
                  for rt in range(G1R // 16) for q in range(NQ)]
        work = []
        nu = D // 32
        for i in range(nu):
            js = relayout_jobs(pslot, c + 1, i)
            work += [js[k:k + JGROUP] for k in range(0, len(js), JGROUP)]
            work += [[job] for job in small[i * len(small) // nu:(i + 1) * len(small) // nu]]
        npin = 7 * (HG // 2) * (PH // MB)
        jobs = [[] for _ in range(npin)]
        for k, group in enumerate(work):
            pos = k * (npin - P1_TAIL) * 8 // len(work)
            jobs[pos // 8] += [(job, pos % 8 if FINE else 0) for job in group]
        jobs = iter(jobs)

        def prod(n, q, mb):
            ref, r0, c0 = tq_place(c, n)
            w = ref[r0:r0 + D // 4, _ct(2 * q + (n == 4) if c0 is None else c0 + q)]
            m = _dot(_up(hpre_s[n, mb * MB // 2:(mb + 1) * MB // 2, :]), _up(w))
            pending.append(m)
            if len(pending) > P1_LAG:
                anchor = pltpu.bitcast(pending.pop(0), u32)
                for job, g in next(jobs):
                    job(anchor[8 * g:8 * g + 8] & zero_s[...])
            return m

        pending = []
        ns = MB // M
        for q in range(HG // 2):
            for mb in range(PH // MB):
                cs = _strassen(lambda n: prod(n, q, mb))
                for hf in range(2):
                    y = jnp.concatenate([cs[2 * hf + k][sg * M:(sg + 1) * M]
                                         for sg in range(ns) for k in range(2)], axis=0)
                    s0 = hf * (NSEG // 2) + mb * ns
                    pre_s.at[c][s0 * M:(s0 + ns) * M, _ct(q)] = _pk(y)

        for t in range(3):
            @pl.when((c + 3) >> 2 == t)
            def _():
                w_copy(t, (c + 3) & 3, pslot).start()

        @pl.when(c + 2 < NC)
        def _():
            for cp in bg_copies(c + 1, pslot):
                cp.start()

        @pl.when(c < NC - 3)
        def _():
            wm_copy(2 * D // E + c, c, SEM_WMR).start()

        @pl.when(c == NC - 3)
        def _():
            def issue(k, carry2):
                wm_copy(2 * D // E + k, k, SEM_WMR).start()
                return carry2

            x_copy(0).start()
            for k in range(2):
                for cp in mlp_w_copies(k, k):
                    cp.start()
            lax.fori_loop(NC - 3, 3 * D // E, issue, 0)

        return carry

    lax.fori_loop(0, NC, _scoped("p1", p1_body), 0)
    x_copy(1).start()
    x_copy(0).wait()
    wm_wait(0, 3 * D // E, SEM_WMR)
    mod_tiles(0, 3 * D // E, 2 * D // E)
    for k in range(D // E):
        wm_copy(5 * D // E + k, k, SEM_WM).start()

    def h_rows(s):
        return modulate_a(x_s[s, 0:TC, :].astype(f32))

    hn_s[...] = h_rows(0)

    def chain_step(s, mem, htok, odef_prev, jobs=(), hooks=None):
        hs = jnp.concatenate([mem, htok], axis=0).astype(bf16)
        qkv = [[None] * 3 for _ in range(NP)]
        ps = [None] * NP
        os_ = [None] * H
        odef = [None] * H

        def proj(p, ts=(0, 1, 2)):
            for t in ts:
                c, q = t * NG + p // (HG // 2), p % (HG // 2)
                a = _dot(hs, _up(w_s[c, :, _ct(2 * q)]))
                b = _dot(hs, _up(w_s[c, :, _ct(2 * q + 1)]))
                if hooks and t == 2 and p - NP in hooks:
                    hooks[p - NP](b)
                pre = pre_s[c, pl.ds(pl.multiple_of(s * M, M), M), _ct(q)]
                if t == 1:
                    kf = jnp.concatenate([a, b, _up(pre).astype(f32), jnp.zeros((E - NR, E), f32)],
                                         axis=0)
                    qkv[p][t] = kf.T.astype(bf16)
                    continue
                parts = [_pk(a), _pk(b), pre]
                if t == 2:
                    parts.append(jnp.zeros(((E - NR) // 2, E), u32))
                qkv[p][t] = _up(jnp.concatenate(parts, axis=0))

        def scores(p):
            sc_ = _dot(qkv[p][0], qkv[p][1])
            fill = fill_s[...]
            sc_ = jnp.where(fill == 0.0, sc_ * SCALE, fill)
            m = jnp.max(sc_, axis=-1, keepdims=True)
            e = jnp.exp(sc_ - m)
            l = jnp.sum(e, axis=-1, keepdims=True)
            r = pl.reciprocal(l, approx=True)
            r = r * (2.0 - l * r)
            ps[p] = (e * r).astype(bf16)

        def fin(p):
            o = _dot(ps[p], qkv[p][2])
            for hh in range(2):
                h = 2 * p + hh
                rows = o[32 * hh:32 * hh + 32]
                odef[h] = o[64 + 8 * hh:72 + 8 * hh]
                if odef_prev is not None:
                    rows = jnp.concatenate([rows, odef_prev[h], odef[h]], axis=0)
                os_[h] = _pk(rows)

        acc = [None] * 8
        jobs = iter(jobs)

        def wo(h0, h1, js):
            lhs = _up(jnp.concatenate(os_[h0:h1], axis=1))
            for j in js:
                ws = []
                for r0 in range(h0 * E // 2, h1 * E // 2, PIN_ROWS):
                    ws.append(pinned(lambda: wo_s[r0:r0 + PIN_ROWS, j * E:(j + 1) * E],
                                     next(jobs, None)))
                part = _dot(lhs, _up(jnp.concatenate(ws, axis=0)))
                if hooks and acc[j] is None and j in hooks:
                    hooks[j](part)
                acc[j] = part if acc[j] is None else part + acc[j]

        for p in range(NP):
            if ORDER == 0:
                proj(p)
                if p >= LAG_S:
                    scores(p - LAG_S)
                if p >= LAG_O:
                    fin(p - LAG_O)
            elif ORDER == 1:
                proj(p, (1, 0))
                if p >= LAG_O:
                    fin(p - LAG_O)
                proj(p, (2,))
                if p >= LAG_S:
                    scores(p - LAG_S)
            elif ORDER == 2:
                proj(p, (1,))
                if p >= LAG_S:
                    scores(p - LAG_S)
                proj(p, (0,))
                if p >= LAG_O:
                    fin(p - LAG_O)
                proj(p, (2,))
            else:
                proj(p, (1, 0, 2))
                if p >= LAG_O:
                    fin(p - LAG_O)
                if p >= LAG_S:
                    scores(p - LAG_S)
        tail = []
        for k in range(LAG_O):
            step = []
            if NP - LAG_S + k < NP:
                step.append(functools.partial(scores, NP - LAG_S + k))
            step.append(functools.partial(fin, NP - LAG_O + k))
            tail.append(step)
        hsplit = min(24, 2 * (NP - LAG_O))
        cuts = {3: (2, 3, 5), 2: (2, 5), 4: (1, 2, 4, 6), 5: (1, 2, 3, 4, 6)}[LAG_O]
        j0 = 0
        for k, step in enumerate(tail):
            wo(0, hsplit, range(j0, cuts[k]))
            j0 = cuts[k]
            for f in step:
                f()
        wo(0, hsplit, range(j0, 8))
        wo(hsplit, H, range(8))
        return jnp.concatenate(acc, axis=1), odef

    def mixer_prep(i, r0, n, anchor=None):
        r = pl.ds(aligned(i * 64 + r0, 16), n)
        xr = x_s[2 * i + r0 // SEG, r0 % SEG:r0 % SEG + n, :].astype(f32)
        x2 = xr + mod_rows(2, n) * after(aout_s[r0:r0 + n, :], anchor)
        x2_s[r, :] = x2.astype(bf16)
        hb = _ln(x2) * mod_rows(4, n) + mod_rows(3, n)
        hb_s[r, :] = hb.astype(bf16)
        return _ln(hb)

    def mixer_sets(ya, yb, r0):
        n = ya.shape[0]
        for m, v in enumerate(_lhs_set(ya[:, :HD], ya[:, HD:], yb[:, :HD], yb[:, HD:])):
            l1_s.at[m][r0 // 2:(r0 + n) // 2, :] = _pk(v)

    def mixer_mm(i):
        for q in range(NQ):
            cs = _strassen(lambda n: _dot(_up(l1_s[n]), _up(t1_s[n, :, _ct(q)])))
            for k, cc in enumerate(cs):
                r0 = aligned(i * 64 + 8 + (k // 2) * SEG, 8)
                t_s[pl.ds(r0, SEG), _ct(q + NQ * (k % 2))] = _gelu(cc)

    def p2_body(i, carry):
        slot = i & 1
        for cp in mlp_w_copies(0, slot):
            cp.wait()

        @pl.when(i == 1)
        def _():
            x_copy(1).wait()

        work = [functools.partial(rhs_job, g3, slot, 0, q, NF + q, t3_s, q, i * 8)
                for q in range(NF)]
        work += [functools.partial(rhs_job, g2, slot, 0, q, NQ + q, t2_s, q, i * 8)
                 for q in range(NQ)]
        row4 = clamp(i, FH // G4R - 1) * (G4R // 2)
        work += [functools.partial(rhs_job, g4, slot, 16 * rt, q, NQ + q, t4_s, q, row4 + 8 * rt)
                 for rt in range(G4R // 16) for q in range(NQ)]
        npin = 60
        jobs = [None] * npin
        for k, job in enumerate(work):
            jobs[1 + k * (npin - 1) // len(work)] = job

        sa_ = 2 * i
        sb_ = 2 * i + 1
        hb_tok = h_rows(sb_)
        oa, odef_a = chain_step(sa_, mem_s[...], hn_s[...], None)
        mixer_mm(jnp.maximum(i - 2, 0))
        ys = []

        def hook(k, anchor):
            if k >= PREP_CH:
                anchor = anchor[0:8] + ys[-PREP_CH][0:8, 0:E] + ys[-PREP_CH][8:16, 0:E]
            ys.append(mixer_prep(jnp.maximum(i - 1, 0), (k % 2) * SEG + (k // 2) * 16, 16, anchor))
            if k % 2:
                mixer_sets(ys[-2], ys[-1], (k // 2) * 16)

        hooks = {j: functools.partial(hook, k) for k, j in enumerate(PREP_AT)}
        ob, _ = chain_step(sb_, oa[0:M], hb_tok, odef_a, jobs, hooks)
        mem_s[...] = ob[0:M]
        aout_s[0:TC, :] = oa[M:SEG]
        aout_s[TC:SEG, :] = ob[SEG:SEG + M]
        aout_s[SEG:SEG + TC, :] = ob[M:SEG]
        aout_s[SEG + TC:2 * SEG, :] = ob[SEG + M:SEG + 2 * M]
        hn_s[...] = h_rows(jnp.minimum(sb_ + 1, NSEG - 1))
        for cp in mlp_w_copies(i + 2, slot):
            cp.start()
        return carry

    lax.fori_loop(0, _N2, _scoped("p2", p2_body), 0)

    TH = TB // 2
    SHIFT = (-1, -1, 1, 1, -2, -2, 2, 2)

    def g_job(j, rt, q, n=16, anchor=None):
        blk = []
        for hf in range(2):
            for ct in (q, NQ + q):
                win = t_s[pl.ds(aligned(j * TB + hf * TH + rt * n, 16), n + 16), ct * E:(ct + 1) * E]
                blk.append(win[8 + SHIFT[ct]:8 + SHIFT[ct] + n])
        blk[0] = after(blk[0], anchor)
        blk[3] = after(blk[3], anchor)
        for k, v in enumerate(_lhs_set(*blk)):
            g_s.at[k][rt * n // 2:(rt + 1) * n // 2, q * E:(q + 1) * E] = _pk(v)

    def mix(j):
        r0 = aligned(j * TB, TB)
        for q in range(NQ):
            cs = _strassen(lambda n: _dot(_up(g_s[n]), _up(t2_s[n, :, _ct(q)])))
            for k, cc in enumerate(cs):
                rr = pl.ds(r0 + (k // 2) * TH, TH)
                c0 = (q + NQ * (k % 2)) * E
                x1 = hb_s[rr, c0:c0 + E].astype(f32) + cc
                x1_s[(k // 2) * TH:(k // 2 + 1) * TH, c0:c0 + E] = x1
                hb_s[rr, c0:c0 + E] = x1.astype(bf16)

    def out_copy(j, slot):
        return copy(o_s.at[slot], out_hbm.at[pl.ds(aligned(j * TB, TB), TB)], SEM_OUT + slot)

    prev_y = [None]

    def put_y(rt=0, n=TH, anchor=None):
        if anchor is not None and rt > 0:
            anchor = anchor[0:8] + prev_y[0]
        ya = _ln(after(x1_s[rt * n:(rt + 1) * n, :], anchor))
        yb = _ln(after(x1_s[TH + rt * n:TH + (rt + 1) * n, :], anchor))
        sets = _lhs_set(ya[:, :HD], ya[:, HD:], yb[:, :HD], yb[:, HD:])
        prev_y[0] = sets[0][0:8, 0:E] + sets[0][8:16, 0:E]
        for k, v in enumerate(sets):
            y_s.at[k][rt * n // 2:(rt + 1) * n // 2, :] = _pk(v)

    wm_wait(0, D // E, SEM_WM)
    mod_tiles(0, D // E, 5 * D // E)
    mixer_mm(NI - 2)
    mixer_sets(mixer_prep(NI - 1, 0, SEG), mixer_prep(NI - 1, SEG, SEG), 0)
    for q in range(NQ):
        g_job(0, 0, q, TH)
    mix(0)
    mixer_mm(NI - 1)
    put_y()
    for q in range(NQ):
        g_job(1, 0, q, TH)

    def mlp_block(j, last):
        slot = j & 1
        r0 = aligned(j * TB, TB)
        for q in range(NF):
            cs = _strassen(lambda n: _dot(_up(y_s[n]), _up(t3_s[n, :, _ct(q)])))
            for n, v in enumerate(_lhs_set(*[_gelu(cc) for cc in cs])):
                u_s.at[n][:, q * E:(q + 1) * E] = _pk(v)
        jobs = {}
        if not last:
            mix(j + 1)
            jn = clamp(j + 2, NB - 1)
            for rt in range(TH // 16):
                jobs[Y_AT[rt]] = functools.partial(put_y, rt, 16)
            free = [k for k in range(G_AT, 7 * NQ) if k not in jobs]
            for k in range(TH // 16 * NQ):
                jobs[free[k]] = functools.partial(g_job, jn, k // NQ, k % NQ, 16)

        def prod(n, q):
            m = _dot(_up(u_s[n]), _up(t4_s[n, :, _ct(q)]))
            job = jobs.get(count[0])
            count[0] += 1
            if job is not None:
                job(anchor=m)
            return m

        count = [0]
        for q in range(NQ):
            if last and q == 0:
                ks = FH - 2 * E
                head = [_dot(_up(u_s[n, :, 0:ks]), _up(t4_s[n, 0:ks // 2, _ct(q)])) for n in range(7)]
                cs = _strassen(lambda n: _dot(_up(u_s[n, :, ks:FH]), _up(t4_s[n, ks // 2:, _ct(q)]))
                               + head[n])
            else:
                cs = _strassen(lambda n: prod(n, q))
            for k, cc in enumerate(cs):
                rr = pl.ds(r0 + (k // 2) * TH, TH)
                c0 = (q + NQ * (k % 2)) * E
                gb = mod_rows(5, TH, c0, E)
                o_s[slot, (k // 2) * TH:(k // 2 + 1) * TH, c0:c0 + E] = (
                    x2_s[rr, c0:c0 + E].astype(f32)
                    + gb * (hb_s[rr, c0:c0 + E].astype(f32) + cc)).astype(bf16)
        out_copy(j, slot).start()

    def p3_body(j, carry):
        @pl.when(j >= 2)
        def _():
            out_copy(j - 2, j & 1).wait()

        mlp_block(j, False)
        return carry

    lax.fori_loop(0, NB - 1, _scoped("p3", p3_body), 0)
    for k in range(2):
        for cp in mlp_w_copies(0, k):
            cp.wait()
    out_copy(NB - 3, (NB - 3) % 2).wait()
    mlp_block(NB - 1, True)
    out_copy(NB - 2, (NB - 2) % 2).wait()
    out_copy(NB - 1, (NB - 1) % 2).wait()


@jax.jit
def pallas_adaLN_cond__memory_aug_recurrent_mem_tr__mixer_s_mlp__prompt_kernel(
    A_x: jax.Array,
    A_mem0: jax.Array,
    A_Wq: jax.Array,
    A_Wk: jax.Array,
    A_Wv: jax.Array,
    A_Wo: jax.Array,
    A_seg_len,
    B_x: jax.Array,
    B_w1: jax.Array,
    B_w2: jax.Array,
    B_w3: jax.Array,
    B_w4: jax.Array,
    c: jax.Array,
    w_mod: jax.Array,
):
    del A_seg_len, B_x
    assert A_x.shape == (1, S, D) and A_mem0.shape == (1, M, D)
    hbm = pl.BlockSpec(memory_space=pl.ANY)
    scratch = [
        pltpu.VMEM((NSEG, SEG, D), bf16),
        pltpu.VMEM((NSEG, M, D), bf16),
        pltpu.VMEM((7, NSEG * M // 4, D // 2), u32),
        pltpu.VMEM((3 * D // E, D, E), bf16),
        pltpu.VMEM((2, D, HG, E), bf16),
        pltpu.VMEM((NC + 3, D // 2, HG * E), u32),
        pltpu.VMEM((H * E // 2, D), u32),
        pltpu.VMEM((7, D // 4, D // 2), u32),
        pltpu.VMEM((2, 2, G1R, D), bf16),
        pltpu.VMEM((7, D // 4, D // 2), u32),
        pltpu.VMEM((7, D // 4, FH), u32),
        pltpu.VMEM((7, FH // 2, D // 2), u32),
        pltpu.VMEM((2, 2, 16, D), bf16),
        pltpu.VMEM((2, 2, 16, F), bf16),
        pltpu.VMEM((2, 2, G4R, D), bf16),
        pltpu.VMEM((NC + 2, NSEG * M, HG // 2 * E), u32),
        pltpu.VMEM((8, 6 * D), f32),
        pltpu.VMEM((M, D), f32),
        pltpu.VMEM((TC, D), f32),
        pltpu.VMEM((2 * SEG, D), f32),
        pltpu.VMEM((NR, E), f32),
        pltpu.VMEM((S, D), bf16),
        pltpu.VMEM((S, D), bf16),
        pltpu.VMEM((S + 16, D), f32),
        pltpu.VMEM((7, SEG // 2, D // 2), u32),
        pltpu.VMEM((TB, D), f32),
        pltpu.VMEM((7, TB // 4, D // 2), u32),
        pltpu.VMEM((7, TB // 4, D // 2), u32),
        pltpu.VMEM((7, TB // 4, FH), u32),
        pltpu.VMEM((2, TB, D), bf16),
        pltpu.VMEM((8, E), u32),
        pltpu.VMEM((2, BGR, D), bf16),
        pltpu.VMEM((1, D), bf16),
        pltpu.VMEM((M, D), bf16),
        pltpu.SemaphoreType.DMA((24,)),
    ]
    out = pl.pallas_call(
        _kernel,
        out_shape=jax.ShapeDtypeStruct((S, D), bf16),
        in_specs=[hbm] * 12,
        out_specs=hbm,
        scratch_shapes=scratch,
        compiler_params=pltpu.CompilerParams(vmem_limit_bytes=126 * 1024 * 1024,
                                             disable_bounds_checks=NO_BOUNDS),
    )(A_x.reshape(NSEG, SEG, D), A_mem0.reshape(M, D), A_Wq, A_Wk, A_Wv,
      A_Wo.reshape(H * E, D), B_w1.reshape(2, D // 2, D), B_w2.reshape(2, D // 2, D), B_w3.reshape(2, D // 2, F),
      B_w4.reshape(2, FH, D), c, w_mod)
    return out.reshape(1, S, D)
```

```python
import functools

import jax
import jax.numpy as jnp
from jax import lax
import jax.experimental.pallas as pl
import jax.experimental.pallas.tpu as pltpu

bf16, f32, u32 = jnp.bfloat16, jnp.float32, jnp.uint32

S, D, H, E, M, SEG, F = 2048, 1024, 32, 128, 8, 32, 3584
NSEG = S // SEG
NP = H // 2
TC = SEG - M
HG = 8
NG = H // HG
TB = 128
NB = S // TB
FH = F // 2
NF = FH // E
G4R = 64
NI = NSEG // 2
NQ = D // E // 2
NC = 3 * NG
BGR = 384
G1R = 48
HD = D // 2
X0 = 4
NR = 2 * (M + SEG)
NO_BOUNDS = True
PIN_ROWS = 256
Y_AT = (0, 7, 14, 21)
G_AT = 2
PREP_AT = (0, 1, 3, 4)
PREP_CH = 2
SORD = 0
FINE = 1
JGROUP = 1
P1_TAIL = 5
P1_LAG = 4
SCHED_A = (2, 1, 3)
SCHED_B = (3, 1, 3)
EPS = 1e-5
SCALE = E ** -0.5
_SCOPES = False
_N2 = NSEG // 2


def _scoped(name, fn):
    def wrapped(*a):
        if not _SCOPES:
            return fn(*a)
        with jax.named_scope(name):
            return fn(*a)
    return wrapped


def _pk(x):
    return pltpu.bitcast(x.astype(bf16), u32)


def _up(x):
    return pltpu.bitcast(x, bf16)


def _ct(k):
    return slice(k * E, (k + 1) * E)


def _dot(a, b):
    return jnp.dot(a, b, preferred_element_type=f32)


def _ln(x):
    m = jnp.mean(x, axis=-1, keepdims=True)
    xc = x - m
    v = jnp.mean(xc * xc, axis=-1, keepdims=True)
    return xc * lax.rsqrt(v + EPS)


def _gelu(x):
    c = 0.7978845608028654
    return 0.5 * x * (1.0 + jnp.tanh(c * (x + 0.044715 * (x * x * x))))


def _lhs_set(a11, a12, a21, a22):
    return (a11 + a22, a21 + a22, a11, a22, a11 + a12, a21 - a11, a12 - a22)


def _rhs_set(b11, b12, b21, b22):
    return (b11 + b22, b11, b12 - b22, b21 - b11, b22, b11 + b12, b21 + b22)


def _strassen(m):
    if SORD == 0:
        m1 = m(0)
        m2 = m(1)
        c22 = m1 - m2
        m3 = m(2)
        c22 = c22 + m3
        c22 = m(5) + c22
        m4 = m(3)
        c21 = m2 + m4
        c11 = m1 + m4
        m5 = m(4)
        c12 = m3 + m5
        c11 = c11 - m5
        c11 = m(6) + c11
    else:
        m2 = m(1)
        c22 = m(5) - m2
        m4 = m(3)
        c21 = m2 + m4
        m1 = m(0)
        c22 = c22 + m1
        c11 = m4 + m1
        m3 = m(2)
        c22 = c22 + m3
        m5 = m(4)
        c12 = m3 + m5
        c11 = c11 - m5
        c11 = m(6) + c11
    return c11, c12, c21, c22


def _mask_fill():
    shape = (NR, E)
    r = lax.broadcasted_iota(jnp.int32, shape, 0)
    c = lax.broadcasted_iota(jnp.int32, shape, 1)

    def headpos(i):
        head = jnp.where(i < 64, i >> 5, (i - 64) >> 3)
        pos = jnp.where(i < 64, i & 31, 32 + (i & 7))
        return head, pos

    hr, pr = headpos(r)
    hc, pc = headpos(c)
    same = hr == hc
    valid = same & ((pr < M) | (pr >= pc))
    return jnp.where(valid, 0.0, jnp.where(same, -1e9, -jnp.inf)).astype(f32)


def _kernel(x_hbm, mem0_hbm, wq_hbm, wk_hbm, wv_hbm, wo_hbm, w1_hbm, w2_hbm, w3_hbm,
            w4_hbm, c_hbm, wm_hbm,
            out_hbm,
            x_s, xpre_s, hpre_s, wm_s, stg, w_s, wo_s,
            t1_s, g1, t2_s, t3_s, t4_s, g2, g3, g4, pre_s, mod_s, mem_s, hn_s, aout_s, fill_s,
            x2_s, hb_s, t_s, l1_s, x1_s, g_s, y_s, u_s, o_s, zero_s, bg, c_s, mem0_s, sems):
    w_hbm = (wq_hbm, wk_hbm, wv_hbm)

    (SEM_C, SEM_MEM, SEM_XPRE, SEM_X, SEM_STG, SEM_BG, SEM_OUT,
     SEM_WMR, SEM_G2, SEM_G3, SEM_G4, SEM_WM, SEM_G1) = (0, 1, 2, 3, 4, 6, 8, 10, 12, 14, 16, 18, 22)

    def copy(src, dst, k):
        return pltpu.make_async_copy(src, dst, sems.at[k])

    def w_copy(t, g, slot):
        return copy(w_hbm[t].at[:, pl.ds(pl.multiple_of(g * HG, HG), HG), :], stg.at[slot],
                    SEM_STG + slot)

    def bg_rows(k):
        return clamp(k * BGR, H * E - BGR), clamp(k * G1R, HD - G1R)

    def bg_copies(k, slot):
        ro, r1 = bg_rows(k)
        return (copy(wo_hbm.at[pl.ds(aligned(ro, 16), BGR)], bg.at[slot], SEM_BG + slot),
                copy(w1_hbm.at[:, pl.ds(aligned(r1, 16), G1R), :], g1.at[slot], SEM_G1 + slot))

    def wm_copy(src_tile, dst_tile, sem):
        return copy(wm_hbm.at[:, pl.ds(aligned(src_tile * E, E), E)], wm_s.at[dst_tile], sem)

    def wm_wait(t0, n, sem):
        copy(wm_s.at[t0:t0 + n], wm_s.at[t0:t0 + n], sem).wait()

    def aligned(x, n):
        return x if isinstance(x, int) else pl.multiple_of(x, n)

    def clamp(k, hi):
        return min(k, hi) if isinstance(k, int) else jnp.minimum(k, hi)

    def mlp_w_copies(k, slot):
        r = pl.ds(aligned(clamp(k, NI - 1) * 16, 16), 16)
        r4 = pl.ds(aligned(clamp(k, FH // G4R - 1) * G4R, 16), G4R)
        return (copy(w2_hbm.at[:, r, :], g2.at[slot], SEM_G2 + slot),
                copy(w3_hbm.at[:, r, :], g3.at[slot], SEM_G3 + slot),
                copy(w4_hbm.at[:, r4, :], g4.at[slot], SEM_G4 + slot))

    def pinned(w, job):
        if job is None:
            return w()
        z = job() & zero_s[...]
        w = w()
        return jnp.concatenate([w[0:8] | z, w[8:]], axis=0)

    def after(x, anchor):
        if anchor is None:
            return x
        z = pltpu.bitcast(pltpu.bitcast(anchor[0:8], u32) & zero_s[...], f32)
        z = jnp.concatenate([z] * (x.shape[0] // 8), axis=0)
        return jnp.concatenate([x[:, 0:E] + z, x[:, E:]], axis=1) if x.shape[1] > E else x + z

    def rhs_job(src, slot, r0, c1, c2, dst, q, row, z=None):
        blk = [src[slot, kh, r0:r0 + 16, cc * E:(cc + 1) * E].astype(f32)
               for kh in range(2) for cc in (c1, c2)]
        if z is not None:
            zf = pltpu.bitcast(jnp.concatenate([z, z], axis=0), f32)
            blk[0] = blk[0] + zf
            blk[3] = blk[3] + zf
        sets = _rhs_set(*blk)
        for n, v in enumerate(sets):
            dst.at[n][pl.ds(pl.multiple_of(row, 8), 8), _ct(q)] = _pk(v)
        out = pltpu.bitcast(sets[2], u32) | pltpu.bitcast(sets[3], u32)
        return out[0:8] | out[8:16]

    def mod_rows(k, n, c0=0, w=D):
        return jnp.concatenate([mod_s[:, k * D + c0:k * D + c0 + w]] * (n // 8), axis=0)

    def tq_place(c, n):
        if n == 1:
            return w_s.at[c], 0, None
        if n == 4:
            return w_s.at[c], D // 4, None
        if n == 6:
            return pre_s.at[c + 1], 0, 0
        k = (0, 2, 3, 5).index(n)
        return w_s.at[c + 2], (k // 2) * (D // 4), (k % 2) * (HG // 2)

    def relayout_jobs(slot, c, i):
        memo = []
        r = aligned(i * 8, 8)

        def job(j, z=None):
            if not memo:
                for d0 in (i * 16, HD + i * 16):
                    memo.append(jnp.swapaxes(pltpu.bitcast(stg[slot, pl.ds(d0, 16)], u32), 0, 1))
            blk = []
            for kh in range(2):
                u = memo[kh][j]
                if z is not None:
                    u = u | jnp.concatenate([z, z], axis=0)
                blk.append(pltpu.bitcast(u << 16, f32))
                blk.append(pltpu.bitcast(u & jnp.uint32(0xFFFF0000), f32))
            for k, v in enumerate(blk):
                w_s.at[c][pl.ds((k // 2) * (D // 4) + r, 8), _ct(2 * j + k % 2)] = _pk(v)
            for n, v in enumerate(_rhs_set(*blk)):
                if n not in (1, 4):
                    ref, r0, c0 = tq_place(c, n)
                    ref[pl.ds(r0 + r, 8), _ct(c0 + j)] = _pk(v)

        return [functools.partial(job, j) for j in range(HG // 2)]

    def repack(slot, row, i, z):
        v = pltpu.bitcast(bg[slot, 16 * i:16 * i + 16, :], u32)
        v = v | jnp.concatenate([z] * (D // E), axis=1)
        wo_s[pl.ds(pl.multiple_of(row + 8 * i, 8), 8), :] = v

    cp_c = copy(c_hbm, c_s, SEM_C)
    cp_mem = copy(mem0_hbm, mem0_s, SEM_MEM)
    cp_xpre = copy(x_hbm.at[:, TC:SEG, :], xpre_s, SEM_XPRE)
    w_copy(0, 0, 0).start()
    cp_xpre.start()
    cp_c.start()
    cp_mem.start()
    for k in range(2 * D // E):
        wm_copy(k, k, SEM_WM + k // 4).start()
    w_copy(0, 1, 1).start()

    zero_s[...] = jnp.zeros(zero_s.shape, u32)
    fill_s[...] = _mask_fill()
    aout_s[...] = jnp.zeros(aout_s.shape, f32)
    l1_s[...] = jnp.zeros(l1_s.shape, u32)
    bg[1] = jnp.zeros(bg.shape[1:], bf16)
    g1[1] = jnp.zeros(g1.shape[1:], bf16)

    w_copy(0, 0, 0).wait()

    def rl0_body(i, carry):
        for job in relayout_jobs(0, 0, i):
            job()
        return carry

    lax.fori_loop(0, D // 32, rl0_body, 0)
    w_copy(0, 2, 0).start()
    for cp in bg_copies(0, 0):
        cp.start()

    cp_xpre.wait()

    def npre_body(i, carry):
        xr = xpre_s[pl.ds(pl.multiple_of(i * 8, 8), 8)].astype(f32).reshape(64, D)
        t_s[pl.ds(pl.multiple_of(i * 64, 64), 64), :] = _ln(xr)
        return carry

    lax.fori_loop(0, NSEG // 8, _scoped("npre", npre_body), 0)

    cp_c.wait()
    cp_mem.wait()
    mem_s[...] = mem0_s[...].astype(f32)
    cf = c_s[...].astype(f32)
    sc = cf * (1.0 / (1.0 + jnp.exp(-cf)))
    sc8 = jnp.broadcast_to(sc, (8, D)).astype(bf16)

    def mod_tiles(t0, n, dst_tile):
        for k in range(n):
            v = _dot(sc8, wm_s[t0 + k])
            if (dst_tile + k) // (D // E) in (1, 4):
                v = 1.0 + v
            mod_s[:, _ct(dst_tile + k)] = v

    for k in range(4):
        wm_wait(4 * k, 4, SEM_WM + k)
        mod_tiles(4 * k, 4, 4 * k)

    PH = NSEG * M // 2

    def hpre_body(i, carry):
        h = [t_s[pl.ds(pl.multiple_of(hf * PH + i * 16, 16), 16), :] * mod_rows(1, 16) + mod_rows(0, 16)
             for hf in range(2)]
        for n, v in enumerate(_lhs_set(h[0][:, :HD], h[0][:, HD:], h[1][:, :HD], h[1][:, HD:])):
            hpre_s.at[n][pl.ds(pl.multiple_of(i * 8, 8), 8), :] = _pk(v)
        return carry

    lax.fori_loop(0, PH // 16, _scoped("hpre", hpre_body), 0)

    t_s[0:8, :] = jnp.zeros((8, D), f32)
    t_s[S + 8:S + 16, :] = jnp.zeros((8, D), f32)

    def modulate_a(xr):
        return _ln(xr) * mod_rows(1, xr.shape[0]) + mod_rows(0, xr.shape[0])

    MB = 64

    def x_copy(k):
        r = slice(0, X0) if k == 0 else slice(X0, NSEG)
        return copy(x_hbm.at[r], x_s.at[r], SEM_XPRE if k == 0 else SEM_X)


    def p1_body(c, carry):
        slot = c & 1
        pslot = 1 - slot
        ro, r1 = bg_rows(jnp.maximum(c - 1, 0))

        @pl.when(c >= 1)
        def _():
            for cp in bg_copies(0, pslot):
                cp.wait()

        @pl.when(c + 1 < NC)
        def _():
            w_copy(0, 0, pslot).wait()

        small = [functools.partial(repack, pslot, ro >> 1, i) for i in range(BGR // 16)]
        small += [functools.partial(rhs_job, g1, pslot, 16 * rt, q, NQ + q, t1_s, q, (r1 >> 1) + 8 * rt)
                  for rt in range(G1R // 16) for q in range(NQ)]
        work = []
        nu = D // 32
        for i in range(nu):
            js = relayout_jobs(pslot, c + 1, i)
            work += [js[k:k + JGROUP] for k in range(0, len(js), JGROUP)]
            work += [[job] for job in small[i * len(small) // nu:(i + 1) * len(small) // nu]]
        npin = 7 * (HG // 2) * (PH // MB)
        jobs = [[] for _ in range(npin)]
        for k, group in enumerate(work):
            pos = k * (npin - P1_TAIL) * 8 // len(work)
            jobs[pos // 8] += [(job, pos % 8 if FINE else 0) for job in group]
        jobs = iter(jobs)

        def prod(n, q, mb):
            ref, r0, c0 = tq_place(c, n)
            w = ref[r0:r0 + D // 4, _ct(2 * q + (n == 4) if c0 is None else c0 + q)]
            m = _dot(_up(hpre_s[n, mb * MB // 2:(mb + 1) * MB // 2, :]), _up(w))
            pending.append(m)
            if len(pending) > P1_LAG:
                anchor = pltpu.bitcast(pending.pop(0), u32)
                for job, g in next(jobs):
                    job(anchor[8 * g:8 * g + 8] & zero_s[...])
            return m

        pending = []
        ns = MB // M
        for q in range(HG // 2):
            for mb in range(PH // MB):
                cs = _strassen(lambda n: prod(n, q, mb))
                for hf in range(2):
                    y = jnp.concatenate([cs[2 * hf + k][sg * M:(sg + 1) * M]
                                         for sg in range(ns) for k in range(2)], axis=0)
                    s0 = hf * (NSEG // 2) + mb * ns
                    pre_s.at[c][s0 * M:(s0 + ns) * M, _ct(q)] = _pk(y)

        for t in range(3):
            @pl.when((c + 3) >> 2 == t)
            def _():
                w_copy(t, (c + 3) & 3, pslot).start()

        @pl.when(c + 2 < NC)
        def _():
            for cp in bg_copies(c + 1, pslot):
                cp.start()

        @pl.when(c < NC - 3)
        def _():
            wm_copy(2 * D // E + c, c, SEM_WMR).start()

        @pl.when(c == NC - 3)
        def _():
            def issue(k, carry2):
                wm_copy(2 * D // E + k, k, SEM_WMR).start()
                return carry2

            x_copy(0).start()
            for k in range(2):
                for cp in mlp_w_copies(k, k):
                    cp.start()
            lax.fori_loop(NC - 3, 3 * D // E, issue, 0)

        return carry

    lax.fori_loop(0, NC, _scoped("p1", p1_body), 0)
    x_copy(1).start()
    x_copy(0).wait()
    wm_wait(0, 3 * D // E, SEM_WMR)
    mod_tiles(0, 3 * D // E, 2 * D // E)
    for k in range(D // E):
        wm_copy(5 * D // E + k, k, SEM_WM).start()

    def h_rows(s):
        return modulate_a(x_s[s, 0:TC, :].astype(f32))

    hn_s[...] = h_rows(0)

    def chain_step(s, mem, htok, odef_prev, jobs=(), hooks=None):
        hs = jnp.concatenate([mem, htok], axis=0).astype(bf16)
        qkv = [[None] * 3 for _ in range(NP)]
        ps = [None] * NP
        os_ = [None] * H
        odef = [None] * H

        def proj(p, ts=(0, 1, 2)):
            for t in ts:
                c, q = t * NG + p // (HG // 2), p % (HG // 2)
                a = _dot(hs, _up(w_s[c, :, _ct(2 * q)]))
                b = _dot(hs, _up(w_s[c, :, _ct(2 * q + 1)]))
                if hooks and t == 2 and p - NP in hooks:
                    hooks[p - NP](b)
                pre = pre_s[c, pl.ds(pl.multiple_of(s * M, M), M), _ct(q)]
                if t == 1:
                    kf = jnp.concatenate([a, b, _up(pre).astype(f32), jnp.zeros((E - NR, E), f32)],
                                         axis=0)
                    qkv[p][t] = kf.T.astype(bf16)
                    continue
                parts = [_pk(a), _pk(b), pre]
                if t == 2:
                    parts.append(jnp.zeros(((E - NR) // 2, E), u32))
                qkv[p][t] = _up(jnp.concatenate(parts, axis=0))

        def scores(p):
            sc_ = _dot(qkv[p][0], qkv[p][1])
            fill = fill_s[...]
            sc_ = jnp.where(fill == 0.0, sc_ * SCALE, fill)
            m = jnp.max(sc_, axis=-1, keepdims=True)
            e = jnp.exp(sc_ - m)
            l = jnp.sum(e, axis=-1, keepdims=True)
            r = pl.reciprocal(l, approx=True)
            r = r * (2.0 - l * r)
            ps[p] = (e * r).astype(bf16)

        def fin(p):
            o = _dot(ps[p], qkv[p][2])
            for hh in range(2):
                h = 2 * p + hh
                rows = o[32 * hh:32 * hh + 32]
                odef[h] = o[64 + 8 * hh:72 + 8 * hh]
                if odef_prev is not None:
                    rows = jnp.concatenate([rows, odef_prev[h], odef[h]], axis=0)
                os_[h] = _pk(rows)

        acc = [None] * 8
        jobs = iter(jobs)

        def wo(h0, h1, js):
            lhs = _up(jnp.concatenate(os_[h0:h1], axis=1))
            for j in js:
                ws = []
                for r0 in range(h0 * E // 2, h1 * E // 2, PIN_ROWS):
                    ws.append(pinned(lambda: wo_s[r0:r0 + PIN_ROWS, j * E:(j + 1) * E],
                                     next(jobs, None)))
                part = _dot(lhs, _up(jnp.concatenate(ws, axis=0)))
                if hooks and acc[j] is None and j in hooks:
                    hooks[j](part)
                acc[j] = part if acc[j] is None else part + acc[j]

        ORDER, LAG_S, LAG_O = SCHED_A if odef_prev is None else SCHED_B
        for p in range(NP):
            if ORDER == 0:
                proj(p)
                if p >= LAG_S:
                    scores(p - LAG_S)
                if p >= LAG_O:
                    fin(p - LAG_O)
            elif ORDER == 1:
                proj(p, (1, 0))
                if p >= LAG_O:
                    fin(p - LAG_O)
                proj(p, (2,))
                if p >= LAG_S:
                    scores(p - LAG_S)
            elif ORDER == 2:
                proj(p, (1,))
                if p >= LAG_S:
                    scores(p - LAG_S)
                proj(p, (0,))
                if p >= LAG_O:
                    fin(p - LAG_O)
                proj(p, (2,))
            elif ORDER == 3:
                proj(p, (1,))
                if p >= LAG_O:
                    fin(p - LAG_O)
                proj(p, (0,))
                if p >= LAG_S:
                    scores(p - LAG_S)
                proj(p, (2,))
            elif ORDER == 4:
                proj(p, (1,))
                if p >= LAG_S:
                    scores(p - LAG_S)
                proj(p, (0, 2))
                if p >= LAG_O:
                    fin(p - LAG_O)
            else:
                proj(p, (0,))
                if p >= LAG_S:
                    scores(p - LAG_S)
                proj(p, (1,))
                if p >= LAG_O:
                    fin(p - LAG_O)
                proj(p, (2,))
        tail = []
        for k in range(LAG_O):
            step = []
            if NP - LAG_S + k < NP:
                step.append(functools.partial(scores, NP - LAG_S + k))
            step.append(functools.partial(fin, NP - LAG_O + k))
            tail.append(step)
        hsplit = min(24, 2 * (NP - LAG_O))
        cuts = {3: (2, 3, 5), 2: (2, 5), 4: (1, 2, 4, 6), 5: (1, 2, 3, 4, 6)}[LAG_O]
        j0 = 0
        for k, step in enumerate(tail):
            wo(0, hsplit, range(j0, cuts[k]))
            j0 = cuts[k]
            for f in step:
                f()
        wo(0, hsplit, range(j0, 8))
        wo(hsplit, H, range(8))
        return jnp.concatenate(acc, axis=1), odef

    def mixer_prep(i, r0, n, anchor=None):
        r = pl.ds(aligned(i * 64 + r0, 16), n)
        xr = x_s[2 * i + r0 // SEG, r0 % SEG:r0 % SEG + n, :].astype(f32)
        x2 = xr + mod_rows(2, n) * after(aout_s[r0:r0 + n, :], anchor)
        x2_s[r, :] = x2.astype(bf16)
        hb = _ln(x2) * mod_rows(4, n) + mod_rows(3, n)
        hb_s[r, :] = hb.astype(bf16)
        return _ln(hb)

    def mixer_sets(ya, yb, r0):
        n = ya.shape[0]
        for m, v in enumerate(_lhs_set(ya[:, :HD], ya[:, HD:], yb[:, :HD], yb[:, HD:])):
            l1_s.at[m][r0 // 2:(r0 + n) // 2, :] = _pk(v)

    def mixer_mm(i):
        for q in range(NQ):
            cs = _strassen(lambda n: _dot(_up(l1_s[n]), _up(t1_s[n, :, _ct(q)])))
            for k, cc in enumerate(cs):
                r0 = aligned(i * 64 + 8 + (k // 2) * SEG, 8)
                t_s[pl.ds(r0, SEG), _ct(q + NQ * (k % 2))] = _gelu(cc)

    def p2_body(i, carry):
        slot = i & 1
        for cp in mlp_w_copies(0, slot):
            cp.wait()

        @pl.when(i == 1)
        def _():
            x_copy(1).wait()

        work = [functools.partial(rhs_job, g3, slot, 0, q, NF + q, t3_s, q, i * 8)
                for q in range(NF)]
        work += [functools.partial(rhs_job, g2, slot, 0, q, NQ + q, t2_s, q, i * 8)
                 for q in range(NQ)]
        row4 = clamp(i, FH // G4R - 1) * (G4R // 2)
        work += [functools.partial(rhs_job, g4, slot, 16 * rt, q, NQ + q, t4_s, q, row4 + 8 * rt)
                 for rt in range(G4R // 16) for q in range(NQ)]
        npin = 60
        jobs = [None] * npin
        for k, job in enumerate(work):
            jobs[1 + k * (npin - 1) // len(work)] = job

        sa_ = 2 * i
        sb_ = 2 * i + 1
        hb_tok = h_rows(sb_)
        oa, odef_a = chain_step(sa_, mem_s[...], hn_s[...], None)
        mixer_mm(jnp.maximum(i - 2, 0))
        ys = []

        def hook(k, anchor):
            if k >= PREP_CH:
                anchor = anchor[0:8] + ys[-PREP_CH][0:8, 0:E] + ys[-PREP_CH][8:16, 0:E]
            ys.append(mixer_prep(jnp.maximum(i - 1, 0), (k % 2) * SEG + (k // 2) * 16, 16, anchor))
            if k % 2:
                mixer_sets(ys[-2], ys[-1], (k // 2) * 16)

        hooks = {j: functools.partial(hook, k) for k, j in enumerate(PREP_AT)}
        ob, _ = chain_step(sb_, oa[0:M], hb_tok, odef_a, jobs, hooks)
        mem_s[...] = ob[0:M]
        aout_s[0:TC, :] = oa[M:SEG]
        aout_s[TC:SEG, :] = ob[SEG:SEG + M]
        aout_s[SEG:SEG + TC, :] = ob[M:SEG]
        aout_s[SEG + TC:2 * SEG, :] = ob[SEG + M:SEG + 2 * M]
        hn_s[...] = h_rows(jnp.minimum(sb_ + 1, NSEG - 1))
        for cp in mlp_w_copies(i + 2, slot):
            cp.start()
        return carry

    lax.fori_loop(0, _N2, _scoped("p2", p2_body), 0)

    TH = TB // 2
    SHIFT = (-1, -1, 1, 1, -2, -2, 2, 2)

    def g_job(j, rt, q, n=16, anchor=None):
        blk = []
        for hf in range(2):
            for ct in (q, NQ + q):
                win = t_s[pl.ds(aligned(j * TB + hf * TH + rt * n, 16), n + 16), ct * E:(ct + 1) * E]
                blk.append(win[8 + SHIFT[ct]:8 + SHIFT[ct] + n])
        blk[0] = after(blk[0], anchor)
        blk[3] = after(blk[3], anchor)
        for k, v in enumerate(_lhs_set(*blk)):
            g_s.at[k][rt * n // 2:(rt + 1) * n // 2, q * E:(q + 1) * E] = _pk(v)

    def mix(j):
        r0 = aligned(j * TB, TB)
        for q in range(NQ):
            cs = _strassen(lambda n: _dot(_up(g_s[n]), _up(t2_s[n, :, _ct(q)])))
            for k, cc in enumerate(cs):
                rr = pl.ds(r0 + (k // 2) * TH, TH)
                c0 = (q + NQ * (k % 2)) * E
                x1 = hb_s[rr, c0:c0 + E].astype(f32) + cc
                x1_s[(k // 2) * TH:(k // 2 + 1) * TH, c0:c0 + E] = x1
                hb_s[rr, c0:c0 + E] = x1.astype(bf16)

    def out_copy(j, slot):
        return copy(o_s.at[slot], out_hbm.at[pl.ds(aligned(j * TB, TB), TB)], SEM_OUT + slot)

    prev_y = [None]

    def put_y(rt=0, n=TH, anchor=None):
        if anchor is not None and rt > 0:
            anchor = anchor[0:8] + prev_y[0]
        ya = _ln(after(x1_s[rt * n:(rt + 1) * n, :], anchor))
        yb = _ln(after(x1_s[TH + rt * n:TH + (rt + 1) * n, :], anchor))
        sets = _lhs_set(ya[:, :HD], ya[:, HD:], yb[:, :HD], yb[:, HD:])
        prev_y[0] = sets[0][0:8, 0:E] + sets[0][8:16, 0:E]
        for k, v in enumerate(sets):
            y_s.at[k][rt * n // 2:(rt + 1) * n // 2, :] = _pk(v)

    wm_wait(0, D // E, SEM_WM)
    mod_tiles(0, D // E, 5 * D // E)
    mixer_mm(NI - 2)
    mixer_sets(mixer_prep(NI - 1, 0, SEG), mixer_prep(NI - 1, SEG, SEG), 0)
    for q in range(NQ):
        g_job(0, 0, q, TH)
    mix(0)
    mixer_mm(NI - 1)
    put_y()
    for q in range(NQ):
        g_job(1, 0, q, TH)

    def mlp_block(j, last):
        slot = j & 1
        r0 = aligned(j * TB, TB)
        for q in range(NF):
            cs = _strassen(lambda n: _dot(_up(y_s[n]), _up(t3_s[n, :, _ct(q)])))
            for n, v in enumerate(_lhs_set(*[_gelu(cc) for cc in cs])):
                u_s.at[n][:, q * E:(q + 1) * E] = _pk(v)
        jobs = {}
        if not last:
            mix(j + 1)
            jn = clamp(j + 2, NB - 1)
            for rt in range(TH // 16):
                jobs[Y_AT[rt]] = functools.partial(put_y, rt, 16)
            free = [k for k in range(G_AT, 7 * NQ) if k not in jobs]
            for k in range(TH // 16 * NQ):
                jobs[free[k]] = functools.partial(g_job, jn, k // NQ, k % NQ, 16)

        def prod(n, q):
            m = _dot(_up(u_s[n]), _up(t4_s[n, :, _ct(q)]))
            job = jobs.get(count[0])
            count[0] += 1
            if job is not None:
                job(anchor=m)
            return m

        count = [0]
        for q in range(NQ):
            if last and q == 0:
                ks = FH - 2 * E
                head = [_dot(_up(u_s[n, :, 0:ks]), _up(t4_s[n, 0:ks // 2, _ct(q)])) for n in range(7)]
                cs = _strassen(lambda n: _dot(_up(u_s[n, :, ks:FH]), _up(t4_s[n, ks // 2:, _ct(q)]))
                               + head[n])
            else:
                cs = _strassen(lambda n: prod(n, q))
            for k, cc in enumerate(cs):
                rr = pl.ds(r0 + (k // 2) * TH, TH)
                c0 = (q + NQ * (k % 2)) * E
                gb = mod_rows(5, TH, c0, E)
                o_s[slot, (k // 2) * TH:(k // 2 + 1) * TH, c0:c0 + E] = (
                    x2_s[rr, c0:c0 + E].astype(f32)
                    + gb * (hb_s[rr, c0:c0 + E].astype(f32) + cc)).astype(bf16)
        out_copy(j, slot).start()

    def p3_body(j, carry):
        @pl.when(j >= 2)
        def _():
            out_copy(j - 2, j & 1).wait()

        mlp_block(j, False)
        return carry

    lax.fori_loop(0, NB - 1, _scoped("p3", p3_body), 0)
    for k in range(2):
        for cp in mlp_w_copies(0, k):
            cp.wait()
    out_copy(NB - 3, (NB - 3) % 2).wait()
    mlp_block(NB - 1, True)
    out_copy(NB - 2, (NB - 2) % 2).wait()
    out_copy(NB - 1, (NB - 1) % 2).wait()


@jax.jit
def pallas_adaLN_cond__memory_aug_recurrent_mem_tr__mixer_s_mlp__prompt_kernel(
    A_x: jax.Array,
    A_mem0: jax.Array,
    A_Wq: jax.Array,
    A_Wk: jax.Array,
    A_Wv: jax.Array,
    A_Wo: jax.Array,
    A_seg_len,
    B_x: jax.Array,
    B_w1: jax.Array,
    B_w2: jax.Array,
    B_w3: jax.Array,
    B_w4: jax.Array,
    c: jax.Array,
    w_mod: jax.Array,
):
    del A_seg_len, B_x
    assert A_x.shape == (1, S, D) and A_mem0.shape == (1, M, D)
    hbm = pl.BlockSpec(memory_space=pl.ANY)
    scratch = [
        pltpu.VMEM((NSEG, SEG, D), bf16),
        pltpu.VMEM((NSEG, M, D), bf16),
        pltpu.VMEM((7, NSEG * M // 4, D // 2), u32),
        pltpu.VMEM((3 * D // E, D, E), bf16),
        pltpu.VMEM((2, D, HG, E), bf16),
        pltpu.VMEM((NC + 3, D // 2, HG * E), u32),
        pltpu.VMEM((H * E // 2, D), u32),
        pltpu.VMEM((7, D // 4, D // 2), u32),
        pltpu.VMEM((2, 2, G1R, D), bf16),
        pltpu.VMEM((7, D // 4, D // 2), u32),
        pltpu.VMEM((7, D // 4, FH), u32),
        pltpu.VMEM((7, FH // 2, D // 2), u32),
        pltpu.VMEM((2, 2, 16, D), bf16),
        pltpu.VMEM((2, 2, 16, F), bf16),
        pltpu.VMEM((2, 2, G4R, D), bf16),
        pltpu.VMEM((NC + 2, NSEG * M, HG // 2 * E), u32),
        pltpu.VMEM((8, 6 * D), f32),
        pltpu.VMEM((M, D), f32),
        pltpu.VMEM((TC, D), f32),
        pltpu.VMEM((2 * SEG, D), f32),
        pltpu.VMEM((NR, E), f32),
        pltpu.VMEM((S, D), bf16),
        pltpu.VMEM((S, D), bf16),
        pltpu.VMEM((S + 16, D), f32),
        pltpu.VMEM((7, SEG // 2, D // 2), u32),
        pltpu.VMEM((TB, D), f32),
        pltpu.VMEM((7, TB // 4, D // 2), u32),
        pltpu.VMEM((7, TB // 4, D // 2), u32),
        pltpu.VMEM((7, TB // 4, FH), u32),
        pltpu.VMEM((2, TB, D), bf16),
        pltpu.VMEM((8, E), u32),
        pltpu.VMEM((2, BGR, D), bf16),
        pltpu.VMEM((1, D), bf16),
        pltpu.VMEM((M, D), bf16),
        pltpu.SemaphoreType.DMA((24,)),
    ]
    out = pl.pallas_call(
        _kernel,
        out_shape=jax.ShapeDtypeStruct((S, D), bf16),
        in_specs=[hbm] * 12,
        out_specs=hbm,
        scratch_shapes=scratch,
        compiler_params=pltpu.CompilerParams(vmem_limit_bytes=126 * 1024 * 1024,
                                             disable_bounds_checks=NO_BOUNDS),
    )(A_x.reshape(NSEG, SEG, D), A_mem0.reshape(M, D), A_Wq, A_Wk, A_Wv,
      A_Wo.reshape(H * E, D), B_w1.reshape(2, D // 2, D), B_w2.reshape(2, D // 2, D), B_w3.reshape(2, D // 2, F),
      B_w4.reshape(2, FH, D), c, w_mod)
    return out.reshape(1, S, D)
```

```python
import functools

import jax
import jax.numpy as jnp
from jax import lax
import jax.experimental.pallas as pl
import jax.experimental.pallas.tpu as pltpu

bf16, f32, u32 = jnp.bfloat16, jnp.float32, jnp.uint32

S, D, H, E, M, SEG, F = 2048, 1024, 32, 128, 8, 32, 3584
NSEG = S // SEG
NP = H // 2
TC = SEG - M
HG = 8
NG = H // HG
TB = 128
NB = S // TB
FH = F // 2
NF = FH // E
G4R = 64
NI = NSEG // 2
NQ = D // E // 2
NC = 3 * NG
BGR = 384
G1R = 48
HD = D // 2
X0 = 4
NR = 2 * (M + SEG)
NO_BOUNDS = True
PIN_ROWS = 256
Y_AT = (0, 7, 14, 21)
G_AT = 2
B_AT = 1
PREP_AT = (0, 1, 3, 4)
PREP_CH = 2
SORD = 0
FINE = 1
JGROUP = 1
P1_TAIL = 5
P1_LAG = 4
SCHED_A = (2, 1, 3)
SCHED_B = (3, 1, 3)
EPS = 1e-5
SCALE = E ** -0.5
_SCOPES = False
_N2 = NSEG // 2


def _scoped(name, fn):
    def wrapped(*a):
        if not _SCOPES:
            return fn(*a)
        with jax.named_scope(name):
            return fn(*a)
    return wrapped


def _pk(x):
    return pltpu.bitcast(x.astype(bf16), u32)


def _up(x):
    return pltpu.bitcast(x, bf16)


def _ct(k):
    return slice(k * E, (k + 1) * E)


def _dot(a, b):
    return jnp.dot(a, b, preferred_element_type=f32)


def _ln(x):
    m = jnp.mean(x, axis=-1, keepdims=True)
    xc = x - m
    v = jnp.mean(xc * xc, axis=-1, keepdims=True)
    return xc * lax.rsqrt(v + EPS)


def _gelu(x):
    c = 0.7978845608028654
    return 0.5 * x * (1.0 + jnp.tanh(c * (x + 0.044715 * (x * x * x))))


def _lhs_set(a11, a12, a21, a22):
    return (a11 + a22, a21 + a22, a11, a22, a11 + a12, a21 - a11, a12 - a22)


def _rhs_set(b11, b12, b21, b22):
    return (b11 + b22, b11, b12 - b22, b21 - b11, b22, b11 + b12, b21 + b22)


def _strassen(m):
    if SORD == 0:
        m1 = m(0)
        m2 = m(1)
        c22 = m1 - m2
        m3 = m(2)
        c22 = c22 + m3
        c22 = m(5) + c22
        m4 = m(3)
        c21 = m2 + m4
        c11 = m1 + m4
        m5 = m(4)
        c12 = m3 + m5
        c11 = c11 - m5
        c11 = m(6) + c11
    else:
        m2 = m(1)
        c22 = m(5) - m2
        m4 = m(3)
        c21 = m2 + m4
        m1 = m(0)
        c22 = c22 + m1
        c11 = m4 + m1
        m3 = m(2)
        c22 = c22 + m3
        m5 = m(4)
        c12 = m3 + m5
        c11 = c11 - m5
        c11 = m(6) + c11
    return c11, c12, c21, c22


def _mask_fill():
    shape = (NR, E)
    r = lax.broadcasted_iota(jnp.int32, shape, 0)
    c = lax.broadcasted_iota(jnp.int32, shape, 1)

    def headpos(i):
        head = jnp.where(i < 64, i >> 5, (i - 64) >> 3)
        pos = jnp.where(i < 64, i & 31, 32 + (i & 7))
        return head, pos

    hr, pr = headpos(r)
    hc, pc = headpos(c)
    same = hr == hc
    valid = same & ((pr < M) | (pr >= pc))
    return jnp.where(valid, 0.0, jnp.where(same, -1e9, -jnp.inf)).astype(f32)


def _kernel(x_hbm, mem0_hbm, wq_hbm, wk_hbm, wv_hbm, wo_hbm, w1_hbm, w2_hbm, w3_hbm,
            w4_hbm, c_hbm, wm_hbm,
            out_hbm,
            x_s, xpre_s, hpre_s, wm_s, stg, w_s, wo_s,
            t1_s, g1, t2_s, t3_s, t4_s, g2, g3, g4, pre_s, mod_s, mem_s, hn_s, aout_s, fill_s,
            x2_s, hb_s, t_s, l1_s, x1_s, base_s, g_s, y_s, u_s, o_s, zero_s, bg, c_s, mem0_s, sems):
    w_hbm = (wq_hbm, wk_hbm, wv_hbm)

    (SEM_C, SEM_MEM, SEM_XPRE, SEM_X, SEM_STG, SEM_BG, SEM_OUT,
     SEM_WMR, SEM_G2, SEM_G3, SEM_G4, SEM_WM, SEM_G1) = (0, 1, 2, 3, 4, 6, 8, 10, 12, 14, 16, 18, 22)

    def copy(src, dst, k):
        return pltpu.make_async_copy(src, dst, sems.at[k])

    def w_copy(t, g, slot):
        return copy(w_hbm[t].at[:, pl.ds(pl.multiple_of(g * HG, HG), HG), :], stg.at[slot],
                    SEM_STG + slot)

    def bg_rows(k):
        return clamp(k * BGR, H * E - BGR), clamp(k * G1R, HD - G1R)

    def bg_copies(k, slot):
        ro, r1 = bg_rows(k)
        return (copy(wo_hbm.at[pl.ds(aligned(ro, 16), BGR)], bg.at[slot], SEM_BG + slot),
                copy(w1_hbm.at[:, pl.ds(aligned(r1, 16), G1R), :], g1.at[slot], SEM_G1 + slot))

    def wm_copy(src_tile, dst_tile, sem):
        return copy(wm_hbm.at[:, pl.ds(aligned(src_tile * E, E), E)], wm_s.at[dst_tile], sem)

    def wm_wait(t0, n, sem):
        copy(wm_s.at[t0:t0 + n], wm_s.at[t0:t0 + n], sem).wait()

    def aligned(x, n):
        return x if isinstance(x, int) else pl.multiple_of(x, n)

    def clamp(k, hi):
        return min(k, hi) if isinstance(k, int) else jnp.minimum(k, hi)

    def mlp_w_copies(k, slot):
        r = pl.ds(aligned(clamp(k, NI - 1) * 16, 16), 16)
        r4 = pl.ds(aligned(clamp(k, FH // G4R - 1) * G4R, 16), G4R)
        return (copy(w2_hbm.at[:, r, :], g2.at[slot], SEM_G2 + slot),
                copy(w3_hbm.at[:, r, :], g3.at[slot], SEM_G3 + slot),
                copy(w4_hbm.at[:, r4, :], g4.at[slot], SEM_G4 + slot))

    def pinned(w, job):
        if job is None:
            return w()
        z = job() & zero_s[...]
        w = w()
        return jnp.concatenate([w[0:8] | z, w[8:]], axis=0)

    def after(x, anchor):
        if anchor is None:
            return x
        z = pltpu.bitcast(pltpu.bitcast(anchor[0:8], u32) & zero_s[...], f32)
        z = jnp.concatenate([z] * (x.shape[0] // 8), axis=0)
        return jnp.concatenate([x[:, 0:E] + z, x[:, E:]], axis=1) if x.shape[1] > E else x + z

    def rhs_job(src, slot, r0, c1, c2, dst, q, row, z=None):
        blk = [src[slot, kh, r0:r0 + 16, cc * E:(cc + 1) * E].astype(f32)
               for kh in range(2) for cc in (c1, c2)]
        if z is not None:
            zf = pltpu.bitcast(jnp.concatenate([z, z], axis=0), f32)
            blk[0] = blk[0] + zf
            blk[3] = blk[3] + zf
        sets = _rhs_set(*blk)
        for n, v in enumerate(sets):
            dst.at[n][pl.ds(pl.multiple_of(row, 8), 8), _ct(q)] = _pk(v)
        out = pltpu.bitcast(sets[2], u32) | pltpu.bitcast(sets[3], u32)
        return out[0:8] | out[8:16]

    def mod_rows(k, n, c0=0, w=D):
        return jnp.concatenate([mod_s[:, k * D + c0:k * D + c0 + w]] * (n // 8), axis=0)

    def tq_place(c, n):
        if n == 1:
            return w_s.at[c], 0, None
        if n == 4:
            return w_s.at[c], D // 4, None
        if n == 6:
            return pre_s.at[c + 1], 0, 0
        k = (0, 2, 3, 5).index(n)
        return w_s.at[c + 2], (k // 2) * (D // 4), (k % 2) * (HG // 2)

    def relayout_jobs(slot, c, i):
        memo = []
        r = aligned(i * 8, 8)

        def job(j, z=None):
            if not memo:
                for d0 in (i * 16, HD + i * 16):
                    memo.append(jnp.swapaxes(pltpu.bitcast(stg[slot, pl.ds(d0, 16)], u32), 0, 1))
            blk = []
            for kh in range(2):
                u = memo[kh][j]
                if z is not None:
                    u = u | jnp.concatenate([z, z], axis=0)
                blk.append(pltpu.bitcast(u << 16, f32))
                blk.append(pltpu.bitcast(u & jnp.uint32(0xFFFF0000), f32))
            for k, v in enumerate(blk):
                w_s.at[c][pl.ds((k // 2) * (D // 4) + r, 8), _ct(2 * j + k % 2)] = _pk(v)
            for n, v in enumerate(_rhs_set(*blk)):
                if n not in (1, 4):
                    ref, r0, c0 = tq_place(c, n)
                    ref[pl.ds(r0 + r, 8), _ct(c0 + j)] = _pk(v)

        return [functools.partial(job, j) for j in range(HG // 2)]

    def repack(slot, row, i, z):
        v = pltpu.bitcast(bg[slot, 16 * i:16 * i + 16, :], u32)
        v = v | jnp.concatenate([z] * (D // E), axis=1)
        wo_s[pl.ds(pl.multiple_of(row + 8 * i, 8), 8), :] = v

    cp_c = copy(c_hbm, c_s, SEM_C)
    cp_mem = copy(mem0_hbm, mem0_s, SEM_MEM)
    cp_xpre = copy(x_hbm.at[:, TC:SEG, :], xpre_s, SEM_XPRE)
    w_copy(0, 0, 0).start()
    cp_xpre.start()
    cp_c.start()
    cp_mem.start()
    for k in range(2 * D // E):
        wm_copy(k, k, SEM_WM + k // 4).start()
    w_copy(0, 1, 1).start()

    zero_s[...] = jnp.zeros(zero_s.shape, u32)
    fill_s[...] = _mask_fill()
    aout_s[...] = jnp.zeros(aout_s.shape, f32)
    l1_s[...] = jnp.zeros(l1_s.shape, u32)
    bg[1] = jnp.zeros(bg.shape[1:], bf16)
    g1[1] = jnp.zeros(g1.shape[1:], bf16)

    w_copy(0, 0, 0).wait()

    def rl0_body(i, carry):
        for job in relayout_jobs(0, 0, i):
            job()
        return carry

    lax.fori_loop(0, D // 32, rl0_body, 0)
    w_copy(0, 2, 0).start()
    for cp in bg_copies(0, 0):
        cp.start()

    cp_xpre.wait()

    def npre_body(i, carry):
        xr = xpre_s[pl.ds(pl.multiple_of(i * 8, 8), 8)].astype(f32).reshape(64, D)
        t_s[pl.ds(pl.multiple_of(i * 64, 64), 64), :] = _ln(xr)
        return carry

    lax.fori_loop(0, NSEG // 8, _scoped("npre", npre_body), 0)

    cp_c.wait()
    cp_mem.wait()
    mem_s[...] = mem0_s[...].astype(f32)
    cf = c_s[...].astype(f32)
    sc = cf * (1.0 / (1.0 + jnp.exp(-cf)))
    sc8 = jnp.broadcast_to(sc, (8, D)).astype(bf16)

    def mod_tiles(t0, n, dst_tile):
        for k in range(n):
            v = _dot(sc8, wm_s[t0 + k])
            if (dst_tile + k) // (D // E) in (1, 4):
                v = 1.0 + v
            mod_s[:, _ct(dst_tile + k)] = v

    for k in range(4):
        wm_wait(4 * k, 4, SEM_WM + k)
        mod_tiles(4 * k, 4, 4 * k)

    PH = NSEG * M // 2

    def hpre_body(i, carry):
        h = [t_s[pl.ds(pl.multiple_of(hf * PH + i * 16, 16), 16), :] * mod_rows(1, 16) + mod_rows(0, 16)
             for hf in range(2)]
        for n, v in enumerate(_lhs_set(h[0][:, :HD], h[0][:, HD:], h[1][:, :HD], h[1][:, HD:])):
            hpre_s.at[n][pl.ds(pl.multiple_of(i * 8, 8), 8), :] = _pk(v)
        return carry

    lax.fori_loop(0, PH // 16, _scoped("hpre", hpre_body), 0)

    t_s[0:8, :] = jnp.zeros((8, D), f32)
    t_s[S + 8:S + 16, :] = jnp.zeros((8, D), f32)

    def modulate_a(xr):
        return _ln(xr) * mod_rows(1, xr.shape[0]) + mod_rows(0, xr.shape[0])

    MB = 64

    def x_copy(k):
        r = slice(0, X0) if k == 0 else slice(X0, NSEG)
        return copy(x_hbm.at[r], x_s.at[r], SEM_XPRE if k == 0 else SEM_X)


    def p1_body(c, carry):
        slot = c & 1
        pslot = 1 - slot
        ro, r1 = bg_rows(jnp.maximum(c - 1, 0))

        @pl.when(c >= 1)
        def _():
            for cp in bg_copies(0, pslot):
                cp.wait()

        @pl.when(c + 1 < NC)
        def _():
            w_copy(0, 0, pslot).wait()

        small = [functools.partial(repack, pslot, ro >> 1, i) for i in range(BGR // 16)]
        small += [functools.partial(rhs_job, g1, pslot, 16 * rt, q, NQ + q, t1_s, q, (r1 >> 1) + 8 * rt)
                  for rt in range(G1R // 16) for q in range(NQ)]
        work = []
        nu = D // 32
        for i in range(nu):
            js = relayout_jobs(pslot, c + 1, i)
            work += [js[k:k + JGROUP] for k in range(0, len(js), JGROUP)]
            work += [[job] for job in small[i * len(small) // nu:(i + 1) * len(small) // nu]]
        npin = 7 * (HG // 2) * (PH // MB)
        jobs = [[] for _ in range(npin)]
        for k, group in enumerate(work):
            pos = k * (npin - P1_TAIL) * 8 // len(work)
            jobs[pos // 8] += [(job, pos % 8 if FINE else 0) for job in group]
        jobs = iter(jobs)

        def prod(n, q, mb):
            ref, r0, c0 = tq_place(c, n)
            w = ref[r0:r0 + D // 4, _ct(2 * q + (n == 4) if c0 is None else c0 + q)]
            m = _dot(_up(hpre_s[n, mb * MB // 2:(mb + 1) * MB // 2, :]), _up(w))
            pending.append(m)
            if len(pending) > P1_LAG:
                anchor = pltpu.bitcast(pending.pop(0), u32)
                for job, g in next(jobs):
                    job(anchor[8 * g:8 * g + 8] & zero_s[...])
            return m

        pending = []
        ns = MB // M
        for q in range(HG // 2):
            for mb in range(PH // MB):
                cs = _strassen(lambda n: prod(n, q, mb))
                for hf in range(2):
                    y = jnp.concatenate([cs[2 * hf + k][sg * M:(sg + 1) * M]
                                         for sg in range(ns) for k in range(2)], axis=0)
                    s0 = hf * (NSEG // 2) + mb * ns
                    pre_s.at[c][s0 * M:(s0 + ns) * M, _ct(q)] = _pk(y)

        for t in range(3):
            @pl.when((c + 3) >> 2 == t)
            def _():
                w_copy(t, (c + 3) & 3, pslot).start()

        @pl.when(c + 2 < NC)
        def _():
            for cp in bg_copies(c + 1, pslot):
                cp.start()

        @pl.when(c < NC - 3)
        def _():
            wm_copy(2 * D // E + c, c, SEM_WMR).start()

        @pl.when(c == NC - 3)
        def _():
            def issue(k, carry2):
                wm_copy(2 * D // E + k, k, SEM_WMR).start()
                return carry2

            x_copy(0).start()
            for k in range(2):
                for cp in mlp_w_copies(k, k):
                    cp.start()
            lax.fori_loop(NC - 3, 3 * D // E, issue, 0)

        return carry

    lax.fori_loop(0, NC, _scoped("p1", p1_body), 0)
    x_copy(1).start()
    x_copy(0).wait()
    wm_wait(0, 3 * D // E, SEM_WMR)
    mod_tiles(0, 3 * D // E, 2 * D // E)
    for k in range(D // E):
        wm_copy(5 * D // E + k, k, SEM_WM).start()

    def h_rows(s):
        return modulate_a(x_s[s, 0:TC, :].astype(f32))

    hn_s[...] = h_rows(0)

    def chain_step(s, mem, htok, odef_prev, jobs=(), hooks=None):
        hs = jnp.concatenate([mem, htok], axis=0).astype(bf16)
        qkv = [[None] * 3 for _ in range(NP)]
        ps = [None] * NP
        os_ = [None] * H
        odef = [None] * H

        def proj(p, ts=(0, 1, 2)):
            for t in ts:
                c, q = t * NG + p // (HG // 2), p % (HG // 2)
                a = _dot(hs, _up(w_s[c, :, _ct(2 * q)]))
                b = _dot(hs, _up(w_s[c, :, _ct(2 * q + 1)]))
                if hooks and t == 2 and p - NP in hooks:
                    hooks[p - NP](b)
                pre = pre_s[c, pl.ds(pl.multiple_of(s * M, M), M), _ct(q)]
                if t == 1:
                    kf = jnp.concatenate([a, b, _up(pre).astype(f32), jnp.zeros((E - NR, E), f32)],
                                         axis=0)
                    qkv[p][t] = kf.T.astype(bf16)
                    continue
                parts = [_pk(a), _pk(b), pre]
                if t == 2:
                    parts.append(jnp.zeros(((E - NR) // 2, E), u32))
                qkv[p][t] = _up(jnp.concatenate(parts, axis=0))

        def scores(p):
            sc_ = _dot(qkv[p][0], qkv[p][1])
            fill = fill_s[...]
            sc_ = jnp.where(fill == 0.0, sc_ * SCALE, fill)
            m = jnp.max(sc_, axis=-1, keepdims=True)
            e = jnp.exp(sc_ - m)
            l = jnp.sum(e, axis=-1, keepdims=True)
            r = pl.reciprocal(l, approx=True)
            r = r * (2.0 - l * r)
            ps[p] = (e * r).astype(bf16)

        def fin(p):
            o = _dot(ps[p], qkv[p][2])
            for hh in range(2):
                h = 2 * p + hh
                rows = o[32 * hh:32 * hh + 32]
                odef[h] = o[64 + 8 * hh:72 + 8 * hh]
                if odef_prev is not None:
                    rows = jnp.concatenate([rows, odef_prev[h], odef[h]], axis=0)
                os_[h] = _pk(rows)

        acc = [None] * 8
        jobs = iter(jobs)

        def wo(h0, h1, js):
            lhs = _up(jnp.concatenate(os_[h0:h1], axis=1))
            for j in js:
                ws = []
                for r0 in range(h0 * E // 2, h1 * E // 2, PIN_ROWS):
                    ws.append(pinned(lambda: wo_s[r0:r0 + PIN_ROWS, j * E:(j + 1) * E],
                                     next(jobs, None)))
                part = _dot(lhs, _up(jnp.concatenate(ws, axis=0)))
                if hooks and acc[j] is None and j in hooks:
                    hooks[j](part)
                acc[j] = part if acc[j] is None else part + acc[j]

        ORDER, LAG_S, LAG_O = SCHED_A if odef_prev is None else SCHED_B
        for p in range(NP):
            if ORDER == 0:
                proj(p)
                if p >= LAG_S:
                    scores(p - LAG_S)
                if p >= LAG_O:
                    fin(p - LAG_O)
            elif ORDER == 1:
                proj(p, (1, 0))
                if p >= LAG_O:
                    fin(p - LAG_O)
                proj(p, (2,))
                if p >= LAG_S:
                    scores(p - LAG_S)
            elif ORDER == 2:
                proj(p, (1,))
                if p >= LAG_S:
                    scores(p - LAG_S)
                proj(p, (0,))
                if p >= LAG_O:
                    fin(p - LAG_O)
                proj(p, (2,))
            elif ORDER == 3:
                proj(p, (1,))
                if p >= LAG_O:
                    fin(p - LAG_O)
                proj(p, (0,))
                if p >= LAG_S:
                    scores(p - LAG_S)
                proj(p, (2,))
            elif ORDER == 4:
                proj(p, (1,))
                if p >= LAG_S:
                    scores(p - LAG_S)
                proj(p, (0, 2))
                if p >= LAG_O:
                    fin(p - LAG_O)
            else:
                proj(p, (0,))
                if p >= LAG_S:
                    scores(p - LAG_S)
                proj(p, (1,))
                if p >= LAG_O:
                    fin(p - LAG_O)
                proj(p, (2,))
        tail = []
        for k in range(LAG_O):
            step = []
            if NP - LAG_S + k < NP:
                step.append(functools.partial(scores, NP - LAG_S + k))
            step.append(functools.partial(fin, NP - LAG_O + k))
            tail.append(step)
        hsplit = min(24, 2 * (NP - LAG_O))
        cuts = {3: (2, 3, 5), 2: (2, 5), 4: (1, 2, 4, 6), 5: (1, 2, 3, 4, 6)}[LAG_O]
        j0 = 0
        for k, step in enumerate(tail):
            wo(0, hsplit, range(j0, cuts[k]))
            j0 = cuts[k]
            for f in step:
                f()
        wo(0, hsplit, range(j0, 8))
        wo(hsplit, H, range(8))
        return jnp.concatenate(acc, axis=1), odef

    def mixer_prep(i, r0, n, anchor=None):
        r = pl.ds(aligned(i * 64 + r0, 16), n)
        xr = x_s[2 * i + r0 // SEG, r0 % SEG:r0 % SEG + n, :].astype(f32)
        x2 = xr + mod_rows(2, n) * after(aout_s[r0:r0 + n, :], anchor)
        x2_s[r, :] = x2.astype(bf16)
        hb = _ln(x2) * mod_rows(4, n) + mod_rows(3, n)
        hb_s[r, :] = hb.astype(bf16)
        return _ln(hb)

    def mixer_sets(ya, yb, r0):
        n = ya.shape[0]
        for m, v in enumerate(_lhs_set(ya[:, :HD], ya[:, HD:], yb[:, :HD], yb[:, HD:])):
            l1_s.at[m][r0 // 2:(r0 + n) // 2, :] = _pk(v)

    def mixer_mm(i):
        for q in range(NQ):
            cs = _strassen(lambda n: _dot(_up(l1_s[n]), _up(t1_s[n, :, _ct(q)])))
            for k, cc in enumerate(cs):
                r0 = aligned(i * 64 + 8 + (k // 2) * SEG, 8)
                t_s[pl.ds(r0, SEG), _ct(q + NQ * (k % 2))] = _gelu(cc)

    def p2_body(i, carry):
        slot = i & 1
        for cp in mlp_w_copies(0, slot):
            cp.wait()

        @pl.when(i == 1)
        def _():
            x_copy(1).wait()

        work = [functools.partial(rhs_job, g3, slot, 0, q, NF + q, t3_s, q, i * 8)
                for q in range(NF)]
        work += [functools.partial(rhs_job, g2, slot, 0, 2 * q, 2 * q + 1, t2_s, q, i * 8)
                 for q in range(NQ)]
        row4 = clamp(i, FH // G4R - 1) * (G4R // 2)
        work += [functools.partial(rhs_job, g4, slot, 16 * rt, 2 * q, 2 * q + 1, t4_s, q, row4 + 8 * rt)
                 for rt in range(G4R // 16) for q in range(NQ)]
        npin = 60
        jobs = [None] * npin
        for k, job in enumerate(work):
            jobs[1 + k * (npin - 1) // len(work)] = job

        sa_ = 2 * i
        sb_ = 2 * i + 1
        hb_tok = h_rows(sb_)
        oa, odef_a = chain_step(sa_, mem_s[...], hn_s[...], None)
        mixer_mm(jnp.maximum(i - 2, 0))
        ys = []

        def hook(k, anchor):
            if k >= PREP_CH:
                anchor = anchor[0:8] + ys[-PREP_CH][0:8, 0:E] + ys[-PREP_CH][8:16, 0:E]
            ys.append(mixer_prep(jnp.maximum(i - 1, 0), (k % 2) * SEG + (k // 2) * 16, 16, anchor))
            if k % 2:
                mixer_sets(ys[-2], ys[-1], (k // 2) * 16)

        hooks = {j: functools.partial(hook, k) for k, j in enumerate(PREP_AT)}
        ob, _ = chain_step(sb_, oa[0:M], hb_tok, odef_a, jobs, hooks)
        mem_s[...] = ob[0:M]
        aout_s[0:TC, :] = oa[M:SEG]
        aout_s[TC:SEG, :] = ob[SEG:SEG + M]
        aout_s[SEG:SEG + TC, :] = ob[M:SEG]
        aout_s[SEG + TC:2 * SEG, :] = ob[SEG + M:SEG + 2 * M]
        hn_s[...] = h_rows(jnp.minimum(sb_ + 1, NSEG - 1))
        for cp in mlp_w_copies(i + 2, slot):
            cp.start()
        return carry

    lax.fori_loop(0, _N2, _scoped("p2", p2_body), 0)

    TH = TB // 2
    SHIFT = (-1, -1, 1, 1, -2, -2, 2, 2)

    def g_job(j, rt, q, n=16, anchor=None):
        blk = []
        for hf in range(2):
            for ct in (q, NQ + q):
                win = t_s[pl.ds(aligned(j * TB + hf * TH + rt * n, 16), n + 16), ct * E:(ct + 1) * E]
                blk.append(win[8 + SHIFT[ct]:8 + SHIFT[ct] + n])
        blk[0] = after(blk[0], anchor)
        blk[3] = after(blk[3], anchor)
        for k, v in enumerate(_lhs_set(*blk)):
            g_s.at[k][rt * n // 2:(rt + 1) * n // 2, q * E:(q + 1) * E] = _pk(v)

    def mix(j):
        r0 = aligned(j * TB, TB)
        for q in range(NQ):
            cs = _strassen(lambda n: _dot(_up(g_s[n]), _up(t2_s[n, :, _ct(q)])))
            cols = slice(2 * q * E, (2 * q + 2) * E)
            for hf in range(2):
                x1_s[hf * TH:(hf + 1) * TH, cols] = (
                    hb_s[pl.ds(r0 + hf * TH, TH), cols].astype(f32)
                    + jnp.concatenate(cs[2 * hf:2 * hf + 2], axis=1))

    def base_job(j, rt, anchor):
        rows = slice(rt * 16, (rt + 1) * 16)
        z = pltpu.bitcast(pltpu.bitcast(anchor[0:8], u32) & zero_s[...], f32)
        gb = mod_rows(5, 8) + jnp.concatenate([z] * (D // E), axis=1)
        base_s[rows, :] = (x2_s[pl.ds(aligned(j * TB + rt * 16, 16), 16), :].astype(f32)
                           + jnp.concatenate([gb, gb], axis=0) * x1_s[rows, :])

    def out_copy(j, slot):
        return copy(o_s.at[slot], out_hbm.at[pl.ds(aligned(j * TB, TB), TB)], SEM_OUT + slot)

    prev_y = [None]

    def put_y(rt=0, n=TH, anchor=None):
        if anchor is not None and rt > 0:
            anchor = anchor[0:8] + prev_y[0]
        ya = _ln(after(x1_s[rt * n:(rt + 1) * n, :], anchor))
        yb = _ln(after(x1_s[TH + rt * n:TH + (rt + 1) * n, :], anchor))
        sets = _lhs_set(ya[:, :HD], ya[:, HD:], yb[:, :HD], yb[:, HD:])
        prev_y[0] = sets[0][0:8, 0:E] + sets[0][8:16, 0:E]
        for k, v in enumerate(sets):
            y_s.at[k][rt * n // 2:(rt + 1) * n // 2, :] = _pk(v)

    wm_wait(0, D // E, SEM_WM)
    mod_tiles(0, D // E, 5 * D // E)
    mixer_mm(NI - 2)
    mixer_sets(mixer_prep(NI - 1, 0, SEG), mixer_prep(NI - 1, SEG, SEG), 0)
    for q in range(NQ):
        g_job(0, 0, q, TH)
    mix(0)
    mixer_mm(NI - 1)
    put_y()
    for q in range(NQ):
        g_job(1, 0, q, TH)

    def mlp_block(j, last):
        slot = j & 1
        for q in range(NF):
            cs = _strassen(lambda n: _dot(_up(y_s[n]), _up(t3_s[n, :, _ct(q)])))
            if 0 <= q - B_AT < TB // 16:
                base_job(j, q - B_AT, cs[0])
            for n, v in enumerate(_lhs_set(*[_gelu(cc) for cc in cs])):
                u_s.at[n][:, q * E:(q + 1) * E] = _pk(v)
        jobs = {}
        if not last:
            mix(j + 1)
            jn = clamp(j + 2, NB - 1)
            for rt in range(TH // 16):
                jobs[Y_AT[rt]] = functools.partial(put_y, rt, 16)
            free = [k for k in range(G_AT, 7 * NQ) if k not in jobs]
            for k in range(TH // 16 * NQ):
                jobs[free[k]] = functools.partial(g_job, jn, k // NQ, k % NQ, 16)

        def prod(n, q):
            m = _dot(_up(u_s[n]), _up(t4_s[n, :, _ct(q)]))
            job = jobs.get(count[0])
            count[0] += 1
            if job is not None:
                job(anchor=m)
            return m

        count = [0]
        for q in range(NQ):
            if last and q == 0:
                ks = FH - 2 * E
                head = [_dot(_up(u_s[n, :, 0:ks]), _up(t4_s[n, 0:ks // 2, _ct(q)])) for n in range(7)]
                cs = _strassen(lambda n: _dot(_up(u_s[n, :, ks:FH]), _up(t4_s[n, ks // 2:, _ct(q)]))
                               + head[n])
            else:
                cs = _strassen(lambda n: prod(n, q))
            cols = slice(2 * q * E, (2 * q + 2) * E)
            for hf in range(2):
                rows = slice(hf * TH, (hf + 1) * TH)
                o_s.at[slot][rows, cols] = (
                    base_s[rows, cols] + mod_rows(5, TH, 2 * q * E, 2 * E)
                    * jnp.concatenate(cs[2 * hf:2 * hf + 2], axis=1)).astype(bf16)
        out_copy(j, slot).start()

    def p3_body(j, carry):
        @pl.when(j >= 2)
        def _():
            out_copy(j - 2, j & 1).wait()

        mlp_block(j, False)
        return carry

    lax.fori_loop(0, NB - 1, _scoped("p3", p3_body), 0)
    for k in range(2):
        for cp in mlp_w_copies(0, k):
            cp.wait()
    out_copy(NB - 3, (NB - 3) % 2).wait()
    mlp_block(NB - 1, True)
    out_copy(NB - 2, (NB - 2) % 2).wait()
    out_copy(NB - 1, (NB - 1) % 2).wait()


@jax.jit
def pallas_adaLN_cond__memory_aug_recurrent_mem_tr__mixer_s_mlp__prompt_kernel(
    A_x: jax.Array,
    A_mem0: jax.Array,
    A_Wq: jax.Array,
    A_Wk: jax.Array,
    A_Wv: jax.Array,
    A_Wo: jax.Array,
    A_seg_len,
    B_x: jax.Array,
    B_w1: jax.Array,
    B_w2: jax.Array,
    B_w3: jax.Array,
    B_w4: jax.Array,
    c: jax.Array,
    w_mod: jax.Array,
):
    del A_seg_len, B_x
    assert A_x.shape == (1, S, D) and A_mem0.shape == (1, M, D)
    hbm = pl.BlockSpec(memory_space=pl.ANY)
    scratch = [
        pltpu.VMEM((NSEG, SEG, D), bf16),
        pltpu.VMEM((NSEG, M, D), bf16),
        pltpu.VMEM((7, NSEG * M // 4, D // 2), u32),
        pltpu.VMEM((3 * D // E, D, E), bf16),
        pltpu.VMEM((2, D, HG, E), bf16),
        pltpu.VMEM((NC + 3, D // 2, HG * E), u32),
        pltpu.VMEM((H * E // 2, D), u32),
        pltpu.VMEM((7, D // 4, D // 2), u32),
        pltpu.VMEM((2, 2, G1R, D), bf16),
        pltpu.VMEM((7, D // 4, D // 2), u32),
        pltpu.VMEM((7, D // 4, FH), u32),
        pltpu.VMEM((7, FH // 2, D // 2), u32),
        pltpu.VMEM((2, 2, 16, D), bf16),
        pltpu.VMEM((2, 2, 16, F), bf16),
        pltpu.VMEM((2, 2, G4R, D), bf16),
        pltpu.VMEM((NC + 2, NSEG * M, HG // 2 * E), u32),
        pltpu.VMEM((8, 6 * D), f32),
        pltpu.VMEM((M, D), f32),
        pltpu.VMEM((TC, D), f32),
        pltpu.VMEM((2 * SEG, D), f32),
        pltpu.VMEM((NR, E), f32),
        pltpu.VMEM((S, D), bf16),
        pltpu.VMEM((S, D), bf16),
        pltpu.VMEM((S + 16, D), f32),
        pltpu.VMEM((7, SEG // 2, D // 2), u32),
        pltpu.VMEM((TB, D), f32),
        pltpu.VMEM((TB, D), f32),
        pltpu.VMEM((7, TB // 4, D // 2), u32),
        pltpu.VMEM((7, TB // 4, D // 2), u32),
        pltpu.VMEM((7, TB // 4, FH), u32),
        pltpu.VMEM((2, TB, D), bf16),
        pltpu.VMEM((8, E), u32),
        pltpu.VMEM((2, BGR, D), bf16),
        pltpu.VMEM((1, D), bf16),
        pltpu.VMEM((M, D), bf16),
        pltpu.SemaphoreType.DMA((24,)),
    ]
    out = pl.pallas_call(
        _kernel,
        out_shape=jax.ShapeDtypeStruct((S, D), bf16),
        in_specs=[hbm] * 12,
        out_specs=hbm,
        scratch_shapes=scratch,
        compiler_params=pltpu.CompilerParams(vmem_limit_bytes=126 * 1024 * 1024,
                                             disable_bounds_checks=NO_BOUNDS),
    )(A_x.reshape(NSEG, SEG, D), A_mem0.reshape(M, D), A_Wq, A_Wk, A_Wv,
      A_Wo.reshape(H * E, D), B_w1.reshape(2, D // 2, D), B_w2.reshape(2, D // 2, D), B_w3.reshape(2, D // 2, F),
      B_w4.reshape(2, FH, D), c, w_mod)
    return out.reshape(1, S, D)
```

```python
import functools

import jax
import jax.numpy as jnp
from jax import lax
import jax.experimental.pallas as pl
import jax.experimental.pallas.tpu as pltpu

bf16, f32, u32 = jnp.bfloat16, jnp.float32, jnp.uint32

S, D, H, E, M, SEG, F = 2048, 1024, 32, 128, 8, 32, 3584
NSEG = S // SEG
NP = H // 2
TC = SEG - M
HG = 8
NG = H // HG
TB = 128
NB = S // TB
NFG = F // (4 * E)
NOG = D // (4 * E)
NI = NSEG // 2
NQ = D // E // 2
NC = 3 * NG
BGR = 384
G1R = 48
HD = D // 2
X0 = 4
NR = 2 * (M + SEG)
NO_BOUNDS = True
PIN_ROWS = 256
Y_AT = 4
S_AT = (26, 44)
G_AT = 62
HEAD = 14
PREP_AT = (0, 1, 3, 4)
PREP_CH = 2
SORD = 0
FINE = 1
JGROUP = 1
P1_TAIL = 5
P1_LAG = 4
SCHED_A = (2, 1, 3)
SCHED_B = (3, 1, 3)
EPS = 1e-5
SCALE = E ** -0.5
_SCOPES = False
_N2 = NSEG // 2


def _scoped(name, fn):
    def wrapped(*a):
        if not _SCOPES:
            return fn(*a)
        with jax.named_scope(name):
            return fn(*a)
    return wrapped


def _pk(x):
    return pltpu.bitcast(x.astype(bf16), u32)


def _up(x):
    return pltpu.bitcast(x, bf16)


def _ct(k):
    return slice(k * E, (k + 1) * E)


def _dot(a, b):
    return jnp.dot(a, b, preferred_element_type=f32)


def _ln(x):
    m = jnp.mean(x, axis=-1, keepdims=True)
    xc = x - m
    v = jnp.mean(xc * xc, axis=-1, keepdims=True)
    return xc * lax.rsqrt(v + EPS)


def _gelu(x):
    c = 0.7978845608028654
    return 0.5 * x * (1.0 + jnp.tanh(c * (x + 0.044715 * (x * x * x))))


def _lhs_set(a11, a12, a21, a22):
    return (a11 + a22, a21 + a22, a11, a22, a11 + a12, a21 - a11, a12 - a22)


def _rhs_set(b11, b12, b21, b22):
    return (b11 + b22, b11, b12 - b22, b21 - b11, b22, b11 + b12, b21 + b22)


_LHS_TERMS = (((0, 1), (3, 1)), ((2, 1), (3, 1)), ((0, 1),), ((3, 1),),
              ((0, 1), (1, 1)), ((2, 1), (0, -1)), ((1, 1), (3, -1)))
_RHS_TERMS = (((0, 1), (3, 1)), ((0, 1),), ((1, 1), (3, -1)), ((2, 1), (0, -1)),
              ((3, 1),), ((0, 1), (1, 1)), ((2, 1), (3, 1)))


def _outer_operand(tile, terms):
    out = []
    for i in range(2):
        for j in range(2):
            v = None
            for o, sign in terms:
                t = tile(2 * (o // 2) + i, 2 * (o % 2) + j)
                v = t if v is None else (v + t if sign > 0 else v - t)
            out.append(v)
    return out


class _Quad:
    def __init__(self, tiles):
        self.t = tuple(tiles)

    def __add__(self, other):
        return _Quad([a + b for a, b in zip(self.t, other.t)])

    def __sub__(self, other):
        return _Quad([a - b for a, b in zip(self.t, other.t)])


def _strassen2(m):
    cs = _strassen(lambda n1: _Quad(_strassen(lambda n2: m(7 * n1 + n2))))
    return lambda i, j: cs[2 * (i // 2) + j // 2].t[2 * (i % 2) + j % 2]


def _strassen(m):
    if SORD == 0:
        m1 = m(0)
        m2 = m(1)
        c22 = m1 - m2
        m3 = m(2)
        c22 = c22 + m3
        c22 = m(5) + c22
        m4 = m(3)
        c21 = m2 + m4
        c11 = m1 + m4
        m5 = m(4)
        c12 = m3 + m5
        c11 = c11 - m5
        c11 = m(6) + c11
    else:
        m2 = m(1)
        c22 = m(5) - m2
        m4 = m(3)
        c21 = m2 + m4
        m1 = m(0)
        c22 = c22 + m1
        c11 = m4 + m1
        m3 = m(2)
        c22 = c22 + m3
        m5 = m(4)
        c12 = m3 + m5
        c11 = c11 - m5
        c11 = m(6) + c11
    return c11, c12, c21, c22


def _mask_fill():
    shape = (NR, E)
    r = lax.broadcasted_iota(jnp.int32, shape, 0)
    c = lax.broadcasted_iota(jnp.int32, shape, 1)

    def headpos(i):
        head = jnp.where(i < 64, i >> 5, (i - 64) >> 3)
        pos = jnp.where(i < 64, i & 31, 32 + (i & 7))
        return head, pos

    hr, pr = headpos(r)
    hc, pc = headpos(c)
    same = hr == hc
    valid = same & ((pr < M) | (pr >= pc))
    return jnp.where(valid, 0.0, jnp.where(same, -1e9, -jnp.inf)).astype(f32)


def _kernel(x_hbm, mem0_hbm, wq_hbm, wk_hbm, wv_hbm, wo_hbm, w1_hbm, w2_hbm, w3_hbm,
            w4_hbm, c_hbm, wm_hbm,
            out_hbm,
            x_s, w_s, wo_s, t1_s, g2, g3, g4, pre_s, mod_s, mem_s, hn_s, aout_s, fill_s,
            hb_s, t_s, l1_s, zero_s, c_s, mem0_s, sems):
    w_hbm = (wq_hbm, wk_hbm, wv_hbm)

    (SEM_C, SEM_MEM, SEM_XPRE, SEM_X, SEM_STG, SEM_BG, SEM_OUT,
     SEM_WMR, SEM_G2, SEM_G3, SEM_G4, SEM_WM, SEM_G1) = (0, 1, 2, 3, 4, 6, 8, 10, 12, 14, 16, 18, 22)

    def copy(src, dst, k):
        return pltpu.make_async_copy(src, dst, sems.at[k])

    def aligned(x, n):
        return x if isinstance(x, int) else pl.multiple_of(x, n)

    def clamp(k, hi):
        return min(k, hi) if isinstance(k, int) else jnp.minimum(k, hi)

    def mlp_piece(k):
        k = clamp(k, 4 * NFG - 1)
        return k >> 2, k & 3

    def mlp_w_copies(k, slot):
        g, rr = mlp_piece(k)
        r = pl.ds(aligned(clamp(k, NI - 1) * 16, 16), 16)
        return (copy(w2_hbm.at[:, r, :], g2.at[slot], SEM_G2 + slot),
                copy(w3_hbm.at[:, pl.ds(aligned(rr * 64, 64), 64), pl.ds(aligned(g * 4 * E, E), 4 * E)],
                     g3.at[slot], SEM_G3 + slot),
                copy(w4_hbm.at[g, :, pl.ds(aligned(rr * 32, 32), 32), :], g4.at[slot], SEM_G4 + slot))

    def pinned(w, job):
        if job is None:
            return w()
        z = job() & zero_s[...]
        w = w()
        return jnp.concatenate([w[0:8] | z, w[8:]], axis=0)

    def after(x, anchor):
        if anchor is None:
            return x
        z = pltpu.bitcast(pltpu.bitcast(anchor[0:8], u32) & zero_s[...], f32)
        z = jnp.concatenate([z] * (x.shape[0] // 8), axis=0)
        return jnp.concatenate([x[:, 0:E] + z, x[:, E:]], axis=1) if x.shape[1] > E else x + z

    def rhs_job(src, slot, r0, c1, c2, dst, q, row, z=None):
        blk = [src[slot, kh, r0:r0 + 16, cc * E:(cc + 1) * E].astype(f32)
               for kh in range(2) for cc in (c1, c2)]
        if z is not None:
            zf = pltpu.bitcast(jnp.concatenate([z, z], axis=0), f32)
            blk[0] = blk[0] + zf
            blk[3] = blk[3] + zf
        sets = _rhs_set(*blk)
        for n, v in enumerate(sets):
            dst.at[n][pl.ds(pl.multiple_of(row, 8), 8), _ct(q)] = _pk(v)
        out = pltpu.bitcast(sets[2], u32) | pltpu.bitcast(sets[3], u32)
        return out[0:8] | out[8:16]

    def rhs2_job(src, slot, r0, c0, n1, dst, row):
        blk = _outer_operand(lambda i, j: src[slot, i, r0:r0 + 16, _ct(c0 + j)].astype(f32),
                             _RHS_TERMS[n1])
        sets = _rhs_set(*blk)
        for n2, v in enumerate(sets):
            dst[pl.ds(pl.multiple_of(row, 8), 8), _ct(7 * n1 + n2)] = _pk(v)
        out = pltpu.bitcast(sets[2], u32) | pltpu.bitcast(sets[3], u32)
        return out[0:8] | out[8:16]

    def silu_c():
        cf = c_s[...].astype(f32)
        return jnp.broadcast_to(cf * (1.0 / (1.0 + jnp.exp(-cf))), (8, D)).astype(bf16)

    def wm_copy(wm_s, src_tile, dst_tile, sem):
        return copy(wm_hbm.at[:, pl.ds(aligned(src_tile * E, E), E)], wm_s.at[dst_tile], sem)

    def wm_wait(wm_s, t0, n, sem):
        copy(wm_s.at[t0:t0 + n], wm_s.at[t0:t0 + n], sem).wait()

    def mod_tiles(wm_s, t0, n, dst_tile):
        sc8 = silu_c()
        for k in range(n):
            v = _dot(sc8, wm_s[t0 + k])
            if (dst_tile + k) // (D // E) in (1, 4):
                v = 1.0 + v
            mod_s[:, _ct(dst_tile + k)] = v

    def x_copy(k):
        r = slice(0, X0) if k == 0 else slice(X0, NSEG)
        return copy(x_hbm.at[r], x_s.at[r], SEM_XPRE if k == 0 else SEM_X)

    def h_rows(s):
        return _ln(x_s[s, 0:TC, :].astype(f32)) * mod_rows(1, TC) + mod_rows(0, TC)

    def mod_rows(k, n, c0=0, w=D):
        return jnp.concatenate([mod_s[:, k * D + c0:k * D + c0 + w]] * (n // 8), axis=0)

    def tq_place(c, n):
        if n == 1:
            return w_s.at[c], 0, None
        if n == 4:
            return w_s.at[c], D // 4, None
        if n == 6:
            return pre_s.at[c + 1], 0, 0
        k = (0, 2, 3, 5).index(n)
        return w_s.at[c + 2], (k // 2) * (D // 4), (k % 2) * (HG // 2)

    def phase_a(xpre_s, hpre_s, wm_s, stg, bg, g1):
        def w_copy(t, g, slot):
            return copy(w_hbm[t].at[:, pl.ds(pl.multiple_of(g * HG, HG), HG), :], stg.at[slot],
                        SEM_STG + slot)

        def bg_rows(k):
            return clamp(k * BGR, H * E - BGR), clamp(k * G1R, HD - G1R)

        def bg_copies(k, slot):
            ro, r1 = bg_rows(k)
            return (copy(wo_hbm.at[pl.ds(aligned(ro, 16), BGR)], bg.at[slot], SEM_BG + slot),
                    copy(w1_hbm.at[:, pl.ds(aligned(r1, 16), G1R), :], g1.at[slot], SEM_G1 + slot))

        def relayout_jobs(slot, c, i):
            memo = []
            r = aligned(i * 8, 8)

            def job(j, z=None):
                if not memo:
                    for d0 in (i * 16, HD + i * 16):
                        memo.append(jnp.swapaxes(pltpu.bitcast(stg[slot, pl.ds(d0, 16)], u32), 0, 1))
                blk = []
                for kh in range(2):
                    u = memo[kh][j]
                    if z is not None:
                        u = u | jnp.concatenate([z, z], axis=0)
                    blk.append(pltpu.bitcast(u << 16, f32))
                    blk.append(pltpu.bitcast(u & jnp.uint32(0xFFFF0000), f32))
                for k, v in enumerate(blk):
                    w_s.at[c][pl.ds((k // 2) * (D // 4) + r, 8), _ct(2 * j + k % 2)] = _pk(v)
                for n, v in enumerate(_rhs_set(*blk)):
                    if n not in (1, 4):
                        ref, r0, c0 = tq_place(c, n)
                        ref[pl.ds(r0 + r, 8), _ct(c0 + j)] = _pk(v)

            return [functools.partial(job, j) for j in range(HG // 2)]

        def repack(slot, row, i, z):
            v = pltpu.bitcast(bg[slot, 16 * i:16 * i + 16, :], u32)
            v = v | jnp.concatenate([z] * (D // E), axis=1)
            wo_s[pl.ds(pl.multiple_of(row + 8 * i, 8), 8), :] = v

        cp_c = copy(c_hbm, c_s, SEM_C)
        cp_mem = copy(mem0_hbm, mem0_s, SEM_MEM)
        cp_xpre = copy(x_hbm.at[:, TC:SEG, :], xpre_s, SEM_XPRE)
        w_copy(0, 0, 0).start()
        cp_xpre.start()
        cp_c.start()
        cp_mem.start()
        for k in range(2 * D // E):
            wm_copy(wm_s, k, k, SEM_WM + k // 4).start()
        w_copy(0, 1, 1).start()

        zero_s[...] = jnp.zeros(zero_s.shape, u32)
        fill_s[...] = _mask_fill()
        aout_s[...] = jnp.zeros(aout_s.shape, f32)
        l1_s[...] = jnp.zeros(l1_s.shape, u32)
        bg[1] = jnp.zeros(bg.shape[1:], bf16)
        g1[1] = jnp.zeros(g1.shape[1:], bf16)

        w_copy(0, 0, 0).wait()

        def rl0_body(i, carry):
            for job in relayout_jobs(0, 0, i):
                job()
            return carry

        lax.fori_loop(0, D // 32, rl0_body, 0)
        w_copy(0, 2, 0).start()
        for cp in bg_copies(0, 0):
            cp.start()

        cp_xpre.wait()

        def npre_body(i, carry):
            xr = xpre_s[pl.ds(pl.multiple_of(i * 8, 8), 8)].astype(f32).reshape(64, D)
            t_s[pl.ds(pl.multiple_of(i * 64, 64), 64), :] = _ln(xr)
            return carry

        lax.fori_loop(0, NSEG // 8, _scoped("npre", npre_body), 0)

        cp_c.wait()
        cp_mem.wait()
        mem_s[...] = mem0_s[...].astype(f32)

        for k in range(4):
            wm_wait(wm_s, 4 * k, 4, SEM_WM + k)
            mod_tiles(wm_s, 4 * k, 4, 4 * k)

        PH = NSEG * M // 2

        def hpre_body(i, carry):
            h = [t_s[pl.ds(pl.multiple_of(hf * PH + i * 16, 16), 16), :] * mod_rows(1, 16) + mod_rows(0, 16)
                 for hf in range(2)]
            for n, v in enumerate(_lhs_set(h[0][:, :HD], h[0][:, HD:], h[1][:, :HD], h[1][:, HD:])):
                hpre_s.at[n][pl.ds(pl.multiple_of(i * 8, 8), 8), :] = _pk(v)
            return carry

        lax.fori_loop(0, PH // 16, _scoped("hpre", hpre_body), 0)

        t_s[0:8, :] = jnp.zeros((8, D), f32)
        t_s[S + 8:S + 16, :] = jnp.zeros((8, D), f32)

        MB = 64

        def p1_body(c, carry):
            slot = c & 1
            pslot = 1 - slot
            ro, r1 = bg_rows(jnp.maximum(c - 1, 0))

            @pl.when(c >= 1)
            def _():
                for cp in bg_copies(0, pslot):
                    cp.wait()

            @pl.when(c + 1 < NC)
            def _():
                w_copy(0, 0, pslot).wait()

            small = [functools.partial(repack, pslot, ro >> 1, i) for i in range(BGR // 16)]
            small += [functools.partial(rhs_job, g1, pslot, 16 * rt, q, NQ + q, t1_s, q, (r1 >> 1) + 8 * rt)
                      for rt in range(G1R // 16) for q in range(NQ)]
            work = []
            nu = D // 32
            for i in range(nu):
                js = relayout_jobs(pslot, c + 1, i)
                work += [js[k:k + JGROUP] for k in range(0, len(js), JGROUP)]
                work += [[job] for job in small[i * len(small) // nu:(i + 1) * len(small) // nu]]
            npin = 7 * (HG // 2) * (PH // MB)
            jobs = [[] for _ in range(npin)]
            for k, group in enumerate(work):
                pos = k * (npin - P1_TAIL) * 8 // len(work)
                jobs[pos // 8] += [(job, pos % 8 if FINE else 0) for job in group]
            jobs = iter(jobs)

            def prod(n, q, mb):
                ref, r0, c0 = tq_place(c, n)
                w = ref[r0:r0 + D // 4, _ct(2 * q + (n == 4) if c0 is None else c0 + q)]
                m = _dot(_up(hpre_s[n, mb * MB // 2:(mb + 1) * MB // 2, :]), _up(w))
                pending.append(m)
                if len(pending) > P1_LAG:
                    anchor = pltpu.bitcast(pending.pop(0), u32)
                    for job, g in next(jobs):
                        job(anchor[8 * g:8 * g + 8] & zero_s[...])
                return m

            pending = []
            ns = MB // M
            for q in range(HG // 2):
                for mb in range(PH // MB):
                    cs = _strassen(lambda n: prod(n, q, mb))
                    for hf in range(2):
                        y = jnp.concatenate([cs[2 * hf + k][sg * M:(sg + 1) * M]
                                             for sg in range(ns) for k in range(2)], axis=0)
                        s0 = hf * (NSEG // 2) + mb * ns
                        pre_s.at[c][s0 * M:(s0 + ns) * M, _ct(q)] = _pk(y)

            for t in range(3):
                @pl.when((c + 3) >> 2 == t)
                def _():
                    w_copy(t, (c + 3) & 3, pslot).start()

            @pl.when(c + 2 < NC)
            def _():
                for cp in bg_copies(c + 1, pslot):
                    cp.start()

            @pl.when(c < NC - 3)
            def _():
                wm_copy(wm_s, 2 * D // E + c, c, SEM_WMR).start()

            @pl.when(c == NC - 3)
            def _():
                def issue(k, carry2):
                    wm_copy(wm_s, 2 * D // E + k, k, SEM_WMR).start()
                    return carry2

                x_copy(0).start()
                for k in range(2):
                    for cp in mlp_w_copies(k, k):
                        cp.start()
                lax.fori_loop(NC - 3, 3 * D // E, issue, 0)

            return carry

        lax.fori_loop(0, NC, _scoped("p1", p1_body), 0)
        x_copy(1).start()
        x_copy(0).wait()
        wm_wait(wm_s, 0, 3 * D // E, SEM_WMR)
        mod_tiles(wm_s, 0, 3 * D // E, 2 * D // E)
        hn_s[...] = h_rows(0)

    def phase_b(t2_s, t3_s, t4_s, wg_s, x1_s, base_s, yn_s, o_s):
        for k in range(D // E):
            wm_copy(wg_s, 5 * D // E + k, k, SEM_WM).start()

        def chain_step(s, mem, htok, odef_prev, jobs=(), hooks=None):
            hs = jnp.concatenate([mem, htok], axis=0).astype(bf16)
            qkv = [[None] * 3 for _ in range(NP)]
            ps = [None] * NP
            os_ = [None] * H
            odef = [None] * H

            def proj(p, ts=(0, 1, 2)):
                for t in ts:
                    c, q = t * NG + p // (HG // 2), p % (HG // 2)
                    a = _dot(hs, _up(w_s[c, :, _ct(2 * q)]))
                    b = _dot(hs, _up(w_s[c, :, _ct(2 * q + 1)]))
                    if hooks and t == 2 and p - NP in hooks:
                        hooks[p - NP](b)
                    pre = pre_s[c, pl.ds(pl.multiple_of(s * M, M), M), _ct(q)]
                    if t == 1:
                        kf = jnp.concatenate([a, b, _up(pre).astype(f32), jnp.zeros((E - NR, E), f32)],
                                             axis=0)
                        qkv[p][t] = kf.T.astype(bf16)
                        continue
                    parts = [_pk(a), _pk(b), pre]
                    if t == 2:
                        parts.append(jnp.zeros(((E - NR) // 2, E), u32))
                    qkv[p][t] = _up(jnp.concatenate(parts, axis=0))

            def scores(p):
                sc_ = _dot(qkv[p][0], qkv[p][1])
                fill = fill_s[...]
                sc_ = jnp.where(fill == 0.0, sc_ * SCALE, fill)
                m = jnp.max(sc_, axis=-1, keepdims=True)
                e = jnp.exp(sc_ - m)
                l = jnp.sum(e, axis=-1, keepdims=True)
                r = pl.reciprocal(l, approx=True)
                r = r * (2.0 - l * r)
                ps[p] = (e * r).astype(bf16)

            def fin(p):
                o = _dot(ps[p], qkv[p][2])
                for hh in range(2):
                    h = 2 * p + hh
                    rows = o[32 * hh:32 * hh + 32]
                    odef[h] = o[64 + 8 * hh:72 + 8 * hh]
                    if odef_prev is not None:
                        rows = jnp.concatenate([rows, odef_prev[h], odef[h]], axis=0)
                    os_[h] = _pk(rows)

            acc = [None] * 8
            jobs = iter(jobs)

            def wo(h0, h1, js):
                lhs = _up(jnp.concatenate(os_[h0:h1], axis=1))
                for j in js:
                    ws = []
                    for r0 in range(h0 * E // 2, h1 * E // 2, PIN_ROWS):
                        ws.append(pinned(lambda: wo_s[r0:r0 + PIN_ROWS, j * E:(j + 1) * E],
                                         next(jobs, None)))
                    part = _dot(lhs, _up(jnp.concatenate(ws, axis=0)))
                    if hooks and acc[j] is None and j in hooks:
                        hooks[j](part)
                    acc[j] = part if acc[j] is None else part + acc[j]

            ORDER, LAG_S, LAG_O = SCHED_A if odef_prev is None else SCHED_B
            for p in range(NP):
                if ORDER == 0:
                    proj(p)
                    if p >= LAG_S:
                        scores(p - LAG_S)
                    if p >= LAG_O:
                        fin(p - LAG_O)
                elif ORDER == 1:
                    proj(p, (1, 0))
                    if p >= LAG_O:
                        fin(p - LAG_O)
                    proj(p, (2,))
                    if p >= LAG_S:
                        scores(p - LAG_S)
                elif ORDER == 2:
                    proj(p, (1,))
                    if p >= LAG_S:
                        scores(p - LAG_S)
                    proj(p, (0,))
                    if p >= LAG_O:
                        fin(p - LAG_O)
                    proj(p, (2,))
                elif ORDER == 3:
                    proj(p, (1,))
                    if p >= LAG_O:
                        fin(p - LAG_O)
                    proj(p, (0,))
                    if p >= LAG_S:
                        scores(p - LAG_S)
                    proj(p, (2,))
                elif ORDER == 4:
                    proj(p, (1,))
                    if p >= LAG_S:
                        scores(p - LAG_S)
                    proj(p, (0, 2))
                    if p >= LAG_O:
                        fin(p - LAG_O)
                else:
                    proj(p, (0,))
                    if p >= LAG_S:
                        scores(p - LAG_S)
                    proj(p, (1,))
                    if p >= LAG_O:
                        fin(p - LAG_O)
                    proj(p, (2,))
            tail = []
            for k in range(LAG_O):
                step = []
                if NP - LAG_S + k < NP:
                    step.append(functools.partial(scores, NP - LAG_S + k))
                step.append(functools.partial(fin, NP - LAG_O + k))
                tail.append(step)
            hsplit = min(24, 2 * (NP - LAG_O))
            cuts = {3: (2, 3, 5), 2: (2, 5), 4: (1, 2, 4, 6), 5: (1, 2, 3, 4, 6)}[LAG_O]
            j0 = 0
            for k, step in enumerate(tail):
                wo(0, hsplit, range(j0, cuts[k]))
                j0 = cuts[k]
                for f in step:
                    f()
            wo(0, hsplit, range(j0, 8))
            wo(hsplit, H, range(8))
            return jnp.concatenate(acc, axis=1), odef

        def mixer_prep(i, r0, n, anchor=None):
            r = pl.ds(aligned(i * 64 + r0, 16), n)
            xr = x_s[2 * i + r0 // SEG, r0 % SEG:r0 % SEG + n, :].astype(f32)
            x2 = xr + mod_rows(2, n) * after(aout_s[r0:r0 + n, :], anchor)
            x_s.at[2 * i + r0 // SEG][r0 % SEG:r0 % SEG + n, :] = x2.astype(bf16)
            hb = _ln(x2) * mod_rows(4, n) + mod_rows(3, n)
            hb_s[r, :] = hb.astype(bf16)
            return _ln(hb)

        def mixer_sets(ya, yb, r0):
            n = ya.shape[0]
            for m, v in enumerate(_lhs_set(ya[:, :HD], ya[:, HD:], yb[:, :HD], yb[:, HD:])):
                l1_s.at[m][r0 // 2:(r0 + n) // 2, :] = _pk(v)

        def mixer_mm(i):
            for q in range(NQ):
                cs = _strassen(lambda n: _dot(_up(l1_s[n]), _up(t1_s[n, :, _ct(q)])))
                for k, cc in enumerate(cs):
                    r0 = aligned(i * 64 + 8 + (k // 2) * SEG, 8)
                    t_s[pl.ds(r0, SEG), _ct(q + NQ * (k % 2))] = _gelu(cc)

        def p2_body(i, carry):
            slot = i & 1
            for cp in mlp_w_copies(0, slot):
                cp.wait()

            @pl.when(i == 1)
            def _():
                x_copy(1).wait()

            g, rr = mlp_piece(i)
            work = [functools.partial(rhs_job, g2, slot, 0, 2 * q, 2 * q + 1, t2_s, q, i * 8)
                    for q in range(NQ)]
            work += [functools.partial(rhs2_job, g3, slot, 16 * rt, 0, n1, t3_s.at[g], rr * 32 + 8 * rt)
                     for rt in range(4) for n1 in range(7)]
            work += [functools.partial(rhs2_job, g4, slot, 16 * rt, 4 * og, n1, t4_s.at[og],
                                       g * (E // 2) + rr * 16 + 8 * rt)
                     for rt in range(2) for og in range(NOG) for n1 in range(7)]
            jobs = [None] + work

            sa_ = 2 * i
            sb_ = 2 * i + 1
            hb_tok = h_rows(sb_)
            oa, odef_a = chain_step(sa_, mem_s[...], hn_s[...], None)
            mixer_mm(jnp.maximum(i - 2, 0))
            ys = []

            def hook(k, anchor):
                if k >= PREP_CH:
                    anchor = anchor[0:8] + ys[-PREP_CH][0:8, 0:E] + ys[-PREP_CH][8:16, 0:E]
                ys.append(mixer_prep(jnp.maximum(i - 1, 0), (k % 2) * SEG + (k // 2) * 16, 16, anchor))
                if k % 2:
                    mixer_sets(ys[-2], ys[-1], (k // 2) * 16)

            hooks = {j: functools.partial(hook, k) for k, j in enumerate(PREP_AT)}
            ob, _ = chain_step(sb_, oa[0:M], hb_tok, odef_a, jobs, hooks)
            mem_s[...] = ob[0:M]
            aout_s[0:TC, :] = oa[M:SEG]
            aout_s[TC:SEG, :] = ob[SEG:SEG + M]
            aout_s[SEG:SEG + TC, :] = ob[M:SEG]
            aout_s[SEG + TC:2 * SEG, :] = ob[SEG + M:SEG + 2 * M]
            hn_s[...] = h_rows(jnp.minimum(sb_ + 1, NSEG - 1))
            for cp in mlp_w_copies(i + 2, slot):
                cp.start()
            return carry

        lax.fori_loop(0, _N2, _scoped("p2", p2_body), 0)

        TH = TB // 2
        TQ = TB // 4
        SHIFT = (-1, -1, 1, 1, -2, -2, 2, 2)

        def u_set(n):
            return w_s.at[n // 32], slice((n % 32) * (TQ // 2), (n % 32 + 1) * (TQ // 2))

        def y_set(n):
            return w_s.at[2], (n // 4) * (TQ // 2), (n % 4) * 2

        def g_rows(n, r0=0, n_rows=TH // 2):
            return slice(n * (TH // 2) + r0, n * (TH // 2) + r0 + n_rows)

        g_s = w_s.at[3]

        def g_job(j, rt, q, n=16, anchor=None):
            blk = []
            for hf in range(2):
                for ct in (q, NQ + q):
                    win = t_s[pl.ds(aligned(j * TB + hf * TH + rt * n, 16), n + 16), _ct(ct)]
                    blk.append(win[8 + SHIFT[ct]:8 + SHIFT[ct] + n])
            blk[0] = after(blk[0], anchor)
            blk[3] = after(blk[3], anchor)
            for k, v in enumerate(_lhs_set(*blk)):
                g_s[g_rows(k, rt * n // 2, n // 2), _ct(q)] = _pk(v)

        def mix(j):
            r0 = aligned(j * TB, TB)
            for q in range(NQ):
                cs = _strassen(lambda n: _dot(_up(g_s[g_rows(n), 0:HD]), _up(t2_s[n, :, _ct(q)])))
                cols = slice(2 * q * E, (2 * q + 2) * E)
                for hf in range(2):
                    x1_s[hf * TH:(hf + 1) * TH, cols] = (
                        hb_s[pl.ds(r0 + hf * TH, TH), cols].astype(f32)
                        + jnp.concatenate(cs[2 * hf:2 * hf + 2], axis=1))

        def base_job(j, rt, anchor):
            rows = slice(rt * 16, (rt + 1) * 16)
            z = pltpu.bitcast(pltpu.bitcast(anchor[0:8], u32) & zero_s[...], f32)
            gb = mod_rows(5, 8) + jnp.concatenate([z] * (D // E), axis=1)
            x2 = x_s[j * (TB // SEG) + rt // 2, (rt % 2) * 16:(rt % 2) * 16 + 16, :]
            base_s[rows, :] = x2.astype(f32) + jnp.concatenate([gb, gb], axis=0) * x1_s[rows, :]

        def out_copy(j, slot):
            return copy(o_s.at[slot], out_hbm.at[pl.ds(aligned(j * TB, TB), TB)], SEM_OUT + slot)

        def ln_job(r0, n, prev, anchor=None):
            if anchor is not None and len(prev) >= 2:
                anchor = anchor[0:8] + prev[-2]
            y = _ln(after(x1_s[r0:r0 + n, :], anchor))
            yn_s[r0:r0 + n, :] = y
            prev.append(y[0:8, 0:E] + y[8:16, 0:E])

        def yset_job(rt, ct, n1, n=16, anchor=None):
            blk = _outer_operand(lambda i, k: yn_s[i * TQ + rt * n:i * TQ + (rt + 1) * n, _ct(2 * k + ct)],
                                 _LHS_TERMS[n1])
            blk[0] = after(blk[0], anchor)
            blk[3] = after(blk[3], anchor)
            for n2, v in enumerate(_lhs_set(*blk)):
                ref, r0, c0 = y_set(7 * n1 + n2)
                ref[r0 + rt * n // 2:r0 + (rt + 1) * n // 2, _ct(c0 + ct)] = _pk(v)

        wm_wait(wg_s, 0, D // E, SEM_WM)
        mod_tiles(wg_s, 0, D // E, 5 * D // E)
        mixer_mm(NI - 2)
        mixer_sets(mixer_prep(NI - 1, 0, SEG), mixer_prep(NI - 1, SEG, SEG), 0)
        for q in range(NQ):
            g_job(0, 0, q, TH)
        mix(0)
        mixer_mm(NI - 1)
        ln_job(0, TB, [])
        for ct in range(2):
            for n1 in range(7):
                yset_job(0, ct, n1, TQ)
        for q in range(NQ):
            g_job(1, 0, q, TH)

        def mlp_block(j, last):
            slot = j & 1

            def up_prod(n, g):
                ref, r0, c0 = y_set(n)
                m = _dot(_up(ref[r0:r0 + TQ // 2, c0 * E:(c0 + 2) * E]), _up(t3_s[g, :, _ct(n)]))
                if n in (10, 34) and 2 * g + (n == 34) < TB // 16:
                    base_job(j, 2 * g + (n == 34), m)
                return m

            for g in range(NFG):
                c = _strassen2(lambda n: up_prod(n, g))
                act = [[_gelu(c(i, k)) for k in range(4)] for i in range(4)]
                for n1 in range(7):
                    blk = _outer_operand(lambda i, k: act[i][k], _LHS_TERMS[n1])
                    for n2, v in enumerate(_lhs_set(*blk)):
                        ref, rows = u_set(7 * n1 + n2)
                        ref[rows, _ct(g)] = _pk(v)
            jobs = {}
            if not last:
                mix(j + 1)
                jn = clamp(j + 2, NB - 1)
                prev = []
                for k in range(TB // 16):
                    jobs[k * Y_AT] = functools.partial(ln_job, (k % 4) * TQ + (k // 4) * 16, 16, prev)

                def place(start, fns):
                    for fn in fns:
                        while start in jobs:
                            start += 1
                        jobs[start] = fn

                for rt in range(2):
                    place(S_AT[rt], [functools.partial(yset_job, rt, ct, n1, 16)
                                     for ct in range(2) for n1 in range(7)])
                place(G_AT, [functools.partial(g_job, jn, k // NQ, k % NQ, 16)
                             for k in range(TH // 16 * NQ)])

            def down_part(n, og, k0, k1):
                ref, rows = u_set(n)
                return _dot(_up(ref[rows, k0 * E:k1 * E]),
                            _up(t4_s[og, k0 * E // 2:k1 * E // 2, _ct(n)]))

            head = {}
            if last:
                head = {n: down_part(n, 0, 0, NFG - 1) for n in range(HEAD)}
            count = [0]

            def down_prod(n, og):
                if og == 0 and n in head:
                    return down_part(n, og, NFG - 1, NFG) + head[n]
                m = down_part(n, og, 0, NFG)
                job = jobs.get(count[0])
                count[0] += 1
                if job is not None:
                    job(anchor=m)
                return m

            for og in range(NOG):
                c = _strassen2(lambda n: down_prod(n, og))
                for i in range(4):
                    rows = slice(i * TQ, (i + 1) * TQ)
                    for k in range(2):
                        c0 = (4 * og + 2 * k) * E
                        o_s.at[slot][rows, c0:c0 + 2 * E] = (
                            base_s[rows, c0:c0 + 2 * E] + mod_rows(5, TQ, c0, 2 * E)
                            * jnp.concatenate([c(i, 2 * k), c(i, 2 * k + 1)], axis=1)).astype(bf16)
            out_copy(j, slot).start()

        def p3_body(j, carry):
            @pl.when(j >= 2)
            def _():
                out_copy(j - 2, j & 1).wait()

            mlp_block(j, False)
            return carry

        lax.fori_loop(0, NB - 1, _scoped("p3", p3_body), 0)
        for k in range(2):
            for cp in mlp_w_copies(0, k):
                cp.wait()
        out_copy(NB - 3, (NB - 3) % 2).wait()
        mlp_block(NB - 1, True)
        out_copy(NB - 2, (NB - 2) % 2).wait()
        out_copy(NB - 1, (NB - 1) % 2).wait()

    pl.run_scoped(
        phase_a,
        pltpu.VMEM((NSEG, M, D), bf16),
        pltpu.VMEM((7, NSEG * M // 4, D // 2), u32),
        pltpu.VMEM((3 * D // E, D, E), bf16),
        pltpu.VMEM((2, D, HG, E), bf16),
        pltpu.VMEM((2, BGR, D), bf16),
        pltpu.VMEM((2, 2, G1R, D), bf16),
    )
    pl.run_scoped(
        phase_b,
        pltpu.VMEM((7, D // 4, D // 2), u32),
        pltpu.VMEM((NFG, D // 8, 49 * E), u32),
        pltpu.VMEM((NOG, F // 8, 49 * E), u32),
        pltpu.VMEM((D // E, D, E), bf16),
        pltpu.VMEM((TB, D), f32),
        pltpu.VMEM((TB, D), f32),
        pltpu.VMEM((TB, D), f32),
        pltpu.VMEM((2, TB, D), bf16),
    )


@jax.jit
def pallas_adaLN_cond__memory_aug_recurrent_mem_tr__mixer_s_mlp__prompt_kernel(
    A_x: jax.Array,
    A_mem0: jax.Array,
    A_Wq: jax.Array,
    A_Wk: jax.Array,
    A_Wv: jax.Array,
    A_Wo: jax.Array,
    A_seg_len,
    B_x: jax.Array,
    B_w1: jax.Array,
    B_w2: jax.Array,
    B_w3: jax.Array,
    B_w4: jax.Array,
    c: jax.Array,
    w_mod: jax.Array,
):
    del A_seg_len, B_x
    assert A_x.shape == (1, S, D) and A_mem0.shape == (1, M, D)
    hbm = pl.BlockSpec(memory_space=pl.ANY)
    scratch = [
        pltpu.VMEM((NSEG, SEG, D), bf16),
        pltpu.VMEM((NC + 3, D // 2, HG * E), u32),
        pltpu.VMEM((H * E // 2, D), u32),
        pltpu.VMEM((7, D // 4, D // 2), u32),
        pltpu.VMEM((2, 2, 16, D), bf16),
        pltpu.VMEM((2, 4, 64, 4 * E), bf16),
        pltpu.VMEM((2, 4, 32, D), bf16),
        pltpu.VMEM((NC + 2, NSEG * M, HG // 2 * E), u32),
        pltpu.VMEM((8, 6 * D), f32),
        pltpu.VMEM((M, D), f32),
        pltpu.VMEM((TC, D), f32),
        pltpu.VMEM((2 * SEG, D), f32),
        pltpu.VMEM((NR, E), f32),
        pltpu.VMEM((S, D), bf16),
        pltpu.VMEM((S + 16, D), f32),
        pltpu.VMEM((7, SEG // 2, D // 2), u32),
        pltpu.VMEM((8, E), u32),
        pltpu.VMEM((1, D), bf16),
        pltpu.VMEM((M, D), bf16),
        pltpu.SemaphoreType.DMA((24,)),
    ]
    out = pl.pallas_call(
        _kernel,
        out_shape=jax.ShapeDtypeStruct((S, D), bf16),
        in_specs=[hbm] * 12,
        out_specs=hbm,
        scratch_shapes=scratch,
        compiler_params=pltpu.CompilerParams(vmem_limit_bytes=127 * 1024 * 1024,
                                             disable_bounds_checks=NO_BOUNDS),
    )(A_x.reshape(NSEG, SEG, D), A_mem0.reshape(M, D), A_Wq, A_Wk, A_Wv,
      A_Wo.reshape(H * E, D), B_w1.reshape(2, D // 2, D), B_w2.reshape(2, D // 2, D), B_w3.reshape(4, D // 4, F),
      B_w4.reshape(NFG, 4, E, D), c, w_mod)
    return out.reshape(1, S, D)
```

```python
import functools

import jax
import jax.numpy as jnp
from jax import lax
import jax.experimental.pallas as pl
import jax.experimental.pallas.tpu as pltpu

bf16, f32, u32 = jnp.bfloat16, jnp.float32, jnp.uint32

S, D, H, E, M, SEG, F = 2048, 1024, 32, 128, 8, 32, 3584
NSEG = S // SEG
NP = H // 2
TC = SEG - M
HG = 8
NG = H // HG
TB = 128
NB = S // TB
NFG = F // (4 * E)
NOG = D // (4 * E)
NI = NSEG // 2
NQ = D // E // 2
NC = 3 * NG
BGR = 384
G1R = 48
HD = D // 2
X0 = 4
NR = 2 * (M + SEG)
NO_BOUNDS = True
ZPAD = 2
PIN_ROWS = 256
Y_AT = 4
S_AT = (26, 44)
G_AT = 62
HEAD = 14
PREP_AT = (0, 1, 3, 4)
PREP_CH = 2
SORD = 0
FINE = 1
JGROUP = 1
P1_TAIL = 5
P1_LAG = 4
SCHED_A = (2, 1, 3)
SCHED_B = (3, 1, 3)
EPS = 1e-5
SCALE = E ** -0.5
_SCOPES = False
_N2 = NSEG // 2


def _scoped(name, fn):
    def wrapped(*a):
        if not _SCOPES:
            return fn(*a)
        with jax.named_scope(name):
            return fn(*a)
    return wrapped


def _pk(x):
    return pltpu.bitcast(x.astype(bf16), u32)


def _up(x):
    return pltpu.bitcast(x, bf16)


def _ct(k):
    return slice(k * E, (k + 1) * E)


def _dot(a, b):
    return jnp.dot(a, b, preferred_element_type=f32)


def _ln(x):
    m = jnp.mean(x, axis=-1, keepdims=True)
    xc = x - m
    v = jnp.mean(xc * xc, axis=-1, keepdims=True)
    return xc * lax.rsqrt(v + EPS)


def _gelu(x):
    c = 0.7978845608028654
    return 0.5 * x * (1.0 + jnp.tanh(c * (x + 0.044715 * (x * x * x))))


def _lhs_set(a11, a12, a21, a22):
    return (a11 + a22, a21 + a22, a11, a22, a11 + a12, a21 - a11, a12 - a22)


def _rhs_set(b11, b12, b21, b22):
    return (b11 + b22, b11, b12 - b22, b21 - b11, b22, b11 + b12, b21 + b22)


_LHS_TERMS = (((0, 1), (3, 1)), ((2, 1), (3, 1)), ((0, 1),), ((3, 1),),
              ((0, 1), (1, 1)), ((2, 1), (0, -1)), ((1, 1), (3, -1)))
_RHS_TERMS = (((0, 1), (3, 1)), ((0, 1),), ((1, 1), (3, -1)), ((2, 1), (0, -1)),
              ((3, 1),), ((0, 1), (1, 1)), ((2, 1), (3, 1)))


def _outer_operand(tile, terms):
    out = []
    for i in range(2):
        for j in range(2):
            v = None
            for o, sign in terms:
                t = tile(2 * (o // 2) + i, 2 * (o % 2) + j)
                v = t if v is None else (v + t if sign > 0 else v - t)
            out.append(v)
    return out


class _Quad:
    def __init__(self, tiles):
        self.t = tuple(tiles)

    def __add__(self, other):
        return _Quad([a + b for a, b in zip(self.t, other.t)])

    def __sub__(self, other):
        return _Quad([a - b for a, b in zip(self.t, other.t)])


def _strassen2(m):
    cs = _strassen(lambda n1: _Quad(_strassen(lambda n2: m(7 * n1 + n2))))
    return lambda i, j: cs[2 * (i // 2) + j // 2].t[2 * (i % 2) + j % 2]


def _strassen(m):
    if SORD == 0:
        m1 = m(0)
        m2 = m(1)
        c22 = m1 - m2
        m3 = m(2)
        c22 = c22 + m3
        c22 = m(5) + c22
        m4 = m(3)
        c21 = m2 + m4
        c11 = m1 + m4
        m5 = m(4)
        c12 = m3 + m5
        c11 = c11 - m5
        c11 = m(6) + c11
    else:
        m2 = m(1)
        c22 = m(5) - m2
        m4 = m(3)
        c21 = m2 + m4
        m1 = m(0)
        c22 = c22 + m1
        c11 = m4 + m1
        m3 = m(2)
        c22 = c22 + m3
        m5 = m(4)
        c12 = m3 + m5
        c11 = c11 - m5
        c11 = m(6) + c11
    return c11, c12, c21, c22


def _mask_fill():
    shape = (NR, E)
    r = lax.broadcasted_iota(jnp.int32, shape, 0)
    c = lax.broadcasted_iota(jnp.int32, shape, 1)

    def headpos(i):
        head = jnp.where(i < 64, i >> 5, (i - 64) >> 3)
        pos = jnp.where(i < 64, i & 31, 32 + (i & 7))
        return head, pos

    hr, pr = headpos(r)
    hc, pc = headpos(c)
    same = hr == hc
    valid = same & ((pr < M) | (pr >= pc))
    return jnp.where(valid, 0.0, jnp.where(same, -1e9, -jnp.inf)).astype(f32)


def _kernel(x_hbm, mem0_hbm, wq_hbm, wk_hbm, wv_hbm, wo_hbm, w1_hbm, w2_hbm, w3_hbm,
            w4_hbm, c_hbm, wm_hbm,
            out_hbm,
            x_s, w_s, wo_s, t1_s, g2, g3, g4, pre_s, mod_s, mem_s, hn_s, aout_s, fill_s,
            hb_s, t_s, l1_s, zero_s, c_s, mem0_s, sems):
    w_hbm = (wq_hbm, wk_hbm, wv_hbm)

    (SEM_C, SEM_MEM, SEM_XPRE, SEM_X, SEM_STG, SEM_BG, SEM_OUT,
     SEM_WMR, SEM_G2, SEM_G3, SEM_G4, SEM_WM, SEM_G1) = (0, 1, 2, 3, 4, 6, 8, 10, 12, 14, 16, 18, 22)

    def copy(src, dst, k):
        return pltpu.make_async_copy(src, dst, sems.at[k])

    def aligned(x, n):
        return x if isinstance(x, int) else pl.multiple_of(x, n)

    def clamp(k, hi):
        return min(k, hi) if isinstance(k, int) else jnp.minimum(k, hi)

    def mlp_piece(k):
        k = clamp(k, 4 * NFG - 1)
        return k >> 2, k & 3

    def mlp_w_copies(k, slot):
        g, rr = mlp_piece(k)
        r = pl.ds(aligned(clamp(k, NI - 1) * 16, 16), 16)
        return (copy(w2_hbm.at[:, r, :], g2.at[slot], SEM_G2 + slot),
                copy(w3_hbm.at[:, pl.ds(aligned(rr * 64, 64), 64), pl.ds(aligned(g * 4 * E, E), 4 * E)],
                     g3.at[slot], SEM_G3 + slot),
                copy(w4_hbm.at[g, :, pl.ds(aligned(rr * 32, 32), 32), :], g4.at[slot], SEM_G4 + slot))

    def pinned(w, job):
        if job is None:
            return w()
        z = job() & zero_s[0:8, :]
        w = w()
        return jnp.concatenate([w[0:8] | z, w[8:]], axis=0)

    def after(x, anchor):
        if anchor is None:
            return x
        z = pltpu.bitcast(pltpu.bitcast(anchor[0:8], u32) & zero_s[0:8, :], f32)
        z = jnp.concatenate([z] * (x.shape[0] // 8), axis=0)
        return jnp.concatenate([x[:, 0:E] + z, x[:, E:]], axis=1) if x.shape[1] > E else x + z

    def rhs_job(src, slot, r0, c1, c2, dst, q, row, z=None):
        blk = [src[slot, kh, r0:r0 + 16, cc * E:(cc + 1) * E].astype(f32)
               for kh in range(2) for cc in (c1, c2)]
        if z is not None:
            zf = pltpu.bitcast(jnp.concatenate([z, z], axis=0), f32)
            blk[0] = blk[0] + zf
            blk[3] = blk[3] + zf
        sets = _rhs_set(*blk)
        for n, v in enumerate(sets):
            dst.at[n][pl.ds(pl.multiple_of(row, 8), 8), _ct(q)] = _pk(v)
        out = pltpu.bitcast(sets[2], u32) | pltpu.bitcast(sets[3], u32)
        return out[0:8] | out[8:16]

    def rhs2_job(src, slot, r0, c0, n1, dst, row):
        blk = _outer_operand(lambda i, j: src[slot, i, r0:r0 + 16, _ct(c0 + j)].astype(f32),
                             _RHS_TERMS[n1])
        sets = _rhs_set(*blk)
        for n2, v in enumerate(sets):
            dst[pl.ds(pl.multiple_of(row, 8), 8), _ct(7 * n1 + n2)] = _pk(v)
        out = pltpu.bitcast(sets[2], u32) | pltpu.bitcast(sets[3], u32)
        return out[0:8] | out[8:16]

    def silu_c():
        cf = c_s[...].astype(f32)
        return jnp.broadcast_to(cf * (1.0 / (1.0 + jnp.exp(-cf))), (8, D)).astype(bf16)

    def wm_copy(wm_s, src_tile, dst_tile, sem):
        return copy(wm_hbm.at[:, pl.ds(aligned(src_tile * E, E), E)], wm_s.at[dst_tile], sem)

    def wm_wait(wm_s, t0, n, sem):
        copy(wm_s.at[t0:t0 + n], wm_s.at[t0:t0 + n], sem).wait()

    def mod_tiles(wm_s, t0, n, dst_tile):
        sc8 = silu_c()
        for k in range(n):
            v = _dot(sc8, wm_s[t0 + k])
            if (dst_tile + k) // (D // E) in (1, 4):
                v = 1.0 + v
            mod_s[:, _ct(dst_tile + k)] = v

    def x_copy(k):
        r = slice(0, X0) if k == 0 else slice(X0, NSEG)
        return copy(x_hbm.at[r], x_s.at[r], SEM_XPRE if k == 0 else SEM_X)

    def h_rows(s):
        return _ln(x_s[s, 0:TC, :].astype(f32)) * mod_rows(1, TC) + mod_rows(0, TC)

    def mod_rows(k, n, c0=0, w=D):
        return jnp.concatenate([mod_s[:, k * D + c0:k * D + c0 + w]] * (n // 8), axis=0)

    def tq_place(c, n):
        if n == 1:
            return w_s.at[c], 0, None
        if n == 4:
            return w_s.at[c], D // 4, None
        if n == 6:
            return pre_s.at[c + 1], 0, 0
        k = (0, 2, 3, 5).index(n)
        return w_s.at[c + 2], (k // 2) * (D // 4), (k % 2) * (HG // 2)

    def phase_a(xpre_s, hpre_s, wm_s, stg, bg, g1):
        def w_copy(t, g, slot):
            return copy(w_hbm[t].at[:, pl.ds(pl.multiple_of(g * HG, HG), HG), :], stg.at[slot],
                        SEM_STG + slot)

        def bg_rows(k):
            return clamp(k * BGR, H * E - BGR), clamp(k * G1R, HD - G1R)

        def bg_copies(k, slot):
            ro, r1 = bg_rows(k)
            return (copy(wo_hbm.at[pl.ds(aligned(ro, 16), BGR)], bg.at[slot], SEM_BG + slot),
                    copy(w1_hbm.at[:, pl.ds(aligned(r1, 16), G1R), :], g1.at[slot], SEM_G1 + slot))

        def relayout_jobs(slot, c, i):
            memo = []
            r = aligned(i * 8, 8)

            def job(j, z=None):
                if not memo:
                    for d0 in (i * 16, HD + i * 16):
                        memo.append(jnp.swapaxes(pltpu.bitcast(stg[slot, pl.ds(d0, 16)], u32), 0, 1))
                blk = []
                for kh in range(2):
                    u = memo[kh][j]
                    if z is not None:
                        u = u | jnp.concatenate([z, z], axis=0)
                    blk.append(pltpu.bitcast(u << 16, f32))
                    blk.append(pltpu.bitcast(u & jnp.uint32(0xFFFF0000), f32))
                for k, v in enumerate(blk):
                    w_s.at[c][pl.ds((k // 2) * (D // 4) + r, 8), _ct(2 * j + k % 2)] = _pk(v)
                for n, v in enumerate(_rhs_set(*blk)):
                    if n not in (1, 4):
                        ref, r0, c0 = tq_place(c, n)
                        ref[pl.ds(r0 + r, 8), _ct(c0 + j)] = _pk(v)

            return [functools.partial(job, j) for j in range(HG // 2)]

        def repack(slot, row, i, z):
            v = pltpu.bitcast(bg[slot, 16 * i:16 * i + 16, :], u32)
            v = v | jnp.concatenate([z] * (D // E), axis=1)
            wo_s[pl.ds(pl.multiple_of(row + 8 * i, 8), 8), :] = v

        cp_c = copy(c_hbm, c_s, SEM_C)
        cp_mem = copy(mem0_hbm, mem0_s, SEM_MEM)
        cp_xpre = copy(x_hbm.at[:, TC:SEG, :], xpre_s, SEM_XPRE)
        w_copy(0, 0, 0).start()
        cp_xpre.start()
        cp_c.start()
        cp_mem.start()
        for k in range(2 * D // E):
            wm_copy(wm_s, k, k, SEM_WM + k // 4).start()
        w_copy(0, 1, 1).start()

        zero_s[0:8, :] = jnp.zeros((8, E), u32)
        fill_s[0:NR, :] = _mask_fill()
        aout_s[...] = jnp.zeros(aout_s.shape, f32)
        l1_s[...] = jnp.zeros(l1_s.shape, u32)
        bg[1] = jnp.zeros(bg.shape[1:], bf16)
        g1[1] = jnp.zeros(g1.shape[1:], bf16)

        w_copy(0, 0, 0).wait()

        def rl0_body(i, carry):
            for job in relayout_jobs(0, 0, i):
                job()
            return carry

        lax.fori_loop(0, D // 32, rl0_body, 0)
        w_copy(0, 2, 0).start()
        for cp in bg_copies(0, 0):
            cp.start()

        cp_xpre.wait()

        def npre_body(i, carry):
            xr = xpre_s[pl.ds(pl.multiple_of(i * 8, 8), 8)].astype(f32).reshape(64, D)
            t_s[pl.ds(pl.multiple_of(i * 64, 64), 64), :] = _ln(xr)
            return carry

        lax.fori_loop(0, NSEG // 8, _scoped("npre", npre_body), 0)

        cp_c.wait()
        cp_mem.wait()
        mem_s[...] = mem0_s[...].astype(f32)

        for k in range(4):
            wm_wait(wm_s, 4 * k, 4, SEM_WM + k)
            mod_tiles(wm_s, 4 * k, 4, 4 * k)

        PH = NSEG * M // 2

        def hpre_body(i, carry):
            h = [t_s[pl.ds(pl.multiple_of(hf * PH + i * 16, 16), 16), :] * mod_rows(1, 16) + mod_rows(0, 16)
                 for hf in range(2)]
            for n, v in enumerate(_lhs_set(h[0][:, :HD], h[0][:, HD:], h[1][:, :HD], h[1][:, HD:])):
                hpre_s.at[n][pl.ds(pl.multiple_of(i * 8, 8), 8), :] = _pk(v)
            return carry

        lax.fori_loop(0, PH // 16, _scoped("hpre", hpre_body), 0)

        t_s[0:8, :] = jnp.zeros((8, D), f32)
        t_s[S + 8:S + 16, :] = jnp.zeros((8, D), f32)

        MB = 64

        def p1_body(c, carry):
            slot = c & 1
            pslot = 1 - slot
            ro, r1 = bg_rows(jnp.maximum(c - 1, 0))

            @pl.when(c >= 1)
            def _():
                for cp in bg_copies(0, pslot):
                    cp.wait()

            @pl.when(c + 1 < NC)
            def _():
                w_copy(0, 0, pslot).wait()

            small = [functools.partial(repack, pslot, ro >> 1, i) for i in range(BGR // 16)]
            small += [functools.partial(rhs_job, g1, pslot, 16 * rt, q, NQ + q, t1_s, q, (r1 >> 1) + 8 * rt)
                      for rt in range(G1R // 16) for q in range(NQ)]
            work = []
            nu = D // 32
            for i in range(nu):
                js = relayout_jobs(pslot, c + 1, i)
                work += [js[k:k + JGROUP] for k in range(0, len(js), JGROUP)]
                work += [[job] for job in small[i * len(small) // nu:(i + 1) * len(small) // nu]]
            npin = 7 * (HG // 2) * (PH // MB)
            jobs = [[] for _ in range(npin)]
            for k, group in enumerate(work):
                pos = k * (npin - P1_TAIL) * 8 // len(work)
                jobs[pos // 8] += [(job, pos % 8 if FINE else 0) for job in group]
            jobs = iter(jobs)

            def prod(n, q, mb):
                ref, r0, c0 = tq_place(c, n)
                w = ref[r0:r0 + D // 4, _ct(2 * q + (n == 4) if c0 is None else c0 + q)]
                m = _dot(_up(hpre_s[n, mb * MB // 2:(mb + 1) * MB // 2, :]), _up(w))
                pending.append(m)
                if len(pending) > P1_LAG:
                    anchor = pltpu.bitcast(pending.pop(0), u32)
                    for job, g in next(jobs):
                        job(anchor[8 * g:8 * g + 8] & zero_s[0:8, :])
                return m

            pending = []
            ns = MB // M
            for q in range(HG // 2):
                for mb in range(PH // MB):
                    cs = _strassen(lambda n: prod(n, q, mb))
                    for hf in range(2):
                        y = jnp.concatenate([cs[2 * hf + k][sg * M:(sg + 1) * M]
                                             for sg in range(ns) for k in range(2)], axis=0)
                        s0 = hf * (NSEG // 2) + mb * ns
                        pre_s.at[c][s0 * M:(s0 + ns) * M, _ct(q)] = _pk(y)

            for t in range(3):
                @pl.when((c + 3) >> 2 == t)
                def _():
                    w_copy(t, (c + 3) & 3, pslot).start()

            @pl.when(c + 2 < NC)
            def _():
                for cp in bg_copies(c + 1, pslot):
                    cp.start()

            @pl.when(c < NC - 3)
            def _():
                wm_copy(wm_s, 2 * D // E + c, c, SEM_WMR).start()

            @pl.when(c == NC - 3)
            def _():
                def issue(k, carry2):
                    wm_copy(wm_s, 2 * D // E + k, k, SEM_WMR).start()
                    return carry2

                x_copy(0).start()
                for k in range(2):
                    for cp in mlp_w_copies(k, k):
                        cp.start()
                lax.fori_loop(NC - 3, 3 * D // E, issue, 0)

            return carry

        lax.fori_loop(0, NC, _scoped("p1", p1_body), 0)
        x_copy(1).start()
        x_copy(0).wait()
        wm_wait(wm_s, 0, 3 * D // E, SEM_WMR)
        mod_tiles(wm_s, 0, 3 * D // E, 2 * D // E)
        hn_s[...] = h_rows(0)

    def phase_b(t2_s, t3_s, t4_s, wg_s, x1_s, base_s, yn_s, o_s):
        for k in range(D // E):
            wm_copy(wg_s, 5 * D // E + k, k, SEM_WM).start()

        def chain_step(s, mem, htok, odef_prev, jobs=(), hooks=None):
            hs = jnp.concatenate([mem, htok], axis=0).astype(bf16)
            qkv = [[None] * 3 for _ in range(NP)]
            ps = [None] * NP
            os_ = [None] * H
            odef = [None] * H

            def proj(p, ts=(0, 1, 2)):
                for t in ts:
                    c, q = t * NG + p // (HG // 2), p % (HG // 2)
                    a = _dot(hs, _up(w_s[c, :, _ct(2 * q)]))
                    b = _dot(hs, _up(w_s[c, :, _ct(2 * q + 1)]))
                    if hooks and t == 2 and p - NP in hooks:
                        hooks[p - NP](b)
                    pre = pre_s[c, pl.ds(pl.multiple_of(s * M, M), M), _ct(q)]
                    if t == 1:
                        kf = jnp.concatenate([a, b, _up(pre).astype(f32), jnp.zeros((E - NR, E), f32)],
                                             axis=0)
                        qkv[p][t] = kf.T.astype(bf16)
                        continue
                    parts = [_pk(a), _pk(b), pre]
                    if t == 2:
                        parts.append(jnp.zeros(((E - NR) // 2, E), u32))
                    qkv[p][t] = _up(jnp.concatenate(parts, axis=0))

            def scores(p):
                sc_ = _dot(qkv[p][0], qkv[p][1])
                fill = fill_s[0:NR, :]
                sc_ = jnp.where(fill == 0.0, sc_ * SCALE, fill)
                m = jnp.max(sc_, axis=-1, keepdims=True)
                e = jnp.exp(sc_ - m)
                l = jnp.sum(e, axis=-1, keepdims=True)
                r = pl.reciprocal(l, approx=True)
                r = r * (2.0 - l * r)
                ps[p] = (e * r).astype(bf16)

            def fin(p):
                o = _dot(ps[p], qkv[p][2])
                for hh in range(2):
                    h = 2 * p + hh
                    rows = o[32 * hh:32 * hh + 32]
                    odef[h] = o[64 + 8 * hh:72 + 8 * hh]
                    if odef_prev is not None:
                        rows = jnp.concatenate([rows, odef_prev[h], odef[h]], axis=0)
                    os_[h] = _pk(rows)

            acc = [None] * 8
            jobs = iter(jobs)

            def wo(h0, h1, js):
                lhs = _up(jnp.concatenate(os_[h0:h1], axis=1))
                for j in js:
                    ws = []
                    for r0 in range(h0 * E // 2, h1 * E // 2, PIN_ROWS):
                        ws.append(pinned(lambda: wo_s[r0:r0 + PIN_ROWS, j * E:(j + 1) * E],
                                         next(jobs, None)))
                    part = _dot(lhs, _up(jnp.concatenate(ws, axis=0)))
                    if hooks and acc[j] is None and j in hooks:
                        hooks[j](part)
                    acc[j] = part if acc[j] is None else part + acc[j]

            ORDER, LAG_S, LAG_O = SCHED_A if odef_prev is None else SCHED_B
            for p in range(NP):
                if ORDER == 0:
                    proj(p)
                    if p >= LAG_S:
                        scores(p - LAG_S)
                    if p >= LAG_O:
                        fin(p - LAG_O)
                elif ORDER == 1:
                    proj(p, (1, 0))
                    if p >= LAG_O:
                        fin(p - LAG_O)
                    proj(p, (2,))
                    if p >= LAG_S:
                        scores(p - LAG_S)
                elif ORDER == 2:
                    proj(p, (1,))
                    if p >= LAG_S:
                        scores(p - LAG_S)
                    proj(p, (0,))
                    if p >= LAG_O:
                        fin(p - LAG_O)
                    proj(p, (2,))
                elif ORDER == 3:
                    proj(p, (1,))
                    if p >= LAG_O:
                        fin(p - LAG_O)
                    proj(p, (0,))
                    if p >= LAG_S:
                        scores(p - LAG_S)
                    proj(p, (2,))
                elif ORDER == 4:
                    proj(p, (1,))
                    if p >= LAG_S:
                        scores(p - LAG_S)
                    proj(p, (0, 2))
                    if p >= LAG_O:
                        fin(p - LAG_O)
                else:
                    proj(p, (0,))
                    if p >= LAG_S:
                        scores(p - LAG_S)
                    proj(p, (1,))
                    if p >= LAG_O:
                        fin(p - LAG_O)
                    proj(p, (2,))
            tail = []
            for k in range(LAG_O):
                step = []
                if NP - LAG_S + k < NP:
                    step.append(functools.partial(scores, NP - LAG_S + k))
                step.append(functools.partial(fin, NP - LAG_O + k))
                tail.append(step)
            hsplit = min(24, 2 * (NP - LAG_O))
            cuts = {3: (2, 3, 5), 2: (2, 5), 4: (1, 2, 4, 6), 5: (1, 2, 3, 4, 6)}[LAG_O]
            j0 = 0
            for k, step in enumerate(tail):
                wo(0, hsplit, range(j0, cuts[k]))
                j0 = cuts[k]
                for f in step:
                    f()
            wo(0, hsplit, range(j0, 8))
            wo(hsplit, H, range(8))
            return jnp.concatenate(acc, axis=1), odef

        def mixer_prep(i, r0, n, anchor=None):
            r = pl.ds(aligned(i * 64 + r0, 16), n)
            xr = x_s[2 * i + r0 // SEG, r0 % SEG:r0 % SEG + n, :].astype(f32)
            x2 = xr + mod_rows(2, n) * after(aout_s[r0:r0 + n, :], anchor)
            x_s.at[2 * i + r0 // SEG][r0 % SEG:r0 % SEG + n, :] = x2.astype(bf16)
            hb = _ln(x2) * mod_rows(4, n) + mod_rows(3, n)
            hb_s[r, :] = hb.astype(bf16)
            return _ln(hb)

        def mixer_sets(ya, yb, r0):
            n = ya.shape[0]
            for m, v in enumerate(_lhs_set(ya[:, :HD], ya[:, HD:], yb[:, :HD], yb[:, HD:])):
                l1_s.at[m][r0 // 2:(r0 + n) // 2, :] = _pk(v)

        def mixer_mm(i):
            for q in range(NQ):
                cs = _strassen(lambda n: _dot(_up(l1_s[n]), _up(t1_s[n, :, _ct(q)])))
                for k, cc in enumerate(cs):
                    r0 = aligned(i * 64 + 8 + (k // 2) * SEG, 8)
                    t_s[pl.ds(r0, SEG), _ct(q + NQ * (k % 2))] = _gelu(cc)

        def p2_body(i, carry):
            slot = i & 1
            for cp in mlp_w_copies(0, slot):
                cp.wait()

            @pl.when(i == 1)
            def _():
                x_copy(1).wait()

            g, rr = mlp_piece(i)
            work = [functools.partial(rhs_job, g2, slot, 0, 2 * q, 2 * q + 1, t2_s, q, i * 8)
                    for q in range(NQ)]
            work += [functools.partial(rhs2_job, g3, slot, 16 * rt, 0, n1, t3_s.at[g], rr * 32 + 8 * rt)
                     for rt in range(4) for n1 in range(7)]
            work += [functools.partial(rhs2_job, g4, slot, 16 * rt, 4 * og, n1, t4_s.at[og],
                                       g * (E // 2) + rr * 16 + 8 * rt)
                     for rt in range(2) for og in range(NOG) for n1 in range(7)]
            jobs = [None] + work

            sa_ = 2 * i
            sb_ = 2 * i + 1
            hb_tok = h_rows(sb_)
            oa, odef_a = chain_step(sa_, mem_s[...], hn_s[...], None)
            mixer_mm(jnp.maximum(i - 2, 0))
            ys = []

            def hook(k, anchor):
                if k >= PREP_CH:
                    anchor = anchor[0:8] + ys[-PREP_CH][0:8, 0:E] + ys[-PREP_CH][8:16, 0:E]
                ys.append(mixer_prep(jnp.maximum(i - 1, 0), (k % 2) * SEG + (k // 2) * 16, 16, anchor))
                if k % 2:
                    mixer_sets(ys[-2], ys[-1], (k // 2) * 16)

            hooks = {j: functools.partial(hook, k) for k, j in enumerate(PREP_AT)}
            ob, _ = chain_step(sb_, oa[0:M], hb_tok, odef_a, jobs, hooks)
            mem_s[...] = ob[0:M]
            aout_s[0:TC, :] = oa[M:SEG]
            aout_s[TC:SEG, :] = ob[SEG:SEG + M]
            aout_s[SEG:SEG + TC, :] = ob[M:SEG]
            aout_s[SEG + TC:2 * SEG, :] = ob[SEG + M:SEG + 2 * M]
            hn_s[...] = h_rows(jnp.minimum(sb_ + 1, NSEG - 1))
            for cp in mlp_w_copies(i + 2, slot):
                cp.start()
            return carry

        lax.fori_loop(0, _N2, _scoped("p2", p2_body), 0)

        TH = TB // 2
        TQ = TB // 4
        SHIFT = (-1, -1, 1, 1, -2, -2, 2, 2)

        def u_set(n):
            return w_s.at[n // 32], slice((n % 32) * (TQ // 2), (n % 32 + 1) * (TQ // 2))

        def y_set(n):
            return w_s.at[2], (n // 4) * (TQ // 2), (n % 4) * 2

        def g_rows(n, r0=0, n_rows=TH // 2):
            return slice(n * (TH // 2) + r0, n * (TH // 2) + r0 + n_rows)

        g_s = w_s.at[3]

        def g_job(j, rt, q, n=16, anchor=None):
            blk = []
            for hf in range(2):
                for ct in (q, NQ + q):
                    win = t_s[pl.ds(aligned(j * TB + hf * TH + rt * n, 16), n + 16), _ct(ct)]
                    blk.append(pltpu.roll(win, (-SHIFT[ct]) % (n + 16), 0)[8:8 + n])
            blk[0] = after(blk[0], anchor)
            blk[3] = after(blk[3], anchor)
            for k, v in enumerate(_lhs_set(*blk)):
                g_s[g_rows(k, rt * n // 2, n // 2), _ct(q)] = _pk(v)

        def mix(j):
            r0 = aligned(j * TB, TB)
            for q in range(NQ):
                cs = _strassen(lambda n: _dot(_up(g_s[g_rows(n), 0:HD]), _up(t2_s[n, :, _ct(q)])))
                cols = slice(2 * q * E, (2 * q + 2) * E)
                for hf in range(2):
                    x1_s[hf * TH:(hf + 1) * TH, cols] = (
                        hb_s[pl.ds(r0 + hf * TH, TH), cols].astype(f32)
                        + jnp.concatenate(cs[2 * hf:2 * hf + 2], axis=1))

        def base_job(j, rt, anchor):
            rows = slice(rt * 16, (rt + 1) * 16)
            z = pltpu.bitcast(pltpu.bitcast(anchor[0:8], u32) & zero_s[0:8, :], f32)
            gb = mod_rows(5, 8) + jnp.concatenate([z] * (D // E), axis=1)
            x2 = x_s[j * (TB // SEG) + rt // 2, (rt % 2) * 16:(rt % 2) * 16 + 16, :]
            base_s[rows, :] = x2.astype(f32) + jnp.concatenate([gb, gb], axis=0) * x1_s[rows, :]

        def out_copy(j, slot):
            return copy(o_s.at[slot], out_hbm.at[pl.ds(aligned(j * TB, TB), TB)], SEM_OUT + slot)

        def ln_job(r0, n, prev, anchor=None):
            if anchor is not None and len(prev) >= 2:
                anchor = anchor[0:8] + prev[-2]
            y = _ln(after(x1_s[r0:r0 + n, :], anchor))
            yn_s[r0:r0 + n, :] = y
            prev.append(y[0:8, 0:E] + y[8:16, 0:E])

        def yset_job(rt, ct, n1, n=16, anchor=None):
            blk = _outer_operand(lambda i, k: yn_s[i * TQ + rt * n:i * TQ + (rt + 1) * n, _ct(2 * k + ct)],
                                 _LHS_TERMS[n1])
            blk[0] = after(blk[0], anchor)
            blk[3] = after(blk[3], anchor)
            for n2, v in enumerate(_lhs_set(*blk)):
                ref, r0, c0 = y_set(7 * n1 + n2)
                ref[r0 + rt * n // 2:r0 + (rt + 1) * n // 2, _ct(c0 + ct)] = _pk(v)

        wm_wait(wg_s, 0, D // E, SEM_WM)
        mod_tiles(wg_s, 0, D // E, 5 * D // E)
        mixer_mm(NI - 2)
        mixer_sets(mixer_prep(NI - 1, 0, SEG), mixer_prep(NI - 1, SEG, SEG), 0)
        for q in range(NQ):
            g_job(0, 0, q, TH)
        mix(0)
        mixer_mm(NI - 1)
        ln_job(0, TB, [])
        for ct in range(2):
            for n1 in range(7):
                yset_job(0, ct, n1, TQ)
        for q in range(NQ):
            g_job(1, 0, q, TH)

        def mlp_block(j, last):
            slot = j & 1

            def up_prod(n, g):
                ref, r0, c0 = y_set(n)
                m = _dot(_up(ref[r0:r0 + TQ // 2, c0 * E:(c0 + 2) * E]), _up(t3_s[g, :, _ct(n)]))
                if n in (10, 34) and 2 * g + (n == 34) < TB // 16:
                    base_job(j, 2 * g + (n == 34), m)
                return m

            for g in range(NFG):
                c = _strassen2(lambda n: up_prod(n, g))
                act = [[_gelu(c(i, k)) for k in range(4)] for i in range(4)]
                for n1 in range(7):
                    blk = _outer_operand(lambda i, k: act[i][k], _LHS_TERMS[n1])
                    for n2, v in enumerate(_lhs_set(*blk)):
                        ref, rows = u_set(7 * n1 + n2)
                        ref[rows, _ct(g)] = _pk(v)
            jobs = {}
            if not last:
                mix(j + 1)
                jn = clamp(j + 2, NB - 1)
                prev = []
                for k in range(TB // 16):
                    jobs[k * Y_AT] = functools.partial(ln_job, (k % 4) * TQ + (k // 4) * 16, 16, prev)

                def place(start, fns):
                    for fn in fns:
                        while start in jobs:
                            start += 1
                        jobs[start] = fn

                for rt in range(2):
                    place(S_AT[rt], [functools.partial(yset_job, rt, ct, n1, 16)
                                     for ct in range(2) for n1 in range(7)])
                place(G_AT, [functools.partial(g_job, jn, k // NQ, k % NQ, 16)
                             for k in range(TH // 16 * NQ)])

            def down_part(n, og, k0, k1):
                ref, rows = u_set(n)
                return _dot(_up(ref[rows, k0 * E:k1 * E]),
                            _up(t4_s[og, k0 * E // 2:k1 * E // 2, _ct(n)]))

            head = {}
            if last:
                head = {n: down_part(n, 0, 0, NFG - 1) for n in range(HEAD)}
            count = [0]

            def down_prod(n, og):
                if og == 0 and n in head:
                    return down_part(n, og, NFG - 1, NFG) + head[n]
                m = down_part(n, og, 0, NFG)
                job = jobs.get(count[0])
                count[0] += 1
                if job is not None:
                    job(anchor=m)
                return m

            for og in range(NOG):
                c = _strassen2(lambda n: down_prod(n, og))
                for i in range(4):
                    rows = slice(i * TQ, (i + 1) * TQ)
                    for k in range(2):
                        c0 = (4 * og + 2 * k) * E
                        o_s.at[slot][rows, c0:c0 + 2 * E] = (
                            base_s[rows, c0:c0 + 2 * E] + mod_rows(5, TQ, c0, 2 * E)
                            * jnp.concatenate([c(i, 2 * k), c(i, 2 * k + 1)], axis=1)).astype(bf16)
            out_copy(j, slot).start()

        def p3_body(j, carry):
            @pl.when(j >= 2)
            def _():
                out_copy(j - 2, j & 1).wait()

            mlp_block(j, False)
            return carry

        lax.fori_loop(0, NB - 1, _scoped("p3", p3_body), 0)
        for k in range(2):
            for cp in mlp_w_copies(0, k):
                cp.wait()
        out_copy(NB - 3, (NB - 3) % 2).wait()
        mlp_block(NB - 1, True)
        out_copy(NB - 2, (NB - 2) % 2).wait()
        out_copy(NB - 1, (NB - 1) % 2).wait()

    pl.run_scoped(
        phase_a,
        pltpu.VMEM((NSEG, M, D), bf16),
        pltpu.VMEM((7, NSEG * M // 4, D // 2), u32),
        pltpu.VMEM((3 * D // E, D, E), bf16),
        pltpu.VMEM((2, D, HG, E), bf16),
        pltpu.VMEM((2, BGR, D), bf16),
        pltpu.VMEM((2, 2, G1R, D), bf16),
    )
    pl.run_scoped(
        phase_b,
        pltpu.VMEM((7, D // 4, D // 2), u32),
        pltpu.VMEM((NFG, D // 8, 49 * E), u32),
        pltpu.VMEM((NOG, F // 8, 49 * E), u32),
        pltpu.VMEM((D // E, D, E), bf16),
        pltpu.VMEM((TB, D), f32),
        pltpu.VMEM((TB, D), f32),
        pltpu.VMEM((TB, D), f32),
        pltpu.VMEM((2, TB, D), bf16),
    )


@jax.jit
def pallas_adaLN_cond__memory_aug_recurrent_mem_tr__mixer_s_mlp__prompt_kernel(
    A_x: jax.Array,
    A_mem0: jax.Array,
    A_Wq: jax.Array,
    A_Wk: jax.Array,
    A_Wv: jax.Array,
    A_Wo: jax.Array,
    A_seg_len,
    B_x: jax.Array,
    B_w1: jax.Array,
    B_w2: jax.Array,
    B_w3: jax.Array,
    B_w4: jax.Array,
    c: jax.Array,
    w_mod: jax.Array,
):
    del A_seg_len, B_x
    assert A_x.shape == (1, S, D) and A_mem0.shape == (1, M, D)
    hbm = pl.BlockSpec(memory_space=pl.ANY)
    scratch = [
        pltpu.VMEM((NSEG, SEG, D), bf16),
        pltpu.VMEM((NC + 3, D // 2, HG * E), u32),
        pltpu.VMEM((H * E // 2, D), u32),
        pltpu.VMEM((7, D // 4, D // 2), u32),
        pltpu.VMEM((2, 2, 16, D), bf16),
        pltpu.VMEM((2, 4, 64, 4 * E), bf16),
        pltpu.VMEM((2, 4, 32, D), bf16),
        pltpu.VMEM((NC + 2, NSEG * M, HG // 2 * E), u32),
        pltpu.VMEM((8, 6 * D), f32),
        pltpu.VMEM((M, D), f32),
        pltpu.VMEM((TC, D), f32),
        pltpu.VMEM((2 * SEG, D), f32),
        pltpu.VMEM((E, E), f32),
        pltpu.VMEM((S, D), bf16),
        pltpu.VMEM((S + 16, D), f32),
        pltpu.VMEM((7, SEG // 2, D // 2), u32),
        pltpu.VMEM((8 * ZPAD, E), u32),
        pltpu.VMEM((1, D), bf16),
        pltpu.VMEM((M, D), bf16),
        pltpu.SemaphoreType.DMA((24,)),
    ]
    out = pl.pallas_call(
        _kernel,
        out_shape=jax.ShapeDtypeStruct((S, D), bf16),
        in_specs=[hbm] * 12,
        out_specs=hbm,
        scratch_shapes=scratch,
        compiler_params=pltpu.CompilerParams(vmem_limit_bytes=127 * 1024 * 1024,
                                             disable_bounds_checks=NO_BOUNDS),
    )(A_x.reshape(NSEG, SEG, D), A_mem0.reshape(M, D), A_Wq, A_Wk, A_Wv,
      A_Wo.reshape(H * E, D), B_w1.reshape(2, D // 2, D), B_w2.reshape(2, D // 2, D), B_w3.reshape(4, D // 4, F),
      B_w4.reshape(NFG, 4, E, D), c, w_mod)
    return out.reshape(1, S, D)
```

```python
import functools

import jax
import jax.numpy as jnp
from jax import lax
import jax.experimental.pallas as pl
import jax.experimental.pallas.tpu as pltpu

bf16, f32, u32 = jnp.bfloat16, jnp.float32, jnp.uint32

S, D, H, E, M, SEG, F = 2048, 1024, 32, 128, 8, 32, 3584
NSEG = S // SEG
NP = H // 2
TC = SEG - M
HG = 8
NG = H // HG
TB = 128
NB = S // TB
NFG = F // (4 * E)
NOG = D // (4 * E)
NI = NSEG // 2
NQ = D // E // 2
NC = 3 * NG
BGR = 384
G1R = 48
HD = D // 2
X0 = 4
NR = 2 * (M + SEG)
NO_BOUNDS = True
ZPAD = 2
PIN_ROWS = 256
Y_AT = 4
S_AT = (26, 44)
G_AT = 62
HEAD = 14
PREP_AT = (0, 1, 3, 4)
PREP_CH = 2
O3 = (1, 0)
O4 = (0, 0)
G_STEP = 1
FINE = 1
JGROUP = 1
P1_TAIL = 5
P1_LAG = 4
SCHED_A = (2, 1, 3)
SCHED_B = (3, 1, 3)
EPS = 1e-5
SCALE = E ** -0.5
_SCOPES = False
_N2 = NSEG // 2


def _scoped(name, fn):
    def wrapped(*a):
        if not _SCOPES:
            return fn(*a)
        with jax.named_scope(name):
            return fn(*a)
    return wrapped


def _pk(x):
    return pltpu.bitcast(x.astype(bf16), u32)


def _up(x):
    return pltpu.bitcast(x, bf16)


def _ct(k):
    return slice(k * E, (k + 1) * E)


def _dot(a, b):
    return jnp.dot(a, b, preferred_element_type=f32)


def _ln(x):
    m = jnp.mean(x, axis=-1, keepdims=True)
    xc = x - m
    v = jnp.mean(xc * xc, axis=-1, keepdims=True)
    return xc * lax.rsqrt(v + EPS)


def _gelu(x):
    c = 0.7978845608028654
    return 0.5 * x * (1.0 + jnp.tanh(c * (x + 0.044715 * (x * x * x))))


def _lhs_set(a11, a12, a21, a22):
    return (a11 + a22, a21 + a22, a11, a22, a11 + a12, a21 - a11, a12 - a22)


def _rhs_set(b11, b12, b21, b22):
    return (b11 + b22, b11, b12 - b22, b21 - b11, b22, b11 + b12, b21 + b22)


_LHS_TERMS = (((0, 1), (3, 1)), ((2, 1), (3, 1)), ((0, 1),), ((3, 1),),
              ((0, 1), (1, 1)), ((2, 1), (0, -1)), ((1, 1), (3, -1)))
_RHS_TERMS = (((0, 1), (3, 1)), ((0, 1),), ((1, 1), (3, -1)), ((2, 1), (0, -1)),
              ((3, 1),), ((0, 1), (1, 1)), ((2, 1), (3, 1)))


def _outer_operand(tile, terms):
    out = []
    for i in range(2):
        for j in range(2):
            v = None
            for o, sign in terms:
                t = tile(2 * (o // 2) + i, 2 * (o % 2) + j)
                v = t if v is None else (v + t if sign > 0 else v - t)
            out.append(v)
    return out


class _Quad:
    def __init__(self, tiles):
        self.t = tuple(tiles)

    def __add__(self, other):
        return _Quad([a + b for a, b in zip(self.t, other.t)])

    def __sub__(self, other):
        return _Quad([a - b for a, b in zip(self.t, other.t)])


def _strassen2(m, oo=0, oi=0):
    cs = _strassen(lambda n1: _Quad(_strassen(lambda n2: m(7 * n1 + n2), oi)), oo)
    return lambda i, j: cs[2 * (i // 2) + j // 2].t[2 * (i % 2) + j % 2]


def _strassen(m, order=0):
    if order == 0:
        m1 = m(0)
        m2 = m(1)
        c22 = m1 - m2
        m3 = m(2)
        c22 = c22 + m3
        c22 = m(5) + c22
        m4 = m(3)
        c21 = m2 + m4
        c11 = m1 + m4
        m5 = m(4)
        c12 = m3 + m5
        c11 = c11 - m5
        c11 = m(6) + c11
    else:
        m2 = m(1)
        c22 = m(5) - m2
        m4 = m(3)
        c21 = m2 + m4
        m1 = m(0)
        c22 = c22 + m1
        c11 = m4 + m1
        m3 = m(2)
        c22 = c22 + m3
        m5 = m(4)
        c12 = m3 + m5
        c11 = c11 - m5
        c11 = m(6) + c11
    return c11, c12, c21, c22


def _mask_fill():
    shape = (NR, E)
    r = lax.broadcasted_iota(jnp.int32, shape, 0)
    c = lax.broadcasted_iota(jnp.int32, shape, 1)

    def headpos(i):
        head = jnp.where(i < 64, i >> 5, (i - 64) >> 3)
        pos = jnp.where(i < 64, i & 31, 32 + (i & 7))
        return head, pos

    hr, pr = headpos(r)
    hc, pc = headpos(c)
    same = hr == hc
    valid = same & ((pr < M) | (pr >= pc))
    return jnp.where(valid, 0.0, jnp.where(same, -1e9, -jnp.inf)).astype(f32)


def _kernel(x_hbm, mem0_hbm, wq_hbm, wk_hbm, wv_hbm, wo_hbm, w1_hbm, w2_hbm, w3_hbm,
            w4_hbm, c_hbm, wm_hbm,
            out_hbm,
            x_s, w_s, wo_s, t1_s, g2, g3, g4, pre_s, mod_s, mem_s, hn_s, aout_s, fill_s,
            hb_s, t_s, l1_s, zero_s, c_s, mem0_s, sems):
    w_hbm = (wq_hbm, wk_hbm, wv_hbm)

    (SEM_C, SEM_MEM, SEM_XPRE, SEM_X, SEM_STG, SEM_BG, SEM_OUT,
     SEM_WMR, SEM_G2, SEM_G3, SEM_G4, SEM_WM, SEM_G1) = (0, 1, 2, 3, 4, 6, 8, 10, 12, 14, 16, 18, 22)

    def copy(src, dst, k):
        return pltpu.make_async_copy(src, dst, sems.at[k])

    def aligned(x, n):
        return x if isinstance(x, int) else pl.multiple_of(x, n)

    def clamp(k, hi):
        return min(k, hi) if isinstance(k, int) else jnp.minimum(k, hi)

    def mlp_piece(k):
        k = clamp(k, 4 * NFG - 1)
        return k >> 2, k & 3

    def mlp_w_copies(k, slot):
        g, rr = mlp_piece(k)
        r = pl.ds(aligned(clamp(k, NI - 1) * 16, 16), 16)
        return (copy(w2_hbm.at[:, r, :], g2.at[slot], SEM_G2 + slot),
                copy(w3_hbm.at[:, pl.ds(aligned(rr * 64, 64), 64), pl.ds(aligned(g * 4 * E, E), 4 * E)],
                     g3.at[slot], SEM_G3 + slot),
                copy(w4_hbm.at[g, :, pl.ds(aligned(rr * 32, 32), 32), :], g4.at[slot], SEM_G4 + slot))

    def pinned(w, job):
        if job is None:
            return w()
        z = job() & zero_s[0:8, :]
        w = w()
        return jnp.concatenate([w[0:8] | z, w[8:]], axis=0)

    def after(x, anchor):
        if anchor is None:
            return x
        z = pltpu.bitcast(pltpu.bitcast(anchor[0:8], u32) & zero_s[0:8, :], f32)
        z = jnp.concatenate([z] * (x.shape[0] // 8), axis=0)
        return jnp.concatenate([x[:, 0:E] + z, x[:, E:]], axis=1) if x.shape[1] > E else x + z

    def rhs_job(src, slot, r0, c1, c2, dst, q, row, z=None):
        blk = [src[slot, kh, r0:r0 + 16, cc * E:(cc + 1) * E].astype(f32)
               for kh in range(2) for cc in (c1, c2)]
        if z is not None:
            zf = pltpu.bitcast(jnp.concatenate([z, z], axis=0), f32)
            blk[0] = blk[0] + zf
            blk[3] = blk[3] + zf
        sets = _rhs_set(*blk)
        for n, v in enumerate(sets):
            dst.at[n][pl.ds(pl.multiple_of(row, 8), 8), _ct(q)] = _pk(v)
        out = pltpu.bitcast(sets[2], u32) | pltpu.bitcast(sets[3], u32)
        return out[0:8] | out[8:16]

    def rhs2_job(src, slot, r0, c0, n1, dst, row):
        blk = _outer_operand(lambda i, j: src[slot, i, r0:r0 + 16, _ct(c0 + j)].astype(f32),
                             _RHS_TERMS[n1])
        sets = _rhs_set(*blk)
        for n2, v in enumerate(sets):
            dst[pl.ds(pl.multiple_of(row, 8), 8), _ct(7 * n1 + n2)] = _pk(v)
        out = pltpu.bitcast(sets[2], u32) | pltpu.bitcast(sets[3], u32)
        return out[0:8] | out[8:16]

    def silu_c():
        cf = c_s[...].astype(f32)
        return jnp.broadcast_to(cf * (1.0 / (1.0 + jnp.exp(-cf))), (8, D)).astype(bf16)

    def wm_copy(wm_s, src_tile, dst_tile, sem):
        return copy(wm_hbm.at[:, pl.ds(aligned(src_tile * E, E), E)], wm_s.at[dst_tile], sem)

    def wm_wait(wm_s, t0, n, sem):
        copy(wm_s.at[t0:t0 + n], wm_s.at[t0:t0 + n], sem).wait()

    def mod_tiles(wm_s, t0, n, dst_tile):
        sc8 = silu_c()
        for k in range(n):
            v = _dot(sc8, wm_s[t0 + k])
            if (dst_tile + k) // (D // E) in (1, 4):
                v = 1.0 + v
            mod_s[:, _ct(dst_tile + k)] = v

    def x_copy(k):
        r = slice(0, X0) if k == 0 else slice(X0, NSEG)
        return copy(x_hbm.at[r], x_s.at[r], SEM_XPRE if k == 0 else SEM_X)

    def h_rows(s):
        return _ln(x_s[s, 0:TC, :].astype(f32)) * mod_rows(1, TC) + mod_rows(0, TC)

    def mod_rows(k, n, c0=0, w=D):
        return jnp.concatenate([mod_s[:, k * D + c0:k * D + c0 + w]] * (n // 8), axis=0)

    def tq_place(c, n):
        if n == 1:
            return w_s.at[c], 0, None
        if n == 4:
            return w_s.at[c], D // 4, None
        if n == 6:
            return pre_s.at[c + 1], 0, 0
        k = (0, 2, 3, 5).index(n)
        return w_s.at[c + 2], (k // 2) * (D // 4), (k % 2) * (HG // 2)

    def phase_a(xpre_s, hpre_s, wm_s, stg, bg, g1):
        def w_copy(t, g, slot):
            return copy(w_hbm[t].at[:, pl.ds(pl.multiple_of(g * HG, HG), HG), :], stg.at[slot],
                        SEM_STG + slot)

        def bg_rows(k):
            return clamp(k * BGR, H * E - BGR), clamp(k * G1R, HD - G1R)

        def bg_copies(k, slot):
            ro, r1 = bg_rows(k)
            return (copy(wo_hbm.at[pl.ds(aligned(ro, 16), BGR)], bg.at[slot], SEM_BG + slot),
                    copy(w1_hbm.at[:, pl.ds(aligned(r1, 16), G1R), :], g1.at[slot], SEM_G1 + slot))

        def relayout_jobs(slot, c, i):
            memo = []
            r = aligned(i * 8, 8)

            def job(j, z=None):
                if not memo:
                    for d0 in (i * 16, HD + i * 16):
                        memo.append(jnp.swapaxes(pltpu.bitcast(stg[slot, pl.ds(d0, 16)], u32), 0, 1))
                blk = []
                for kh in range(2):
                    u = memo[kh][j]
                    if z is not None:
                        u = u | jnp.concatenate([z, z], axis=0)
                    blk.append(pltpu.bitcast(u << 16, f32))
                    blk.append(pltpu.bitcast(u & jnp.uint32(0xFFFF0000), f32))
                for k, v in enumerate(blk):
                    w_s.at[c][pl.ds((k // 2) * (D // 4) + r, 8), _ct(2 * j + k % 2)] = _pk(v)
                for n, v in enumerate(_rhs_set(*blk)):
                    if n not in (1, 4):
                        ref, r0, c0 = tq_place(c, n)
                        ref[pl.ds(r0 + r, 8), _ct(c0 + j)] = _pk(v)

            return [functools.partial(job, j) for j in range(HG // 2)]

        def repack(slot, row, i, z):
            v = pltpu.bitcast(bg[slot, 16 * i:16 * i + 16, :], u32)
            v = v | jnp.concatenate([z] * (D // E), axis=1)
            wo_s[pl.ds(pl.multiple_of(row + 8 * i, 8), 8), :] = v

        cp_c = copy(c_hbm, c_s, SEM_C)
        cp_mem = copy(mem0_hbm, mem0_s, SEM_MEM)
        cp_xpre = copy(x_hbm.at[:, TC:SEG, :], xpre_s, SEM_XPRE)
        w_copy(0, 0, 0).start()
        cp_xpre.start()
        cp_c.start()
        cp_mem.start()
        for k in range(2 * D // E):
            wm_copy(wm_s, k, k, SEM_WM + k // 4).start()
        w_copy(0, 1, 1).start()

        zero_s[0:8, :] = jnp.zeros((8, E), u32)
        fill_s[0:NR, :] = _mask_fill()
        aout_s[...] = jnp.zeros(aout_s.shape, f32)
        l1_s[...] = jnp.zeros(l1_s.shape, u32)
        bg[1] = jnp.zeros(bg.shape[1:], bf16)
        g1[1] = jnp.zeros(g1.shape[1:], bf16)

        w_copy(0, 0, 0).wait()

        def rl0_body(i, carry):
            for job in relayout_jobs(0, 0, i):
                job()
            return carry

        lax.fori_loop(0, D // 32, rl0_body, 0)
        w_copy(0, 2, 0).start()
        for cp in bg_copies(0, 0):
            cp.start()

        cp_xpre.wait()

        def npre_body(i, carry):
            xr = xpre_s[pl.ds(pl.multiple_of(i * 8, 8), 8)].astype(f32).reshape(64, D)
            t_s[pl.ds(pl.multiple_of(i * 64, 64), 64), :] = _ln(xr)
            return carry

        lax.fori_loop(0, NSEG // 8, _scoped("npre", npre_body), 0)

        cp_c.wait()
        cp_mem.wait()
        mem_s[...] = mem0_s[...].astype(f32)

        for k in range(4):
            wm_wait(wm_s, 4 * k, 4, SEM_WM + k)
            mod_tiles(wm_s, 4 * k, 4, 4 * k)

        PH = NSEG * M // 2

        def hpre_body(i, carry):
            h = [t_s[pl.ds(pl.multiple_of(hf * PH + i * 16, 16), 16), :] * mod_rows(1, 16) + mod_rows(0, 16)
                 for hf in range(2)]
            for n, v in enumerate(_lhs_set(h[0][:, :HD], h[0][:, HD:], h[1][:, :HD], h[1][:, HD:])):
                hpre_s.at[n][pl.ds(pl.multiple_of(i * 8, 8), 8), :] = _pk(v)
            return carry

        lax.fori_loop(0, PH // 16, _scoped("hpre", hpre_body), 0)

        t_s[0:8, :] = jnp.zeros((8, D), f32)
        t_s[S + 8:S + 16, :] = jnp.zeros((8, D), f32)

        MB = 64

        def p1_body(c, carry):
            slot = c & 1
            pslot = 1 - slot
            ro, r1 = bg_rows(jnp.maximum(c - 1, 0))

            @pl.when(c >= 1)
            def _():
                for cp in bg_copies(0, pslot):
                    cp.wait()

            @pl.when(c + 1 < NC)
            def _():
                w_copy(0, 0, pslot).wait()

            small = [functools.partial(repack, pslot, ro >> 1, i) for i in range(BGR // 16)]
            small += [functools.partial(rhs_job, g1, pslot, 16 * rt, q, NQ + q, t1_s, q, (r1 >> 1) + 8 * rt)
                      for rt in range(G1R // 16) for q in range(NQ)]
            work = []
            nu = D // 32
            for i in range(nu):
                js = relayout_jobs(pslot, c + 1, i)
                work += [js[k:k + JGROUP] for k in range(0, len(js), JGROUP)]
                work += [[job] for job in small[i * len(small) // nu:(i + 1) * len(small) // nu]]
            npin = 7 * (HG // 2) * (PH // MB)
            jobs = [[] for _ in range(npin)]
            for k, group in enumerate(work):
                pos = k * (npin - P1_TAIL) * 8 // len(work)
                jobs[pos // 8] += [(job, pos % 8 if FINE else 0) for job in group]
            jobs = iter(jobs)

            def prod(n, q, mb):
                ref, r0, c0 = tq_place(c, n)
                w = ref[r0:r0 + D // 4, _ct(2 * q + (n == 4) if c0 is None else c0 + q)]
                m = _dot(_up(hpre_s[n, mb * MB // 2:(mb + 1) * MB // 2, :]), _up(w))
                pending.append(m)
                if len(pending) > P1_LAG:
                    anchor = pltpu.bitcast(pending.pop(0), u32)
                    for job, g in next(jobs):
                        job(anchor[8 * g:8 * g + 8] & zero_s[0:8, :])
                return m

            pending = []
            ns = MB // M
            for q in range(HG // 2):
                for mb in range(PH // MB):
                    cs = _strassen(lambda n: prod(n, q, mb))
                    for hf in range(2):
                        y = jnp.concatenate([cs[2 * hf + k][sg * M:(sg + 1) * M]
                                             for sg in range(ns) for k in range(2)], axis=0)
                        s0 = hf * (NSEG // 2) + mb * ns
                        pre_s.at[c][s0 * M:(s0 + ns) * M, _ct(q)] = _pk(y)

            for t in range(3):
                @pl.when((c + 3) >> 2 == t)
                def _():
                    w_copy(t, (c + 3) & 3, pslot).start()

            @pl.when(c + 2 < NC)
            def _():
                for cp in bg_copies(c + 1, pslot):
                    cp.start()

            @pl.when(c < NC - 3)
            def _():
                wm_copy(wm_s, 2 * D // E + c, c, SEM_WMR).start()

            @pl.when(c == NC - 3)
            def _():
                def issue(k, carry2):
                    wm_copy(wm_s, 2 * D // E + k, k, SEM_WMR).start()
                    return carry2

                x_copy(0).start()
                for k in range(2):
                    for cp in mlp_w_copies(k, k):
                        cp.start()
                lax.fori_loop(NC - 3, 3 * D // E, issue, 0)

            return carry

        lax.fori_loop(0, NC, _scoped("p1", p1_body), 0)
        x_copy(1).start()
        x_copy(0).wait()
        wm_wait(wm_s, 0, 3 * D // E, SEM_WMR)
        mod_tiles(wm_s, 0, 3 * D // E, 2 * D // E)
        hn_s[...] = h_rows(0)

    def phase_b(t2_s, t3_s, t4_s, wg_s, x1_s, base_s, yn_s, o_s):
        for k in range(D // E):
            wm_copy(wg_s, 5 * D // E + k, k, SEM_WM).start()

        def chain_step(s, mem, htok, odef_prev, jobs=(), hooks=None):
            hs = jnp.concatenate([mem, htok], axis=0).astype(bf16)
            qkv = [[None] * 3 for _ in range(NP)]
            ps = [None] * NP
            os_ = [None] * H
            odef = [None] * H

            def proj(p, ts=(0, 1, 2)):
                for t in ts:
                    c, q = t * NG + p // (HG // 2), p % (HG // 2)
                    a = _dot(hs, _up(w_s[c, :, _ct(2 * q)]))
                    b = _dot(hs, _up(w_s[c, :, _ct(2 * q + 1)]))
                    if hooks and t == 2 and p - NP in hooks:
                        hooks[p - NP](b)
                    pre = pre_s[c, pl.ds(pl.multiple_of(s * M, M), M), _ct(q)]
                    if t == 1:
                        kf = jnp.concatenate([a, b, _up(pre).astype(f32), jnp.zeros((E - NR, E), f32)],
                                             axis=0)
                        qkv[p][t] = kf.T.astype(bf16)
                        continue
                    parts = [_pk(a), _pk(b), pre]
                    if t == 2:
                        parts.append(jnp.zeros(((E - NR) // 2, E), u32))
                    qkv[p][t] = _up(jnp.concatenate(parts, axis=0))

            def scores(p):
                sc_ = _dot(qkv[p][0], qkv[p][1])
                fill = fill_s[0:NR, :]
                sc_ = jnp.where(fill == 0.0, sc_ * SCALE, fill)
                m = jnp.max(sc_, axis=-1, keepdims=True)
                e = jnp.exp(sc_ - m)
                l = jnp.sum(e, axis=-1, keepdims=True)
                r = pl.reciprocal(l, approx=True)
                r = r * (2.0 - l * r)
                ps[p] = (e * r).astype(bf16)

            def fin(p):
                o = _dot(ps[p], qkv[p][2])
                for hh in range(2):
                    h = 2 * p + hh
                    rows = o[32 * hh:32 * hh + 32]
                    odef[h] = o[64 + 8 * hh:72 + 8 * hh]
                    if odef_prev is not None:
                        rows = jnp.concatenate([rows, odef_prev[h], odef[h]], axis=0)
                    os_[h] = _pk(rows)

            acc = [None] * 8
            jobs = iter(jobs)

            def wo(h0, h1, js):
                lhs = _up(jnp.concatenate(os_[h0:h1], axis=1))
                for j in js:
                    ws = []
                    for r0 in range(h0 * E // 2, h1 * E // 2, PIN_ROWS):
                        ws.append(pinned(lambda: wo_s[r0:r0 + PIN_ROWS, j * E:(j + 1) * E],
                                         next(jobs, None)))
                    part = _dot(lhs, _up(jnp.concatenate(ws, axis=0)))
                    if hooks and acc[j] is None and j in hooks:
                        hooks[j](part)
                    acc[j] = part if acc[j] is None else part + acc[j]

            ORDER, LAG_S, LAG_O = SCHED_A if odef_prev is None else SCHED_B
            for p in range(NP):
                if ORDER == 0:
                    proj(p)
                    if p >= LAG_S:
                        scores(p - LAG_S)
                    if p >= LAG_O:
                        fin(p - LAG_O)
                elif ORDER == 1:
                    proj(p, (1, 0))
                    if p >= LAG_O:
                        fin(p - LAG_O)
                    proj(p, (2,))
                    if p >= LAG_S:
                        scores(p - LAG_S)
                elif ORDER == 2:
                    proj(p, (1,))
                    if p >= LAG_S:
                        scores(p - LAG_S)
                    proj(p, (0,))
                    if p >= LAG_O:
                        fin(p - LAG_O)
                    proj(p, (2,))
                elif ORDER == 3:
                    proj(p, (1,))
                    if p >= LAG_O:
                        fin(p - LAG_O)
                    proj(p, (0,))
                    if p >= LAG_S:
                        scores(p - LAG_S)
                    proj(p, (2,))
                elif ORDER == 4:
                    proj(p, (1,))
                    if p >= LAG_S:
                        scores(p - LAG_S)
                    proj(p, (0, 2))
                    if p >= LAG_O:
                        fin(p - LAG_O)
                else:
                    proj(p, (0,))
                    if p >= LAG_S:
                        scores(p - LAG_S)
                    proj(p, (1,))
                    if p >= LAG_O:
                        fin(p - LAG_O)
                    proj(p, (2,))
            tail = []
            for k in range(LAG_O):
                step = []
                if NP - LAG_S + k < NP:
                    step.append(functools.partial(scores, NP - LAG_S + k))
                step.append(functools.partial(fin, NP - LAG_O + k))
                tail.append(step)
            hsplit = min(24, 2 * (NP - LAG_O))
            cuts = {3: (2, 3, 5), 2: (2, 5), 4: (1, 2, 4, 6), 5: (1, 2, 3, 4, 6)}[LAG_O]
            j0 = 0
            for k, step in enumerate(tail):
                wo(0, hsplit, range(j0, cuts[k]))
                j0 = cuts[k]
                for f in step:
                    f()
            wo(0, hsplit, range(j0, 8))
            wo(hsplit, H, range(8))
            return jnp.concatenate(acc, axis=1), odef

        def mixer_prep(i, r0, n, anchor=None):
            r = pl.ds(aligned(i * 64 + r0, 16), n)
            xr = x_s[2 * i + r0 // SEG, r0 % SEG:r0 % SEG + n, :].astype(f32)
            x2 = xr + mod_rows(2, n) * after(aout_s[r0:r0 + n, :], anchor)
            x_s.at[2 * i + r0 // SEG][r0 % SEG:r0 % SEG + n, :] = x2.astype(bf16)
            hb = _ln(x2) * mod_rows(4, n) + mod_rows(3, n)
            hb_s[r, :] = hb.astype(bf16)
            return _ln(hb)

        def mixer_sets(ya, yb, r0):
            n = ya.shape[0]
            for m, v in enumerate(_lhs_set(ya[:, :HD], ya[:, HD:], yb[:, :HD], yb[:, HD:])):
                l1_s.at[m][r0 // 2:(r0 + n) // 2, :] = _pk(v)

        def mixer_mm(i):
            for q in range(NQ):
                cs = _strassen(lambda n: _dot(_up(l1_s[n]), _up(t1_s[n, :, _ct(q)])))
                for k, cc in enumerate(cs):
                    r0 = aligned(i * 64 + 8 + (k // 2) * SEG, 8)
                    t_s[pl.ds(r0, SEG), _ct(q + NQ * (k % 2))] = _gelu(cc)

        def p2_body(i, carry):
            slot = i & 1
            for cp in mlp_w_copies(0, slot):
                cp.wait()

            @pl.when(i == 1)
            def _():
                x_copy(1).wait()

            g, rr = mlp_piece(i)
            work = [functools.partial(rhs_job, g2, slot, 0, 2 * q, 2 * q + 1, t2_s, q, i * 8)
                    for q in range(NQ)]
            work += [functools.partial(rhs2_job, g3, slot, 16 * rt, 0, n1, t3_s.at[g], rr * 32 + 8 * rt)
                     for rt in range(4) for n1 in range(7)]
            work += [functools.partial(rhs2_job, g4, slot, 16 * rt, 4 * og, n1, t4_s.at[og],
                                       g * (E // 2) + rr * 16 + 8 * rt)
                     for rt in range(2) for og in range(NOG) for n1 in range(7)]
            jobs = [None] + work

            sa_ = 2 * i
            sb_ = 2 * i + 1
            hb_tok = h_rows(sb_)
            oa, odef_a = chain_step(sa_, mem_s[...], hn_s[...], None)
            mixer_mm(jnp.maximum(i - 2, 0))
            ys = []

            def hook(k, anchor):
                if k >= PREP_CH:
                    anchor = anchor[0:8] + ys[-PREP_CH][0:8, 0:E] + ys[-PREP_CH][8:16, 0:E]
                ys.append(mixer_prep(jnp.maximum(i - 1, 0), (k % 2) * SEG + (k // 2) * 16, 16, anchor))
                if k % 2:
                    mixer_sets(ys[-2], ys[-1], (k // 2) * 16)

            hooks = {j: functools.partial(hook, k) for k, j in enumerate(PREP_AT)}
            ob, _ = chain_step(sb_, oa[0:M], hb_tok, odef_a, jobs, hooks)
            mem_s[...] = ob[0:M]
            aout_s[0:TC, :] = oa[M:SEG]
            aout_s[TC:SEG, :] = ob[SEG:SEG + M]
            aout_s[SEG:SEG + TC, :] = ob[M:SEG]
            aout_s[SEG + TC:2 * SEG, :] = ob[SEG + M:SEG + 2 * M]
            hn_s[...] = h_rows(jnp.minimum(sb_ + 1, NSEG - 1))
            for cp in mlp_w_copies(i + 2, slot):
                cp.start()
            return carry

        lax.fori_loop(0, _N2, _scoped("p2", p2_body), 0)

        TH = TB // 2
        TQ = TB // 4
        SHIFT = (-1, -1, 1, 1, -2, -2, 2, 2)

        def u_set(n):
            return w_s.at[n // 32], slice((n % 32) * (TQ // 2), (n % 32 + 1) * (TQ // 2))

        def y_set(n):
            return w_s.at[2], (n // 4) * (TQ // 2), (n % 4) * 2

        def g_rows(n, r0=0, n_rows=TH // 2):
            return slice(n * (TH // 2) + r0, n * (TH // 2) + r0 + n_rows)

        g_s = w_s.at[3]

        def g_job(j, rt, q, n=16, anchor=None):
            blk = []
            for hf in range(2):
                for ct in (q, NQ + q):
                    win = t_s[pl.ds(aligned(j * TB + hf * TH + rt * n, 16), n + 16), _ct(ct)]
                    blk.append(pltpu.roll(win, (-SHIFT[ct]) % (n + 16), 0)[8:8 + n])
            blk[0] = after(blk[0], anchor)
            blk[3] = after(blk[3], anchor)
            for k, v in enumerate(_lhs_set(*blk)):
                g_s[g_rows(k, rt * n // 2, n // 2), _ct(q)] = _pk(v)

        def mix(j):
            r0 = aligned(j * TB, TB)
            for q in range(NQ):
                cs = _strassen(lambda n: _dot(_up(g_s[g_rows(n), 0:HD]), _up(t2_s[n, :, _ct(q)])))
                cols = slice(2 * q * E, (2 * q + 2) * E)
                for hf in range(2):
                    x1_s[hf * TH:(hf + 1) * TH, cols] = (
                        hb_s[pl.ds(r0 + hf * TH, TH), cols].astype(f32)
                        + jnp.concatenate(cs[2 * hf:2 * hf + 2], axis=1))

        def base_job(j, rt, anchor):
            rows = slice(rt * 16, (rt + 1) * 16)
            z = pltpu.bitcast(pltpu.bitcast(anchor[0:8], u32) & zero_s[0:8, :], f32)
            gb = mod_rows(5, 8) + jnp.concatenate([z] * (D // E), axis=1)
            x2 = x_s[j * (TB // SEG) + rt // 2, (rt % 2) * 16:(rt % 2) * 16 + 16, :]
            base_s[rows, :] = x2.astype(f32) + jnp.concatenate([gb, gb], axis=0) * x1_s[rows, :]

        def out_copy(j, slot):
            return copy(o_s.at[slot], out_hbm.at[pl.ds(aligned(j * TB, TB), TB)], SEM_OUT + slot)

        def ln_job(r0, n, prev, anchor=None):
            if anchor is not None and len(prev) >= 2:
                anchor = anchor[0:8] + prev[-2]
            y = _ln(after(x1_s[r0:r0 + n, :], anchor))
            yn_s[r0:r0 + n, :] = y
            prev.append(y[0:8, 0:E] + y[8:16, 0:E])

        def yset_job(rt, ct, n1, n=16, anchor=None):
            blk = _outer_operand(lambda i, k: yn_s[i * TQ + rt * n:i * TQ + (rt + 1) * n, _ct(2 * k + ct)],
                                 _LHS_TERMS[n1])
            blk[0] = after(blk[0], anchor)
            blk[3] = after(blk[3], anchor)
            for n2, v in enumerate(_lhs_set(*blk)):
                ref, r0, c0 = y_set(7 * n1 + n2)
                ref[r0 + rt * n // 2:r0 + (rt + 1) * n // 2, _ct(c0 + ct)] = _pk(v)

        wm_wait(wg_s, 0, D // E, SEM_WM)
        mod_tiles(wg_s, 0, D // E, 5 * D // E)
        mixer_mm(NI - 2)
        mixer_sets(mixer_prep(NI - 1, 0, SEG), mixer_prep(NI - 1, SEG, SEG), 0)
        for q in range(NQ):
            g_job(0, 0, q, TH)
        mix(0)
        mixer_mm(NI - 1)
        ln_job(0, TB, [])
        for ct in range(2):
            for n1 in range(7):
                yset_job(0, ct, n1, TQ)
        for q in range(NQ):
            g_job(1, 0, q, TH)

        def mlp_block(j, last):
            slot = j & 1

            def up_prod(n, g):
                ref, r0, c0 = y_set(n)
                m = _dot(_up(ref[r0:r0 + TQ // 2, c0 * E:(c0 + 2) * E]), _up(t3_s[g, :, _ct(n)]))
                if n in (10, 34) and 2 * g + (n == 34) < TB // 16:
                    base_job(j, 2 * g + (n == 34), m)
                return m

            for g in range(NFG):
                c = _strassen2(lambda n: up_prod(n, g), *O3)
                act = [[_gelu(c(i, k)) for k in range(4)] for i in range(4)]
                for n1 in range(7):
                    blk = _outer_operand(lambda i, k: act[i][k], _LHS_TERMS[n1])
                    for n2, v in enumerate(_lhs_set(*blk)):
                        ref, rows = u_set(7 * n1 + n2)
                        ref[rows, _ct(g)] = _pk(v)
            jobs = {}
            if not last:
                mix(j + 1)
                jn = clamp(j + 2, NB - 1)
                prev = []
                for k in range(TB // 16):
                    jobs[k * Y_AT] = functools.partial(ln_job, (k % 4) * TQ + (k // 4) * 16, 16, prev)

                def place(start, fns, step=1):
                    for fn in fns:
                        while start in jobs:
                            start += 1
                        jobs[start] = fn
                        start += step

                for rt in range(2):
                    place(S_AT[rt], [functools.partial(yset_job, rt, ct, n1, 16)
                                     for ct in range(2) for n1 in range(7)])
                place(G_AT, [functools.partial(g_job, jn, k // NQ, k % NQ, 16)
                             for k in range(TH // 16 * NQ)], G_STEP)

            def down_part(n, og, k0, k1):
                ref, rows = u_set(n)
                return _dot(_up(ref[rows, k0 * E:k1 * E]),
                            _up(t4_s[og, k0 * E // 2:k1 * E // 2, _ct(n)]))

            head = {}
            if last:
                head = {n: down_part(n, 0, 0, NFG - 1) for n in range(HEAD)}
            count = [0]

            def down_prod(n, og):
                if og == 0 and n in head:
                    return down_part(n, og, NFG - 1, NFG) + head[n]
                m = down_part(n, og, 0, NFG)
                job = jobs.get(count[0])
                count[0] += 1
                if job is not None:
                    job(anchor=m)
                return m

            for og in range(NOG):
                c = _strassen2(lambda n: down_prod(n, og), *(O4 if not last else (0, O4[1])))
                for i in range(4):
                    rows = slice(i * TQ, (i + 1) * TQ)
                    for k in range(2):
                        c0 = (4 * og + 2 * k) * E
                        o_s.at[slot][rows, c0:c0 + 2 * E] = (
                            base_s[rows, c0:c0 + 2 * E] + mod_rows(5, TQ, c0, 2 * E)
                            * jnp.concatenate([c(i, 2 * k), c(i, 2 * k + 1)], axis=1)).astype(bf16)
            out_copy(j, slot).start()

        def p3_body(j, carry):
            @pl.when(j >= 2)
            def _():
                out_copy(j - 2, j & 1).wait()

            mlp_block(j, False)
            return carry

        lax.fori_loop(0, NB - 1, _scoped("p3", p3_body), 0)
        for k in range(2):
            for cp in mlp_w_copies(0, k):
                cp.wait()
        out_copy(NB - 3, (NB - 3) % 2).wait()
        mlp_block(NB - 1, True)
        out_copy(NB - 2, (NB - 2) % 2).wait()
        out_copy(NB - 1, (NB - 1) % 2).wait()

    pl.run_scoped(
        phase_a,
        pltpu.VMEM((NSEG, M, D), bf16),
        pltpu.VMEM((7, NSEG * M // 4, D // 2), u32),
        pltpu.VMEM((3 * D // E, D, E), bf16),
        pltpu.VMEM((2, D, HG, E), bf16),
        pltpu.VMEM((2, BGR, D), bf16),
        pltpu.VMEM((2, 2, G1R, D), bf16),
    )
    pl.run_scoped(
        phase_b,
        pltpu.VMEM((7, D // 4, D // 2), u32),
        pltpu.VMEM((NFG, D // 8, 49 * E), u32),
        pltpu.VMEM((NOG, F // 8, 49 * E), u32),
        pltpu.VMEM((D // E, D, E), bf16),
        pltpu.VMEM((TB, D), f32),
        pltpu.VMEM((TB, D), f32),
        pltpu.VMEM((TB, D), f32),
        pltpu.VMEM((2, TB, D), bf16),
    )


@jax.jit
def pallas_adaLN_cond__memory_aug_recurrent_mem_tr__mixer_s_mlp__prompt_kernel(
    A_x: jax.Array,
    A_mem0: jax.Array,
    A_Wq: jax.Array,
    A_Wk: jax.Array,
    A_Wv: jax.Array,
    A_Wo: jax.Array,
    A_seg_len,
    B_x: jax.Array,
    B_w1: jax.Array,
    B_w2: jax.Array,
    B_w3: jax.Array,
    B_w4: jax.Array,
    c: jax.Array,
    w_mod: jax.Array,
):
    del A_seg_len, B_x
    assert A_x.shape == (1, S, D) and A_mem0.shape == (1, M, D)
    hbm = pl.BlockSpec(memory_space=pl.ANY)
    scratch = [
        pltpu.VMEM((NSEG, SEG, D), bf16),
        pltpu.VMEM((NC + 3, D // 2, HG * E), u32),
        pltpu.VMEM((H * E // 2, D), u32),
        pltpu.VMEM((7, D // 4, D // 2), u32),
        pltpu.VMEM((2, 2, 16, D), bf16),
        pltpu.VMEM((2, 4, 64, 4 * E), bf16),
        pltpu.VMEM((2, 4, 32, D), bf16),
        pltpu.VMEM((NC + 2, NSEG * M, HG // 2 * E), u32),
        pltpu.VMEM((8, 6 * D), f32),
        pltpu.VMEM((M, D), f32),
        pltpu.VMEM((TC, D), f32),
        pltpu.VMEM((2 * SEG, D), f32),
        pltpu.VMEM((E, E), f32),
        pltpu.VMEM((S, D), bf16),
        pltpu.VMEM((S + 16, D), f32),
        pltpu.VMEM((7, SEG // 2, D // 2), u32),
        pltpu.VMEM((8 * ZPAD, E), u32),
        pltpu.VMEM((1, D), bf16),
        pltpu.VMEM((M, D), bf16),
        pltpu.SemaphoreType.DMA((24,)),
    ]
    out = pl.pallas_call(
        _kernel,
        out_shape=jax.ShapeDtypeStruct((S, D), bf16),
        in_specs=[hbm] * 12,
        out_specs=hbm,
        scratch_shapes=scratch,
        compiler_params=pltpu.CompilerParams(vmem_limit_bytes=127 * 1024 * 1024,
                                             disable_bounds_checks=NO_BOUNDS),
    )(A_x.reshape(NSEG, SEG, D), A_mem0.reshape(M, D), A_Wq, A_Wk, A_Wv,
      A_Wo.reshape(H * E, D), B_w1.reshape(2, D // 2, D), B_w2.reshape(2, D // 2, D), B_w3.reshape(4, D // 4, F),
      B_w4.reshape(NFG, 4, E, D), c, w_mod)
    return out.reshape(1, S, D)
```

```python
import functools

import jax
import jax.numpy as jnp
from jax import lax
import jax.experimental.pallas as pl
import jax.experimental.pallas.tpu as pltpu

bf16, f32, u32 = jnp.bfloat16, jnp.float32, jnp.uint32

S, D, H, E, M, SEG, F = 2048, 1024, 32, 128, 8, 32, 3584
NSEG = S // SEG
NP = H // 2
TC = SEG - M
HG = 8
NG = H // HG
TB = 128
NB = S // TB
NFG = F // (4 * E)
NOG = D // (4 * E)
NI = NSEG // 2
NQ = D // E // 2
NC = 3 * NG
BGR = 384
G1R = 48
HD = D // 2
X0 = 4
NR = 2 * (M + SEG)
NO_BOUNDS = True
ZPAD = 2
PIN_ROWS = 256
Y_AT = 4
S_AT = (26, 44)
G_AT = 62
HEAD = 14
PREP_AT = (0, 1, 3, 4)
PREP_CH = 2
O3 = (1, 0)
O4 = (0, 0)
O2 = (0, 0)
E_AT = (10, 24, 34)
FINE = 1
JGROUP = 1
P1_TAIL = 5
P1_LAG = 4
SCHED_A = (2, 1, 3)
SCHED_B = (3, 1, 3)
EPS = 1e-5
SCALE = E ** -0.5
_SCOPES = False
_N2 = NSEG // 2


def _scoped(name, fn):
    def wrapped(*a):
        if not _SCOPES:
            return fn(*a)
        with jax.named_scope(name):
            return fn(*a)
    return wrapped


def _pk(x):
    return pltpu.bitcast(x.astype(bf16), u32)


def _up(x):
    return pltpu.bitcast(x, bf16)


def _ct(k):
    return slice(k * E, (k + 1) * E)


def _dot(a, b):
    return jnp.dot(a, b, preferred_element_type=f32)


def _ln(x):
    m = jnp.mean(x, axis=-1, keepdims=True)
    xc = x - m
    v = jnp.mean(xc * xc, axis=-1, keepdims=True)
    return xc * lax.rsqrt(v + EPS)


def _gelu(x):
    c = 0.7978845608028654
    return 0.5 * x * (1.0 + jnp.tanh(c * (x + 0.044715 * (x * x * x))))


def _lhs_set(a11, a12, a21, a22):
    return (a11 + a22, a21 + a22, a11, a22, a11 + a12, a21 - a11, a12 - a22)


def _rhs_set(b11, b12, b21, b22):
    return (b11 + b22, b11, b12 - b22, b21 - b11, b22, b11 + b12, b21 + b22)


_LHS_TERMS = (((0, 1), (3, 1)), ((2, 1), (3, 1)), ((0, 1),), ((3, 1),),
              ((0, 1), (1, 1)), ((2, 1), (0, -1)), ((1, 1), (3, -1)))
_RHS_TERMS = (((0, 1), (3, 1)), ((0, 1),), ((1, 1), (3, -1)), ((2, 1), (0, -1)),
              ((3, 1),), ((0, 1), (1, 1)), ((2, 1), (3, 1)))


def _outer_operand(tile, terms):
    out = []
    for i in range(2):
        for j in range(2):
            v = None
            for o, sign in terms:
                t = tile(2 * (o // 2) + i, 2 * (o % 2) + j)
                v = t if v is None else (v + t if sign > 0 else v - t)
            out.append(v)
    return out


class _Quad:
    def __init__(self, tiles):
        self.t = tuple(tiles)

    def __add__(self, other):
        return _Quad([a + b for a, b in zip(self.t, other.t)])

    def __sub__(self, other):
        return _Quad([a - b for a, b in zip(self.t, other.t)])


def _strassen2(m, oo=0, oi=0):
    cs = _strassen(lambda n1: _Quad(_strassen(lambda n2: m(7 * n1 + n2), oi)), oo)
    return lambda i, j: cs[2 * (i // 2) + j // 2].t[2 * (i % 2) + j % 2]


def _strassen(m, order=0):
    if order == 0:
        m1 = m(0)
        m2 = m(1)
        c22 = m1 - m2
        m3 = m(2)
        c22 = c22 + m3
        c22 = m(5) + c22
        m4 = m(3)
        c21 = m2 + m4
        c11 = m1 + m4
        m5 = m(4)
        c12 = m3 + m5
        c11 = c11 - m5
        c11 = m(6) + c11
    else:
        m2 = m(1)
        c22 = m(5) - m2
        m4 = m(3)
        c21 = m2 + m4
        m1 = m(0)
        c22 = c22 + m1
        c11 = m4 + m1
        m3 = m(2)
        c22 = c22 + m3
        m5 = m(4)
        c12 = m3 + m5
        c11 = c11 - m5
        c11 = m(6) + c11
    return c11, c12, c21, c22


def _mask_fill():
    shape = (NR, E)
    r = lax.broadcasted_iota(jnp.int32, shape, 0)
    c = lax.broadcasted_iota(jnp.int32, shape, 1)

    def headpos(i):
        head = jnp.where(i < 64, i >> 5, (i - 64) >> 3)
        pos = jnp.where(i < 64, i & 31, 32 + (i & 7))
        return head, pos

    hr, pr = headpos(r)
    hc, pc = headpos(c)
    same = hr == hc
    valid = same & ((pr < M) | (pr >= pc))
    return jnp.where(valid, 0.0, jnp.where(same, -1e9, -jnp.inf)).astype(f32)


def _kernel(x_hbm, mem0_hbm, wq_hbm, wk_hbm, wv_hbm, wo_hbm, w1_hbm, w2_hbm, w3_hbm,
            w4_hbm, c_hbm, wm_hbm,
            out_hbm,
            x_s, w_s, wo_s, t1_s, g2, g3, g4, pre_s, mod_s, mem_s, hn_s, aout_s, fill_s,
            hb_s, t_s, l1_s, zero_s, c_s, mem0_s, sems):
    w_hbm = (wq_hbm, wk_hbm, wv_hbm)

    (SEM_C, SEM_MEM, SEM_XPRE, SEM_X, SEM_STG, SEM_BG, SEM_OUT,
     SEM_WMR, SEM_G2, SEM_G3, SEM_G4, SEM_WM, SEM_G1) = (0, 1, 2, 3, 4, 6, 8, 10, 12, 14, 16, 18, 22)

    def copy(src, dst, k):
        return pltpu.make_async_copy(src, dst, sems.at[k])

    def aligned(x, n):
        return x if isinstance(x, int) else pl.multiple_of(x, n)

    def clamp(k, hi):
        return min(k, hi) if isinstance(k, int) else jnp.minimum(k, hi)

    def mlp_piece(k):
        k = clamp(k, 4 * NFG - 1)
        return k >> 2, k & 3

    def mlp_w_copies(k, slot):
        g, rr = mlp_piece(k)
        k2 = clamp(k, NI - 1)
        return (copy(w2_hbm.at[:, pl.ds(aligned((k2 >> 1) * 16, 16), 16),
                               pl.ds(aligned((k2 & 1) * 4 * E, E), 4 * E)], g2.at[slot], SEM_G2 + slot),
                copy(w3_hbm.at[:, pl.ds(aligned(rr * 64, 64), 64), pl.ds(aligned(g * 4 * E, E), 4 * E)],
                     g3.at[slot], SEM_G3 + slot),
                copy(w4_hbm.at[g, :, pl.ds(aligned(rr * 32, 32), 32), :], g4.at[slot], SEM_G4 + slot))

    def pinned(w, job):
        if job is None:
            return w()
        z = job() & zero_s[0:8, :]
        w = w()
        return jnp.concatenate([w[0:8] | z, w[8:]], axis=0)

    def after(x, anchor):
        if anchor is None:
            return x
        z = pltpu.bitcast(pltpu.bitcast(anchor[0:8], u32) & zero_s[0:8, :], f32)
        z = jnp.concatenate([z] * (x.shape[0] // 8), axis=0)
        return jnp.concatenate([x[:, 0:E] + z, x[:, E:]], axis=1) if x.shape[1] > E else x + z

    def rhs_job(src, slot, r0, c1, c2, dst, q, row, z=None):
        blk = [src[slot, kh, r0:r0 + 16, cc * E:(cc + 1) * E].astype(f32)
               for kh in range(2) for cc in (c1, c2)]
        if z is not None:
            zf = pltpu.bitcast(jnp.concatenate([z, z], axis=0), f32)
            blk[0] = blk[0] + zf
            blk[3] = blk[3] + zf
        sets = _rhs_set(*blk)
        for n, v in enumerate(sets):
            dst.at[n][pl.ds(pl.multiple_of(row, 8), 8), _ct(q)] = _pk(v)
        out = pltpu.bitcast(sets[2], u32) | pltpu.bitcast(sets[3], u32)
        return out[0:8] | out[8:16]

    def rhs2_job(src, slot, r0, c0, n1, dst, row):
        blk = _outer_operand(lambda i, j: src[slot, i, r0:r0 + 16, _ct(c0 + j)].astype(f32),
                             _RHS_TERMS[n1])
        sets = _rhs_set(*blk)
        for n2, v in enumerate(sets):
            dst[pl.ds(pl.multiple_of(row, 8), 8), _ct(7 * n1 + n2)] = _pk(v)
        out = pltpu.bitcast(sets[2], u32) | pltpu.bitcast(sets[3], u32)
        return out[0:8] | out[8:16]

    def silu_c():
        cf = c_s[...].astype(f32)
        return jnp.broadcast_to(cf * (1.0 / (1.0 + jnp.exp(-cf))), (8, D)).astype(bf16)

    def wm_copy(wm_s, src_tile, dst_tile, sem):
        return copy(wm_hbm.at[:, pl.ds(aligned(src_tile * E, E), E)], wm_s.at[dst_tile], sem)

    def wm_wait(wm_s, t0, n, sem):
        copy(wm_s.at[t0:t0 + n], wm_s.at[t0:t0 + n], sem).wait()

    def mod_tiles(wm_s, t0, n, dst_tile):
        sc8 = silu_c()
        for k in range(n):
            v = _dot(sc8, wm_s[t0 + k])
            if (dst_tile + k) // (D // E) in (1, 4):
                v = 1.0 + v
            mod_s[:, _ct(dst_tile + k)] = v

    def x_copy(k):
        r = slice(0, X0) if k == 0 else slice(X0, NSEG)
        return copy(x_hbm.at[r], x_s.at[r], SEM_XPRE if k == 0 else SEM_X)

    def h_rows(s):
        return _ln(x_s[s, 0:TC, :].astype(f32)) * mod_rows(1, TC) + mod_rows(0, TC)

    def mod_rows(k, n, c0=0, w=D):
        return jnp.concatenate([mod_s[:, k * D + c0:k * D + c0 + w]] * (n // 8), axis=0)

    def phase_a(xpre_s, hpre_s, wm_s, stg, bg, g1, tq_s):
        def tq_place(c, n):
            if n == 1:
                return w_s.at[c], 0, None
            if n == 4:
                return w_s.at[c], D // 4, None
            return tq_s.at[c], 0, (0, 2, 3, 5, 6).index(n) * (HG // 2)

        def w_copy(t, g, slot):
            return copy(w_hbm[t].at[:, pl.ds(pl.multiple_of(g * HG, HG), HG), :], stg.at[slot],
                        SEM_STG + slot)

        def bg_rows(k):
            return clamp(k * BGR, H * E - BGR), clamp(k * G1R, HD - G1R)

        def bg_copies(k, slot):
            ro, r1 = bg_rows(k)
            return (copy(wo_hbm.at[pl.ds(aligned(ro, 16), BGR)], bg.at[slot], SEM_BG + slot),
                    copy(w1_hbm.at[:, pl.ds(aligned(r1, 16), G1R), :], g1.at[slot], SEM_G1 + slot))

        def relayout_jobs(slot, c, i):
            memo = []
            r = aligned(i * 8, 8)

            def job(j, z=None):
                if not memo:
                    for d0 in (i * 16, HD + i * 16):
                        memo.append(jnp.swapaxes(pltpu.bitcast(stg[slot, pl.ds(d0, 16)], u32), 0, 1))
                blk = []
                for kh in range(2):
                    u = memo[kh][j]
                    if z is not None:
                        u = u | jnp.concatenate([z, z], axis=0)
                    blk.append(pltpu.bitcast(u << 16, f32))
                    blk.append(pltpu.bitcast(u & jnp.uint32(0xFFFF0000), f32))
                for k, v in enumerate(blk):
                    w_s.at[c][pl.ds((k // 2) * (D // 4) + r, 8), _ct(2 * j + k % 2)] = _pk(v)
                for n, v in enumerate(_rhs_set(*blk)):
                    if n not in (1, 4):
                        ref, r0, c0 = tq_place(c, n)
                        ref[pl.ds(r0 + r, 8), _ct(c0 + j)] = _pk(v)

            return [functools.partial(job, j) for j in range(HG // 2)]

        def repack(slot, row, i, z):
            v = pltpu.bitcast(bg[slot, 16 * i:16 * i + 16, :], u32)
            v = v | jnp.concatenate([z] * (D // E), axis=1)
            wo_s[pl.ds(pl.multiple_of(row + 8 * i, 8), 8), :] = v

        cp_c = copy(c_hbm, c_s, SEM_C)
        cp_mem = copy(mem0_hbm, mem0_s, SEM_MEM)
        cp_xpre = copy(x_hbm.at[:, TC:SEG, :], xpre_s, SEM_XPRE)
        w_copy(0, 0, 0).start()
        cp_xpre.start()
        cp_c.start()
        cp_mem.start()
        for k in range(2 * D // E):
            wm_copy(wm_s, k, k, SEM_WM + k // 4).start()
        w_copy(0, 1, 1).start()

        zero_s[0:8, :] = jnp.zeros((8, E), u32)
        fill_s[0:NR, :] = _mask_fill()
        aout_s[...] = jnp.zeros(aout_s.shape, f32)
        l1_s[...] = jnp.zeros(l1_s.shape, u32)
        bg[1] = jnp.zeros(bg.shape[1:], bf16)
        g1[1] = jnp.zeros(g1.shape[1:], bf16)

        w_copy(0, 0, 0).wait()

        def rl0_body(i, carry):
            for job in relayout_jobs(0, 0, i):
                job()
            return carry

        lax.fori_loop(0, D // 32, rl0_body, 0)
        w_copy(0, 2, 0).start()
        for cp in bg_copies(0, 0):
            cp.start()

        cp_xpre.wait()

        def npre_body(i, carry):
            xr = xpre_s[pl.ds(pl.multiple_of(i * 8, 8), 8)].astype(f32).reshape(64, D)
            t_s[pl.ds(pl.multiple_of(i * 64, 64), 64), :] = _ln(xr)
            return carry

        lax.fori_loop(0, NSEG // 8, _scoped("npre", npre_body), 0)

        cp_c.wait()
        cp_mem.wait()
        mem_s[...] = mem0_s[...].astype(f32)

        for k in range(4):
            wm_wait(wm_s, 4 * k, 4, SEM_WM + k)
            mod_tiles(wm_s, 4 * k, 4, 4 * k)

        PH = NSEG * M // 2

        def hpre_body(i, carry):
            h = [t_s[pl.ds(pl.multiple_of(hf * PH + i * 16, 16), 16), :] * mod_rows(1, 16) + mod_rows(0, 16)
                 for hf in range(2)]
            for n, v in enumerate(_lhs_set(h[0][:, :HD], h[0][:, HD:], h[1][:, :HD], h[1][:, HD:])):
                hpre_s.at[n][pl.ds(pl.multiple_of(i * 8, 8), 8), :] = _pk(v)
            return carry

        lax.fori_loop(0, PH // 16, _scoped("hpre", hpre_body), 0)

        t_s[0:8, :] = jnp.zeros((8, D), f32)
        t_s[S + 8:S + 16, :] = jnp.zeros((8, D), f32)

        MB = 64

        def p1_body(c, carry):
            slot = c & 1
            pslot = 1 - slot
            ro, r1 = bg_rows(jnp.maximum(c - 1, 0))

            @pl.when(c >= 1)
            def _():
                for cp in bg_copies(0, pslot):
                    cp.wait()

            @pl.when(c + 1 < NC)
            def _():
                w_copy(0, 0, pslot).wait()

            small = [functools.partial(repack, pslot, ro >> 1, i) for i in range(BGR // 16)]
            small += [functools.partial(rhs_job, g1, pslot, 16 * rt, q, NQ + q, t1_s, q, (r1 >> 1) + 8 * rt)
                      for rt in range(G1R // 16) for q in range(NQ)]
            work = []
            nu = D // 32
            for i in range(nu):
                js = relayout_jobs(pslot, c + 1, i)
                work += [js[k:k + JGROUP] for k in range(0, len(js), JGROUP)]
                work += [[job] for job in small[i * len(small) // nu:(i + 1) * len(small) // nu]]
            npin = 7 * (HG // 2) * (PH // MB)
            jobs = [[] for _ in range(npin)]
            for k, group in enumerate(work):
                pos = k * (npin - P1_TAIL) * 8 // len(work)
                jobs[pos // 8] += [(job, pos % 8 if FINE else 0) for job in group]
            jobs = iter(jobs)

            def prod(n, q, mb):
                ref, r0, c0 = tq_place(c, n)
                w = ref[r0:r0 + D // 4, _ct(2 * q + (n == 4) if c0 is None else c0 + q)]
                m = _dot(_up(hpre_s[n, mb * MB // 2:(mb + 1) * MB // 2, :]), _up(w))
                pending.append(m)
                if len(pending) > P1_LAG:
                    anchor = pltpu.bitcast(pending.pop(0), u32)
                    for job, g in next(jobs):
                        job(anchor[8 * g:8 * g + 8] & zero_s[0:8, :])
                return m

            pending = []
            ns = MB // M
            for q in range(HG // 2):
                for mb in range(PH // MB):
                    cs = _strassen(lambda n: prod(n, q, mb))
                    for hf in range(2):
                        y = jnp.concatenate([cs[2 * hf + k][sg * M:(sg + 1) * M]
                                             for sg in range(ns) for k in range(2)], axis=0)
                        s0 = hf * (NSEG // 2) + mb * ns
                        pre_s.at[c][s0 * M:(s0 + ns) * M, _ct(q)] = _pk(y)

            for t in range(3):
                @pl.when((c + 3) >> 2 == t)
                def _():
                    w_copy(t, (c + 3) & 3, pslot).start()

            @pl.when(c + 2 < NC)
            def _():
                for cp in bg_copies(c + 1, pslot):
                    cp.start()

            @pl.when(c < NC - 3)
            def _():
                wm_copy(wm_s, 2 * D // E + c, c, SEM_WMR).start()

            @pl.when(c == NC - 3)
            def _():
                def issue(k, carry2):
                    wm_copy(wm_s, 2 * D // E + k, k, SEM_WMR).start()
                    return carry2

                x_copy(0).start()
                for k in range(2):
                    for cp in mlp_w_copies(k, k):
                        cp.start()
                lax.fori_loop(NC - 3, 3 * D // E, issue, 0)

            return carry

        lax.fori_loop(0, NC, _scoped("p1", p1_body), 0)
        x_copy(1).start()
        x_copy(0).wait()
        wm_wait(wm_s, 0, 3 * D // E, SEM_WMR)
        mod_tiles(wm_s, 0, 3 * D // E, 2 * D // E)
        hn_s[...] = h_rows(0)

    def phase_b(t2_s, t3_s, t4_s, wg_s, x1_s, base_s, yn_s, gs_s, o_s):
        for k in range(D // E):
            wm_copy(wg_s, 5 * D // E + k, k, SEM_WM).start()

        def chain_step(s, mem, htok, odef_prev, jobs=(), hooks=None):
            hs = jnp.concatenate([mem, htok], axis=0).astype(bf16)
            qkv = [[None] * 3 for _ in range(NP)]
            ps = [None] * NP
            os_ = [None] * H
            odef = [None] * H

            def proj(p, ts=(0, 1, 2)):
                for t in ts:
                    c, q = t * NG + p // (HG // 2), p % (HG // 2)
                    a = _dot(hs, _up(w_s[c, :, _ct(2 * q)]))
                    b = _dot(hs, _up(w_s[c, :, _ct(2 * q + 1)]))
                    if hooks and t == 2 and p - NP in hooks:
                        hooks[p - NP](b)
                    pre = pre_s[c, pl.ds(pl.multiple_of(s * M, M), M), _ct(q)]
                    if t == 1:
                        kf = jnp.concatenate([a, b, _up(pre).astype(f32), jnp.zeros((E - NR, E), f32)],
                                             axis=0)
                        qkv[p][t] = kf.T.astype(bf16)
                        continue
                    parts = [_pk(a), _pk(b), pre]
                    if t == 2:
                        parts.append(jnp.zeros(((E - NR) // 2, E), u32))
                    qkv[p][t] = _up(jnp.concatenate(parts, axis=0))

            def scores(p):
                sc_ = _dot(qkv[p][0], qkv[p][1])
                fill = fill_s[0:NR, :]
                sc_ = jnp.where(fill == 0.0, sc_ * SCALE, fill)
                m = jnp.max(sc_, axis=-1, keepdims=True)
                e = jnp.exp(sc_ - m)
                l = jnp.sum(e, axis=-1, keepdims=True)
                r = pl.reciprocal(l, approx=True)
                r = r * (2.0 - l * r)
                ps[p] = (e * r).astype(bf16)

            def fin(p):
                o = _dot(ps[p], qkv[p][2])
                for hh in range(2):
                    h = 2 * p + hh
                    rows = o[32 * hh:32 * hh + 32]
                    odef[h] = o[64 + 8 * hh:72 + 8 * hh]
                    if odef_prev is not None:
                        rows = jnp.concatenate([rows, odef_prev[h], odef[h]], axis=0)
                    os_[h] = _pk(rows)

            acc = [None] * 8
            jobs = iter(jobs)

            def wo(h0, h1, js):
                lhs = _up(jnp.concatenate(os_[h0:h1], axis=1))
                for j in js:
                    ws = []
                    for r0 in range(h0 * E // 2, h1 * E // 2, PIN_ROWS):
                        ws.append(pinned(lambda: wo_s[r0:r0 + PIN_ROWS, j * E:(j + 1) * E],
                                         next(jobs, None)))
                    part = _dot(lhs, _up(jnp.concatenate(ws, axis=0)))
                    if hooks and acc[j] is None and j in hooks:
                        hooks[j](part)
                    acc[j] = part if acc[j] is None else part + acc[j]

            ORDER, LAG_S, LAG_O = SCHED_A if odef_prev is None else SCHED_B
            for p in range(NP):
                if ORDER == 0:
                    proj(p)
                    if p >= LAG_S:
                        scores(p - LAG_S)
                    if p >= LAG_O:
                        fin(p - LAG_O)
                elif ORDER == 1:
                    proj(p, (1, 0))
                    if p >= LAG_O:
                        fin(p - LAG_O)
                    proj(p, (2,))
                    if p >= LAG_S:
                        scores(p - LAG_S)
                elif ORDER == 2:
                    proj(p, (1,))
                    if p >= LAG_S:
                        scores(p - LAG_S)
                    proj(p, (0,))
                    if p >= LAG_O:
                        fin(p - LAG_O)
                    proj(p, (2,))
                elif ORDER == 3:
                    proj(p, (1,))
                    if p >= LAG_O:
                        fin(p - LAG_O)
                    proj(p, (0,))
                    if p >= LAG_S:
                        scores(p - LAG_S)
                    proj(p, (2,))
                elif ORDER == 4:
                    proj(p, (1,))
                    if p >= LAG_S:
                        scores(p - LAG_S)
                    proj(p, (0, 2))
                    if p >= LAG_O:
                        fin(p - LAG_O)
                else:
                    proj(p, (0,))
                    if p >= LAG_S:
                        scores(p - LAG_S)
                    proj(p, (1,))
                    if p >= LAG_O:
                        fin(p - LAG_O)
                    proj(p, (2,))
            tail = []
            for k in range(LAG_O):
                step = []
                if NP - LAG_S + k < NP:
                    step.append(functools.partial(scores, NP - LAG_S + k))
                step.append(functools.partial(fin, NP - LAG_O + k))
                tail.append(step)
            hsplit = min(24, 2 * (NP - LAG_O))
            cuts = {3: (2, 3, 5), 2: (2, 5), 4: (1, 2, 4, 6), 5: (1, 2, 3, 4, 6)}[LAG_O]
            j0 = 0
            for k, step in enumerate(tail):
                wo(0, hsplit, range(j0, cuts[k]))
                j0 = cuts[k]
                for f in step:
                    f()
            wo(0, hsplit, range(j0, 8))
            wo(hsplit, H, range(8))
            return jnp.concatenate(acc, axis=1), odef

        def mixer_prep(i, r0, n, anchor=None):
            r = pl.ds(aligned(i * 64 + r0, 16), n)
            xr = x_s[2 * i + r0 // SEG, r0 % SEG:r0 % SEG + n, :].astype(f32)
            x2 = xr + mod_rows(2, n) * after(aout_s[r0:r0 + n, :], anchor)
            x_s.at[2 * i + r0 // SEG][r0 % SEG:r0 % SEG + n, :] = x2.astype(bf16)
            hb = _ln(x2) * mod_rows(4, n) + mod_rows(3, n)
            hb_s[r, :] = hb.astype(bf16)
            return _ln(hb)

        def mixer_sets(ya, yb, r0):
            n = ya.shape[0]
            for m, v in enumerate(_lhs_set(ya[:, :HD], ya[:, HD:], yb[:, :HD], yb[:, HD:])):
                l1_s.at[m][r0 // 2:(r0 + n) // 2, :] = _pk(v)

        def mixer_mm(i):
            for q in range(NQ):
                cs = _strassen(lambda n: _dot(_up(l1_s[n]), _up(t1_s[n, :, _ct(q)])))
                for k, cc in enumerate(cs):
                    r0 = aligned(i * 64 + 8 + (k // 2) * SEG, 8)
                    t_s[pl.ds(r0, SEG), _ct(q + NQ * (k % 2))] = _gelu(cc)

        def p2_body(i, carry):
            slot = i & 1
            for cp in mlp_w_copies(0, slot):
                cp.wait()

            @pl.when(i == 1)
            def _():
                x_copy(1).wait()

            g, rr = mlp_piece(i)
            work = [functools.partial(rhs2_job, g2, slot, 0, 0, n1, t2_s.at[slot], (i >> 1) * 8)
                    for n1 in range(7)]
            work += [functools.partial(rhs2_job, g3, slot, 16 * rt, 0, n1, t3_s.at[g], rr * 32 + 8 * rt)
                     for rt in range(4) for n1 in range(7)]
            work += [functools.partial(rhs2_job, g4, slot, 16 * rt, 4 * og, n1, t4_s.at[og],
                                       g * (E // 2) + rr * 16 + 8 * rt)
                     for rt in range(2) for og in range(NOG) for n1 in range(7)]
            jobs = [None] + work

            sa_ = 2 * i
            sb_ = 2 * i + 1
            hb_tok = h_rows(sb_)
            oa, odef_a = chain_step(sa_, mem_s[...], hn_s[...], None)
            mixer_mm(jnp.maximum(i - 2, 0))
            ys = []

            def hook(k, anchor):
                if k >= PREP_CH:
                    anchor = anchor[0:8] + ys[-PREP_CH][0:8, 0:E] + ys[-PREP_CH][8:16, 0:E]
                ys.append(mixer_prep(jnp.maximum(i - 1, 0), (k % 2) * SEG + (k // 2) * 16, 16, anchor))
                if k % 2:
                    mixer_sets(ys[-2], ys[-1], (k // 2) * 16)

            hooks = {j: functools.partial(hook, k) for k, j in enumerate(PREP_AT)}
            ob, _ = chain_step(sb_, oa[0:M], hb_tok, odef_a, jobs, hooks)
            mem_s[...] = ob[0:M]
            aout_s[0:TC, :] = oa[M:SEG]
            aout_s[TC:SEG, :] = ob[SEG:SEG + M]
            aout_s[SEG:SEG + TC, :] = ob[M:SEG]
            aout_s[SEG + TC:2 * SEG, :] = ob[SEG + M:SEG + 2 * M]
            hn_s[...] = h_rows(jnp.minimum(sb_ + 1, NSEG - 1))
            for cp in mlp_w_copies(i + 2, slot):
                cp.start()
            return carry

        lax.fori_loop(0, _N2, _scoped("p2", p2_body), 0)

        TQ = TB // 4
        SHIFT = (-1, -1, 1, 1, -2, -2, 2, 2)

        def u_set(n):
            return w_s.at[n // 32], slice((n % 32) * (TQ // 2), (n % 32 + 1) * (TQ // 2))

        def d_set(slot, n):
            return w_s.at[slot], (n // 4) * (TQ // 2), (n % 4) * 2

        def d_lhs(slot, n):
            ref, r0, c0 = d_set(slot, n)
            return _up(ref[r0:r0 + TQ // 2, c0 * E:(c0 + 2) * E])

        def shift_job(j, r0, n, anchor=None):
            for ct in range(D // E):
                win = t_s[pl.ds(aligned(j * TB + r0, 16), n + 16), _ct(ct)]
                gs_s[r0:r0 + n, _ct(ct)] = after(
                    pltpu.roll(win, (-SHIFT[ct]) % (n + 16), 0)[8:8 + n], anchor)

        def mix(j):
            r0 = aligned(j * TB, TB)
            for og in range(NOG):
                c = _strassen2(lambda n: _dot(d_lhs(3, n), _up(t2_s[og, :, _ct(n)])), *O2)
                for i in range(4):
                    for k in range(2):
                        cols = slice((4 * og + 2 * k) * E, (4 * og + 2 * k + 2) * E)
                        x1_s[i * TQ:(i + 1) * TQ, cols] = (
                            hb_s[pl.ds(r0 + i * TQ, TQ), cols].astype(f32)
                            + jnp.concatenate([c(i, 2 * k), c(i, 2 * k + 1)], axis=1))

        def base_job(j, rt, anchor):
            rows = slice(rt * 16, (rt + 1) * 16)
            z = pltpu.bitcast(pltpu.bitcast(anchor[0:8], u32) & zero_s[0:8, :], f32)
            gb = mod_rows(5, 8) + jnp.concatenate([z] * (D // E), axis=1)
            x2 = x_s[j * (TB // SEG) + rt // 2, (rt % 2) * 16:(rt % 2) * 16 + 16, :]
            base_s[rows, :] = x2.astype(f32) + jnp.concatenate([gb, gb], axis=0) * x1_s[rows, :]

        def out_copy(j, slot):
            return copy(o_s.at[slot], out_hbm.at[pl.ds(aligned(j * TB, TB), TB)], SEM_OUT + slot)

        def ln_job(r0, n, prev, anchor=None):
            if anchor is not None and len(prev) >= 2:
                anchor = anchor[0:8] + prev[-2]
            y = _ln(after(x1_s[r0:r0 + n, :], anchor))
            yn_s[r0:r0 + n, :] = y
            prev.append(y[0:8, 0:E] + y[8:16, 0:E])

        def set_job(src, slot, rt, ct, n1, n=16, anchor=None):
            blk = _outer_operand(lambda i, k: src[i * TQ + rt * n:i * TQ + (rt + 1) * n, _ct(2 * k + ct)],
                                 _LHS_TERMS[n1])
            blk[0] = after(blk[0], anchor)
            blk[3] = after(blk[3], anchor)
            for n2, v in enumerate(_lhs_set(*blk)):
                ref, r0, c0 = d_set(slot, 7 * n1 + n2)
                ref[r0 + rt * n // 2:r0 + (rt + 1) * n // 2, _ct(c0 + ct)] = _pk(v)

        def all_sets(src, slot):
            for n1 in range(7):
                for ct in range(2):
                    set_job(src, slot, 0, ct, n1, TQ)

        wm_wait(wg_s, 0, D // E, SEM_WM)
        mod_tiles(wg_s, 0, D // E, 5 * D // E)
        mixer_mm(NI - 2)
        mixer_sets(mixer_prep(NI - 1, 0, SEG), mixer_prep(NI - 1, SEG, SEG), 0)
        shift_job(0, 0, TB)
        all_sets(gs_s, 3)
        mix(0)
        mixer_mm(NI - 1)
        ln_job(0, TB, [])
        all_sets(yn_s, 2)
        shift_job(1, 0, TB)
        all_sets(gs_s, 3)

        def mlp_block(j, last):
            slot = j & 1

            jn = clamp(j + 2, NB - 1)
            early = [functools.partial(base_job, j, k) for k in range(TB // 16)]
            if not last:
                early += [functools.partial(shift_job, jn, 16 * k, 16) for k in range(TB // 16)]
            early = iter(early)

            def up_prod(n, g):
                m = _dot(d_lhs(2, n), _up(t3_s[g, :, _ct(n)]))
                if n in E_AT:
                    job = next(early, None)
                    if job is not None:
                        job(anchor=m)
                return m

            for g in range(NFG):
                c = _strassen2(lambda n: up_prod(n, g), *O3)
                act = [[_gelu(c(i, k)) for k in range(4)] for i in range(4)]
                for n1 in range(7):
                    blk = _outer_operand(lambda i, k: act[i][k], _LHS_TERMS[n1])
                    for n2, v in enumerate(_lhs_set(*blk)):
                        ref, rows = u_set(7 * n1 + n2)
                        ref[rows, _ct(g)] = _pk(v)
            jobs = {}
            if not last:
                mix(j + 1)
                prev = []
                for k in range(TB // 16):
                    jobs[k * Y_AT] = functools.partial(ln_job, (k % 4) * TQ + (k // 4) * 16, 16, prev)

                def place(start, fns, step=1):
                    for fn in fns:
                        while start in jobs:
                            start += 1
                        jobs[start] = fn
                        start += step

                for rt in range(2):
                    place(S_AT[rt], [functools.partial(set_job, yn_s, 2, rt, ct, n1, 16)
                                     for ct in range(2) for n1 in range(7)])
                place(G_AT, [functools.partial(set_job, gs_s, 3, rt, ct, n1, 16)
                             for rt in range(2) for ct in range(2) for n1 in range(7)])

            def down_part(n, og, k0, k1):
                ref, rows = u_set(n)
                return _dot(_up(ref[rows, k0 * E:k1 * E]),
                            _up(t4_s[og, k0 * E // 2:k1 * E // 2, _ct(n)]))

            head = {}
            if last:
                head = {n: down_part(n, 0, 0, NFG - 1) for n in range(HEAD)}
            count = [0]

            def down_prod(n, og):
                if og == 0 and n in head:
                    return down_part(n, og, NFG - 1, NFG) + head[n]
                m = down_part(n, og, 0, NFG)
                job = jobs.get(count[0])
                count[0] += 1
                if job is not None:
                    job(anchor=m)
                return m

            for og in range(NOG):
                c = _strassen2(lambda n: down_prod(n, og), *(O4 if not last else (0, O4[1])))
                for i in range(4):
                    rows = slice(i * TQ, (i + 1) * TQ)
                    for k in range(2):
                        c0 = (4 * og + 2 * k) * E
                        o_s.at[slot][rows, c0:c0 + 2 * E] = (
                            base_s[rows, c0:c0 + 2 * E] + mod_rows(5, TQ, c0, 2 * E)
                            * jnp.concatenate([c(i, 2 * k), c(i, 2 * k + 1)], axis=1)).astype(bf16)
            out_copy(j, slot).start()

        def p3_body(j, carry):
            @pl.when(j >= 2)
            def _():
                out_copy(j - 2, j & 1).wait()

            mlp_block(j, False)
            return carry

        lax.fori_loop(0, NB - 1, _scoped("p3", p3_body), 0)
        for k in range(2):
            for cp in mlp_w_copies(0, k):
                cp.wait()
        out_copy(NB - 3, (NB - 3) % 2).wait()
        mlp_block(NB - 1, True)
        out_copy(NB - 2, (NB - 2) % 2).wait()
        out_copy(NB - 1, (NB - 1) % 2).wait()

    pl.run_scoped(
        phase_a,
        pltpu.VMEM((NSEG, M, D), bf16),
        pltpu.VMEM((7, NSEG * M // 4, D // 2), u32),
        pltpu.VMEM((3 * D // E, D, E), bf16),
        pltpu.VMEM((2, D, HG, E), bf16),
        pltpu.VMEM((2, BGR, D), bf16),
        pltpu.VMEM((2, 2, G1R, D), bf16),
        pltpu.VMEM((NC + 1, D // 4, 5 * HG // 2 * E), u32),
    )
    pl.run_scoped(
        phase_b,
        pltpu.VMEM((NOG, D // 8, 49 * E), u32),
        pltpu.VMEM((NFG, D // 8, 49 * E), u32),
        pltpu.VMEM((NOG, F // 8, 49 * E), u32),
        pltpu.VMEM((D // E, D, E), bf16),
        pltpu.VMEM((TB, D), f32),
        pltpu.VMEM((TB, D), f32),
        pltpu.VMEM((TB, D), f32),
        pltpu.VMEM((TB, D), f32),
        pltpu.VMEM((2, TB, D), bf16),
    )


@jax.jit
def pallas_adaLN_cond__memory_aug_recurrent_mem_tr__mixer_s_mlp__prompt_kernel(
    A_x: jax.Array,
    A_mem0: jax.Array,
    A_Wq: jax.Array,
    A_Wk: jax.Array,
    A_Wv: jax.Array,
    A_Wo: jax.Array,
    A_seg_len,
    B_x: jax.Array,
    B_w1: jax.Array,
    B_w2: jax.Array,
    B_w3: jax.Array,
    B_w4: jax.Array,
    c: jax.Array,
    w_mod: jax.Array,
):
    del A_seg_len, B_x
    assert A_x.shape == (1, S, D) and A_mem0.shape == (1, M, D)
    hbm = pl.BlockSpec(memory_space=pl.ANY)
    scratch = [
        pltpu.VMEM((NSEG, SEG, D), bf16),
        pltpu.VMEM((NC + 1, D // 2, HG * E), u32),
        pltpu.VMEM((H * E // 2, D), u32),
        pltpu.VMEM((7, D // 4, D // 2), u32),
        pltpu.VMEM((2, 4, 16, 4 * E), bf16),
        pltpu.VMEM((2, 4, 64, 4 * E), bf16),
        pltpu.VMEM((2, 4, 32, D), bf16),
        pltpu.VMEM((NC, NSEG * M, HG // 2 * E), u32),
        pltpu.VMEM((8, 6 * D), f32),
        pltpu.VMEM((M, D), f32),
        pltpu.VMEM((TC, D), f32),
        pltpu.VMEM((2 * SEG, D), f32),
        pltpu.VMEM((E, E), f32),
        pltpu.VMEM((S, D), bf16),
        pltpu.VMEM((S + 16, D), f32),
        pltpu.VMEM((7, SEG // 2, D // 2), u32),
        pltpu.VMEM((8 * ZPAD, E), u32),
        pltpu.VMEM((1, D), bf16),
        pltpu.VMEM((M, D), bf16),
        pltpu.SemaphoreType.DMA((24,)),
    ]
    out = pl.pallas_call(
        _kernel,
        out_shape=jax.ShapeDtypeStruct((S, D), bf16),
        in_specs=[hbm] * 12,
        out_specs=hbm,
        scratch_shapes=scratch,
        compiler_params=pltpu.CompilerParams(vmem_limit_bytes=127 * 1024 * 1024,
                                             disable_bounds_checks=NO_BOUNDS),
    )(A_x.reshape(NSEG, SEG, D), A_mem0.reshape(M, D), A_Wq, A_Wk, A_Wv,
      A_Wo.reshape(H * E, D), B_w1.reshape(2, D // 2, D), B_w2.reshape(4, D // 4, D), B_w3.reshape(4, D // 4, F),
      B_w4.reshape(NFG, 4, E, D), c, w_mod)
    return out.reshape(1, S, D)
```

```python
import functools

import jax
import jax.numpy as jnp
from jax import lax
import jax.experimental.pallas as pl
import jax.experimental.pallas.tpu as pltpu

bf16, f32, u32 = jnp.bfloat16, jnp.float32, jnp.uint32

S, D, H, E, M, SEG, F = 2048, 1024, 32, 128, 8, 32, 3584
NSEG = S // SEG
NP = H // 2
TC = SEG - M
HG = 8
NG = H // HG
TB = 128
NB = S // TB
NFG = F // (4 * E)
NOG = D // (4 * E)
NI = NSEG // 2
NQ = D // E // 2
NC = 3 * NG
BGR = 384
G1R = 48
HD = D // 2
X0 = 4
NR = 2 * (M + SEG)
NO_BOUNDS = True
ZPAD = 2
PIN_ROWS = 256
Y_AT = 4
S_AT = (26, 44)
G_AT = 62
HEAD = 14
PREP_AT = (0, 1, 4, 5)
PREP_CH = 2
O3 = (1, 0)
O4 = (0, 0)
O2 = (0, 0)
FREE_JOBS = 0
SH_AT = None
E_AT = (10, 24, 34)
FINE = 1
JGROUP = 1
P1_TAIL = 5
P1_LAG = 4
SCHED_A = (2, 1, 3)
SCHED_B = (3, 1, 3)
EPS = 1e-5
SCALE = E ** -0.5
_SCOPES = False
_N2 = NSEG // 2


def _scoped(name, fn):
    def wrapped(*a):
        if not _SCOPES:
            return fn(*a)
        with jax.named_scope(name):
            return fn(*a)
    return wrapped


def _pk(x):
    return pltpu.bitcast(x.astype(bf16), u32)


def _up(x):
    return pltpu.bitcast(x, bf16)


def _ct(k):
    return slice(k * E, (k + 1) * E)


def _dot(a, b):
    return jnp.dot(a, b, preferred_element_type=f32)


def _ln(x):
    m = jnp.mean(x, axis=-1, keepdims=True)
    xc = x - m
    v = jnp.mean(xc * xc, axis=-1, keepdims=True)
    return xc * lax.rsqrt(v + EPS)


def _gelu(x):
    c = 0.7978845608028654
    return 0.5 * x * (1.0 + jnp.tanh(c * (x + 0.044715 * (x * x * x))))


def _lhs_set(a11, a12, a21, a22):
    return (a11 + a22, a21 + a22, a11, a22, a11 + a12, a21 - a11, a12 - a22)


def _rhs_set(b11, b12, b21, b22):
    return (b11 + b22, b11, b12 - b22, b21 - b11, b22, b11 + b12, b21 + b22)


_LHS_TERMS = (((0, 1), (3, 1)), ((2, 1), (3, 1)), ((0, 1),), ((3, 1),),
              ((0, 1), (1, 1)), ((2, 1), (0, -1)), ((1, 1), (3, -1)))
_RHS_TERMS = (((0, 1), (3, 1)), ((0, 1),), ((1, 1), (3, -1)), ((2, 1), (0, -1)),
              ((3, 1),), ((0, 1), (1, 1)), ((2, 1), (3, 1)))


def _outer_operand(tile, terms):
    out = []
    for i in range(2):
        for j in range(2):
            v = None
            for o, sign in terms:
                t = tile(2 * (o // 2) + i, 2 * (o % 2) + j)
                v = t if v is None else (v + t if sign > 0 else v - t)
            out.append(v)
    return out


class _Quad:
    def __init__(self, tiles):
        self.t = tuple(tiles)

    def __add__(self, other):
        return _Quad([a + b for a, b in zip(self.t, other.t)])

    def __sub__(self, other):
        return _Quad([a - b for a, b in zip(self.t, other.t)])


def _strassen2(m, oo=0, oi=0):
    cs = _strassen(lambda n1: _Quad(_strassen(lambda n2: m(7 * n1 + n2), oi)), oo)
    return lambda i, j: cs[2 * (i // 2) + j // 2].t[2 * (i % 2) + j % 2]


def _strassen(m, order=0):
    if order == 0:
        m1 = m(0)
        m2 = m(1)
        c22 = m1 - m2
        m3 = m(2)
        c22 = c22 + m3
        c22 = m(5) + c22
        m4 = m(3)
        c21 = m2 + m4
        c11 = m1 + m4
        m5 = m(4)
        c12 = m3 + m5
        c11 = c11 - m5
        c11 = m(6) + c11
    else:
        m2 = m(1)
        c22 = m(5) - m2
        m4 = m(3)
        c21 = m2 + m4
        m1 = m(0)
        c22 = c22 + m1
        c11 = m4 + m1
        m3 = m(2)
        c22 = c22 + m3
        m5 = m(4)
        c12 = m3 + m5
        c11 = c11 - m5
        c11 = m(6) + c11
    return c11, c12, c21, c22


def _mask_fill():
    shape = (NR, E)
    r = lax.broadcasted_iota(jnp.int32, shape, 0)
    c = lax.broadcasted_iota(jnp.int32, shape, 1)

    def headpos(i):
        head = jnp.where(i < 64, i >> 5, (i - 64) >> 3)
        pos = jnp.where(i < 64, i & 31, 32 + (i & 7))
        return head, pos

    hr, pr = headpos(r)
    hc, pc = headpos(c)
    same = hr == hc
    valid = same & ((pr < M) | (pr >= pc))
    return jnp.where(valid, 0.0, jnp.where(same, -1e9, -jnp.inf)).astype(f32)


def _kernel(x_hbm, mem0_hbm, wq_hbm, wk_hbm, wv_hbm, wo_hbm, w1_hbm, w2_hbm, w3_hbm,
            w4_hbm, c_hbm, wm_hbm,
            out_hbm,
            x_s, w_s, wo_s, t1_s, g2, g3, g4, pre_s, mod_s, mem_s, hn_s, aout_s, fill_s,
            hb_s, t_s, l1_s, zero_s, c_s, mem0_s, sems):
    w_hbm = (wq_hbm, wk_hbm, wv_hbm)

    (SEM_C, SEM_MEM, SEM_XPRE, SEM_X, SEM_STG, SEM_BG, SEM_OUT,
     SEM_WMR, SEM_G2, SEM_G3, SEM_G4, SEM_WM, SEM_G1) = (0, 1, 2, 3, 4, 6, 8, 10, 12, 14, 16, 18, 22)

    def copy(src, dst, k):
        return pltpu.make_async_copy(src, dst, sems.at[k])

    def aligned(x, n):
        return x if isinstance(x, int) else pl.multiple_of(x, n)

    def clamp(k, hi):
        return min(k, hi) if isinstance(k, int) else jnp.minimum(k, hi)

    def mlp_piece(k):
        k = clamp(k, 4 * NFG - 1)
        return k >> 2, k & 3

    def mlp_w_copies(k, slot):
        g, rr = mlp_piece(k)
        k2 = clamp(k, NI - 1)
        return (copy(w2_hbm.at[:, pl.ds(aligned((k2 >> 1) * 16, 16), 16),
                               pl.ds(aligned((k2 & 1) * 4 * E, E), 4 * E)], g2.at[slot], SEM_G2 + slot),
                copy(w3_hbm.at[:, pl.ds(aligned(rr * 64, 64), 64), pl.ds(aligned(g * 4 * E, E), 4 * E)],
                     g3.at[slot], SEM_G3 + slot),
                copy(w4_hbm.at[g, :, pl.ds(aligned(rr * 32, 32), 32), :], g4.at[slot], SEM_G4 + slot))

    def pinned(w, job):
        if job is None:
            return w()
        z = job() & zero_s[0:8, :]
        w = w()
        return jnp.concatenate([w[0:8] | z, w[8:]], axis=0)

    def after(x, anchor):
        if anchor is None:
            return x
        z = pltpu.bitcast(pltpu.bitcast(anchor[0:8], u32) & zero_s[0:8, :], f32)
        z = jnp.concatenate([z] * (x.shape[0] // 8), axis=0)
        return jnp.concatenate([x[:, 0:E] + z, x[:, E:]], axis=1) if x.shape[1] > E else x + z

    def rhs_job(src, slot, r0, c1, c2, dst, q, row, z=None):
        blk = [src[slot, kh, r0:r0 + 16, cc * E:(cc + 1) * E].astype(f32)
               for kh in range(2) for cc in (c1, c2)]
        if z is not None:
            zf = pltpu.bitcast(jnp.concatenate([z, z], axis=0), f32)
            blk[0] = blk[0] + zf
            blk[3] = blk[3] + zf
        sets = _rhs_set(*blk)
        for n, v in enumerate(sets):
            dst.at[n][pl.ds(pl.multiple_of(row, 8), 8), _ct(q)] = _pk(v)
        out = pltpu.bitcast(sets[2], u32) | pltpu.bitcast(sets[3], u32)
        return out[0:8] | out[8:16]

    def rhs2_job(src, slot, r0, c0, n1, dst, row):
        blk = _outer_operand(lambda i, j: src[slot, i, r0:r0 + 16, _ct(c0 + j)].astype(f32),
                             _RHS_TERMS[n1])
        sets = _rhs_set(*blk)
        for n2, v in enumerate(sets):
            dst[pl.ds(pl.multiple_of(row, 8), 8), _ct(7 * n1 + n2)] = _pk(v)
        out = pltpu.bitcast(sets[2], u32) | pltpu.bitcast(sets[3], u32)
        return out[0:8] | out[8:16]

    def silu_c():
        cf = c_s[...].astype(f32)
        return jnp.broadcast_to(cf * (1.0 / (1.0 + jnp.exp(-cf))), (8, D)).astype(bf16)

    def wm_copy(wm_s, src_tile, dst_tile, sem):
        return copy(wm_hbm.at[:, pl.ds(aligned(src_tile * E, E), E)], wm_s.at[dst_tile], sem)

    def wm_wait(wm_s, t0, n, sem):
        copy(wm_s.at[t0:t0 + n], wm_s.at[t0:t0 + n], sem).wait()

    def mod_tiles(wm_s, t0, n, dst_tile):
        sc8 = silu_c()
        for k in range(n):
            v = _dot(sc8, wm_s[t0 + k])
            if (dst_tile + k) // (D // E) in (1, 4):
                v = 1.0 + v
            mod_s[:, _ct(dst_tile + k)] = v

    def x_copy(k):
        r = slice(0, X0) if k == 0 else slice(X0, NSEG)
        return copy(x_hbm.at[r], x_s.at[r], SEM_XPRE if k == 0 else SEM_X)

    def h_rows(s):
        return _ln(x_s[s, 0:TC, :].astype(f32)) * mod_rows(1, TC) + mod_rows(0, TC)

    def mod_rows(k, n, c0=0, w=D):
        return jnp.concatenate([mod_s[:, k * D + c0:k * D + c0 + w]] * (n // 8), axis=0)

    def phase_a(xpre_s, hpre_s, wm_s, stg, bg, g1, tq_s):
        def tq_place(c, n):
            if n == 1:
                return w_s.at[c], 0, None
            if n == 4:
                return w_s.at[c], D // 4, None
            return tq_s.at[c], 0, (0, 2, 3, 5, 6).index(n) * (HG // 2)

        def w_copy(t, g, slot):
            return copy(w_hbm[t].at[:, pl.ds(pl.multiple_of(g * HG, HG), HG), :], stg.at[slot],
                        SEM_STG + slot)

        def bg_rows(k):
            return clamp(k * BGR, H * E - BGR), clamp(k * G1R, HD - G1R)

        def bg_copies(k, slot):
            ro, r1 = bg_rows(k)
            return (copy(wo_hbm.at[pl.ds(aligned(ro, 16), BGR)], bg.at[slot], SEM_BG + slot),
                    copy(w1_hbm.at[:, pl.ds(aligned(r1, 16), G1R), :], g1.at[slot], SEM_G1 + slot))

        def relayout_jobs(slot, c, i):
            memo = []
            r = aligned(i * 8, 8)

            def job(j, z=None):
                if not memo:
                    for d0 in (i * 16, HD + i * 16):
                        memo.append(jnp.swapaxes(pltpu.bitcast(stg[slot, pl.ds(d0, 16)], u32), 0, 1))
                blk = []
                for kh in range(2):
                    u = memo[kh][j]
                    if z is not None:
                        u = u | jnp.concatenate([z, z], axis=0)
                    blk.append(pltpu.bitcast(u << 16, f32))
                    blk.append(pltpu.bitcast(u & jnp.uint32(0xFFFF0000), f32))
                for k, v in enumerate(blk):
                    w_s.at[c][pl.ds((k // 2) * (D // 4) + r, 8), _ct(2 * j + k % 2)] = _pk(v)
                for n, v in enumerate(_rhs_set(*blk)):
                    if n not in (1, 4):
                        ref, r0, c0 = tq_place(c, n)
                        ref[pl.ds(r0 + r, 8), _ct(c0 + j)] = _pk(v)

            return [functools.partial(job, j) for j in range(HG // 2)]

        def repack(slot, row, i, z):
            v = pltpu.bitcast(bg[slot, 16 * i:16 * i + 16, :], u32)
            v = v | jnp.concatenate([z] * (D // E), axis=1)
            wo_s[pl.ds(pl.multiple_of(row + 8 * i, 8), 8), :] = v

        cp_c = copy(c_hbm, c_s, SEM_C)
        cp_mem = copy(mem0_hbm, mem0_s, SEM_MEM)
        cp_xpre = copy(x_hbm.at[:, TC:SEG, :], xpre_s, SEM_XPRE)
        w_copy(0, 0, 0).start()
        cp_xpre.start()
        cp_c.start()
        cp_mem.start()
        for k in range(2 * D // E):
            wm_copy(wm_s, k, k, SEM_WM + k // 4).start()
        w_copy(0, 1, 1).start()

        zero_s[0:8, :] = jnp.zeros((8, E), u32)
        fill_s[0:NR, :] = _mask_fill()
        aout_s[...] = jnp.zeros(aout_s.shape, f32)
        l1_s[...] = jnp.zeros(l1_s.shape, u32)
        bg[1] = jnp.zeros(bg.shape[1:], bf16)
        g1[1] = jnp.zeros(g1.shape[1:], bf16)

        w_copy(0, 0, 0).wait()

        def rl0_body(i, carry):
            for job in relayout_jobs(0, 0, i):
                job()
            return carry

        lax.fori_loop(0, D // 32, rl0_body, 0)
        w_copy(0, 2, 0).start()
        for cp in bg_copies(0, 0):
            cp.start()

        cp_xpre.wait()

        def npre_body(i, carry):
            xr = xpre_s[pl.ds(pl.multiple_of(i * 8, 8), 8)].astype(f32).reshape(64, D)
            t_s[pl.ds(pl.multiple_of(i * 64, 64), 64), :] = _ln(xr)
            return carry

        lax.fori_loop(0, NSEG // 8, _scoped("npre", npre_body), 0)

        cp_c.wait()
        cp_mem.wait()
        mem_s[...] = mem0_s[...].astype(f32)

        for k in range(4):
            wm_wait(wm_s, 4 * k, 4, SEM_WM + k)
            mod_tiles(wm_s, 4 * k, 4, 4 * k)

        PH = NSEG * M // 2

        def hpre_body(i, carry):
            h = [t_s[pl.ds(pl.multiple_of(hf * PH + i * 16, 16), 16), :] * mod_rows(1, 16) + mod_rows(0, 16)
                 for hf in range(2)]
            for n, v in enumerate(_lhs_set(h[0][:, :HD], h[0][:, HD:], h[1][:, :HD], h[1][:, HD:])):
                hpre_s.at[n][pl.ds(pl.multiple_of(i * 8, 8), 8), :] = _pk(v)
            return carry

        lax.fori_loop(0, PH // 16, _scoped("hpre", hpre_body), 0)

        t_s[0:8, :] = jnp.zeros((8, D), f32)
        t_s[S + 8:S + 16, :] = jnp.zeros((8, D), f32)

        MB = 64

        def p1_body(c, carry):
            slot = c & 1
            pslot = 1 - slot
            ro, r1 = bg_rows(jnp.maximum(c - 1, 0))

            @pl.when(c >= 1)
            def _():
                for cp in bg_copies(0, pslot):
                    cp.wait()

            @pl.when(c + 1 < NC)
            def _():
                w_copy(0, 0, pslot).wait()

            small = [functools.partial(repack, pslot, ro >> 1, i) for i in range(BGR // 16)]
            small += [functools.partial(rhs_job, g1, pslot, 16 * rt, q, NQ + q, t1_s, q, (r1 >> 1) + 8 * rt)
                      for rt in range(G1R // 16) for q in range(NQ)]
            work = []
            nu = D // 32
            for i in range(nu):
                js = relayout_jobs(pslot, c + 1, i)
                work += [js[k:k + JGROUP] for k in range(0, len(js), JGROUP)]
                work += [[job] for job in small[i * len(small) // nu:(i + 1) * len(small) // nu]]
            npin = 7 * (HG // 2) * (PH // MB)
            jobs = [[] for _ in range(npin)]
            for k, group in enumerate(work):
                pos = k * (npin - P1_TAIL) * 8 // len(work)
                jobs[pos // 8] += [(job, pos % 8 if FINE else 0) for job in group]
            jobs = iter(jobs)

            def prod(n, q, mb):
                ref, r0, c0 = tq_place(c, n)
                w = ref[r0:r0 + D // 4, _ct(2 * q + (n == 4) if c0 is None else c0 + q)]
                m = _dot(_up(hpre_s[n, mb * MB // 2:(mb + 1) * MB // 2, :]), _up(w))
                pending.append(m)
                if len(pending) > P1_LAG:
                    anchor = pltpu.bitcast(pending.pop(0), u32)
                    for job, g in next(jobs):
                        job(anchor[8 * g:8 * g + 8] & zero_s[0:8, :])
                return m

            pending = []
            ns = MB // M
            for q in range(HG // 2):
                for mb in range(PH // MB):
                    cs = _strassen(lambda n: prod(n, q, mb))
                    for hf in range(2):
                        y = jnp.concatenate([cs[2 * hf + k][sg * M:(sg + 1) * M]
                                             for sg in range(ns) for k in range(2)], axis=0)
                        s0 = hf * (NSEG // 2) + mb * ns
                        pre_s.at[c][s0 * M:(s0 + ns) * M, _ct(q)] = _pk(y)

            for t in range(3):
                @pl.when((c + 3) >> 2 == t)
                def _():
                    w_copy(t, (c + 3) & 3, pslot).start()

            @pl.when(c + 2 < NC)
            def _():
                for cp in bg_copies(c + 1, pslot):
                    cp.start()

            @pl.when(c < NC - 3)
            def _():
                wm_copy(wm_s, 2 * D // E + c, c, SEM_WMR).start()

            @pl.when(c == NC - 3)
            def _():
                def issue(k, carry2):
                    wm_copy(wm_s, 2 * D // E + k, k, SEM_WMR).start()
                    return carry2

                x_copy(0).start()
                for k in range(2):
                    for cp in mlp_w_copies(k, k):
                        cp.start()
                lax.fori_loop(NC - 3, 3 * D // E, issue, 0)

            return carry

        lax.fori_loop(0, NC, _scoped("p1", p1_body), 0)
        x_copy(1).start()
        x_copy(0).wait()
        wm_wait(wm_s, 0, 3 * D // E, SEM_WMR)
        mod_tiles(wm_s, 0, 3 * D // E, 2 * D // E)
        hn_s[...] = h_rows(0)

    def phase_b(t2_s, t3_s, t4_s, wg_s, x1_s, base_s, yn_s, gs_s, o_s):
        for k in range(D // E):
            wm_copy(wg_s, 5 * D // E + k, k, SEM_WM).start()

        def chain_step(s, mem, htok, odef_prev, jobs=(), hooks=None):
            hs = jnp.concatenate([mem, htok], axis=0).astype(bf16)
            qkv = [[None] * 3 for _ in range(NP)]
            ps = [None] * NP
            os_ = [None] * H
            odef = [None] * H

            def proj(p, ts=(0, 1, 2)):
                for t in ts:
                    c, q = t * NG + p // (HG // 2), p % (HG // 2)
                    a = _dot(hs, _up(w_s[c, :, _ct(2 * q)]))
                    b = _dot(hs, _up(w_s[c, :, _ct(2 * q + 1)]))
                    if hooks and t == 2 and p - NP in hooks:
                        hooks[p - NP](b)
                    pre = pre_s[c, pl.ds(pl.multiple_of(s * M, M), M), _ct(q)]
                    if t == 1:
                        kf = jnp.concatenate([a, b, _up(pre).astype(f32), jnp.zeros((E - NR, E), f32)],
                                             axis=0)
                        qkv[p][t] = kf.T.astype(bf16)
                        continue
                    parts = [_pk(a), _pk(b), pre]
                    if t == 2:
                        parts.append(jnp.zeros(((E - NR) // 2, E), u32))
                    qkv[p][t] = _up(jnp.concatenate(parts, axis=0))

            def scores(p):
                sc_ = _dot(qkv[p][0], qkv[p][1])
                fill = fill_s[0:NR, :]
                sc_ = jnp.where(fill == 0.0, sc_ * SCALE, fill)
                m = jnp.max(sc_, axis=-1, keepdims=True)
                e = jnp.exp(sc_ - m)
                l = jnp.sum(e, axis=-1, keepdims=True)
                r = pl.reciprocal(l, approx=True)
                r = r * (2.0 - l * r)
                ps[p] = (e * r).astype(bf16)

            def fin(p):
                o = _dot(ps[p], qkv[p][2])
                for hh in range(2):
                    h = 2 * p + hh
                    rows = o[32 * hh:32 * hh + 32]
                    odef[h] = o[64 + 8 * hh:72 + 8 * hh]
                    if odef_prev is not None:
                        rows = jnp.concatenate([rows, odef_prev[h], odef[h]], axis=0)
                    os_[h] = _pk(rows)

            acc = [None] * 8
            jobs = iter(jobs)

            def wo(h0, h1, js):
                lhs = _up(jnp.concatenate(os_[h0:h1], axis=1))
                for j in js:
                    ws = []
                    for r0 in range(h0 * E // 2, h1 * E // 2, PIN_ROWS):
                        ws.append(pinned(lambda: wo_s[r0:r0 + PIN_ROWS, j * E:(j + 1) * E],
                                         next(jobs, None)))
                    part = _dot(lhs, _up(jnp.concatenate(ws, axis=0)))
                    if hooks and acc[j] is None and j in hooks:
                        hooks[j](part)
                    acc[j] = part if acc[j] is None else part + acc[j]

            ORDER, LAG_S, LAG_O = SCHED_A if odef_prev is None else SCHED_B
            for p in range(NP):
                if ORDER == 0:
                    proj(p)
                    if p >= LAG_S:
                        scores(p - LAG_S)
                    if p >= LAG_O:
                        fin(p - LAG_O)
                elif ORDER == 1:
                    proj(p, (1, 0))
                    if p >= LAG_O:
                        fin(p - LAG_O)
                    proj(p, (2,))
                    if p >= LAG_S:
                        scores(p - LAG_S)
                elif ORDER == 2:
                    proj(p, (1,))
                    if p >= LAG_S:
                        scores(p - LAG_S)
                    proj(p, (0,))
                    if p >= LAG_O:
                        fin(p - LAG_O)
                    proj(p, (2,))
                elif ORDER == 3:
                    proj(p, (1,))
                    if p >= LAG_O:
                        fin(p - LAG_O)
                    proj(p, (0,))
                    if p >= LAG_S:
                        scores(p - LAG_S)
                    proj(p, (2,))
                elif ORDER == 4:
                    proj(p, (1,))
                    if p >= LAG_S:
                        scores(p - LAG_S)
                    proj(p, (0, 2))
                    if p >= LAG_O:
                        fin(p - LAG_O)
                else:
                    proj(p, (0,))
                    if p >= LAG_S:
                        scores(p - LAG_S)
                    proj(p, (1,))
                    if p >= LAG_O:
                        fin(p - LAG_O)
                    proj(p, (2,))
            tail = []
            for k in range(LAG_O):
                step = []
                if NP - LAG_S + k < NP:
                    step.append(functools.partial(scores, NP - LAG_S + k))
                step.append(functools.partial(fin, NP - LAG_O + k))
                tail.append(step)
            hsplit = min(24, 2 * (NP - LAG_O))
            cuts = {3: (2, 3, 5), 2: (2, 5), 4: (1, 2, 4, 6), 5: (1, 2, 3, 4, 6)}[LAG_O]
            j0 = 0
            for k, step in enumerate(tail):
                wo(0, hsplit, range(j0, cuts[k]))
                j0 = cuts[k]
                for f in step:
                    f()
            wo(0, hsplit, range(j0, 8))
            wo(hsplit, H, range(8))
            return jnp.concatenate(acc, axis=1), odef

        def mixer_prep(i, r0, n, anchor=None):
            r = pl.ds(aligned(i * 64 + r0, 16), n)
            xr = x_s[2 * i + r0 // SEG, r0 % SEG:r0 % SEG + n, :].astype(f32)
            x2 = xr + mod_rows(2, n) * after(aout_s[r0:r0 + n, :], anchor)
            x_s.at[2 * i + r0 // SEG][r0 % SEG:r0 % SEG + n, :] = x2.astype(bf16)
            hb = _ln(x2) * mod_rows(4, n) + mod_rows(3, n)
            hb_s[r, :] = hb.astype(bf16)
            return _ln(hb)

        def mixer_sets(ya, yb, r0, dst=l1_s):
            n = ya.shape[0]
            for m, v in enumerate(_lhs_set(ya[:, :HD], ya[:, HD:], yb[:, :HD], yb[:, HD:])):
                dst[m * (SEG // 2) + r0 // 2:m * (SEG // 2) + (r0 + n) // 2, 0:HD] = _pk(v)

        def mixer_mm(i, src=l1_s):
            for q in range(NQ):
                cs = _strassen(lambda n: _dot(_up(src[n * (SEG // 2):(n + 1) * (SEG // 2), 0:HD]),
                                              _up(t1_s[n, :, _ct(q)])))
                for k, cc in enumerate(cs):
                    r0 = aligned(i * 64 + 8 + (k // 2) * SEG, 8)
                    t_s[pl.ds(r0, SEG), _ct(q + NQ * (k % 2))] = _gelu(cc)

        def p2_body(i, carry):
            slot = i & 1
            for cp in mlp_w_copies(0, slot):
                cp.wait()

            @pl.when(i == 1)
            def _():
                x_copy(1).wait()

            g, rr = mlp_piece(i)
            work = [functools.partial(rhs2_job, g2, slot, 0, 0, n1, t2_s.at[slot], (i >> 1) * 8)
                    for n1 in range(7)]
            work += [functools.partial(rhs2_job, g3, slot, 16 * rt, 0, n1, t3_s.at[g], rr * 32 + 8 * rt)
                     for rt in range(4) for n1 in range(7)]
            work += [functools.partial(rhs2_job, g4, slot, 16 * rt, 4 * og, n1, t4_s.at[og],
                                       g * (E // 2) + rr * 16 + 8 * rt)
                     for rt in range(2) for og in range(NOG) for n1 in range(7)]
            npin = len(work) - FREE_JOBS
            jobs = [None] * 64
            for k in range(npin):
                jobs[1 + k * 63 // npin] = work[k]

            sa_ = 2 * i
            sb_ = 2 * i + 1
            hb_tok = h_rows(sb_)
            oa, odef_a = chain_step(sa_, mem_s[...], hn_s[...], None)
            mixer_mm(jnp.maximum(i - 2, 0))
            ys = []

            def hook(k, anchor):
                if k >= PREP_CH:
                    anchor = anchor[0:8] + ys[-PREP_CH][0:8, 0:E] + ys[-PREP_CH][8:16, 0:E]
                ys.append(mixer_prep(jnp.maximum(i - 1, 0), (k % 2) * SEG + (k // 2) * 16, 16, anchor))
                if k % 2:
                    mixer_sets(ys[-2], ys[-1], (k // 2) * 16)

            hooks = {j: functools.partial(hook, k) for k, j in enumerate(PREP_AT)}
            ob, _ = chain_step(sb_, oa[0:M], hb_tok, odef_a, jobs, hooks)
            for job in work[npin:]:
                job()
            mem_s[...] = ob[0:M]
            aout_s[0:TC, :] = oa[M:SEG]
            aout_s[TC:SEG, :] = ob[SEG:SEG + M]
            aout_s[SEG:SEG + TC, :] = ob[M:SEG]
            aout_s[SEG + TC:2 * SEG, :] = ob[SEG + M:SEG + 2 * M]
            hn_s[...] = h_rows(jnp.minimum(sb_ + 1, NSEG - 1))
            for cp in mlp_w_copies(i + 2, slot):
                cp.start()
            return carry

        lax.fori_loop(0, _N2, _scoped("p2", p2_body), 0)

        TQ = TB // 4
        SHIFT = (-1, -1, 1, 1, -2, -2, 2, 2)

        def u_set(n):
            return w_s.at[n // 32], slice((n % 32) * (TQ // 2), (n % 32 + 1) * (TQ // 2))

        def d_set(slot, n):
            return w_s.at[slot], (n // 4) * (TQ // 2), (n % 4) * 2

        def d_lhs(slot, n):
            ref, r0, c0 = d_set(slot, n)
            return _up(ref[r0:r0 + TQ // 2, c0 * E:(c0 + 2) * E])

        def shift_job(j, r0, n, anchor=None):
            for ct in range(D // E):
                win = t_s[pl.ds(aligned(j * TB + r0, 16), n + 16), _ct(ct)]
                gs_s[r0:r0 + n, _ct(ct)] = after(
                    pltpu.roll(win, (-SHIFT[ct]) % (n + 16), 0)[8:8 + n], anchor)

        def mix(j):
            r0 = aligned(j * TB, TB)
            for og in range(NOG):
                c = _strassen2(lambda n: _dot(d_lhs(3, n), _up(t2_s[og, :, _ct(n)])), *O2)
                for i in range(4):
                    for k in range(2):
                        cols = slice((4 * og + 2 * k) * E, (4 * og + 2 * k + 2) * E)
                        x1_s[i * TQ:(i + 1) * TQ, cols] = (
                            hb_s[pl.ds(r0 + i * TQ, TQ), cols].astype(f32)
                            + jnp.concatenate([c(i, 2 * k), c(i, 2 * k + 1)], axis=1))

        def base_job(j, rt, anchor):
            rows = slice(rt * 16, (rt + 1) * 16)
            z = pltpu.bitcast(pltpu.bitcast(anchor[0:8], u32) & zero_s[0:8, :], f32)
            gb = mod_rows(5, 8) + jnp.concatenate([z] * (D // E), axis=1)
            x2 = x_s[j * (TB // SEG) + rt // 2, (rt % 2) * 16:(rt % 2) * 16 + 16, :]
            base_s[rows, :] = x2.astype(f32) + jnp.concatenate([gb, gb], axis=0) * x1_s[rows, :]

        def out_copy(j, slot):
            return copy(o_s.at[slot], out_hbm.at[pl.ds(aligned(j * TB, TB), TB)], SEM_OUT + slot)

        def ln_job(r0, n, prev, anchor=None):
            if anchor is not None and len(prev) >= 2:
                anchor = anchor[0:8] + prev[-2]
            y = _ln(after(x1_s[r0:r0 + n, :], anchor))
            yn_s[r0:r0 + n, :] = y
            prev.append(y[0:8, 0:E] + y[8:16, 0:E])

        def set_job(src, slot, rt, ct, n1, n=16, anchor=None):
            blk = _outer_operand(lambda i, k: src[i * TQ + rt * n:i * TQ + (rt + 1) * n, _ct(2 * k + ct)],
                                 _LHS_TERMS[n1])
            blk[0] = after(blk[0], anchor)
            blk[3] = after(blk[3], anchor)
            for n2, v in enumerate(_lhs_set(*blk)):
                ref, r0, c0 = d_set(slot, 7 * n1 + n2)
                ref[r0 + rt * n // 2:r0 + (rt + 1) * n // 2, _ct(c0 + ct)] = _pk(v)

        def all_sets(src, slot):
            for n1 in range(7):
                for ct in range(2):
                    set_job(src, slot, 0, ct, n1, TQ)

        wm_wait(wg_s, 0, D // E, SEM_WM)
        mod_tiles(wg_s, 0, D // E, 5 * D // E)
        shift_job(0, 0, TB)
        all_sets(gs_s, 3)
        mix(0)
        mixer_mm(NI - 2)
        mixer_sets(mixer_prep(NI - 1, 0, SEG), mixer_prep(NI - 1, SEG, SEG), 0, w_s.at[4])
        mixer_mm(NI - 1, w_s.at[4])
        ln_job(0, TB, [])
        all_sets(yn_s, 2)
        shift_job(1, 0, TB)
        all_sets(gs_s, 3)

        def mlp_block(j, last):
            slot = j & 1

            jn = clamp(j + 2, NB - 1)
            early = [functools.partial(base_job, j, k) for k in range(TB // 16)]
            shifts = [functools.partial(shift_job, jn, (k % 4) * TQ + (k // 4) * 16, 16)
                      for k in range(TB // 16)]
            if not last and SH_AT is None:
                early += shifts
            early = iter(early)

            def up_prod(n, g):
                m = _dot(d_lhs(2, n), _up(t3_s[g, :, _ct(n)]))
                if n in E_AT:
                    job = next(early, None)
                    if job is not None:
                        job(anchor=m)
                return m

            for g in range(NFG):
                c = _strassen2(lambda n: up_prod(n, g), *O3)
                act = [[_gelu(c(i, k)) for k in range(4)] for i in range(4)]
                for n1 in range(7):
                    blk = _outer_operand(lambda i, k: act[i][k], _LHS_TERMS[n1])
                    for n2, v in enumerate(_lhs_set(*blk)):
                        ref, rows = u_set(7 * n1 + n2)
                        ref[rows, _ct(g)] = _pk(v)
            jobs = {}
            if not last:
                mix(j + 1)
                prev = []
                for k in range(TB // 16):
                    jobs[k * Y_AT] = functools.partial(ln_job, (k % 4) * TQ + (k // 4) * 16, 16, prev)

                def place(start, fns, step=1):
                    for fn in fns:
                        while start in jobs:
                            start += 1
                        jobs[start] = fn
                        start += step

                if SH_AT is not None:
                    place(SH_AT[0], shifts, SH_AT[1])
                for rt in range(2):
                    place(S_AT[rt], [functools.partial(set_job, yn_s, 2, rt, ct, n1, 16)
                                     for ct in range(2) for n1 in range(7)])
                place(G_AT, [functools.partial(set_job, gs_s, 3, rt, ct, n1, 16)
                             for rt in range(2) for ct in range(2) for n1 in range(7)])

            def down_part(n, og, k0, k1):
                ref, rows = u_set(n)
                return _dot(_up(ref[rows, k0 * E:k1 * E]),
                            _up(t4_s[og, k0 * E // 2:k1 * E // 2, _ct(n)]))

            head = {}
            if last:
                head = {n: down_part(n, 0, 0, NFG - 1) for n in range(HEAD)}
            count = [0]

            def down_prod(n, og):
                if og == 0 and n in head:
                    return down_part(n, og, NFG - 1, NFG) + head[n]
                m = down_part(n, og, 0, NFG)
                job = jobs.get(count[0])
                count[0] += 1
                if job is not None:
                    job(anchor=m)
                return m

            for og in range(NOG):
                c = _strassen2(lambda n: down_prod(n, og), *(O4 if not last else (0, O4[1])))
                for i in range(4):
                    rows = slice(i * TQ, (i + 1) * TQ)
                    for k in range(2):
                        c0 = (4 * og + 2 * k) * E
                        o_s.at[slot][rows, c0:c0 + 2 * E] = (
                            base_s[rows, c0:c0 + 2 * E] + mod_rows(5, TQ, c0, 2 * E)
                            * jnp.concatenate([c(i, 2 * k), c(i, 2 * k + 1)], axis=1)).astype(bf16)
            out_copy(j, slot).start()

        def p3_body(j, carry):
            @pl.when(j >= 2)
            def _():
                out_copy(j - 2, j & 1).wait()

            mlp_block(j, False)
            return carry

        lax.fori_loop(0, NB - 1, _scoped("p3", p3_body), 0)
        for k in range(2):
            for cp in mlp_w_copies(0, k):
                cp.wait()
        out_copy(NB - 3, (NB - 3) % 2).wait()
        mlp_block(NB - 1, True)
        out_copy(NB - 2, (NB - 2) % 2).wait()
        out_copy(NB - 1, (NB - 1) % 2).wait()

    pl.run_scoped(
        phase_a,
        pltpu.VMEM((NSEG, M, D), bf16),
        pltpu.VMEM((7, NSEG * M // 4, D // 2), u32),
        pltpu.VMEM((3 * D // E, D, E), bf16),
        pltpu.VMEM((2, D, HG, E), bf16),
        pltpu.VMEM((2, BGR, D), bf16),
        pltpu.VMEM((2, 2, G1R, D), bf16),
        pltpu.VMEM((NC + 1, D // 4, 5 * HG // 2 * E), u32),
    )
    pl.run_scoped(
        phase_b,
        pltpu.VMEM((NOG, D // 8, 49 * E), u32),
        pltpu.VMEM((NFG, D // 8, 49 * E), u32),
        pltpu.VMEM((NOG, F // 8, 49 * E), u32),
        pltpu.VMEM((D // E, D, E), bf16),
        pltpu.VMEM((TB, D), f32),
        pltpu.VMEM((TB, D), f32),
        pltpu.VMEM((TB, D), f32),
        pltpu.VMEM((TB, D), f32),
        pltpu.VMEM((2, TB, D), bf16),
    )


@jax.jit
def pallas_adaLN_cond__memory_aug_recurrent_mem_tr__mixer_s_mlp__prompt_kernel(
    A_x: jax.Array,
    A_mem0: jax.Array,
    A_Wq: jax.Array,
    A_Wk: jax.Array,
    A_Wv: jax.Array,
    A_Wo: jax.Array,
    A_seg_len,
    B_x: jax.Array,
    B_w1: jax.Array,
    B_w2: jax.Array,
    B_w3: jax.Array,
    B_w4: jax.Array,
    c: jax.Array,
    w_mod: jax.Array,
):
    del A_seg_len, B_x
    assert A_x.shape == (1, S, D) and A_mem0.shape == (1, M, D)
    hbm = pl.BlockSpec(memory_space=pl.ANY)
    scratch = [
        pltpu.VMEM((NSEG, SEG, D), bf16),
        pltpu.VMEM((NC + 1, D // 2, HG * E), u32),
        pltpu.VMEM((H * E // 2, D), u32),
        pltpu.VMEM((7, D // 4, D // 2), u32),
        pltpu.VMEM((2, 4, 16, 4 * E), bf16),
        pltpu.VMEM((2, 4, 64, 4 * E), bf16),
        pltpu.VMEM((2, 4, 32, D), bf16),
        pltpu.VMEM((NC, NSEG * M, HG // 2 * E), u32),
        pltpu.VMEM((8, 6 * D), f32),
        pltpu.VMEM((M, D), f32),
        pltpu.VMEM((TC, D), f32),
        pltpu.VMEM((2 * SEG, D), f32),
        pltpu.VMEM((E, E), f32),
        pltpu.VMEM((S, D), bf16),
        pltpu.VMEM((S + 16, D), f32),
        pltpu.VMEM((7 * SEG // 2, D // 2), u32),
        pltpu.VMEM((8 * ZPAD, E), u32),
        pltpu.VMEM((1, D), bf16),
        pltpu.VMEM((M, D), bf16),
        pltpu.SemaphoreType.DMA((24,)),
    ]
    out = pl.pallas_call(
        _kernel,
        out_shape=jax.ShapeDtypeStruct((S, D), bf16),
        in_specs=[hbm] * 12,
        out_specs=hbm,
        scratch_shapes=scratch,
        compiler_params=pltpu.CompilerParams(vmem_limit_bytes=127 * 1024 * 1024,
                                             disable_bounds_checks=NO_BOUNDS),
    )(A_x.reshape(NSEG, SEG, D), A_mem0.reshape(M, D), A_Wq, A_Wk, A_Wv,
      A_Wo.reshape(H * E, D), B_w1.reshape(2, D // 2, D), B_w2.reshape(4, D // 4, D), B_w3.reshape(4, D // 4, F),
      B_w4.reshape(NFG, 4, E, D), c, w_mod)
    return out.reshape(1, S, D)
```

```python
import functools

import jax
import jax.numpy as jnp
from jax import lax
import jax.experimental.pallas as pl
import jax.experimental.pallas.tpu as pltpu

bf16, f32, u32 = jnp.bfloat16, jnp.float32, jnp.uint32

S, D, H, E, M, SEG, F = 2048, 1024, 32, 128, 8, 32, 3584
NSEG = S // SEG
NP = H // 2
TC = SEG - M
HG = 8
NG = H // HG
TB = 128
NB = S // TB
NFG = F // (4 * E)
NOG = D // (4 * E)
NI = NSEG // 2
NQ = D // E // 2
NC = 3 * NG
BGR = 384
G1R = 48
HD = D // 2
X0 = 4
NR = 2 * (M + SEG)
NO_BOUNDS = True
ZPAD = 2
PIN_ROWS = 256
Y_AT = 4
S_AT = (26, 44)
G_AT = 62
HEAD = 14
PREP_AT = (0, 1, 4, 5)
PREP_CH = 2
O3 = (1, 0)
O4 = (0, 0)
O2 = (0, 0)
U_AT = (6, 3, 16)
FREE_JOBS = 0
SH_AT = None
E_AT = (10, 24, 34)
FINE = 1
JGROUP = 1
P1_TAIL = 5
P1_LAG = 4
SCHED_A = (2, 1, 3)
SCHED_B = (3, 1, 3)
EPS = 1e-5
SCALE = E ** -0.5
_SCOPES = False
_N2 = NSEG // 2


def _scoped(name, fn):
    def wrapped(*a):
        if not _SCOPES:
            return fn(*a)
        with jax.named_scope(name):
            return fn(*a)
    return wrapped


def _pk(x):
    return pltpu.bitcast(x.astype(bf16), u32)


def _up(x):
    return pltpu.bitcast(x, bf16)


def _ct(k):
    return slice(k * E, (k + 1) * E)


def _dot(a, b):
    return jnp.dot(a, b, preferred_element_type=f32)


def _ln(x):
    m = jnp.mean(x, axis=-1, keepdims=True)
    xc = x - m
    v = jnp.mean(xc * xc, axis=-1, keepdims=True)
    return xc * lax.rsqrt(v + EPS)


def _gelu(x):
    c = 0.7978845608028654
    return 0.5 * x * (1.0 + jnp.tanh(c * (x + 0.044715 * (x * x * x))))


def _lhs_set(a11, a12, a21, a22):
    return (a11 + a22, a21 + a22, a11, a22, a11 + a12, a21 - a11, a12 - a22)


def _rhs_set(b11, b12, b21, b22):
    return (b11 + b22, b11, b12 - b22, b21 - b11, b22, b11 + b12, b21 + b22)


_LHS_TERMS = (((0, 1), (3, 1)), ((2, 1), (3, 1)), ((0, 1),), ((3, 1),),
              ((0, 1), (1, 1)), ((2, 1), (0, -1)), ((1, 1), (3, -1)))
_RHS_TERMS = (((0, 1), (3, 1)), ((0, 1),), ((1, 1), (3, -1)), ((2, 1), (0, -1)),
              ((3, 1),), ((0, 1), (1, 1)), ((2, 1), (3, 1)))


def _outer_operand(tile, terms):
    out = []
    for i in range(2):
        for j in range(2):
            v = None
            for o, sign in terms:
                t = tile(2 * (o // 2) + i, 2 * (o % 2) + j)
                v = t if v is None else (v + t if sign > 0 else v - t)
            out.append(v)
    return out


class _Quad:
    def __init__(self, tiles):
        self.t = tuple(tiles)

    def __add__(self, other):
        return _Quad([a + b for a, b in zip(self.t, other.t)])

    def __sub__(self, other):
        return _Quad([a - b for a, b in zip(self.t, other.t)])


def _strassen2(m, oo=0, oi=0):
    cs = _strassen(lambda n1: _Quad(_strassen(lambda n2: m(7 * n1 + n2), oi)), oo)
    return lambda i, j: cs[2 * (i // 2) + j // 2].t[2 * (i % 2) + j % 2]


def _strassen(m, order=0):
    if order == 0:
        m1 = m(0)
        m2 = m(1)
        c22 = m1 - m2
        m3 = m(2)
        c22 = c22 + m3
        c22 = m(5) + c22
        m4 = m(3)
        c21 = m2 + m4
        c11 = m1 + m4
        m5 = m(4)
        c12 = m3 + m5
        c11 = c11 - m5
        c11 = m(6) + c11
    else:
        m2 = m(1)
        c22 = m(5) - m2
        m4 = m(3)
        c21 = m2 + m4
        m1 = m(0)
        c22 = c22 + m1
        c11 = m4 + m1
        m3 = m(2)
        c22 = c22 + m3
        m5 = m(4)
        c12 = m3 + m5
        c11 = c11 - m5
        c11 = m(6) + c11
    return c11, c12, c21, c22


def _mask_fill():
    shape = (NR, E)
    r = lax.broadcasted_iota(jnp.int32, shape, 0)
    c = lax.broadcasted_iota(jnp.int32, shape, 1)

    def headpos(i):
        head = jnp.where(i < 64, i >> 5, (i - 64) >> 3)
        pos = jnp.where(i < 64, i & 31, 32 + (i & 7))
        return head, pos

    hr, pr = headpos(r)
    hc, pc = headpos(c)
    same = hr == hc
    valid = same & ((pr < M) | (pr >= pc))
    return jnp.where(valid, 0.0, jnp.where(same, -1e9, -jnp.inf)).astype(f32)


def _kernel(x_hbm, mem0_hbm, wq_hbm, wk_hbm, wv_hbm, wo_hbm, w1_hbm, w2_hbm, w3_hbm,
            w4_hbm, c_hbm, wm_hbm,
            out_hbm,
            x_s, w_s, wo_s, t1_s, g2, g3, g4, pre_s, mod_s, mem_s, hn_s, aout_s, fill_s,
            hb_s, t_s, l1_s, zero_s, c_s, mem0_s, sems):
    w_hbm = (wq_hbm, wk_hbm, wv_hbm)

    (SEM_C, SEM_MEM, SEM_XPRE, SEM_X, SEM_STG, SEM_BG, SEM_OUT,
     SEM_WMR, SEM_G2, SEM_G3, SEM_G4, SEM_WM, SEM_G1) = (0, 1, 2, 3, 4, 6, 8, 10, 12, 14, 16, 18, 22)

    def copy(src, dst, k):
        return pltpu.make_async_copy(src, dst, sems.at[k])

    def aligned(x, n):
        return x if isinstance(x, int) else pl.multiple_of(x, n)

    def clamp(k, hi):
        return min(k, hi) if isinstance(k, int) else jnp.minimum(k, hi)

    def mlp_piece(k):
        k = clamp(k, 4 * NFG - 1)
        return k >> 2, k & 3

    def mlp_w_copies(k, slot):
        g, rr = mlp_piece(k)
        k2 = clamp(k, NI - 1)
        return (copy(w2_hbm.at[:, pl.ds(aligned((k2 >> 1) * 16, 16), 16),
                               pl.ds(aligned((k2 & 1) * 4 * E, E), 4 * E)], g2.at[slot], SEM_G2 + slot),
                copy(w3_hbm.at[:, pl.ds(aligned(rr * 64, 64), 64), pl.ds(aligned(g * 4 * E, E), 4 * E)],
                     g3.at[slot], SEM_G3 + slot),
                copy(w4_hbm.at[g, :, pl.ds(aligned(rr * 32, 32), 32), :], g4.at[slot], SEM_G4 + slot))

    def pinned(w, job):
        if job is None:
            return w()
        z = job() & zero_s[0:8, :]
        w = w()
        return jnp.concatenate([w[0:8] | z, w[8:]], axis=0)

    def after(x, anchor):
        if anchor is None:
            return x
        z = pltpu.bitcast(pltpu.bitcast(anchor[0:8], u32) & zero_s[0:8, :], f32)
        z = jnp.concatenate([z] * (x.shape[0] // 8), axis=0)
        return jnp.concatenate([x[:, 0:E] + z, x[:, E:]], axis=1) if x.shape[1] > E else x + z

    def rhs_job(src, slot, r0, c1, c2, dst, q, row, z=None):
        blk = [src[slot, kh, r0:r0 + 16, cc * E:(cc + 1) * E].astype(f32)
               for kh in range(2) for cc in (c1, c2)]
        if z is not None:
            zf = pltpu.bitcast(jnp.concatenate([z, z], axis=0), f32)
            blk[0] = blk[0] + zf
            blk[3] = blk[3] + zf
        sets = _rhs_set(*blk)
        for n, v in enumerate(sets):
            dst.at[n][pl.ds(pl.multiple_of(row, 8), 8), _ct(q)] = _pk(v)
        out = pltpu.bitcast(sets[2], u32) | pltpu.bitcast(sets[3], u32)
        return out[0:8] | out[8:16]

    def rhs2_job(src, slot, r0, c0, n1, dst, row):
        blk = _outer_operand(lambda i, j: src[slot, i, r0:r0 + 16, _ct(c0 + j)].astype(f32),
                             _RHS_TERMS[n1])
        sets = _rhs_set(*blk)
        for n2, v in enumerate(sets):
            dst[pl.ds(pl.multiple_of(row, 8), 8), _ct(7 * n1 + n2)] = _pk(v)
        out = pltpu.bitcast(sets[2], u32) | pltpu.bitcast(sets[3], u32)
        return out[0:8] | out[8:16]

    def silu_c():
        cf = c_s[...].astype(f32)
        return jnp.broadcast_to(cf * (1.0 / (1.0 + jnp.exp(-cf))), (8, D)).astype(bf16)

    def wm_copy(wm_s, src_tile, dst_tile, sem):
        return copy(wm_hbm.at[:, pl.ds(aligned(src_tile * E, E), E)], wm_s.at[dst_tile], sem)

    def wm_wait(wm_s, t0, n, sem):
        copy(wm_s.at[t0:t0 + n], wm_s.at[t0:t0 + n], sem).wait()

    def mod_tiles(wm_s, t0, n, dst_tile):
        sc8 = silu_c()
        for k in range(n):
            v = _dot(sc8, wm_s[t0 + k])
            if (dst_tile + k) // (D // E) in (1, 4):
                v = 1.0 + v
            mod_s[:, _ct(dst_tile + k)] = v

    def x_copy(k):
        r = slice(0, X0) if k == 0 else slice(X0, NSEG)
        return copy(x_hbm.at[r], x_s.at[r], SEM_XPRE if k == 0 else SEM_X)

    def h_rows(s):
        return _ln(x_s[s, 0:TC, :].astype(f32)) * mod_rows(1, TC) + mod_rows(0, TC)

    def mod_rows(k, n, c0=0, w=D):
        return jnp.concatenate([mod_s[:, k * D + c0:k * D + c0 + w]] * (n // 8), axis=0)

    def phase_a(xpre_s, hpre_s, wm_s, stg, bg, g1, tq_s):
        def tq_place(c, n):
            if n == 1:
                return w_s.at[c], 0, None
            if n == 4:
                return w_s.at[c], D // 4, None
            return tq_s.at[c], 0, (0, 2, 3, 5, 6).index(n) * (HG // 2)

        def w_copy(t, g, slot):
            return copy(w_hbm[t].at[:, pl.ds(pl.multiple_of(g * HG, HG), HG), :], stg.at[slot],
                        SEM_STG + slot)

        def bg_rows(k):
            return clamp(k * BGR, H * E - BGR), clamp(k * G1R, HD - G1R)

        def bg_copies(k, slot):
            ro, r1 = bg_rows(k)
            return (copy(wo_hbm.at[pl.ds(aligned(ro, 16), BGR)], bg.at[slot], SEM_BG + slot),
                    copy(w1_hbm.at[:, pl.ds(aligned(r1, 16), G1R), :], g1.at[slot], SEM_G1 + slot))

        def relayout_jobs(slot, c, i):
            memo = []
            r = aligned(i * 8, 8)

            def job(j, z=None):
                if not memo:
                    for d0 in (i * 16, HD + i * 16):
                        memo.append(jnp.swapaxes(pltpu.bitcast(stg[slot, pl.ds(d0, 16)], u32), 0, 1))
                blk = []
                for kh in range(2):
                    u = memo[kh][j]
                    if z is not None:
                        u = u | jnp.concatenate([z, z], axis=0)
                    blk.append(pltpu.bitcast(u << 16, f32))
                    blk.append(pltpu.bitcast(u & jnp.uint32(0xFFFF0000), f32))
                for k, v in enumerate(blk):
                    w_s.at[c][pl.ds((k // 2) * (D // 4) + r, 8), _ct(2 * j + k % 2)] = _pk(v)
                for n, v in enumerate(_rhs_set(*blk)):
                    if n not in (1, 4):
                        ref, r0, c0 = tq_place(c, n)
                        ref[pl.ds(r0 + r, 8), _ct(c0 + j)] = _pk(v)

            return [functools.partial(job, j) for j in range(HG // 2)]

        def repack(slot, row, i, z):
            v = pltpu.bitcast(bg[slot, 16 * i:16 * i + 16, :], u32)
            v = v | jnp.concatenate([z] * (D // E), axis=1)
            wo_s[pl.ds(pl.multiple_of(row + 8 * i, 8), 8), :] = v

        cp_c = copy(c_hbm, c_s, SEM_C)
        cp_mem = copy(mem0_hbm, mem0_s, SEM_MEM)
        cp_xpre = copy(x_hbm.at[:, TC:SEG, :], xpre_s, SEM_XPRE)
        w_copy(0, 0, 0).start()
        cp_xpre.start()
        cp_c.start()
        cp_mem.start()
        for k in range(2 * D // E):
            wm_copy(wm_s, k, k, SEM_WM + k // 4).start()
        w_copy(0, 1, 1).start()

        zero_s[0:8, :] = jnp.zeros((8, E), u32)
        fill_s[0:NR, :] = _mask_fill()
        aout_s[...] = jnp.zeros(aout_s.shape, f32)
        l1_s[...] = jnp.zeros(l1_s.shape, u32)
        bg[1] = jnp.zeros(bg.shape[1:], bf16)
        g1[1] = jnp.zeros(g1.shape[1:], bf16)

        w_copy(0, 0, 0).wait()

        def rl0_body(i, carry):
            for job in relayout_jobs(0, 0, i):
                job()
            return carry

        lax.fori_loop(0, D // 32, rl0_body, 0)
        w_copy(0, 2, 0).start()
        for cp in bg_copies(0, 0):
            cp.start()

        cp_xpre.wait()

        def npre_body(i, carry):
            xr = xpre_s[pl.ds(pl.multiple_of(i * 8, 8), 8)].astype(f32).reshape(64, D)
            t_s[pl.ds(pl.multiple_of(i * 64, 64), 64), :] = _ln(xr)
            return carry

        lax.fori_loop(0, NSEG // 8, _scoped("npre", npre_body), 0)

        cp_c.wait()
        cp_mem.wait()
        mem_s[...] = mem0_s[...].astype(f32)

        for k in range(4):
            wm_wait(wm_s, 4 * k, 4, SEM_WM + k)
            mod_tiles(wm_s, 4 * k, 4, 4 * k)

        PH = NSEG * M // 2

        def hpre_body(i, carry):
            h = [t_s[pl.ds(pl.multiple_of(hf * PH + i * 16, 16), 16), :] * mod_rows(1, 16) + mod_rows(0, 16)
                 for hf in range(2)]
            for n, v in enumerate(_lhs_set(h[0][:, :HD], h[0][:, HD:], h[1][:, :HD], h[1][:, HD:])):
                hpre_s.at[n][pl.ds(pl.multiple_of(i * 8, 8), 8), :] = _pk(v)
            return carry

        lax.fori_loop(0, PH // 16, _scoped("hpre", hpre_body), 0)

        t_s[0:8, :] = jnp.zeros((8, D), f32)
        t_s[S + 8:S + 16, :] = jnp.zeros((8, D), f32)

        MB = 64

        def p1_body(c, carry):
            slot = c & 1
            pslot = 1 - slot
            ro, r1 = bg_rows(jnp.maximum(c - 1, 0))

            @pl.when(c >= 1)
            def _():
                for cp in bg_copies(0, pslot):
                    cp.wait()

            @pl.when(c + 1 < NC)
            def _():
                w_copy(0, 0, pslot).wait()

            small = [functools.partial(repack, pslot, ro >> 1, i) for i in range(BGR // 16)]
            small += [functools.partial(rhs_job, g1, pslot, 16 * rt, q, NQ + q, t1_s, q, (r1 >> 1) + 8 * rt)
                      for rt in range(G1R // 16) for q in range(NQ)]
            work = []
            nu = D // 32
            for i in range(nu):
                js = relayout_jobs(pslot, c + 1, i)
                work += [js[k:k + JGROUP] for k in range(0, len(js), JGROUP)]
                work += [[job] for job in small[i * len(small) // nu:(i + 1) * len(small) // nu]]
            npin = 7 * (HG // 2) * (PH // MB)
            jobs = [[] for _ in range(npin)]
            for k, group in enumerate(work):
                pos = k * (npin - P1_TAIL) * 8 // len(work)
                jobs[pos // 8] += [(job, pos % 8 if FINE else 0) for job in group]
            jobs = iter(jobs)

            def prod(n, q, mb):
                ref, r0, c0 = tq_place(c, n)
                w = ref[r0:r0 + D // 4, _ct(2 * q + (n == 4) if c0 is None else c0 + q)]
                m = _dot(_up(hpre_s[n, mb * MB // 2:(mb + 1) * MB // 2, :]), _up(w))
                pending.append(m)
                if len(pending) > P1_LAG:
                    anchor = pltpu.bitcast(pending.pop(0), u32)
                    for job, g in next(jobs):
                        job(anchor[8 * g:8 * g + 8] & zero_s[0:8, :])
                return m

            pending = []
            ns = MB // M
            for q in range(HG // 2):
                for mb in range(PH // MB):
                    cs = _strassen(lambda n: prod(n, q, mb))
                    for hf in range(2):
                        y = jnp.concatenate([cs[2 * hf + k][sg * M:(sg + 1) * M]
                                             for sg in range(ns) for k in range(2)], axis=0)
                        s0 = hf * (NSEG // 2) + mb * ns
                        pre_s.at[c][s0 * M:(s0 + ns) * M, _ct(q)] = _pk(y)

            for t in range(3):
                @pl.when((c + 3) >> 2 == t)
                def _():
                    w_copy(t, (c + 3) & 3, pslot).start()

            @pl.when(c + 2 < NC)
            def _():
                for cp in bg_copies(c + 1, pslot):
                    cp.start()

            @pl.when(c < NC - 3)
            def _():
                wm_copy(wm_s, 2 * D // E + c, c, SEM_WMR).start()

            @pl.when(c == NC - 3)
            def _():
                def issue(k, carry2):
                    wm_copy(wm_s, 2 * D // E + k, k, SEM_WMR).start()
                    return carry2

                x_copy(0).start()
                for k in range(2):
                    for cp in mlp_w_copies(k, k):
                        cp.start()
                lax.fori_loop(NC - 3, 3 * D // E, issue, 0)

            return carry

        lax.fori_loop(0, NC, _scoped("p1", p1_body), 0)
        x_copy(1).start()
        x_copy(0).wait()
        wm_wait(wm_s, 0, 3 * D // E, SEM_WMR)
        mod_tiles(wm_s, 0, 3 * D // E, 2 * D // E)
        hn_s[...] = h_rows(0)

    def phase_b(t2_s, t3_s, t4_s, wg_s, x1_s, base_s, yn_s, gs_s, act_s, o_s):
        for k in range(D // E):
            wm_copy(wg_s, 5 * D // E + k, k, SEM_WM).start()

        def chain_step(s, mem, htok, odef_prev, jobs=(), hooks=None):
            hs = jnp.concatenate([mem, htok], axis=0).astype(bf16)
            qkv = [[None] * 3 for _ in range(NP)]
            ps = [None] * NP
            os_ = [None] * H
            odef = [None] * H

            def proj(p, ts=(0, 1, 2)):
                for t in ts:
                    c, q = t * NG + p // (HG // 2), p % (HG // 2)
                    a = _dot(hs, _up(w_s[c, :, _ct(2 * q)]))
                    b = _dot(hs, _up(w_s[c, :, _ct(2 * q + 1)]))
                    if hooks and t == 2 and p - NP in hooks:
                        hooks[p - NP](b)
                    pre = pre_s[c, pl.ds(pl.multiple_of(s * M, M), M), _ct(q)]
                    if t == 1:
                        kf = jnp.concatenate([a, b, _up(pre).astype(f32), jnp.zeros((E - NR, E), f32)],
                                             axis=0)
                        qkv[p][t] = kf.T.astype(bf16)
                        continue
                    parts = [_pk(a), _pk(b), pre]
                    if t == 2:
                        parts.append(jnp.zeros(((E - NR) // 2, E), u32))
                    qkv[p][t] = _up(jnp.concatenate(parts, axis=0))

            def scores(p):
                sc_ = _dot(qkv[p][0], qkv[p][1])
                fill = fill_s[0:NR, :]
                sc_ = jnp.where(fill == 0.0, sc_ * SCALE, fill)
                m = jnp.max(sc_, axis=-1, keepdims=True)
                e = jnp.exp(sc_ - m)
                l = jnp.sum(e, axis=-1, keepdims=True)
                r = pl.reciprocal(l, approx=True)
                r = r * (2.0 - l * r)
                ps[p] = (e * r).astype(bf16)

            def fin(p):
                o = _dot(ps[p], qkv[p][2])
                for hh in range(2):
                    h = 2 * p + hh
                    rows = o[32 * hh:32 * hh + 32]
                    odef[h] = o[64 + 8 * hh:72 + 8 * hh]
                    if odef_prev is not None:
                        rows = jnp.concatenate([rows, odef_prev[h], odef[h]], axis=0)
                    os_[h] = _pk(rows)

            acc = [None] * 8
            jobs = iter(jobs)

            def wo(h0, h1, js):
                lhs = _up(jnp.concatenate(os_[h0:h1], axis=1))
                for j in js:
                    ws = []
                    for r0 in range(h0 * E // 2, h1 * E // 2, PIN_ROWS):
                        ws.append(pinned(lambda: wo_s[r0:r0 + PIN_ROWS, j * E:(j + 1) * E],
                                         next(jobs, None)))
                    part = _dot(lhs, _up(jnp.concatenate(ws, axis=0)))
                    if hooks and acc[j] is None and j in hooks:
                        hooks[j](part)
                    acc[j] = part if acc[j] is None else part + acc[j]

            ORDER, LAG_S, LAG_O = SCHED_A if odef_prev is None else SCHED_B
            for p in range(NP):
                if ORDER == 0:
                    proj(p)
                    if p >= LAG_S:
                        scores(p - LAG_S)
                    if p >= LAG_O:
                        fin(p - LAG_O)
                elif ORDER == 1:
                    proj(p, (1, 0))
                    if p >= LAG_O:
                        fin(p - LAG_O)
                    proj(p, (2,))
                    if p >= LAG_S:
                        scores(p - LAG_S)
                elif ORDER == 2:
                    proj(p, (1,))
                    if p >= LAG_S:
                        scores(p - LAG_S)
                    proj(p, (0,))
                    if p >= LAG_O:
                        fin(p - LAG_O)
                    proj(p, (2,))
                elif ORDER == 3:
                    proj(p, (1,))
                    if p >= LAG_O:
                        fin(p - LAG_O)
                    proj(p, (0,))
                    if p >= LAG_S:
                        scores(p - LAG_S)
                    proj(p, (2,))
                elif ORDER == 4:
                    proj(p, (1,))
                    if p >= LAG_S:
                        scores(p - LAG_S)
                    proj(p, (0, 2))
                    if p >= LAG_O:
                        fin(p - LAG_O)
                else:
                    proj(p, (0,))
                    if p >= LAG_S:
                        scores(p - LAG_S)
                    proj(p, (1,))
                    if p >= LAG_O:
                        fin(p - LAG_O)
                    proj(p, (2,))
            tail = []
            for k in range(LAG_O):
                step = []
                if NP - LAG_S + k < NP:
                    step.append(functools.partial(scores, NP - LAG_S + k))
                step.append(functools.partial(fin, NP - LAG_O + k))
                tail.append(step)
            hsplit = min(24, 2 * (NP - LAG_O))
            cuts = {3: (2, 3, 5), 2: (2, 5), 4: (1, 2, 4, 6), 5: (1, 2, 3, 4, 6)}[LAG_O]
            j0 = 0
            for k, step in enumerate(tail):
                wo(0, hsplit, range(j0, cuts[k]))
                j0 = cuts[k]
                for f in step:
                    f()
            wo(0, hsplit, range(j0, 8))
            wo(hsplit, H, range(8))
            return jnp.concatenate(acc, axis=1), odef

        def mixer_prep(i, r0, n, anchor=None):
            r = pl.ds(aligned(i * 64 + r0, 16), n)
            xr = x_s[2 * i + r0 // SEG, r0 % SEG:r0 % SEG + n, :].astype(f32)
            x2 = xr + mod_rows(2, n) * after(aout_s[r0:r0 + n, :], anchor)
            x_s.at[2 * i + r0 // SEG][r0 % SEG:r0 % SEG + n, :] = x2.astype(bf16)
            hb = _ln(x2) * mod_rows(4, n) + mod_rows(3, n)
            hb_s[r, :] = hb.astype(bf16)
            return _ln(hb)

        def mixer_sets(ya, yb, r0, dst=l1_s):
            n = ya.shape[0]
            for m, v in enumerate(_lhs_set(ya[:, :HD], ya[:, HD:], yb[:, :HD], yb[:, HD:])):
                dst[m * (SEG // 2) + r0 // 2:m * (SEG // 2) + (r0 + n) // 2, 0:HD] = _pk(v)

        def mixer_mm(i, src=l1_s):
            for q in range(NQ):
                cs = _strassen(lambda n: _dot(_up(src[n * (SEG // 2):(n + 1) * (SEG // 2), 0:HD]),
                                              _up(t1_s[n, :, _ct(q)])))
                for k, cc in enumerate(cs):
                    r0 = aligned(i * 64 + 8 + (k // 2) * SEG, 8)
                    t_s[pl.ds(r0, SEG), _ct(q + NQ * (k % 2))] = _gelu(cc)

        def p2_body(i, carry):
            slot = i & 1
            for cp in mlp_w_copies(0, slot):
                cp.wait()

            @pl.when(i == 1)
            def _():
                x_copy(1).wait()

            g, rr = mlp_piece(i)
            work = [functools.partial(rhs2_job, g2, slot, 0, 0, n1, t2_s.at[slot], (i >> 1) * 8)
                    for n1 in range(7)]
            work += [functools.partial(rhs2_job, g3, slot, 16 * rt, 0, n1, t3_s.at[g], rr * 32 + 8 * rt)
                     for rt in range(4) for n1 in range(7)]
            work += [functools.partial(rhs2_job, g4, slot, 16 * rt, 4 * og, n1, t4_s.at[og],
                                       g * (E // 2) + rr * 16 + 8 * rt)
                     for rt in range(2) for og in range(NOG) for n1 in range(7)]
            npin = len(work) - FREE_JOBS
            jobs = [None] * 64
            for k in range(npin):
                jobs[1 + k * 63 // npin] = work[k]

            sa_ = 2 * i
            sb_ = 2 * i + 1
            hb_tok = h_rows(sb_)
            oa, odef_a = chain_step(sa_, mem_s[...], hn_s[...], None)
            mixer_mm(jnp.maximum(i - 2, 0))
            ys = []

            def hook(k, anchor):
                if k >= PREP_CH:
                    anchor = anchor[0:8] + ys[-PREP_CH][0:8, 0:E] + ys[-PREP_CH][8:16, 0:E]
                ys.append(mixer_prep(jnp.maximum(i - 1, 0), (k % 2) * SEG + (k // 2) * 16, 16, anchor))
                if k % 2:
                    mixer_sets(ys[-2], ys[-1], (k // 2) * 16)

            hooks = {j: functools.partial(hook, k) for k, j in enumerate(PREP_AT)}
            ob, _ = chain_step(sb_, oa[0:M], hb_tok, odef_a, jobs, hooks)
            for job in work[npin:]:
                job()
            mem_s[...] = ob[0:M]
            aout_s[0:TC, :] = oa[M:SEG]
            aout_s[TC:SEG, :] = ob[SEG:SEG + M]
            aout_s[SEG:SEG + TC, :] = ob[M:SEG]
            aout_s[SEG + TC:2 * SEG, :] = ob[SEG + M:SEG + 2 * M]
            hn_s[...] = h_rows(jnp.minimum(sb_ + 1, NSEG - 1))
            for cp in mlp_w_copies(i + 2, slot):
                cp.start()
            return carry

        lax.fori_loop(0, _N2, _scoped("p2", p2_body), 0)

        TQ = TB // 4
        SHIFT = (-1, -1, 1, 1, -2, -2, 2, 2)

        def u_set(n):
            return w_s.at[n // 32], slice((n % 32) * (TQ // 2), (n % 32 + 1) * (TQ // 2))

        def d_set(slot, n):
            return w_s.at[slot], (n // 4) * (TQ // 2), (n % 4) * 2

        def d_lhs(slot, n):
            ref, r0, c0 = d_set(slot, n)
            return _up(ref[r0:r0 + TQ // 2, c0 * E:(c0 + 2) * E])

        def shift_job(j, r0, n, anchor=None):
            for ct in range(D // E):
                win = t_s[pl.ds(aligned(j * TB + r0, 16), n + 16), _ct(ct)]
                gs_s[r0:r0 + n, _ct(ct)] = after(
                    pltpu.roll(win, (-SHIFT[ct]) % (n + 16), 0)[8:8 + n], anchor)

        def mix(j, hook=None):
            r0 = aligned(j * TB, TB)
            for og in range(NOG):
                def prod(n):
                    m = _dot(d_lhs(3, n), _up(t2_s[og, :, _ct(n)]))
                    if hook is not None:
                        hook(m)
                    return m

                c = _strassen2(prod, *O2)
                for i in range(4):
                    for k in range(2):
                        cols = slice((4 * og + 2 * k) * E, (4 * og + 2 * k + 2) * E)
                        x1_s[i * TQ:(i + 1) * TQ, cols] = (
                            hb_s[pl.ds(r0 + i * TQ, TQ), cols].astype(f32)
                            + jnp.concatenate([c(i, 2 * k), c(i, 2 * k + 1)], axis=1))

        def base_job(j, rt, anchor):
            rows = slice(rt * 16, (rt + 1) * 16)
            z = pltpu.bitcast(pltpu.bitcast(anchor[0:8], u32) & zero_s[0:8, :], f32)
            gb = mod_rows(5, 8) + jnp.concatenate([z] * (D // E), axis=1)
            x2 = x_s[j * (TB // SEG) + rt // 2, (rt % 2) * 16:(rt % 2) * 16 + 16, :]
            base_s[rows, :] = x2.astype(f32) + jnp.concatenate([gb, gb], axis=0) * x1_s[rows, :]

        def out_copy(j, slot):
            return copy(o_s.at[slot], out_hbm.at[pl.ds(aligned(j * TB, TB), TB)], SEM_OUT + slot)

        def ln_job(r0, n, prev, anchor=None):
            if anchor is not None and len(prev) >= 2:
                anchor = anchor[0:8] + prev[-2]
            y = _ln(after(x1_s[r0:r0 + n, :], anchor))
            yn_s[r0:r0 + n, :] = y
            prev.append(y[0:8, 0:E] + y[8:16, 0:E])

        def set_job(src, slot, rt, ct, n1, n=16, anchor=None):
            blk = _outer_operand(lambda i, k: src[i * TQ + rt * n:i * TQ + (rt + 1) * n, _ct(2 * k + ct)],
                                 _LHS_TERMS[n1])
            blk[0] = after(blk[0], anchor)
            blk[3] = after(blk[3], anchor)
            for n2, v in enumerate(_lhs_set(*blk)):
                ref, r0, c0 = d_set(slot, 7 * n1 + n2)
                ref[r0 + rt * n // 2:r0 + (rt + 1) * n // 2, _ct(c0 + ct)] = _pk(v)

        def all_sets(src, slot):
            for n1 in range(7):
                for ct in range(2):
                    set_job(src, slot, 0, ct, n1, TQ)

        wm_wait(wg_s, 0, D // E, SEM_WM)
        mod_tiles(wg_s, 0, D // E, 5 * D // E)
        shift_job(0, 0, TB)
        all_sets(gs_s, 3)
        mix(0)
        mixer_mm(NI - 2)
        mixer_sets(mixer_prep(NI - 1, 0, SEG), mixer_prep(NI - 1, SEG, SEG), 0, w_s.at[4])
        mixer_mm(NI - 1, w_s.at[4])
        ln_job(0, TB, [])
        all_sets(yn_s, 2)
        shift_job(1, 0, TB)
        all_sets(gs_s, 3)

        def mlp_block(j, last):
            slot = j & 1

            jn = clamp(j + 2, NB - 1)
            early = [functools.partial(base_job, j, k) for k in range(TB // 16)]
            shifts = [functools.partial(shift_job, jn, (k % 4) * TQ + (k // 4) * 16, 16)
                      for k in range(TB // 16)]
            if not last and SH_AT is None:
                early += shifts
            early = iter(early)

            pend = []
            tick = [0]

            def drain(m):
                tick[0] += 1
                if pend and tick[0] >= U_AT[0] and (tick[0] - U_AT[0]) % U_AT[1] == 0:
                    pend.pop(0)(m)

            def up_prod(n, g):
                m = _dot(d_lhs(2, n), _up(t3_s[g, :, _ct(n)]))
                if n in E_AT:
                    job = next(early, None)
                    if job is not None:
                        job(anchor=m)
                drain(m)
                return m

            def uset_job(tile, g, n1, r0, n, anchor=None):
                blk = _outer_operand(lambda i, k: tile(i, k, r0, n), _LHS_TERMS[n1])
                blk[0] = after(blk[0], anchor)
                blk[3] = after(blk[3], anchor)
                for n2, v in enumerate(_lhs_set(*blk)):
                    ref, rows = u_set(7 * n1 + n2)
                    ref[rows.start + r0 // 2:rows.start + (r0 + n) // 2, _ct(g)] = _pk(v)

            for g in range(NFG):
                c = _strassen2(lambda n: up_prod(n, g), *O3)
                assert not pend
                tick[0] = 0
                if U_AT[1] == 0 or (last and g == NFG - 1):
                    act = [[_gelu(c(i, k)) for k in range(4)] for i in range(4)]
                    for n1 in range(7):
                        uset_job(lambda i, k, r0, n: act[i][k], g, n1, 0, TQ)
                    continue
                c0 = 4 * (g % 2)
                for i in range(4):
                    for k in range(4):
                        act_s[i * TQ:(i + 1) * TQ, _ct(c0 + k)] = _gelu(c(i, k))

                def tile(i, k, r0, n, c0=c0):
                    return act_s[i * TQ + r0:i * TQ + r0 + n, _ct(c0 + k)]

                pend += [functools.partial(uset_job, tile, g, n1, r0, U_AT[2])
                         for n1 in range(7) for r0 in range(0, TQ, U_AT[2])]
            jobs = {}
            if not last:
                mix(j + 1, drain)
                assert not pend
                prev = []
                for k in range(TB // 16):
                    jobs[k * Y_AT] = functools.partial(ln_job, (k % 4) * TQ + (k // 4) * 16, 16, prev)

                def place(start, fns, step=1):
                    for fn in fns:
                        while start in jobs:
                            start += 1
                        jobs[start] = fn
                        start += step

                if SH_AT is not None:
                    place(SH_AT[0], shifts, SH_AT[1])
                for rt in range(2):
                    place(S_AT[rt], [functools.partial(set_job, yn_s, 2, rt, ct, n1, 16)
                                     for ct in range(2) for n1 in range(7)])
                place(G_AT, [functools.partial(set_job, gs_s, 3, rt, ct, n1, 16)
                             for rt in range(2) for ct in range(2) for n1 in range(7)])

            def down_part(n, og, k0, k1):
                ref, rows = u_set(n)
                return _dot(_up(ref[rows, k0 * E:k1 * E]),
                            _up(t4_s[og, k0 * E // 2:k1 * E // 2, _ct(n)]))

            head = {}
            if last:
                head = {n: down_part(n, 0, 0, NFG - 1) for n in range(HEAD)}
            count = [0]

            def down_prod(n, og):
                if og == 0 and n in head:
                    return down_part(n, og, NFG - 1, NFG) + head[n]
                m = down_part(n, og, 0, NFG)
                job = jobs.get(count[0])
                count[0] += 1
                if job is not None:
                    job(anchor=m)
                return m

            for og in range(NOG):
                c = _strassen2(lambda n: down_prod(n, og), *(O4 if not last else (0, O4[1])))
                for i in range(4):
                    rows = slice(i * TQ, (i + 1) * TQ)
                    for k in range(2):
                        c0 = (4 * og + 2 * k) * E
                        o_s.at[slot][rows, c0:c0 + 2 * E] = (
                            base_s[rows, c0:c0 + 2 * E] + mod_rows(5, TQ, c0, 2 * E)
                            * jnp.concatenate([c(i, 2 * k), c(i, 2 * k + 1)], axis=1)).astype(bf16)
            out_copy(j, slot).start()

        def p3_body(j, carry):
            @pl.when(j >= 2)
            def _():
                out_copy(j - 2, j & 1).wait()

            mlp_block(j, False)
            return carry

        lax.fori_loop(0, NB - 1, _scoped("p3", p3_body), 0)
        for k in range(2):
            for cp in mlp_w_copies(0, k):
                cp.wait()
        out_copy(NB - 3, (NB - 3) % 2).wait()
        mlp_block(NB - 1, True)
        out_copy(NB - 2, (NB - 2) % 2).wait()
        out_copy(NB - 1, (NB - 1) % 2).wait()

    pl.run_scoped(
        phase_a,
        pltpu.VMEM((NSEG, M, D), bf16),
        pltpu.VMEM((7, NSEG * M // 4, D // 2), u32),
        pltpu.VMEM((3 * D // E, D, E), bf16),
        pltpu.VMEM((2, D, HG, E), bf16),
        pltpu.VMEM((2, BGR, D), bf16),
        pltpu.VMEM((2, 2, G1R, D), bf16),
        pltpu.VMEM((NC + 1, D // 4, 5 * HG // 2 * E), u32),
    )
    pl.run_scoped(
        phase_b,
        pltpu.VMEM((NOG, D // 8, 49 * E), u32),
        pltpu.VMEM((NFG, D // 8, 49 * E), u32),
        pltpu.VMEM((NOG, F // 8, 49 * E), u32),
        pltpu.VMEM((D // E, D, E), bf16),
        pltpu.VMEM((TB, D), f32),
        pltpu.VMEM((TB, D), f32),
        pltpu.VMEM((TB, D), f32),
        pltpu.VMEM((TB, D), f32),
        pltpu.VMEM((TB, D), f32),
        pltpu.VMEM((2, TB, D), bf16),
    )


@jax.jit
def pallas_adaLN_cond__memory_aug_recurrent_mem_tr__mixer_s_mlp__prompt_kernel(
    A_x: jax.Array,
    A_mem0: jax.Array,
    A_Wq: jax.Array,
    A_Wk: jax.Array,
    A_Wv: jax.Array,
    A_Wo: jax.Array,
    A_seg_len,
    B_x: jax.Array,
    B_w1: jax.Array,
    B_w2: jax.Array,
    B_w3: jax.Array,
    B_w4: jax.Array,
    c: jax.Array,
    w_mod: jax.Array,
):
    del A_seg_len, B_x
    assert A_x.shape == (1, S, D) and A_mem0.shape == (1, M, D)
    hbm = pl.BlockSpec(memory_space=pl.ANY)
    scratch = [
        pltpu.VMEM((NSEG, SEG, D), bf16),
        pltpu.VMEM((NC + 1, D // 2, HG * E), u32),
        pltpu.VMEM((H * E // 2, D), u32),
        pltpu.VMEM((7, D // 4, D // 2), u32),
        pltpu.VMEM((2, 4, 16, 4 * E), bf16),
        pltpu.VMEM((2, 4, 64, 4 * E), bf16),
        pltpu.VMEM((2, 4, 32, D), bf16),
        pltpu.VMEM((NC, NSEG * M, HG // 2 * E), u32),
        pltpu.VMEM((8, 6 * D), f32),
        pltpu.VMEM((M, D), f32),
        pltpu.VMEM((TC, D), f32),
        pltpu.VMEM((2 * SEG, D), f32),
        pltpu.VMEM((E, E), f32),
        pltpu.VMEM((S, D), bf16),
        pltpu.VMEM((S + 16, D), f32),
        pltpu.VMEM((7 * SEG // 2, D // 2), u32),
        pltpu.VMEM((8 * ZPAD, E), u32),
        pltpu.VMEM((1, D), bf16),
        pltpu.VMEM((M, D), bf16),
        pltpu.SemaphoreType.DMA((24,)),
    ]
    out = pl.pallas_call(
        _kernel,
        out_shape=jax.ShapeDtypeStruct((S, D), bf16),
        in_specs=[hbm] * 12,
        out_specs=hbm,
        scratch_shapes=scratch,
        compiler_params=pltpu.CompilerParams(vmem_limit_bytes=127 * 1024 * 1024,
                                             disable_bounds_checks=NO_BOUNDS),
    )(A_x.reshape(NSEG, SEG, D), A_mem0.reshape(M, D), A_Wq, A_Wk, A_Wv,
      A_Wo.reshape(H * E, D), B_w1.reshape(2, D // 2, D), B_w2.reshape(4, D // 4, D), B_w3.reshape(4, D // 4, F),
      B_w4.reshape(NFG, 4, E, D), c, w_mod)
    return out.reshape(1, S, D)
```

```python
import functools

import jax
import jax.numpy as jnp
from jax import lax
import jax.experimental.pallas as pl
import jax.experimental.pallas.tpu as pltpu

bf16, f32, u32 = jnp.bfloat16, jnp.float32, jnp.uint32

S, D, H, E, M, SEG, F = 2048, 1024, 32, 128, 8, 32, 3584
NSEG = S // SEG
NP = H // 2
TC = SEG - M
HG = 8
NG = H // HG
TB = 128
NB = S // TB
NFG = F // (4 * E)
NOG = D // (4 * E)
NI = NSEG // 2
NQ = D // E // 2
NC = 3 * NG
BGR = 384
G1R = 48
HD = D // 2
X0 = 4
NR = 2 * (M + SEG)
NO_BOUNDS = True
ZPAD = 2
PIN_ROWS = 256
Y_AT = 4
S_AT = (26, 44)
G_AT = 62
HEAD = 14
PREP_AT = (0, 1, 4, 5)
PREP_CH = 2
O3 = (1, 0)
O4 = (0, 0)
O2 = (0, 0)
T_AT = (7, 28, 52)
U_AT = (6, 3, 16)
FREE_JOBS = 0
SH_AT = None
E_AT = (10, 24, 34)
FINE = 1
JGROUP = 1
P1_TAIL = 5
P1_LAG = 4
SCHED_A = (2, 1, 3)
SCHED_B = (3, 1, 3)
EPS = 1e-5
SCALE = E ** -0.5
_SCOPES = False
_N2 = NSEG // 2


def _scoped(name, fn):
    def wrapped(*a):
        if not _SCOPES:
            return fn(*a)
        with jax.named_scope(name):
            return fn(*a)
    return wrapped


def _pk(x):
    return pltpu.bitcast(x.astype(bf16), u32)


def _up(x):
    return pltpu.bitcast(x, bf16)


def _ct(k):
    return slice(k * E, (k + 1) * E)


def _dot(a, b):
    return jnp.dot(a, b, preferred_element_type=f32)


def _ln(x):
    m = jnp.mean(x, axis=-1, keepdims=True)
    xc = x - m
    v = jnp.mean(xc * xc, axis=-1, keepdims=True)
    return xc * lax.rsqrt(v + EPS)


def _gelu(x):
    c = 0.7978845608028654
    return 0.5 * x * (1.0 + jnp.tanh(c * (x + 0.044715 * (x * x * x))))


def _lhs_set(a11, a12, a21, a22):
    return (a11 + a22, a21 + a22, a11, a22, a11 + a12, a21 - a11, a12 - a22)


def _rhs_set(b11, b12, b21, b22):
    return (b11 + b22, b11, b12 - b22, b21 - b11, b22, b11 + b12, b21 + b22)


_LHS_TERMS = (((0, 1), (3, 1)), ((2, 1), (3, 1)), ((0, 1),), ((3, 1),),
              ((0, 1), (1, 1)), ((2, 1), (0, -1)), ((1, 1), (3, -1)))
_RHS_TERMS = (((0, 1), (3, 1)), ((0, 1),), ((1, 1), (3, -1)), ((2, 1), (0, -1)),
              ((3, 1),), ((0, 1), (1, 1)), ((2, 1), (3, 1)))


def _outer_operand(tile, terms):
    out = []
    for i in range(2):
        for j in range(2):
            v = None
            for o, sign in terms:
                t = tile(2 * (o // 2) + i, 2 * (o % 2) + j)
                v = t if v is None else (v + t if sign > 0 else v - t)
            out.append(v)
    return out


class _Quad:
    def __init__(self, tiles):
        self.t = tuple(tiles)

    def __add__(self, other):
        return _Quad([a + b for a, b in zip(self.t, other.t)])

    def __sub__(self, other):
        return _Quad([a - b for a, b in zip(self.t, other.t)])


def _strassen2(m, oo=0, oi=0):
    cs = _strassen(lambda n1: _Quad(_strassen(lambda n2: m(7 * n1 + n2), oi)), oo)
    return lambda i, j: cs[2 * (i // 2) + j // 2].t[2 * (i % 2) + j % 2]


def _strassen(m, order=0):
    if order == 0:
        m1 = m(0)
        m2 = m(1)
        c22 = m1 - m2
        m3 = m(2)
        c22 = c22 + m3
        c22 = m(5) + c22
        m4 = m(3)
        c21 = m2 + m4
        c11 = m1 + m4
        m5 = m(4)
        c12 = m3 + m5
        c11 = c11 - m5
        c11 = m(6) + c11
    else:
        m2 = m(1)
        c22 = m(5) - m2
        m4 = m(3)
        c21 = m2 + m4
        m1 = m(0)
        c22 = c22 + m1
        c11 = m4 + m1
        m3 = m(2)
        c22 = c22 + m3
        m5 = m(4)
        c12 = m3 + m5
        c11 = c11 - m5
        c11 = m(6) + c11
    return c11, c12, c21, c22


def _mask_fill():
    shape = (NR, E)
    r = lax.broadcasted_iota(jnp.int32, shape, 0)
    c = lax.broadcasted_iota(jnp.int32, shape, 1)

    def headpos(i):
        head = jnp.where(i < 64, i >> 5, (i - 64) >> 3)
        pos = jnp.where(i < 64, i & 31, 32 + (i & 7))
        return head, pos

    hr, pr = headpos(r)
    hc, pc = headpos(c)
    same = hr == hc
    valid = same & ((pr < M) | (pr >= pc))
    return jnp.where(valid, 0.0, jnp.where(same, -1e9, -jnp.inf)).astype(f32)


def _kernel(x_hbm, mem0_hbm, wq_hbm, wk_hbm, wv_hbm, wo_hbm, w1_hbm, w2_hbm, w3_hbm,
            w4_hbm, c_hbm, wm_hbm,
            out_hbm,
            x_s, w_s, wo_s, t1_s, g2, g3, g4, pre_s, mod_s, mem_s, hn_s, aout_s, fill_s,
            hb_s, t_s, l1_s, zero_s, c_s, mem0_s, sems):
    w_hbm = (wq_hbm, wk_hbm, wv_hbm)

    (SEM_C, SEM_MEM, SEM_XPRE, SEM_X, SEM_STG, SEM_BG, SEM_OUT,
     SEM_WMR, SEM_G2, SEM_G3, SEM_G4, SEM_WM, SEM_G1) = (0, 1, 2, 3, 4, 6, 8, 10, 12, 14, 16, 18, 22)

    def copy(src, dst, k):
        return pltpu.make_async_copy(src, dst, sems.at[k])

    def aligned(x, n):
        return x if isinstance(x, int) else pl.multiple_of(x, n)

    def clamp(k, hi):
        return min(k, hi) if isinstance(k, int) else jnp.minimum(k, hi)

    def mlp_piece(k):
        k = clamp(k, 4 * NFG - 1)
        return k >> 2, k & 3

    def mlp_w_copies(k, slot):
        g, rr = mlp_piece(k)
        k2 = clamp(k, NI - 1)
        return (copy(w2_hbm.at[:, pl.ds(aligned((k2 >> 1) * 16, 16), 16),
                               pl.ds(aligned((k2 & 1) * 4 * E, E), 4 * E)], g2.at[slot], SEM_G2 + slot),
                copy(w3_hbm.at[:, pl.ds(aligned(rr * 64, 64), 64), pl.ds(aligned(g * 4 * E, E), 4 * E)],
                     g3.at[slot], SEM_G3 + slot),
                copy(w4_hbm.at[g, :, pl.ds(aligned(rr * 32, 32), 32), :], g4.at[slot], SEM_G4 + slot))

    def pinned(w, job):
        if job is None:
            return w()
        z = job() & zero_s[0:8, :]
        w = w()
        return jnp.concatenate([w[0:8] | z, w[8:]], axis=0)

    def after(x, anchor):
        if anchor is None:
            return x
        z = pltpu.bitcast(pltpu.bitcast(anchor[0:8], u32) & zero_s[0:8, :], f32)
        z = jnp.concatenate([z] * (x.shape[0] // 8), axis=0)
        return jnp.concatenate([x[:, 0:E] + z, x[:, E:]], axis=1) if x.shape[1] > E else x + z

    def rhs_job(src, slot, r0, c1, c2, dst, q, row, z=None):
        blk = [src[slot, kh, r0:r0 + 16, cc * E:(cc + 1) * E].astype(f32)
               for kh in range(2) for cc in (c1, c2)]
        if z is not None:
            zf = pltpu.bitcast(jnp.concatenate([z, z], axis=0), f32)
            blk[0] = blk[0] + zf
            blk[3] = blk[3] + zf
        sets = _rhs_set(*blk)
        for n, v in enumerate(sets):
            dst.at[n][pl.ds(pl.multiple_of(row, 8), 8), _ct(q)] = _pk(v)
        out = pltpu.bitcast(sets[2], u32) | pltpu.bitcast(sets[3], u32)
        return out[0:8] | out[8:16]

    def rhs2_job(src, slot, r0, c0, n1, dst, row):
        blk = _outer_operand(lambda i, j: src[slot, i, r0:r0 + 16, _ct(c0 + j)].astype(f32),
                             _RHS_TERMS[n1])
        sets = _rhs_set(*blk)
        for n2, v in enumerate(sets):
            dst[pl.ds(pl.multiple_of(row, 8), 8), _ct(7 * n1 + n2)] = _pk(v)
        out = pltpu.bitcast(sets[2], u32) | pltpu.bitcast(sets[3], u32)
        return out[0:8] | out[8:16]

    def silu_c():
        cf = c_s[...].astype(f32)
        return jnp.broadcast_to(cf * (1.0 / (1.0 + jnp.exp(-cf))), (8, D)).astype(bf16)

    def wm_copy(wm_s, src_tile, dst_tile, sem):
        return copy(wm_hbm.at[:, pl.ds(aligned(src_tile * E, E), E)], wm_s.at[dst_tile], sem)

    def wm_wait(wm_s, t0, n, sem):
        copy(wm_s.at[t0:t0 + n], wm_s.at[t0:t0 + n], sem).wait()

    def mod_tiles(wm_s, t0, n, dst_tile):
        sc8 = silu_c()
        for k in range(n):
            v = _dot(sc8, wm_s[t0 + k])
            if (dst_tile + k) // (D // E) in (1, 4):
                v = 1.0 + v
            mod_s[:, _ct(dst_tile + k)] = v

    def x_copy(k):
        r = slice(0, X0) if k == 0 else slice(X0, NSEG)
        return copy(x_hbm.at[r], x_s.at[r], SEM_XPRE if k == 0 else SEM_X)

    def h_rows(s):
        return _ln(x_s[s, 0:TC, :].astype(f32)) * mod_rows(1, TC) + mod_rows(0, TC)

    def mod_rows(k, n, c0=0, w=D):
        return jnp.concatenate([mod_s[:, k * D + c0:k * D + c0 + w]] * (n // 8), axis=0)

    def phase_a(xpre_s, hpre_s, wm_s, stg, bg, g1, tq_s):
        def tq_place(c, n):
            if n == 1:
                return w_s.at[c], 0, None
            if n == 4:
                return w_s.at[c], D // 4, None
            return tq_s.at[c], 0, (0, 2, 3, 5, 6).index(n) * (HG // 2)

        def w_copy(t, g, slot):
            return copy(w_hbm[t].at[:, pl.ds(pl.multiple_of(g * HG, HG), HG), :], stg.at[slot],
                        SEM_STG + slot)

        def bg_rows(k):
            return clamp(k * BGR, H * E - BGR), clamp(k * G1R, HD - G1R)

        def bg_copies(k, slot):
            ro, r1 = bg_rows(k)
            return (copy(wo_hbm.at[pl.ds(aligned(ro, 16), BGR)], bg.at[slot], SEM_BG + slot),
                    copy(w1_hbm.at[:, pl.ds(aligned(r1, 16), G1R), :], g1.at[slot], SEM_G1 + slot))

        def relayout_jobs(slot, c, i):
            memo = []
            r = aligned(i * 8, 8)

            def job(j, z=None):
                if not memo:
                    for d0 in (i * 16, HD + i * 16):
                        memo.append(jnp.swapaxes(pltpu.bitcast(stg[slot, pl.ds(d0, 16)], u32), 0, 1))
                blk = []
                for kh in range(2):
                    u = memo[kh][j]
                    if z is not None:
                        u = u | jnp.concatenate([z, z], axis=0)
                    blk.append(pltpu.bitcast(u << 16, f32))
                    blk.append(pltpu.bitcast(u & jnp.uint32(0xFFFF0000), f32))
                for k, v in enumerate(blk):
                    w_s.at[c][pl.ds((k // 2) * (D // 4) + r, 8), _ct(2 * j + k % 2)] = _pk(v)
                for n, v in enumerate(_rhs_set(*blk)):
                    if n not in (1, 4):
                        ref, r0, c0 = tq_place(c, n)
                        ref[pl.ds(r0 + r, 8), _ct(c0 + j)] = _pk(v)

            return [functools.partial(job, j) for j in range(HG // 2)]

        def repack(slot, row, i, z):
            v = pltpu.bitcast(bg[slot, 16 * i:16 * i + 16, :], u32)
            v = v | jnp.concatenate([z] * (D // E), axis=1)
            wo_s[pl.ds(pl.multiple_of(row + 8 * i, 8), 8), :] = v

        cp_c = copy(c_hbm, c_s, SEM_C)
        cp_mem = copy(mem0_hbm, mem0_s, SEM_MEM)
        cp_xpre = copy(x_hbm.at[:, TC:SEG, :], xpre_s, SEM_XPRE)
        w_copy(0, 0, 0).start()
        cp_xpre.start()
        cp_c.start()
        cp_mem.start()
        for k in range(2 * D // E):
            wm_copy(wm_s, k, k, SEM_WM + k // 4).start()
        w_copy(0, 1, 1).start()

        zero_s[0:8, :] = jnp.zeros((8, E), u32)
        fill_s[0:NR, :] = _mask_fill()
        aout_s[...] = jnp.zeros(aout_s.shape, f32)
        l1_s[...] = jnp.zeros(l1_s.shape, u32)
        bg[1] = jnp.zeros(bg.shape[1:], bf16)
        g1[1] = jnp.zeros(g1.shape[1:], bf16)

        w_copy(0, 0, 0).wait()

        def rl0_body(i, carry):
            for job in relayout_jobs(0, 0, i):
                job()
            return carry

        lax.fori_loop(0, D // 32, rl0_body, 0)
        w_copy(0, 2, 0).start()
        for cp in bg_copies(0, 0):
            cp.start()

        cp_xpre.wait()

        def npre_body(i, carry):
            xr = xpre_s[pl.ds(pl.multiple_of(i * 8, 8), 8)].astype(f32).reshape(64, D)
            t_s[pl.ds(pl.multiple_of(i * 64, 64), 64), :] = _ln(xr)
            return carry

        lax.fori_loop(0, NSEG // 8, _scoped("npre", npre_body), 0)

        cp_c.wait()
        cp_mem.wait()
        mem_s[...] = mem0_s[...].astype(f32)

        for k in range(4):
            wm_wait(wm_s, 4 * k, 4, SEM_WM + k)
            mod_tiles(wm_s, 4 * k, 4, 4 * k)

        PH = NSEG * M // 2

        def hpre_body(i, carry):
            h = [t_s[pl.ds(pl.multiple_of(hf * PH + i * 16, 16), 16), :] * mod_rows(1, 16) + mod_rows(0, 16)
                 for hf in range(2)]
            for n, v in enumerate(_lhs_set(h[0][:, :HD], h[0][:, HD:], h[1][:, :HD], h[1][:, HD:])):
                hpre_s.at[n][pl.ds(pl.multiple_of(i * 8, 8), 8), :] = _pk(v)
            return carry

        lax.fori_loop(0, PH // 16, _scoped("hpre", hpre_body), 0)

        t_s[0:8, :] = jnp.zeros((8, D), f32)
        t_s[S + 8:S + 16, :] = jnp.zeros((8, D), f32)

        MB = 64

        def p1_body(c, carry):
            slot = c & 1
            pslot = 1 - slot
            ro, r1 = bg_rows(jnp.maximum(c - 1, 0))

            @pl.when(c >= 1)
            def _():
                for cp in bg_copies(0, pslot):
                    cp.wait()

            @pl.when(c + 1 < NC)
            def _():
                w_copy(0, 0, pslot).wait()

            small = [functools.partial(repack, pslot, ro >> 1, i) for i in range(BGR // 16)]
            small += [functools.partial(rhs_job, g1, pslot, 16 * rt, q, NQ + q, t1_s, q, (r1 >> 1) + 8 * rt)
                      for rt in range(G1R // 16) for q in range(NQ)]
            work = []
            nu = D // 32
            for i in range(nu):
                js = relayout_jobs(pslot, c + 1, i)
                work += [js[k:k + JGROUP] for k in range(0, len(js), JGROUP)]
                work += [[job] for job in small[i * len(small) // nu:(i + 1) * len(small) // nu]]
            npin = 7 * (HG // 2) * (PH // MB)
            jobs = [[] for _ in range(npin)]
            for k, group in enumerate(work):
                pos = k * (npin - P1_TAIL) * 8 // len(work)
                jobs[pos // 8] += [(job, pos % 8 if FINE else 0) for job in group]
            jobs = iter(jobs)

            def prod(n, q, mb):
                ref, r0, c0 = tq_place(c, n)
                w = ref[r0:r0 + D // 4, _ct(2 * q + (n == 4) if c0 is None else c0 + q)]
                m = _dot(_up(hpre_s[n, mb * MB // 2:(mb + 1) * MB // 2, :]), _up(w))
                pending.append(m)
                if len(pending) > P1_LAG:
                    anchor = pltpu.bitcast(pending.pop(0), u32)
                    for job, g in next(jobs):
                        job(anchor[8 * g:8 * g + 8] & zero_s[0:8, :])
                return m

            pending = []
            ns = MB // M
            for q in range(HG // 2):
                for mb in range(PH // MB):
                    cs = _strassen(lambda n: prod(n, q, mb))
                    for hf in range(2):
                        y = jnp.concatenate([cs[2 * hf + k][sg * M:(sg + 1) * M]
                                             for sg in range(ns) for k in range(2)], axis=0)
                        s0 = hf * (NSEG // 2) + mb * ns
                        pre_s.at[c][s0 * M:(s0 + ns) * M, _ct(q)] = _pk(y)

            for t in range(3):
                @pl.when((c + 3) >> 2 == t)
                def _():
                    w_copy(t, (c + 3) & 3, pslot).start()

            @pl.when(c + 2 < NC)
            def _():
                for cp in bg_copies(c + 1, pslot):
                    cp.start()

            @pl.when(c < NC - 3)
            def _():
                wm_copy(wm_s, 2 * D // E + c, c, SEM_WMR).start()

            @pl.when(c == NC - 3)
            def _():
                def issue(k, carry2):
                    wm_copy(wm_s, 2 * D // E + k, k, SEM_WMR).start()
                    return carry2

                x_copy(0).start()
                for k in range(2):
                    for cp in mlp_w_copies(k, k):
                        cp.start()
                lax.fori_loop(NC - 3, 3 * D // E, issue, 0)

            return carry

        lax.fori_loop(0, NC, _scoped("p1", p1_body), 0)
        x_copy(1).start()
        x_copy(0).wait()
        wm_wait(wm_s, 0, 3 * D // E, SEM_WMR)
        mod_tiles(wm_s, 0, 3 * D // E, 2 * D // E)
        hn_s[...] = h_rows(0)

    def phase_b(t2_s, t3_s, t4_s, wg_s, x1_s, base_s, yn_s, gs_s, act_s, o_s):
        for k in range(D // E):
            wm_copy(wg_s, 5 * D // E + k, k, SEM_WM).start()

        def chain_step(s, mem, htok, odef_prev, jobs=(), hooks=None):
            hs = jnp.concatenate([mem, htok], axis=0).astype(bf16)
            qkv = [[None] * 3 for _ in range(NP)]
            ps = [None] * NP
            os_ = [None] * H
            odef = [None] * H

            def proj(p, ts=(0, 1, 2)):
                for t in ts:
                    c, q = t * NG + p // (HG // 2), p % (HG // 2)
                    a = _dot(hs, _up(w_s[c, :, _ct(2 * q)]))
                    b = _dot(hs, _up(w_s[c, :, _ct(2 * q + 1)]))
                    if hooks and t == 2 and p - NP in hooks:
                        hooks[p - NP](b)
                    pre = pre_s[c, pl.ds(pl.multiple_of(s * M, M), M), _ct(q)]
                    if t == 1:
                        kf = jnp.concatenate([a, b, _up(pre).astype(f32), jnp.zeros((E - NR, E), f32)],
                                             axis=0)
                        qkv[p][t] = kf.T.astype(bf16)
                        continue
                    parts = [_pk(a), _pk(b), pre]
                    if t == 2:
                        parts.append(jnp.zeros(((E - NR) // 2, E), u32))
                    qkv[p][t] = _up(jnp.concatenate(parts, axis=0))

            def scores(p):
                sc_ = _dot(qkv[p][0], qkv[p][1])
                fill = fill_s[0:NR, :]
                sc_ = jnp.where(fill == 0.0, sc_ * SCALE, fill)
                m = jnp.max(sc_, axis=-1, keepdims=True)
                e = jnp.exp(sc_ - m)
                l = jnp.sum(e, axis=-1, keepdims=True)
                r = pl.reciprocal(l, approx=True)
                r = r * (2.0 - l * r)
                ps[p] = (e * r).astype(bf16)

            def fin(p):
                o = _dot(ps[p], qkv[p][2])
                for hh in range(2):
                    h = 2 * p + hh
                    rows = o[32 * hh:32 * hh + 32]
                    odef[h] = o[64 + 8 * hh:72 + 8 * hh]
                    if odef_prev is not None:
                        rows = jnp.concatenate([rows, odef_prev[h], odef[h]], axis=0)
                    os_[h] = _pk(rows)

            acc = [None] * 8
            jobs = iter(jobs)

            def wo(h0, h1, js):
                lhs = _up(jnp.concatenate(os_[h0:h1], axis=1))
                for j in js:
                    ws = []
                    for r0 in range(h0 * E // 2, h1 * E // 2, PIN_ROWS):
                        ws.append(pinned(lambda: wo_s[r0:r0 + PIN_ROWS, j * E:(j + 1) * E],
                                         next(jobs, None)))
                    part = _dot(lhs, _up(jnp.concatenate(ws, axis=0)))
                    if hooks and acc[j] is None and j in hooks:
                        hooks[j](part)
                    acc[j] = part if acc[j] is None else part + acc[j]

            ORDER, LAG_S, LAG_O = SCHED_A if odef_prev is None else SCHED_B
            for p in range(NP):
                if ORDER == 0:
                    proj(p)
                    if p >= LAG_S:
                        scores(p - LAG_S)
                    if p >= LAG_O:
                        fin(p - LAG_O)
                elif ORDER == 1:
                    proj(p, (1, 0))
                    if p >= LAG_O:
                        fin(p - LAG_O)
                    proj(p, (2,))
                    if p >= LAG_S:
                        scores(p - LAG_S)
                elif ORDER == 2:
                    proj(p, (1,))
                    if p >= LAG_S:
                        scores(p - LAG_S)
                    proj(p, (0,))
                    if p >= LAG_O:
                        fin(p - LAG_O)
                    proj(p, (2,))
                elif ORDER == 3:
                    proj(p, (1,))
                    if p >= LAG_O:
                        fin(p - LAG_O)
                    proj(p, (0,))
                    if p >= LAG_S:
                        scores(p - LAG_S)
                    proj(p, (2,))
                elif ORDER == 4:
                    proj(p, (1,))
                    if p >= LAG_S:
                        scores(p - LAG_S)
                    proj(p, (0, 2))
                    if p >= LAG_O:
                        fin(p - LAG_O)
                else:
                    proj(p, (0,))
                    if p >= LAG_S:
                        scores(p - LAG_S)
                    proj(p, (1,))
                    if p >= LAG_O:
                        fin(p - LAG_O)
                    proj(p, (2,))
            tail = []
            for k in range(LAG_O):
                step = []
                if NP - LAG_S + k < NP:
                    step.append(functools.partial(scores, NP - LAG_S + k))
                step.append(functools.partial(fin, NP - LAG_O + k))
                tail.append(step)
            hsplit = min(24, 2 * (NP - LAG_O))
            cuts = {3: (2, 3, 5), 2: (2, 5), 4: (1, 2, 4, 6), 5: (1, 2, 3, 4, 6)}[LAG_O]
            j0 = 0
            for k, step in enumerate(tail):
                wo(0, hsplit, range(j0, cuts[k]))
                j0 = cuts[k]
                for f in step:
                    f()
            wo(0, hsplit, range(j0, 8))
            wo(hsplit, H, range(8))
            return jnp.concatenate(acc, axis=1), odef

        def mixer_prep(i, r0, n, anchor=None):
            r = pl.ds(aligned(i * 64 + r0, 16), n)
            xr = x_s[2 * i + r0 // SEG, r0 % SEG:r0 % SEG + n, :].astype(f32)
            x2 = xr + mod_rows(2, n) * after(aout_s[r0:r0 + n, :], anchor)
            x_s.at[2 * i + r0 // SEG][r0 % SEG:r0 % SEG + n, :] = x2.astype(bf16)
            hb = _ln(x2) * mod_rows(4, n) + mod_rows(3, n)
            hb_s[r, :] = hb.astype(bf16)
            return _ln(hb)

        def mixer_sets(ya, yb, r0, dst=l1_s):
            n = ya.shape[0]
            for m, v in enumerate(_lhs_set(ya[:, :HD], ya[:, HD:], yb[:, :HD], yb[:, HD:])):
                dst[m * (SEG // 2) + r0 // 2:m * (SEG // 2) + (r0 + n) // 2, 0:HD] = _pk(v)

        def mixer_mm(i, src=l1_s, hook=None):
            for q in range(NQ):
                def prod(n):
                    m = _dot(_up(src[n * (SEG // 2):(n + 1) * (SEG // 2), 0:HD]),
                             _up(t1_s[n, :, _ct(q)]))
                    if hook is not None:
                        hook(m)
                    return m

                cs = _strassen(prod)
                for k, cc in enumerate(cs):
                    r0 = aligned(i * 64 + 8 + (k // 2) * SEG, 8)
                    t_s[pl.ds(r0, SEG), _ct(q + NQ * (k % 2))] = _gelu(cc)

        def p2_body(i, carry):
            slot = i & 1
            for cp in mlp_w_copies(0, slot):
                cp.wait()

            @pl.when(i == 1)
            def _():
                x_copy(1).wait()

            g, rr = mlp_piece(i)
            work = [functools.partial(rhs2_job, g2, slot, 0, 0, n1, t2_s.at[slot], (i >> 1) * 8)
                    for n1 in range(7)]
            work += [functools.partial(rhs2_job, g3, slot, 16 * rt, 0, n1, t3_s.at[g], rr * 32 + 8 * rt)
                     for rt in range(4) for n1 in range(7)]
            work += [functools.partial(rhs2_job, g4, slot, 16 * rt, 4 * og, n1, t4_s.at[og],
                                       g * (E // 2) + rr * 16 + 8 * rt)
                     for rt in range(2) for og in range(NOG) for n1 in range(7)]
            npin = len(work) - FREE_JOBS
            jobs = [None] * 64
            for k in range(npin):
                jobs[1 + k * 63 // npin] = work[k]

            sa_ = 2 * i
            sb_ = 2 * i + 1
            hb_tok = h_rows(sb_)
            oa, odef_a = chain_step(sa_, mem_s[...], hn_s[...], None)
            mixer_mm(jnp.maximum(i - 2, 0))
            ys = []

            def hook(k, anchor):
                if k >= PREP_CH:
                    anchor = anchor[0:8] + ys[-PREP_CH][0:8, 0:E] + ys[-PREP_CH][8:16, 0:E]
                ys.append(mixer_prep(jnp.maximum(i - 1, 0), (k % 2) * SEG + (k // 2) * 16, 16, anchor))
                if k % 2:
                    mixer_sets(ys[-2], ys[-1], (k // 2) * 16)

            hooks = {j: functools.partial(hook, k) for k, j in enumerate(PREP_AT)}
            ob, _ = chain_step(sb_, oa[0:M], hb_tok, odef_a, jobs, hooks)
            for job in work[npin:]:
                job()
            mem_s[...] = ob[0:M]
            aout_s[0:TC, :] = oa[M:SEG]
            aout_s[TC:SEG, :] = ob[SEG:SEG + M]
            aout_s[SEG:SEG + TC, :] = ob[M:SEG]
            aout_s[SEG + TC:2 * SEG, :] = ob[SEG + M:SEG + 2 * M]
            hn_s[...] = h_rows(jnp.minimum(sb_ + 1, NSEG - 1))
            for cp in mlp_w_copies(i + 2, slot):
                cp.start()
            return carry

        lax.fori_loop(0, _N2, _scoped("p2", p2_body), 0)

        TQ = TB // 4
        SHIFT = (-1, -1, 1, 1, -2, -2, 2, 2)

        def u_set(n):
            return w_s.at[n // 32], slice((n % 32) * (TQ // 2), (n % 32 + 1) * (TQ // 2))

        def d_set(slot, n):
            return w_s.at[slot], (n // 4) * (TQ // 2), (n % 4) * 2

        def d_lhs(slot, n):
            ref, r0, c0 = d_set(slot, n)
            return _up(ref[r0:r0 + TQ // 2, c0 * E:(c0 + 2) * E])

        def shift_job(j, r0, n, anchor=None):
            for ct in range(D // E):
                win = t_s[pl.ds(aligned(j * TB + r0, 16), n + 16), _ct(ct)]
                gs_s[r0:r0 + n, _ct(ct)] = after(
                    pltpu.roll(win, (-SHIFT[ct]) % (n + 16), 0)[8:8 + n], anchor)

        def mix(j, hook=None):
            r0 = aligned(j * TB, TB)
            for og in range(NOG):
                def prod(n):
                    m = _dot(d_lhs(3, n), _up(t2_s[og, :, _ct(n)]))
                    if hook is not None:
                        hook(m)
                    return m

                c = _strassen2(prod, *O2)
                for i in range(4):
                    for k in range(2):
                        cols = slice((4 * og + 2 * k) * E, (4 * og + 2 * k + 2) * E)
                        x1_s[i * TQ:(i + 1) * TQ, cols] = (
                            hb_s[pl.ds(r0 + i * TQ, TQ), cols].astype(f32)
                            + jnp.concatenate([c(i, 2 * k), c(i, 2 * k + 1)], axis=1))

        def base_job(j, rt, anchor):
            rows = slice(rt * 16, (rt + 1) * 16)
            z = pltpu.bitcast(pltpu.bitcast(anchor[0:8], u32) & zero_s[0:8, :], f32)
            gb = mod_rows(5, 8) + jnp.concatenate([z] * (D // E), axis=1)
            x2 = x_s[j * (TB // SEG) + rt // 2, (rt % 2) * 16:(rt % 2) * 16 + 16, :]
            base_s[rows, :] = x2.astype(f32) + jnp.concatenate([gb, gb], axis=0) * x1_s[rows, :]

        def out_copy(j, slot):
            return copy(o_s.at[slot], out_hbm.at[pl.ds(aligned(j * TB, TB), TB)], SEM_OUT + slot)

        def ln_job(r0, n, prev, anchor=None):
            if anchor is not None and len(prev) >= 2:
                anchor = anchor[0:8] + prev[-2]
            y = _ln(after(x1_s[r0:r0 + n, :], anchor))
            yn_s[r0:r0 + n, :] = y
            prev.append(y[0:8, 0:E] + y[8:16, 0:E])

        def set_job(src, slot, rt, ct, n1, n=16, anchor=None):
            blk = _outer_operand(lambda i, k: src[i * TQ + rt * n:i * TQ + (rt + 1) * n, _ct(2 * k + ct)],
                                 _LHS_TERMS[n1])
            blk[0] = after(blk[0], anchor)
            blk[3] = after(blk[3], anchor)
            for n2, v in enumerate(_lhs_set(*blk)):
                ref, r0, c0 = d_set(slot, 7 * n1 + n2)
                ref[r0 + rt * n // 2:r0 + (rt + 1) * n // 2, _ct(c0 + ct)] = _pk(v)

        def all_sets(src, slot):
            for n1 in range(7):
                for ct in range(2):
                    set_job(src, slot, 0, ct, n1, TQ)

        wm_wait(wg_s, 0, D // E, SEM_WM)
        mod_tiles(wg_s, 0, D // E, 5 * D // E)
        shift_job(0, 0, TB)
        all_sets(gs_s, 3)
        mix(0)
        prev0 = []
        plan = {}
        for k in range(TB // 16):
            plan[T_AT[0] * (k // 2) + k % 2] = [
                functools.partial(ln_job, (k % 4) * TQ + (k // 4) * 16, 16, prev0)]
        rest = [functools.partial(shift_job, 1, (k % 4) * TQ + (k // 4) * 16, 16)
                for k in range(TB // 16)]
        rest += [functools.partial(set_job, gs_s, 3, rt, ct, n1, 16)
                 for rt in range(2) for ct in range(2) for n1 in range(7)]
        for k, job in enumerate(rest):
            plan.setdefault(k * T_AT[1] // len(rest), []).append(job)
        rest = [functools.partial(set_job, yn_s, 2, rt, ct, n1, 16)
                for rt in range(2) for ct in range(2) for n1 in range(7)]
        for k, job in enumerate(rest):
            plan.setdefault(T_AT[1] + k * (T_AT[2] - T_AT[1]) // len(rest), []).append(job)
        tick0 = [0]

        def hook0(m):
            for job in plan.pop(tick0[0], ()):
                job(anchor=m)
            tick0[0] += 1

        mixer_mm(NI - 2, hook=hook0)
        mixer_sets(mixer_prep(NI - 1, 0, SEG), mixer_prep(NI - 1, SEG, SEG), 0, w_s.at[4])
        mixer_mm(NI - 1, w_s.at[4], hook0)
        assert not plan

        def mlp_block(j, last):
            slot = j & 1

            jn = clamp(j + 2, NB - 1)
            early = [functools.partial(base_job, j, k) for k in range(TB // 16)]
            shifts = [functools.partial(shift_job, jn, (k % 4) * TQ + (k // 4) * 16, 16)
                      for k in range(TB // 16)]
            if not last and SH_AT is None:
                early += shifts
            early = iter(early)

            pend = []
            tick = [0]

            def drain(m):
                tick[0] += 1
                if pend and tick[0] >= U_AT[0] and (tick[0] - U_AT[0]) % U_AT[1] == 0:
                    pend.pop(0)(m)

            def up_prod(n, g):
                m = _dot(d_lhs(2, n), _up(t3_s[g, :, _ct(n)]))
                if n in E_AT:
                    job = next(early, None)
                    if job is not None:
                        job(anchor=m)
                drain(m)
                return m

            def uset_job(tile, g, n1, r0, n, anchor=None):
                blk = _outer_operand(lambda i, k: tile(i, k, r0, n), _LHS_TERMS[n1])
                blk[0] = after(blk[0], anchor)
                blk[3] = after(blk[3], anchor)
                for n2, v in enumerate(_lhs_set(*blk)):
                    ref, rows = u_set(7 * n1 + n2)
                    ref[rows.start + r0 // 2:rows.start + (r0 + n) // 2, _ct(g)] = _pk(v)

            for g in range(NFG):
                c = _strassen2(lambda n: up_prod(n, g), *O3)
                assert not pend
                tick[0] = 0
                if U_AT[1] == 0 or (last and g == NFG - 1):
                    act = [[_gelu(c(i, k)) for k in range(4)] for i in range(4)]
                    for n1 in range(7):
                        uset_job(lambda i, k, r0, n: act[i][k], g, n1, 0, TQ)
                    continue
                c0 = 4 * (g % 2)
                for i in range(4):
                    for k in range(4):
                        act_s[i * TQ:(i + 1) * TQ, _ct(c0 + k)] = _gelu(c(i, k))

                def tile(i, k, r0, n, c0=c0):
                    return act_s[i * TQ + r0:i * TQ + r0 + n, _ct(c0 + k)]

                pend += [functools.partial(uset_job, tile, g, n1, r0, U_AT[2])
                         for n1 in range(7) for r0 in range(0, TQ, U_AT[2])]
            jobs = {}
            if not last:
                mix(j + 1, drain)
                assert not pend
                prev = []
                for k in range(TB // 16):
                    jobs[k * Y_AT] = functools.partial(ln_job, (k % 4) * TQ + (k // 4) * 16, 16, prev)

                def place(start, fns, step=1):
                    for fn in fns:
                        while start in jobs:
                            start += 1
                        jobs[start] = fn
                        start += step

                if SH_AT is not None:
                    place(SH_AT[0], shifts, SH_AT[1])
                for rt in range(2):
                    place(S_AT[rt], [functools.partial(set_job, yn_s, 2, rt, ct, n1, 16)
                                     for ct in range(2) for n1 in range(7)])
                place(G_AT, [functools.partial(set_job, gs_s, 3, rt, ct, n1, 16)
                             for rt in range(2) for ct in range(2) for n1 in range(7)])

            def down_part(n, og, k0, k1):
                ref, rows = u_set(n)
                return _dot(_up(ref[rows, k0 * E:k1 * E]),
                            _up(t4_s[og, k0 * E // 2:k1 * E // 2, _ct(n)]))

            head = {}
            if last:
                head = {n: down_part(n, 0, 0, NFG - 1) for n in range(HEAD)}
            count = [0]

            def down_prod(n, og):
                if og == 0 and n in head:
                    return down_part(n, og, NFG - 1, NFG) + head[n]
                m = down_part(n, og, 0, NFG)
                job = jobs.get(count[0])
                count[0] += 1
                if job is not None:
                    job(anchor=m)
                return m

            for og in range(NOG):
                c = _strassen2(lambda n: down_prod(n, og), *(O4 if not last else (0, O4[1])))
                for i in range(4):
                    rows = slice(i * TQ, (i + 1) * TQ)
                    for k in range(2):
                        c0 = (4 * og + 2 * k) * E
                        o_s.at[slot][rows, c0:c0 + 2 * E] = (
                            base_s[rows, c0:c0 + 2 * E] + mod_rows(5, TQ, c0, 2 * E)
                            * jnp.concatenate([c(i, 2 * k), c(i, 2 * k + 1)], axis=1)).astype(bf16)
            out_copy(j, slot).start()

        def p3_body(j, carry):
            @pl.when(j >= 2)
            def _():
                out_copy(j - 2, j & 1).wait()

            mlp_block(j, False)
            return carry

        lax.fori_loop(0, NB - 1, _scoped("p3", p3_body), 0)
        for k in range(2):
            for cp in mlp_w_copies(0, k):
                cp.wait()
        out_copy(NB - 3, (NB - 3) % 2).wait()
        mlp_block(NB - 1, True)
        out_copy(NB - 2, (NB - 2) % 2).wait()
        out_copy(NB - 1, (NB - 1) % 2).wait()

    pl.run_scoped(
        phase_a,
        pltpu.VMEM((NSEG, M, D), bf16),
        pltpu.VMEM((7, NSEG * M // 4, D // 2), u32),
        pltpu.VMEM((3 * D // E, D, E), bf16),
        pltpu.VMEM((2, D, HG, E), bf16),
        pltpu.VMEM((2, BGR, D), bf16),
        pltpu.VMEM((2, 2, G1R, D), bf16),
        pltpu.VMEM((NC + 1, D // 4, 5 * HG // 2 * E), u32),
    )
    pl.run_scoped(
        phase_b,
        pltpu.VMEM((NOG, D // 8, 49 * E), u32),
        pltpu.VMEM((NFG, D // 8, 49 * E), u32),
        pltpu.VMEM((NOG, F // 8, 49 * E), u32),
        pltpu.VMEM((D // E, D, E), bf16),
        pltpu.VMEM((TB, D), f32),
        pltpu.VMEM((TB, D), f32),
        pltpu.VMEM((TB, D), f32),
        pltpu.VMEM((TB, D), f32),
        pltpu.VMEM((TB, D), f32),
        pltpu.VMEM((2, TB, D), bf16),
    )


@jax.jit
def pallas_adaLN_cond__memory_aug_recurrent_mem_tr__mixer_s_mlp__prompt_kernel(
    A_x: jax.Array,
    A_mem0: jax.Array,
    A_Wq: jax.Array,
    A_Wk: jax.Array,
    A_Wv: jax.Array,
    A_Wo: jax.Array,
    A_seg_len,
    B_x: jax.Array,
    B_w1: jax.Array,
    B_w2: jax.Array,
    B_w3: jax.Array,
    B_w4: jax.Array,
    c: jax.Array,
    w_mod: jax.Array,
):
    del A_seg_len, B_x
    assert A_x.shape == (1, S, D) and A_mem0.shape == (1, M, D)
    hbm = pl.BlockSpec(memory_space=pl.ANY)
    scratch = [
        pltpu.VMEM((NSEG, SEG, D), bf16),
        pltpu.VMEM((NC + 1, D // 2, HG * E), u32),
        pltpu.VMEM((H * E // 2, D), u32),
        pltpu.VMEM((7, D // 4, D // 2), u32),
        pltpu.VMEM((2, 4, 16, 4 * E), bf16),
        pltpu.VMEM((2, 4, 64, 4 * E), bf16),
        pltpu.VMEM((2, 4, 32, D), bf16),
        pltpu.VMEM((NC, NSEG * M, HG // 2 * E), u32),
        pltpu.VMEM((8, 6 * D), f32),
        pltpu.VMEM((M, D), f32),
        pltpu.VMEM((TC, D), f32),
        pltpu.VMEM((2 * SEG, D), f32),
        pltpu.VMEM((E, E), f32),
        pltpu.VMEM((S, D), bf16),
        pltpu.VMEM((S + 16, D), f32),
        pltpu.VMEM((7 * SEG // 2, D // 2), u32),
        pltpu.VMEM((8 * ZPAD, E), u32),
        pltpu.VMEM((1, D), bf16),
        pltpu.VMEM((M, D), bf16),
        pltpu.SemaphoreType.DMA((24,)),
    ]
    out = pl.pallas_call(
        _kernel,
        out_shape=jax.ShapeDtypeStruct((S, D), bf16),
        in_specs=[hbm] * 12,
        out_specs=hbm,
        scratch_shapes=scratch,
        compiler_params=pltpu.CompilerParams(vmem_limit_bytes=127 * 1024 * 1024,
                                             disable_bounds_checks=NO_BOUNDS,
                                             disable_semaphore_checks=NO_BOUNDS),
    )(A_x.reshape(NSEG, SEG, D), A_mem0.reshape(M, D), A_Wq, A_Wk, A_Wv,
      A_Wo.reshape(H * E, D), B_w1.reshape(2, D // 2, D), B_w2.reshape(4, D // 4, D), B_w3.reshape(4, D // 4, F),
      B_w4.reshape(NFG, 4, E, D), c, w_mod)
    return out.reshape(1, S, D)
```

```python
import functools

import jax
import jax.numpy as jnp
from jax import lax
import jax.experimental.pallas as pl
import jax.experimental.pallas.tpu as pltpu

bf16, f32, u32 = jnp.bfloat16, jnp.float32, jnp.uint32

S, D, H, E, M, SEG, F = 2048, 1024, 32, 128, 8, 32, 3584
NSEG = S // SEG
NP = H // 2
TC = SEG - M
HG = 8
NG = H // HG
TB = 128
NB = S // TB
NFG = F // (4 * E)
NOG = D // (4 * E)
NI = NSEG // 2
NQ = D // E // 2
NC = 3 * NG
BGR = 384
G1R = 48
HD = D // 2
X0 = 4
NR = 2 * (M + SEG)
NO_BOUNDS = True
ZPAD = 2
PIN_ROWS = 256
Y_AT = 4
S_AT = (26, 44)
G_AT = 62
HEAD = 14
PREP_AT = (0, 1, 4, 5)
PREP_CH = 2
O3 = (1, 0)
O4 = (0, 0)
O2 = (0, 0)
QV32 = 1
OSREF = 0
T_AT = (7, 28, 52)
U_AT = (6, 3, 16)
FREE_JOBS = 0
SH_AT = None
E_AT = (10, 24, 34)
FINE = 1
JGROUP = 1
P1_TAIL = 5
P1_LAG = 4
SCHED_A = (2, 1, 3)
SCHED_B = (3, 1, 3)
EPS = 1e-5
SCALE = E ** -0.5
_SCOPES = False
_N2 = NSEG // 2


def _scoped(name, fn):
    def wrapped(*a):
        if not _SCOPES:
            return fn(*a)
        with jax.named_scope(name):
            return fn(*a)
    return wrapped


def _pk(x):
    return pltpu.bitcast(x.astype(bf16), u32)


def _up(x):
    return pltpu.bitcast(x, bf16)


def _ct(k):
    return slice(k * E, (k + 1) * E)


def _dot(a, b):
    return jnp.dot(a, b, preferred_element_type=f32)


def _ln(x):
    m = jnp.mean(x, axis=-1, keepdims=True)
    xc = x - m
    v = jnp.mean(xc * xc, axis=-1, keepdims=True)
    return xc * lax.rsqrt(v + EPS)


def _gelu(x):
    c = 0.7978845608028654
    return 0.5 * x * (1.0 + jnp.tanh(c * (x + 0.044715 * (x * x * x))))


def _lhs_set(a11, a12, a21, a22):
    return (a11 + a22, a21 + a22, a11, a22, a11 + a12, a21 - a11, a12 - a22)


def _rhs_set(b11, b12, b21, b22):
    return (b11 + b22, b11, b12 - b22, b21 - b11, b22, b11 + b12, b21 + b22)


_LHS_TERMS = (((0, 1), (3, 1)), ((2, 1), (3, 1)), ((0, 1),), ((3, 1),),
              ((0, 1), (1, 1)), ((2, 1), (0, -1)), ((1, 1), (3, -1)))
_RHS_TERMS = (((0, 1), (3, 1)), ((0, 1),), ((1, 1), (3, -1)), ((2, 1), (0, -1)),
              ((3, 1),), ((0, 1), (1, 1)), ((2, 1), (3, 1)))


def _outer_operand(tile, terms):
    out = []
    for i in range(2):
        for j in range(2):
            v = None
            for o, sign in terms:
                t = tile(2 * (o // 2) + i, 2 * (o % 2) + j)
                v = t if v is None else (v + t if sign > 0 else v - t)
            out.append(v)
    return out


class _Quad:
    def __init__(self, tiles):
        self.t = tuple(tiles)

    def __add__(self, other):
        return _Quad([a + b for a, b in zip(self.t, other.t)])

    def __sub__(self, other):
        return _Quad([a - b for a, b in zip(self.t, other.t)])


def _strassen2(m, oo=0, oi=0):
    cs = _strassen(lambda n1: _Quad(_strassen(lambda n2: m(7 * n1 + n2), oi)), oo)
    return lambda i, j: cs[2 * (i // 2) + j // 2].t[2 * (i % 2) + j % 2]


def _strassen(m, order=0):
    if order == 0:
        m1 = m(0)
        m2 = m(1)
        c22 = m1 - m2
        m3 = m(2)
        c22 = c22 + m3
        c22 = m(5) + c22
        m4 = m(3)
        c21 = m2 + m4
        c11 = m1 + m4
        m5 = m(4)
        c12 = m3 + m5
        c11 = c11 - m5
        c11 = m(6) + c11
    else:
        m2 = m(1)
        c22 = m(5) - m2
        m4 = m(3)
        c21 = m2 + m4
        m1 = m(0)
        c22 = c22 + m1
        c11 = m4 + m1
        m3 = m(2)
        c22 = c22 + m3
        m5 = m(4)
        c12 = m3 + m5
        c11 = c11 - m5
        c11 = m(6) + c11
    return c11, c12, c21, c22


def _mask_fill():
    shape = (NR, E)
    r = lax.broadcasted_iota(jnp.int32, shape, 0)
    c = lax.broadcasted_iota(jnp.int32, shape, 1)

    def headpos(i):
        head = jnp.where(i < 64, i >> 5, (i - 64) >> 3)
        pos = jnp.where(i < 64, i & 31, 32 + (i & 7))
        return head, pos

    hr, pr = headpos(r)
    hc, pc = headpos(c)
    same = hr == hc
    valid = same & ((pr < M) | (pr >= pc))
    return jnp.where(valid, 0.0, jnp.where(same, -1e9, -jnp.inf)).astype(f32)


def _kernel(x_hbm, mem0_hbm, wq_hbm, wk_hbm, wv_hbm, wo_hbm, w1_hbm, w2_hbm, w3_hbm,
            w4_hbm, c_hbm, wm_hbm,
            out_hbm,
            x_s, w_s, wo_s, t1_s, g2, g3, g4, pre_s, mod_s, mem_s, hn_s, aout_s, fill_s,
            hb_s, t_s, l1_s, zero_s, c_s, mem0_s, sems):
    w_hbm = (wq_hbm, wk_hbm, wv_hbm)

    (SEM_C, SEM_MEM, SEM_XPRE, SEM_X, SEM_STG, SEM_BG, SEM_OUT,
     SEM_WMR, SEM_G2, SEM_G3, SEM_G4, SEM_WM, SEM_G1) = (0, 1, 2, 3, 4, 6, 8, 10, 12, 14, 16, 18, 22)

    def copy(src, dst, k):
        return pltpu.make_async_copy(src, dst, sems.at[k])

    def aligned(x, n):
        return x if isinstance(x, int) else pl.multiple_of(x, n)

    def clamp(k, hi):
        return min(k, hi) if isinstance(k, int) else jnp.minimum(k, hi)

    def mlp_piece(k):
        k = clamp(k, 4 * NFG - 1)
        return k >> 2, k & 3

    def mlp_w_copies(k, slot):
        g, rr = mlp_piece(k)
        k2 = clamp(k, NI - 1)
        return (copy(w2_hbm.at[:, pl.ds(aligned((k2 >> 1) * 16, 16), 16),
                               pl.ds(aligned((k2 & 1) * 4 * E, E), 4 * E)], g2.at[slot], SEM_G2 + slot),
                copy(w3_hbm.at[:, pl.ds(aligned(rr * 64, 64), 64), pl.ds(aligned(g * 4 * E, E), 4 * E)],
                     g3.at[slot], SEM_G3 + slot),
                copy(w4_hbm.at[g, :, pl.ds(aligned(rr * 32, 32), 32), :], g4.at[slot], SEM_G4 + slot))

    def pinned(w, job):
        if job is None:
            return w()
        z = job() & zero_s[0:8, :]
        w = w()
        return jnp.concatenate([w[0:8] | z, w[8:]], axis=0)

    def after(x, anchor):
        if anchor is None:
            return x
        z = pltpu.bitcast(pltpu.bitcast(anchor[0:8], u32) & zero_s[0:8, :], f32)
        z = jnp.concatenate([z] * (x.shape[0] // 8), axis=0)
        return jnp.concatenate([x[:, 0:E] + z, x[:, E:]], axis=1) if x.shape[1] > E else x + z

    def rhs_job(src, slot, r0, c1, c2, dst, q, row, z=None):
        blk = [src[slot, kh, r0:r0 + 16, cc * E:(cc + 1) * E].astype(f32)
               for kh in range(2) for cc in (c1, c2)]
        if z is not None:
            zf = pltpu.bitcast(jnp.concatenate([z, z], axis=0), f32)
            blk[0] = blk[0] + zf
            blk[3] = blk[3] + zf
        sets = _rhs_set(*blk)
        for n, v in enumerate(sets):
            dst.at[n][pl.ds(pl.multiple_of(row, 8), 8), _ct(q)] = _pk(v)
        out = pltpu.bitcast(sets[2], u32) | pltpu.bitcast(sets[3], u32)
        return out[0:8] | out[8:16]

    def rhs2_job(src, slot, r0, c0, n1, dst, row):
        blk = _outer_operand(lambda i, j: src[slot, i, r0:r0 + 16, _ct(c0 + j)].astype(f32),
                             _RHS_TERMS[n1])
        sets = _rhs_set(*blk)
        for n2, v in enumerate(sets):
            dst[pl.ds(pl.multiple_of(row, 8), 8), _ct(7 * n1 + n2)] = _pk(v)
        out = pltpu.bitcast(sets[2], u32) | pltpu.bitcast(sets[3], u32)
        return out[0:8] | out[8:16]

    def silu_c():
        cf = c_s[...].astype(f32)
        return jnp.broadcast_to(cf * (1.0 / (1.0 + jnp.exp(-cf))), (8, D)).astype(bf16)

    def wm_copy(wm_s, src_tile, dst_tile, sem):
        return copy(wm_hbm.at[:, pl.ds(aligned(src_tile * E, E), E)], wm_s.at[dst_tile], sem)

    def wm_wait(wm_s, t0, n, sem):
        copy(wm_s.at[t0:t0 + n], wm_s.at[t0:t0 + n], sem).wait()

    def mod_tiles(wm_s, t0, n, dst_tile):
        sc8 = silu_c()
        for k in range(n):
            v = _dot(sc8, wm_s[t0 + k])
            if (dst_tile + k) // (D // E) in (1, 4):
                v = 1.0 + v
            mod_s[:, _ct(dst_tile + k)] = v

    def x_copy(k):
        r = slice(0, X0) if k == 0 else slice(X0, NSEG)
        return copy(x_hbm.at[r], x_s.at[r], SEM_XPRE if k == 0 else SEM_X)

    def h_rows(s):
        return _ln(x_s[s, 0:TC, :].astype(f32)) * mod_rows(1, TC) + mod_rows(0, TC)

    def mod_rows(k, n, c0=0, w=D):
        return jnp.concatenate([mod_s[:, k * D + c0:k * D + c0 + w]] * (n // 8), axis=0)

    def phase_a(xpre_s, hpre_s, wm_s, stg, bg, g1, tq_s):
        def tq_place(c, n):
            if n == 1:
                return w_s.at[c], 0, None
            if n == 4:
                return w_s.at[c], D // 4, None
            return tq_s.at[c], 0, (0, 2, 3, 5, 6).index(n) * (HG // 2)

        def w_copy(t, g, slot):
            return copy(w_hbm[t].at[:, pl.ds(pl.multiple_of(g * HG, HG), HG), :], stg.at[slot],
                        SEM_STG + slot)

        def bg_rows(k):
            return clamp(k * BGR, H * E - BGR), clamp(k * G1R, HD - G1R)

        def bg_copies(k, slot):
            ro, r1 = bg_rows(k)
            return (copy(wo_hbm.at[pl.ds(aligned(ro, 16), BGR)], bg.at[slot], SEM_BG + slot),
                    copy(w1_hbm.at[:, pl.ds(aligned(r1, 16), G1R), :], g1.at[slot], SEM_G1 + slot))

        def relayout_jobs(slot, c, i):
            memo = []
            r = aligned(i * 8, 8)

            def job(j, z=None):
                if not memo:
                    for d0 in (i * 16, HD + i * 16):
                        memo.append(jnp.swapaxes(pltpu.bitcast(stg[slot, pl.ds(d0, 16)], u32), 0, 1))
                blk = []
                for kh in range(2):
                    u = memo[kh][j]
                    if z is not None:
                        u = u | jnp.concatenate([z, z], axis=0)
                    blk.append(pltpu.bitcast(u << 16, f32))
                    blk.append(pltpu.bitcast(u & jnp.uint32(0xFFFF0000), f32))
                for k, v in enumerate(blk):
                    w_s.at[c][pl.ds((k // 2) * (D // 4) + r, 8), _ct(2 * j + k % 2)] = _pk(v)
                for n, v in enumerate(_rhs_set(*blk)):
                    if n not in (1, 4):
                        ref, r0, c0 = tq_place(c, n)
                        ref[pl.ds(r0 + r, 8), _ct(c0 + j)] = _pk(v)

            return [functools.partial(job, j) for j in range(HG // 2)]

        def repack(slot, row, i, z):
            v = pltpu.bitcast(bg[slot, 16 * i:16 * i + 16, :], u32)
            v = v | jnp.concatenate([z] * (D // E), axis=1)
            wo_s[pl.ds(pl.multiple_of(row + 8 * i, 8), 8), :] = v

        cp_c = copy(c_hbm, c_s, SEM_C)
        cp_mem = copy(mem0_hbm, mem0_s, SEM_MEM)
        cp_xpre = copy(x_hbm.at[:, TC:SEG, :], xpre_s, SEM_XPRE)
        w_copy(0, 0, 0).start()
        cp_xpre.start()
        cp_c.start()
        cp_mem.start()
        for k in range(2 * D // E):
            wm_copy(wm_s, k, k, SEM_WM + k // 4).start()
        w_copy(0, 1, 1).start()

        zero_s[0:8, :] = jnp.zeros((8, E), u32)
        fill_s[0:NR, :] = _mask_fill()
        aout_s[...] = jnp.zeros(aout_s.shape, f32)
        l1_s[...] = jnp.zeros(l1_s.shape, u32)
        bg[1] = jnp.zeros(bg.shape[1:], bf16)
        g1[1] = jnp.zeros(g1.shape[1:], bf16)

        w_copy(0, 0, 0).wait()

        def rl0_body(i, carry):
            for job in relayout_jobs(0, 0, i):
                job()
            return carry

        lax.fori_loop(0, D // 32, rl0_body, 0)
        w_copy(0, 2, 0).start()
        for cp in bg_copies(0, 0):
            cp.start()

        cp_xpre.wait()

        def npre_body(i, carry):
            xr = xpre_s[pl.ds(pl.multiple_of(i * 8, 8), 8)].astype(f32).reshape(64, D)
            t_s[pl.ds(pl.multiple_of(i * 64, 64), 64), :] = _ln(xr)
            return carry

        lax.fori_loop(0, NSEG // 8, _scoped("npre", npre_body), 0)

        cp_c.wait()
        cp_mem.wait()
        mem_s[...] = mem0_s[...].astype(f32)

        for k in range(4):
            wm_wait(wm_s, 4 * k, 4, SEM_WM + k)
            mod_tiles(wm_s, 4 * k, 4, 4 * k)

        PH = NSEG * M // 2

        def hpre_body(i, carry):
            h = [t_s[pl.ds(pl.multiple_of(hf * PH + i * 16, 16), 16), :] * mod_rows(1, 16) + mod_rows(0, 16)
                 for hf in range(2)]
            for n, v in enumerate(_lhs_set(h[0][:, :HD], h[0][:, HD:], h[1][:, :HD], h[1][:, HD:])):
                hpre_s.at[n][pl.ds(pl.multiple_of(i * 8, 8), 8), :] = _pk(v)
            return carry

        lax.fori_loop(0, PH // 16, _scoped("hpre", hpre_body), 0)

        t_s[0:8, :] = jnp.zeros((8, D), f32)
        t_s[S + 8:S + 16, :] = jnp.zeros((8, D), f32)

        MB = 64

        def p1_body(c, carry):
            slot = c & 1
            pslot = 1 - slot
            ro, r1 = bg_rows(jnp.maximum(c - 1, 0))

            @pl.when(c >= 1)
            def _():
                for cp in bg_copies(0, pslot):
                    cp.wait()

            @pl.when(c + 1 < NC)
            def _():
                w_copy(0, 0, pslot).wait()

            small = [functools.partial(repack, pslot, ro >> 1, i) for i in range(BGR // 16)]
            small += [functools.partial(rhs_job, g1, pslot, 16 * rt, q, NQ + q, t1_s, q, (r1 >> 1) + 8 * rt)
                      for rt in range(G1R // 16) for q in range(NQ)]
            work = []
            nu = D // 32
            for i in range(nu):
                js = relayout_jobs(pslot, c + 1, i)
                work += [js[k:k + JGROUP] for k in range(0, len(js), JGROUP)]
                work += [[job] for job in small[i * len(small) // nu:(i + 1) * len(small) // nu]]
            npin = 7 * (HG // 2) * (PH // MB)
            jobs = [[] for _ in range(npin)]
            for k, group in enumerate(work):
                pos = k * (npin - P1_TAIL) * 8 // len(work)
                jobs[pos // 8] += [(job, pos % 8 if FINE else 0) for job in group]
            jobs = iter(jobs)

            def prod(n, q, mb):
                ref, r0, c0 = tq_place(c, n)
                w = ref[r0:r0 + D // 4, _ct(2 * q + (n == 4) if c0 is None else c0 + q)]
                m = _dot(_up(hpre_s[n, mb * MB // 2:(mb + 1) * MB // 2, :]), _up(w))
                pending.append(m)
                if len(pending) > P1_LAG:
                    anchor = pltpu.bitcast(pending.pop(0), u32)
                    for job, g in next(jobs):
                        job(anchor[8 * g:8 * g + 8] & zero_s[0:8, :])
                return m

            pending = []
            ns = MB // M
            for q in range(HG // 2):
                for mb in range(PH // MB):
                    cs = _strassen(lambda n: prod(n, q, mb))
                    for hf in range(2):
                        y = jnp.concatenate([cs[2 * hf + k][sg * M:(sg + 1) * M]
                                             for sg in range(ns) for k in range(2)], axis=0)
                        s0 = hf * (NSEG // 2) + mb * ns
                        pre_s.at[c][s0 * M:(s0 + ns) * M, _ct(q)] = _pk(y)

            for t in range(3):
                @pl.when((c + 3) >> 2 == t)
                def _():
                    w_copy(t, (c + 3) & 3, pslot).start()

            @pl.when(c + 2 < NC)
            def _():
                for cp in bg_copies(c + 1, pslot):
                    cp.start()

            @pl.when(c < NC - 3)
            def _():
                wm_copy(wm_s, 2 * D // E + c, c, SEM_WMR).start()

            @pl.when(c == NC - 3)
            def _():
                def issue(k, carry2):
                    wm_copy(wm_s, 2 * D // E + k, k, SEM_WMR).start()
                    return carry2

                x_copy(0).start()
                for k in range(2):
                    for cp in mlp_w_copies(k, k):
                        cp.start()
                lax.fori_loop(NC - 3, 3 * D // E, issue, 0)

            return carry

        lax.fori_loop(0, NC, _scoped("p1", p1_body), 0)
        x_copy(1).start()
        x_copy(0).wait()
        wm_wait(wm_s, 0, 3 * D // E, SEM_WMR)
        mod_tiles(wm_s, 0, 3 * D // E, 2 * D // E)
        hn_s[...] = h_rows(0)

    def phase_b(t2_s, t3_s, t4_s, wg_s, x1_s, base_s, yn_s, gs_s, act_s, o_s, os_s):
        for k in range(D // E):
            wm_copy(wg_s, 5 * D // E + k, k, SEM_WM).start()

        def chain_step(s, mem, htok, odef_prev, jobs=(), hooks=None):
            hs = jnp.concatenate([mem, htok], axis=0).astype(bf16)
            qkv = [[None] * 3 for _ in range(NP)]
            ps = [None] * NP
            os_ = [None] * H
            odef = [None] * H
            os_r = os_s.at[0:16] if odef_prev is None else os_s.at[16:40]

            def proj(p, ts=(0, 1, 2)):
                for t in ts:
                    c, q = t * NG + p // (HG // 2), p % (HG // 2)
                    a = _dot(hs, _up(w_s[c, :, _ct(2 * q)]))
                    b = _dot(hs, _up(w_s[c, :, _ct(2 * q + 1)]))
                    if hooks and t == 2 and p - NP in hooks:
                        hooks[p - NP](b)
                    pre = pre_s[c, pl.ds(pl.multiple_of(s * M, M), M), _ct(q)]
                    if t == 1:
                        kf = jnp.concatenate([a, b, _up(pre).astype(f32), jnp.zeros((E - NR, E), f32)],
                                             axis=0)
                        qkv[p][t] = kf.T.astype(bf16)
                        continue
                    if QV32:
                        parts = [a, b, _up(pre).astype(f32)]
                        if t == 2:
                            parts.append(jnp.zeros((E - NR, E), f32))
                        qkv[p][t] = jnp.concatenate(parts, axis=0).astype(bf16)
                        continue
                    parts = [_pk(a), _pk(b), pre]
                    if t == 2:
                        parts.append(jnp.zeros(((E - NR) // 2, E), u32))
                    qkv[p][t] = _up(jnp.concatenate(parts, axis=0))

            def scores(p):
                sc_ = _dot(qkv[p][0], qkv[p][1])
                fill = fill_s[0:NR, :]
                sc_ = jnp.where(fill == 0.0, sc_ * SCALE, fill)
                m = jnp.max(sc_, axis=-1, keepdims=True)
                e = jnp.exp(sc_ - m)
                l = jnp.sum(e, axis=-1, keepdims=True)
                r = pl.reciprocal(l, approx=True)
                r = r * (2.0 - l * r)
                ps[p] = (e * r).astype(bf16)

            def fin(p):
                o = _dot(ps[p], qkv[p][2])
                for hh in range(2):
                    h = 2 * p + hh
                    rows = o[32 * hh:32 * hh + 32]
                    odef[h] = o[64 + 8 * hh:72 + 8 * hh]
                    if odef_prev is not None:
                        rows = jnp.concatenate([rows, odef_prev[h], odef[h]], axis=0)
                    if OSREF:
                        os_r[:, _ct(h)] = _pk(rows)
                    else:
                        os_[h] = _pk(rows)

            acc = [None] * 8
            jobs = iter(jobs)

            def wo(h0, h1, js):
                if not OSREF:
                    lhs = _up(jnp.concatenate(os_[h0:h1], axis=1))
                for j in js:
                    if OSREF:
                        lhs = _up(os_r[:, h0 * E:h1 * E])
                    ws = []
                    for r0 in range(h0 * E // 2, h1 * E // 2, PIN_ROWS):
                        ws.append(pinned(lambda: wo_s[r0:r0 + PIN_ROWS, j * E:(j + 1) * E],
                                         next(jobs, None)))
                    part = _dot(lhs, _up(jnp.concatenate(ws, axis=0)))
                    if hooks and acc[j] is None and j in hooks:
                        hooks[j](part)
                    acc[j] = part if acc[j] is None else part + acc[j]

            ORDER, LAG_S, LAG_O = SCHED_A if odef_prev is None else SCHED_B
            for p in range(NP):
                if ORDER == 0:
                    proj(p)
                    if p >= LAG_S:
                        scores(p - LAG_S)
                    if p >= LAG_O:
                        fin(p - LAG_O)
                elif ORDER == 1:
                    proj(p, (1, 0))
                    if p >= LAG_O:
                        fin(p - LAG_O)
                    proj(p, (2,))
                    if p >= LAG_S:
                        scores(p - LAG_S)
                elif ORDER == 2:
                    proj(p, (1,))
                    if p >= LAG_S:
                        scores(p - LAG_S)
                    proj(p, (0,))
                    if p >= LAG_O:
                        fin(p - LAG_O)
                    proj(p, (2,))
                elif ORDER == 3:
                    proj(p, (1,))
                    if p >= LAG_O:
                        fin(p - LAG_O)
                    proj(p, (0,))
                    if p >= LAG_S:
                        scores(p - LAG_S)
                    proj(p, (2,))
                elif ORDER == 4:
                    proj(p, (1,))
                    if p >= LAG_S:
                        scores(p - LAG_S)
                    proj(p, (0, 2))
                    if p >= LAG_O:
                        fin(p - LAG_O)
                else:
                    proj(p, (0,))
                    if p >= LAG_S:
                        scores(p - LAG_S)
                    proj(p, (1,))
                    if p >= LAG_O:
                        fin(p - LAG_O)
                    proj(p, (2,))
            tail = []
            for k in range(LAG_O):
                step = []
                if NP - LAG_S + k < NP:
                    step.append(functools.partial(scores, NP - LAG_S + k))
                step.append(functools.partial(fin, NP - LAG_O + k))
                tail.append(step)
            hsplit = min(24, 2 * (NP - LAG_O))
            cuts = {3: (2, 3, 5), 2: (2, 5), 4: (1, 2, 4, 6), 5: (1, 2, 3, 4, 6)}[LAG_O]
            j0 = 0
            for k, step in enumerate(tail):
                wo(0, hsplit, range(j0, cuts[k]))
                j0 = cuts[k]
                for f in step:
                    f()
            wo(0, hsplit, range(j0, 8))
            wo(hsplit, H, range(8))
            return jnp.concatenate(acc, axis=1), odef

        def mixer_prep(i, r0, n, anchor=None):
            r = pl.ds(aligned(i * 64 + r0, 16), n)
            xr = x_s[2 * i + r0 // SEG, r0 % SEG:r0 % SEG + n, :].astype(f32)
            x2 = xr + mod_rows(2, n) * after(aout_s[r0:r0 + n, :], anchor)
            x_s.at[2 * i + r0 // SEG][r0 % SEG:r0 % SEG + n, :] = x2.astype(bf16)
            hb = _ln(x2) * mod_rows(4, n) + mod_rows(3, n)
            hb_s[r, :] = hb.astype(bf16)
            return _ln(hb)

        def mixer_sets(ya, yb, r0, dst=l1_s):
            n = ya.shape[0]
            for m, v in enumerate(_lhs_set(ya[:, :HD], ya[:, HD:], yb[:, :HD], yb[:, HD:])):
                dst[m * (SEG // 2) + r0 // 2:m * (SEG // 2) + (r0 + n) // 2, 0:HD] = _pk(v)

        def mixer_mm(i, src=l1_s, hook=None):
            for q in range(NQ):
                def prod(n):
                    m = _dot(_up(src[n * (SEG // 2):(n + 1) * (SEG // 2), 0:HD]),
                             _up(t1_s[n, :, _ct(q)]))
                    if hook is not None:
                        hook(m)
                    return m

                cs = _strassen(prod)
                for k, cc in enumerate(cs):
                    r0 = aligned(i * 64 + 8 + (k // 2) * SEG, 8)
                    t_s[pl.ds(r0, SEG), _ct(q + NQ * (k % 2))] = _gelu(cc)

        def p2_body(i, carry):
            slot = i & 1
            for cp in mlp_w_copies(0, slot):
                cp.wait()

            @pl.when(i == 1)
            def _():
                x_copy(1).wait()

            g, rr = mlp_piece(i)
            work = [functools.partial(rhs2_job, g2, slot, 0, 0, n1, t2_s.at[slot], (i >> 1) * 8)
                    for n1 in range(7)]
            work += [functools.partial(rhs2_job, g3, slot, 16 * rt, 0, n1, t3_s.at[g], rr * 32 + 8 * rt)
                     for rt in range(4) for n1 in range(7)]
            work += [functools.partial(rhs2_job, g4, slot, 16 * rt, 4 * og, n1, t4_s.at[og],
                                       g * (E // 2) + rr * 16 + 8 * rt)
                     for rt in range(2) for og in range(NOG) for n1 in range(7)]
            npin = len(work) - FREE_JOBS
            jobs = [None] * 64
            for k in range(npin):
                jobs[1 + k * 63 // npin] = work[k]

            sa_ = 2 * i
            sb_ = 2 * i + 1
            hb_tok = h_rows(sb_)
            oa, odef_a = chain_step(sa_, mem_s[...], hn_s[...], None)
            mixer_mm(jnp.maximum(i - 2, 0))
            ys = []

            def hook(k, anchor):
                if k >= PREP_CH:
                    anchor = anchor[0:8] + ys[-PREP_CH][0:8, 0:E] + ys[-PREP_CH][8:16, 0:E]
                ys.append(mixer_prep(jnp.maximum(i - 1, 0), (k % 2) * SEG + (k // 2) * 16, 16, anchor))
                if k % 2:
                    mixer_sets(ys[-2], ys[-1], (k // 2) * 16)

            hooks = {j: functools.partial(hook, k) for k, j in enumerate(PREP_AT)}
            ob, _ = chain_step(sb_, oa[0:M], hb_tok, odef_a, jobs, hooks)
            for job in work[npin:]:
                job()
            mem_s[...] = ob[0:M]
            aout_s[0:TC, :] = oa[M:SEG]
            aout_s[TC:SEG, :] = ob[SEG:SEG + M]
            aout_s[SEG:SEG + TC, :] = ob[M:SEG]
            aout_s[SEG + TC:2 * SEG, :] = ob[SEG + M:SEG + 2 * M]
            hn_s[...] = h_rows(jnp.minimum(sb_ + 1, NSEG - 1))
            for cp in mlp_w_copies(i + 2, slot):
                cp.start()
            return carry

        lax.fori_loop(0, _N2, _scoped("p2", p2_body), 0)

        TQ = TB // 4
        SHIFT = (-1, -1, 1, 1, -2, -2, 2, 2)

        def u_set(n):
            return w_s.at[n // 32], slice((n % 32) * (TQ // 2), (n % 32 + 1) * (TQ // 2))

        def d_set(slot, n):
            return w_s.at[slot], (n // 4) * (TQ // 2), (n % 4) * 2

        def d_lhs(slot, n):
            ref, r0, c0 = d_set(slot, n)
            return _up(ref[r0:r0 + TQ // 2, c0 * E:(c0 + 2) * E])

        def shift_job(j, r0, n, anchor=None):
            for ct in range(D // E):
                win = t_s[pl.ds(aligned(j * TB + r0, 16), n + 16), _ct(ct)]
                gs_s[r0:r0 + n, _ct(ct)] = after(
                    pltpu.roll(win, (-SHIFT[ct]) % (n + 16), 0)[8:8 + n], anchor)

        def mix(j, hook=None):
            r0 = aligned(j * TB, TB)
            for og in range(NOG):
                def prod(n):
                    m = _dot(d_lhs(3, n), _up(t2_s[og, :, _ct(n)]))
                    if hook is not None:
                        hook(m)
                    return m

                c = _strassen2(prod, *O2)
                for i in range(4):
                    for k in range(2):
                        cols = slice((4 * og + 2 * k) * E, (4 * og + 2 * k + 2) * E)
                        x1_s[i * TQ:(i + 1) * TQ, cols] = (
                            hb_s[pl.ds(r0 + i * TQ, TQ), cols].astype(f32)
                            + jnp.concatenate([c(i, 2 * k), c(i, 2 * k + 1)], axis=1))

        def base_job(j, rt, anchor):
            rows = slice(rt * 16, (rt + 1) * 16)
            z = pltpu.bitcast(pltpu.bitcast(anchor[0:8], u32) & zero_s[0:8, :], f32)
            gb = mod_rows(5, 8) + jnp.concatenate([z] * (D // E), axis=1)
            x2 = x_s[j * (TB // SEG) + rt // 2, (rt % 2) * 16:(rt % 2) * 16 + 16, :]
            base_s[rows, :] = x2.astype(f32) + jnp.concatenate([gb, gb], axis=0) * x1_s[rows, :]

        def out_copy(j, slot):
            return copy(o_s.at[slot], out_hbm.at[pl.ds(aligned(j * TB, TB), TB)], SEM_OUT + slot)

        def ln_job(r0, n, prev, anchor=None):
            if anchor is not None and len(prev) >= 2:
                anchor = anchor[0:8] + prev[-2]
            y = _ln(after(x1_s[r0:r0 + n, :], anchor))
            yn_s[r0:r0 + n, :] = y
            prev.append(y[0:8, 0:E] + y[8:16, 0:E])

        def set_job(src, slot, rt, ct, n1, n=16, anchor=None):
            blk = _outer_operand(lambda i, k: src[i * TQ + rt * n:i * TQ + (rt + 1) * n, _ct(2 * k + ct)],
                                 _LHS_TERMS[n1])
            blk[0] = after(blk[0], anchor)
            blk[3] = after(blk[3], anchor)
            for n2, v in enumerate(_lhs_set(*blk)):
                ref, r0, c0 = d_set(slot, 7 * n1 + n2)
                ref[r0 + rt * n // 2:r0 + (rt + 1) * n // 2, _ct(c0 + ct)] = _pk(v)

        def all_sets(src, slot):
            for n1 in range(7):
                for ct in range(2):
                    set_job(src, slot, 0, ct, n1, TQ)

        wm_wait(wg_s, 0, D // E, SEM_WM)
        mod_tiles(wg_s, 0, D // E, 5 * D // E)
        shift_job(0, 0, TB)
        all_sets(gs_s, 3)
        mix(0)
        prev0 = []
        plan = {}
        for k in range(TB // 16):
            plan[T_AT[0] * (k // 2) + k % 2] = [
                functools.partial(ln_job, (k % 4) * TQ + (k // 4) * 16, 16, prev0)]
        rest = [functools.partial(shift_job, 1, (k % 4) * TQ + (k // 4) * 16, 16)
                for k in range(TB // 16)]
        rest += [functools.partial(set_job, gs_s, 3, rt, ct, n1, 16)
                 for rt in range(2) for ct in range(2) for n1 in range(7)]
        for k, job in enumerate(rest):
            plan.setdefault(k * T_AT[1] // len(rest), []).append(job)
        rest = [functools.partial(set_job, yn_s, 2, rt, ct, n1, 16)
                for rt in range(2) for ct in range(2) for n1 in range(7)]
        for k, job in enumerate(rest):
            plan.setdefault(T_AT[1] + k * (T_AT[2] - T_AT[1]) // len(rest), []).append(job)
        tick0 = [0]

        def hook0(m):
            for job in plan.pop(tick0[0], ()):
                job(anchor=m)
            tick0[0] += 1

        mixer_mm(NI - 2, hook=hook0)
        mixer_sets(mixer_prep(NI - 1, 0, SEG), mixer_prep(NI - 1, SEG, SEG), 0, w_s.at[4])
        mixer_mm(NI - 1, w_s.at[4], hook0)
        assert not plan

        def mlp_block(j, last):
            slot = j & 1

            jn = clamp(j + 2, NB - 1)
            early = [functools.partial(base_job, j, k) for k in range(TB // 16)]
            shifts = [functools.partial(shift_job, jn, (k % 4) * TQ + (k // 4) * 16, 16)
                      for k in range(TB // 16)]
            if not last and SH_AT is None:
                early += shifts
            early = iter(early)

            pend = []
            tick = [0]

            def drain(m):
                tick[0] += 1
                if pend and tick[0] >= U_AT[0] and (tick[0] - U_AT[0]) % U_AT[1] == 0:
                    pend.pop(0)(m)

            def up_prod(n, g):
                m = _dot(d_lhs(2, n), _up(t3_s[g, :, _ct(n)]))
                if n in E_AT:
                    job = next(early, None)
                    if job is not None:
                        job(anchor=m)
                drain(m)
                return m

            def uset_job(tile, g, n1, r0, n, anchor=None):
                blk = _outer_operand(lambda i, k: tile(i, k, r0, n), _LHS_TERMS[n1])
                blk[0] = after(blk[0], anchor)
                blk[3] = after(blk[3], anchor)
                for n2, v in enumerate(_lhs_set(*blk)):
                    ref, rows = u_set(7 * n1 + n2)
                    ref[rows.start + r0 // 2:rows.start + (r0 + n) // 2, _ct(g)] = _pk(v)

            for g in range(NFG):
                c = _strassen2(lambda n: up_prod(n, g), *O3)
                assert not pend
                tick[0] = 0
                if U_AT[1] == 0 or (last and g == NFG - 1):
                    act = [[_gelu(c(i, k)) for k in range(4)] for i in range(4)]
                    for n1 in range(7):
                        uset_job(lambda i, k, r0, n: act[i][k], g, n1, 0, TQ)
                    continue
                c0 = 4 * (g % 2)
                for i in range(4):
                    for k in range(4):
                        act_s[i * TQ:(i + 1) * TQ, _ct(c0 + k)] = _gelu(c(i, k))

                def tile(i, k, r0, n, c0=c0):
                    return act_s[i * TQ + r0:i * TQ + r0 + n, _ct(c0 + k)]

                pend += [functools.partial(uset_job, tile, g, n1, r0, U_AT[2])
                         for n1 in range(7) for r0 in range(0, TQ, U_AT[2])]
            jobs = {}
            if not last:
                mix(j + 1, drain)
                assert not pend
                prev = []
                for k in range(TB // 16):
                    jobs[k * Y_AT] = functools.partial(ln_job, (k % 4) * TQ + (k // 4) * 16, 16, prev)

                def place(start, fns, step=1):
                    for fn in fns:
                        while start in jobs:
                            start += 1
                        jobs[start] = fn
                        start += step

                if SH_AT is not None:
                    place(SH_AT[0], shifts, SH_AT[1])
                for rt in range(2):
                    place(S_AT[rt], [functools.partial(set_job, yn_s, 2, rt, ct, n1, 16)
                                     for ct in range(2) for n1 in range(7)])
                place(G_AT, [functools.partial(set_job, gs_s, 3, rt, ct, n1, 16)
                             for rt in range(2) for ct in range(2) for n1 in range(7)])

            def down_part(n, og, k0, k1):
                ref, rows = u_set(n)
                return _dot(_up(ref[rows, k0 * E:k1 * E]),
                            _up(t4_s[og, k0 * E // 2:k1 * E // 2, _ct(n)]))

            head = {}
            if last:
                head = {n: down_part(n, 0, 0, NFG - 1) for n in range(HEAD)}
            count = [0]

            def down_prod(n, og):
                if og == 0 and n in head:
                    return down_part(n, og, NFG - 1, NFG) + head[n]
                m = down_part(n, og, 0, NFG)
                job = jobs.get(count[0])
                count[0] += 1
                if job is not None:
                    job(anchor=m)
                return m

            for og in range(NOG):
                c = _strassen2(lambda n: down_prod(n, og), *(O4 if not last else (0, O4[1])))
                for i in range(4):
                    rows = slice(i * TQ, (i + 1) * TQ)
                    for k in range(2):
                        c0 = (4 * og + 2 * k) * E
                        o_s.at[slot][rows, c0:c0 + 2 * E] = (
                            base_s[rows, c0:c0 + 2 * E] + mod_rows(5, TQ, c0, 2 * E)
                            * jnp.concatenate([c(i, 2 * k), c(i, 2 * k + 1)], axis=1)).astype(bf16)
            out_copy(j, slot).start()

        def p3_body(j, carry):
            @pl.when(j >= 2)
            def _():
                out_copy(j - 2, j & 1).wait()

            mlp_block(j, False)
            return carry

        lax.fori_loop(0, NB - 1, _scoped("p3", p3_body), 0)
        for k in range(2):
            for cp in mlp_w_copies(0, k):
                cp.wait()
        out_copy(NB - 3, (NB - 3) % 2).wait()
        mlp_block(NB - 1, True)
        out_copy(NB - 2, (NB - 2) % 2).wait()
        out_copy(NB - 1, (NB - 1) % 2).wait()

    pl.run_scoped(
        phase_a,
        pltpu.VMEM((NSEG, M, D), bf16),
        pltpu.VMEM((7, NSEG * M // 4, D // 2), u32),
        pltpu.VMEM((3 * D // E, D, E), bf16),
        pltpu.VMEM((2, D, HG, E), bf16),
        pltpu.VMEM((2, BGR, D), bf16),
        pltpu.VMEM((2, 2, G1R, D), bf16),
        pltpu.VMEM((NC + 1, D // 4, 5 * HG // 2 * E), u32),
    )
    pl.run_scoped(
        phase_b,
        pltpu.VMEM((NOG, D // 8, 49 * E), u32),
        pltpu.VMEM((NFG, D // 8, 49 * E), u32),
        pltpu.VMEM((NOG, F // 8, 49 * E), u32),
        pltpu.VMEM((D // E, D, E), bf16),
        pltpu.VMEM((TB, D), f32),
        pltpu.VMEM((TB, D), f32),
        pltpu.VMEM((TB, D), f32),
        pltpu.VMEM((TB, D), f32),
        pltpu.VMEM((TB, D), f32),
        pltpu.VMEM((2, TB, D), bf16),
        pltpu.VMEM((40, H * E), u32),
    )


@jax.jit
def pallas_adaLN_cond__memory_aug_recurrent_mem_tr__mixer_s_mlp__prompt_kernel(
    A_x: jax.Array,
    A_mem0: jax.Array,
    A_Wq: jax.Array,
    A_Wk: jax.Array,
    A_Wv: jax.Array,
    A_Wo: jax.Array,
    A_seg_len,
    B_x: jax.Array,
    B_w1: jax.Array,
    B_w2: jax.Array,
    B_w3: jax.Array,
    B_w4: jax.Array,
    c: jax.Array,
    w_mod: jax.Array,
):
    del A_seg_len, B_x
    assert A_x.shape == (1, S, D) and A_mem0.shape == (1, M, D)
    hbm = pl.BlockSpec(memory_space=pl.ANY)
    scratch = [
        pltpu.VMEM((NSEG, SEG, D), bf16),
        pltpu.VMEM((NC + 1, D // 2, HG * E), u32),
        pltpu.VMEM((H * E // 2, D), u32),
        pltpu.VMEM((7, D // 4, D // 2), u32),
        pltpu.VMEM((2, 4, 16, 4 * E), bf16),
        pltpu.VMEM((2, 4, 64, 4 * E), bf16),
        pltpu.VMEM((2, 4, 32, D), bf16),
        pltpu.VMEM((NC, NSEG * M, HG // 2 * E), u32),
        pltpu.VMEM((8, 6 * D), f32),
        pltpu.VMEM((M, D), f32),
        pltpu.VMEM((TC, D), f32),
        pltpu.VMEM((2 * SEG, D), f32),
        pltpu.VMEM((E, E), f32),
        pltpu.VMEM((S, D), bf16),
        pltpu.VMEM((S + 16, D), f32),
        pltpu.VMEM((7 * SEG // 2, D // 2), u32),
        pltpu.VMEM((8 * ZPAD, E), u32),
        pltpu.VMEM((1, D), bf16),
        pltpu.VMEM((M, D), bf16),
        pltpu.SemaphoreType.DMA((24,)),
    ]
    out = pl.pallas_call(
        _kernel,
        out_shape=jax.ShapeDtypeStruct((S, D), bf16),
        in_specs=[hbm] * 12,
        out_specs=hbm,
        scratch_shapes=scratch,
        compiler_params=pltpu.CompilerParams(vmem_limit_bytes=127 * 1024 * 1024,
                                             disable_bounds_checks=NO_BOUNDS,
                                             disable_semaphore_checks=NO_BOUNDS),
    )(A_x.reshape(NSEG, SEG, D), A_mem0.reshape(M, D), A_Wq, A_Wk, A_Wv,
      A_Wo.reshape(H * E, D), B_w1.reshape(2, D // 2, D), B_w2.reshape(4, D // 4, D), B_w3.reshape(4, D // 4, F),
      B_w4.reshape(NFG, 4, E, D), c, w_mod)
    return out.reshape(1, S, D)
```

```python
import functools

import jax
import jax.numpy as jnp
from jax import lax
import jax.experimental.pallas as pl
import jax.experimental.pallas.tpu as pltpu

bf16, f32, u32 = jnp.bfloat16, jnp.float32, jnp.uint32

S, D, H, E, M, SEG, F = 2048, 1024, 32, 128, 8, 32, 3584
EPS = 1e-5
SCALE = E ** -0.5
NSEG = S // SEG
NI = NSEG // 2
NP = H // 2
NR = 2 * (M + SEG)
TC = SEG - M
HG = 8
NG = H // HG
NC = 3 * NG
BGR = 384
G1R = 48
X0 = 4
TB = 128
NB = S // TB
HD = D // 2
NQ = D // E // 2
NFG = F // (4 * E)
NOG = D // (4 * E)

PIN_ROWS = 256
P1_LAG, P1_TAIL = 4, 5
PREP_AT = (0, 1, 4, 5)
T_AT = (7, 28, 52)
E_AT = (10, 24, 34)
U_AT = (6, 3)
Y_AT, S_AT, G_AT = 4, (26, 44), 62
HEAD = 14
NO_CHECKS = True
_SCOPES = False


def _scoped(name, fn):
    def wrapped(*a):
        if not _SCOPES:
            return fn(*a)
        with jax.named_scope(name):
            return fn(*a)
    return wrapped


def _pk(x):
    return pltpu.bitcast(x.astype(bf16), u32)


def _up(x):
    return pltpu.bitcast(x, bf16)


def _ct(k):
    return slice(k * E, (k + 1) * E)


def _dot(a, b):
    return jnp.dot(a, b, preferred_element_type=f32)


def _ln(x):
    m = jnp.mean(x, axis=-1, keepdims=True)
    xc = x - m
    v = jnp.mean(xc * xc, axis=-1, keepdims=True)
    return xc * lax.rsqrt(v + EPS)


def _gelu(x):
    c = 0.7978845608028654
    return 0.5 * x * (1.0 + jnp.tanh(c * (x + 0.044715 * (x * x * x))))


def _lhs_set(a11, a12, a21, a22):
    return (a11 + a22, a21 + a22, a11, a22, a11 + a12, a21 - a11, a12 - a22)


def _rhs_set(b11, b12, b21, b22):
    return (b11 + b22, b11, b12 - b22, b21 - b11, b22, b11 + b12, b21 + b22)


_LHS_TERMS = (((0, 1), (3, 1)), ((2, 1), (3, 1)), ((0, 1),), ((3, 1),),
              ((0, 1), (1, 1)), ((2, 1), (0, -1)), ((1, 1), (3, -1)))
_RHS_TERMS = (((0, 1), (3, 1)), ((0, 1),), ((1, 1), (3, -1)), ((2, 1), (0, -1)),
              ((3, 1),), ((0, 1), (1, 1)), ((2, 1), (3, 1)))


def _outer_operand(tile, terms):
    out = []
    for i in range(2):
        for j in range(2):
            v = None
            for o, sign in terms:
                t = tile(2 * (o // 2) + i, 2 * (o % 2) + j)
                v = t if v is None else (v + t if sign > 0 else v - t)
            out.append(v)
    return out


class _Quad:
    def __init__(self, tiles):
        self.t = tuple(tiles)

    def __add__(self, other):
        return _Quad([a + b for a, b in zip(self.t, other.t)])

    def __sub__(self, other):
        return _Quad([a - b for a, b in zip(self.t, other.t)])


def _strassen2(m, order=0):
    cs = _strassen(lambda n1: _Quad(_strassen(lambda n2: m(7 * n1 + n2))), order)
    return lambda i, j: cs[2 * (i // 2) + j // 2].t[2 * (i % 2) + j % 2]


def _strassen(m, order=0):
    if order == 0:
        m1 = m(0)
        m2 = m(1)
        c22 = m1 - m2
        m3 = m(2)
        c22 = c22 + m3
        c22 = m(5) + c22
        m4 = m(3)
        c21 = m2 + m4
        c11 = m1 + m4
        m5 = m(4)
        c12 = m3 + m5
        c11 = c11 - m5
        c11 = m(6) + c11
    else:
        m2 = m(1)
        c22 = m(5) - m2
        m4 = m(3)
        c21 = m2 + m4
        m1 = m(0)
        c22 = c22 + m1
        c11 = m4 + m1
        m3 = m(2)
        c22 = c22 + m3
        m5 = m(4)
        c12 = m3 + m5
        c11 = c11 - m5
        c11 = m(6) + c11
    return c11, c12, c21, c22


def _mask_fill():
    shape = (NR, E)
    r = lax.broadcasted_iota(jnp.int32, shape, 0)
    c = lax.broadcasted_iota(jnp.int32, shape, 1)

    def headpos(i):
        head = jnp.where(i < 64, i >> 5, (i - 64) >> 3)
        pos = jnp.where(i < 64, i & 31, 32 + (i & 7))
        return head, pos

    hr, pr = headpos(r)
    hc, pc = headpos(c)
    same = hr == hc
    valid = same & ((pr < M) | (pr >= pc))
    return jnp.where(valid, 0.0, jnp.where(same, -1e9, -jnp.inf)).astype(f32)


def _kernel(x_hbm, mem0_hbm, wq_hbm, wk_hbm, wv_hbm, wo_hbm, w1_hbm, w2_hbm, w3_hbm,
            w4_hbm, c_hbm, wm_hbm,
            out_hbm,
            x_s, w_s, wo_s, t1_s, g2, g3, g4, pre_s, mod_s, mem_s, hn_s, aout_s, fill_s,
            hb_s, t_s, l1_s, zero_s, c_s, mem0_s, sems):
    w_hbm = (wq_hbm, wk_hbm, wv_hbm)

    (SEM_C, SEM_MEM, SEM_XPRE, SEM_X, SEM_STG, SEM_BG, SEM_OUT,
     SEM_WMR, SEM_G2, SEM_G3, SEM_G4, SEM_WM, SEM_G1) = (0, 1, 2, 3, 4, 6, 8, 10, 12, 14, 16, 18, 22)

    def copy(src, dst, k):
        return pltpu.make_async_copy(src, dst, sems.at[k])

    def aligned(x, n):
        return x if isinstance(x, int) else pl.multiple_of(x, n)

    def clamp(k, hi):
        return min(k, hi) if isinstance(k, int) else jnp.minimum(k, hi)

    def mlp_piece(k):
        k = clamp(k, 4 * NFG - 1)
        return k >> 2, k & 3

    def mlp_w_copies(k, slot):
        g, rr = mlp_piece(k)
        k2 = clamp(k, NI - 1)
        return (copy(w2_hbm.at[:, pl.ds(aligned((k2 >> 1) * 16, 16), 16),
                               pl.ds(aligned((k2 & 1) * 4 * E, E), 4 * E)], g2.at[slot], SEM_G2 + slot),
                copy(w3_hbm.at[:, pl.ds(aligned(rr * 64, 64), 64), pl.ds(aligned(g * 4 * E, E), 4 * E)],
                     g3.at[slot], SEM_G3 + slot),
                copy(w4_hbm.at[g, :, pl.ds(aligned(rr * 32, 32), 32), :], g4.at[slot], SEM_G4 + slot))

    def pinned(w, job):
        if job is None:
            return w()
        z = job() & zero_s[0:8, :]
        w = w()
        return jnp.concatenate([w[0:8] | z, w[8:]], axis=0)

    def after(x, anchor):
        if anchor is None:
            return x
        z = pltpu.bitcast(pltpu.bitcast(anchor[0:8], u32) & zero_s[0:8, :], f32)
        z = jnp.concatenate([z] * (x.shape[0] // 8), axis=0)
        return jnp.concatenate([x[:, 0:E] + z, x[:, E:]], axis=1) if x.shape[1] > E else x + z

    def rhs_job(src, slot, r0, q, dst, row, z):
        blk = [src[slot, kh, r0:r0 + 16, _ct(cc)].astype(f32)
               for kh in range(2) for cc in (q, NQ + q)]
        zf = pltpu.bitcast(jnp.concatenate([z, z], axis=0), f32)
        blk[0] = blk[0] + zf
        blk[3] = blk[3] + zf
        for n, v in enumerate(_rhs_set(*blk)):
            dst.at[n][pl.ds(pl.multiple_of(row, 8), 8), _ct(q)] = _pk(v)

    def rhs2_job(src, slot, r0, c0, n1, dst, row):
        blk = _outer_operand(lambda i, j: src[slot, i, r0:r0 + 16, _ct(c0 + j)].astype(f32),
                             _RHS_TERMS[n1])
        sets = _rhs_set(*blk)
        for n2, v in enumerate(sets):
            dst[pl.ds(pl.multiple_of(row, 8), 8), _ct(7 * n1 + n2)] = _pk(v)
        out = pltpu.bitcast(sets[2], u32) | pltpu.bitcast(sets[3], u32)
        return out[0:8] | out[8:16]

    def silu_c():
        cf = c_s[...].astype(f32)
        return jnp.broadcast_to(cf * (1.0 / (1.0 + jnp.exp(-cf))), (8, D)).astype(bf16)

    def wm_copy(wm_s, src_tile, dst_tile, sem):
        return copy(wm_hbm.at[:, pl.ds(aligned(src_tile * E, E), E)], wm_s.at[dst_tile], sem)

    def wm_wait(wm_s, t0, n, sem):
        copy(wm_s.at[t0:t0 + n], wm_s.at[t0:t0 + n], sem).wait()

    def mod_tiles(wm_s, t0, n, dst_tile):
        sc8 = silu_c()
        for k in range(n):
            v = _dot(sc8, wm_s[t0 + k])
            if (dst_tile + k) // (D // E) in (1, 4):
                v = 1.0 + v
            mod_s[:, _ct(dst_tile + k)] = v

    def x_copy(k):
        r = slice(0, X0) if k == 0 else slice(X0, NSEG)
        return copy(x_hbm.at[r], x_s.at[r], SEM_XPRE if k == 0 else SEM_X)

    def h_rows(s):
        return _ln(x_s[s, 0:TC, :].astype(f32)) * mod_rows(1, TC) + mod_rows(0, TC)

    def mod_rows(k, n, c0=0, w=D):
        return jnp.concatenate([mod_s[:, k * D + c0:k * D + c0 + w]] * (n // 8), axis=0)

    def phase_a(xpre_s, hpre_s, wm_s, stg, bg, g1, tq_s):
        def tq_place(c, n):
            if n == 1:
                return w_s.at[c], 0, None
            if n == 4:
                return w_s.at[c], D // 4, None
            return tq_s.at[c], 0, (0, 2, 3, 5, 6).index(n) * (HG // 2)

        def w_copy(t, g, slot):
            return copy(w_hbm[t].at[:, pl.ds(pl.multiple_of(g * HG, HG), HG), :], stg.at[slot],
                        SEM_STG + slot)

        def bg_rows(k):
            return clamp(k * BGR, H * E - BGR), clamp(k * G1R, HD - G1R)

        def bg_copies(k, slot):
            ro, r1 = bg_rows(k)
            return (copy(wo_hbm.at[pl.ds(aligned(ro, 16), BGR)], bg.at[slot], SEM_BG + slot),
                    copy(w1_hbm.at[:, pl.ds(aligned(r1, 16), G1R), :], g1.at[slot], SEM_G1 + slot))

        def relayout_jobs(slot, c, i):
            memo = []
            r = aligned(i * 8, 8)

            def job(j, z=None):
                if not memo:
                    for d0 in (i * 16, HD + i * 16):
                        memo.append(jnp.swapaxes(pltpu.bitcast(stg[slot, pl.ds(d0, 16)], u32), 0, 1))
                blk = []
                for kh in range(2):
                    u = memo[kh][j]
                    if z is not None:
                        u = u | jnp.concatenate([z, z], axis=0)
                    blk.append(pltpu.bitcast(u << 16, f32))
                    blk.append(pltpu.bitcast(u & jnp.uint32(0xFFFF0000), f32))
                for k, v in enumerate(blk):
                    w_s.at[c][pl.ds((k // 2) * (D // 4) + r, 8), _ct(2 * j + k % 2)] = _pk(v)
                for n, v in enumerate(_rhs_set(*blk)):
                    if n not in (1, 4):
                        ref, r0, c0 = tq_place(c, n)
                        ref[pl.ds(r0 + r, 8), _ct(c0 + j)] = _pk(v)

            return [functools.partial(job, j) for j in range(HG // 2)]

        def repack(slot, row, i, z):
            v = pltpu.bitcast(bg[slot, 16 * i:16 * i + 16, :], u32)
            v = v | jnp.concatenate([z] * (D // E), axis=1)
            wo_s[pl.ds(pl.multiple_of(row + 8 * i, 8), 8), :] = v

        cp_c = copy(c_hbm, c_s, SEM_C)
        cp_mem = copy(mem0_hbm, mem0_s, SEM_MEM)
        cp_xpre = copy(x_hbm.at[:, TC:SEG, :], xpre_s, SEM_XPRE)
        w_copy(0, 0, 0).start()
        cp_xpre.start()
        cp_c.start()
        cp_mem.start()
        for k in range(2 * D // E):
            wm_copy(wm_s, k, k, SEM_WM + k // 4).start()
        w_copy(0, 1, 1).start()

        zero_s[0:8, :] = jnp.zeros((8, E), u32)
        fill_s[0:NR, :] = _mask_fill()
        aout_s[...] = jnp.zeros(aout_s.shape, f32)
        l1_s[...] = jnp.zeros(l1_s.shape, u32)
        bg[1] = jnp.zeros(bg.shape[1:], bf16)
        g1[1] = jnp.zeros(g1.shape[1:], bf16)

        w_copy(0, 0, 0).wait()

        def rl0_body(i, carry):
            for job in relayout_jobs(0, 0, i):
                job()
            return carry

        lax.fori_loop(0, D // 32, rl0_body, 0)
        w_copy(0, 2, 0).start()
        for cp in bg_copies(0, 0):
            cp.start()

        cp_xpre.wait()

        def npre_body(i, carry):
            xr = xpre_s[pl.ds(pl.multiple_of(i * 8, 8), 8)].astype(f32).reshape(64, D)
            t_s[pl.ds(pl.multiple_of(i * 64, 64), 64), :] = _ln(xr)
            return carry

        lax.fori_loop(0, NSEG // 8, _scoped("npre", npre_body), 0)

        cp_c.wait()
        cp_mem.wait()
        mem_s[...] = mem0_s[...].astype(f32)

        for k in range(4):
            wm_wait(wm_s, 4 * k, 4, SEM_WM + k)
            mod_tiles(wm_s, 4 * k, 4, 4 * k)

        PH = NSEG * M // 2

        def hpre_body(i, carry):
            h = [t_s[pl.ds(pl.multiple_of(hf * PH + i * 16, 16), 16), :] * mod_rows(1, 16) + mod_rows(0, 16)
                 for hf in range(2)]
            for n, v in enumerate(_lhs_set(h[0][:, :HD], h[0][:, HD:], h[1][:, :HD], h[1][:, HD:])):
                hpre_s.at[n][pl.ds(pl.multiple_of(i * 8, 8), 8), :] = _pk(v)
            return carry

        lax.fori_loop(0, PH // 16, _scoped("hpre", hpre_body), 0)

        t_s[0:8, :] = jnp.zeros((8, D), f32)
        t_s[S + 8:S + 16, :] = jnp.zeros((8, D), f32)

        MB = 64

        def p1_body(c, carry):
            slot = c & 1
            pslot = 1 - slot
            ro, r1 = bg_rows(jnp.maximum(c - 1, 0))

            @pl.when(c >= 1)
            def _():
                for cp in bg_copies(0, pslot):
                    cp.wait()

            @pl.when(c + 1 < NC)
            def _():
                w_copy(0, 0, pslot).wait()

            small = [functools.partial(repack, pslot, ro >> 1, i) for i in range(BGR // 16)]
            small += [functools.partial(rhs_job, g1, pslot, 16 * rt, q, t1_s, (r1 >> 1) + 8 * rt)
                      for rt in range(G1R // 16) for q in range(NQ)]
            work = []
            nu = D // 32
            for i in range(nu):
                work += relayout_jobs(pslot, c + 1, i)
                work += small[i * len(small) // nu:(i + 1) * len(small) // nu]
            npin = 7 * (HG // 2) * (PH // MB)
            jobs = [[] for _ in range(npin)]
            for k, job in enumerate(work):
                pos = k * (npin - P1_TAIL) * 8 // len(work)
                jobs[pos // 8].append((job, pos % 8))
            jobs = iter(jobs)

            def prod(n, q, mb):
                ref, r0, c0 = tq_place(c, n)
                w = ref[r0:r0 + D // 4, _ct(2 * q + (n == 4) if c0 is None else c0 + q)]
                m = _dot(_up(hpre_s[n, mb * MB // 2:(mb + 1) * MB // 2, :]), _up(w))
                pending.append(m)
                if len(pending) > P1_LAG:
                    anchor = pltpu.bitcast(pending.pop(0), u32)
                    for job, g in next(jobs):
                        job(anchor[8 * g:8 * g + 8] & zero_s[0:8, :])
                return m

            pending = []
            ns = MB // M
            for q in range(HG // 2):
                for mb in range(PH // MB):
                    cs = _strassen(lambda n: prod(n, q, mb))
                    for hf in range(2):
                        y = jnp.concatenate([cs[2 * hf + k][sg * M:(sg + 1) * M]
                                             for sg in range(ns) for k in range(2)], axis=0)
                        s0 = hf * (NSEG // 2) + mb * ns
                        pre_s.at[c][s0 * M:(s0 + ns) * M, _ct(q)] = _pk(y)

            for t in range(3):
                @pl.when((c + 3) >> 2 == t)
                def _():
                    w_copy(t, (c + 3) & 3, pslot).start()

            @pl.when(c + 2 < NC)
            def _():
                for cp in bg_copies(c + 1, pslot):
                    cp.start()

            @pl.when(c < NC - 3)
            def _():
                wm_copy(wm_s, 2 * D // E + c, c, SEM_WMR).start()

            @pl.when(c == NC - 3)
            def _():
                def issue(k, carry2):
                    wm_copy(wm_s, 2 * D // E + k, k, SEM_WMR).start()
                    return carry2

                x_copy(0).start()
                for k in range(2):
                    for cp in mlp_w_copies(k, k):
                        cp.start()
                lax.fori_loop(NC - 3, 3 * D // E, issue, 0)

            return carry

        lax.fori_loop(0, NC, _scoped("p1", p1_body), 0)
        x_copy(1).start()
        x_copy(0).wait()
        wm_wait(wm_s, 0, 3 * D // E, SEM_WMR)
        mod_tiles(wm_s, 0, 3 * D // E, 2 * D // E)
        hn_s[...] = after(h_rows(0), pltpu.bitcast(tq_s[NC, 0:8, 0:E], f32))

    def phase_b(t2_s, t3_s, t4_s, wg_s, x1_s, base_s, yn_s, gs_s, act_s, o_s):
        for k in range(D // E):
            wm_copy(wg_s, 5 * D // E + k, k, SEM_WM).start()

        def chain_step(s, mem, htok, odef_prev, jobs=(), hooks=None):
            hs = jnp.concatenate([mem, htok], axis=0).astype(bf16)
            qkv = [[None] * 3 for _ in range(NP)]
            ps = [None] * NP
            os_ = [None] * H
            odef = [None] * H

            def proj(p, t):
                c, q = t * NG + p // (HG // 2), p % (HG // 2)
                a = _dot(hs, _up(w_s[c, :, _ct(2 * q)]))
                b = _dot(hs, _up(w_s[c, :, _ct(2 * q + 1)]))
                pre = pre_s[c, pl.ds(pl.multiple_of(s * M, M), M), _ct(q)]
                parts = [a, b, _up(pre).astype(f32)]
                if t > 0:
                    parts.append(jnp.zeros((E - NR, E), f32))
                v = jnp.concatenate(parts, axis=0)
                qkv[p][t] = (v.T if t == 1 else v).astype(bf16)

            def scores(p):
                sc_ = _dot(qkv[p][0], qkv[p][1])
                fill = fill_s[0:NR, :]
                sc_ = jnp.where(fill == 0.0, sc_ * SCALE, fill)
                m = jnp.max(sc_, axis=-1, keepdims=True)
                e = jnp.exp(sc_ - m)
                l = jnp.sum(e, axis=-1, keepdims=True)
                r = pl.reciprocal(l, approx=True)
                r = r * (2.0 - l * r)
                ps[p] = (e * r).astype(bf16)

            def fin(p):
                o = _dot(ps[p], qkv[p][2])
                for hh in range(2):
                    h = 2 * p + hh
                    rows = o[32 * hh:32 * hh + 32]
                    odef[h] = o[64 + 8 * hh:72 + 8 * hh]
                    if odef_prev is not None:
                        rows = jnp.concatenate([rows, odef_prev[h], odef[h]], axis=0)
                    os_[h] = _pk(rows)

            acc = [None] * 8
            jobs = iter(jobs)

            def wo(h0, h1, js):
                lhs = _up(jnp.concatenate(os_[h0:h1], axis=1))
                for j in js:
                    ws = []
                    for r0 in range(h0 * E // 2, h1 * E // 2, PIN_ROWS):
                        ws.append(pinned(lambda: wo_s[r0:r0 + PIN_ROWS, j * E:(j + 1) * E],
                                         next(jobs, None)))
                    part = _dot(lhs, _up(jnp.concatenate(ws, axis=0)))
                    if hooks and acc[j] is None and j in hooks:
                        hooks[j](part)
                    acc[j] = part if acc[j] is None else part + acc[j]

            for p in range(NP):
                attn = [functools.partial(scores, p - 1) if p >= 1 else None,
                        functools.partial(fin, p - 3) if p >= 3 else None]
                if odef_prev is not None:
                    attn.reverse()
                for t, f in zip((1, 0, 2), attn + [None]):
                    proj(p, t)
                    if f is not None:
                        f()
            hsplit = 24
            wo(0, hsplit, range(0, 2))
            scores(NP - 1)
            fin(NP - 3)
            wo(0, hsplit, range(2, 3))
            fin(NP - 2)
            wo(0, hsplit, range(3, 5))
            fin(NP - 1)
            wo(0, hsplit, range(5, 8))
            wo(hsplit, H, range(8))
            return jnp.concatenate(acc, axis=1), odef

        def mixer_prep(i, r0, n, anchor=None):
            r = pl.ds(aligned(i * 64 + r0, 16), n)
            xr = x_s[2 * i + r0 // SEG, r0 % SEG:r0 % SEG + n, :].astype(f32)
            x2 = xr + mod_rows(2, n) * after(aout_s[r0:r0 + n, :], anchor)
            x_s.at[2 * i + r0 // SEG][r0 % SEG:r0 % SEG + n, :] = x2.astype(bf16)
            hb = _ln(x2) * mod_rows(4, n) + mod_rows(3, n)
            hb_s[r, :] = hb.astype(bf16)
            return _ln(hb)

        def mixer_sets(ya, yb, r0, dst=l1_s):
            n = ya.shape[0]
            for m, v in enumerate(_lhs_set(ya[:, :HD], ya[:, HD:], yb[:, :HD], yb[:, HD:])):
                dst[m * (SEG // 2) + r0 // 2:m * (SEG // 2) + (r0 + n) // 2, 0:HD] = _pk(v)

        def mixer_mm(i, src=l1_s, hook=None):
            for q in range(NQ):
                def prod(n):
                    m = _dot(_up(src[n * (SEG // 2):(n + 1) * (SEG // 2), 0:HD]),
                             _up(t1_s[n, :, _ct(q)]))
                    if hook is not None:
                        hook(m)
                    return m

                cs = _strassen(prod)
                for k, cc in enumerate(cs):
                    r0 = aligned(i * 64 + 8 + (k // 2) * SEG, 8)
                    t_s[pl.ds(r0, SEG), _ct(q + NQ * (k % 2))] = _gelu(cc)

        def p2_body(i, carry):
            slot = i & 1
            for cp in mlp_w_copies(0, slot):
                cp.wait()

            @pl.when(i == 1)
            def _():
                x_copy(1).wait()

            g, rr = mlp_piece(i)
            work = [functools.partial(rhs2_job, g2, slot, 0, 0, n1, t2_s.at[slot], (i >> 1) * 8)
                    for n1 in range(7)]
            work += [functools.partial(rhs2_job, g3, slot, 16 * rt, 0, n1, t3_s.at[g], rr * 32 + 8 * rt)
                     for rt in range(4) for n1 in range(7)]
            work += [functools.partial(rhs2_job, g4, slot, 16 * rt, 4 * og, n1, t4_s.at[og],
                                       g * (E // 2) + rr * 16 + 8 * rt)
                     for rt in range(2) for og in range(NOG) for n1 in range(7)]
            jobs = [None] + work

            sa_ = 2 * i
            sb_ = 2 * i + 1
            hb_tok = h_rows(sb_)
            oa, odef_a = chain_step(sa_, mem_s[...], hn_s[...], None)
            mixer_mm(jnp.maximum(i - 2, 0))
            ys = []

            def hook(k, anchor):
                if k >= 2:
                    anchor = anchor[0:8] + ys[-2][0:8, 0:E] + ys[-2][8:16, 0:E]
                ys.append(mixer_prep(jnp.maximum(i - 1, 0), (k % 2) * SEG + (k // 2) * 16, 16, anchor))
                if k % 2:
                    mixer_sets(ys[-2], ys[-1], (k // 2) * 16)

            hooks = {j: functools.partial(hook, k) for k, j in enumerate(PREP_AT)}
            ob, _ = chain_step(sb_, oa[0:M], hb_tok, odef_a, jobs, hooks)
            mem_s[...] = ob[0:M]
            aout_s[0:TC, :] = oa[M:SEG]
            aout_s[TC:SEG, :] = ob[SEG:SEG + M]
            aout_s[SEG:SEG + TC, :] = ob[M:SEG]
            aout_s[SEG + TC:2 * SEG, :] = ob[SEG + M:SEG + 2 * M]
            hn_s[...] = h_rows(jnp.minimum(sb_ + 1, NSEG - 1))
            for cp in mlp_w_copies(i + 2, slot):
                cp.start()
            return carry

        lax.fori_loop(0, NI, _scoped("p2", p2_body), 0)

        TQ = TB // 4
        SHIFT = (-1, -1, 1, 1, -2, -2, 2, 2)

        def u_set(n):
            return w_s.at[n // 32], slice((n % 32) * (TQ // 2), (n % 32 + 1) * (TQ // 2))

        def d_set(slot, n):
            return w_s.at[slot], (n // 4) * (TQ // 2), (n % 4) * 2

        def d_lhs(slot, n):
            ref, r0, c0 = d_set(slot, n)
            return _up(ref[r0:r0 + TQ // 2, c0 * E:(c0 + 2) * E])

        def shift_job(j, r0, n, anchor=None):
            for ct in range(D // E):
                win = t_s[pl.ds(aligned(j * TB + r0, 16), n + 16), _ct(ct)]
                gs_s[r0:r0 + n, _ct(ct)] = after(
                    pltpu.roll(win, (-SHIFT[ct]) % (n + 16), 0)[8:8 + n], anchor)

        def mix(j, hook=None):
            r0 = aligned(j * TB, TB)
            for og in range(NOG):
                def prod(n):
                    m = _dot(d_lhs(3, n), _up(t2_s[og, :, _ct(n)]))
                    if hook is not None:
                        hook(m)
                    return m

                c = _strassen2(prod)
                for i in range(4):
                    for k in range(2):
                        cols = slice((4 * og + 2 * k) * E, (4 * og + 2 * k + 2) * E)
                        x1_s[i * TQ:(i + 1) * TQ, cols] = (
                            hb_s[pl.ds(r0 + i * TQ, TQ), cols].astype(f32)
                            + jnp.concatenate([c(i, 2 * k), c(i, 2 * k + 1)], axis=1))

        def base_job(j, rt, anchor):
            rows = slice(rt * 16, (rt + 1) * 16)
            z = pltpu.bitcast(pltpu.bitcast(anchor[0:8], u32) & zero_s[0:8, :], f32)
            gb = mod_rows(5, 8) + jnp.concatenate([z] * (D // E), axis=1)
            x2 = x_s[j * (TB // SEG) + rt // 2, (rt % 2) * 16:(rt % 2) * 16 + 16, :]
            base_s[rows, :] = x2.astype(f32) + jnp.concatenate([gb, gb], axis=0) * x1_s[rows, :]

        def out_copy(j, slot):
            return copy(o_s.at[slot], out_hbm.at[pl.ds(aligned(j * TB, TB), TB)], SEM_OUT + slot)

        def ln_job(r0, n, prev, anchor=None):
            if anchor is not None and len(prev) >= 2:
                anchor = anchor[0:8] + prev[-2]
            y = _ln(after(x1_s[r0:r0 + n, :], anchor))
            yn_s[r0:r0 + n, :] = y
            prev.append(y[0:8, 0:E] + y[8:16, 0:E])

        def set_job(src, slot, rt, ct, n1, n=16, anchor=None):
            blk = _outer_operand(lambda i, k: src[i * TQ + rt * n:i * TQ + (rt + 1) * n, _ct(2 * k + ct)],
                                 _LHS_TERMS[n1])
            blk[0] = after(blk[0], anchor)
            blk[3] = after(blk[3], anchor)
            for n2, v in enumerate(_lhs_set(*blk)):
                ref, r0, c0 = d_set(slot, 7 * n1 + n2)
                ref[r0 + rt * n // 2:r0 + (rt + 1) * n // 2, _ct(c0 + ct)] = _pk(v)

        def all_sets(src, slot):
            for n1 in range(7):
                for ct in range(2):
                    set_job(src, slot, 0, ct, n1, TQ)

        wm_wait(wg_s, 0, D // E, SEM_WM)
        mod_tiles(wg_s, 0, D // E, 5 * D // E)
        shift_job(0, 0, TB)
        all_sets(gs_s, 3)
        mix(0)
        prev0 = []
        plan = {}
        for k in range(TB // 16):
            plan[T_AT[0] * (k // 2) + k % 2] = [
                functools.partial(ln_job, (k % 4) * TQ + (k // 4) * 16, 16, prev0)]
        rest = [functools.partial(shift_job, 1, (k % 4) * TQ + (k // 4) * 16, 16)
                for k in range(TB // 16)]
        rest += [functools.partial(set_job, gs_s, 3, rt, ct, n1, 16)
                 for rt in range(2) for ct in range(2) for n1 in range(7)]
        for k, job in enumerate(rest):
            plan.setdefault(k * T_AT[1] // len(rest), []).append(job)
        rest = [functools.partial(set_job, yn_s, 2, rt, ct, n1, 16)
                for rt in range(2) for ct in range(2) for n1 in range(7)]
        for k, job in enumerate(rest):
            plan.setdefault(T_AT[1] + k * (T_AT[2] - T_AT[1]) // len(rest), []).append(job)
        tick0 = [0]

        def hook0(m):
            for job in plan.pop(tick0[0], ()):
                job(anchor=m)
            tick0[0] += 1

        mixer_mm(NI - 2, hook=hook0)
        mixer_sets(mixer_prep(NI - 1, 0, SEG), mixer_prep(NI - 1, SEG, SEG), 0, w_s.at[4])
        mixer_mm(NI - 1, w_s.at[4], hook0)
        assert not plan

        def mlp_block(j, last):
            slot = j & 1

            jn = clamp(j + 2, NB - 1)
            early = [functools.partial(base_job, j, k) for k in range(TB // 16)]
            if not last:
                early += [functools.partial(shift_job, jn, (k % 4) * TQ + (k // 4) * 16, 16)
                          for k in range(TB // 16)]
            early = iter(early)

            pend = []
            tick = [0]

            def drain(m):
                tick[0] += 1
                if pend and tick[0] >= U_AT[0] and (tick[0] - U_AT[0]) % U_AT[1] == 0:
                    pend.pop(0)(m)

            def up_prod(n, g):
                m = _dot(d_lhs(2, n), _up(t3_s[g, :, _ct(n)]))
                if n in E_AT:
                    job = next(early, None)
                    if job is not None:
                        job(anchor=m)
                drain(m)
                return m

            def uset_job(tile, g, n1, r0, n, anchor=None):
                blk = _outer_operand(lambda i, k: tile(i, k, r0, n), _LHS_TERMS[n1])
                blk[0] = after(blk[0], anchor)
                blk[3] = after(blk[3], anchor)
                for n2, v in enumerate(_lhs_set(*blk)):
                    ref, rows = u_set(7 * n1 + n2)
                    ref[rows.start + r0 // 2:rows.start + (r0 + n) // 2, _ct(g)] = _pk(v)

            for g in range(NFG):
                c = _strassen2(lambda n: up_prod(n, g), 1)
                assert not pend
                tick[0] = 0
                if last and g == NFG - 1:
                    act = [[_gelu(c(i, k)) for k in range(4)] for i in range(4)]
                    for n1 in range(7):
                        uset_job(lambda i, k, r0, n: act[i][k], g, n1, 0, TQ)
                    continue
                c0 = 4 * (g % 2)
                for i in range(4):
                    for k in range(4):
                        act_s[i * TQ:(i + 1) * TQ, _ct(c0 + k)] = _gelu(c(i, k))

                def tile(i, k, r0, n, c0=c0):
                    return act_s[i * TQ + r0:i * TQ + r0 + n, _ct(c0 + k)]

                pend += [functools.partial(uset_job, tile, g, n1, r0, 16)
                         for n1 in range(7) for r0 in range(0, TQ, 16)]
            jobs = {}
            if not last:
                mix(j + 1, drain)
                assert not pend
                prev = []
                for k in range(TB // 16):
                    jobs[k * Y_AT] = functools.partial(ln_job, (k % 4) * TQ + (k // 4) * 16, 16, prev)

                def place(start, fns):
                    for fn in fns:
                        while start in jobs:
                            start += 1
                        jobs[start] = fn

                for rt in range(2):
                    place(S_AT[rt], [functools.partial(set_job, yn_s, 2, rt, ct, n1, 16)
                                     for ct in range(2) for n1 in range(7)])
                place(G_AT, [functools.partial(set_job, gs_s, 3, rt, ct, n1, 16)
                             for rt in range(2) for ct in range(2) for n1 in range(7)])

            def down_part(n, og, k0, k1):
                ref, rows = u_set(n)
                return _dot(_up(ref[rows, k0 * E:k1 * E]),
                            _up(t4_s[og, k0 * E // 2:k1 * E // 2, _ct(n)]))

            head = {}
            if last:
                head = {n: down_part(n, 0, 0, NFG - 1) for n in range(HEAD)}
            count = [0]

            def down_prod(n, og):
                if og == 0 and n in head:
                    return down_part(n, og, NFG - 1, NFG) + head[n]
                m = down_part(n, og, 0, NFG)
                job = jobs.get(count[0])
                count[0] += 1
                if job is not None:
                    job(anchor=m)
                return m

            for og in range(NOG):
                c = _strassen2(lambda n: down_prod(n, og))
                for i in range(4):
                    rows = slice(i * TQ, (i + 1) * TQ)
                    for k in range(2):
                        c0 = (4 * og + 2 * k) * E
                        o_s.at[slot][rows, c0:c0 + 2 * E] = (
                            base_s[rows, c0:c0 + 2 * E] + mod_rows(5, TQ, c0, 2 * E)
                            * jnp.concatenate([c(i, 2 * k), c(i, 2 * k + 1)], axis=1)).astype(bf16)
            out_copy(j, slot).start()

        def p3_body(j, carry):
            @pl.when(j >= 2)
            def _():
                out_copy(j - 2, j & 1).wait()

            mlp_block(j, False)
            return carry

        lax.fori_loop(0, NB - 1, _scoped("p3", p3_body), 0)
        for k in range(2):
            for cp in mlp_w_copies(0, k):
                cp.wait()
        out_copy(NB - 3, (NB - 3) % 2).wait()
        mlp_block(NB - 1, True)
        out_copy(NB - 2, (NB - 2) % 2).wait()
        out_copy(NB - 1, (NB - 1) % 2).wait()

    pl.run_scoped(
        phase_a,
        pltpu.VMEM((NSEG, M, D), bf16),
        pltpu.VMEM((7, NSEG * M // 4, D // 2), u32),
        pltpu.VMEM((3 * D // E, D, E), bf16),
        pltpu.VMEM((2, D, HG, E), bf16),
        pltpu.VMEM((2, BGR, D), bf16),
        pltpu.VMEM((2, 2, G1R, D), bf16),
        pltpu.VMEM((NC + 1, D // 4, 5 * HG // 2 * E), u32),
    )
    pl.run_scoped(
        phase_b,
        pltpu.VMEM((NOG, D // 8, 49 * E), u32),
        pltpu.VMEM((NFG, D // 8, 49 * E), u32),
        pltpu.VMEM((NOG, F // 8, 49 * E), u32),
        pltpu.VMEM((D // E, D, E), bf16),
        pltpu.VMEM((TB, D), f32),
        pltpu.VMEM((TB, D), f32),
        pltpu.VMEM((TB, D), f32),
        pltpu.VMEM((TB, D), f32),
        pltpu.VMEM((TB, D), f32),
        pltpu.VMEM((2, TB, D), bf16),
    )


@jax.jit
def pallas_adaLN_cond__memory_aug_recurrent_mem_tr__mixer_s_mlp__prompt_kernel(
    A_x: jax.Array,
    A_mem0: jax.Array,
    A_Wq: jax.Array,
    A_Wk: jax.Array,
    A_Wv: jax.Array,
    A_Wo: jax.Array,
    A_seg_len,
    B_x: jax.Array,
    B_w1: jax.Array,
    B_w2: jax.Array,
    B_w3: jax.Array,
    B_w4: jax.Array,
    c: jax.Array,
    w_mod: jax.Array,
):
    del A_seg_len, B_x
    assert A_x.shape == (1, S, D) and A_mem0.shape == (1, M, D)
    hbm = pl.BlockSpec(memory_space=pl.ANY)
    scratch = [
        pltpu.VMEM((NSEG, SEG, D), bf16),
        pltpu.VMEM((NC + 1, D // 2, HG * E), u32),
        pltpu.VMEM((H * E // 2, D), u32),
        pltpu.VMEM((7, D // 4, D // 2), u32),
        pltpu.VMEM((2, 4, 16, 4 * E), bf16),
        pltpu.VMEM((2, 4, 64, 4 * E), bf16),
        pltpu.VMEM((2, 4, 32, D), bf16),
        pltpu.VMEM((NC, NSEG * M, HG // 2 * E), u32),
        pltpu.VMEM((8, 6 * D), f32),
        pltpu.VMEM((M, D), f32),
        pltpu.VMEM((TC, D), f32),
        pltpu.VMEM((2 * SEG, D), f32),
        pltpu.VMEM((E, E), f32),
        pltpu.VMEM((S, D), bf16),
        pltpu.VMEM((S + 16, D), f32),
        pltpu.VMEM((7 * SEG // 2, D // 2), u32),
        pltpu.VMEM((16, E), u32),
        pltpu.VMEM((1, D), bf16),
        pltpu.VMEM((M, D), bf16),
        pltpu.SemaphoreType.DMA((24,)),
    ]
    out = pl.pallas_call(
        _kernel,
        out_shape=jax.ShapeDtypeStruct((S, D), bf16),
        in_specs=[hbm] * 12,
        out_specs=hbm,
        scratch_shapes=scratch,
        compiler_params=pltpu.CompilerParams(vmem_limit_bytes=127 * 1024 * 1024,
                                             disable_bounds_checks=NO_CHECKS,
                                             disable_semaphore_checks=NO_CHECKS),
    )(A_x.reshape(NSEG, SEG, D), A_mem0.reshape(M, D), A_Wq, A_Wk, A_Wv,
      A_Wo.reshape(H * E, D), B_w1.reshape(2, D // 2, D), B_w2.reshape(4, D // 4, D), B_w3.reshape(4, D // 4, F),
      B_w4.reshape(NFG, 4, E, D), c, w_mod)
    return out.reshape(1, S, D)
```

```python
import functools

import jax
import jax.numpy as jnp
from jax import lax
import jax.experimental.pallas as pl
import jax.experimental.pallas.tpu as pltpu

bf16, f32, u32 = jnp.bfloat16, jnp.float32, jnp.uint32

S, D, H, E, M, SEG, F = 2048, 1024, 32, 128, 8, 32, 3584
EPS = 1e-5
SCALE = E ** -0.5
NSEG = S // SEG
NI = NSEG // 2
NP = H // 2
NR = 2 * (M + SEG)
TC = SEG - M
HG = 8
HH = HG // 2
NG = H // HG
NC = 3 * NG
BGR = 384
G1R = 48
X0 = 4
TB = 128
NB = S // TB
HD = D // 2
NQ = D // E // 2
NFG = F // (4 * E)
NOG = D // (4 * E)

PIN_ROWS = 256
P1_LAG, P1_TAIL, P1_PIN, P1_FROM = 4, 5, 48, 46
PREP_AT = (0, 1, 4, 5)
T_AT = (7, 28, 52)
E_AT = (10, 24, 34)
U_AT = (6, 3)
Y_AT, S_AT, G_AT = 4, (26, 44), 62
HEAD = 14
NO_CHECKS = True
_SCOPES = False


def _scoped(name, fn):
    def wrapped(*a):
        if not _SCOPES:
            return fn(*a)
        with jax.named_scope(name):
            return fn(*a)
    return wrapped


def _pk(x):
    return pltpu.bitcast(x.astype(bf16), u32)


def _up(x):
    return pltpu.bitcast(x, bf16)


def _ct(k):
    return slice(k * E, (k + 1) * E)


def _dot(a, b):
    return jnp.dot(a, b, preferred_element_type=f32)


def _ln(x):
    m = jnp.mean(x, axis=-1, keepdims=True)
    xc = x - m
    v = jnp.mean(xc * xc, axis=-1, keepdims=True)
    return xc * lax.rsqrt(v + EPS)


def _gelu(x):
    c = 0.7978845608028654
    return 0.5 * x * (1.0 + jnp.tanh(c * (x + 0.044715 * (x * x * x))))


def _lhs_set(a11, a12, a21, a22):
    return (a11 + a22, a21 + a22, a11, a22, a11 + a12, a21 - a11, a12 - a22)


def _rhs_set(b11, b12, b21, b22):
    return (b11 + b22, b11, b12 - b22, b21 - b11, b22, b11 + b12, b21 + b22)


_LHS_TERMS = (((0, 1), (3, 1)), ((2, 1), (3, 1)), ((0, 1),), ((3, 1),),
              ((0, 1), (1, 1)), ((2, 1), (0, -1)), ((1, 1), (3, -1)))
_RHS_TERMS = (((0, 1), (3, 1)), ((0, 1),), ((1, 1), (3, -1)), ((2, 1), (0, -1)),
              ((3, 1),), ((0, 1), (1, 1)), ((2, 1), (3, 1)))


def _outer_operand(tile, terms):
    out = []
    for i in range(2):
        for j in range(2):
            v = None
            for o, sign in terms:
                t = tile(2 * (o // 2) + i, 2 * (o % 2) + j)
                v = t if v is None else (v + t if sign > 0 else v - t)
            out.append(v)
    return out


class _Quad:
    def __init__(self, tiles):
        self.t = tuple(tiles)

    def __add__(self, other):
        return _Quad([a + b for a, b in zip(self.t, other.t)])

    def __sub__(self, other):
        return _Quad([a - b for a, b in zip(self.t, other.t)])


def _strassen2(m, order=0):
    cs = _strassen(lambda n1: _Quad(_strassen(lambda n2: m(7 * n1 + n2))), order)
    return lambda i, j: cs[2 * (i // 2) + j // 2].t[2 * (i % 2) + j % 2]


def _strassen(m, order=0):
    if order == 0:
        m1 = m(0)
        m2 = m(1)
        c22 = m1 - m2
        m3 = m(2)
        c22 = c22 + m3
        c22 = m(5) + c22
        m4 = m(3)
        c21 = m2 + m4
        c11 = m1 + m4
        m5 = m(4)
        c12 = m3 + m5
        c11 = c11 - m5
        c11 = m(6) + c11
    else:
        m2 = m(1)
        c22 = m(5) - m2
        m4 = m(3)
        c21 = m2 + m4
        m1 = m(0)
        c22 = c22 + m1
        c11 = m4 + m1
        m3 = m(2)
        c22 = c22 + m3
        m5 = m(4)
        c12 = m3 + m5
        c11 = c11 - m5
        c11 = m(6) + c11
    return c11, c12, c21, c22


def _mask_fill():
    shape = (NR, E)
    r = lax.broadcasted_iota(jnp.int32, shape, 0)
    c = lax.broadcasted_iota(jnp.int32, shape, 1)

    def headpos(i):
        head = jnp.where(i < 64, i >> 5, (i - 64) >> 3)
        pos = jnp.where(i < 64, i & 31, 32 + (i & 7))
        return head, pos

    hr, pr = headpos(r)
    hc, pc = headpos(c)
    same = hr == hc
    valid = same & ((pr < M) | (pr >= pc))
    return jnp.where(valid, 0.0, jnp.where(same, -1e9, -jnp.inf)).astype(f32)


def _kernel(x_hbm, mem0_hbm, wq_hbm, wk_hbm, wv_hbm, wo_hbm, w1_hbm, w2_hbm, w3_hbm,
            w4_hbm, c_hbm, wm_hbm,
            out_hbm,
            x_s, w_s, wo_s, t1_s, g2, g3, g4, pre_s, mod_s, mem_s, hn_s, aout_s, fill_s,
            hb_s, t_s, l1_s, zero_s, c_s, mem0_s, sems):
    w_hbm = (wq_hbm, wk_hbm, wv_hbm)

    (SEM_C, SEM_MEM, SEM_XPRE, SEM_X, SEM_WMR, SEM_BG, SEM_OUT, SEM_G1,
     SEM_G2, SEM_G3, SEM_G4, SEM_WM, SEM_STG) = (0, 1, 2, 3, 4, 6, 8, 10, 12, 14, 16, 18, 22)

    def copy(src, dst, k):
        return pltpu.make_async_copy(src, dst, sems.at[k])

    def aligned(x, n):
        return x if isinstance(x, int) else pl.multiple_of(x, n)

    def clamp(k, hi):
        return min(k, hi) if isinstance(k, int) else jnp.minimum(k, hi)

    def mlp_piece(k):
        k = clamp(k, 4 * NFG - 1)
        return k >> 2, k & 3

    def mlp_w_copies(k, slot):
        g, rr = mlp_piece(k)
        k2 = clamp(k, NI - 1)
        return (copy(w2_hbm.at[:, pl.ds(aligned((k2 >> 1) * 16, 16), 16),
                               pl.ds(aligned((k2 & 1) * 4 * E, E), 4 * E)], g2.at[slot], SEM_G2 + slot),
                copy(w3_hbm.at[:, pl.ds(aligned(rr * 64, 64), 64), pl.ds(aligned(g * 4 * E, E), 4 * E)],
                     g3.at[slot], SEM_G3 + slot),
                copy(w4_hbm.at[g, :, pl.ds(aligned(rr * 32, 32), 32), :], g4.at[slot], SEM_G4 + slot))

    def pinned(w, job):
        if job is None:
            return w()
        z = job() & zero_s[0:8, :]
        w = w()
        return jnp.concatenate([w[0:8] | z, w[8:]], axis=0)

    def after(x, anchor):
        if anchor is None:
            return x
        z = pltpu.bitcast(pltpu.bitcast(anchor[0:8], u32) & zero_s[0:8, :], f32)
        z = jnp.concatenate([z] * (x.shape[0] // 8), axis=0)
        return jnp.concatenate([x[:, 0:E] + z, x[:, E:]], axis=1) if x.shape[1] > E else x + z

    def rhs_job(src, slot, r0, q, dst, row, z):
        blk = [src[slot, kh, r0:r0 + 16, _ct(cc)].astype(f32)
               for kh in range(2) for cc in (q, NQ + q)]
        zf = pltpu.bitcast(jnp.concatenate([z, z], axis=0), f32)
        blk[0] = blk[0] + zf
        blk[3] = blk[3] + zf
        for n, v in enumerate(_rhs_set(*blk)):
            dst.at[n][pl.ds(pl.multiple_of(row, 8), 8), _ct(q)] = _pk(v)

    def rhs2_job(src, slot, r0, c0, n1, dst, row):
        blk = _outer_operand(lambda i, j: src[slot, i, r0:r0 + 16, _ct(c0 + j)].astype(f32),
                             _RHS_TERMS[n1])
        sets = _rhs_set(*blk)
        for n2, v in enumerate(sets):
            dst[pl.ds(pl.multiple_of(row, 8), 8), _ct(7 * n1 + n2)] = _pk(v)
        out = pltpu.bitcast(sets[2], u32) | pltpu.bitcast(sets[3], u32)
        return out[0:8] | out[8:16]

    def silu_c():
        cf = c_s[...].astype(f32)
        return jnp.broadcast_to(cf * (1.0 / (1.0 + jnp.exp(-cf))), (8, D)).astype(bf16)

    def wm_copy(wm_s, src_tile, dst_tile, sem):
        return copy(wm_hbm.at[:, pl.ds(aligned(src_tile * E, E), E)], wm_s.at[dst_tile], sem)

    def wm_wait(wm_s, t0, n, sem):
        copy(wm_s.at[t0:t0 + n], wm_s.at[t0:t0 + n], sem).wait()

    def mod_tiles(wm_s, t0, n, dst_tile):
        sc8 = silu_c()
        for k in range(n):
            v = _dot(sc8, wm_s[t0 + k])
            if (dst_tile + k) // (D // E) in (1, 4):
                v = 1.0 + v
            mod_s[:, _ct(dst_tile + k)] = v

    def x_copy(k):
        r = slice(0, X0) if k == 0 else slice(X0, NSEG)
        return copy(x_hbm.at[r], x_s.at[r], SEM_XPRE if k == 0 else SEM_X)

    def h_rows(s):
        return _ln(x_s[s, 0:TC, :].astype(f32)) * mod_rows(1, TC) + mod_rows(0, TC)

    def mod_rows(k, n, c0=0, w=D):
        return jnp.concatenate([mod_s[:, k * D + c0:k * D + c0 + w]] * (n // 8), axis=0)

    def phase_a(xpre_s, hpre_s, wm_s, stg, bg, g1, tq_s):
        def tq_place(c, n):
            if n == 1:
                return w_s.at[c], 0, None
            if n == 4:
                return w_s.at[c], D // 4, None
            return tq_s.at[c], 0, (0, 2, 3, 5, 6).index(n) * (HG // 2)

        def w_copy(t, g, slot, hf):
            return copy(w_hbm[t].at[:, pl.ds(aligned(g * HH, HH), HH), :], stg.at[slot, hf],
                        SEM_STG + 2 * slot + hf)

        def bg_rows(k):
            return clamp(k * BGR, H * E - BGR), clamp(k * G1R, HD - G1R)

        def bg_copies(k, slot):
            ro, r1 = bg_rows(k)
            return (copy(wo_hbm.at[pl.ds(aligned(ro, 16), BGR)], bg.at[slot], SEM_BG + slot),
                    copy(w1_hbm.at[:, pl.ds(aligned(r1, 16), G1R), :], g1.at[slot], SEM_G1 + slot))

        def relayout_jobs(slot, hf, c, j0, i):
            memo = []
            r = aligned(i * 8, 8)

            def job(jj, z=None):
                if not memo:
                    for d0 in (i * 16, HD + i * 16):
                        memo.append(jnp.swapaxes(pltpu.bitcast(stg[slot, hf, pl.ds(d0, 16)], u32), 0, 1))
                j = j0 + jj
                blk = []
                for kh in range(2):
                    u = memo[kh][jj]
                    if z is not None:
                        u = u | jnp.concatenate([z, z], axis=0)
                    blk.append(pltpu.bitcast(u << 16, f32))
                    blk.append(pltpu.bitcast(u & jnp.uint32(0xFFFF0000), f32))
                for k, v in enumerate(blk):
                    w_s.at[c][pl.ds((k // 2) * (D // 4) + r, 8), _ct(2 * j + k % 2)] = _pk(v)
                sets = _rhs_set(*blk)
                for n, v in enumerate(sets):
                    if n not in (1, 4):
                        ref, r0, c0 = tq_place(c, n)
                        ref[pl.ds(r0 + r, 8), _ct(c0 + j)] = _pk(v)
                out = pltpu.bitcast(sets[2], u32) | pltpu.bitcast(sets[3], u32)
                return out[0:8] | out[8:16]

            return [functools.partial(job, jj) for jj in range(2)]

        def repack(slot, row, i, z):
            v = pltpu.bitcast(bg[slot, 16 * i:16 * i + 16, :], u32)
            v = v | jnp.concatenate([z] * (D // E), axis=1)
            wo_s[pl.ds(pl.multiple_of(row + 8 * i, 8), 8), :] = v

        cp_c = copy(c_hbm, c_s, SEM_C)
        cp_mem = copy(mem0_hbm, mem0_s, SEM_MEM)
        cp_xpre = copy(x_hbm.at[:, TC:SEG, :], xpre_s, SEM_XPRE)
        w_copy(0, 0, 0, 1).start()
        cp_xpre.start()
        cp_c.start()
        cp_mem.start()
        for k in range(2 * D // E):
            wm_copy(wm_s, k, k, SEM_WM + k // 4).start()
        w_copy(0, 1, 1, 0).start()
        w_copy(0, 2, 1, 1).start()

        zero_s[0:8, :] = jnp.zeros((8, E), u32)
        fill_s[0:NR, :] = _mask_fill()
        aout_s[...] = jnp.zeros(aout_s.shape, f32)
        l1_s[...] = jnp.zeros(l1_s.shape, u32)
        bg[1] = jnp.zeros(bg.shape[1:], bf16)
        g1[1] = jnp.zeros(g1.shape[1:], bf16)

        w_copy(0, 0, 0, 1).wait()

        def rl0_body(i, carry):
            for job in relayout_jobs(0, 1, 0, 0, i):
                job()
            return carry

        lax.fori_loop(0, D // 32, rl0_body, 0)
        w_copy(0, 3, 0, 0).start()
        w_copy(0, 4, 0, 1).start()
        for cp in bg_copies(0, 0):
            cp.start()

        cp_xpre.wait()

        def npre_body(i, carry):
            xr = xpre_s[pl.ds(pl.multiple_of(i * 8, 8), 8)].astype(f32).reshape(64, D)
            t_s[pl.ds(pl.multiple_of(i * 64, 64), 64), :] = _ln(xr)
            return carry

        lax.fori_loop(0, NSEG // 8, _scoped("npre", npre_body), 0)

        cp_c.wait()
        cp_mem.wait()
        mem_s[...] = mem0_s[...].astype(f32)

        for k in range(4):
            wm_wait(wm_s, 4 * k, 4, SEM_WM + k)
            mod_tiles(wm_s, 4 * k, 4, 4 * k)

        PH = NSEG * M // 2

        def hpre_body(i, carry):
            h = [t_s[pl.ds(pl.multiple_of(hf * PH + i * 16, 16), 16), :] * mod_rows(1, 16) + mod_rows(0, 16)
                 for hf in range(2)]
            for n, v in enumerate(_lhs_set(h[0][:, :HD], h[0][:, HD:], h[1][:, :HD], h[1][:, HD:])):
                hpre_s.at[n][pl.ds(pl.multiple_of(i * 8, 8), 8), :] = _pk(v)
            return carry

        lax.fori_loop(0, PH // 16, _scoped("hpre", hpre_body), 0)

        t_s[0:8, :] = jnp.zeros((8, D), f32)
        t_s[S + 8:S + 16, :] = jnp.zeros((8, D), f32)

        MB = 64

        def p1_body(c, carry):
            slot = c & 1
            pslot = 1 - slot
            ro, r1 = bg_rows(jnp.maximum(c - 1, 0))

            @pl.when(c >= 1)
            def _():
                for cp in bg_copies(0, pslot):
                    cp.wait()

            w_copy(0, 0, pslot, 0).wait()

            @pl.when(c + 1 < NC)
            def _():
                w_copy(0, 0, pslot, 1).wait()

            small = [functools.partial(repack, pslot, ro >> 1, i) for i in range(BGR // 16)]
            small += [functools.partial(rhs_job, g1, pslot, 16 * rt, q, t1_s, (r1 >> 1) + 8 * rt)
                      for rt in range(G1R // 16) for q in range(NQ)]
            nu = D // 32
            npin = 7 * (HG // 2) * (PH // MB)
            first = [job for i in range(nu) for job in relayout_jobs(pslot, 0, c, 2, i)]
            pins = [[] for _ in range(npin)]
            for k, job in enumerate(first):
                pins[1 + k * (P1_PIN - 1) // len(first)].append(job)
            pins = iter(pins)
            work = []
            for i in range(nu):
                work += relayout_jobs(pslot, 1, c + 1, 0, i)
                work += small[i * len(small) // nu:(i + 1) * len(small) // nu]
            jobs = [[] for _ in range(npin)]
            for k, job in enumerate(work):
                pos = P1_FROM * 8 + k * (npin - P1_TAIL - P1_FROM) * 8 // len(work)
                jobs[pos // 8].append((job, pos % 8))
            jobs = iter(jobs)

            def run(group):
                z = group[0]()
                for job in group[1:]:
                    z = z | job()
                return z

            def prod(n, q, mb):
                ref, r0, c0 = tq_place(c, n)
                group = next(pins)
                w = pinned(lambda: ref[r0:r0 + D // 4, _ct(2 * q + (n == 4) if c0 is None else c0 + q)],
                           functools.partial(run, group) if group else None)
                m = _dot(_up(hpre_s[n, mb * MB // 2:(mb + 1) * MB // 2, :]), _up(w))
                pending.append(m)
                if len(pending) > P1_LAG:
                    anchor = pltpu.bitcast(pending.pop(0), u32)
                    for job, g in next(jobs):
                        job(anchor[8 * g:8 * g + 8] & zero_s[0:8, :])
                return m

            pending = []
            ns = MB // M
            for q in range(HG // 2):
                for mb in range(PH // MB):
                    cs = _strassen(lambda n: prod(n, q, mb))
                    for hf in range(2):
                        y = jnp.concatenate([cs[2 * hf + k][sg * M:(sg + 1) * M]
                                             for sg in range(ns) for k in range(2)], axis=0)
                        s0 = hf * (NSEG // 2) + mb * ns
                        pre_s.at[c][s0 * M:(s0 + ns) * M, _ct(q)] = _pk(y)

            for hf in range(2):
                h = 2 * c + 5 + hf
                for t in range(3):
                    @pl.when(h >> 3 == t)
                    def _():
                        w_copy(t, h & 7, pslot, hf).start()

            @pl.when(c + 2 < NC)
            def _():
                for cp in bg_copies(c + 1, pslot):
                    cp.start()

            @pl.when(c < NC - 3)
            def _():
                wm_copy(wm_s, 2 * D // E + c, c, SEM_WMR).start()

            @pl.when(c == NC - 3)
            def _():
                def issue(k, carry2):
                    wm_copy(wm_s, 2 * D // E + k, k, SEM_WMR).start()
                    return carry2

                x_copy(0).start()
                lax.fori_loop(NC - 3, 3 * D // E, issue, 0)
                for k in range(2):
                    for cp in mlp_w_copies(k, k):
                        cp.start()

            return carry

        lax.fori_loop(0, NC, _scoped("p1", p1_body), 0)
        x_copy(1).start()
        x_copy(0).wait()
        wm_wait(wm_s, 0, 3 * D // E, SEM_WMR)
        mod_tiles(wm_s, 0, 3 * D // E, 2 * D // E)
        hn_s[...] = after(h_rows(0), pltpu.bitcast(tq_s[NC, 0:8, 0:E], f32))

    def phase_b(t2_s, t3_s, t4_s, wg_s, x1_s, base_s, yn_s, gs_s, act_s, o_s):
        for k in range(D // E):
            wm_copy(wg_s, 5 * D // E + k, k, SEM_WM).start()

        def chain_step(s, mem, htok, odef_prev, jobs=(), hooks=None):
            hs = jnp.concatenate([mem, htok], axis=0).astype(bf16)
            qkv = [[None] * 3 for _ in range(NP)]
            ps = [None] * NP
            os_ = [None] * H
            odef = [None] * H

            def proj(p, t):
                c, q = t * NG + p // (HG // 2), p % (HG // 2)
                a = _dot(hs, _up(w_s[c, :, _ct(2 * q)]))
                b = _dot(hs, _up(w_s[c, :, _ct(2 * q + 1)]))
                pre = pre_s[c, pl.ds(pl.multiple_of(s * M, M), M), _ct(q)]
                parts = [a, b, _up(pre).astype(f32)]
                if t > 0:
                    parts.append(jnp.zeros((E - NR, E), f32))
                v = jnp.concatenate(parts, axis=0)
                qkv[p][t] = (v.T if t == 1 else v).astype(bf16)

            def scores(p):
                sc_ = _dot(qkv[p][0], qkv[p][1])
                fill = fill_s[0:NR, :]
                sc_ = jnp.where(fill == 0.0, sc_ * SCALE, fill)
                m = jnp.max(sc_, axis=-1, keepdims=True)
                e = jnp.exp(sc_ - m)
                l = jnp.sum(e, axis=-1, keepdims=True)
                r = pl.reciprocal(l, approx=True)
                r = r * (2.0 - l * r)
                ps[p] = (e * r).astype(bf16)

            def fin(p):
                o = _dot(ps[p], qkv[p][2])
                for hh in range(2):
                    h = 2 * p + hh
                    rows = o[32 * hh:32 * hh + 32]
                    odef[h] = o[64 + 8 * hh:72 + 8 * hh]
                    if odef_prev is not None:
                        rows = jnp.concatenate([rows, odef_prev[h], odef[h]], axis=0)
                    os_[h] = _pk(rows)

            acc = [None] * 8
            jobs = iter(jobs)

            def wo(h0, h1, js):
                lhs = _up(jnp.concatenate(os_[h0:h1], axis=1))
                for j in js:
                    ws = []
                    for r0 in range(h0 * E // 2, h1 * E // 2, PIN_ROWS):
                        ws.append(pinned(lambda: wo_s[r0:r0 + PIN_ROWS, j * E:(j + 1) * E],
                                         next(jobs, None)))
                    part = _dot(lhs, _up(jnp.concatenate(ws, axis=0)))
                    if hooks and acc[j] is None and j in hooks:
                        hooks[j](part)
                    acc[j] = part if acc[j] is None else part + acc[j]

            for p in range(NP):
                attn = [functools.partial(scores, p - 1) if p >= 1 else None,
                        functools.partial(fin, p - 3) if p >= 3 else None]
                if odef_prev is not None:
                    attn.reverse()
                for t, f in zip((1, 0, 2), attn + [None]):
                    proj(p, t)
                    if f is not None:
                        f()
            hsplit = 24
            wo(0, hsplit, range(0, 2))
            scores(NP - 1)
            fin(NP - 3)
            wo(0, hsplit, range(2, 3))
            fin(NP - 2)
            wo(0, hsplit, range(3, 5))
            fin(NP - 1)
            wo(0, hsplit, range(5, 8))
            wo(hsplit, H, range(8))
            return jnp.concatenate(acc, axis=1), odef

        def mixer_prep(i, r0, n, anchor=None):
            r = pl.ds(aligned(i * 64 + r0, 16), n)
            xr = x_s[2 * i + r0 // SEG, r0 % SEG:r0 % SEG + n, :].astype(f32)
            x2 = xr + mod_rows(2, n) * after(aout_s[r0:r0 + n, :], anchor)
            x_s.at[2 * i + r0 // SEG][r0 % SEG:r0 % SEG + n, :] = x2.astype(bf16)
            hb = _ln(x2) * mod_rows(4, n) + mod_rows(3, n)
            hb_s[r, :] = hb.astype(bf16)
            return _ln(hb)

        def mixer_sets(ya, yb, r0, dst=l1_s):
            n = ya.shape[0]
            for m, v in enumerate(_lhs_set(ya[:, :HD], ya[:, HD:], yb[:, :HD], yb[:, HD:])):
                dst[m * (SEG // 2) + r0 // 2:m * (SEG // 2) + (r0 + n) // 2, 0:HD] = _pk(v)

        def mixer_mm(i, src=l1_s, hook=None):
            for q in range(NQ):
                def prod(n):
                    m = _dot(_up(src[n * (SEG // 2):(n + 1) * (SEG // 2), 0:HD]),
                             _up(t1_s[n, :, _ct(q)]))
                    if hook is not None:
                        hook(m)
                    return m

                cs = _strassen(prod)
                for k, cc in enumerate(cs):
                    r0 = aligned(i * 64 + 8 + (k // 2) * SEG, 8)
                    t_s[pl.ds(r0, SEG), _ct(q + NQ * (k % 2))] = _gelu(cc)

        def p2_body(i, carry):
            slot = i & 1
            for cp in mlp_w_copies(0, slot):
                cp.wait()

            @pl.when(i == 1)
            def _():
                x_copy(1).wait()

            g, rr = mlp_piece(i)
            work = [functools.partial(rhs2_job, g2, slot, 0, 0, n1, t2_s.at[slot], (i >> 1) * 8)
                    for n1 in range(7)]
            work += [functools.partial(rhs2_job, g3, slot, 16 * rt, 0, n1, t3_s.at[g], rr * 32 + 8 * rt)
                     for rt in range(4) for n1 in range(7)]
            work += [functools.partial(rhs2_job, g4, slot, 16 * rt, 4 * og, n1, t4_s.at[og],
                                       g * (E // 2) + rr * 16 + 8 * rt)
                     for rt in range(2) for og in range(NOG) for n1 in range(7)]
            jobs = [None] + work

            sa_ = 2 * i
            sb_ = 2 * i + 1
            hb_tok = h_rows(sb_)
            oa, odef_a = chain_step(sa_, mem_s[...], hn_s[...], None)
            mixer_mm(jnp.maximum(i - 2, 0))
            ys = []

            def hook(k, anchor):
                if k >= 2:
                    anchor = anchor[0:8] + ys[-2][0:8, 0:E] + ys[-2][8:16, 0:E]
                ys.append(mixer_prep(jnp.maximum(i - 1, 0), (k % 2) * SEG + (k // 2) * 16, 16, anchor))
                if k % 2:
                    mixer_sets(ys[-2], ys[-1], (k // 2) * 16)

            hooks = {j: functools.partial(hook, k) for k, j in enumerate(PREP_AT)}
            ob, _ = chain_step(sb_, oa[0:M], hb_tok, odef_a, jobs, hooks)
            mem_s[...] = ob[0:M]
            aout_s[0:TC, :] = oa[M:SEG]
            aout_s[TC:SEG, :] = ob[SEG:SEG + M]
            aout_s[SEG:SEG + TC, :] = ob[M:SEG]
            aout_s[SEG + TC:2 * SEG, :] = ob[SEG + M:SEG + 2 * M]
            hn_s[...] = h_rows(jnp.minimum(sb_ + 1, NSEG - 1))
            for cp in mlp_w_copies(i + 2, slot):
                cp.start()
            return carry

        lax.fori_loop(0, NI, _scoped("p2", p2_body), 0)

        TQ = TB // 4
        SHIFT = (-1, -1, 1, 1, -2, -2, 2, 2)

        def u_set(n):
            return w_s.at[n // 32], slice((n % 32) * (TQ // 2), (n % 32 + 1) * (TQ // 2))

        def d_set(slot, n):
            return w_s.at[slot], (n // 4) * (TQ // 2), (n % 4) * 2

        def d_lhs(slot, n):
            ref, r0, c0 = d_set(slot, n)
            return _up(ref[r0:r0 + TQ // 2, c0 * E:(c0 + 2) * E])

        def shift_job(j, r0, n, anchor=None):
            for ct in range(D // E):
                win = t_s[pl.ds(aligned(j * TB + r0, 16), n + 16), _ct(ct)]
                gs_s[r0:r0 + n, _ct(ct)] = after(
                    pltpu.roll(win, (-SHIFT[ct]) % (n + 16), 0)[8:8 + n], anchor)

        def mix(j, hook=None):
            r0 = aligned(j * TB, TB)
            for og in range(NOG):
                def prod(n):
                    m = _dot(d_lhs(3, n), _up(t2_s[og, :, _ct(n)]))
                    if hook is not None:
                        hook(m)
                    return m

                c = _strassen2(prod)
                for i in range(4):
                    for k in range(2):
                        cols = slice((4 * og + 2 * k) * E, (4 * og + 2 * k + 2) * E)
                        x1_s[i * TQ:(i + 1) * TQ, cols] = (
                            hb_s[pl.ds(r0 + i * TQ, TQ), cols].astype(f32)
                            + jnp.concatenate([c(i, 2 * k), c(i, 2 * k + 1)], axis=1))

        def base_job(j, rt, anchor):
            rows = slice(rt * 16, (rt + 1) * 16)
            z = pltpu.bitcast(pltpu.bitcast(anchor[0:8], u32) & zero_s[0:8, :], f32)
            gb = mod_rows(5, 8) + jnp.concatenate([z] * (D // E), axis=1)
            x2 = x_s[j * (TB // SEG) + rt // 2, (rt % 2) * 16:(rt % 2) * 16 + 16, :]
            base_s[rows, :] = x2.astype(f32) + jnp.concatenate([gb, gb], axis=0) * x1_s[rows, :]

        def out_copy(j, slot):
            return copy(o_s.at[slot], out_hbm.at[pl.ds(aligned(j * TB, TB), TB)], SEM_OUT + slot)

        def ln_job(r0, n, prev, anchor=None):
            if anchor is not None and len(prev) >= 2:
                anchor = anchor[0:8] + prev[-2]
            y = _ln(after(x1_s[r0:r0 + n, :], anchor))
            yn_s[r0:r0 + n, :] = y
            prev.append(y[0:8, 0:E] + y[8:16, 0:E])

        def set_job(src, slot, rt, ct, n1, n=16, anchor=None):
            blk = _outer_operand(lambda i, k: src[i * TQ + rt * n:i * TQ + (rt + 1) * n, _ct(2 * k + ct)],
                                 _LHS_TERMS[n1])
            blk[0] = after(blk[0], anchor)
            blk[3] = after(blk[3], anchor)
            for n2, v in enumerate(_lhs_set(*blk)):
                ref, r0, c0 = d_set(slot, 7 * n1 + n2)
                ref[r0 + rt * n // 2:r0 + (rt + 1) * n // 2, _ct(c0 + ct)] = _pk(v)

        def all_sets(src, slot):
            for n1 in range(7):
                for ct in range(2):
                    set_job(src, slot, 0, ct, n1, TQ)

        wm_wait(wg_s, 0, D // E, SEM_WM)
        mod_tiles(wg_s, 0, D // E, 5 * D // E)
        shift_job(0, 0, TB)
        all_sets(gs_s, 3)
        mix(0)
        prev0 = []
        plan = {}
        for k in range(TB // 16):
            plan[T_AT[0] * (k // 2) + k % 2] = [
                functools.partial(ln_job, (k % 4) * TQ + (k // 4) * 16, 16, prev0)]
        rest = [functools.partial(shift_job, 1, (k % 4) * TQ + (k // 4) * 16, 16)
                for k in range(TB // 16)]
        rest += [functools.partial(set_job, gs_s, 3, rt, ct, n1, 16)
                 for rt in range(2) for ct in range(2) for n1 in range(7)]
        for k, job in enumerate(rest):
            plan.setdefault(k * T_AT[1] // len(rest), []).append(job)
        rest = [functools.partial(set_job, yn_s, 2, rt, ct, n1, 16)
                for rt in range(2) for ct in range(2) for n1 in range(7)]
        for k, job in enumerate(rest):
            plan.setdefault(T_AT[1] + k * (T_AT[2] - T_AT[1]) // len(rest), []).append(job)
        tick0 = [0]

        def hook0(m):
            for job in plan.pop(tick0[0], ()):
                job(anchor=m)
            tick0[0] += 1

        mixer_mm(NI - 2, hook=hook0)
        mixer_sets(mixer_prep(NI - 1, 0, SEG), mixer_prep(NI - 1, SEG, SEG), 0, w_s.at[4])
        mixer_mm(NI - 1, w_s.at[4], hook0)
        assert not plan

        def mlp_block(j, last):
            slot = j & 1

            jn = clamp(j + 2, NB - 1)
            early = [functools.partial(base_job, j, k) for k in range(TB // 16)]
            if not last:
                early += [functools.partial(shift_job, jn, (k % 4) * TQ + (k // 4) * 16, 16)
                          for k in range(TB // 16)]
            early = iter(early)

            pend = []
            tick = [0]

            def drain(m):
                tick[0] += 1
                if pend and tick[0] >= U_AT[0] and (tick[0] - U_AT[0]) % U_AT[1] == 0:
                    pend.pop(0)(m)

            def up_prod(n, g):
                m = _dot(d_lhs(2, n), _up(t3_s[g, :, _ct(n)]))
                if n in E_AT:
                    job = next(early, None)
                    if job is not None:
                        job(anchor=m)
                drain(m)
                return m

            def uset_job(tile, g, n1, r0, n, anchor=None):
                blk = _outer_operand(lambda i, k: tile(i, k, r0, n), _LHS_TERMS[n1])
                blk[0] = after(blk[0], anchor)
                blk[3] = after(blk[3], anchor)
                for n2, v in enumerate(_lhs_set(*blk)):
                    ref, rows = u_set(7 * n1 + n2)
                    ref[rows.start + r0 // 2:rows.start + (r0 + n) // 2, _ct(g)] = _pk(v)

            for g in range(NFG):
                c = _strassen2(lambda n: up_prod(n, g), 1)
                assert not pend
                tick[0] = 0
                if last and g == NFG - 1:
                    act = [[_gelu(c(i, k)) for k in range(4)] for i in range(4)]
                    for n1 in range(7):
                        uset_job(lambda i, k, r0, n: act[i][k], g, n1, 0, TQ)
                    continue
                c0 = 4 * (g % 2)
                for i in range(4):
                    for k in range(4):
                        act_s[i * TQ:(i + 1) * TQ, _ct(c0 + k)] = _gelu(c(i, k))

                def tile(i, k, r0, n, c0=c0):
                    return act_s[i * TQ + r0:i * TQ + r0 + n, _ct(c0 + k)]

                pend += [functools.partial(uset_job, tile, g, n1, r0, 16)
                         for n1 in range(7) for r0 in range(0, TQ, 16)]
            jobs = {}
            if not last:
                mix(j + 1, drain)
                assert not pend
                prev = []
                for k in range(TB // 16):
                    jobs[k * Y_AT] = functools.partial(ln_job, (k % 4) * TQ + (k // 4) * 16, 16, prev)

                def place(start, fns):
                    for fn in fns:
                        while start in jobs:
                            start += 1
                        jobs[start] = fn

                for rt in range(2):
                    place(S_AT[rt], [functools.partial(set_job, yn_s, 2, rt, ct, n1, 16)
                                     for ct in range(2) for n1 in range(7)])
                place(G_AT, [functools.partial(set_job, gs_s, 3, rt, ct, n1, 16)
                             for rt in range(2) for ct in range(2) for n1 in range(7)])

            def down_part(n, og, k0, k1):
                ref, rows = u_set(n)
                return _dot(_up(ref[rows, k0 * E:k1 * E]),
                            _up(t4_s[og, k0 * E // 2:k1 * E // 2, _ct(n)]))

            head = {}
            if last:
                head = {n: down_part(n, 0, 0, NFG - 1) for n in range(HEAD)}
            count = [0]

            def down_prod(n, og):
                if og == 0 and n in head:
                    return down_part(n, og, NFG - 1, NFG) + head[n]
                m = down_part(n, og, 0, NFG)
                job = jobs.get(count[0])
                count[0] += 1
                if job is not None:
                    job(anchor=m)
                return m

            for og in range(NOG):
                c = _strassen2(lambda n: down_prod(n, og))
                for i in range(4):
                    rows = slice(i * TQ, (i + 1) * TQ)
                    for k in range(2):
                        c0 = (4 * og + 2 * k) * E
                        o_s.at[slot][rows, c0:c0 + 2 * E] = (
                            base_s[rows, c0:c0 + 2 * E] + mod_rows(5, TQ, c0, 2 * E)
                            * jnp.concatenate([c(i, 2 * k), c(i, 2 * k + 1)], axis=1)).astype(bf16)
            out_copy(j, slot).start()

        def p3_body(j, carry):
            @pl.when(j >= 2)
            def _():
                out_copy(j - 2, j & 1).wait()

            mlp_block(j, False)
            return carry

        lax.fori_loop(0, NB - 1, _scoped("p3", p3_body), 0)
        for k in range(2):
            for cp in mlp_w_copies(0, k):
                cp.wait()
        out_copy(NB - 3, (NB - 3) % 2).wait()
        mlp_block(NB - 1, True)
        out_copy(NB - 2, (NB - 2) % 2).wait()
        out_copy(NB - 1, (NB - 1) % 2).wait()

    pl.run_scoped(
        phase_a,
        pltpu.VMEM((NSEG, M, D), bf16),
        pltpu.VMEM((7, NSEG * M // 4, D // 2), u32),
        pltpu.VMEM((3 * D // E, D, E), bf16),
        pltpu.VMEM((2, 2, D, HH, E), bf16),
        pltpu.VMEM((2, BGR, D), bf16),
        pltpu.VMEM((2, 2, G1R, D), bf16),
        pltpu.VMEM((NC + 1, D // 4, 5 * HG // 2 * E), u32),
    )
    pl.run_scoped(
        phase_b,
        pltpu.VMEM((NOG, D // 8, 49 * E), u32),
        pltpu.VMEM((NFG, D // 8, 49 * E), u32),
        pltpu.VMEM((NOG, F // 8, 49 * E), u32),
        pltpu.VMEM((D // E, D, E), bf16),
        pltpu.VMEM((TB, D), f32),
        pltpu.VMEM((TB, D), f32),
        pltpu.VMEM((TB, D), f32),
        pltpu.VMEM((TB, D), f32),
        pltpu.VMEM((TB, D), f32),
        pltpu.VMEM((2, TB, D), bf16),
    )


@jax.jit
def pallas_adaLN_cond__memory_aug_recurrent_mem_tr__mixer_s_mlp__prompt_kernel(
    A_x: jax.Array,
    A_mem0: jax.Array,
    A_Wq: jax.Array,
    A_Wk: jax.Array,
    A_Wv: jax.Array,
    A_Wo: jax.Array,
    A_seg_len,
    B_x: jax.Array,
    B_w1: jax.Array,
    B_w2: jax.Array,
    B_w3: jax.Array,
    B_w4: jax.Array,
    c: jax.Array,
    w_mod: jax.Array,
):
    del A_seg_len, B_x
    assert A_x.shape == (1, S, D) and A_mem0.shape == (1, M, D)
    hbm = pl.BlockSpec(memory_space=pl.ANY)
    scratch = [
        pltpu.VMEM((NSEG, SEG, D), bf16),
        pltpu.VMEM((NC + 1, D // 2, HG * E), u32),
        pltpu.VMEM((H * E // 2, D), u32),
        pltpu.VMEM((7, D // 4, D // 2), u32),
        pltpu.VMEM((2, 4, 16, 4 * E), bf16),
        pltpu.VMEM((2, 4, 64, 4 * E), bf16),
        pltpu.VMEM((2, 4, 32, D), bf16),
        pltpu.VMEM((NC, NSEG * M, HG // 2 * E), u32),
        pltpu.VMEM((8, 6 * D), f32),
        pltpu.VMEM((M, D), f32),
        pltpu.VMEM((TC, D), f32),
        pltpu.VMEM((2 * SEG, D), f32),
        pltpu.VMEM((E, E), f32),
        pltpu.VMEM((S, D), bf16),
        pltpu.VMEM((S + 16, D), f32),
        pltpu.VMEM((7 * SEG // 2, D // 2), u32),
        pltpu.VMEM((16, E), u32),
        pltpu.VMEM((1, D), bf16),
        pltpu.VMEM((M, D), bf16),
        pltpu.SemaphoreType.DMA((26,)),
    ]
    out = pl.pallas_call(
        _kernel,
        out_shape=jax.ShapeDtypeStruct((S, D), bf16),
        in_specs=[hbm] * 12,
        out_specs=hbm,
        scratch_shapes=scratch,
        compiler_params=pltpu.CompilerParams(vmem_limit_bytes=127 * 1024 * 1024,
                                             disable_bounds_checks=NO_CHECKS,
                                             disable_semaphore_checks=NO_CHECKS),
    )(A_x.reshape(NSEG, SEG, D), A_mem0.reshape(M, D), A_Wq, A_Wk, A_Wv,
      A_Wo.reshape(H * E, D), B_w1.reshape(2, D // 2, D), B_w2.reshape(4, D // 4, D), B_w3.reshape(4, D // 4, F),
      B_w4.reshape(NFG, 4, E, D), c, w_mod)
    return out.reshape(1, S, D)
```

```python
import functools

import jax
import jax.numpy as jnp
from jax import lax
import jax.experimental.pallas as pl
import jax.experimental.pallas.tpu as pltpu

bf16, f32, u32 = jnp.bfloat16, jnp.float32, jnp.uint32

S, D, H, E, M, SEG, F = 2048, 1024, 32, 128, 8, 32, 3584
EPS = 1e-5
SCALE = E ** -0.5
NSEG = S // SEG
NI = NSEG // 2
NP = H // 2
NR = 2 * (M + SEG)
TC = SEG - M
HG = 8
HH = HG // 2
NG = H // HG
NC = 3 * NG
BGR = 384
G1R = 48
X0 = 4
TB = 128
NB = S // TB
HD = D // 2
NQ = D // E // 2
NFG = F // (4 * E)
NOG = D // (4 * E)

PIN_ROWS = 256
P1_LAG, P1_TAIL, P1_PIN, P1_FROM = 4, 5, 48, 46
PREP_AT = (0, 1, 4, 5)
T_AT = (7, 28, 52)
E_AT = (10, 24, 34)
U_AT = (6, 3)
Y_AT, S_AT, G_AT = 4, (26, 44), 62
HEAD = 14
NO_CHECKS = True
_SCOPES = False


def _scoped(name, fn):
    def wrapped(*a):
        if not _SCOPES:
            return fn(*a)
        with jax.named_scope(name):
            return fn(*a)
    return wrapped


def _pk(x):
    return pltpu.bitcast(x.astype(bf16), u32)


def _up(x):
    return pltpu.bitcast(x, bf16)


def _ct(k):
    return slice(k * E, (k + 1) * E)


def _dot(a, b):
    return jnp.dot(a, b, preferred_element_type=f32)


def _ln(x):
    m = jnp.mean(x, axis=-1, keepdims=True)
    xc = x - m
    v = jnp.mean(xc * xc, axis=-1, keepdims=True)
    return xc * lax.rsqrt(v + EPS)


def _gelu(x):
    c = 0.7978845608028654
    return 0.5 * x * (1.0 + jnp.tanh(c * (x + 0.044715 * (x * x * x))))


def _lhs_set(a11, a12, a21, a22):
    return (a11 + a22, a21 + a22, a11, a22, a11 + a12, a21 - a11, a12 - a22)


def _rhs_set(b11, b12, b21, b22):
    return (b11 + b22, b11, b12 - b22, b21 - b11, b22, b11 + b12, b21 + b22)


_LHS_TERMS = (((0, 1), (3, 1)), ((2, 1), (3, 1)), ((0, 1),), ((3, 1),),
              ((0, 1), (1, 1)), ((2, 1), (0, -1)), ((1, 1), (3, -1)))
_RHS_TERMS = (((0, 1), (3, 1)), ((0, 1),), ((1, 1), (3, -1)), ((2, 1), (0, -1)),
              ((3, 1),), ((0, 1), (1, 1)), ((2, 1), (3, 1)))


def _outer_operand(tile, terms):
    out = []
    for i in range(2):
        for j in range(2):
            v = None
            for o, sign in terms:
                t = tile(2 * (o // 2) + i, 2 * (o % 2) + j)
                v = t if v is None else (v + t if sign > 0 else v - t)
            out.append(v)
    return out


class _Quad:
    def __init__(self, tiles):
        self.t = tuple(tiles)

    def __add__(self, other):
        return _Quad([a + b for a, b in zip(self.t, other.t)])

    def __sub__(self, other):
        return _Quad([a - b for a, b in zip(self.t, other.t)])


def _strassen2(m, order=0):
    cs = _strassen(lambda n1: _Quad(_strassen(lambda n2: m(7 * n1 + n2))), order)
    return lambda i, j: cs[2 * (i // 2) + j // 2].t[2 * (i % 2) + j % 2]


def _strassen(m, order=0):
    if order == 0:
        m1 = m(0)
        m2 = m(1)
        c22 = m1 - m2
        m3 = m(2)
        c22 = c22 + m3
        c22 = m(5) + c22
        m4 = m(3)
        c21 = m2 + m4
        c11 = m1 + m4
        m5 = m(4)
        c12 = m3 + m5
        c11 = c11 - m5
        c11 = m(6) + c11
    else:
        m2 = m(1)
        c22 = m(5) - m2
        m4 = m(3)
        c21 = m2 + m4
        m1 = m(0)
        c22 = c22 + m1
        c11 = m4 + m1
        m3 = m(2)
        c22 = c22 + m3
        m5 = m(4)
        c12 = m3 + m5
        c11 = c11 - m5
        c11 = m(6) + c11
    return c11, c12, c21, c22


def _mask_fill():
    shape = (NR, E)
    r = lax.broadcasted_iota(jnp.int32, shape, 0)
    c = lax.broadcasted_iota(jnp.int32, shape, 1)

    def headpos(i):
        head = jnp.where(i < 64, i >> 5, (i - 64) >> 3)
        pos = jnp.where(i < 64, i & 31, 32 + (i & 7))
        return head, pos

    hr, pr = headpos(r)
    hc, pc = headpos(c)
    same = hr == hc
    valid = same & ((pr < M) | (pr >= pc))
    return jnp.where(valid, 0.0, jnp.where(same, -1e9, -jnp.inf)).astype(f32)


def _kernel(x_hbm, mem0_hbm, wq_hbm, wk_hbm, wv_hbm, wo_hbm, w1_hbm, w2_hbm, w3_hbm,
            w4_hbm, c_hbm, wm_hbm,
            out_hbm,
            x_s, w_s, wo_s, t1_s, g2, g3, g4, pre_s, mod_s, mem_s, hn_s, aout_s, fill_s,
            hb_s, t_s, l1_s, zero_s, c_s, mem0_s, sems):
    w_hbm = (wq_hbm, wk_hbm, wv_hbm)

    (SEM_C, SEM_MEM, SEM_XPRE, SEM_X, SEM_WMR, SEM_BG, SEM_OUT, SEM_G1,
     SEM_G2, SEM_G3, SEM_G4, SEM_WM, SEM_STG) = (0, 1, 2, 3, 4, 6, 8, 10, 12, 14, 16, 18, 22)

    def copy(src, dst, k):
        return pltpu.make_async_copy(src, dst, sems.at[k])

    def aligned(x, n):
        return x if isinstance(x, int) else pl.multiple_of(x, n)

    def clamp(k, hi):
        return min(k, hi) if isinstance(k, int) else jnp.minimum(k, hi)

    def mlp_piece(k):
        k = clamp(k, 4 * NFG - 1)
        return k >> 2, k & 3

    def mlp_w_copies(k, slot):
        g, rr = mlp_piece(k)
        k2 = clamp(k, NI - 1)
        return (copy(w2_hbm.at[:, pl.ds(aligned((k2 >> 1) * 16, 16), 16),
                               pl.ds(aligned((k2 & 1) * 4 * E, E), 4 * E)], g2.at[slot], SEM_G2 + slot),
                copy(w3_hbm.at[:, pl.ds(aligned(rr * 64, 64), 64), pl.ds(aligned(g * 4 * E, E), 4 * E)],
                     g3.at[slot], SEM_G3 + slot),
                copy(w4_hbm.at[g, :, pl.ds(aligned(rr * 32, 32), 32), :], g4.at[slot], SEM_G4 + slot))

    def pinned(w, job):
        if job is None:
            return w()
        z = job() & zero_s[0:8, :]
        w = w()
        return jnp.concatenate([w[0:8] | z, w[8:]], axis=0)

    def after(x, anchor):
        if anchor is None:
            return x
        z = pltpu.bitcast(pltpu.bitcast(anchor[0:8], u32) & zero_s[0:8, :], f32)
        z = jnp.concatenate([z] * (x.shape[0] // 8), axis=0)
        return jnp.concatenate([x[:, 0:E] + z, x[:, E:]], axis=1) if x.shape[1] > E else x + z

    def rhs_job(src, slot, r0, q, dst, row, z):
        blk = [src[slot, kh, r0:r0 + 16, _ct(cc)].astype(f32)
               for kh in range(2) for cc in (q, NQ + q)]
        zf = pltpu.bitcast(jnp.concatenate([z, z], axis=0), f32)
        blk[0] = blk[0] + zf
        blk[3] = blk[3] + zf
        for n, v in enumerate(_rhs_set(*blk)):
            dst.at[n][pl.ds(aligned(row, 8), 8), _ct(q)] = _pk(v)

    def rhs2_job(src, slot, r0, c0, n1, dst, row):
        blk = _outer_operand(lambda i, j: src[slot, i, r0:r0 + 16, _ct(c0 + j)].astype(f32),
                             _RHS_TERMS[n1])
        sets = _rhs_set(*blk)
        for n2, v in enumerate(sets):
            dst[pl.ds(pl.multiple_of(row, 8), 8), _ct(7 * n1 + n2)] = _pk(v)
        out = pltpu.bitcast(sets[2], u32) | pltpu.bitcast(sets[3], u32)
        return out[0:8] | out[8:16]

    def silu_c():
        cf = c_s[...].astype(f32)
        return jnp.broadcast_to(cf * (1.0 / (1.0 + jnp.exp(-cf))), (8, D)).astype(bf16)

    def wm_copy(wm_s, src_tile, dst_tile, sem):
        return copy(wm_hbm.at[:, pl.ds(aligned(src_tile * E, E), E)], wm_s.at[dst_tile], sem)

    def wm_wait(wm_s, t0, n, sem):
        copy(wm_s.at[t0:t0 + n], wm_s.at[t0:t0 + n], sem).wait()

    def mod_tiles(wm_s, t0, n, dst_tile):
        sc8 = silu_c()
        for k in range(n):
            v = _dot(sc8, wm_s[t0 + k])
            if (dst_tile + k) // (D // E) in (1, 4):
                v = 1.0 + v
            mod_s[:, _ct(dst_tile + k)] = v

    def x_copy(k):
        r = slice(0, X0) if k == 0 else slice(X0, NSEG)
        return copy(x_hbm.at[r], x_s.at[r], SEM_XPRE if k == 0 else SEM_X)

    def h_rows(s):
        return _ln(x_s[s, 0:TC, :].astype(f32)) * mod_rows(1, TC) + mod_rows(0, TC)

    def mod_rows(k, n, c0=0, w=D):
        return jnp.concatenate([mod_s[:, k * D + c0:k * D + c0 + w]] * (n // 8), axis=0)

    def phase_a(xpre_s, hpre_s, wm_s, stg, bg, g1, tq_s):
        def tq_place(c, n):
            if n == 1:
                return w_s.at[c], 0, None
            if n == 4:
                return w_s.at[c], D // 4, None
            return tq_s.at[c], 0, (0, 2, 3, 5, 6).index(n) * (HG // 2)

        def w_copy(t, g, slot, hf):
            return copy(w_hbm[t].at[:, pl.ds(aligned(g * HH, HH), HH), :], stg.at[slot, hf],
                        SEM_STG + 2 * slot + hf)

        def bg_rows(k):
            return clamp(k * BGR, H * E - BGR), clamp(k * G1R, HD - G1R)

        def bg_copies(k, slot):
            ro, r1 = bg_rows(k)
            return (copy(wo_hbm.at[pl.ds(aligned(ro, 16), BGR)], bg.at[slot], SEM_BG + slot),
                    copy(w1_hbm.at[:, pl.ds(aligned(r1, 16), G1R), :], g1.at[slot], SEM_G1 + slot))

        def relayout_jobs(slot, hf, c, j0, i):
            memo = []
            r = aligned(i * 8, 8)

            def job(jj, z=None):
                if not memo:
                    for d0 in (i * 16, HD + i * 16):
                        memo.append(jnp.swapaxes(pltpu.bitcast(stg[slot, hf, pl.ds(d0, 16)], u32), 0, 1))
                j = j0 + jj
                blk = []
                for kh in range(2):
                    u = memo[kh][jj]
                    if z is not None:
                        u = u | jnp.concatenate([z, z], axis=0)
                    blk.append(pltpu.bitcast(u << 16, f32))
                    blk.append(pltpu.bitcast(u & jnp.uint32(0xFFFF0000), f32))
                for k, v in enumerate(blk):
                    w_s.at[c][pl.ds((k // 2) * (D // 4) + r, 8), _ct(2 * j + k % 2)] = _pk(v)
                sets = _rhs_set(*blk)
                for n, v in enumerate(sets):
                    if n not in (1, 4):
                        ref, r0, c0 = tq_place(c, n)
                        ref[pl.ds(r0 + r, 8), _ct(c0 + j)] = _pk(v)
                out = pltpu.bitcast(sets[2], u32) | pltpu.bitcast(sets[3], u32)
                return out[0:8] | out[8:16]

            return [functools.partial(job, jj) for jj in range(2)]

        def repack(slot, row, i, z):
            v = pltpu.bitcast(bg[slot, 16 * i:16 * i + 16, :], u32)
            v = v | jnp.concatenate([z] * (D // E), axis=1)
            wo_s[pl.ds(aligned(row + 8 * i, 8), 8), :] = v

        cp_c = copy(c_hbm, c_s, SEM_C)
        cp_mem = copy(mem0_hbm, mem0_s, SEM_MEM)
        cp_xpre = copy(x_hbm.at[:, TC:SEG, :], xpre_s, SEM_XPRE)
        w_copy(0, 0, 0, 0).start()
        cp_xpre.start()
        cp_c.start()
        cp_mem.start()
        for k in range(2 * D // E):
            wm_copy(wm_s, k, k, SEM_WM + k // 4).start()
        w_copy(0, 1, 0, 1).start()
        w_copy(0, 2, 1, 0).start()
        w_copy(0, 3, 1, 1).start()

        zero_s[0:8, :] = jnp.zeros((8, E), u32)
        fill_s[0:NR, :] = _mask_fill()
        aout_s[...] = jnp.zeros(aout_s.shape, f32)
        l1_s[...] = jnp.zeros(l1_s.shape, u32)
        bg[1] = jnp.zeros(bg.shape[1:], bf16)
        g1[1] = jnp.zeros(g1.shape[1:], bf16)

        w_copy(0, 0, 0, 0).wait()

        def rl0_body(i, carry):
            for job in relayout_jobs(0, 0, 0, 0, i):
                job()
            return carry

        lax.fori_loop(0, D // 32, rl0_body, 0)
        cp_xpre.wait()

        def npre_body(i, carry):
            xr = xpre_s[pl.ds(pl.multiple_of(i * 8, 8), 8)].astype(f32).reshape(64, D)
            t_s[pl.ds(pl.multiple_of(i * 64, 64), 64), :] = _ln(xr)
            return carry

        lax.fori_loop(0, NSEG // 8, _scoped("npre", npre_body), 0)

        cp_c.wait()
        cp_mem.wait()
        mem_s[...] = mem0_s[...].astype(f32)

        for k in range(4):
            wm_wait(wm_s, 4 * k, 4, SEM_WM + k)
            mod_tiles(wm_s, 4 * k, 4, 4 * k)

        PH = NSEG * M // 2

        def hpre_body(i, carry):
            h = [t_s[pl.ds(pl.multiple_of(hf * PH + i * 16, 16), 16), :] * mod_rows(1, 16) + mod_rows(0, 16)
                 for hf in range(2)]
            for n, v in enumerate(_lhs_set(h[0][:, :HD], h[0][:, HD:], h[1][:, :HD], h[1][:, HD:])):
                hpre_s.at[n][pl.ds(pl.multiple_of(i * 8, 8), 8), :] = _pk(v)
            return carry

        lax.fori_loop(0, PH // 16, _scoped("hpre", hpre_body), 0)

        t_s[0:8, :] = jnp.zeros((8, D), f32)
        t_s[S + 8:S + 16, :] = jnp.zeros((8, D), f32)

        MB = 64

        nu = D // 32

        def small_jobs(slot, k):
            ro, r1 = bg_rows(k)
            return ([functools.partial(repack, slot, ro >> 1, i) for i in range(BGR // 16)]
                    + [functools.partial(rhs_job, g1, slot, 16 * rt, q, t1_s, (r1 >> 1) + 8 * rt)
                       for rt in range(G1R // 16) for q in range(NQ)])

        def p1_pairs(pairs, first, work, start, extra=None):
            npin = 7 * len(pairs) * (PH // MB)
            pins = [[] for _ in range(npin)]
            for k, job in enumerate(first):
                pins[1 + k * (P1_PIN - 1) // len(first)].append(job)
            pins = iter(pins)
            jobs = [[] for _ in range(npin)]
            for k, job in enumerate(work):
                pos = start * 8 + k * (npin - P1_TAIL - start) * 8 // len(work)
                jobs[pos // 8].append((job, pos % 8))
            jobs = iter(jobs)
            pending = []

            def run(group):
                z = group[0]()
                for job in group[1:]:
                    z = z | job()
                return z

            def prod(n, c, q, mb):
                ref, r0, c0 = tq_place(c, n)
                group = next(pins)
                w = pinned(lambda: ref[r0:r0 + D // 4, _ct(2 * q + (n == 4) if c0 is None else c0 + q)],
                           functools.partial(run, group) if group else None)
                m = _dot(_up(hpre_s[n, mb * MB // 2:(mb + 1) * MB // 2, :]), _up(w))
                pending.append(m)
                if len(pending) > P1_LAG:
                    anchor = pltpu.bitcast(pending.pop(0), u32)
                    for job, g in next(jobs):
                        job(anchor[8 * g:8 * g + 8] & zero_s[0:8, :])
                if extra is not None:
                    extra()
                return m

            ns = MB // M
            for c, q in pairs:
                for mb in range(PH // MB):
                    cs = _strassen(lambda n: prod(n, c, q, mb))
                    for hf in range(2):
                        y = jnp.concatenate([cs[2 * hf + k][sg * M:(sg + 1) * M]
                                             for sg in range(ns) for k in range(2)], axis=0)
                        s0 = hf * (NSEG // 2) + mb * ns
                        pre_s.at[c][s0 * M:(s0 + ns) * M, _ct(q)] = _pk(y)

        w_copy(0, 0, 0, 1).wait()
        p1_pairs([(0, 0), (0, 1)], [], [job for i in range(nu) for job in relayout_jobs(0, 1, 0, 2, i)], 0)
        for hf in range(2):
            w_copy(0, 4 + hf, 0, hf).start()
        for cp in bg_copies(0, 0):
            cp.start()

        def wm_rest(k):
            for kk in (k, k + 1):
                wm_copy(wm_s, 2 * D // E + kk, kk, SEM_WMR).start()

        wm_rest(0)

        def p1_body(c, carry):
            pslot = 1 - (c & 1)

            @pl.when(c >= 1)
            def _():
                for cp in bg_copies(0, pslot):
                    cp.wait()

            for hf in range(2):
                w_copy(0, 0, pslot, hf).wait()

            small = small_jobs(pslot, jnp.maximum(c - 1, 0))
            work = []
            for i in range(nu):
                work += relayout_jobs(pslot, 1, c + 1, 2, i)
                work += small[i * len(small) // nu:(i + 1) * len(small) // nu]
            p1_pairs([(c, 2), (c, 3), (c + 1, 0), (c + 1, 1)],
                     [job for i in range(nu) for job in relayout_jobs(pslot, 0, c + 1, 0, i)],
                     work, P1_FROM)

            for t in range(3):
                @pl.when((c + 3) >> 2 == t)
                def _():
                    for hf in range(2):
                        w_copy(t, 2 * ((c + 3) & 3) + hf, pslot, hf).start()

            @pl.when(c + 2 < NC)
            def _():
                for cp in bg_copies(c + 1, pslot):
                    cp.start()
                wm_rest(2 * c + 2)

            @pl.when(c == NC - 3)
            def _():
                wm_rest(2 * NC - 2)
                x_copy(0).start()

            return carry

        lax.fori_loop(0, NC - 1, _scoped("p1", p1_body), 0)
        for k in range(2):
            for cp in mlp_w_copies(k, k):
                cp.start()
        x_copy(1).start()
        for cp in bg_copies(0, NC & 1):
            cp.wait()
        x_copy(0).wait()
        wm_wait(wm_s, 0, 3 * D // E, SEM_WMR)

        sc8 = silu_c()
        halves = iter(range(2 * 3 * D // E))
        part = []

        def mod_half():
            k = next(halves, None)
            if k is None:
                return
            rows = slice((k % 2) * HD, (k % 2 + 1) * HD)
            v = _dot(sc8[:, rows], wm_s[k // 2, rows, :])
            if k % 2 == 0:
                part.append(v)
            else:
                v = v + part.pop()
                tile = 2 * D // E + k // 2
                mod_s[:, _ct(tile)] = 1.0 + v if tile // (D // E) == 4 else v

        p1_pairs([(NC - 1, 2), (NC - 1, 3)], [], small_jobs(NC & 1, NC - 2), 0, mod_half)
        hn_s[...] = h_rows(0)

    def phase_b(t2_s, t3_s, t4_s, wg_s, x1_s, base_s, yn_s, gs_s, act_s, o_s):
        for k in range(D // E):
            wm_copy(wg_s, 5 * D // E + k, k, SEM_WM).start()

        def chain_step(s, mem, htok, odef_prev, jobs=(), hooks=None):
            hs = jnp.concatenate([mem, htok], axis=0).astype(bf16)
            qkv = [[None] * 3 for _ in range(NP)]
            ps = [None] * NP
            os_ = [None] * H
            odef = [None] * H

            def proj(p, t):
                c, q = t * NG + p // (HG // 2), p % (HG // 2)
                a = _dot(hs, _up(w_s[c, :, _ct(2 * q)]))
                b = _dot(hs, _up(w_s[c, :, _ct(2 * q + 1)]))
                pre = pre_s[c, pl.ds(pl.multiple_of(s * M, M), M), _ct(q)]
                parts = [a, b, _up(pre).astype(f32)]
                if t > 0:
                    parts.append(jnp.zeros((E - NR, E), f32))
                v = jnp.concatenate(parts, axis=0)
                qkv[p][t] = (v.T if t == 1 else v).astype(bf16)

            def scores(p):
                sc_ = _dot(qkv[p][0], qkv[p][1])
                fill = fill_s[0:NR, :]
                sc_ = jnp.where(fill == 0.0, sc_ * SCALE, fill)
                m = jnp.max(sc_, axis=-1, keepdims=True)
                e = jnp.exp(sc_ - m)
                l = jnp.sum(e, axis=-1, keepdims=True)
                r = pl.reciprocal(l, approx=True)
                r = r * (2.0 - l * r)
                ps[p] = (e * r).astype(bf16)

            def fin(p):
                o = _dot(ps[p], qkv[p][2])
                for hh in range(2):
                    h = 2 * p + hh
                    rows = o[32 * hh:32 * hh + 32]
                    odef[h] = o[64 + 8 * hh:72 + 8 * hh]
                    if odef_prev is not None:
                        rows = jnp.concatenate([rows, odef_prev[h], odef[h]], axis=0)
                    os_[h] = _pk(rows)

            acc = [None] * 8
            jobs = iter(jobs)

            def wo(h0, h1, js):
                lhs = _up(jnp.concatenate(os_[h0:h1], axis=1))
                for j in js:
                    ws = []
                    for r0 in range(h0 * E // 2, h1 * E // 2, PIN_ROWS):
                        ws.append(pinned(lambda: wo_s[r0:r0 + PIN_ROWS, j * E:(j + 1) * E],
                                         next(jobs, None)))
                    part = _dot(lhs, _up(jnp.concatenate(ws, axis=0)))
                    if hooks and acc[j] is None and j in hooks:
                        hooks[j](part)
                    acc[j] = part if acc[j] is None else part + acc[j]

            for p in range(NP):
                attn = [functools.partial(scores, p - 1) if p >= 1 else None,
                        functools.partial(fin, p - 3) if p >= 3 else None]
                if odef_prev is not None:
                    attn.reverse()
                for t, f in zip((1, 0, 2), attn + [None]):
                    proj(p, t)
                    if f is not None:
                        f()
            hsplit = 24
            wo(0, hsplit, range(0, 2))
            scores(NP - 1)
            fin(NP - 3)
            wo(0, hsplit, range(2, 3))
            fin(NP - 2)
            wo(0, hsplit, range(3, 5))
            fin(NP - 1)
            wo(0, hsplit, range(5, 8))
            wo(hsplit, H, range(8))
            return jnp.concatenate(acc, axis=1), odef

        def mixer_prep(i, r0, n, anchor=None):
            r = pl.ds(aligned(i * 64 + r0, 16), n)
            xr = x_s[2 * i + r0 // SEG, r0 % SEG:r0 % SEG + n, :].astype(f32)
            x2 = xr + mod_rows(2, n) * after(aout_s[r0:r0 + n, :], anchor)
            x_s.at[2 * i + r0 // SEG][r0 % SEG:r0 % SEG + n, :] = x2.astype(bf16)
            hb = _ln(x2) * mod_rows(4, n) + mod_rows(3, n)
            hb_s[r, :] = hb.astype(bf16)
            return _ln(hb)

        def mixer_sets(ya, yb, r0, dst=l1_s):
            n = ya.shape[0]
            for m, v in enumerate(_lhs_set(ya[:, :HD], ya[:, HD:], yb[:, :HD], yb[:, HD:])):
                dst[m * (SEG // 2) + r0 // 2:m * (SEG // 2) + (r0 + n) // 2, 0:HD] = _pk(v)

        def mixer_mm(i, src=l1_s, hook=None):
            for q in range(NQ):
                def prod(n):
                    m = _dot(_up(src[n * (SEG // 2):(n + 1) * (SEG // 2), 0:HD]),
                             _up(t1_s[n, :, _ct(q)]))
                    if hook is not None:
                        hook(m)
                    return m

                cs = _strassen(prod)
                for k, cc in enumerate(cs):
                    r0 = aligned(i * 64 + 8 + (k // 2) * SEG, 8)
                    t_s[pl.ds(r0, SEG), _ct(q + NQ * (k % 2))] = _gelu(cc)

        def p2_body(i, carry):
            slot = i & 1
            for cp in mlp_w_copies(0, slot):
                cp.wait()

            @pl.when(i == 1)
            def _():
                x_copy(1).wait()

            g, rr = mlp_piece(i)
            work = [functools.partial(rhs2_job, g2, slot, 0, 0, n1, t2_s.at[slot], (i >> 1) * 8)
                    for n1 in range(7)]
            work += [functools.partial(rhs2_job, g3, slot, 16 * rt, 0, n1, t3_s.at[g], rr * 32 + 8 * rt)
                     for rt in range(4) for n1 in range(7)]
            work += [functools.partial(rhs2_job, g4, slot, 16 * rt, 4 * og, n1, t4_s.at[og],
                                       g * (E // 2) + rr * 16 + 8 * rt)
                     for rt in range(2) for og in range(NOG) for n1 in range(7)]
            jobs = [None] + work

            sa_ = 2 * i
            sb_ = 2 * i + 1
            hb_tok = h_rows(sb_)
            oa, odef_a = chain_step(sa_, mem_s[...], hn_s[...], None)
            mixer_mm(jnp.maximum(i - 2, 0))
            ys = []

            def hook(k, anchor):
                if k >= 2:
                    anchor = anchor[0:8] + ys[-2][0:8, 0:E] + ys[-2][8:16, 0:E]
                ys.append(mixer_prep(jnp.maximum(i - 1, 0), (k % 2) * SEG + (k // 2) * 16, 16, anchor))
                if k % 2:
                    mixer_sets(ys[-2], ys[-1], (k // 2) * 16)

            hooks = {j: functools.partial(hook, k) for k, j in enumerate(PREP_AT)}
            ob, _ = chain_step(sb_, oa[0:M], hb_tok, odef_a, jobs, hooks)
            mem_s[...] = ob[0:M]
            aout_s[0:TC, :] = oa[M:SEG]
            aout_s[TC:SEG, :] = ob[SEG:SEG + M]
            aout_s[SEG:SEG + TC, :] = ob[M:SEG]
            aout_s[SEG + TC:2 * SEG, :] = ob[SEG + M:SEG + 2 * M]
            hn_s[...] = h_rows(jnp.minimum(sb_ + 1, NSEG - 1))
            for cp in mlp_w_copies(i + 2, slot):
                cp.start()
            return carry

        lax.fori_loop(0, NI, _scoped("p2", p2_body), 0)

        TQ = TB // 4
        SHIFT = (-1, -1, 1, 1, -2, -2, 2, 2)

        def u_set(n):
            return w_s.at[n // 32], slice((n % 32) * (TQ // 2), (n % 32 + 1) * (TQ // 2))

        def d_set(slot, n):
            return w_s.at[slot], (n // 4) * (TQ // 2), (n % 4) * 2

        def d_lhs(slot, n):
            ref, r0, c0 = d_set(slot, n)
            return _up(ref[r0:r0 + TQ // 2, c0 * E:(c0 + 2) * E])

        def shift_job(j, r0, n, anchor=None):
            for ct in range(D // E):
                win = t_s[pl.ds(aligned(j * TB + r0, 16), n + 16), _ct(ct)]
                gs_s[r0:r0 + n, _ct(ct)] = after(
                    pltpu.roll(win, (-SHIFT[ct]) % (n + 16), 0)[8:8 + n], anchor)

        def mix(j, hook=None):
            r0 = aligned(j * TB, TB)
            for og in range(NOG):
                def prod(n):
                    m = _dot(d_lhs(3, n), _up(t2_s[og, :, _ct(n)]))
                    if hook is not None:
                        hook(m)
                    return m

                c = _strassen2(prod)
                for i in range(4):
                    for k in range(2):
                        cols = slice((4 * og + 2 * k) * E, (4 * og + 2 * k + 2) * E)
                        x1_s[i * TQ:(i + 1) * TQ, cols] = (
                            hb_s[pl.ds(r0 + i * TQ, TQ), cols].astype(f32)
                            + jnp.concatenate([c(i, 2 * k), c(i, 2 * k + 1)], axis=1))

        def base_job(j, rt, anchor):
            rows = slice(rt * 16, (rt + 1) * 16)
            z = pltpu.bitcast(pltpu.bitcast(anchor[0:8], u32) & zero_s[0:8, :], f32)
            gb = mod_rows(5, 8) + jnp.concatenate([z] * (D // E), axis=1)
            x2 = x_s[j * (TB // SEG) + rt // 2, (rt % 2) * 16:(rt % 2) * 16 + 16, :]
            base_s[rows, :] = x2.astype(f32) + jnp.concatenate([gb, gb], axis=0) * x1_s[rows, :]

        def out_copy(j, slot):
            return copy(o_s.at[slot], out_hbm.at[pl.ds(aligned(j * TB, TB), TB)], SEM_OUT + slot)

        def ln_job(r0, n, prev, anchor=None):
            if anchor is not None and len(prev) >= 2:
                anchor = anchor[0:8] + prev[-2]
            y = _ln(after(x1_s[r0:r0 + n, :], anchor))
            yn_s[r0:r0 + n, :] = y
            prev.append(y[0:8, 0:E] + y[8:16, 0:E])

        def set_job(src, slot, rt, ct, n1, n=16, anchor=None):
            blk = _outer_operand(lambda i, k: src[i * TQ + rt * n:i * TQ + (rt + 1) * n, _ct(2 * k + ct)],
                                 _LHS_TERMS[n1])
            blk[0] = after(blk[0], anchor)
            blk[3] = after(blk[3], anchor)
            for n2, v in enumerate(_lhs_set(*blk)):
                ref, r0, c0 = d_set(slot, 7 * n1 + n2)
                ref[r0 + rt * n // 2:r0 + (rt + 1) * n // 2, _ct(c0 + ct)] = _pk(v)

        def all_sets(src, slot):
            for n1 in range(7):
                for ct in range(2):
                    set_job(src, slot, 0, ct, n1, TQ)

        wm_wait(wg_s, 0, D // E, SEM_WM)
        mod_tiles(wg_s, 0, D // E, 5 * D // E)
        shift_job(0, 0, TB)
        all_sets(gs_s, 3)
        mix(0)
        prev0 = []
        plan = {}
        for k in range(TB // 16):
            plan[T_AT[0] * (k // 2) + k % 2] = [
                functools.partial(ln_job, (k % 4) * TQ + (k // 4) * 16, 16, prev0)]
        rest = [functools.partial(shift_job, 1, (k % 4) * TQ + (k // 4) * 16, 16)
                for k in range(TB // 16)]
        rest += [functools.partial(set_job, gs_s, 3, rt, ct, n1, 16)
                 for rt in range(2) for ct in range(2) for n1 in range(7)]
        for k, job in enumerate(rest):
            plan.setdefault(k * T_AT[1] // len(rest), []).append(job)
        rest = [functools.partial(set_job, yn_s, 2, rt, ct, n1, 16)
                for rt in range(2) for ct in range(2) for n1 in range(7)]
        for k, job in enumerate(rest):
            plan.setdefault(T_AT[1] + k * (T_AT[2] - T_AT[1]) // len(rest), []).append(job)
        tick0 = [0]

        def hook0(m):
            for job in plan.pop(tick0[0], ()):
                job(anchor=m)
            tick0[0] += 1

        mixer_mm(NI - 2, hook=hook0)
        mixer_sets(mixer_prep(NI - 1, 0, SEG), mixer_prep(NI - 1, SEG, SEG), 0, w_s.at[4])
        mixer_mm(NI - 1, w_s.at[4], hook0)
        assert not plan

        def mlp_block(j, last):
            slot = j & 1

            jn = clamp(j + 2, NB - 1)
            early = [functools.partial(base_job, j, k) for k in range(TB // 16)]
            if not last:
                early += [functools.partial(shift_job, jn, (k % 4) * TQ + (k // 4) * 16, 16)
                          for k in range(TB // 16)]
            early = iter(early)

            pend = []
            tick = [0]

            def drain(m):
                tick[0] += 1
                if pend and tick[0] >= U_AT[0] and (tick[0] - U_AT[0]) % U_AT[1] == 0:
                    pend.pop(0)(m)

            def up_prod(n, g):
                m = _dot(d_lhs(2, n), _up(t3_s[g, :, _ct(n)]))
                if n in E_AT:
                    job = next(early, None)
                    if job is not None:
                        job(anchor=m)
                drain(m)
                return m

            def uset_job(tile, g, n1, r0, n, anchor=None):
                blk = _outer_operand(lambda i, k: tile(i, k, r0, n), _LHS_TERMS[n1])
                blk[0] = after(blk[0], anchor)
                blk[3] = after(blk[3], anchor)
                for n2, v in enumerate(_lhs_set(*blk)):
                    ref, rows = u_set(7 * n1 + n2)
                    ref[rows.start + r0 // 2:rows.start + (r0 + n) // 2, _ct(g)] = _pk(v)

            for g in range(NFG):
                c = _strassen2(lambda n: up_prod(n, g), 1)
                assert not pend
                tick[0] = 0
                if last and g == NFG - 1:
                    act = [[_gelu(c(i, k)) for k in range(4)] for i in range(4)]
                    for n1 in range(7):
                        uset_job(lambda i, k, r0, n: act[i][k], g, n1, 0, TQ)
                    continue
                c0 = 4 * (g % 2)
                for i in range(4):
                    for k in range(4):
                        act_s[i * TQ:(i + 1) * TQ, _ct(c0 + k)] = _gelu(c(i, k))

                def tile(i, k, r0, n, c0=c0):
                    return act_s[i * TQ + r0:i * TQ + r0 + n, _ct(c0 + k)]

                pend += [functools.partial(uset_job, tile, g, n1, r0, 16)
                         for n1 in range(7) for r0 in range(0, TQ, 16)]
            jobs = {}
            if not last:
                mix(j + 1, drain)
                assert not pend
                prev = []
                for k in range(TB // 16):
                    jobs[k * Y_AT] = functools.partial(ln_job, (k % 4) * TQ + (k // 4) * 16, 16, prev)

                def place(start, fns):
                    for fn in fns:
                        while start in jobs:
                            start += 1
                        jobs[start] = fn

                for rt in range(2):
                    place(S_AT[rt], [functools.partial(set_job, yn_s, 2, rt, ct, n1, 16)
                                     for ct in range(2) for n1 in range(7)])
                place(G_AT, [functools.partial(set_job, gs_s, 3, rt, ct, n1, 16)
                             for rt in range(2) for ct in range(2) for n1 in range(7)])

            def down_part(n, og, k0, k1):
                ref, rows = u_set(n)
                return _dot(_up(ref[rows, k0 * E:k1 * E]),
                            _up(t4_s[og, k0 * E // 2:k1 * E // 2, _ct(n)]))

            head = {}
            if last:
                head = {n: down_part(n, 0, 0, NFG - 1) for n in range(HEAD)}
            count = [0]

            def down_prod(n, og):
                if og == 0 and n in head:
                    return down_part(n, og, NFG - 1, NFG) + head[n]
                m = down_part(n, og, 0, NFG)
                job = jobs.get(count[0])
                count[0] += 1
                if job is not None:
                    job(anchor=m)
                return m

            for og in range(NOG):
                c = _strassen2(lambda n: down_prod(n, og))
                for i in range(4):
                    rows = slice(i * TQ, (i + 1) * TQ)
                    for k in range(2):
                        c0 = (4 * og + 2 * k) * E
                        o_s.at[slot][rows, c0:c0 + 2 * E] = (
                            base_s[rows, c0:c0 + 2 * E] + mod_rows(5, TQ, c0, 2 * E)
                            * jnp.concatenate([c(i, 2 * k), c(i, 2 * k + 1)], axis=1)).astype(bf16)
            out_copy(j, slot).start()

        def p3_body(j, carry):
            @pl.when(j >= 2)
            def _():
                out_copy(j - 2, j & 1).wait()

            mlp_block(j, False)
            return carry

        lax.fori_loop(0, NB - 1, _scoped("p3", p3_body), 0)
        for k in range(2):
            for cp in mlp_w_copies(0, k):
                cp.wait()
        out_copy(NB - 3, (NB - 3) % 2).wait()
        mlp_block(NB - 1, True)
        out_copy(NB - 2, (NB - 2) % 2).wait()
        out_copy(NB - 1, (NB - 1) % 2).wait()

    pl.run_scoped(
        phase_a,
        pltpu.VMEM((NSEG, M, D), bf16),
        pltpu.VMEM((7, NSEG * M // 4, D // 2), u32),
        pltpu.VMEM((3 * D // E, D, E), bf16),
        pltpu.VMEM((2, 2, D, HH, E), bf16),
        pltpu.VMEM((2, BGR, D), bf16),
        pltpu.VMEM((2, 2, G1R, D), bf16),
        pltpu.VMEM((NC, D // 4, 5 * HG // 2 * E), u32),
    )
    pl.run_scoped(
        phase_b,
        pltpu.VMEM((NOG, D // 8, 49 * E), u32),
        pltpu.VMEM((NFG, D // 8, 49 * E), u32),
        pltpu.VMEM((NOG, F // 8, 49 * E), u32),
        pltpu.VMEM((D // E, D, E), bf16),
        pltpu.VMEM((TB, D), f32),
        pltpu.VMEM((TB, D), f32),
        pltpu.VMEM((TB, D), f32),
        pltpu.VMEM((TB, D), f32),
        pltpu.VMEM((TB, D), f32),
        pltpu.VMEM((2, TB, D), bf16),
    )


@jax.jit
def pallas_adaLN_cond__memory_aug_recurrent_mem_tr__mixer_s_mlp__prompt_kernel(
    A_x: jax.Array,
    A_mem0: jax.Array,
    A_Wq: jax.Array,
    A_Wk: jax.Array,
    A_Wv: jax.Array,
    A_Wo: jax.Array,
    A_seg_len,
    B_x: jax.Array,
    B_w1: jax.Array,
    B_w2: jax.Array,
    B_w3: jax.Array,
    B_w4: jax.Array,
    c: jax.Array,
    w_mod: jax.Array,
):
    del A_seg_len, B_x
    assert A_x.shape == (1, S, D) and A_mem0.shape == (1, M, D)
    hbm = pl.BlockSpec(memory_space=pl.ANY)
    scratch = [
        pltpu.VMEM((NSEG, SEG, D), bf16),
        pltpu.VMEM((NC, D // 2, HG * E), u32),
        pltpu.VMEM((H * E // 2, D), u32),
        pltpu.VMEM((7, D // 4, D // 2), u32),
        pltpu.VMEM((2, 4, 16, 4 * E), bf16),
        pltpu.VMEM((2, 4, 64, 4 * E), bf16),
        pltpu.VMEM((2, 4, 32, D), bf16),
        pltpu.VMEM((NC, NSEG * M, HG // 2 * E), u32),
        pltpu.VMEM((8, 6 * D), f32),
        pltpu.VMEM((M, D), f32),
        pltpu.VMEM((TC, D), f32),
        pltpu.VMEM((2 * SEG, D), f32),
        pltpu.VMEM((E, E), f32),
        pltpu.VMEM((S, D), bf16),
        pltpu.VMEM((S + 16, D), f32),
        pltpu.VMEM((7 * SEG // 2, D // 2), u32),
        pltpu.VMEM((16, E), u32),
        pltpu.VMEM((1, D), bf16),
        pltpu.VMEM((M, D), bf16),
        pltpu.SemaphoreType.DMA((26,)),
    ]
    out = pl.pallas_call(
        _kernel,
        out_shape=jax.ShapeDtypeStruct((S, D), bf16),
        in_specs=[hbm] * 12,
        out_specs=hbm,
        scratch_shapes=scratch,
        compiler_params=pltpu.CompilerParams(vmem_limit_bytes=127 * 1024 * 1024,
                                             disable_bounds_checks=NO_CHECKS,
                                             disable_semaphore_checks=NO_CHECKS),
    )(A_x.reshape(NSEG, SEG, D), A_mem0.reshape(M, D), A_Wq, A_Wk, A_Wv,
      A_Wo.reshape(H * E, D), B_w1.reshape(2, D // 2, D), B_w2.reshape(4, D // 4, D), B_w3.reshape(4, D // 4, F),
      B_w4.reshape(NFG, 4, E, D), c, w_mod)
    return out.reshape(1, S, D)
```

```python
import functools

import jax
import jax.numpy as jnp
from jax import lax
import jax.experimental.pallas as pl
import jax.experimental.pallas.tpu as pltpu

bf16, f32, u32 = jnp.bfloat16, jnp.float32, jnp.uint32

S, D, H, E, M, SEG, F = 2048, 1024, 32, 128, 8, 32, 3584
EPS = 1e-5
SCALE = E ** -0.5
NSEG = S // SEG
NI = NSEG // 2
NP = H // 2
NR = 2 * (M + SEG)
TC = SEG - M
HG = 8
HH = HG // 2
NG = H // HG
NC = 3 * NG
BGR = 384
G1R = 48
X0 = 4
TB = 128
NB = S // TB
HD = D // 2
NQ = D // E // 2
NFG = F // (4 * E)
NOG = D // (4 * E)

PIN_ROWS = 256
P1_LAG, P1_TAIL, P1_PIN, P1_FROM = 4, 4, 55, 55
PREP_AT = (0, 1, 4, 5)
T_AT = (7, 28, 52)
E_AT = (10, 24, 34)
U_AT = (6, 3)
Y_AT, S_AT, G_AT = 4, (26, 44), 62
HEAD = 14
NO_CHECKS = True
_SCOPES = False


def _scoped(name, fn):
    def wrapped(*a):
        if not _SCOPES:
            return fn(*a)
        with jax.named_scope(name):
            return fn(*a)
    return wrapped


def _pk(x):
    return pltpu.bitcast(x.astype(bf16), u32)


def _up(x):
    return pltpu.bitcast(x, bf16)


def _ct(k):
    return slice(k * E, (k + 1) * E)


def _dot(a, b):
    return jnp.dot(a, b, preferred_element_type=f32)


def _ln(x):
    m = jnp.mean(x, axis=-1, keepdims=True)
    xc = x - m
    v = jnp.mean(xc * xc, axis=-1, keepdims=True)
    return xc * lax.rsqrt(v + EPS)


def _gelu(x):
    c = 0.7978845608028654
    return 0.5 * x * (1.0 + jnp.tanh(c * (x + 0.044715 * (x * x * x))))


def _lhs_set(a11, a12, a21, a22):
    return (a11 + a22, a21 + a22, a11, a22, a11 + a12, a21 - a11, a12 - a22)


def _rhs_set(b11, b12, b21, b22):
    return (b11 + b22, b11, b12 - b22, b21 - b11, b22, b11 + b12, b21 + b22)


_LHS_TERMS = (((0, 1), (3, 1)), ((2, 1), (3, 1)), ((0, 1),), ((3, 1),),
              ((0, 1), (1, 1)), ((2, 1), (0, -1)), ((1, 1), (3, -1)))
_RHS_TERMS = (((0, 1), (3, 1)), ((0, 1),), ((1, 1), (3, -1)), ((2, 1), (0, -1)),
              ((3, 1),), ((0, 1), (1, 1)), ((2, 1), (3, 1)))


def _outer_operand(tile, terms):
    out = []
    for i in range(2):
        for j in range(2):
            v = None
            for o, sign in terms:
                t = tile(2 * (o // 2) + i, 2 * (o % 2) + j)
                v = t if v is None else (v + t if sign > 0 else v - t)
            out.append(v)
    return out


class _Quad:
    def __init__(self, tiles):
        self.t = tuple(tiles)

    def __add__(self, other):
        return _Quad([a + b for a, b in zip(self.t, other.t)])

    def __sub__(self, other):
        return _Quad([a - b for a, b in zip(self.t, other.t)])


def _strassen2(m, order=0):
    cs = _strassen(lambda n1: _Quad(_strassen(lambda n2: m(7 * n1 + n2))), order)
    return lambda i, j: cs[2 * (i // 2) + j // 2].t[2 * (i % 2) + j % 2]


def _strassen(m, order=0):
    if order == 0:
        m1 = m(0)
        m2 = m(1)
        c22 = m1 - m2
        m3 = m(2)
        c22 = c22 + m3
        c22 = m(5) + c22
        m4 = m(3)
        c21 = m2 + m4
        c11 = m1 + m4
        m5 = m(4)
        c12 = m3 + m5
        c11 = c11 - m5
        c11 = m(6) + c11
    else:
        m2 = m(1)
        c22 = m(5) - m2
        m4 = m(3)
        c21 = m2 + m4
        m1 = m(0)
        c22 = c22 + m1
        c11 = m4 + m1
        m3 = m(2)
        c22 = c22 + m3
        m5 = m(4)
        c12 = m3 + m5
        c11 = c11 - m5
        c11 = m(6) + c11
    return c11, c12, c21, c22


def _mask_fill():
    shape = (NR, E)
    r = lax.broadcasted_iota(jnp.int32, shape, 0)
    c = lax.broadcasted_iota(jnp.int32, shape, 1)

    def headpos(i):
        head = jnp.where(i < 64, i >> 5, (i - 64) >> 3)
        pos = jnp.where(i < 64, i & 31, 32 + (i & 7))
        return head, pos

    hr, pr = headpos(r)
    hc, pc = headpos(c)
    same = hr == hc
    valid = same & ((pr < M) | (pr >= pc))
    return jnp.where(valid, 0.0, jnp.where(same, -1e9, -jnp.inf)).astype(f32)


def _kernel(x_hbm, mem0_hbm, wq_hbm, wk_hbm, wv_hbm, wo_hbm, w1_hbm, w2_hbm, w3_hbm,
            w4_hbm, c_hbm, wm_hbm,
            out_hbm,
            x_s, w_s, wo_s, t1_s, g2, g3, g4, pre_s, mod_s, mem_s, hn_s, aout_s, fill_s,
            hb_s, t_s, l1_s, zero_s, c_s, mem0_s, sems):
    w_hbm = (wq_hbm, wk_hbm, wv_hbm)

    (SEM_C, SEM_MEM, SEM_XPRE, SEM_X, SEM_WMR, SEM_BG, SEM_OUT, SEM_G1,
     SEM_G2, SEM_G3, SEM_G4, SEM_WM, SEM_STG) = (0, 1, 2, 3, 4, 6, 8, 10, 12, 14, 16, 18, 22)

    def copy(src, dst, k):
        return pltpu.make_async_copy(src, dst, sems.at[k])

    def aligned(x, n):
        return x if isinstance(x, int) else pl.multiple_of(x, n)

    def clamp(k, hi):
        return min(k, hi) if isinstance(k, int) else jnp.minimum(k, hi)

    def mlp_piece(k):
        k = clamp(k, 4 * NFG - 1)
        return k >> 2, k & 3

    def mlp_w_copies(k, slot):
        g, rr = mlp_piece(k)
        k2 = clamp(k, NI - 1)
        return (copy(w2_hbm.at[:, pl.ds(aligned((k2 >> 1) * 16, 16), 16),
                               pl.ds(aligned((k2 & 1) * 4 * E, E), 4 * E)], g2.at[slot], SEM_G2 + slot),
                copy(w3_hbm.at[:, pl.ds(aligned(rr * 64, 64), 64), pl.ds(aligned(g * 4 * E, E), 4 * E)],
                     g3.at[slot], SEM_G3 + slot),
                copy(w4_hbm.at[g, :, pl.ds(aligned(rr * 32, 32), 32), :], g4.at[slot], SEM_G4 + slot))

    def pinned(w, job):
        if job is None:
            return w()
        z = job() & zero_s[0:8, :]
        w = w()
        return jnp.concatenate([w[0:8] | z, w[8:]], axis=0)

    def after(x, anchor):
        if anchor is None:
            return x
        z = pltpu.bitcast(pltpu.bitcast(anchor[0:8], u32) & zero_s[0:8, :], f32)
        z = jnp.concatenate([z] * (x.shape[0] // 8), axis=0)
        return jnp.concatenate([x[:, 0:E] + z, x[:, E:]], axis=1) if x.shape[1] > E else x + z

    def rhs_job(src, slot, r0, q, dst, row, z):
        blk = [src[slot, kh, r0:r0 + 16, _ct(cc)].astype(f32)
               for kh in range(2) for cc in (q, NQ + q)]
        zf = pltpu.bitcast(jnp.concatenate([z, z], axis=0), f32)
        blk[0] = blk[0] + zf
        blk[3] = blk[3] + zf
        for n, v in enumerate(_rhs_set(*blk)):
            dst.at[n][pl.ds(aligned(row, 8), 8), _ct(q)] = _pk(v)

    def rhs2_job(src, slot, r0, c0, n1, dst, row):
        blk = _outer_operand(lambda i, j: src[slot, i, r0:r0 + 16, _ct(c0 + j)].astype(f32),
                             _RHS_TERMS[n1])
        sets = _rhs_set(*blk)
        for n2, v in enumerate(sets):
            dst[pl.ds(pl.multiple_of(row, 8), 8), _ct(7 * n1 + n2)] = _pk(v)
        out = pltpu.bitcast(sets[2], u32) | pltpu.bitcast(sets[3], u32)
        return out[0:8] | out[8:16]

    def silu_c():
        cf = c_s[...].astype(f32)
        return jnp.broadcast_to(cf * (1.0 / (1.0 + jnp.exp(-cf))), (8, D)).astype(bf16)

    def wm_copy(wm_s, src_tile, dst_tile, sem):
        return copy(wm_hbm.at[:, pl.ds(aligned(src_tile * E, E), E)], wm_s.at[dst_tile], sem)

    def wm_wait(wm_s, t0, n, sem):
        copy(wm_s.at[pl.ds(t0, n)], wm_s.at[pl.ds(t0, n)], sem).wait()

    def x_copy(k):
        r = slice(0, X0) if k == 0 else slice(X0, NSEG)
        return copy(x_hbm.at[r], x_s.at[r], SEM_XPRE if k == 0 else SEM_X)

    def h_rows(s):
        return _ln(x_s[s, 0:TC, :].astype(f32)) * mod_rows(1, TC) + mod_rows(0, TC)

    def mod_rows(k, n, c0=0, w=D):
        return jnp.concatenate([mod_s[:, k * D + c0:k * D + c0 + w]] * (n // 8), axis=0)

    def phase_a(xpre_s, hpre_s, wm_s, stg, bg, g1, tq_s, modt_s):
        def tq_place(c, n):
            if n == 1:
                return w_s.at[c], 0, None
            if n == 4:
                return w_s.at[c], D // 4, None
            return tq_s.at[c], 0, (0, 2, 3, 5, 6).index(n) * (HG // 2)

        def w_copy(t, g, slot, hf):
            return copy(w_hbm[t].at[:, pl.ds(aligned(g * HH, HH), HH), :], stg.at[slot, hf],
                        SEM_STG + 2 * slot + hf)

        def bg_rows(k):
            return clamp(k * BGR, H * E - BGR), clamp(k * G1R, HD - G1R)

        def bg_copies(k, slot):
            ro, r1 = bg_rows(k)
            return (copy(wo_hbm.at[pl.ds(aligned(ro, 16), BGR)], bg.at[slot], SEM_BG + slot),
                    copy(w1_hbm.at[:, pl.ds(aligned(r1, 16), G1R), :], g1.at[slot], SEM_G1 + slot))

        def relayout_jobs(slot, hf, c, j0, i):
            memo = []
            r = aligned(i * 8, 8)

            def job(jj, z=None):
                if not memo:
                    for d0 in (i * 16, HD + i * 16):
                        memo.append(jnp.swapaxes(pltpu.bitcast(stg[slot, hf, pl.ds(d0, 16)], u32), 0, 1))
                j = j0 + jj
                blk = []
                for kh in range(2):
                    u = memo[kh][jj]
                    if z is not None:
                        u = u | jnp.concatenate([z, z], axis=0)
                    blk.append(pltpu.bitcast(u << 16, f32))
                    blk.append(pltpu.bitcast(u & jnp.uint32(0xFFFF0000), f32))
                for k, v in enumerate(blk):
                    w_s.at[c][pl.ds((k // 2) * (D // 4) + r, 8), _ct(2 * j + k % 2)] = _pk(v)
                sets = _rhs_set(*blk)
                for n, v in enumerate(sets):
                    if n not in (1, 4):
                        ref, r0, c0 = tq_place(c, n)
                        ref[pl.ds(r0 + r, 8), _ct(c0 + j)] = _pk(v)
                out = pltpu.bitcast(sets[2], u32) | pltpu.bitcast(sets[3], u32)
                return out[0:8] | out[8:16]

            return [functools.partial(job, jj) for jj in range(2)]

        def repack(slot, row, i, z):
            v = pltpu.bitcast(bg[slot, 16 * i:16 * i + 16, :], u32)
            v = v | jnp.concatenate([z] * (D // E), axis=1)
            wo_s[pl.ds(aligned(row + 8 * i, 8), 8), :] = v

        cp_c = copy(c_hbm, c_s, SEM_C)
        cp_mem = copy(mem0_hbm, mem0_s, SEM_MEM)
        cp_xpre = copy(x_hbm.at[:, TC:SEG, :], xpre_s, SEM_XPRE)
        w_copy(0, 0, 0, 0).start()
        cp_xpre.start()
        cp_c.start()
        cp_mem.start()
        for k in range(2 * D // E):
            wm_copy(wm_s, k, k, SEM_WM + k // 4).start()
        w_copy(0, 1, 0, 1).start()
        w_copy(0, 2, 1, 0).start()
        w_copy(0, 3, 1, 1).start()

        zero_s[0:8, :] = jnp.zeros((8, E), u32)
        fill_s[0:NR, :] = _mask_fill()
        aout_s[...] = jnp.zeros(aout_s.shape, f32)
        l1_s[...] = jnp.zeros(l1_s.shape, u32)
        bg[1] = jnp.zeros(bg.shape[1:], bf16)
        g1[1] = jnp.zeros(g1.shape[1:], bf16)

        w_copy(0, 0, 0, 0).wait()

        def rl0_body(i, carry):
            for job in relayout_jobs(0, 0, 0, 0, i):
                job()
            return carry

        lax.fori_loop(0, D // 32, rl0_body, 0)
        cp_xpre.wait()

        def npre_body(i, carry):
            xr = xpre_s[pl.ds(pl.multiple_of(i * 8, 8), 8)].astype(f32).reshape(64, D)
            t_s[pl.ds(pl.multiple_of(i * 64, 64), 64), :] = _ln(xr)
            return carry

        lax.fori_loop(0, NSEG // 8, _scoped("npre", npre_body), 0)

        cp_c.wait()
        cp_mem.wait()
        mem_s[...] = mem0_s[...].astype(f32)

        sc8 = silu_c()

        def mod_body(k, carry):
            wm_wait(wm_s, 4 * k, 4, SEM_WM + k)
            for kk in range(4):
                modt_s[4 * k + kk] = _dot(sc8, wm_s[4 * k + kk])
            return carry

        lax.fori_loop(0, 4, mod_body, 0)
        for k in range(2 * D // E):
            mod_s[:, _ct(k)] = modt_s[k] if k < D // E else 1.0 + modt_s[k]

        PH = NSEG * M // 2

        def hpre_body(i, carry):
            h = [t_s[pl.ds(pl.multiple_of(hf * PH + i * 16, 16), 16), :] * mod_rows(1, 16) + mod_rows(0, 16)
                 for hf in range(2)]
            for n, v in enumerate(_lhs_set(h[0][:, :HD], h[0][:, HD:], h[1][:, :HD], h[1][:, HD:])):
                hpre_s.at[n][pl.ds(pl.multiple_of(i * 8, 8), 8), :] = _pk(v)
            return carry

        lax.fori_loop(0, PH // 16, _scoped("hpre", hpre_body), 0)

        t_s[0:8, :] = jnp.zeros((8, D), f32)
        t_s[S + 8:S + 16, :] = jnp.zeros((8, D), f32)

        MB = 64

        nu = D // 32

        def small_jobs(slot, k):
            ro, r1 = bg_rows(k)
            return ([functools.partial(repack, slot, ro >> 1, i) for i in range(BGR // 16)]
                    + [functools.partial(rhs_job, g1, slot, 16 * rt, q, t1_s, (r1 >> 1) + 8 * rt)
                       for rt in range(G1R // 16) for q in range(NQ)])

        def p1_pairs(pairs, first, work, start, extra=None):
            npin = 7 * len(pairs) * (PH // MB)
            pins = [[] for _ in range(npin)]
            for k, job in enumerate(first):
                pins[1 + k * (P1_PIN - 1) // len(first)].append(job)
            pins = iter(pins)
            jobs = [[] for _ in range(npin)]
            for k, job in enumerate(work):
                pos = start * 8 + k * (npin - P1_TAIL - start) * 8 // len(work)
                jobs[pos // 8].append((job, pos % 8))
            jobs = iter(jobs)
            pending = []

            def run(group):
                z = group[0]()
                for job in group[1:]:
                    z = z | job()
                return z

            def prod(n, c, q, mb):
                ref, r0, c0 = tq_place(c, n)
                group = next(pins)
                w = pinned(lambda: ref[r0:r0 + D // 4, _ct(2 * q + (n == 4) if c0 is None else c0 + q)],
                           functools.partial(run, group) if group else None)
                m = _dot(_up(hpre_s[n, mb * MB // 2:(mb + 1) * MB // 2, :]), _up(w))
                pending.append(m)
                if len(pending) > P1_LAG:
                    anchor = pltpu.bitcast(pending.pop(0), u32)
                    for job, g in next(jobs):
                        job(anchor[8 * g:8 * g + 8] & zero_s[0:8, :])
                if extra is not None:
                    extra()
                return m

            ns = MB // M
            for c, q in pairs:
                for mb in range(PH // MB):
                    cs = _strassen(lambda n: prod(n, c, q, mb))
                    for hf in range(2):
                        y = jnp.concatenate([cs[2 * hf + k][sg * M:(sg + 1) * M]
                                             for sg in range(ns) for k in range(2)], axis=0)
                        s0 = hf * (NSEG // 2) + mb * ns
                        pre_s.at[c][s0 * M:(s0 + ns) * M, _ct(q)] = _pk(y)

        w_copy(0, 0, 0, 1).wait()
        p1_pairs([(0, 0), (0, 1)], [], [job for i in range(nu) for job in relayout_jobs(0, 1, 0, 2, i)], 0)
        for hf in range(2):
            w_copy(0, 4 + hf, 0, hf).start()
        for cp in bg_copies(0, 0):
            cp.start()

        def wm_rest(k):
            for kk in (k, k + 1):
                wm_copy(wm_s, 2 * D // E + kk, kk, SEM_WMR).start()

        wm_rest(0)

        def p1_body(c, carry):
            pslot = 1 - (c & 1)

            @pl.when(c >= 1)
            def _():
                for cp in bg_copies(0, pslot):
                    cp.wait()

            for hf in range(2):
                w_copy(0, 0, pslot, hf).wait()

            small = small_jobs(pslot, jnp.maximum(c - 1, 0))
            work = []
            for i in range(nu):
                work += relayout_jobs(pslot, 1, c + 1, 2, i)
                work += small[i * len(small) // nu:(i + 1) * len(small) // nu]
            p1_pairs([(c, 2), (c, 3), (c + 1, 0), (c + 1, 1)],
                     [job for i in range(nu) for job in relayout_jobs(pslot, 0, c + 1, 0, i)],
                     work, P1_FROM)

            for t in range(3):
                @pl.when((c + 3) >> 2 == t)
                def _():
                    for hf in range(2):
                        w_copy(t, 2 * ((c + 3) & 3) + hf, pslot, hf).start()

            @pl.when(c + 2 < NC)
            def _():
                for cp in bg_copies(c + 1, pslot):
                    cp.start()
                wm_rest(2 * c + 2)

            @pl.when(c == NC - 3)
            def _():
                wm_rest(2 * NC - 2)
                x_copy(0).start()

            return carry

        lax.fori_loop(0, NC - 1, _scoped("p1", p1_body), 0)
        for k in range(2):
            for cp in mlp_w_copies(k, k):
                cp.start()
        x_copy(1).start()
        for cp in bg_copies(0, NC & 1):
            cp.wait()
        x_copy(0).wait()
        wm_wait(wm_s, 0, 3 * D // E, SEM_WMR)

        halves = iter(range(2 * 3 * D // E))
        part = []

        def mod_half():
            k = next(halves, None)
            if k is None:
                return
            rows = slice((k % 2) * HD, (k % 2 + 1) * HD)
            v = _dot(sc8[:, rows], wm_s[k // 2, rows, :])
            if k % 2 == 0:
                part.append(v)
            else:
                v = v + part.pop()
                tile = 2 * D // E + k // 2
                mod_s[:, _ct(tile)] = 1.0 + v if tile // (D // E) == 4 else v

        p1_pairs([(NC - 1, 2), (NC - 1, 3)], [], small_jobs(NC & 1, NC - 2), 0, mod_half)
        hn_s[...] = h_rows(0)

    def phase_b(t2_s, t3_s, t4_s, wg_s, x1_s, base_s, yn_s, gs_s, act_s, o_s):
        for k in range(D // E):
            wm_copy(wg_s, 5 * D // E + k, k, SEM_WM).start()

        def chain_step(s, mem, htok, odef_prev, jobs=(), hooks=None):
            hs = jnp.concatenate([mem, htok], axis=0).astype(bf16)
            qkv = [[None] * 3 for _ in range(NP)]
            ps = [None] * NP
            os_ = [None] * H
            odef = [None] * H

            def proj(p, t):
                c, q = t * NG + p // (HG // 2), p % (HG // 2)
                a = _dot(hs, _up(w_s[c, :, _ct(2 * q)]))
                b = _dot(hs, _up(w_s[c, :, _ct(2 * q + 1)]))
                pre = pre_s[c, pl.ds(pl.multiple_of(s * M, M), M), _ct(q)]
                parts = [a, b, _up(pre).astype(f32)]
                if t > 0:
                    parts.append(jnp.zeros((E - NR, E), f32))
                v = jnp.concatenate(parts, axis=0)
                qkv[p][t] = (v.T if t == 1 else v).astype(bf16)

            def scores(p):
                sc_ = _dot(qkv[p][0], qkv[p][1])
                fill = fill_s[0:NR, :]
                sc_ = jnp.where(fill == 0.0, sc_ * SCALE, fill)
                m = jnp.max(sc_, axis=-1, keepdims=True)
                e = jnp.exp(sc_ - m)
                l = jnp.sum(e, axis=-1, keepdims=True)
                r = pl.reciprocal(l, approx=True)
                r = r * (2.0 - l * r)
                ps[p] = (e * r).astype(bf16)

            def fin(p):
                o = _dot(ps[p], qkv[p][2])
                for hh in range(2):
                    h = 2 * p + hh
                    rows = o[32 * hh:32 * hh + 32]
                    odef[h] = o[64 + 8 * hh:72 + 8 * hh]
                    if odef_prev is not None:
                        rows = jnp.concatenate([rows, odef_prev[h], odef[h]], axis=0)
                    os_[h] = _pk(rows)

            acc = [None] * 8
            jobs = iter(jobs)

            def wo(h0, h1, js):
                lhs = _up(jnp.concatenate(os_[h0:h1], axis=1))
                for j in js:
                    ws = []
                    for r0 in range(h0 * E // 2, h1 * E // 2, PIN_ROWS):
                        ws.append(pinned(lambda: wo_s[r0:r0 + PIN_ROWS, j * E:(j + 1) * E],
                                         next(jobs, None)))
                    part = _dot(lhs, _up(jnp.concatenate(ws, axis=0)))
                    if hooks and acc[j] is None and j in hooks:
                        hooks[j](part)
                    acc[j] = part if acc[j] is None else part + acc[j]

            for p in range(NP):
                attn = [functools.partial(scores, p - 1) if p >= 1 else None,
                        functools.partial(fin, p - 3) if p >= 3 else None]
                if odef_prev is not None:
                    attn.reverse()
                for t, f in zip((1, 0, 2), attn + [None]):
                    proj(p, t)
                    if f is not None:
                        f()
            hsplit = 24
            wo(0, hsplit, range(0, 2))
            scores(NP - 1)
            fin(NP - 3)
            wo(0, hsplit, range(2, 3))
            fin(NP - 2)
            wo(0, hsplit, range(3, 5))
            fin(NP - 1)
            wo(0, hsplit, range(5, 8))
            wo(hsplit, H, range(8))
            return jnp.concatenate(acc, axis=1), odef

        def mixer_prep(i, r0, n, anchor=None):
            r = pl.ds(aligned(i * 64 + r0, 16), n)
            xr = x_s[2 * i + r0 // SEG, r0 % SEG:r0 % SEG + n, :].astype(f32)
            x2 = xr + mod_rows(2, n) * after(aout_s[r0:r0 + n, :], anchor)
            x_s.at[2 * i + r0 // SEG][r0 % SEG:r0 % SEG + n, :] = x2.astype(bf16)
            hb = _ln(x2) * mod_rows(4, n) + mod_rows(3, n)
            hb_s[r, :] = hb.astype(bf16)
            return _ln(hb)

        def mixer_sets(ya, yb, r0, dst=l1_s):
            n = ya.shape[0]
            for m, v in enumerate(_lhs_set(ya[:, :HD], ya[:, HD:], yb[:, :HD], yb[:, HD:])):
                dst[m * (SEG // 2) + r0 // 2:m * (SEG // 2) + (r0 + n) // 2, 0:HD] = _pk(v)

        def mixer_mm(i, src=l1_s, hook=None):
            for q in range(NQ):
                def prod(n):
                    m = _dot(_up(src[n * (SEG // 2):(n + 1) * (SEG // 2), 0:HD]),
                             _up(t1_s[n, :, _ct(q)]))
                    if hook is not None:
                        hook(m)
                    return m

                cs = _strassen(prod)
                for k, cc in enumerate(cs):
                    r0 = aligned(i * 64 + 8 + (k // 2) * SEG, 8)
                    t_s[pl.ds(r0, SEG), _ct(q + NQ * (k % 2))] = _gelu(cc)

        def p2_body(i, carry):
            slot = i & 1
            for cp in mlp_w_copies(0, slot):
                cp.wait()

            @pl.when(i == 1)
            def _():
                x_copy(1).wait()

            g, rr = mlp_piece(i)
            work = [functools.partial(rhs2_job, g2, slot, 0, 0, n1, t2_s.at[slot], (i >> 1) * 8)
                    for n1 in range(7)]
            work += [functools.partial(rhs2_job, g3, slot, 16 * rt, 0, n1, t3_s.at[g], rr * 32 + 8 * rt)
                     for rt in range(4) for n1 in range(7)]
            work += [functools.partial(rhs2_job, g4, slot, 16 * rt, 4 * og, n1, t4_s.at[og],
                                       g * (E // 2) + rr * 16 + 8 * rt)
                     for rt in range(2) for og in range(NOG) for n1 in range(7)]
            jobs = [None] + work

            sa_ = 2 * i
            sb_ = 2 * i + 1
            hb_tok = h_rows(sb_)
            oa, odef_a = chain_step(sa_, mem_s[...], hn_s[...], None)
            mixer_mm(jnp.maximum(i - 2, 0))
            ys = []

            def hook(k, anchor):
                if k >= 2:
                    anchor = anchor[0:8] + ys[-2][0:8, 0:E] + ys[-2][8:16, 0:E]
                ys.append(mixer_prep(jnp.maximum(i - 1, 0), (k % 2) * SEG + (k // 2) * 16, 16, anchor))
                if k % 2:
                    mixer_sets(ys[-2], ys[-1], (k // 2) * 16)

            hooks = {j: functools.partial(hook, k) for k, j in enumerate(PREP_AT)}
            ob, _ = chain_step(sb_, oa[0:M], hb_tok, odef_a, jobs, hooks)
            mem_s[...] = ob[0:M]
            aout_s[0:TC, :] = oa[M:SEG]
            aout_s[TC:SEG, :] = ob[SEG:SEG + M]
            aout_s[SEG:SEG + TC, :] = ob[M:SEG]
            aout_s[SEG + TC:2 * SEG, :] = ob[SEG + M:SEG + 2 * M]
            hn_s[...] = h_rows(jnp.minimum(sb_ + 1, NSEG - 1))
            for cp in mlp_w_copies(i + 2, slot):
                cp.start()
            return carry

        lax.fori_loop(0, NI, _scoped("p2", p2_body), 0)

        TQ = TB // 4
        SHIFT = (-1, -1, 1, 1, -2, -2, 2, 2)

        def u_set(n):
            return w_s.at[n // 32], slice((n % 32) * (TQ // 2), (n % 32 + 1) * (TQ // 2))

        def d_set(slot, n):
            return w_s.at[slot], (n // 4) * (TQ // 2), (n % 4) * 2

        def d_lhs(slot, n):
            ref, r0, c0 = d_set(slot, n)
            return _up(ref[r0:r0 + TQ // 2, c0 * E:(c0 + 2) * E])

        def shift_job(j, r0, n, anchor=None):
            for ct in range(D // E):
                win = t_s[pl.ds(aligned(j * TB + r0, 16), n + 16), _ct(ct)]
                gs_s[r0:r0 + n, _ct(ct)] = after(
                    pltpu.roll(win, (-SHIFT[ct]) % (n + 16), 0)[8:8 + n], anchor)

        def mix(j, hook=None):
            r0 = aligned(j * TB, TB)
            for og in range(NOG):
                def prod(n):
                    m = _dot(d_lhs(3, n), _up(t2_s[og, :, _ct(n)]))
                    if hook is not None:
                        hook(m)
                    return m

                c = _strassen2(prod)
                for i in range(4):
                    for k in range(2):
                        cols = slice((4 * og + 2 * k) * E, (4 * og + 2 * k + 2) * E)
                        x1_s[i * TQ:(i + 1) * TQ, cols] = (
                            hb_s[pl.ds(r0 + i * TQ, TQ), cols].astype(f32)
                            + jnp.concatenate([c(i, 2 * k), c(i, 2 * k + 1)], axis=1))

        def base_job(j, rt, anchor):
            rows = slice(rt * 16, (rt + 1) * 16)
            z = pltpu.bitcast(pltpu.bitcast(anchor[0:8], u32) & zero_s[0:8, :], f32)
            gb = mod_rows(5, 8) + jnp.concatenate([z] * (D // E), axis=1)
            x2 = x_s[j * (TB // SEG) + rt // 2, (rt % 2) * 16:(rt % 2) * 16 + 16, :]
            base_s[rows, :] = x2.astype(f32) + jnp.concatenate([gb, gb], axis=0) * x1_s[rows, :]

        def out_copy(j, slot):
            return copy(o_s.at[slot], out_hbm.at[pl.ds(aligned(j * TB, TB), TB)], SEM_OUT + slot)

        def ln_job(r0, n, prev, anchor=None):
            if anchor is not None and len(prev) >= 2:
                anchor = anchor[0:8] + prev[-2]
            y = _ln(after(x1_s[r0:r0 + n, :], anchor))
            yn_s[r0:r0 + n, :] = y
            prev.append(y[0:8, 0:E] + y[8:16, 0:E])

        def set_job(src, slot, rt, ct, n1, n=16, anchor=None):
            blk = _outer_operand(lambda i, k: src[i * TQ + rt * n:i * TQ + (rt + 1) * n, _ct(2 * k + ct)],
                                 _LHS_TERMS[n1])
            blk[0] = after(blk[0], anchor)
            blk[3] = after(blk[3], anchor)
            for n2, v in enumerate(_lhs_set(*blk)):
                ref, r0, c0 = d_set(slot, 7 * n1 + n2)
                ref[r0 + rt * n // 2:r0 + (rt + 1) * n // 2, _ct(c0 + ct)] = _pk(v)

        def all_sets(src, slot):
            for n1 in range(7):
                for ct in range(2):
                    set_job(src, slot, 0, ct, n1, TQ)

        wm_wait(wg_s, 0, D // E, SEM_WM)
        sc8 = silu_c()
        for k in range(D // E):
            mod_s[:, _ct(5 * D // E + k)] = _dot(sc8, wg_s[k])
        shift_job(0, 0, TB)
        all_sets(gs_s, 3)
        mix(0)
        prev0 = []
        plan = {}
        for k in range(TB // 16):
            plan[T_AT[0] * (k // 2) + k % 2] = [
                functools.partial(ln_job, (k % 4) * TQ + (k // 4) * 16, 16, prev0)]
        rest = [functools.partial(shift_job, 1, (k % 4) * TQ + (k // 4) * 16, 16)
                for k in range(TB // 16)]
        rest += [functools.partial(set_job, gs_s, 3, rt, ct, n1, 16)
                 for rt in range(2) for ct in range(2) for n1 in range(7)]
        for k, job in enumerate(rest):
            plan.setdefault(k * T_AT[1] // len(rest), []).append(job)
        rest = [functools.partial(set_job, yn_s, 2, rt, ct, n1, 16)
                for rt in range(2) for ct in range(2) for n1 in range(7)]
        for k, job in enumerate(rest):
            plan.setdefault(T_AT[1] + k * (T_AT[2] - T_AT[1]) // len(rest), []).append(job)
        tick0 = [0]

        def hook0(m):
            for job in plan.pop(tick0[0], ()):
                job(anchor=m)
            tick0[0] += 1

        mixer_mm(NI - 2, hook=hook0)
        mixer_sets(mixer_prep(NI - 1, 0, SEG), mixer_prep(NI - 1, SEG, SEG), 0, w_s.at[4])
        mixer_mm(NI - 1, w_s.at[4], hook0)
        assert not plan

        def mlp_block(j, last):
            slot = j & 1

            jn = clamp(j + 2, NB - 1)
            early = [functools.partial(base_job, j, k) for k in range(TB // 16)]
            if not last:
                early += [functools.partial(shift_job, jn, (k % 4) * TQ + (k // 4) * 16, 16)
                          for k in range(TB // 16)]
            early = iter(early)

            pend = []
            tick = [0]

            def drain(m):
                tick[0] += 1
                if pend and tick[0] >= U_AT[0] and (tick[0] - U_AT[0]) % U_AT[1] == 0:
                    pend.pop(0)(m)

            def up_prod(n, g):
                m = _dot(d_lhs(2, n), _up(t3_s[g, :, _ct(n)]))
                if n in E_AT:
                    job = next(early, None)
                    if job is not None:
                        job(anchor=m)
                drain(m)
                return m

            def uset_job(tile, g, n1, r0, n, anchor=None):
                blk = _outer_operand(lambda i, k: tile(i, k, r0, n), _LHS_TERMS[n1])
                blk[0] = after(blk[0], anchor)
                blk[3] = after(blk[3], anchor)
                for n2, v in enumerate(_lhs_set(*blk)):
                    ref, rows = u_set(7 * n1 + n2)
                    ref[rows.start + r0 // 2:rows.start + (r0 + n) // 2, _ct(g)] = _pk(v)

            for g in range(NFG):
                c = _strassen2(lambda n: up_prod(n, g), 1)
                assert not pend
                tick[0] = 0
                if last and g == NFG - 1:
                    act = [[_gelu(c(i, k)) for k in range(4)] for i in range(4)]
                    for n1 in range(7):
                        uset_job(lambda i, k, r0, n: act[i][k], g, n1, 0, TQ)
                    continue
                c0 = 4 * (g % 2)
                for i in range(4):
                    for k in range(4):
                        act_s[i * TQ:(i + 1) * TQ, _ct(c0 + k)] = _gelu(c(i, k))

                def tile(i, k, r0, n, c0=c0):
                    return act_s[i * TQ + r0:i * TQ + r0 + n, _ct(c0 + k)]

                pend += [functools.partial(uset_job, tile, g, n1, r0, 16)
                         for n1 in range(7) for r0 in range(0, TQ, 16)]
            jobs = {}
            if not last:
                mix(j + 1, drain)
                assert not pend
                prev = []
                for k in range(TB // 16):
                    jobs[k * Y_AT] = functools.partial(ln_job, (k % 4) * TQ + (k // 4) * 16, 16, prev)

                def place(start, fns):
                    for fn in fns:
                        while start in jobs:
                            start += 1
                        jobs[start] = fn

                for rt in range(2):
                    place(S_AT[rt], [functools.partial(set_job, yn_s, 2, rt, ct, n1, 16)
                                     for ct in range(2) for n1 in range(7)])
                place(G_AT, [functools.partial(set_job, gs_s, 3, rt, ct, n1, 16)
                             for rt in range(2) for ct in range(2) for n1 in range(7)])

            def down_part(n, og, k0, k1):
                ref, rows = u_set(n)
                return _dot(_up(ref[rows, k0 * E:k1 * E]),
                            _up(t4_s[og, k0 * E // 2:k1 * E // 2, _ct(n)]))

            head = {}
            if last:
                head = {n: down_part(n, 0, 0, NFG - 1) for n in range(HEAD)}
            count = [0]

            def down_prod(n, og):
                if og == 0 and n in head:
                    return down_part(n, og, NFG - 1, NFG) + head[n]
                m = down_part(n, og, 0, NFG)
                job = jobs.get(count[0])
                count[0] += 1
                if job is not None:
                    job(anchor=m)
                return m

            for og in range(NOG):
                c = _strassen2(lambda n: down_prod(n, og))
                for i in range(4):
                    rows = slice(i * TQ, (i + 1) * TQ)
                    for k in range(2):
                        c0 = (4 * og + 2 * k) * E
                        o_s.at[slot][rows, c0:c0 + 2 * E] = (
                            base_s[rows, c0:c0 + 2 * E] + mod_rows(5, TQ, c0, 2 * E)
                            * jnp.concatenate([c(i, 2 * k), c(i, 2 * k + 1)], axis=1)).astype(bf16)
            out_copy(j, slot).start()

        def p3_body(j, carry):
            @pl.when(j >= 2)
            def _():
                out_copy(j - 2, j & 1).wait()

            mlp_block(j, False)
            return carry

        lax.fori_loop(0, NB - 1, _scoped("p3", p3_body), 0)
        for k in range(2):
            for cp in mlp_w_copies(0, k):
                cp.wait()
        out_copy(NB - 3, (NB - 3) % 2).wait()
        mlp_block(NB - 1, True)
        out_copy(NB - 2, (NB - 2) % 2).wait()
        out_copy(NB - 1, (NB - 1) % 2).wait()

    pl.run_scoped(
        phase_a,
        pltpu.VMEM((NSEG, M, D), bf16),
        pltpu.VMEM((7, NSEG * M // 4, D // 2), u32),
        pltpu.VMEM((3 * D // E, D, E), bf16),
        pltpu.VMEM((2, 2, D, HH, E), bf16),
        pltpu.VMEM((2, BGR, D), bf16),
        pltpu.VMEM((2, 2, G1R, D), bf16),
        pltpu.VMEM((NC, D // 4, 5 * HG // 2 * E), u32),
        pltpu.VMEM((2 * D // E, 8, E), f32),
    )
    pl.run_scoped(
        phase_b,
        pltpu.VMEM((NOG, D // 8, 49 * E), u32),
        pltpu.VMEM((NFG, D // 8, 49 * E), u32),
        pltpu.VMEM((NOG, F // 8, 49 * E), u32),
        pltpu.VMEM((D // E, D, E), bf16),
        pltpu.VMEM((TB, D), f32),
        pltpu.VMEM((TB, D), f32),
        pltpu.VMEM((TB, D), f32),
        pltpu.VMEM((TB, D), f32),
        pltpu.VMEM((TB, D), f32),
        pltpu.VMEM((2, TB, D), bf16),
    )


@jax.jit
def pallas_adaLN_cond__memory_aug_recurrent_mem_tr__mixer_s_mlp__prompt_kernel(
    A_x: jax.Array,
    A_mem0: jax.Array,
    A_Wq: jax.Array,
    A_Wk: jax.Array,
    A_Wv: jax.Array,
    A_Wo: jax.Array,
    A_seg_len,
    B_x: jax.Array,
    B_w1: jax.Array,
    B_w2: jax.Array,
    B_w3: jax.Array,
    B_w4: jax.Array,
    c: jax.Array,
    w_mod: jax.Array,
):
    del A_seg_len, B_x
    assert A_x.shape == (1, S, D) and A_mem0.shape == (1, M, D)
    hbm = pl.BlockSpec(memory_space=pl.ANY)
    scratch = [
        pltpu.VMEM((NSEG, SEG, D), bf16),
        pltpu.VMEM((NC, D // 2, HG * E), u32),
        pltpu.VMEM((H * E // 2, D), u32),
        pltpu.VMEM((7, D // 4, D // 2), u32),
        pltpu.VMEM((2, 4, 16, 4 * E), bf16),
        pltpu.VMEM((2, 4, 64, 4 * E), bf16),
        pltpu.VMEM((2, 4, 32, D), bf16),
        pltpu.VMEM((NC, NSEG * M, HG // 2 * E), u32),
        pltpu.VMEM((8, 6 * D), f32),
        pltpu.VMEM((M, D), f32),
        pltpu.VMEM((TC, D), f32),
        pltpu.VMEM((2 * SEG, D), f32),
        pltpu.VMEM((E, E), f32),
        pltpu.VMEM((S, D), bf16),
        pltpu.VMEM((S + 16, D), f32),
        pltpu.VMEM((7 * SEG // 2, D // 2), u32),
        pltpu.VMEM((16, E), u32),
        pltpu.VMEM((1, D), bf16),
        pltpu.VMEM((M, D), bf16),
        pltpu.SemaphoreType.DMA((26,)),
    ]
    out = pl.pallas_call(
        _kernel,
        out_shape=jax.ShapeDtypeStruct((S, D), bf16),
        in_specs=[hbm] * 12,
        out_specs=hbm,
        scratch_shapes=scratch,
        compiler_params=pltpu.CompilerParams(vmem_limit_bytes=127 * 1024 * 1024,
                                             disable_bounds_checks=NO_CHECKS,
                                             disable_semaphore_checks=NO_CHECKS),
    )(A_x.reshape(NSEG, SEG, D), A_mem0.reshape(M, D), A_Wq, A_Wk, A_Wv,
      A_Wo.reshape(H * E, D), B_w1.reshape(2, D // 2, D), B_w2.reshape(4, D // 4, D), B_w3.reshape(4, D // 4, F),
      B_w4.reshape(NFG, 4, E, D), c, w_mod)
    return out.reshape(1, S, D)
```

```python
import functools

import jax
import jax.numpy as jnp
from jax import lax
import jax.experimental.pallas as pl
import jax.experimental.pallas.tpu as pltpu

bf16, f32, u32 = jnp.bfloat16, jnp.float32, jnp.uint32

S, D, H, E, M, SEG, F = 2048, 1024, 32, 128, 8, 32, 3584
EPS = 1e-5
SCALE = E ** -0.5
NSEG = S // SEG
NI = NSEG // 2
NP = H // 2
NR = 2 * (M + SEG)
TC = SEG - M
HG = 8
HH = HG // 2
NG = H // HG
NC = 3 * NG
BGR = 384
G1R = 48
X0 = 4
TB = 128
NB = S // TB
HD = D // 2
NQ = D // E // 2
NFG = F // (4 * E)
NOG = D // (4 * E)

PIN_ROWS = 256
P1_LAG, P1_TAIL, P1_PIN, P1_FROM = 4, 4, 55, 55
PREP_AT = (0, 1, 4, 5)
T_AT = (7, 28, 52)
E_AT = (10, 24, 34)
U_AT = (6, 3)
Y_AT, S_AT, G_AT = 4, (26, 44), 62
HEAD = 14
HN_AT = 3
NO_CHECKS = True
_SCOPES = False


def _scoped(name, fn):
    def wrapped(*a):
        if not _SCOPES:
            return fn(*a)
        with jax.named_scope(name):
            return fn(*a)
    return wrapped


def _pk(x):
    return pltpu.bitcast(x.astype(bf16), u32)


def _up(x):
    return pltpu.bitcast(x, bf16)


def _ct(k):
    return slice(k * E, (k + 1) * E)


def _dot(a, b):
    return jnp.dot(a, b, preferred_element_type=f32)


def _ln(x):
    m = jnp.mean(x, axis=-1, keepdims=True)
    xc = x - m
    v = jnp.mean(xc * xc, axis=-1, keepdims=True)
    return xc * lax.rsqrt(v + EPS)


def _gelu(x):
    c = 0.7978845608028654
    return 0.5 * x * (1.0 + jnp.tanh(c * (x + 0.044715 * (x * x * x))))


def _lhs_set(a11, a12, a21, a22):
    return (a11 + a22, a21 + a22, a11, a22, a11 + a12, a21 - a11, a12 - a22)


def _rhs_set(b11, b12, b21, b22):
    return (b11 + b22, b11, b12 - b22, b21 - b11, b22, b11 + b12, b21 + b22)


_LHS_TERMS = (((0, 1), (3, 1)), ((2, 1), (3, 1)), ((0, 1),), ((3, 1),),
              ((0, 1), (1, 1)), ((2, 1), (0, -1)), ((1, 1), (3, -1)))
_RHS_TERMS = (((0, 1), (3, 1)), ((0, 1),), ((1, 1), (3, -1)), ((2, 1), (0, -1)),
              ((3, 1),), ((0, 1), (1, 1)), ((2, 1), (3, 1)))


def _outer_operand(tile, terms):
    out = []
    for i in range(2):
        for j in range(2):
            v = None
            for o, sign in terms:
                t = tile(2 * (o // 2) + i, 2 * (o % 2) + j)
                v = t if v is None else (v + t if sign > 0 else v - t)
            out.append(v)
    return out


class _Quad:
    def __init__(self, tiles):
        self.t = tuple(tiles)

    def __add__(self, other):
        return _Quad([a + b for a, b in zip(self.t, other.t)])

    def __sub__(self, other):
        return _Quad([a - b for a, b in zip(self.t, other.t)])


def _strassen2(m, order=0):
    cs = _strassen(lambda n1: _Quad(_strassen(lambda n2: m(7 * n1 + n2))), order)
    return lambda i, j: cs[2 * (i // 2) + j // 2].t[2 * (i % 2) + j % 2]


def _strassen(m, order=0):
    if order == 0:
        m1 = m(0)
        m2 = m(1)
        c22 = m1 - m2
        m3 = m(2)
        c22 = c22 + m3
        c22 = m(5) + c22
        m4 = m(3)
        c21 = m2 + m4
        c11 = m1 + m4
        m5 = m(4)
        c12 = m3 + m5
        c11 = c11 - m5
        c11 = m(6) + c11
    else:
        m2 = m(1)
        c22 = m(5) - m2
        m4 = m(3)
        c21 = m2 + m4
        m1 = m(0)
        c22 = c22 + m1
        c11 = m4 + m1
        m3 = m(2)
        c22 = c22 + m3
        m5 = m(4)
        c12 = m3 + m5
        c11 = c11 - m5
        c11 = m(6) + c11
    return c11, c12, c21, c22


def _mask_fill():
    shape = (NR, E)
    r = lax.broadcasted_iota(jnp.int32, shape, 0)
    c = lax.broadcasted_iota(jnp.int32, shape, 1)

    def headpos(i):
        head = jnp.where(i < 64, i >> 5, (i - 64) >> 3)
        pos = jnp.where(i < 64, i & 31, 32 + (i & 7))
        return head, pos

    hr, pr = headpos(r)
    hc, pc = headpos(c)
    same = hr == hc
    valid = same & ((pr < M) | (pr >= pc))
    return jnp.where(valid, 0.0, jnp.where(same, -1e9, -jnp.inf)).astype(f32)


def _kernel(x_hbm, mem0_hbm, wq_hbm, wk_hbm, wv_hbm, wo_hbm, w1_hbm, w2_hbm, w3_hbm,
            w4_hbm, c_hbm, wm_hbm,
            out_hbm,
            x_s, w_s, wo_s, t1_s, g2, g3, g4, pre_s, mod_s, mem_s, hn_s, aout_s, fill_s,
            hb_s, t_s, l1_s, zero_s, c_s, mem0_s, sems):
    w_hbm = (wq_hbm, wk_hbm, wv_hbm)

    (SEM_C, SEM_MEM, SEM_XPRE, SEM_X, SEM_WMR, SEM_BG, SEM_OUT, SEM_G1,
     SEM_G2, SEM_G3, SEM_G4, SEM_WM, SEM_STG) = (0, 1, 2, 3, 4, 6, 8, 10, 12, 14, 16, 18, 22)

    def copy(src, dst, k):
        return pltpu.make_async_copy(src, dst, sems.at[k])

    def aligned(x, n):
        return x if isinstance(x, int) else pl.multiple_of(x, n)

    def clamp(k, hi):
        return min(k, hi) if isinstance(k, int) else jnp.minimum(k, hi)

    def mlp_piece(k):
        k = clamp(k, 4 * NFG - 1)
        return k >> 2, k & 3

    def mlp_w_copies(k, slot):
        g, rr = mlp_piece(k)
        k2 = clamp(k, NI - 1)
        return (copy(w2_hbm.at[:, pl.ds(aligned((k2 >> 1) * 16, 16), 16),
                               pl.ds(aligned((k2 & 1) * 4 * E, E), 4 * E)], g2.at[slot], SEM_G2 + slot),
                copy(w3_hbm.at[:, pl.ds(aligned(rr * 64, 64), 64), pl.ds(aligned(g * 4 * E, E), 4 * E)],
                     g3.at[slot], SEM_G3 + slot),
                copy(w4_hbm.at[g, :, pl.ds(aligned(rr * 32, 32), 32), :], g4.at[slot], SEM_G4 + slot))

    def pinned(w, job):
        if job is None:
            return w()
        z = job() & zero_s[0:8, :]
        w = w()
        return jnp.concatenate([w[0:8] | z, w[8:]], axis=0)

    def after(x, anchor):
        if anchor is None:
            return x
        z = pltpu.bitcast(pltpu.bitcast(anchor[0:8], u32) & zero_s[0:8, :], f32)
        z = jnp.concatenate([z] * (x.shape[0] // 8), axis=0)
        return jnp.concatenate([x[:, 0:E] + z, x[:, E:]], axis=1) if x.shape[1] > E else x + z

    def rhs_job(src, slot, r0, q, dst, row, z):
        blk = [src[slot, kh, r0:r0 + 16, _ct(cc)].astype(f32)
               for kh in range(2) for cc in (q, NQ + q)]
        zf = pltpu.bitcast(jnp.concatenate([z, z], axis=0), f32)
        blk[0] = blk[0] + zf
        blk[3] = blk[3] + zf
        for n, v in enumerate(_rhs_set(*blk)):
            dst.at[n][pl.ds(aligned(row, 8), 8), _ct(q)] = _pk(v)

    def rhs2_job(src, slot, r0, c0, n1, dst, row):
        blk = _outer_operand(lambda i, j: src[slot, i, r0:r0 + 16, _ct(c0 + j)].astype(f32),
                             _RHS_TERMS[n1])
        sets = _rhs_set(*blk)
        for n2, v in enumerate(sets):
            dst[pl.ds(pl.multiple_of(row, 8), 8), _ct(7 * n1 + n2)] = _pk(v)
        out = pltpu.bitcast(sets[2], u32) | pltpu.bitcast(sets[3], u32)
        return out[0:8] | out[8:16]

    def silu_c():
        cf = c_s[...].astype(f32)
        return jnp.broadcast_to(cf * (1.0 / (1.0 + jnp.exp(-cf))), (8, D)).astype(bf16)

    def wm_copy(wm_s, src_tile, dst_tile, sem):
        return copy(wm_hbm.at[:, pl.ds(aligned(src_tile * E, E), E)], wm_s.at[dst_tile], sem)

    def wm_wait(wm_s, t0, n, sem):
        copy(wm_s.at[pl.ds(t0, n)], wm_s.at[pl.ds(t0, n)], sem).wait()

    def x_copy(k):
        r = slice(0, X0) if k == 0 else slice(X0, NSEG)
        return copy(x_hbm.at[r], x_s.at[r], SEM_XPRE if k == 0 else SEM_X)

    def h_rows(xr, anchor=None):
        return _ln(after(xr.astype(f32), anchor)) * mod_rows(1, TC) + mod_rows(0, TC)

    def mod_rows(k, n, c0=0, w=D):
        return jnp.concatenate([mod_s[:, k * D + c0:k * D + c0 + w]] * (n // 8), axis=0)

    def phase_a(xpre_s, hpre_s, wm_s, stg, bg, g1, tq_s, modt_s):
        def tq_place(c, n):
            if n == 1:
                return w_s.at[c], 0, None
            if n == 4:
                return w_s.at[c], D // 4, None
            return tq_s.at[c], 0, (0, 2, 3, 5, 6).index(n) * (HG // 2)

        def w_copy(t, g, slot, hf):
            return copy(w_hbm[t].at[:, pl.ds(aligned(g * HH, HH), HH), :], stg.at[slot, hf],
                        SEM_STG + 2 * slot + hf)

        def bg_rows(k):
            return clamp(k * BGR, H * E - BGR), clamp(k * G1R, HD - G1R)

        def bg_copies(k, slot):
            ro, r1 = bg_rows(k)
            return (copy(wo_hbm.at[pl.ds(aligned(ro, 16), BGR)], bg.at[slot], SEM_BG + slot),
                    copy(w1_hbm.at[:, pl.ds(aligned(r1, 16), G1R), :], g1.at[slot], SEM_G1 + slot))

        def relayout_jobs(slot, hf, c, j0, i):
            memo = []
            r = aligned(i * 8, 8)

            def job(jj, z=None):
                if not memo:
                    for d0 in (i * 16, HD + i * 16):
                        memo.append(jnp.swapaxes(pltpu.bitcast(stg[slot, hf, pl.ds(d0, 16)], u32), 0, 1))
                j = j0 + jj
                blk = []
                for kh in range(2):
                    u = memo[kh][jj]
                    if z is not None:
                        u = u | jnp.concatenate([z, z], axis=0)
                    blk.append(pltpu.bitcast(u << 16, f32))
                    blk.append(pltpu.bitcast(u & jnp.uint32(0xFFFF0000), f32))
                for k, v in enumerate(blk):
                    w_s.at[c][pl.ds((k // 2) * (D // 4) + r, 8), _ct(2 * j + k % 2)] = _pk(v)
                sets = _rhs_set(*blk)
                for n, v in enumerate(sets):
                    if n not in (1, 4):
                        ref, r0, c0 = tq_place(c, n)
                        ref[pl.ds(r0 + r, 8), _ct(c0 + j)] = _pk(v)
                out = pltpu.bitcast(sets[2], u32) | pltpu.bitcast(sets[3], u32)
                return out[0:8] | out[8:16]

            return [functools.partial(job, jj) for jj in range(2)]

        def repack(slot, row, i, z):
            v = pltpu.bitcast(bg[slot, 16 * i:16 * i + 16, :], u32)
            v = v | jnp.concatenate([z] * (D // E), axis=1)
            wo_s[pl.ds(aligned(row + 8 * i, 8), 8), :] = v

        cp_c = copy(c_hbm, c_s, SEM_C)
        cp_mem = copy(mem0_hbm, mem0_s, SEM_MEM)
        cp_xpre = copy(x_hbm.at[:, TC:SEG, :], xpre_s, SEM_XPRE)
        w_copy(0, 0, 0, 0).start()
        cp_xpre.start()
        cp_c.start()
        cp_mem.start()
        for k in range(2 * D // E):
            wm_copy(wm_s, k, k, SEM_WM + k // 4).start()
        w_copy(0, 1, 0, 1).start()
        w_copy(0, 2, 1, 0).start()
        w_copy(0, 3, 1, 1).start()

        zero_s[0:8, :] = jnp.zeros((8, E), u32)
        fill_s[0:NR, :] = _mask_fill()
        aout_s[...] = jnp.zeros(aout_s.shape, f32)
        l1_s[...] = jnp.zeros(l1_s.shape, u32)
        bg[1] = jnp.zeros(bg.shape[1:], bf16)
        g1[1] = jnp.zeros(g1.shape[1:], bf16)

        w_copy(0, 0, 0, 0).wait()

        def rl0_body(i, carry):
            for job in relayout_jobs(0, 0, 0, 0, i):
                job()
            return carry

        lax.fori_loop(0, D // 32, rl0_body, 0)
        cp_xpre.wait()

        def npre_body(i, carry):
            xr = xpre_s[pl.ds(pl.multiple_of(i * 8, 8), 8)].astype(f32).reshape(64, D)
            t_s[pl.ds(pl.multiple_of(i * 64, 64), 64), :] = _ln(xr)
            return carry

        lax.fori_loop(0, NSEG // 8, _scoped("npre", npre_body), 0)

        cp_c.wait()
        cp_mem.wait()
        mem_s[...] = mem0_s[...].astype(f32)

        sc8 = silu_c()

        def mod_body(k, carry):
            wm_wait(wm_s, 4 * k, 4, SEM_WM + k)
            for kk in range(4):
                modt_s[4 * k + kk] = _dot(sc8, wm_s[4 * k + kk])
            return carry

        lax.fori_loop(0, 4, mod_body, 0)
        for k in range(2 * D // E):
            mod_s[:, _ct(k)] = modt_s[k] if k < D // E else 1.0 + modt_s[k]

        PH = NSEG * M // 2

        def hpre_body(i, carry):
            h = [t_s[pl.ds(pl.multiple_of(hf * PH + i * 16, 16), 16), :] * mod_rows(1, 16) + mod_rows(0, 16)
                 for hf in range(2)]
            for n, v in enumerate(_lhs_set(h[0][:, :HD], h[0][:, HD:], h[1][:, :HD], h[1][:, HD:])):
                hpre_s.at[n][pl.ds(pl.multiple_of(i * 8, 8), 8), :] = _pk(v)
            return carry

        lax.fori_loop(0, PH // 16, _scoped("hpre", hpre_body), 0)

        t_s[0:8, :] = jnp.zeros((8, D), f32)
        t_s[S + 8:S + 16, :] = jnp.zeros((8, D), f32)

        MB = 64

        nu = D // 32

        def small_jobs(slot, k):
            ro, r1 = bg_rows(k)
            return ([functools.partial(repack, slot, ro >> 1, i) for i in range(BGR // 16)]
                    + [functools.partial(rhs_job, g1, slot, 16 * rt, q, t1_s, (r1 >> 1) + 8 * rt)
                       for rt in range(G1R // 16) for q in range(NQ)])

        def p1_pairs(pairs, first, work, start, extra=None):
            npin = 7 * len(pairs) * (PH // MB)
            pins = [[] for _ in range(npin)]
            for k, job in enumerate(first):
                pins[1 + k * (P1_PIN - 1) // len(first)].append(job)
            pins = iter(pins)
            jobs = [[] for _ in range(npin)]
            for k, job in enumerate(work):
                pos = start * 8 + k * (npin - P1_TAIL - start) * 8 // len(work)
                jobs[pos // 8].append((job, pos % 8))
            jobs = iter(jobs)
            pending = []

            def run(group):
                z = group[0]()
                for job in group[1:]:
                    z = z | job()
                return z

            def prod(n, c, q, mb):
                ref, r0, c0 = tq_place(c, n)
                group = next(pins)
                w = pinned(lambda: ref[r0:r0 + D // 4, _ct(2 * q + (n == 4) if c0 is None else c0 + q)],
                           functools.partial(run, group) if group else None)
                m = _dot(_up(hpre_s[n, mb * MB // 2:(mb + 1) * MB // 2, :]), _up(w))
                pending.append(m)
                if len(pending) > P1_LAG:
                    anchor = pltpu.bitcast(pending.pop(0), u32)
                    for job, g in next(jobs):
                        job(anchor[8 * g:8 * g + 8] & zero_s[0:8, :])
                if extra is not None:
                    extra()
                return m

            ns = MB // M
            for c, q in pairs:
                for mb in range(PH // MB):
                    cs = _strassen(lambda n: prod(n, c, q, mb))
                    for hf in range(2):
                        y = jnp.concatenate([cs[2 * hf + k][sg * M:(sg + 1) * M]
                                             for sg in range(ns) for k in range(2)], axis=0)
                        s0 = hf * (NSEG // 2) + mb * ns
                        pre_s.at[c][s0 * M:(s0 + ns) * M, _ct(q)] = _pk(y)

        w_copy(0, 0, 0, 1).wait()
        p1_pairs([(0, 0), (0, 1)], [], [job for i in range(nu) for job in relayout_jobs(0, 1, 0, 2, i)], 0)
        for hf in range(2):
            w_copy(0, 4 + hf, 0, hf).start()
        for cp in bg_copies(0, 0):
            cp.start()

        def wm_rest(k):
            for kk in (k, k + 1):
                wm_copy(wm_s, 2 * D // E + kk, kk, SEM_WMR).start()

        wm_rest(0)

        def p1_body(c, carry):
            pslot = 1 - (c & 1)

            @pl.when(c >= 1)
            def _():
                for cp in bg_copies(0, pslot):
                    cp.wait()

            for hf in range(2):
                w_copy(0, 0, pslot, hf).wait()

            small = small_jobs(pslot, jnp.maximum(c - 1, 0))
            work = []
            for i in range(nu):
                work += relayout_jobs(pslot, 1, c + 1, 2, i)
                work += small[i * len(small) // nu:(i + 1) * len(small) // nu]
            p1_pairs([(c, 2), (c, 3), (c + 1, 0), (c + 1, 1)],
                     [job for i in range(nu) for job in relayout_jobs(pslot, 0, c + 1, 0, i)],
                     work, P1_FROM)

            for t in range(3):
                @pl.when((c + 3) >> 2 == t)
                def _():
                    for hf in range(2):
                        w_copy(t, 2 * ((c + 3) & 3) + hf, pslot, hf).start()

            @pl.when(c + 2 < NC)
            def _():
                for cp in bg_copies(c + 1, pslot):
                    cp.start()
                wm_rest(2 * c + 2)

            @pl.when(c == NC - 3)
            def _():
                wm_rest(2 * NC - 2)
                x_copy(0).start()

            return carry

        lax.fori_loop(0, NC - 1, _scoped("p1", p1_body), 0)
        for k in range(2):
            for cp in mlp_w_copies(k, k):
                cp.start()
        x_copy(1).start()
        for cp in bg_copies(0, NC & 1):
            cp.wait()
        x_copy(0).wait()
        wm_wait(wm_s, 0, 3 * D // E, SEM_WMR)

        halves = iter(range(2 * 3 * D // E))
        part = []

        def mod_half():
            k = next(halves, None)
            if k is None:
                return
            rows = slice((k % 2) * HD, (k % 2 + 1) * HD)
            v = _dot(sc8[:, rows], wm_s[k // 2, rows, :])
            if k % 2 == 0:
                part.append(v)
            else:
                v = v + part.pop()
                tile = 2 * D // E + k // 2
                mod_s[:, _ct(tile)] = 1.0 + v if tile // (D // E) == 4 else v

        p1_pairs([(NC - 1, 2), (NC - 1, 3)], [], small_jobs(NC & 1, NC - 2), 0, mod_half)
        hn_s[...] = h_rows(x_s[0, 0:TC, :])

    def phase_b(t2_s, t3_s, t4_s, wg_s, x1_s, base_s, yn_s, gs_s, act_s, o_s):
        for k in range(D // E):
            wm_copy(wg_s, 5 * D // E + k, k, SEM_WM).start()

        def chain_step(s, mem, htok, odef_prev, jobs=(), hooks=None):
            hs = jnp.concatenate([mem, htok], axis=0).astype(bf16)
            qkv = [[None] * 3 for _ in range(NP)]
            ps = [None] * NP
            os_ = [None] * H
            odef = [None] * H

            def proj(p, t):
                c, q = t * NG + p // (HG // 2), p % (HG // 2)
                a = _dot(hs, _up(w_s[c, :, _ct(2 * q)]))
                b = _dot(hs, _up(w_s[c, :, _ct(2 * q + 1)]))
                pre = pre_s[c, pl.ds(pl.multiple_of(s * M, M), M), _ct(q)]
                parts = [a, b, _up(pre).astype(f32)]
                if t > 0:
                    parts.append(jnp.zeros((E - NR, E), f32))
                v = jnp.concatenate(parts, axis=0)
                qkv[p][t] = (v.T if t == 1 else v).astype(bf16)

            def scores(p):
                sc_ = _dot(qkv[p][0], qkv[p][1])
                fill = fill_s[0:NR, :]
                sc_ = jnp.where(fill == 0.0, sc_ * SCALE, fill)
                m = jnp.max(sc_, axis=-1, keepdims=True)
                e = jnp.exp(sc_ - m)
                l = jnp.sum(e, axis=-1, keepdims=True)
                r = pl.reciprocal(l, approx=True)
                r = r * (2.0 - l * r)
                ps[p] = (e * r).astype(bf16)

            def fin(p):
                o = _dot(ps[p], qkv[p][2])
                for hh in range(2):
                    h = 2 * p + hh
                    rows = o[32 * hh:32 * hh + 32]
                    odef[h] = o[64 + 8 * hh:72 + 8 * hh]
                    if odef_prev is not None:
                        rows = jnp.concatenate([rows, odef_prev[h], odef[h]], axis=0)
                    os_[h] = _pk(rows)

            acc = [None] * 8
            jobs = iter(jobs)

            def wo(h0, h1, js):
                lhs = _up(jnp.concatenate(os_[h0:h1], axis=1))
                for j in js:
                    ws = []
                    for r0 in range(h0 * E // 2, h1 * E // 2, PIN_ROWS):
                        ws.append(pinned(lambda: wo_s[r0:r0 + PIN_ROWS, j * E:(j + 1) * E],
                                         next(jobs, None)))
                    part = _dot(lhs, _up(jnp.concatenate(ws, axis=0)))
                    if hooks and acc[j] is None and j in hooks:
                        hooks[j](part)
                    acc[j] = part if acc[j] is None else part + acc[j]

            for p in range(NP):
                attn = [functools.partial(scores, p - 1) if p >= 1 else None,
                        functools.partial(fin, p - 3) if p >= 3 else None]
                if odef_prev is not None:
                    attn.reverse()
                for t, f in zip((1, 0, 2), attn + [None]):
                    proj(p, t)
                    if f is not None:
                        f()
            hsplit = 24
            wo(0, hsplit, range(0, 2))
            scores(NP - 1)
            fin(NP - 3)
            wo(0, hsplit, range(2, 3))
            fin(NP - 2)
            wo(0, hsplit, range(3, 5))
            fin(NP - 1)
            wo(0, hsplit, range(5, 8))
            wo(hsplit, H, range(8))
            return jnp.concatenate(acc, axis=1), odef

        def mixer_prep(i, r0, n, anchor=None):
            r = pl.ds(aligned(i * 64 + r0, 16), n)
            xr = x_s[2 * i + r0 // SEG, r0 % SEG:r0 % SEG + n, :].astype(f32)
            x2 = xr + mod_rows(2, n) * after(aout_s[r0:r0 + n, :], anchor)
            x_s.at[2 * i + r0 // SEG][r0 % SEG:r0 % SEG + n, :] = x2.astype(bf16)
            hb = _ln(x2) * mod_rows(4, n) + mod_rows(3, n)
            hb_s[r, :] = hb.astype(bf16)
            return _ln(hb)

        def mixer_sets(ya, yb, r0, dst=l1_s):
            n = ya.shape[0]
            for m, v in enumerate(_lhs_set(ya[:, :HD], ya[:, HD:], yb[:, :HD], yb[:, HD:])):
                dst[m * (SEG // 2) + r0 // 2:m * (SEG // 2) + (r0 + n) // 2, 0:HD] = _pk(v)

        def mixer_mm(i, src=l1_s, hook=None):
            for q in range(NQ):
                def prod(n):
                    m = _dot(_up(src[n * (SEG // 2):(n + 1) * (SEG // 2), 0:HD]),
                             _up(t1_s[n, :, _ct(q)]))
                    if hook is not None:
                        hook(m)
                    return m

                cs = _strassen(prod)
                for k, cc in enumerate(cs):
                    r0 = aligned(i * 64 + 8 + (k // 2) * SEG, 8)
                    t_s[pl.ds(r0, SEG), _ct(q + NQ * (k % 2))] = _gelu(cc)

        def p2_body(i, carry):
            slot = i & 1
            for cp in mlp_w_copies(0, slot):
                cp.wait()

            @pl.when(i == 1)
            def _():
                x_copy(1).wait()

            g, rr = mlp_piece(i)
            work = [functools.partial(rhs2_job, g2, slot, 0, 0, n1, t2_s.at[slot], (i >> 1) * 8)
                    for n1 in range(7)]
            work += [functools.partial(rhs2_job, g3, slot, 16 * rt, 0, n1, t3_s.at[g], rr * 32 + 8 * rt)
                     for rt in range(4) for n1 in range(7)]
            work += [functools.partial(rhs2_job, g4, slot, 16 * rt, 4 * og, n1, t4_s.at[og],
                                       g * (E // 2) + rr * 16 + 8 * rt)
                     for rt in range(2) for og in range(NOG) for n1 in range(7)]
            jobs = [None] + work

            sa_ = 2 * i
            sb_ = 2 * i + 1
            hb_tok = h_rows(x_s[sb_, 0:TC, :])
            oa, odef_a = chain_step(sa_, mem_s[...], hn_s[...], None)
            xn = x_s[jnp.minimum(sb_ + 1, NSEG - 1), 0:TC, :]
            mixer_mm(jnp.maximum(i - 2, 0))
            ys = []

            def hook(k, anchor):
                if k >= 2:
                    anchor = anchor[0:8] + ys[-2][0:8, 0:E] + ys[-2][8:16, 0:E]
                ys.append(mixer_prep(jnp.maximum(i - 1, 0), (k % 2) * SEG + (k // 2) * 16, 16, anchor))
                if k % 2:
                    mixer_sets(ys[-2], ys[-1], (k // 2) * 16)

            hooks = {j: functools.partial(hook, k) for k, j in enumerate(PREP_AT)}
            ob, _ = chain_step(sb_, oa[0:M], hb_tok, odef_a, jobs, hooks)
            mem_s[...] = ob[0:M]
            aout_s[0:TC, :] = oa[M:SEG]
            aout_s[TC:SEG, :] = ob[SEG:SEG + M]
            aout_s[SEG:SEG + TC, :] = ob[M:SEG]
            aout_s[SEG + TC:2 * SEG, :] = ob[SEG + M:SEG + 2 * M]
            hn_s[...] = h_rows(xn, ob[:, _ct(HN_AT)])
            for cp in mlp_w_copies(i + 2, slot):
                cp.start()
            return carry

        lax.fori_loop(0, NI, _scoped("p2", p2_body), 0)

        TQ = TB // 4
        SHIFT = (-1, -1, 1, 1, -2, -2, 2, 2)

        def u_set(n):
            return w_s.at[n // 32], slice((n % 32) * (TQ // 2), (n % 32 + 1) * (TQ // 2))

        def d_set(slot, n):
            return w_s.at[slot], (n // 4) * (TQ // 2), (n % 4) * 2

        def d_lhs(slot, n):
            ref, r0, c0 = d_set(slot, n)
            return _up(ref[r0:r0 + TQ // 2, c0 * E:(c0 + 2) * E])

        def shift_job(j, r0, n, anchor=None):
            for ct in range(D // E):
                win = t_s[pl.ds(aligned(j * TB + r0, 16), n + 16), _ct(ct)]
                gs_s[r0:r0 + n, _ct(ct)] = after(
                    pltpu.roll(win, (-SHIFT[ct]) % (n + 16), 0)[8:8 + n], anchor)

        def mix(j, hook=None):
            r0 = aligned(j * TB, TB)
            for og in range(NOG):
                def prod(n):
                    m = _dot(d_lhs(3, n), _up(t2_s[og, :, _ct(n)]))
                    if hook is not None:
                        hook(m)
                    return m

                c = _strassen2(prod)
                for i in range(4):
                    for k in range(2):
                        cols = slice((4 * og + 2 * k) * E, (4 * og + 2 * k + 2) * E)
                        x1_s[i * TQ:(i + 1) * TQ, cols] = (
                            hb_s[pl.ds(r0 + i * TQ, TQ), cols].astype(f32)
                            + jnp.concatenate([c(i, 2 * k), c(i, 2 * k + 1)], axis=1))

        def base_job(j, rt, anchor):
            rows = slice(rt * 16, (rt + 1) * 16)
            z = pltpu.bitcast(pltpu.bitcast(anchor[0:8], u32) & zero_s[0:8, :], f32)
            gb = mod_rows(5, 8) + jnp.concatenate([z] * (D // E), axis=1)
            x2 = x_s[j * (TB // SEG) + rt // 2, (rt % 2) * 16:(rt % 2) * 16 + 16, :]
            base_s[rows, :] = x2.astype(f32) + jnp.concatenate([gb, gb], axis=0) * x1_s[rows, :]

        def out_copy(j, slot):
            return copy(o_s.at[slot], out_hbm.at[pl.ds(aligned(j * TB, TB), TB)], SEM_OUT + slot)

        def ln_job(r0, n, prev, anchor=None):
            if anchor is not None and len(prev) >= 2:
                anchor = anchor[0:8] + prev[-2]
            y = _ln(after(x1_s[r0:r0 + n, :], anchor))
            yn_s[r0:r0 + n, :] = y
            prev.append(y[0:8, 0:E] + y[8:16, 0:E])

        def set_job(src, slot, rt, ct, n1, n=16, anchor=None):
            blk = _outer_operand(lambda i, k: src[i * TQ + rt * n:i * TQ + (rt + 1) * n, _ct(2 * k + ct)],
                                 _LHS_TERMS[n1])
            blk[0] = after(blk[0], anchor)
            blk[3] = after(blk[3], anchor)
            for n2, v in enumerate(_lhs_set(*blk)):
                ref, r0, c0 = d_set(slot, 7 * n1 + n2)
                ref[r0 + rt * n // 2:r0 + (rt + 1) * n // 2, _ct(c0 + ct)] = _pk(v)

        def all_sets(src, slot):
            for n1 in range(7):
                for ct in range(2):
                    set_job(src, slot, 0, ct, n1, TQ)

        wm_wait(wg_s, 0, D // E, SEM_WM)
        sc8 = silu_c()
        for k in range(D // E):
            mod_s[:, _ct(5 * D // E + k)] = _dot(sc8, wg_s[k])
        shift_job(0, 0, TB)
        all_sets(gs_s, 3)
        mix(0)
        prev0 = []
        plan = {}
        for k in range(TB // 16):
            plan[T_AT[0] * (k // 2) + k % 2] = [
                functools.partial(ln_job, (k % 4) * TQ + (k // 4) * 16, 16, prev0)]
        rest = [functools.partial(shift_job, 1, (k % 4) * TQ + (k // 4) * 16, 16)
                for k in range(TB // 16)]
        rest += [functools.partial(set_job, gs_s, 3, rt, ct, n1, 16)
                 for rt in range(2) for ct in range(2) for n1 in range(7)]
        for k, job in enumerate(rest):
            plan.setdefault(k * T_AT[1] // len(rest), []).append(job)
        rest = [functools.partial(set_job, yn_s, 2, rt, ct, n1, 16)
                for rt in range(2) for ct in range(2) for n1 in range(7)]
        for k, job in enumerate(rest):
            plan.setdefault(T_AT[1] + k * (T_AT[2] - T_AT[1]) // len(rest), []).append(job)
        tick0 = [0]

        def hook0(m):
            for job in plan.pop(tick0[0], ()):
                job(anchor=m)
            tick0[0] += 1

        mixer_mm(NI - 2, hook=hook0)
        mixer_sets(mixer_prep(NI - 1, 0, SEG), mixer_prep(NI - 1, SEG, SEG), 0, w_s.at[4])
        mixer_mm(NI - 1, w_s.at[4], hook0)
        assert not plan

        def mlp_block(j, last):
            slot = j & 1

            jn = clamp(j + 2, NB - 1)
            early = [functools.partial(base_job, j, k) for k in range(TB // 16)]
            if not last:
                early += [functools.partial(shift_job, jn, (k % 4) * TQ + (k // 4) * 16, 16)
                          for k in range(TB // 16)]
            early = iter(early)

            pend = []
            tick = [0]

            def drain(m):
                tick[0] += 1
                if pend and tick[0] >= U_AT[0] and (tick[0] - U_AT[0]) % U_AT[1] == 0:
                    pend.pop(0)(m)

            def up_prod(n, g):
                m = _dot(d_lhs(2, n), _up(t3_s[g, :, _ct(n)]))
                if n in E_AT:
                    job = next(early, None)
                    if job is not None:
                        job(anchor=m)
                drain(m)
                return m

            def uset_job(tile, g, n1, r0, n, anchor=None):
                blk = _outer_operand(lambda i, k: tile(i, k, r0, n), _LHS_TERMS[n1])
                blk[0] = after(blk[0], anchor)
                blk[3] = after(blk[3], anchor)
                for n2, v in enumerate(_lhs_set(*blk)):
                    ref, rows = u_set(7 * n1 + n2)
                    ref[rows.start + r0 // 2:rows.start + (r0 + n) // 2, _ct(g)] = _pk(v)

            for g in range(NFG):
                c = _strassen2(lambda n: up_prod(n, g), 1)
                assert not pend
                tick[0] = 0
                if last and g == NFG - 1:
                    act = [[_gelu(c(i, k)) for k in range(4)] for i in range(4)]
                    for n1 in range(7):
                        uset_job(lambda i, k, r0, n: act[i][k], g, n1, 0, TQ)
                    continue
                c0 = 4 * (g % 2)
                for i in range(4):
                    for k in range(4):
                        act_s[i * TQ:(i + 1) * TQ, _ct(c0 + k)] = _gelu(c(i, k))

                def tile(i, k, r0, n, c0=c0):
                    return act_s[i * TQ + r0:i * TQ + r0 + n, _ct(c0 + k)]

                pend += [functools.partial(uset_job, tile, g, n1, r0, 16)
                         for n1 in range(7) for r0 in range(0, TQ, 16)]
            jobs = {}
            if not last:
                mix(j + 1, drain)
                assert not pend
                prev = []
                for k in range(TB // 16):
                    jobs[k * Y_AT] = functools.partial(ln_job, (k % 4) * TQ + (k // 4) * 16, 16, prev)

                def place(start, fns):
                    for fn in fns:
                        while start in jobs:
                            start += 1
                        jobs[start] = fn

                for rt in range(2):
                    place(S_AT[rt], [functools.partial(set_job, yn_s, 2, rt, ct, n1, 16)
                                     for ct in range(2) for n1 in range(7)])
                place(G_AT, [functools.partial(set_job, gs_s, 3, rt, ct, n1, 16)
                             for rt in range(2) for ct in range(2) for n1 in range(7)])

            def down_part(n, og, k0, k1):
                ref, rows = u_set(n)
                return _dot(_up(ref[rows, k0 * E:k1 * E]),
                            _up(t4_s[og, k0 * E // 2:k1 * E // 2, _ct(n)]))

            head = {}
            if last:
                head = {n: down_part(n, 0, 0, NFG - 1) for n in range(HEAD)}
            count = [0]

            def down_prod(n, og):
                if og == 0 and n in head:
                    return down_part(n, og, NFG - 1, NFG) + head[n]
                m = down_part(n, og, 0, NFG)
                job = jobs.get(count[0])
                count[0] += 1
                if job is not None:
                    job(anchor=m)
                return m

            for og in range(NOG):
                c = _strassen2(lambda n: down_prod(n, og))
                for i in range(4):
                    rows = slice(i * TQ, (i + 1) * TQ)
                    for k in range(2):
                        c0 = (4 * og + 2 * k) * E
                        o_s.at[slot][rows, c0:c0 + 2 * E] = (
                            base_s[rows, c0:c0 + 2 * E] + mod_rows(5, TQ, c0, 2 * E)
                            * jnp.concatenate([c(i, 2 * k), c(i, 2 * k + 1)], axis=1)).astype(bf16)
            out_copy(j, slot).start()

        def p3_body(j, carry):
            @pl.when(j >= 2)
            def _():
                out_copy(j - 2, j & 1).wait()

            mlp_block(j, False)
            return carry

        lax.fori_loop(0, NB - 1, _scoped("p3", p3_body), 0)
        for k in range(2):
            for cp in mlp_w_copies(0, k):
                cp.wait()
        out_copy(NB - 3, (NB - 3) % 2).wait()
        mlp_block(NB - 1, True)
        out_copy(NB - 2, (NB - 2) % 2).wait()
        out_copy(NB - 1, (NB - 1) % 2).wait()

    pl.run_scoped(
        phase_a,
        pltpu.VMEM((NSEG, M, D), bf16),
        pltpu.VMEM((7, NSEG * M // 4, D // 2), u32),
        pltpu.VMEM((3 * D // E, D, E), bf16),
        pltpu.VMEM((2, 2, D, HH, E), bf16),
        pltpu.VMEM((2, BGR, D), bf16),
        pltpu.VMEM((2, 2, G1R, D), bf16),
        pltpu.VMEM((NC, D // 4, 5 * HG // 2 * E), u32),
        pltpu.VMEM((2 * D // E, 8, E), f32),
    )
    pl.run_scoped(
        phase_b,
        pltpu.VMEM((NOG, D // 8, 49 * E), u32),
        pltpu.VMEM((NFG, D // 8, 49 * E), u32),
        pltpu.VMEM((NOG, F // 8, 49 * E), u32),
        pltpu.VMEM((D // E, D, E), bf16),
        pltpu.VMEM((TB, D), f32),
        pltpu.VMEM((TB, D), f32),
        pltpu.VMEM((TB, D), f32),
        pltpu.VMEM((TB, D), f32),
        pltpu.VMEM((TB, D), f32),
        pltpu.VMEM((2, TB, D), bf16),
    )


@jax.jit
def pallas_adaLN_cond__memory_aug_recurrent_mem_tr__mixer_s_mlp__prompt_kernel(
    A_x: jax.Array,
    A_mem0: jax.Array,
    A_Wq: jax.Array,
    A_Wk: jax.Array,
    A_Wv: jax.Array,
    A_Wo: jax.Array,
    A_seg_len,
    B_x: jax.Array,
    B_w1: jax.Array,
    B_w2: jax.Array,
    B_w3: jax.Array,
    B_w4: jax.Array,
    c: jax.Array,
    w_mod: jax.Array,
):
    del A_seg_len, B_x
    assert A_x.shape == (1, S, D) and A_mem0.shape == (1, M, D)
    hbm = pl.BlockSpec(memory_space=pl.ANY)
    scratch = [
        pltpu.VMEM((NSEG, SEG, D), bf16),
        pltpu.VMEM((NC, D // 2, HG * E), u32),
        pltpu.VMEM((H * E // 2, D), u32),
        pltpu.VMEM((7, D // 4, D // 2), u32),
        pltpu.VMEM((2, 4, 16, 4 * E), bf16),
        pltpu.VMEM((2, 4, 64, 4 * E), bf16),
        pltpu.VMEM((2, 4, 32, D), bf16),
        pltpu.VMEM((NC, NSEG * M, HG // 2 * E), u32),
        pltpu.VMEM((8, 6 * D), f32),
        pltpu.VMEM((M, D), f32),
        pltpu.VMEM((TC, D), f32),
        pltpu.VMEM((2 * SEG, D), f32),
        pltpu.VMEM((E, E), f32),
        pltpu.VMEM((S, D), bf16),
        pltpu.VMEM((S + 16, D), f32),
        pltpu.VMEM((7 * SEG // 2, D // 2), u32),
        pltpu.VMEM((16, E), u32),
        pltpu.VMEM((1, D), bf16),
        pltpu.VMEM((M, D), bf16),
        pltpu.SemaphoreType.DMA((26,)),
    ]
    out = pl.pallas_call(
        _kernel,
        out_shape=jax.ShapeDtypeStruct((S, D), bf16),
        in_specs=[hbm] * 12,
        out_specs=hbm,
        scratch_shapes=scratch,
        compiler_params=pltpu.CompilerParams(vmem_limit_bytes=127 * 1024 * 1024,
                                             disable_bounds_checks=NO_CHECKS,
                                             disable_semaphore_checks=NO_CHECKS),
    )(A_x.reshape(NSEG, SEG, D), A_mem0.reshape(M, D), A_Wq, A_Wk, A_Wv,
      A_Wo.reshape(H * E, D), B_w1.reshape(2, D // 2, D), B_w2.reshape(4, D // 4, D), B_w3.reshape(4, D // 4, F),
      B_w4.reshape(NFG, 4, E, D), c, w_mod)
    return out.reshape(1, S, D)
```

```python
import functools

import jax
import jax.numpy as jnp
from jax import lax
import jax.experimental.pallas as pl
import jax.experimental.pallas.tpu as pltpu

bf16, f32, u32 = jnp.bfloat16, jnp.float32, jnp.uint32

S, D, H, E, M, SEG, F = 2048, 1024, 32, 128, 8, 32, 3584
EPS = 1e-5
SCALE = E ** -0.5
NSEG = S // SEG
NI = NSEG // 2
NP = H // 2
NR = 2 * (M + SEG)
TC = SEG - M
HG = 8
HH = HG // 2
NG = H // HG
NC = 3 * NG
BGR = 384
G1R = 48
X0 = 4
TB = 128
NB = S // TB
HD = D // 2
NQ = D // E // 2
NFG = F // (4 * E)
NOG = D // (4 * E)

PIN_ROWS = 256
P1_LAG, P1_TAIL, P1_PIN, P1_FROM = 4, 4, 55, 55
PREP_AT = (0, 1, 4, 5)
T_AT = (7, 28, 52)
E_AT = (10, 24, 34)
U_AT = (6, 3)
Y_AT, S_AT, G_AT = 4, (26, 44), 62
HEAD = 14
HN_AT = 3
NO_CHECKS = True
_SCOPES = False


def _scoped(name, fn):
    def wrapped(*a):
        if not _SCOPES:
            return fn(*a)
        with jax.named_scope(name):
            return fn(*a)
    return wrapped


def _pk(x):
    return pltpu.bitcast(x.astype(bf16), u32)


def _up(x):
    return pltpu.bitcast(x, bf16)


def _ct(k):
    return slice(k * E, (k + 1) * E)


def _dot(a, b):
    return jnp.dot(a, b, preferred_element_type=f32)


def _ln(x):
    m = jnp.mean(x, axis=-1, keepdims=True)
    xc = x - m
    v = jnp.mean(xc * xc, axis=-1, keepdims=True)
    return xc * lax.rsqrt(v + EPS)


def _gelu(x):
    c = 0.7978845608028654
    return 0.5 * x * (1.0 + jnp.tanh(c * (x + 0.044715 * (x * x * x))))


def _lhs_set(a11, a12, a21, a22):
    return (a11 + a22, a21 + a22, a11, a22, a11 + a12, a21 - a11, a12 - a22)


def _rhs_set(b11, b12, b21, b22):
    return (b11 + b22, b11, b12 - b22, b21 - b11, b22, b11 + b12, b21 + b22)


_LHS_TERMS = (((0, 1), (3, 1)), ((2, 1), (3, 1)), ((0, 1),), ((3, 1),),
              ((0, 1), (1, 1)), ((2, 1), (0, -1)), ((1, 1), (3, -1)))
_RHS_TERMS = (((0, 1), (3, 1)), ((0, 1),), ((1, 1), (3, -1)), ((2, 1), (0, -1)),
              ((3, 1),), ((0, 1), (1, 1)), ((2, 1), (3, 1)))


def _outer_operand(tile, terms):
    out = []
    for i in range(2):
        for j in range(2):
            v = None
            for o, sign in terms:
                t = tile(2 * (o // 2) + i, 2 * (o % 2) + j)
                v = t if v is None else (v + t if sign > 0 else v - t)
            out.append(v)
    return out


class _Quad:
    def __init__(self, tiles):
        self.t = tuple(tiles)

    def __add__(self, other):
        return _Quad([a + b for a, b in zip(self.t, other.t)])

    def __sub__(self, other):
        return _Quad([a - b for a, b in zip(self.t, other.t)])


def _strassen2(m, order=0):
    cs = _strassen(lambda n1: _Quad(_strassen(lambda n2: m(7 * n1 + n2))), order)
    return lambda i, j: cs[2 * (i // 2) + j // 2].t[2 * (i % 2) + j % 2]


def _strassen(m, order=0):
    if order == 0:
        m1 = m(0)
        m2 = m(1)
        c22 = m1 - m2
        m3 = m(2)
        c22 = c22 + m3
        c22 = m(5) + c22
        m4 = m(3)
        c21 = m2 + m4
        c11 = m1 + m4
        m5 = m(4)
        c12 = m3 + m5
        c11 = c11 - m5
        c11 = m(6) + c11
    else:
        m2 = m(1)
        c22 = m(5) - m2
        m4 = m(3)
        c21 = m2 + m4
        m1 = m(0)
        c22 = c22 + m1
        c11 = m4 + m1
        m3 = m(2)
        c22 = c22 + m3
        m5 = m(4)
        c12 = m3 + m5
        c11 = c11 - m5
        c11 = m(6) + c11
    return c11, c12, c21, c22


def _mask_fill():
    shape = (NR, E)
    r = lax.broadcasted_iota(jnp.int32, shape, 0)
    c = lax.broadcasted_iota(jnp.int32, shape, 1)

    def headpos(i):
        head = jnp.where(i < 64, i >> 5, (i - 64) >> 3)
        pos = jnp.where(i < 64, i & 31, 32 + (i & 7))
        return head, pos

    hr, pr = headpos(r)
    hc, pc = headpos(c)
    same = hr == hc
    valid = same & ((pr < M) | (pr >= pc))
    return jnp.where(valid, 0.0, jnp.where(same, -1e9, -jnp.inf)).astype(f32)


def _kernel(x_hbm, mem0_hbm, wq_hbm, wk_hbm, wv_hbm, wo_hbm, w1_hbm, w2_hbm, w3_hbm,
            w4_hbm, c_hbm, wm_hbm,
            out_hbm,
            x_s, w_s, wo_s, t1_s, g2, g3, g4, pre_s, mod_s, mem_s, hn_s, aout_s, fill_s,
            hb_s, t_s, l1_s, zero_s, c_s, mem0_s, sems):
    w_hbm = (wq_hbm, wk_hbm, wv_hbm)

    (SEM_C, SEM_MEM, SEM_XPRE, SEM_X, SEM_WMR, SEM_BG, SEM_OUT, SEM_G1,
     SEM_G2, SEM_G3, SEM_G4, SEM_WM, SEM_STG) = (0, 1, 2, 3, 4, 6, 8, 10, 12, 14, 16, 18, 22)

    def copy(src, dst, k):
        return pltpu.make_async_copy(src, dst, sems.at[k])

    def aligned(x, n):
        return x if isinstance(x, int) else pl.multiple_of(x, n)

    def clamp(k, hi):
        return min(k, hi) if isinstance(k, int) else jnp.minimum(k, hi)

    def mlp_piece(k):
        k = clamp(k, 4 * NFG - 1)
        return k >> 2, k & 3

    def mlp_w_copies(k, slot):
        g, rr = mlp_piece(k)
        k2 = clamp(k, NI - 1)
        return (copy(w2_hbm.at[:, pl.ds(aligned((k2 >> 1) * 16, 16), 16),
                               pl.ds(aligned((k2 & 1) * 4 * E, E), 4 * E)], g2.at[slot], SEM_G2 + slot),
                copy(w3_hbm.at[:, pl.ds(aligned(rr * 64, 64), 64), pl.ds(aligned(g * 4 * E, E), 4 * E)],
                     g3.at[slot], SEM_G3 + slot),
                copy(w4_hbm.at[g, :, pl.ds(aligned(rr * 32, 32), 32), :], g4.at[slot], SEM_G4 + slot))

    def pinned(w, job):
        if job is None:
            return w()
        z = job() & zero_s[0:8, :]
        w = w()
        return jnp.concatenate([w[0:8] | z, w[8:]], axis=0)

    def after(x, anchor):
        if anchor is None:
            return x
        z = pltpu.bitcast(pltpu.bitcast(anchor[0:8], u32) & zero_s[0:8, :], f32)
        z = jnp.concatenate([z] * (x.shape[0] // 8), axis=0)
        return jnp.concatenate([x[:, 0:E] + z, x[:, E:]], axis=1) if x.shape[1] > E else x + z

    def rhs_job(src, slot, r0, q, dst, row, z):
        blk = [src[slot, kh, r0:r0 + 16, _ct(cc)].astype(f32)
               for kh in range(2) for cc in (q, NQ + q)]
        zf = pltpu.bitcast(jnp.concatenate([z, z], axis=0), f32)
        blk[0] = blk[0] + zf
        blk[3] = blk[3] + zf
        for n, v in enumerate(_rhs_set(*blk)):
            dst.at[n][pl.ds(aligned(row, 8), 8), _ct(q)] = _pk(v)

    def rhs2_job(src, slot, r0, c0, n1, dst, row):
        blk = _outer_operand(lambda i, j: src[slot, i, r0:r0 + 16, _ct(c0 + j)].astype(f32),
                             _RHS_TERMS[n1])
        sets = _rhs_set(*blk)
        for n2, v in enumerate(sets):
            dst[pl.ds(pl.multiple_of(row, 8), 8), _ct(7 * n1 + n2)] = _pk(v)
        out = pltpu.bitcast(sets[2], u32) | pltpu.bitcast(sets[3], u32)
        return out[0:8] | out[8:16]

    def silu_c():
        cf = c_s[...].astype(f32)
        return jnp.broadcast_to(cf * (1.0 / (1.0 + jnp.exp(-cf))), (8, D)).astype(bf16)

    def wm_copy(wm_s, src_tile, dst_tile, sem):
        return copy(wm_hbm.at[:, pl.ds(aligned(src_tile * E, E), E)], wm_s.at[dst_tile], sem)

    def wm_wait(wm_s, t0, n, sem):
        copy(wm_s.at[pl.ds(t0, n)], wm_s.at[pl.ds(t0, n)], sem).wait()

    def x_copy(k):
        r = slice(0, X0) if k == 0 else slice(X0, NSEG)
        return copy(x_hbm.at[r], x_s.at[r], SEM_XPRE if k == 0 else SEM_X)

    def h_rows(xr, anchor=None):
        return _ln(after(xr.astype(f32), anchor)) * mod_rows(1, TC) + mod_rows(0, TC)

    def mod_rows(k, n, c0=0, w=D):
        return jnp.concatenate([mod_s[:, k * D + c0:k * D + c0 + w]] * (n // 8), axis=0)

    def phase_a(xpre_s, hpre_s, wm_s, stg, bg, g1, tq_s, modt_s):
        def tq_place(c, n):
            if n == 1:
                return w_s.at[c], 0, None
            if n == 4:
                return w_s.at[c], D // 4, None
            return tq_s.at[c], 0, (0, 2, 3, 5, 6).index(n) * (HG // 2)

        def w_copy(t, g, slot, hf):
            return copy(w_hbm[t].at[:, pl.ds(aligned(g * HH, HH), HH), :], stg.at[slot, hf],
                        SEM_STG + 2 * slot + hf)

        def bg_rows(k):
            return clamp(k * BGR, H * E - BGR), clamp(k * G1R, HD - G1R)

        def bg_copies(k, slot):
            ro, r1 = bg_rows(k)
            return (copy(wo_hbm.at[pl.ds(aligned(ro, 16), BGR)], bg.at[slot], SEM_BG + slot),
                    copy(w1_hbm.at[:, pl.ds(aligned(r1, 16), G1R), :], g1.at[slot], SEM_G1 + slot))

        def relayout_jobs(slot, hf, c, j0, i):
            memo = []
            r = aligned(i * 8, 8)

            def job(jj, z=None):
                if not memo:
                    for d0 in (i * 16, HD + i * 16):
                        memo.append(jnp.swapaxes(pltpu.bitcast(stg[slot, hf, pl.ds(d0, 16)], u32), 0, 1))
                j = j0 + jj
                blk = []
                for kh in range(2):
                    u = memo[kh][jj]
                    if z is not None:
                        u = u | jnp.concatenate([z, z], axis=0)
                    blk.append(pltpu.bitcast(u << 16, f32))
                    blk.append(pltpu.bitcast(u & jnp.uint32(0xFFFF0000), f32))
                for k, v in enumerate(blk):
                    w_s.at[c][pl.ds((k // 2) * (D // 4) + r, 8), _ct(2 * j + k % 2)] = _pk(v)
                sets = _rhs_set(*blk)
                for n, v in enumerate(sets):
                    if n not in (1, 4):
                        ref, r0, c0 = tq_place(c, n)
                        ref[pl.ds(r0 + r, 8), _ct(c0 + j)] = _pk(v)
                out = pltpu.bitcast(sets[2], u32) | pltpu.bitcast(sets[3], u32)
                return out[0:8] | out[8:16]

            return [functools.partial(job, jj) for jj in range(2)]

        def repack(slot, row, i, z):
            v = pltpu.bitcast(bg[slot, 16 * i:16 * i + 16, :], u32)
            v = v | jnp.concatenate([z] * (D // E), axis=1)
            wo_s[pl.ds(aligned(row + 8 * i, 8), 8), :] = v

        cp_c = copy(c_hbm, c_s, SEM_C)
        cp_mem = copy(mem0_hbm, mem0_s, SEM_MEM)
        cp_xpre = copy(x_hbm.at[:, TC:SEG, :], xpre_s, SEM_XPRE)
        w_copy(0, 0, 0, 0).start()
        cp_xpre.start()
        cp_c.start()
        cp_mem.start()
        for k in range(2 * D // E):
            wm_copy(wm_s, k, k, SEM_WM + k // 4).start()
        w_copy(0, 1, 0, 1).start()
        w_copy(0, 2, 1, 0).start()
        w_copy(0, 3, 1, 1).start()

        zero_s[0:8, :] = jnp.zeros((8, E), u32)
        fill_s[0:NR, :] = _mask_fill()
        aout_s[...] = jnp.zeros(aout_s.shape, f32)
        l1_s[...] = jnp.zeros(l1_s.shape, u32)
        bg[1] = jnp.zeros(bg.shape[1:], bf16)
        g1[1] = jnp.zeros(g1.shape[1:], bf16)

        w_copy(0, 0, 0, 0).wait()

        def rl0_body(i, carry):
            for job in relayout_jobs(0, 0, 0, 0, i):
                job()
            return carry

        lax.fori_loop(0, D // 32, rl0_body, 0)
        cp_xpre.wait()

        def npre_body(i, carry):
            xr = xpre_s[pl.ds(pl.multiple_of(i * 8, 8), 8)].astype(f32).reshape(64, D)
            t_s[pl.ds(pl.multiple_of(i * 64, 64), 64), :] = _ln(xr)
            return carry

        lax.fori_loop(0, NSEG // 8, _scoped("npre", npre_body), 0)

        cp_c.wait()
        cp_mem.wait()
        mem_s[...] = mem0_s[...].astype(f32)

        sc8 = silu_c()

        def mod_body(k, carry):
            wm_wait(wm_s, 4 * k, 4, SEM_WM + k)
            for kk in range(4):
                modt_s[4 * k + kk] = _dot(sc8, wm_s[4 * k + kk])
            return carry

        lax.fori_loop(0, 4, mod_body, 0)
        for k in range(2 * D // E):
            mod_s[:, _ct(k)] = modt_s[k] if k < D // E else 1.0 + modt_s[k]

        PH = NSEG * M // 2

        def hpre_body(i, carry):
            h = [t_s[pl.ds(pl.multiple_of(hf * PH + i * 16, 16), 16), :] * mod_rows(1, 16) + mod_rows(0, 16)
                 for hf in range(2)]
            for n, v in enumerate(_lhs_set(h[0][:, :HD], h[0][:, HD:], h[1][:, :HD], h[1][:, HD:])):
                hpre_s.at[n][pl.ds(pl.multiple_of(i * 8, 8), 8), :] = _pk(v)
            return carry

        lax.fori_loop(0, PH // 16, _scoped("hpre", hpre_body), 0)

        t_s[0:8, :] = jnp.zeros((8, D), f32)
        t_s[S + 8:S + 16, :] = jnp.zeros((8, D), f32)

        MB = 64

        nu = D // 32

        def small_jobs(slot, k):
            ro, r1 = bg_rows(k)
            return ([functools.partial(repack, slot, ro >> 1, i) for i in range(BGR // 16)]
                    + [functools.partial(rhs_job, g1, slot, 16 * rt, q, t1_s, (r1 >> 1) + 8 * rt)
                       for rt in range(G1R // 16) for q in range(NQ)])

        def p1_pairs(pairs, first, work, start, extra=None):
            npin = 7 * len(pairs) * (PH // MB)
            pins = [[] for _ in range(npin)]
            for k, job in enumerate(first):
                pins[1 + k * (P1_PIN - 1) // len(first)].append(job)
            pins = iter(pins)
            jobs = [[] for _ in range(npin)]
            for k, job in enumerate(work):
                pos = start * 8 + k * (npin - P1_TAIL - start) * 8 // len(work)
                jobs[pos // 8].append((job, pos % 8))
            jobs = iter(jobs)
            pending = []

            def run(group):
                z = group[0]()
                for job in group[1:]:
                    z = z | job()
                return z

            def prod(n, c, q, mb):
                ref, r0, c0 = tq_place(c, n)
                group = next(pins)
                w = pinned(lambda: ref[r0:r0 + D // 4, _ct(2 * q + (n == 4) if c0 is None else c0 + q)],
                           functools.partial(run, group) if group else None)
                m = _dot(_up(hpre_s[n, mb * MB // 2:(mb + 1) * MB // 2, :]), _up(w))
                pending.append(m)
                if len(pending) > P1_LAG:
                    anchor = pltpu.bitcast(pending.pop(0), u32)
                    for job, g in next(jobs):
                        job(anchor[8 * g:8 * g + 8] & zero_s[0:8, :])
                if extra is not None:
                    extra()
                return m

            ns = MB // M
            for c, q in pairs:
                for mb in range(PH // MB):
                    cs = _strassen(lambda n: prod(n, c, q, mb))
                    for hf in range(2):
                        y = jnp.concatenate([cs[2 * hf + k][sg * M:(sg + 1) * M]
                                             for sg in range(ns) for k in range(2)], axis=0)
                        s0 = hf * (NSEG // 2) + mb * ns
                        pre_s.at[c][s0 * M:(s0 + ns) * M, _ct(q)] = _pk(y)

        w_copy(0, 0, 0, 1).wait()
        p1_pairs([(0, 0), (0, 1)], [], [job for i in range(nu) for job in relayout_jobs(0, 1, 0, 2, i)], 0)
        for hf in range(2):
            w_copy(0, 4 + hf, 0, hf).start()
        for cp in bg_copies(0, 0):
            cp.start()

        def wm_rest(k):
            for kk in (k, k + 1):
                wm_copy(wm_s, 2 * D // E + kk, kk, SEM_WMR).start()

        wm_rest(0)

        def p1_body(c, carry):
            pslot = 1 - (c & 1)

            @pl.when(c >= 1)
            def _():
                for cp in bg_copies(0, pslot):
                    cp.wait()

            for hf in range(2):
                w_copy(0, 0, pslot, hf).wait()

            small = small_jobs(pslot, jnp.maximum(c - 1, 0))
            work = []
            for i in range(nu):
                work += relayout_jobs(pslot, 1, c + 1, 2, i)
                work += small[i * len(small) // nu:(i + 1) * len(small) // nu]
            p1_pairs([(c, 2), (c, 3), (c + 1, 0), (c + 1, 1)],
                     [job for i in range(nu) for job in relayout_jobs(pslot, 0, c + 1, 0, i)],
                     work, P1_FROM)

            for t in range(3):
                @pl.when((c + 3) >> 2 == t)
                def _():
                    for hf in range(2):
                        w_copy(t, 2 * ((c + 3) & 3) + hf, pslot, hf).start()

            @pl.when(c + 2 < NC)
            def _():
                for cp in bg_copies(c + 1, pslot):
                    cp.start()
                wm_rest(2 * c + 2)

            @pl.when(c == NC - 3)
            def _():
                wm_rest(2 * NC - 2)
                x_copy(0).start()

            return carry

        lax.fori_loop(0, NC - 1, _scoped("p1", p1_body), 0)
        for k in range(2):
            for cp in mlp_w_copies(k, k):
                cp.start()
        x_copy(1).start()
        for cp in bg_copies(0, NC & 1):
            cp.wait()
        x_copy(0).wait()
        wm_wait(wm_s, 0, 3 * D // E, SEM_WMR)

        halves = iter(range(2 * 3 * D // E))
        part = []

        def mod_half():
            k = next(halves, None)
            if k is None:
                return
            rows = slice((k % 2) * HD, (k % 2 + 1) * HD)
            v = _dot(sc8[:, rows], wm_s[k // 2, rows, :])
            if k % 2 == 0:
                part.append(v)
            else:
                v = v + part.pop()
                tile = 2 * D // E + k // 2
                mod_s[:, _ct(tile)] = 1.0 + v if tile // (D // E) == 4 else v

        p1_pairs([(NC - 1, 2), (NC - 1, 3)], [], small_jobs(NC & 1, NC - 2), 0, mod_half)
        hn_s[...] = h_rows(x_s[0, 0:TC, :])

    def phase_b(t2_s, t3_s, t4_s, wg_s, x1_s, base_s, yn_s, gs_s, act_s, o_s):
        for k in range(D // E):
            wm_copy(wg_s, 5 * D // E + k, k, SEM_WM).start()

        def chain_step(s, mem, htok, odef_prev, jobs=(), hooks=None):
            hs = jnp.concatenate([mem, htok], axis=0).astype(bf16)
            qkv = [[None] * 3 for _ in range(NP)]
            ps = [None] * NP
            os_ = [None] * H
            odef = [None] * H

            def proj(p, t):
                c, q = t * NG + p // (HG // 2), p % (HG // 2)
                a = _dot(hs, _up(w_s[c, :, _ct(2 * q)]))
                b = _dot(hs, _up(w_s[c, :, _ct(2 * q + 1)]))
                pre = pre_s[c, pl.ds(pl.multiple_of(s * M, M), M), _ct(q)]
                parts = [a, b, _up(pre).astype(f32)]
                if t > 0:
                    parts.append(jnp.zeros((E - NR, E), f32))
                v = jnp.concatenate(parts, axis=0)
                qkv[p][t] = (v.T if t == 1 else v).astype(bf16)

            def scores(p):
                sc_ = _dot(qkv[p][0], qkv[p][1])
                fill = fill_s[0:NR, :]
                sc_ = jnp.where(fill == 0.0, sc_ * SCALE, fill)
                m = jnp.max(sc_, axis=-1, keepdims=True)
                e = jnp.exp(sc_ - m)
                l = jnp.sum(e, axis=-1, keepdims=True)
                r = pl.reciprocal(l, approx=True)
                r = r * (2.0 - l * r)
                ps[p] = (e * r).astype(bf16)

            def fin(p):
                o = _dot(ps[p], qkv[p][2])
                for hh in range(2):
                    h = 2 * p + hh
                    rows = o[32 * hh:32 * hh + 32]
                    odef[h] = o[64 + 8 * hh:72 + 8 * hh]
                    if odef_prev is not None:
                        rows = jnp.concatenate([rows, odef_prev[h], odef[h]], axis=0)
                    os_[h] = _pk(rows)

            acc = [None] * 8
            jobs = iter(jobs)

            def wo(h0, h1, js):
                lhs = _up(jnp.concatenate(os_[h0:h1], axis=1))
                for j in js:
                    ws = []
                    for r0 in range(h0 * E // 2, h1 * E // 2, PIN_ROWS):
                        ws.append(pinned(lambda: wo_s[r0:r0 + PIN_ROWS, j * E:(j + 1) * E],
                                         next(jobs, None)))
                    part = _dot(lhs, _up(jnp.concatenate(ws, axis=0)))
                    if hooks and acc[j] is None and j in hooks:
                        hooks[j](part)
                    acc[j] = part if acc[j] is None else part + acc[j]

            for p in range(NP):
                attn = [functools.partial(scores, p - 1) if p >= 1 else None,
                        functools.partial(fin, p - 3) if p >= 3 else None]
                if odef_prev is not None:
                    attn.reverse()
                for t, f in zip((1, 0, 2), attn + [None]):
                    proj(p, t)
                    if f is not None:
                        f()
            hsplit = 24
            wo(0, hsplit, range(0, 2))
            scores(NP - 1)
            fin(NP - 3)
            wo(0, hsplit, range(2, 3))
            fin(NP - 2)
            wo(0, hsplit, range(3, 5))
            fin(NP - 1)
            wo(0, hsplit, range(5, 8))
            wo(hsplit, H, range(8))
            return jnp.concatenate(acc, axis=1), odef

        def mixer_prep(i, r0, n, anchor=None):
            r = pl.ds(aligned(i * 64 + r0, 16), n)
            xr = x_s[2 * i + r0 // SEG, r0 % SEG:r0 % SEG + n, :].astype(f32)
            x2 = xr + mod_rows(2, n) * after(aout_s[r0:r0 + n, :], anchor)
            x_s.at[2 * i + r0 // SEG][r0 % SEG:r0 % SEG + n, :] = x2.astype(bf16)
            hb = _ln(x2) * mod_rows(4, n) + mod_rows(3, n)
            hb_s[r, :] = hb.astype(bf16)
            return _ln(hb)

        def mixer_sets(ya, yb, r0, dst=l1_s):
            n = ya.shape[0]
            for m, v in enumerate(_lhs_set(ya[:, :HD], ya[:, HD:], yb[:, :HD], yb[:, HD:])):
                dst[m * (SEG // 2) + r0 // 2:m * (SEG // 2) + (r0 + n) // 2, 0:HD] = _pk(v)

        def mixer_mm(i, src=l1_s, hook=None):
            for q in range(NQ):
                def prod(n):
                    m = _dot(_up(src[n * (SEG // 2):(n + 1) * (SEG // 2), 0:HD]),
                             _up(t1_s[n, :, _ct(q)]))
                    if hook is not None:
                        hook(m)
                    return m

                cs = _strassen(prod)
                for k, cc in enumerate(cs):
                    r0 = aligned(i * 64 + 8 + (k // 2) * SEG, 8)
                    t_s[pl.ds(r0, SEG), _ct(q + NQ * (k % 2))] = _gelu(cc)

        def p2_body(i, carry):
            slot = i & 1
            for cp in mlp_w_copies(0, slot):
                cp.wait()

            @pl.when(i == 1)
            def _():
                x_copy(1).wait()

            g, rr = mlp_piece(i)
            work = [functools.partial(rhs2_job, g2, slot, 0, 0, n1, t2_s.at[slot], (i >> 1) * 8)
                    for n1 in range(7)]
            work += [functools.partial(rhs2_job, g3, slot, 16 * rt, 0, n1, t3_s.at[g], rr * 32 + 8 * rt)
                     for rt in range(4) for n1 in range(7)]
            work += [functools.partial(rhs2_job, g4, slot, 16 * rt, 4 * og, n1, t4_s.at[og],
                                       g * (E // 2) + rr * 16 + 8 * rt)
                     for rt in range(2) for og in range(NOG) for n1 in range(7)]
            jobs = [None] + work

            sa_ = 2 * i
            sb_ = 2 * i + 1
            hb_tok = h_rows(x_s[sb_, 0:TC, :])
            oa, odef_a = chain_step(sa_, mem_s[...], hn_s[...], None)
            xn = x_s[jnp.minimum(sb_ + 1, NSEG - 1), 0:TC, :]
            mixer_mm(jnp.maximum(i - 2, 0))
            ys = []

            def hook(k, anchor):
                if k >= 2:
                    anchor = anchor[0:8] + ys[-2][0:8, 0:E] + ys[-2][8:16, 0:E]
                ys.append(mixer_prep(jnp.maximum(i - 1, 0), (k % 2) * SEG + (k // 2) * 16, 16, anchor))
                if k % 2:
                    mixer_sets(ys[-2], ys[-1], (k // 2) * 16)

            hooks = {j: functools.partial(hook, k) for k, j in enumerate(PREP_AT)}
            ob, _ = chain_step(sb_, oa[0:M], hb_tok, odef_a, jobs, hooks)
            mem_s[...] = ob[0:M]
            aout_s[0:TC, :] = oa[M:SEG]
            aout_s[TC:SEG, :] = ob[SEG:SEG + M]
            aout_s[SEG:SEG + TC, :] = ob[M:SEG]
            aout_s[SEG + TC:2 * SEG, :] = ob[SEG + M:SEG + 2 * M]
            hn_s[...] = h_rows(xn, ob[:, _ct(HN_AT)])
            for cp in mlp_w_copies(i + 2, slot):
                cp.start()
            return carry

        lax.fori_loop(0, NI, _scoped("p2", p2_body), 0)

        TQ = TB // 4
        SHIFT = (-1, -1, 1, 1, -2, -2, 2, 2)

        def u_set(n):
            return w_s.at[n // 32], slice((n % 32) * (TQ // 2), (n % 32 + 1) * (TQ // 2))

        def d_set(slot, n):
            return w_s.at[slot], (n // 4) * (TQ // 2), (n % 4) * 2

        def d_lhs(slot, n):
            ref, r0, c0 = d_set(slot, n)
            return _up(ref[r0:r0 + TQ // 2, c0 * E:(c0 + 2) * E])

        def shift_job(j, r0, n, anchor=None):
            for ct in range(D // E):
                win = t_s[pl.ds(aligned(j * TB + r0, 16), n + 16), _ct(ct)]
                gs_s[r0:r0 + n, _ct(ct)] = after(
                    pltpu.roll(win, (-SHIFT[ct]) % (n + 16), 0)[8:8 + n], anchor)

        def mix(j, hook=None):
            r0 = aligned(j * TB, TB)
            for og in range(NOG):
                def prod(n):
                    m = _dot(d_lhs(3, n), _up(t2_s[og, :, _ct(n)]))
                    if hook is not None:
                        hook(m)
                    return m

                c = _strassen2(prod)
                for i in range(4):
                    for k in range(2):
                        cols = slice((4 * og + 2 * k) * E, (4 * og + 2 * k + 2) * E)
                        x1_s[i * TQ:(i + 1) * TQ, cols] = (
                            hb_s[pl.ds(r0 + i * TQ, TQ), cols].astype(f32)
                            + jnp.concatenate([c(i, 2 * k), c(i, 2 * k + 1)], axis=1))

        def base_job(j, rt, anchor):
            rows = slice(rt * 16, (rt + 1) * 16)
            z = pltpu.bitcast(pltpu.bitcast(anchor[0:8], u32) & zero_s[0:8, :], f32)
            gb = mod_rows(5, 8) + jnp.concatenate([z] * (D // E), axis=1)
            x2 = x_s[j * (TB // SEG) + rt // 2, (rt % 2) * 16:(rt % 2) * 16 + 16, :]
            base_s[rows, :] = x2.astype(f32) + jnp.concatenate([gb, gb], axis=0) * x1_s[rows, :]

        def out_copy(j, slot):
            return copy(o_s.at[slot], out_hbm.at[pl.ds(aligned(j * TB, TB), TB)], SEM_OUT + slot)

        def ln_job(r0, n, prev, anchor=None):
            if anchor is not None and len(prev) >= 2:
                anchor = anchor[0:8] + prev[-2]
            y = _ln(after(x1_s[r0:r0 + n, :], anchor))
            yn_s[r0:r0 + n, :] = y
            prev.append(y[0:8, 0:E] + y[8:16, 0:E])

        def set_job(src, slot, rt, ct, n1, n=16, anchor=None):
            blk = _outer_operand(lambda i, k: src[i * TQ + rt * n:i * TQ + (rt + 1) * n, _ct(2 * k + ct)],
                                 _LHS_TERMS[n1])
            blk[0] = after(blk[0], anchor)
            blk[3] = after(blk[3], anchor)
            for n2, v in enumerate(_lhs_set(*blk)):
                ref, r0, c0 = d_set(slot, 7 * n1 + n2)
                ref[r0 + rt * n // 2:r0 + (rt + 1) * n // 2, _ct(c0 + ct)] = _pk(v)

        def all_sets(src, slot):
            for n1 in range(7):
                for ct in range(2):
                    set_job(src, slot, 0, ct, n1, TQ)

        wm_wait(wg_s, 0, D // E, SEM_WM)
        sc8 = silu_c()
        for k in range(D // E):
            mod_s[:, _ct(5 * D // E + k)] = _dot(sc8, wg_s[k])
        shift_job(0, 0, TB)
        all_sets(gs_s, 3)
        mix(0)
        prev0 = []
        plan = {}
        for k in range(TB // 16):
            plan[T_AT[0] * (k // 2) + k % 2] = [
                functools.partial(ln_job, (k % 4) * TQ + (k // 4) * 16, 16, prev0)]
        rest = [functools.partial(shift_job, 1, (k % 4) * TQ + (k // 4) * 16, 16)
                for k in range(TB // 16)]
        rest += [functools.partial(set_job, gs_s, 3, rt, ct, n1, 16)
                 for rt in range(2) for ct in range(2) for n1 in range(7)]
        for k, job in enumerate(rest):
            plan.setdefault(k * T_AT[1] // len(rest), []).append(job)
        rest = [functools.partial(set_job, yn_s, 2, rt, ct, n1, 16)
                for rt in range(2) for ct in range(2) for n1 in range(7)]
        for k, job in enumerate(rest):
            plan.setdefault(T_AT[1] + k * (T_AT[2] - T_AT[1]) // len(rest), []).append(job)
        tick0 = [0]

        def hook0(m):
            for job in plan.pop(tick0[0], ()):
                job(anchor=m)
            tick0[0] += 1

        mixer_mm(NI - 2, hook=hook0)
        mixer_sets(mixer_prep(NI - 1, 0, SEG), mixer_prep(NI - 1, SEG, SEG), 0, w_s.at[4])
        mixer_mm(NI - 1, w_s.at[4], hook0)
        assert not plan

        def mlp_block(j, last):
            slot = j & 1

            jn = clamp(j + 2, NB - 1)
            early = [functools.partial(base_job, j, k) for k in range(TB // 16)]
            if not last:
                early += [functools.partial(shift_job, jn, (k % 4) * TQ + (k // 4) * 16, 16)
                          for k in range(TB // 16)]
            early = iter(early)

            pend = []
            tick = [0]

            def drain(m):
                tick[0] += 1
                if pend and tick[0] >= U_AT[0] and (tick[0] - U_AT[0]) % U_AT[1] == 0:
                    pend.pop(0)(m)

            def up_prod(n, g):
                m = _dot(d_lhs(2, n), _up(t3_s[g, :, _ct(n)]))
                if n in E_AT:
                    job = next(early, None)
                    if job is not None:
                        job(anchor=m)
                drain(m)
                return m

            def uset_job(tile, g, n1, r0, n, anchor=None):
                blk = _outer_operand(lambda i, k: tile(i, k, r0, n), _LHS_TERMS[n1])
                blk[0] = after(blk[0], anchor)
                blk[3] = after(blk[3], anchor)
                for n2, v in enumerate(_lhs_set(*blk)):
                    ref, rows = u_set(7 * n1 + n2)
                    ref[rows.start + r0 // 2:rows.start + (r0 + n) // 2, _ct(g)] = _pk(v)

            for g in range(NFG):
                c = _strassen2(lambda n: up_prod(n, g), 1)
                assert not pend
                tick[0] = 0
                if last and g == NFG - 1:
                    act = [[_gelu(c(i, k)) for k in range(4)] for i in range(4)]
                    for n1 in range(7):
                        uset_job(lambda i, k, r0, n: act[i][k], g, n1, 0, TQ)
                    continue
                c0 = 4 * (g % 2)
                for i in range(4):
                    for k in range(4):
                        act_s[i * TQ:(i + 1) * TQ, _ct(c0 + k)] = _gelu(c(i, k))

                def tile(i, k, r0, n, c0=c0):
                    return act_s[i * TQ + r0:i * TQ + r0 + n, _ct(c0 + k)]

                pend += [functools.partial(uset_job, tile, g, n1, r0, 16)
                         for n1 in range(7) for r0 in range(0, TQ, 16)]
            jobs = {}
            if not last:
                mix(j + 1, drain)
                assert not pend
                prev = []
                for k in range(TB // 16):
                    jobs[k * Y_AT] = functools.partial(ln_job, (k % 4) * TQ + (k // 4) * 16, 16, prev)

                def place(start, fns):
                    for fn in fns:
                        while start in jobs:
                            start += 1
                        jobs[start] = fn

                for rt in range(2):
                    place(S_AT[rt], [functools.partial(set_job, yn_s, 2, rt, ct, n1, 16)
                                     for ct in range(2) for n1 in range(7)])
                place(G_AT, [functools.partial(set_job, gs_s, 3, rt, ct, n1, 16)
                             for rt in range(2) for ct in range(2) for n1 in range(7)])

            def down_part(n, og, k0, k1):
                ref, rows = u_set(n)
                return _dot(_up(ref[rows, k0 * E:k1 * E]),
                            _up(t4_s[og, k0 * E // 2:k1 * E // 2, _ct(n)]))

            head = {}
            if last:
                head = {n: down_part(n, 0, 0, NFG - 1) for n in range(HEAD)}
            count = [0]

            def down_prod(n, og):
                if og == 0 and n in head:
                    return down_part(n, og, NFG - 1, NFG) + head[n]
                m = down_part(n, og, 0, NFG)
                job = jobs.get(count[0])
                count[0] += 1
                if job is not None:
                    job(anchor=m)
                return m

            for og in range(NOG):
                c = _strassen2(lambda n: down_prod(n, og))
                for i in (2, 3, 0, 1):
                    rows = slice(i * TQ, (i + 1) * TQ)
                    for k in range(2):
                        c0 = (4 * og + 2 * k) * E
                        o_s.at[slot][rows, c0:c0 + 2 * E] = (
                            base_s[rows, c0:c0 + 2 * E] + mod_rows(5, TQ, c0, 2 * E)
                            * jnp.concatenate([c(i, 2 * k), c(i, 2 * k + 1)], axis=1)).astype(bf16)
                    if last and i % 2:
                        r0, cols = (i - 1) * TQ, slice(og * HD, (og + 1) * HD)
                        copy(o_s.at[slot, r0:r0 + 2 * TQ, cols],
                             out_hbm.at[j * TB + r0:j * TB + r0 + 2 * TQ, cols], SEM_OUT + slot).start()
            if not last:
                out_copy(j, slot).start()

        def p3_body(j, carry):
            @pl.when(j >= 2)
            def _():
                out_copy(j - 2, j & 1).wait()

            mlp_block(j, False)
            return carry

        lax.fori_loop(0, NB - 1, _scoped("p3", p3_body), 0)
        for k in range(2):
            for cp in mlp_w_copies(0, k):
                cp.wait()
        out_copy(NB - 3, (NB - 3) % 2).wait()
        mlp_block(NB - 1, True)
        out_copy(NB - 2, (NB - 2) % 2).wait()
        out_copy(NB - 1, (NB - 1) % 2).wait()

    pl.run_scoped(
        phase_a,
        pltpu.VMEM((NSEG, M, D), bf16),
        pltpu.VMEM((7, NSEG * M // 4, D // 2), u32),
        pltpu.VMEM((3 * D // E, D, E), bf16),
        pltpu.VMEM((2, 2, D, HH, E), bf16),
        pltpu.VMEM((2, BGR, D), bf16),
        pltpu.VMEM((2, 2, G1R, D), bf16),
        pltpu.VMEM((NC, D // 4, 5 * HG // 2 * E), u32),
        pltpu.VMEM((2 * D // E, 8, E), f32),
    )
    pl.run_scoped(
        phase_b,
        pltpu.VMEM((NOG, D // 8, 49 * E), u32),
        pltpu.VMEM((NFG, D // 8, 49 * E), u32),
        pltpu.VMEM((NOG, F // 8, 49 * E), u32),
        pltpu.VMEM((D // E, D, E), bf16),
        pltpu.VMEM((TB, D), f32),
        pltpu.VMEM((TB, D), f32),
        pltpu.VMEM((TB, D), f32),
        pltpu.VMEM((TB, D), f32),
        pltpu.VMEM((TB, D), f32),
        pltpu.VMEM((2, TB, D), bf16),
    )


@jax.jit
def pallas_adaLN_cond__memory_aug_recurrent_mem_tr__mixer_s_mlp__prompt_kernel(
    A_x: jax.Array,
    A_mem0: jax.Array,
    A_Wq: jax.Array,
    A_Wk: jax.Array,
    A_Wv: jax.Array,
    A_Wo: jax.Array,
    A_seg_len,
    B_x: jax.Array,
    B_w1: jax.Array,
    B_w2: jax.Array,
    B_w3: jax.Array,
    B_w4: jax.Array,
    c: jax.Array,
    w_mod: jax.Array,
):
    del A_seg_len, B_x
    assert A_x.shape == (1, S, D) and A_mem0.shape == (1, M, D)
    hbm = pl.BlockSpec(memory_space=pl.ANY)
    scratch = [
        pltpu.VMEM((NSEG, SEG, D), bf16),
        pltpu.VMEM((NC, D // 2, HG * E), u32),
        pltpu.VMEM((H * E // 2, D), u32),
        pltpu.VMEM((7, D // 4, D // 2), u32),
        pltpu.VMEM((2, 4, 16, 4 * E), bf16),
        pltpu.VMEM((2, 4, 64, 4 * E), bf16),
        pltpu.VMEM((2, 4, 32, D), bf16),
        pltpu.VMEM((NC, NSEG * M, HG // 2 * E), u32),
        pltpu.VMEM((8, 6 * D), f32),
        pltpu.VMEM((M, D), f32),
        pltpu.VMEM((TC, D), f32),
        pltpu.VMEM((2 * SEG, D), f32),
        pltpu.VMEM((E, E), f32),
        pltpu.VMEM((S, D), bf16),
        pltpu.VMEM((S + 16, D), f32),
        pltpu.VMEM((7 * SEG // 2, D // 2), u32),
        pltpu.VMEM((16, E), u32),
        pltpu.VMEM((1, D), bf16),
        pltpu.VMEM((M, D), bf16),
        pltpu.SemaphoreType.DMA((26,)),
    ]
    out = pl.pallas_call(
        _kernel,
        out_shape=jax.ShapeDtypeStruct((S, D), bf16),
        in_specs=[hbm] * 12,
        out_specs=hbm,
        scratch_shapes=scratch,
        compiler_params=pltpu.CompilerParams(vmem_limit_bytes=127 * 1024 * 1024,
                                             disable_bounds_checks=NO_CHECKS,
                                             disable_semaphore_checks=NO_CHECKS),
    )(A_x.reshape(NSEG, SEG, D), A_mem0.reshape(M, D), A_Wq, A_Wk, A_Wv,
      A_Wo.reshape(H * E, D), B_w1.reshape(2, D // 2, D), B_w2.reshape(4, D // 4, D), B_w3.reshape(4, D // 4, F),
      B_w4.reshape(NFG, 4, E, D), c, w_mod)
    return out.reshape(1, S, D)
```
